```python
import jax
import jax.numpy as jnp

def _softmax(x, axis=-1):
    return jax.nn.softmax(x, axis=axis)

def _gelu(x):
    return jax.nn.gelu(x, approximate=True)

def _silu(x):
    return jax.nn.silu(x)

def _sigmoid(x):
    return jax.nn.sigmoid(x)

def _layernorm(x, axis=-1, eps=1e-05):
    m = jnp.mean(x, axis=axis, keepdims=True)
    v = jnp.var(x, axis=axis, keepdims=True)
    return (x - m) / jnp.sqrt(v + eps)

def _scatter_add(tgt, idx, src, axis=0):
    return tgt.at[idx].add(src)

def _segment_sum(src, seg, n):
    return jax.ops.segment_sum(src, seg, n)

class _Rng:

    def __init__(self, key):
        self._k = key

    def _next(self):
        self._k, sub = jax.random.split(self._k)
        return sub

    def normal(self, shape):
        return jax.random.normal(self._next(), shape, dtype=jnp.bfloat16)

    def randint(self, lo, hi, shape):
        return jax.random.randint(self._next(), shape, lo, hi, dtype=jnp.int32)

    def uniform(self, shape, lo=0.0, hi=1.0):
        return jax.random.uniform(self._next(), shape, jnp.bfloat16, lo, hi)

    def permutation(self, n):
        return jax.random.permutation(self._next(), n)
kernel_name = 'adaLN_cond__ssm_conv_h3__mixer_s_mlp__prompt'

def setup_inputs():
    _rng = _Rng(jax.random.key(int.from_bytes(__import__("os").urandom(4), "little")))
    _w = lambda a: (lambda t: t.astype(jnp.bfloat16) if jnp.issubdtype(t.dtype, jnp.floating) else t)(jnp.asarray(a))

    def _A_setup():
        B, S, D = (1, 2048, 640)
        ks = 4
        return {'q': _w((lambda *s: _rng.normal(s) * 0.05)(B, S, D)), 'k': _w((lambda *s: _rng.normal(s) * 0.05)(B, S, D)), 'v': _w((lambda *s: _rng.normal(s) * 0.05)(B, S, D)), 'shift_k': _w((lambda *s: _rng.normal(s) * 0.05)(D, ks) * 0.5), 'ssm_k': _w((lambda *s: _rng.normal(s) * 0.05)(D, S) * (1.0 / S ** 0.5)), 'ssm_D': _w((lambda *s: _rng.normal(s) * 0.05)(D))}
    _A_in = _A_setup()

    def _B_setup():
        B, S, D, F = (1, 2048, 640, 1728)
        return {'x': _w((lambda *s: _rng.normal(s) * 0.05)(B, S, D)), 'w1': _w((lambda *s: _rng.normal(s) * 0.05)(D, D) * D ** (-0.5)), 'w2': _w((lambda *s: _rng.normal(s) * 0.05)(D, D) * D ** (-0.5)), 'w3': _w((lambda *s: _rng.normal(s) * 0.05)(D, F) * D ** (-0.5)), 'w4': _w((lambda *s: _rng.normal(s) * 0.05)(F, D) * F ** (-0.5))}
    _B_in = _B_setup()
    return {'A_q': _A_in['q'], 'A_k': _A_in['k'], 'A_v': _A_in['v'], 'A_shift_k': _A_in['shift_k'], 'A_ssm_k': _A_in['ssm_k'], 'A_ssm_D': _A_in['ssm_D'], 'B_x': _B_in['x'], 'B_w1': _B_in['w1'], 'B_w2': _B_in['w2'], 'B_w3': _B_in['w3'], 'B_w4': _B_in['w4'], 'c': _w((lambda *s: _rng.normal(s) * 0.05)(1, 640)), 'w_mod': _w((lambda *s: _rng.normal(s) * 0.05)(640, 6 * 640) * 640 ** (-0.5))}

def reference(A_q, A_k, A_v, A_shift_k, A_ssm_k, A_ssm_D, B_x, B_w1, B_w2, B_w3, B_w4, c, w_mod):

    def _A_ref(q, k, v, shift_k, ssm_k, ssm_D):
        B, S, D = q.shape
        ks = shift_k.shape[-1]
        k_pad = jnp.pad(k, ((0, 0), (ks - 1, 0), (0, 0)))
        k_shift = jnp.zeros_like(k)
        for t in range(ks):
            k_shift = k_shift + k_pad[:, t:t + S, :] * shift_k[:, ks - 1 - t][None, None, :]
        kv = k_shift * v
        L = 2 * S
        kv_pad = jnp.pad(kv, ((0, 0), (0, S), (0, 0)))
        kf_pad = jnp.pad(ssm_k, ((0, 0), (0, S)))
        kv_f = (lambda x, axes=(-2, -1): jnp.fft.rfft2(x.astype(jnp.float32), axes=axes))(kv_pad[:, None, :, :], axes=(1, 2))
        kf_f = (lambda x, axes=(-2, -1): jnp.fft.rfft2(x.astype(jnp.float32), axes=axes))(kf_pad[:, None, :], axes=(1, 2))
        kf_f = (lambda x, *d: x.transpose(*d))(kf_f, 1, 2, 0)
        y_f = kv_f * kf_f[None, :, :, :]
        y = (lambda x, s, axes=(-2, -1): jnp.fft.irfft2(x, s=s, axes=axes).astype(jnp.bfloat16))(y_f, (1, L), axes=(1, 2))[:, 0, :S, :]
        y = y + kv * ssm_D[None, None, :]
        return q * y

    def _B_ref(x, w1, w2, w3, w4):
        B, S, D = x.shape
        h = _gelu(_layernorm(x, axis=-1) @ w1)
        c = D // 4
        g0 = jnp.pad(h[:, :, 0 * c:1 * c], ((0, 0), (1, 0), (0, 0)))[:, :S, :]
        g1 = jnp.pad(h[:, :, 1 * c:2 * c], ((0, 0), (0, 1), (0, 0)))[:, 1:, :]
        g2 = jnp.pad(h[:, :, 2 * c:3 * c], ((0, 0), (2, 0), (0, 0)))[:, :S, :]
        g3 = jnp.pad(h[:, :, 3 * c:], ((0, 0), (0, 2), (0, 0)))[:, 2:, :]
        hs = jnp.concatenate([g0, g1, g2, g3], axis=-1) @ w2
        x1 = x + hs
        h2 = _gelu(_layernorm(x1, axis=-1) @ w3) @ w4
        return x1 + h2
    x = A_q
    mod = (_silu(c) @ w_mod).reshape(c.shape[0], 6, 1, -1)
    sa, ca, ga, sb, cb, gb = (mod[:, 0].copy(), mod[:, 1].copy(), mod[:, 2].copy(), mod[:, 3].copy(), mod[:, 4].copy(), mod[:, 5].copy())
    h = _layernorm(x, axis=-1) * (1 + ca) + sa
    x = x + ga * _A_ref(h, A_k, A_v, A_shift_k, A_ssm_k, A_ssm_D)
    h = _layernorm(x, axis=-1) * (1 + cb) + sb
    x = x + gb * _B_ref(h, B_w1, B_w2, B_w3, B_w4)
    return x
```

```python
import numpy as np
import jax
import jax.numpy as jnp
import jax.experimental.pallas as pl
import jax.experimental.pallas.tpu as pltpu

f32, bf16, u32 = jnp.float32, jnp.bfloat16, jnp.uint32

S, D, F = 2048, 640, 1728
CT = D // 128
NB, BLK, NFFT = 4, 512, 1024
T = 256
NC = S // T
EPS = 1e-5
NT_DIMS = (((1,), (1,)), ((), ()))


def _bf16_bits(x):
    u = np.ascontiguousarray(x, dtype=np.float32).view(np.uint32).astype(np.uint64)
    return ((u + 0x7FFF + ((u >> 16) & 1)) >> 16).astype(np.uint32)


def _pack_rows(x):
    b = _bf16_bits(x)
    return b[..., 0::2, :] | (b[..., 1::2, :] << 16)


def _dft_tables():
    kk = np.arange(128)
    f = np.where(kk < 64, 2 * kk, 2 * (kk - 64) + 1)

    def rows(r):
        th = np.pi * np.outer(2 * f + 1, r) / NFFT
        c, s = np.cos(th), -np.sin(th)
        grouped = np.stack([c.reshape(16, 8, 128), s.reshape(16, 8, 128)], axis=1).reshape(256, 128)
        return grouped, c, s

    fu, fk, g = [], [], []
    lane = np.arange(128)
    for p in range(4):
        o, c, s = rows(4 * lane + p)
        fu.append(o)
        g.append(np.stack([c, s], axis=1).reshape(256, 128).T * (2.0 / NFFT))
        m = (lane - p) % 4
        fk.append(rows(128 * m + (lane - m) % 128)[0])
    return _pack_rows(np.stack(fu)), _pack_rows(np.stack(fk)), _pack_rows(np.stack(g))


_FU, _FK, _G = _dft_tables()


def _lo(w):
    return pltpu.bitcast(w << 16, f32)


def _hi(w):
    return pltpu.bitcast(w & jnp.uint32(0xFFFF0000), f32)


def _ln(x):
    m = jnp.mean(x, axis=-1, keepdims=True)
    d = x - m
    v = jnp.mean(d * d, axis=-1, keepdims=True)
    return d * jax.lax.rsqrt(v + EPS)


def _gelu(x):
    c = 0.7978845608028654
    u = c + (c * 0.044715) * (x * x)
    t = jnp.tanh(x * u)
    hx = 0.5 * x
    return hx + hx * t


def _radix4(re, im, inverse):
    ar, ai = re[0] + re[2], im[0] + im[2]
    br, bi = re[0] - re[2], im[0] - im[2]
    cr, ci = re[1] + re[3], im[1] + im[3]
    dr, di = re[1] - re[3], im[1] - im[3]
    minus_i = (br + di, bi - dr)
    plus_i = (br - di, bi + dr)
    if inverse:
        return [(ar + cr, ai + ci), plus_i, (ar - cr, ai - ci), minus_i]
    return [(ar + cr, ai + ci), minus_i, (ar - cr, ai - ci), plus_i]


def _kernel(q_hbm, k_hbm, v_hbm, sh_hbm, sk_hbm, d_hbm, w1_hbm, w2_hbm, w3_hbm, w4_hbm,
            c_hbm, wm_hbm, fu_hbm, fk_hbm, g_hbm, o_hbm,
            kb, vb, skb, qb, w1b, w2b, w3b, w4b, wmb, shb, db, cb_, fub, fkb, gb_,
            US, KS, KR, ys, modb, h1s, h2s, x2s, ob,
            sem_c, sem_s, sem_m, sem_w, sem_q, sem_o):
    def conv_copies(c):
        return [
            pltpu.make_async_copy(sk_hbm.at[pl.ds(c * 128, 128), :], skb.at[c], sem_c.at[0, c]),
            pltpu.make_async_copy(k_hbm.at[:, pl.ds(c * 128, 128)], kb.at[c, pl.ds(16, S), :], sem_c.at[1, c]),
            pltpu.make_async_copy(v_hbm.at[:, pl.ds(c * 128, 128)], vb.at[c], sem_c.at[2, c]),
        ]

    small = [pltpu.make_async_copy(src, dst, sem_s.at[i]) for i, (src, dst) in enumerate(
        [(fk_hbm, fkb), (d_hbm, db), (fu_hbm, fub), (sh_hbm, shb), (g_hbm, gb_), (c_hbm, cb_)])]

    def mod_copy(i):
        return pltpu.make_async_copy(wm_hbm.at[:, pl.ds(i * D, D)], wmb.at[i], sem_m.at[i])

    w_copies = [pltpu.make_async_copy(src, dst, sem_w.at[i]) for i, (src, dst) in enumerate(
        [(w1_hbm, w1b), (w2_hbm, w2b), (w3_hbm, w3b), (w4_hbm, w4b)])]

    def q_copy(i):
        return pltpu.make_async_copy(q_hbm.at[pl.ds(i * T, T), :], qb.at[pl.ds(i * T, T), :], sem_q.at[i])

    def out_copy(i):
        return pltpu.make_async_copy(ob.at[pl.ds(i * T, T), :], o_hbm.at[pl.ds(i * T, T), :], sem_o.at[i])

    for cp in small:
        cp.start()
    for c in range(2):
        for cp in conv_copies(c):
            cp.start()

    for c in range(CT):
        kb[c, 0:16, :] = jnp.zeros((16, 128), bf16)
    h1s[0:8, :] = jnp.zeros((8, D), f32)
    h1s[S + 8:S + 16, :] = jnp.zeros((8, D), f32)
    kw = kb.bitcast(u32)
    vw = vb.bitcast(u32)

    def grp(ref, idx, g):
        return ref[idx + (slice(g * 16, g * 16 + 8),)], ref[idx + (slice(g * 16 + 8, g * 16 + 16),)]

    def fwd_k(c, slot, j):
        lane = jax.lax.broadcasted_iota(jnp.int32, (64, 128), 1)
        even = (lane & 1) == 0
        l01 = (lane & 2) == 0
        l12 = ((lane + 3) & 2) == 0
        rm = []
        for m in range(4):
            w = pltpu.bitcast(skb[c, :, (4 * j + m) * 128:(4 * j + m + 1) * 128], u32)
            rm.append(pltpu.roll(w, m, 1) if m else w)
        e01 = jnp.where(even, rm[0], rm[1])
        o01 = jnp.where(even, rm[1], rm[0])
        e23 = jnp.where(even, rm[2], rm[3])
        o23 = jnp.where(even, rm[3], rm[2])
        kp = [jnp.where(l01, e01, e23), jnp.where(l12, o01, o23),
              jnp.where(l01, e23, e01), jnp.where(l12, o23, o01)]
        tt = [jax.lax.dot_general(pltpu.bitcast(fkb[p], bf16), pltpu.bitcast(kp[p], bf16), NT_DIMS,
                                  preferred_element_type=f32) for p in range(4)]
        if j == 0:
            dvec = db[:, c * 128:(c + 1) * 128].astype(f32)
        for g in range(16):
            re = [t[g * 16:g * 16 + 8] for t in tt]
            im = [t[g * 16 + 8:g * 16 + 16] for t in tt]
            if j == 0:
                re[0] = re[0] + dvec
            x = _radix4(re, im, False)
            for m in range(4):
                xr, xi = x[m]
                if j < NB - 1:
                    KR[j, m, g * 16:g * 16 + 8, :] = xr
                    KR[j, m, g * 16 + 8:g * 16 + 16, :] = xi
                if j > 0:
                    pr, pi = grp(KR, (j - 1, m), g)
                    if g < 8:
                        xr, xi = xr - pi, xi + pr
                    else:
                        xr, xi = xr + pi, xi - pr
                KS[slot, j, m, g * 16:g * 16 + 8, :] = xr
                KS[slot, j, m, g * 16 + 8:g * 16 + 16, :] = xi

    def fwd_u(c, slot, a):
        w = shb[:, c * 128:(c + 1) * 128].astype(f32)
        w0, w1, w2, w3 = [w[i:i + 1] for i in range(4)]
        base = 8 + a * 256
        ka = kw[c, pl.ds(base, 128, stride=2), :]
        kb2 = kw[c, pl.ds(base + 1, 128, stride=2), :]
        ka1 = kw[c, pl.ds(base - 2, 128, stride=2), :]
        kb1 = kw[c, pl.ds(base - 1, 128, stride=2), :]
        va = vw[c, pl.ds(a * 256, 128, stride=2), :]
        vb2 = vw[c, pl.ds(a * 256 + 1, 128, stride=2), :]
        k0, k1, k2, k3 = _lo(ka), _hi(ka), _lo(kb2), _hi(kb2)
        km3, km2, km1 = _hi(ka1), _lo(kb1), _hi(kb1)
        s0 = w0 * k0 + w1 * km1 + w2 * km2 + w3 * km3
        s1 = w0 * k1 + w1 * k0 + w2 * km1 + w3 * km2
        s2 = w0 * k2 + w1 * k1 + w2 * k0 + w3 * km1
        s3 = w0 * k3 + w1 * k2 + w2 * k1 + w3 * k0
        kv = [s0 * _lo(va), s1 * _hi(va), s2 * _lo(vb2), s3 * _hi(vb2)]
        tt = [jnp.dot(pltpu.bitcast(fub[p], bf16), kv[p].astype(bf16), preferred_element_type=f32)
              for p in range(4)]
        for g in range(16):
            x = _radix4([t[g * 16:g * 16 + 8] for t in tt], [t[g * 16 + 8:g * 16 + 16] for t in tt], False)
            for m in range(4):
                US[slot, a, m, g * 16:g * 16 + 8, :] = x[m][0]
                US[slot, a, m, g * 16 + 8:g * 16 + 16, :] = x[m][1]

    def mac_inv(c, slot, a):
        words = [[] for _ in range(4)]
        for g in range(16):
            yre, yim = [], []
            for m in range(4):
                yr = yi = None
                for j in range(a + 1):
                    kr, ki = grp(KS, (slot, j, m), g)
                    ur, ui = grp(US, (slot, a - j, m), g)
                    tr = kr * ur - ki * ui
                    ti = kr * ui + ki * ur
                    yr = tr if yr is None else yr + tr
                    yi = ti if yi is None else yi + ti
                yre.append(yr)
                yim.append(yi)
            pp = _radix4(yre, yim, True)
            for p in range(4):
                words[p].append(pltpu.pack_elementwise([pp[p][0], pp[p][1]], packed_dtype=bf16))
        for p in range(4):
            pb = pltpu.bitcast(jnp.concatenate(words[p], axis=0), bf16)
            ys[c, pl.ds(a * BLK + p, 128, stride=4), :] = jnp.dot(
                pltpu.bitcast(gb_[p], bf16), pb, preferred_element_type=f32)

    for cp in small:
        cp.wait()
    for s in range(CT + 1):
        if s < CT:
            for cp in conv_copies(s):
                cp.wait()
        if s + 2 < CT:
            for cp in conv_copies(s + 2):
                cp.start()
        if s == CT - 2:
            for i in range(3):
                mod_copy(i).start()
        if s == CT - 1:
            q_copy(0).start()
            q_copy(1).start()
            mod_copy(3).start()
            mod_copy(4).start()
            w_copies[0].start()
        if s == CT:
            mod_copy(0).wait()
            w_copies[1].start()
            q_copy(2).start()
            w_copies[2].start()
            w_copies[3].start()
            mod_copy(5).start()
            for i in range(3, NC):
                q_copy(i).start()
        for j in range(NB):
            if s < CT:
                fwd_k(s, s % 2, j)
            if s >= 1:
                mac_inv(s - 1, (s - 1) % 2, j)
        if s < CT:
            for a in range(NB):
                fwd_u(s, s % 2, a)

    cvec = cb_[...].astype(f32)
    sc = jnp.broadcast_to(cvec * jax.nn.sigmoid(cvec), (16, D)).astype(bf16)

    def mod_compute(i):
        modb[i] = jnp.dot(sc, wmb[i], preferred_element_type=f32)[0:8]

    mod_compute(0)
    for i in range(1, 5):
        mod_copy(i).wait()
        mod_compute(i)

    def mvec(i):
        return modb[i, 0:1, :]

    def stage_a(i):
        r = pl.multiple_of(i * T, T)
        q = qb[pl.ds(r, T), :].astype(f32)
        y = jnp.concatenate([ys[c, pl.ds(r, T), :] for c in range(CT)], axis=-1)
        h = _ln(q) * (1.0 + mvec(1)) + mvec(0)
        x2 = q + mvec(2) * (h * y)
        h2 = _ln(x2) * (1.0 + mvec(4)) + mvec(3)
        z = _ln(h2).astype(bf16)
        h1 = _gelu(jnp.dot(z, w1b[...], preferred_element_type=f32))
        h1s[pl.ds(r + 8, T), :] = h1
        h2s[pl.ds(r, T), :] = h2
        x2s[pl.ds(r, T), :] = x2

    def stage_b(i):
        r = pl.multiple_of(i * T, T)
        win = h1s[pl.ds(r, T + 16), :]
        lane = jax.lax.broadcasted_iota(jnp.int32, (T, 128), 1)

        def sh(k, c):
            return win[8 + k:8 + k + T, c * 128:(c + 1) * 128]

        g = jnp.concatenate([
            sh(-1, 0),
            jnp.where(lane < 32, sh(-1, 1), sh(1, 1)),
            jnp.where(lane < 64, sh(1, 2), sh(-2, 2)),
            jnp.where(lane < 96, sh(-2, 3), sh(2, 3)),
            sh(2, 4)], axis=-1).astype(bf16)
        x1 = h2s[pl.ds(r, T), :] + jnp.dot(g, w2b[...], preferred_element_type=f32)
        z = _ln(x1).astype(bf16)
        a = _gelu(jax.lax.dot_general(z, w3b[...], NT_DIMS, preferred_element_type=f32)).astype(bf16)
        h2 = jnp.dot(a, w4b[...], preferred_element_type=f32)
        ob[pl.ds(r, T), :] = (x2s[pl.ds(r, T), :] + mvec(5) * (x1 + h2)).astype(bf16)

    q_copy(0).wait()
    q_copy(1).wait()
    w_copies[0].wait()
    stage_a(0)
    stage_a(1)
    for i in range(1, 4):
        w_copies[i].wait()
    mod_copy(5).wait()
    mod_compute(5)

    def body(i, carry):
        q_copy(i + 2).wait()
        stage_b(i)
        stage_a(i + 2)
        out_copy(i).start()
        return carry

    jax.lax.fori_loop(0, NC - 2, body, 0)

    def body2(i, carry):
        stage_b(i)
        out_copy(i).start()
        return carry

    jax.lax.fori_loop(NC - 2, NC, body2, 0)
    for i in range(NC):
        out_copy(i).wait()


@jax.jit
def pallas_adaLN_cond__ssm_conv_h3__mixer_s_mlp__prompt_kernel(
    A_q: jax.Array,
    A_k: jax.Array,
    A_v: jax.Array,
    A_shift_k: jax.Array,
    A_ssm_k: jax.Array,
    A_ssm_D: jax.Array,
    B_x: jax.Array,
    B_w1: jax.Array,
    B_w2: jax.Array,
    B_w3: jax.Array,
    B_w4: jax.Array,
    c: jax.Array,
    w_mod: jax.Array,
):
    del B_x
    any_spec = pl.BlockSpec(memory_space=pl.ANY)
    vm = pltpu.VMEM
    out = pl.pallas_call(
        _kernel,
        in_specs=[any_spec] * 15,
        out_specs=any_spec,
        out_shape=jax.ShapeDtypeStruct((S, D), bf16),
        scratch_shapes=[
            vm((CT, S + 16, 128), bf16), vm((CT, S, 128), bf16), vm((CT, 128, S), bf16),
            vm((S, D), bf16), vm((D, D), bf16), vm((D, D), bf16), vm((F, D), bf16), vm((F, D), bf16),
            vm((6, D, D), bf16), vm((4, D), bf16), vm((1, D), bf16), vm((1, D), bf16),
            vm((4, 128, 128), u32), vm((4, 128, 128), u32), vm((4, 64, 256), u32),
            vm((2, NB, 4, 256, 128), f32), vm((2, NB, 4, 256, 128), f32), vm((NB - 1, 4, 256, 128), f32),
            vm((CT, S, 128), f32), vm((6, 8, D), f32),
            vm((S + 16, D), f32), vm((S, D), f32), vm((S, D), f32), vm((S, D), bf16),
            pltpu.SemaphoreType.DMA((3, CT)), pltpu.SemaphoreType.DMA((6,)), pltpu.SemaphoreType.DMA((6,)),
            pltpu.SemaphoreType.DMA((4,)), pltpu.SemaphoreType.DMA((NC,)), pltpu.SemaphoreType.DMA((NC,)),
        ],
        compiler_params=pltpu.CompilerParams(vmem_limit_bytes=110 << 20),
    )(A_q.reshape(S, D), A_k.reshape(S, D), A_v.reshape(S, D), A_shift_k.T, A_ssm_k,
      A_ssm_D.reshape(1, D), B_w1, B_w2, B_w3.T, B_w4, c, w_mod,
      jnp.asarray(_FU), jnp.asarray(_FK), jnp.asarray(_G))
    return out.reshape(1, S, D)
```

```python
import os
import numpy as np
import jax
import jax.numpy as jnp
import jax.experimental.pallas as pl
import jax.experimental.pallas.tpu as pltpu

f32, bf16, u32, i32 = jnp.float32, jnp.bfloat16, jnp.uint32, jnp.int32

S, D, F = 2048, 640, 1728
CT = D // 128
NB, BLK, NFFT = 4, 512, 1024
T = 256
NC = S // T
CONV = 'U3,U2,U1,U0,a3,K3,b3,K2,a2,K1,b2,K0,a1,b1,a0,b0'
P0, P1, PC = 272, 336, 240
RG = 16
EPS = 1e-5
NT_DIMS = (((1,), (1,)), ((), ()))
SCOPES = bool(int(os.environ.get("KSCOPES", "0")))


class _NoScope:
    def __enter__(self):
        return self

    def __exit__(self, *a):
        return False


def _scope(name):
    return jax.named_scope(name) if SCOPES else _NoScope()


def _lo(w):
    return pltpu.bitcast(w << 16, f32)


def _hi(w):
    return pltpu.bitcast(w & jnp.uint32(0xFFFF0000), f32)


def _cos_turn(n32, scale):
    x = 2.0 ** 30 - jnp.abs(n32.astype(f32))
    b = 2.0 * np.pi / 2.0 ** 32
    x = x * b
    x2 = x * x
    c = [scale * v for v in (1.0, -1.0 / 6, 1.0 / 120, -1.0 / 5040, 1.0 / 362880)]
    return x * (c[0] + x2 * (c[1] + x2 * (c[2] + x2 * (c[3] + x2 * c[4]))))


def _odd_freq(k):
    return jnp.where(k < 64, 4 * k + 1, 4 * k - 253) << 21


def _fwd_table(r):
    w = jax.lax.broadcasted_iota(i32, (128, 128), 0)
    halves = []
    for par in range(2):
        row = 2 * w + par
        k = ((row >> 4) << 3) + (row & 7)
        halves.append(_cos_turn(_odd_freq(k) * r + ((row & 8) << 27), 1.0))
    return pltpu.pack_elementwise(halves, packed_dtype=bf16)


def _inv_table(p):
    w = jax.lax.broadcasted_iota(i32, (64, 256), 0)
    col = jax.lax.broadcasted_iota(i32, (64, 256), 1)
    fr = _odd_freq(col >> 1)
    off = (col & 1) << 30
    halves = [_cos_turn(fr * (8 * w + 4 * par + p) + off, 2.0 / NFFT) for par in range(2)]
    return pltpu.pack_elementwise(halves, packed_dtype=bf16)


def _stats(x, floor):
    m = jnp.sum(x, axis=-1, keepdims=True) * (1.0 / D)
    v = jnp.maximum(jnp.sum(x * x, axis=-1, keepdims=True) * (1.0 / D) - m * m, floor)
    return m, jax.lax.rsqrt(v + EPS)


def _gelu(x):
    c = 0.7978845608028654
    u = c + (c * 0.044715) * (x * x)
    t = jnp.tanh(x * u)
    hx = 0.5 * x
    return hx + hx * t


def _radix4(re, im, inverse):
    ar, ai = re[0] + re[2], im[0] + im[2]
    br, bi = re[0] - re[2], im[0] - im[2]
    cr, ci = re[1] + re[3], im[1] + im[3]
    dr, di = re[1] - re[3], im[1] - im[3]
    minus_i = (br + di, bi - dr)
    plus_i = (br - di, bi + dr)
    if inverse:
        return [(ar + cr, ai + ci), plus_i, (ar - cr, ai - ci), minus_i]
    return [(ar + cr, ai + ci), minus_i, (ar - cr, ai - ci), plus_i]


def _kernel(q_hbm, k_hbm, v_hbm, sh_hbm, sk_hbm, d_hbm, w1_hbm, w2_hbm, w3_hbm, w4_hbm,
            c_hbm, wm_hbm, o_hbm,
            kb, vb, skb, qb, w1b, w2b, w3b, w4b, wmb, shb, db, cb_, fub, fkb, gtb, par,
            US, KS, YP, ys, modb, h1s, h2s, x2s, xt, ht, zt, zb, ob,
            sem, sem_o):
    def sk_copy(c):
        return pltpu.make_async_copy(sk_hbm.at[pl.ds(c * 128, 128), :], skb.at[c], sem.at[c])

    def kv_copies(c):
        off = c * 128 if isinstance(c, int) else pl.multiple_of(c * 128, 128)
        return [
            pltpu.make_async_copy(k_hbm.at[:, pl.ds(off, 128)], kb.at[c, pl.ds(16, S), :], sem.at[CT + c]),
            pltpu.make_async_copy(v_hbm.at[:, pl.ds(off, 128)], vb.at[c], sem.at[2 * CT + c]),
        ]

    small = [pltpu.make_async_copy(src, dst, sem.at[15 + i]) for i, (src, dst) in enumerate(
        [(d_hbm, db), (sh_hbm, shb), (c_hbm, cb_)])]

    mod_cols = [(0, 3 * D), (3 * D, 2 * D), (5 * D, D)]
    mod_copies = [pltpu.make_async_copy(wm_hbm.at[:, pl.ds(o, n)], wmb.at[:, pl.ds(o, n)], sem.at[18 + i])
                  for i, (o, n) in enumerate(mod_cols)]
    FH = 896
    w_pairs = [(w1_hbm, w1b), (w2_hbm, w2b), (w3_hbm.at[pl.ds(0, FH), :], w3b.at[pl.ds(0, FH), :]),
               (w3_hbm.at[pl.ds(FH, F - FH), :], w3b.at[pl.ds(FH, F - FH), :]), (w4_hbm, w4b)]
    w_copies = [pltpu.make_async_copy(src, dst, sem.at[21 + i]) for i, (src, dst) in enumerate(w_pairs)]
    q_rows = [(0, P0), (P0, P1), (P0 + P1, PC), (P0 + P1 + PC, S - P0 - P1 - PC)]
    q_copies = [pltpu.make_async_copy(q_hbm.at[pl.ds(o, n), :], qb.at[pl.ds(o, n), :], sem.at[26 + i])
                for i, (o, n) in enumerate(q_rows)]

    def out_copy(i):
        r = i * T if isinstance(i, int) else pl.multiple_of(i * T, T)
        return pltpu.make_async_copy(ob.at[pl.ds(r, T), :], o_hbm.at[pl.ds(r, T), :], sem_o.at[i])

    sk_copy(0).start()
    for cp in small:
        cp.start()
    for cp in kv_copies(0):
        cp.start()
    for c in range(1, CT):
        sk_copy(c).start()
        for cp in kv_copies(c):
            cp.start()
    for cp in [mod_copies[0], q_copies[0], mod_copies[1], w_copies[0], w_copies[1], q_copies[1],
               w_copies[2], w_copies[3], q_copies[2], w_copies[4], mod_copies[2], q_copies[3]]:
        cp.start()

    with _scope("init"):
        def pin(i, carry):
            YP[i, 0:8, :] = jnp.zeros((8, 128), f32)
            return carry

        jax.lax.fori_loop(0, 2, pin, 0)
        lane = jax.lax.broadcasted_iota(i32, (128, 128), 1)
        for p in range(4):
            m = (lane - p) & 3
            fkb[p] = _fwd_table(128 * m + ((lane - m) & 127))
        for c in range(CT):
            kb[c, 0:16, :] = jnp.zeros((16, 128), bf16)
            h1s[c, 0:8, :] = jnp.zeros((8, 128), f32)
            h1s[c, S + 8:S + 16, :] = jnp.zeros((8, 128), f32)
        for p in range(4):
            fub[p] = _fwd_table(4 * lane + p)
        for cp in small:
            cp.wait()
        dv = db[...].astype(f32).reshape(1, D)
        shv = shb[...].astype(f32)
        for c in range(CT):
            for i in range(4):
                par[c, i] = jnp.broadcast_to(shv[i:i + 1, c * 128:(c + 1) * 128], (8, 128))
            par[c, 4] = jnp.broadcast_to(dv[:, c * 128:(c + 1) * 128], (8, 128))
    kw = kb.bitcast(u32)
    vw = vb.bitcast(u32)

    def re_(g):
        return slice(g * 16, g * 16 + 8)

    def im_(g):
        return slice(g * 16 + 8, g * 16 + 16)

    def fwd_k(c, j, sl=0):
        lane = jax.lax.broadcasted_iota(i32, (64, 128), 1)
        even = (lane & 1) == 0
        l01 = (lane & 2) == 0
        l12 = ((lane + 3) & 2) == 0
        rm = []
        for m in range(4):
            w = pltpu.bitcast(skb[c, :, (4 * j + m) * 128:(4 * j + m + 1) * 128], u32)
            rm.append(pltpu.roll(w, m, 1) if m else w)
        e01 = jnp.where(even, rm[0], rm[1])
        o01 = jnp.where(even, rm[1], rm[0])
        e23 = jnp.where(even, rm[2], rm[3])
        o23 = jnp.where(even, rm[3], rm[2])
        kp = [jnp.where(l01, e01, e23), jnp.where(l12, o01, o23),
              jnp.where(l01, e23, e01), jnp.where(l12, o23, o01)]
        tt = [jax.lax.dot_general(pltpu.bitcast(fkb[p], bf16), pltpu.bitcast(kp[p], bf16), NT_DIMS,
                                  preferred_element_type=f32) for p in range(4)]
        dvec = par[c, 4] if j == 0 else None
        for g in range(16):
            re = [t[re_(g)] for t in tt]
            im = [t[im_(g)] for t in tt]
            if j == 0:
                re[0] = re[0] + dvec
            x = _radix4(re, im, False)
            for m in range(4):
                xr, xi = x[m]
                KS[sl, j, m, re_(g), :] = xr
                KS[sl, j, m, im_(g), :] = xi
                if j < NB - 1:
                    nr, ni = KS[sl, j + 1, m, re_(g), :], KS[sl, j + 1, m, im_(g), :]
                    if g < 8:
                        nr, ni = nr - xi, ni + xr
                    else:
                        nr, ni = nr + xi, ni - xr
                    KS[sl, j + 1, m, re_(g), :] = nr
                    KS[sl, j + 1, m, im_(g), :] = ni

    def fwd_u(c, a, sl=0):
        w0, w1, w2, w3 = [jnp.tile(par[c, i], (16, 1)) for i in range(4)]
        base = 8 + a * 256
        ka = kw[c, pl.ds(base, 128, stride=2), :]
        kb2 = kw[c, pl.ds(base + 1, 128, stride=2), :]
        ka1 = kw[c, pl.ds(base - 2, 128, stride=2), :]
        kb1 = kw[c, pl.ds(base - 1, 128, stride=2), :]
        va = vw[c, pl.ds(a * 256, 128, stride=2), :]
        vb2 = vw[c, pl.ds(a * 256 + 1, 128, stride=2), :]
        k0, k1, k2, k3 = _lo(ka), _hi(ka), _lo(kb2), _hi(kb2)
        km3, km2, km1 = _hi(ka1), _lo(kb1), _hi(kb1)
        s0 = w0 * k0 + w1 * km1 + w2 * km2 + w3 * km3
        s1 = w0 * k1 + w1 * k0 + w2 * km1 + w3 * km2
        s2 = w0 * k2 + w1 * k1 + w2 * k0 + w3 * km1
        s3 = w0 * k3 + w1 * k2 + w2 * k1 + w3 * k0
        kv = [s0 * _lo(va), s1 * _hi(va), s2 * _lo(vb2), s3 * _hi(vb2)]
        tt = [jnp.dot(pltpu.bitcast(fub[p], bf16), kv[p].astype(bf16), preferred_element_type=f32)
              for p in range(4)]
        for g in range(16):
            x = _radix4([t[re_(g)] for t in tt], [t[im_(g)] for t in tt], False)
            for m in range(4):
                US[sl, a, m, re_(g), :] = x[m][0]
                US[sl, a, m, im_(g), :] = x[m][1]

    def mac_inv(c, a, sl=0, halves=(0, 1)):
        for h in halves:
            words = [[] for _ in range(4)]
            for g in range(8 * h, 8 * h + 8):
                yre, yim = [], []
                for m in range(4):
                    yr = yi = None
                    for j in range(a + 1):
                        kr, ki = KS[sl, j, m, re_(g), :], KS[sl, j, m, im_(g), :]
                        ur, ui = US[sl, a - j, m, re_(g), :], US[sl, a - j, m, im_(g), :]
                        tr = kr * ur - ki * ui
                        ti = kr * ui + ki * ur
                        yr = tr if yr is None else yr + tr
                        yi = ti if yi is None else yi + ti
                    yre.append(yr)
                    yim.append(yi)
                pp = _radix4(yre, yim, True)
                for p in range(4):
                    words[p].append(pltpu.pack_elementwise([pp[p][0], pp[p][1]], packed_dtype=bf16))
            for p in range(4):
                pb = pltpu.bitcast(jnp.concatenate(words[p], axis=0), bf16)
                r = jnp.dot(pltpu.bitcast(gtb[p, :, h * 128:(h + 1) * 128], bf16), pb,
                            preferred_element_type=f32)
                if h == 0:
                    YP[p] = r
                else:
                    ys[c, pl.ds(a * BLK + p, 128, stride=4), :] = YP[p] + r

    desc = (3, 2, 1, 0)
    with _scope("conv_first"):
        with _scope("w_sk0"):
            sk_copy(0).wait()
        for j in desc:
            fwd_k(0, j)
        for p in range(4):
            gtb[p] = _inv_table(p)
        with _scope("w_kv0"):
            for cp in kv_copies(0):
                cp.wait()
        for a in desc:
            fwd_u(0, a)

    def conv_tile(s, sl):
        with _scope("w_tile"):
            sk_copy(s).wait()
            for cp in kv_copies(s):
                cp.wait()
        for tok in CONV.split(","):
            if tok[0] == "K":
                fwd_k(s, int(tok[1]), sl)
            elif tok[0] == "U":
                fwd_u(s, int(tok[1]), sl)
            else:
                mac_inv(s - 1, int(tok[1]), 1 - sl, (0,) if tok[0] == "a" else (1,))

    def conv_body(t, carry):
        conv_tile(2 * t + 1, 1)
        conv_tile(2 * t + 2, 0)
        return carry

    with _scope("conv_loop"):
        jax.lax.fori_loop(0, 2, conv_body, 0)

    def mod_part(part):
        cvec = cb_[...].astype(f32)
        sc = jnp.broadcast_to(cvec * jax.nn.sigmoid(cvec), (16, D)).astype(bf16)
        o, n = mod_cols[part]
        r = jnp.dot(sc, wmb[:, o:o + n], preferred_element_type=f32)[0:8]
        return [r[:, i * D:(i + 1) * D] for i in range(n // D)]

    def mvec(i):
        return modb[i, 0:1, :]

    def rows(r, n):
        return pl.ds(r, n)

    def floor_of(prev):
        return 0.0 if prev is None else jnp.minimum(prev, 0.0)

    def a_part1(r, o, prev):
        q = qb[rows(r, RG), :].astype(f32)
        m, rs = _stats(q, floor_of(prev))
        y = jnp.concatenate([ys[c, rows(r, RG), :] for c in range(CT)], axis=-1)
        x2 = q + (((q - m) * rs) * mvec(1) + mvec(0)) * y
        xt[o:o + RG, :] = x2
        m, rs = _stats(x2, 0.0)
        return (x2 - m) * rs

    def a_part2(o, n2):
        h2 = n2 * mvec(3) + mvec(2)
        ht[o:o + RG, :] = h2
        m, rs = _stats(h2, 0.0)
        zt[o // 2:(o + RG) // 2, :] = pltpu.bitcast(((h2 - m) * rs).astype(bf16), u32)
        return rs

    def a_chain(r, n):
        prev = None
        for o in range(0, n, RG):
            prev = a_part2(o, a_part1(r + o, o, prev))

    def mm_w1(r, n):
        x2s[rows(r, n), :] = xt[0:n, :]
        h2s[rows(r, n), :] = ht[0:n, :]
        z = pltpu.bitcast(zt[0:n // 2, :], bf16)
        h1 = _gelu(jnp.dot(z, w1b[...], preferred_element_type=f32))
        for c in range(CT):
            h1s[c, rows(r + 8, n), :] = h1[:, c * 128:(c + 1) * 128]

    def mm_w2(r, chained=True):
        lane = jax.lax.broadcasted_iota(i32, (T, 128), 1)

        def sh(k, c):
            return h1s[c, rows(r + 8 + k, T), :]

        g = jnp.concatenate([
            sh(-1, 0),
            jnp.where(lane < 32, sh(-1, 1), sh(1, 1)),
            jnp.where(lane < 64, sh(1, 2), sh(-2, 2)),
            jnp.where(lane < 96, sh(-2, 3), sh(2, 3)),
            sh(2, 4)], axis=-1).astype(bf16)
        h2s[rows(r, T), :] = h2s[rows(r, T), :] + jnp.dot(g, w2b[...], preferred_element_type=f32)
        prev = None
        for o in range(0, T, RG):
            x1 = h2s[rows(r + o, RG), :]
            m, rs = _stats(x1, floor_of(prev))
            zb[o // 2:(o + RG) // 2, :] = pltpu.bitcast(((x1 - m) * rs).astype(bf16), u32)
            if chained:
                prev = rs

    def mm_w3(f0=0, f1=F):
        z = pltpu.bitcast(zb[...], bf16)
        return _gelu(jax.lax.dot_general(z, w3b[f0:f1, :], NT_DIMS, preferred_element_type=f32)).astype(bf16)

    def mm_w4(r, a, n0=0, n1=D):
        h2 = jnp.dot(a, w4b[:, n0:n1], preferred_element_type=f32)
        ob[rows(r, T), n0:n1] = (x2s[rows(r, T), n0:n1]
                                 + modb[4, 0:1, n0:n1] * (h2s[rows(r, T), n0:n1] + h2)).astype(bf16)

    with _scope("pre_a"):
        with _scope("w_modA"):
            mod_copies[0].wait()
            q_copies[0].wait()
        mac_inv(CT - 1, 0, 0)
        sa, ca, ga = mod_part(0)
        modb[0] = ga * sa
        modb[1] = ga * (1.0 + ca)
        for a in (3, 2, 1):
            mac_inv(CT - 1, a, 0)
        for o in range(0, P0, RG):
            ht[o:o + RG, :] = a_part1(o, o, None)
    with _scope("pre_b"):
        with _scope("w_modB"):
            mod_copies[1].wait()
        sb, cb = mod_part(1)
        modb[2] = sb
        modb[3] = 1.0 + cb
        for o in range(0, P0, RG):
            a_part2(o, ht[o:o + RG, :])
    with _scope("r1"):
        with _scope("w_w1"):
            w_copies[0].wait()
        mm_w1(0, P0)
    with _scope("r2"):
        with _scope("w_w2"):
            w_copies[1].wait()
        mm_w2(0, chained=False)
    with _scope("r3"):
        with _scope("w_w3a"):
            q_copies[1].wait()
            w_copies[2].wait()
        act_a = mm_w3(0, FH)
        half = (P1 // RG // 2) * RG
        prev = None
        for o in range(0, half, RG):
            prev = a_part2(o, a_part1(P0 + o, o, prev if o % (2 * RG) == 0 else None))
    with _scope("r4"):
        with _scope("w_w3b"):
            w_copies[3].wait()
        act_b = mm_w3(FH, F)
        prev = None
        for o in range(half, P1, RG):
            prev = a_part2(o, a_part1(P0 + o, o, prev if o % (2 * RG) == 0 else None))
        mm_w1(P0, P1)
    with _scope("r5"):
        with _scope("w_w4"):
            q_copies[2].wait()
            w_copies[4].wait()
            mod_copies[2].wait()
        mm_w2(T)
        modb[4] = mod_part(2)[0]
        mm_w4(0, jnp.concatenate([act_a, act_b], axis=-1))
        a_chain(P0 + P1, PC)
        out_copy(0).start()
        q_copies[3].wait()

    def mlp_body(i, carry):
        r1 = pl.multiple_of(P0 + P1 - PC + PC * i, 16)
        r = pl.multiple_of(i * T, T)
        mm_w1(r1, PC)
        act = mm_w3()
        mm_w2(r + T)
        mm_w4(r, act)
        a_chain(pl.multiple_of(jnp.minimum(r1 + PC, S - PC), 16), PC)
        out_copy(i).start()
        return carry

    with _scope("loop"):
        jax.lax.fori_loop(1, NC - 1, mlp_body, 0)
    with _scope("last"):
        mm_w4(S - T, mm_w3())
        out_copy(NC - 1).start()
    with _scope("fin"):
        for i in range(NC):
            out_copy(i).wait()


@jax.jit
def pallas_adaLN_cond__ssm_conv_h3__mixer_s_mlp__prompt_kernel(
    A_q: jax.Array,
    A_k: jax.Array,
    A_v: jax.Array,
    A_shift_k: jax.Array,
    A_ssm_k: jax.Array,
    A_ssm_D: jax.Array,
    B_x: jax.Array,
    B_w1: jax.Array,
    B_w2: jax.Array,
    B_w3: jax.Array,
    B_w4: jax.Array,
    c: jax.Array,
    w_mod: jax.Array,
):
    del B_x
    any_spec = pl.BlockSpec(memory_space=pl.ANY)
    vm = pltpu.VMEM
    dma = pltpu.SemaphoreType.DMA
    out = pl.pallas_call(
        _kernel,
        in_specs=[any_spec] * 12,
        out_specs=any_spec,
        out_shape=jax.ShapeDtypeStruct((S, D), bf16),
        scratch_shapes=[
            vm((CT, S + 16, 128), bf16), vm((CT, S, 128), bf16), vm((CT, 128, S), bf16),
            vm((S, D), bf16), vm((D, D), bf16), vm((D, D), bf16), vm((F, D), bf16), vm((F, D), bf16),
            vm((D, 6 * D), bf16), vm((4, D), bf16), vm((D,), bf16), vm((1, D), bf16),
            vm((4, 128, 128), u32), vm((4, 128, 128), u32), vm((4, 64, 256), u32),
            vm((CT, 5, 8, 128), f32),
            vm((2, NB, 4, 256, 128), f32), vm((2, NB, 4, 256, 128), f32), vm((4, 128, 128), f32),
            vm((CT, S, 128), f32), vm((5, 8, D), f32),
            vm((CT, S + 16, 128), f32), vm((S, D), f32), vm((S, D), f32),
            vm((P1, D), f32), vm((P1, D), f32), vm((P1 // 2, D), u32), vm((T // 2, D), u32),
            vm((S, D), bf16),
            dma((30,)), dma((NC,)),
        ],
        compiler_params=pltpu.CompilerParams(vmem_limit_bytes=110 << 20),
    )(A_q.reshape(S, D), A_k.reshape(S, D), A_v.reshape(S, D), A_shift_k.T, A_ssm_k,
      A_ssm_D, B_w1, B_w2, B_w3.T, B_w4, c, w_mod)
    return out.reshape(1, S, D)
```

```python
import os
import numpy as np
import jax
import jax.numpy as jnp
import jax.experimental.pallas as pl
import jax.experimental.pallas.tpu as pltpu

f32, bf16, u32, i32 = jnp.float32, jnp.bfloat16, jnp.uint32, jnp.int32

S, D, F = 2048, 640, 1728
CT = D // 128
NB, BLK, NFFT = 4, 512, 1024
T = 256
NC = S // T
CONV = 'U3,U2,U1,U0,a3,K3,b3,K2,a2,K1,b2,K0,a1,b1,a0,b0'
P0, P1, PC = 272, 336, 240
RG = 16
EPS = 1e-5
NT_DIMS = (((1,), (1,)), ((), ()))
SCOPES = bool(int(os.environ.get("KSCOPES", "0")))


class _NoScope:
    def __enter__(self):
        return self

    def __exit__(self, *a):
        return False


def _scope(name):
    return jax.named_scope(name) if SCOPES else _NoScope()


def _lo(w):
    return pltpu.bitcast(w << 16, f32)


def _hi(w):
    return pltpu.bitcast(w & jnp.uint32(0xFFFF0000), f32)


def _cos_turn(n32, scale):
    x = 2.0 ** 30 - jnp.abs(n32.astype(f32))
    b = 2.0 * np.pi / 2.0 ** 32
    x = x * b
    x2 = x * x
    c = [scale * v for v in (1.0, -1.0 / 6, 1.0 / 120, -1.0 / 5040, 1.0 / 362880)]
    return x * (c[0] + x2 * (c[1] + x2 * (c[2] + x2 * (c[3] + x2 * c[4]))))


def _odd_freq(k):
    return jnp.where(k < 64, 4 * k + 1, 4 * k - 253) << 21


def _fwd_table(r):
    w = jax.lax.broadcasted_iota(i32, (128, 128), 0)
    halves = []
    for par in range(2):
        row = 2 * w + par
        k = ((row >> 4) << 3) + (row & 7)
        halves.append(_cos_turn(_odd_freq(k) * r + ((row & 8) << 27), 1.0))
    return pltpu.pack_elementwise(halves, packed_dtype=bf16)


def _inv_table(p):
    w = jax.lax.broadcasted_iota(i32, (64, 256), 0)
    col = jax.lax.broadcasted_iota(i32, (64, 256), 1)
    fr = _odd_freq(col >> 1)
    off = (col & 1) << 30
    halves = [_cos_turn(fr * (8 * w + 4 * par + p) + off, 2.0 / NFFT) for par in range(2)]
    return pltpu.pack_elementwise(halves, packed_dtype=bf16)


def _stats(x, link=None, early=False):
    zero = 0.0 if link is None else jnp.minimum(link, 0.0)
    part = x[:, 0:128]
    for c in range(1, CT):
        part = part + x[:, c * 128:(c + 1) * 128]
    if link is not None and early:
        part = part + zero
        zero = 0.0
    m = jnp.sum(part, axis=-1, keepdims=True) * (1.0 / D)
    v = jnp.maximum(jnp.sum(x * x, axis=-1, keepdims=True) * (1.0 / D) - m * m, zero)
    return m, jax.lax.rsqrt(v + EPS)


def _gelu(x):
    c = 0.7978845608028654
    u = c + (c * 0.044715) * (x * x)
    t = jnp.tanh(x * u)
    hx = 0.5 * x
    return hx + hx * t


def _radix4(re, im, inverse):
    ar, ai = re[0] + re[2], im[0] + im[2]
    br, bi = re[0] - re[2], im[0] - im[2]
    cr, ci = re[1] + re[3], im[1] + im[3]
    dr, di = re[1] - re[3], im[1] - im[3]
    minus_i = (br + di, bi - dr)
    plus_i = (br - di, bi + dr)
    if inverse:
        return [(ar + cr, ai + ci), plus_i, (ar - cr, ai - ci), minus_i]
    return [(ar + cr, ai + ci), minus_i, (ar - cr, ai - ci), plus_i]


def _kernel(q_hbm, k_hbm, v_hbm, sh_hbm, sk_hbm, d_hbm, w1_hbm, w2_hbm, w3_hbm, w4_hbm,
            c_hbm, wm_hbm, o_hbm,
            kb, vb, skb, qb, w1b, w2b, w3b, w4b, wmb, shb, db, cb_, fub, fkb, gtb, par,
            US, KS, YP, ys, modb, h1s, h2s, x2s, zt, zb, ob,
            sem, sem_o):
    def sk_copy(c):
        return pltpu.make_async_copy(sk_hbm.at[pl.ds(c * 128, 128), :], skb.at[c], sem.at[c])

    def kv_copies(c):
        off = c * 128 if isinstance(c, int) else pl.multiple_of(c * 128, 128)
        return [
            pltpu.make_async_copy(k_hbm.at[:, pl.ds(off, 128)], kb.at[c, pl.ds(16, S), :], sem.at[CT + c]),
            pltpu.make_async_copy(v_hbm.at[:, pl.ds(off, 128)], vb.at[c], sem.at[2 * CT + c]),
        ]

    small = [pltpu.make_async_copy(src, dst, sem.at[15 + i]) for i, (src, dst) in enumerate(
        [(d_hbm, db), (sh_hbm, shb), (c_hbm, cb_)])]

    mod_cols = [(0, 3 * D), (3 * D, 2 * D), (5 * D, D)]
    mod_copies = [pltpu.make_async_copy(wm_hbm.at[:, pl.ds(o, n)], wmb.at[:, pl.ds(o, n)], sem.at[18 + i])
                  for i, (o, n) in enumerate(mod_cols)]
    w_pairs = [(w1_hbm, w1b), (w2_hbm, w2b), (w3_hbm, w3b), (w4_hbm, w4b)]
    w_copies = [pltpu.make_async_copy(src, dst, sem.at[21 + i]) for i, (src, dst) in enumerate(w_pairs)]
    q_rows = [(0, P0 + P1), (P0 + P1, PC), (P0 + P1 + PC, S - P0 - P1 - PC)]
    q_copies = [pltpu.make_async_copy(q_hbm.at[pl.ds(o, n), :], qb.at[pl.ds(o, n), :], sem.at[25 + i])
                for i, (o, n) in enumerate(q_rows)]

    def out_copy(i):
        r = i * T if isinstance(i, int) else pl.multiple_of(i * T, T)
        return pltpu.make_async_copy(ob.at[pl.ds(r, T), :], o_hbm.at[pl.ds(r, T), :], sem_o.at[i])

    sk_copy(0).start()
    for cp in small:
        cp.start()
    for cp in kv_copies(0):
        cp.start()
    for c in range(1, CT):
        sk_copy(c).start()
        for cp in kv_copies(c):
            cp.start()
    for cp in [mod_copies[0], q_copies[0], mod_copies[1], w_copies[0], w_copies[1],
               w_copies[2], q_copies[1], w_copies[3], mod_copies[2], q_copies[2]]:
        cp.start()

    with _scope("init"):
        def pin(i, carry):
            YP[i, 0:8, :] = jnp.zeros((8, 128), f32)
            return carry

        jax.lax.fori_loop(0, 2, pin, 0)
        lane = jax.lax.broadcasted_iota(i32, (128, 128), 1)
        for p in range(4):
            m = (lane - p) & 3
            fkb[p] = _fwd_table(128 * m + ((lane - m) & 127))
        for c in range(CT):
            kb[c, 0:16, :] = jnp.zeros((16, 128), bf16)
            h1s[c, 0:8, :] = jnp.zeros((8, 128), f32)
            h1s[c, S + 8:S + 16, :] = jnp.zeros((8, 128), f32)
        for p in range(4):
            fub[p] = _fwd_table(4 * lane + p)
        for cp in small:
            cp.wait()
        dv = db[...].astype(f32).reshape(1, D)
        shv = shb[...].astype(f32)
        for c in range(CT):
            for i in range(4):
                par[c, i] = jnp.broadcast_to(shv[i:i + 1, c * 128:(c + 1) * 128], (8, 128))
            par[c, 4] = jnp.broadcast_to(dv[:, c * 128:(c + 1) * 128], (8, 128))
    kw = kb.bitcast(u32)
    vw = vb.bitcast(u32)

    def re_(g):
        return slice(g * 16, g * 16 + 8)

    def im_(g):
        return slice(g * 16 + 8, g * 16 + 16)

    def fwd_k(c, j, sl=0):
        lane = jax.lax.broadcasted_iota(i32, (64, 128), 1)
        even = (lane & 1) == 0
        l01 = (lane & 2) == 0
        l12 = ((lane + 3) & 2) == 0
        rm = []
        for m in range(4):
            w = pltpu.bitcast(skb[c, :, (4 * j + m) * 128:(4 * j + m + 1) * 128], u32)
            rm.append(pltpu.roll(w, m, 1) if m else w)
        e01 = jnp.where(even, rm[0], rm[1])
        o01 = jnp.where(even, rm[1], rm[0])
        e23 = jnp.where(even, rm[2], rm[3])
        o23 = jnp.where(even, rm[3], rm[2])
        kp = [jnp.where(l01, e01, e23), jnp.where(l12, o01, o23),
              jnp.where(l01, e23, e01), jnp.where(l12, o23, o01)]
        tt = [jax.lax.dot_general(pltpu.bitcast(fkb[p], bf16), pltpu.bitcast(kp[p], bf16), NT_DIMS,
                                  preferred_element_type=f32) for p in range(4)]
        dvec = par[c, 4] if j == 0 else None
        for g in range(16):
            re = [t[re_(g)] for t in tt]
            im = [t[im_(g)] for t in tt]
            if j == 0:
                re[0] = re[0] + dvec
            x = _radix4(re, im, False)
            for m in range(4):
                xr, xi = x[m]
                KS[sl, j, m, re_(g), :] = xr
                KS[sl, j, m, im_(g), :] = xi
                if j < NB - 1:
                    nr, ni = KS[sl, j + 1, m, re_(g), :], KS[sl, j + 1, m, im_(g), :]
                    if g < 8:
                        nr, ni = nr - xi, ni + xr
                    else:
                        nr, ni = nr + xi, ni - xr
                    KS[sl, j + 1, m, re_(g), :] = nr
                    KS[sl, j + 1, m, im_(g), :] = ni

    def fwd_u(c, a, sl=0):
        w0, w1, w2, w3 = [jnp.tile(par[c, i], (16, 1)) for i in range(4)]
        base = 8 + a * 256
        ka = kw[c, pl.ds(base, 128, stride=2), :]
        kb2 = kw[c, pl.ds(base + 1, 128, stride=2), :]
        ka1 = kw[c, pl.ds(base - 2, 128, stride=2), :]
        kb1 = kw[c, pl.ds(base - 1, 128, stride=2), :]
        va = vw[c, pl.ds(a * 256, 128, stride=2), :]
        vb2 = vw[c, pl.ds(a * 256 + 1, 128, stride=2), :]
        k0, k1, k2, k3 = _lo(ka), _hi(ka), _lo(kb2), _hi(kb2)
        km3, km2, km1 = _hi(ka1), _lo(kb1), _hi(kb1)
        s0 = w0 * k0 + w1 * km1 + w2 * km2 + w3 * km3
        s1 = w0 * k1 + w1 * k0 + w2 * km1 + w3 * km2
        s2 = w0 * k2 + w1 * k1 + w2 * k0 + w3 * km1
        s3 = w0 * k3 + w1 * k2 + w2 * k1 + w3 * k0
        kv = [s0 * _lo(va), s1 * _hi(va), s2 * _lo(vb2), s3 * _hi(vb2)]
        tt = [jnp.dot(pltpu.bitcast(fub[p], bf16), kv[p].astype(bf16), preferred_element_type=f32)
              for p in range(4)]
        for g in range(16):
            x = _radix4([t[re_(g)] for t in tt], [t[im_(g)] for t in tt], False)
            for m in range(4):
                US[sl, a, m, re_(g), :] = x[m][0]
                US[sl, a, m, im_(g), :] = x[m][1]

    def mac_inv(c, a, sl=0, halves=(0, 1)):
        for h in halves:
            words = [[] for _ in range(4)]
            for g in range(8 * h, 8 * h + 8):
                yre, yim = [], []
                for m in range(4):
                    yr = yi = None
                    for j in range(a + 1):
                        kr, ki = KS[sl, j, m, re_(g), :], KS[sl, j, m, im_(g), :]
                        ur, ui = US[sl, a - j, m, re_(g), :], US[sl, a - j, m, im_(g), :]
                        tr = kr * ur - ki * ui
                        ti = kr * ui + ki * ur
                        yr = tr if yr is None else yr + tr
                        yi = ti if yi is None else yi + ti
                    yre.append(yr)
                    yim.append(yi)
                pp = _radix4(yre, yim, True)
                for p in range(4):
                    words[p].append(pltpu.pack_elementwise([pp[p][0], pp[p][1]], packed_dtype=bf16))
            for p in range(4):
                pb = pltpu.bitcast(jnp.concatenate(words[p], axis=0), bf16)
                r = jnp.dot(pltpu.bitcast(gtb[p, :, h * 128:(h + 1) * 128], bf16), pb,
                            preferred_element_type=f32)
                if h == 0:
                    YP[p] = r
                else:
                    ys[c, pl.ds(a * BLK + p, 128, stride=4), :] = YP[p] + r

    desc = (3, 2, 1, 0)
    with _scope("conv_first"):
        with _scope("w_sk0"):
            sk_copy(0).wait()
        for j in desc:
            fwd_k(0, j)
        for p in range(4):
            gtb[p] = _inv_table(p)
        with _scope("w_kv0"):
            for cp in kv_copies(0):
                cp.wait()
        for a in desc:
            fwd_u(0, a)

    def conv_tile(s, sl):
        with _scope("w_tile"):
            sk_copy(s).wait()
            for cp in kv_copies(s):
                cp.wait()
        for tok in CONV.split(","):
            if tok[0] == "K":
                fwd_k(s, int(tok[1]), sl)
            elif tok[0] == "U":
                fwd_u(s, int(tok[1]), sl)
            else:
                mac_inv(s - 1, int(tok[1]), 1 - sl, (0,) if tok[0] == "a" else (1,))

    def conv_body(t, carry):
        conv_tile(2 * t + 1, 1)
        conv_tile(2 * t + 2, 0)
        return carry

    with _scope("conv_loop"):
        jax.lax.fori_loop(0, 2, conv_body, 0)

    def mod_part(part):
        cvec = cb_[...].astype(f32)
        sc = jnp.broadcast_to(cvec * jax.nn.sigmoid(cvec), (16, D)).astype(bf16)
        o, n = mod_cols[part]
        r = jnp.dot(sc, wmb[:, o:o + n], preferred_element_type=f32)[0:8]
        return [r[:, i * D:(i + 1) * D] for i in range(n // D)]

    def mvec(i):
        return modb[i, 0:1, :]

    def rows(r, n):
        return pl.ds(r, n)

    def load_q(r):
        return qb[rows(r, RG), :].astype(f32)

    def make_x2(r, q, st):
        y = jnp.concatenate([ys[c, rows(r, RG), :] for c in range(CT)], axis=-1)
        return q + (((q - st[0]) * st[1]) * mvec(1) + mvec(0)) * y

    def make_h2(x2, st):
        return ((x2 - st[0]) * st[1]) * mvec(3) + mvec(2)

    def pack_ln(x, st):
        return pltpu.bitcast(((x - st[0]) * st[1]).astype(bf16), u32)

    def a_chain(r_in, r_out):
        prev = None
        for o in range(0, PC, RG):
            q = load_q(r_in + o)
            x2 = make_x2(r_in + o, q, _stats(q, prev))
            x2s[rows(r_out + o, RG), :] = x2
            h2 = make_h2(x2, _stats(x2))
            h2s[rows(r_out + o, RG), :] = h2
            st = _stats(h2)
            zt[o // 2:(o + RG) // 2, :] = pack_ln(h2, st)
            prev = st[1]

    def mm_w1(r, n, o=0):
        z = pltpu.bitcast(zt[o // 2:(o + n) // 2, :], bf16)
        h1 = _gelu(jnp.dot(z, w1b[...], preferred_element_type=f32))
        for c in range(CT):
            h1s[c, rows(r + 8, n), :] = h1[:, c * 128:(c + 1) * 128]

    def mm_w2a(r):
        lane = jax.lax.broadcasted_iota(i32, (T, 128), 1)

        def sh(k, c):
            return h1s[c, rows(r + 8 + k, T), :]

        g = jnp.concatenate([
            sh(-1, 0),
            jnp.where(lane < 32, sh(-1, 1), sh(1, 1)),
            jnp.where(lane < 64, sh(1, 2), sh(-2, 2)),
            jnp.where(lane < 96, sh(-2, 3), sh(2, 3)),
            sh(2, 4)], axis=-1).astype(bf16)
        h2s[rows(r, T), :] = h2s[rows(r, T), :] + jnp.dot(g, w2b[...], preferred_element_type=f32)

    def mm_w2b(r):
        prev = None
        for o in range(0, T, RG):
            x1 = h2s[rows(r + o, RG), :]
            st = _stats(x1, prev, early=True)
            zb[o // 2:(o + RG) // 2, :] = pack_ln(x1, st)
            prev = st[1]

    def mm_w2(r):
        mm_w2a(r)
        mm_w2b(r)

    def mm_w3(f0=0, f1=F):
        z = pltpu.bitcast(zb[...], bf16)
        return _gelu(jax.lax.dot_general(z, w3b[f0:f1, :], NT_DIMS, preferred_element_type=f32)).astype(bf16)

    def mm_w4(r, a, n0=0, n1=D):
        h2 = jnp.dot(a, w4b[:, n0:n1], preferred_element_type=f32)
        ob[rows(r, T), n0:n1] = (x2s[rows(r, T), n0:n1]
                                 + modb[4, 0:1, n0:n1] * (h2s[rows(r, T), n0:n1] + h2)).astype(bf16)

    groups = list(range(0, P0 + P1, RG))
    with _scope("conv_last"):
        with _scope("w_modA"):
            mod_copies[0].wait()
        sa, ca, ga = mod_part(0)
        modb[0] = ga * sa
        modb[1] = ga * (1.0 + ca)
        for a in desc:
            mac_inv(CT - 1, a, 0)
    with _scope("pre_a"):
        with _scope("w_q0"):
            q_copies[0].wait()
        st1 = {o: _stats(load_q(o)) for o in groups}
        zt[0:8, 0:128] = jnp.zeros((8, 128), u32)
        st2 = {}
        for o in groups:
            x2 = make_x2(o, load_q(o), st1[o])
            x2s[o:o + RG, :] = x2
            st2[o] = _stats(x2)

    def pass_c(os_, links):
        st3 = {}
        prev = [None] * max(links, 1)
        for n, o in enumerate(os_):
            h2 = make_h2(x2s[o:o + RG, :], st2[o])
            h2s[o:o + RG, :] = h2
            st3[o] = _stats(h2, prev[n % len(prev)], early=True)
            if links:
                prev[n % links] = st3[o][1]
                zt[o // 2:(o + RG) // 2, :] = pack_ln(h2, st3[o])
        if not links:
            for o in os_:
                zt[o // 2:(o + RG) // 2, :] = pack_ln(h2s[o:o + RG, :], st3[o])

    with _scope("pre_b"):
        with _scope("w_modB"):
            mod_copies[1].wait()
        sb, cb = mod_part(1)
        modb[2] = sb
        modb[3] = 1.0 + cb
        pass_c([o for o in groups if o < P0], 0)
    with _scope("r1"):
        with _scope("w_w1"):
            w_copies[0].wait()
        mm_w1(0, P0)
        pass_c([o for o in groups if o >= P0], 2)
    with _scope("r2"):
        with _scope("w_w2"):
            w_copies[1].wait()
        mm_w2(0)
        mm_w1(P0, P1, P0)
    with _scope("r3"):
        with _scope("w_w3"):
            w_copies[2].wait()
            q_copies[1].wait()
        a_chain(P0 + P1, P0 + P1)
        act = mm_w3()
        mm_w2a(T)
    with _scope("r4"):
        with _scope("w_w4"):
            w_copies[3].wait()
            mod_copies[2].wait()
        modb[4] = mod_part(2)[0]
        mm_w4(0, act)
        mm_w2b(T)
        out_copy(0).start()
        q_copies[2].wait()

    def mlp_body(i, carry):
        r1 = pl.multiple_of(P0 + P1 - PC + PC * i, 16)
        r = pl.multiple_of(i * T, T)
        mm_w1(r1, PC)
        a_chain(pl.multiple_of(jnp.minimum(r1 + PC, S - PC), 16), r1 + PC)
        act = mm_w3()
        mm_w2(r + T)
        mm_w4(r, act)
        out_copy(i).start()
        return carry

    with _scope("loop"):
        jax.lax.fori_loop(1, NC - 1, mlp_body, 0)
    with _scope("last"):
        mm_w4(S - T, mm_w3())
        out_copy(NC - 1).start()
    with _scope("fin"):
        for i in range(NC):
            out_copy(i).wait()


@jax.jit
def pallas_adaLN_cond__ssm_conv_h3__mixer_s_mlp__prompt_kernel(
    A_q: jax.Array,
    A_k: jax.Array,
    A_v: jax.Array,
    A_shift_k: jax.Array,
    A_ssm_k: jax.Array,
    A_ssm_D: jax.Array,
    B_x: jax.Array,
    B_w1: jax.Array,
    B_w2: jax.Array,
    B_w3: jax.Array,
    B_w4: jax.Array,
    c: jax.Array,
    w_mod: jax.Array,
):
    del B_x
    any_spec = pl.BlockSpec(memory_space=pl.ANY)
    vm = pltpu.VMEM
    dma = pltpu.SemaphoreType.DMA
    out = pl.pallas_call(
        _kernel,
        in_specs=[any_spec] * 12,
        out_specs=any_spec,
        out_shape=jax.ShapeDtypeStruct((S, D), bf16),
        scratch_shapes=[
            vm((CT, S + 16, 128), bf16), vm((CT, S, 128), bf16), vm((CT, 128, S), bf16),
            vm((S, D), bf16), vm((D, D), bf16), vm((D, D), bf16), vm((F, D), bf16), vm((F, D), bf16),
            vm((D, 6 * D), bf16), vm((4, D), bf16), vm((D,), bf16), vm((1, D), bf16),
            vm((4, 128, 128), u32), vm((4, 128, 128), u32), vm((4, 64, 256), u32),
            vm((CT, 5, 8, 128), f32),
            vm((2, NB, 4, 256, 128), f32), vm((2, NB, 4, 256, 128), f32), vm((4, 128, 128), f32),
            vm((CT, S, 128), f32), vm((5, 8, D), f32),
            vm((CT, S + 16, 128), f32), vm((S + PC, D), f32), vm((S + PC, D), f32),
            vm(((P0 + P1) // 2, D), u32), vm((T // 2, D), u32),
            vm((S, D), bf16),
            dma((28,)), dma((NC,)),
        ],
        compiler_params=pltpu.CompilerParams(vmem_limit_bytes=110 << 20, disable_bounds_checks=True,
                                             disable_semaphore_checks=True),
    )(A_q.reshape(S, D), A_k.reshape(S, D), A_v.reshape(S, D), A_shift_k.T, A_ssm_k,
      A_ssm_D, B_w1, B_w2, B_w3.T, B_w4, c, w_mod)
    return out.reshape(1, S, D)
```

```python
import os
import numpy as np
import jax
import jax.numpy as jnp
import jax.experimental.pallas as pl
import jax.experimental.pallas.tpu as pltpu

f32, bf16, u32, i32 = jnp.float32, jnp.bfloat16, jnp.uint32, jnp.int32

S, D, F = 2048, 640, 1728
CT = D // 128
NB, BLK, NFFT = 4, 512, 1024
T = 256
NC = S // T
LBAL = bool(int(os.environ.get('LBAL', '0')))
LAST0 = int(os.environ.get('LAST0', '192'))
FM = (F // 128) * 128
CONV = 'U3,U2,U1,U0,a3,K3,b3,K2,a2,K1,b2,K0,a1,b1,a0,b0'
P0, P1, PC = 320, 288, 240
RG = 16
EPS = 1e-5
NT_DIMS = (((1,), (1,)), ((), ()))
SCOPES = bool(int(os.environ.get("KSCOPES", "0")))


class _NoScope:
    def __enter__(self):
        return self

    def __exit__(self, *a):
        return False


def _scope(name):
    return jax.named_scope(name) if SCOPES else _NoScope()


def _lo(w):
    return pltpu.bitcast(w << 16, f32)


def _hi(w):
    return pltpu.bitcast(w & jnp.uint32(0xFFFF0000), f32)


def _cos_turn(n32, scale):
    x = 2.0 ** 30 - jnp.abs(n32.astype(f32))
    b = 2.0 * np.pi / 2.0 ** 32
    x = x * b
    x2 = x * x
    c = [scale * v for v in (1.0, -1.0 / 6, 1.0 / 120, -1.0 / 5040, 1.0 / 362880)]
    return x * (c[0] + x2 * (c[1] + x2 * (c[2] + x2 * (c[3] + x2 * c[4]))))


def _odd_freq(k):
    return jnp.where(k < 64, 4 * k + 1, 4 * k - 253) << 21


def _fwd_table(r):
    w = jax.lax.broadcasted_iota(i32, (128, 128), 0)
    halves = []
    for par in range(2):
        row = 2 * w + par
        k = ((row >> 4) << 3) + (row & 7)
        halves.append(_cos_turn(_odd_freq(k) * r + ((row & 8) << 27), 1.0))
    return pltpu.pack_elementwise(halves, packed_dtype=bf16)


def _inv_table(p):
    w = jax.lax.broadcasted_iota(i32, (64, 256), 0)
    col = jax.lax.broadcasted_iota(i32, (64, 256), 1)
    fr = _odd_freq(col >> 1)
    off = (col & 1) << 30
    halves = [_cos_turn(fr * (8 * w + 4 * par + p) + off, 2.0 / NFFT) for par in range(2)]
    return pltpu.pack_elementwise(halves, packed_dtype=bf16)


def _stats(x, link=None, early=False):
    zero = 0.0 if link is None else jnp.minimum(link, 0.0)
    part = x[:, 0:128]
    for c in range(1, CT):
        part = part + x[:, c * 128:(c + 1) * 128]
    if link is not None and early:
        part = part + zero
        zero = 0.0
    m = jnp.sum(part, axis=-1, keepdims=True) * (1.0 / D)
    v = jnp.maximum(jnp.sum(x * x, axis=-1, keepdims=True) * (1.0 / D) - m * m, zero)
    return m, jax.lax.rsqrt(v + EPS)


def _gelu(x):
    c = 0.7978845608028654
    u = c + (c * 0.044715) * (x * x)
    t = jnp.tanh(x * u)
    hx = 0.5 * x
    return hx + hx * t


def _row_parts(m, parts):
    base, extra = divmod(m // 16, parts)
    out, o = [], 0
    for i in range(parts):
        n = 16 * (base + (1 if i < extra else 0))
        out.append((o, n))
        o += n
    return out


def _dot_balanced(x, wslice, n_cols, parts, nt=False):
    def mm(a, c0, c1):
        if nt:
            return jax.lax.dot_general(a, wslice(c0, c1), NT_DIMS, preferred_element_type=f32)
        return jnp.dot(a, wslice(c0, c1), preferred_element_type=f32)
    if parts == 1:
        return mm(x, 0, n_cols)
    head = mm(x, 0, n_cols - 128)
    last = jnp.concatenate([mm(x[o:o + n], n_cols - 128, n_cols) for o, n in _row_parts(x.shape[0], parts)],
                           axis=0)
    return jnp.concatenate([head, last], axis=-1)


def _radix4(re, im, inverse):
    ar, ai = re[0] + re[2], im[0] + im[2]
    br, bi = re[0] - re[2], im[0] - im[2]
    cr, ci = re[1] + re[3], im[1] + im[3]
    dr, di = re[1] - re[3], im[1] - im[3]
    minus_i = (br + di, bi - dr)
    plus_i = (br - di, bi + dr)
    if inverse:
        return [(ar + cr, ai + ci), plus_i, (ar - cr, ai - ci), minus_i]
    return [(ar + cr, ai + ci), minus_i, (ar - cr, ai - ci), plus_i]


def _kernel(q_hbm, k_hbm, v_hbm, sh_hbm, sk_hbm, d_hbm, w1_hbm, w2_hbm, w3_hbm, w4_hbm,
            c_hbm, wm_hbm, o_hbm,
            kb, vb, skb, qb, w1b, w2b, w3b, w4b, wmb, shb, db, cb_, fub, fkb, gtb, par,
            US, KS, YP, ys, modb, h1s, h2s, x2s, hss, zt, zb, ob,
            sem, sem_o):
    def sk_copy(c):
        return pltpu.make_async_copy(sk_hbm.at[pl.ds(c * 128, 128), :], skb.at[c], sem.at[c])

    def kv_copies(c):
        off = c * 128 if isinstance(c, int) else pl.multiple_of(c * 128, 128)
        return [
            pltpu.make_async_copy(k_hbm.at[:, pl.ds(off, 128)], kb.at[c, pl.ds(16, S), :], sem.at[CT + c]),
            pltpu.make_async_copy(v_hbm.at[:, pl.ds(off, 128)], vb.at[c], sem.at[2 * CT + c]),
        ]

    small = [pltpu.make_async_copy(src, dst, sem.at[15 + i]) for i, (src, dst) in enumerate(
        [(d_hbm, db), (sh_hbm, shb), (c_hbm, cb_)])]

    mod_cols = [(0, 3 * D), (3 * D, 2 * D), (5 * D, D)]
    mod_copies = [pltpu.make_async_copy(wm_hbm.at[:, pl.ds(o, n)], wmb.at[:, pl.ds(o, n)], sem.at[18 + i])
                  for i, (o, n) in enumerate(mod_cols)]
    w_pairs = [(w1_hbm, w1b), (w2_hbm, w2b), (w3_hbm, w3b), (w4_hbm, w4b)]
    w_copies = [pltpu.make_async_copy(src, dst, sem.at[21 + i]) for i, (src, dst) in enumerate(w_pairs)]
    q_rows = [(0, P0 + P1), (P0 + P1, PC), (P0 + P1 + PC, S - P0 - P1 - PC)]
    q_copies = [pltpu.make_async_copy(q_hbm.at[pl.ds(o, n), :], qb.at[pl.ds(o, n), :], sem.at[25 + i])
                for i, (o, n) in enumerate(q_rows)]

    def out_copy(i):
        r = i * T if isinstance(i, int) else pl.multiple_of(i * T, T)
        return pltpu.make_async_copy(ob.at[pl.ds(r, T), :], o_hbm.at[pl.ds(r, T), :], sem_o.at[i])

    out_tail = [pltpu.make_async_copy(ob.at[pl.ds(o, n), :], o_hbm.at[pl.ds(o, n), :], sem_o.at[NC - 1 + i])
                for i, (o, n) in enumerate([(S - T, LAST0), (S - T + LAST0, T - LAST0)])]

    sk_copy(0).start()
    for cp in small:
        cp.start()
    for cp in kv_copies(0):
        cp.start()
    for c in range(1, CT):
        sk_copy(c).start()
        for cp in kv_copies(c):
            cp.start()
    for cp in [mod_copies[0], q_copies[0], mod_copies[1], w_copies[0], w_copies[1],
               w_copies[2], q_copies[1], w_copies[3], mod_copies[2], q_copies[2]]:
        cp.start()

    with _scope("init"):
        def pin(i, carry):
            YP[i, 0:8, :] = jnp.zeros((8, 128), f32)
            return carry

        jax.lax.fori_loop(0, 2, pin, 0)
        lane = jax.lax.broadcasted_iota(i32, (128, 128), 1)
        for p in range(4):
            m = (lane - p) & 3
            fkb[p] = _fwd_table(128 * m + ((lane - m) & 127))
        for c in range(CT):
            kb[c, 0:16, :] = jnp.zeros((16, 128), bf16)
            h1s[c, 0:8, :] = jnp.zeros((8, 128), f32)
            h1s[c, S + 8:S + 16, :] = jnp.zeros((8, 128), f32)
        for p in range(4):
            fub[p] = _fwd_table(4 * lane + p)
        for cp in small:
            cp.wait()
        dv = db[...].astype(f32).reshape(1, D)
        shv = shb[...].astype(f32)
        for c in range(CT):
            for i in range(4):
                par[c, i] = jnp.broadcast_to(shv[i:i + 1, c * 128:(c + 1) * 128], (8, 128))
            par[c, 4] = jnp.broadcast_to(dv[:, c * 128:(c + 1) * 128], (8, 128))
    kw = kb.bitcast(u32)
    vw = vb.bitcast(u32)

    def re_(g):
        return slice(g * 16, g * 16 + 8)

    def im_(g):
        return slice(g * 16 + 8, g * 16 + 16)

    def fwd_k(c, j, sl=0):
        lane = jax.lax.broadcasted_iota(i32, (64, 128), 1)
        even = (lane & 1) == 0
        l01 = (lane & 2) == 0
        l12 = ((lane + 3) & 2) == 0
        rm = []
        for m in range(4):
            w = pltpu.bitcast(skb[c, :, (4 * j + m) * 128:(4 * j + m + 1) * 128], u32)
            rm.append(pltpu.roll(w, m, 1) if m else w)
        e01 = jnp.where(even, rm[0], rm[1])
        o01 = jnp.where(even, rm[1], rm[0])
        e23 = jnp.where(even, rm[2], rm[3])
        o23 = jnp.where(even, rm[3], rm[2])
        kp = [jnp.where(l01, e01, e23), jnp.where(l12, o01, o23),
              jnp.where(l01, e23, e01), jnp.where(l12, o23, o01)]
        tt = [jax.lax.dot_general(pltpu.bitcast(fkb[p], bf16), pltpu.bitcast(kp[p], bf16), NT_DIMS,
                                  preferred_element_type=f32) for p in range(4)]
        dvec = par[c, 4] if j == 0 else None
        for g in range(16):
            re = [t[re_(g)] for t in tt]
            im = [t[im_(g)] for t in tt]
            if j == 0:
                re[0] = re[0] + dvec
            x = _radix4(re, im, False)
            for m in range(4):
                xr, xi = x[m]
                KS[sl, j, m, re_(g), :] = xr
                KS[sl, j, m, im_(g), :] = xi
                if j < NB - 1:
                    nr, ni = KS[sl, j + 1, m, re_(g), :], KS[sl, j + 1, m, im_(g), :]
                    if g < 8:
                        nr, ni = nr - xi, ni + xr
                    else:
                        nr, ni = nr + xi, ni - xr
                    KS[sl, j + 1, m, re_(g), :] = nr
                    KS[sl, j + 1, m, im_(g), :] = ni

    def fwd_u(c, a, sl=0):
        w0, w1, w2, w3 = [jnp.tile(par[c, i], (16, 1)) for i in range(4)]
        base = 8 + a * 256
        ka = kw[c, pl.ds(base, 128, stride=2), :]
        kb2 = kw[c, pl.ds(base + 1, 128, stride=2), :]
        ka1 = kw[c, pl.ds(base - 2, 128, stride=2), :]
        kb1 = kw[c, pl.ds(base - 1, 128, stride=2), :]
        va = vw[c, pl.ds(a * 256, 128, stride=2), :]
        vb2 = vw[c, pl.ds(a * 256 + 1, 128, stride=2), :]
        k0, k1, k2, k3 = _lo(ka), _hi(ka), _lo(kb2), _hi(kb2)
        km3, km2, km1 = _hi(ka1), _lo(kb1), _hi(kb1)
        s0 = w0 * k0 + w1 * km1 + w2 * km2 + w3 * km3
        s1 = w0 * k1 + w1 * k0 + w2 * km1 + w3 * km2
        s2 = w0 * k2 + w1 * k1 + w2 * k0 + w3 * km1
        s3 = w0 * k3 + w1 * k2 + w2 * k1 + w3 * k0
        kv = [s0 * _lo(va), s1 * _hi(va), s2 * _lo(vb2), s3 * _hi(vb2)]
        tt = [jnp.dot(pltpu.bitcast(fub[p], bf16), kv[p].astype(bf16), preferred_element_type=f32)
              for p in range(4)]
        for g in range(16):
            x = _radix4([t[re_(g)] for t in tt], [t[im_(g)] for t in tt], False)
            for m in range(4):
                US[sl, a, m, re_(g), :] = x[m][0]
                US[sl, a, m, im_(g), :] = x[m][1]

    def mac_inv(c, a, sl=0, halves=(0, 1)):
        for h in halves:
            words = [[] for _ in range(4)]
            for g in range(8 * h, 8 * h + 8):
                yre, yim = [], []
                for m in range(4):
                    yr = yi = None
                    for j in range(a + 1):
                        kr, ki = KS[sl, j, m, re_(g), :], KS[sl, j, m, im_(g), :]
                        ur, ui = US[sl, a - j, m, re_(g), :], US[sl, a - j, m, im_(g), :]
                        tr = kr * ur - ki * ui
                        ti = kr * ui + ki * ur
                        yr = tr if yr is None else yr + tr
                        yi = ti if yi is None else yi + ti
                    yre.append(yr)
                    yim.append(yi)
                pp = _radix4(yre, yim, True)
                for p in range(4):
                    words[p].append(pltpu.pack_elementwise([pp[p][0], pp[p][1]], packed_dtype=bf16))
            for p in range(4):
                pb = pltpu.bitcast(jnp.concatenate(words[p], axis=0), bf16)
                r = jnp.dot(pltpu.bitcast(gtb[p, :, h * 128:(h + 1) * 128], bf16), pb,
                            preferred_element_type=f32)
                if h == 0:
                    YP[p] = r
                else:
                    ys[c, pl.ds(a * BLK + p, 128, stride=4), :] = YP[p] + r

    desc = (3, 2, 1, 0)
    with _scope("conv_first"):
        with _scope("w_sk0"):
            sk_copy(0).wait()
        for j in desc:
            fwd_k(0, j)
        for p in range(4):
            gtb[p] = _inv_table(p)
        with _scope("w_kv0"):
            for cp in kv_copies(0):
                cp.wait()
        for a in desc:
            fwd_u(0, a)

    def conv_tile(s, sl):
        with _scope("w_tile"):
            sk_copy(s).wait()
            for cp in kv_copies(s):
                cp.wait()
        for tok in CONV.split(","):
            if tok[0] == "K":
                fwd_k(s, int(tok[1]), sl)
            elif tok[0] == "U":
                fwd_u(s, int(tok[1]), sl)
            else:
                mac_inv(s - 1, int(tok[1]), 1 - sl, (0,) if tok[0] == "a" else (1,))

    def conv_body(t, carry):
        conv_tile(2 * t + 1, 1)
        conv_tile(2 * t + 2, 0)
        return carry

    with _scope("conv_loop"):
        jax.lax.fori_loop(0, 2, conv_body, 0)

    def mod_part(part, extra):
        cvec = cb_[...].astype(f32)
        act = cvec * jax.nn.sigmoid(cvec)

        def sc(k0, k1):
            return jnp.broadcast_to(act[:, k0:k1], (16, k1 - k0)).astype(bf16)

        o, n = mod_cols[part]
        e = 128 * extra
        r = jnp.dot(sc(0, D), wmb[:, o + e:o + n], preferred_element_type=f32)
        if extra:
            r0 = (jnp.dot(sc(0, D - 64), wmb[0:D - 64, o:o + e], preferred_element_type=f32)
                  + jnp.dot(sc(D - 64, D), wmb[D - 64:D, o:o + e], preferred_element_type=f32))
            r = jnp.concatenate([r0, r], axis=-1)
        r = r[0:8]
        return [r[:, i * D:(i + 1) * D] for i in range(n // D)]

    def mvec(i):
        return modb[i, 0:1, :]

    def rows(r, n):
        return pl.ds(r, n)

    def load_q(r):
        return qb[rows(r, RG), :].astype(f32)

    def make_x2(r, q, st):
        y = jnp.concatenate([ys[c, rows(r, RG), :] for c in range(CT)], axis=-1)
        return q + (((q - st[0]) * st[1]) * mvec(1) + mvec(0)) * y

    def make_h2(x2, st):
        return ((x2 - st[0]) * st[1]) * mvec(3) + mvec(2)

    def pack_ln(x, st):
        return pltpu.bitcast(((x - st[0]) * st[1]).astype(bf16), u32)

    def a_chain(r_in, r_out):
        prev = None
        for o in range(0, PC, RG):
            q = load_q(r_in + o)
            x2 = make_x2(r_in + o, q, _stats(q, prev))
            x2s[rows(r_out + o, RG), :] = x2
            st = _stats(x2)
            h2 = make_h2(x2s[rows(r_out + o, RG), :], st)
            h2s[rows(r_out + o, RG), :] = h2
            st = _stats(h2)
            zt[o // 2:(o + RG) // 2, :] = pack_ln(h2s[rows(r_out + o, RG), :], st)
            prev = st[1]

    def mm_w1(r, n, o=0, bal=True):
        z = pltpu.bitcast(zt[o // 2:(o + n) // 2, :], bf16)
        h1 = _gelu(_dot_balanced(z, lambda a, b: w1b[:, a:b], D, 4 if bal else 1))
        for c in range(CT):
            h1s[c, rows(r + 8, n), :] = h1[:, c * 128:(c + 1) * 128]

    def mm_w2a(r, bal=True):
        lane = jax.lax.broadcasted_iota(i32, (T, 128), 1)

        def sh(k, c):
            return h1s[c, rows(r + 8 + k, T), :]

        g = jnp.concatenate([
            sh(-1, 0),
            jnp.where(lane < 32, sh(-1, 1), sh(1, 1)),
            jnp.where(lane < 64, sh(1, 2), sh(-2, 2)),
            jnp.where(lane < 96, sh(-2, 3), sh(2, 3)),
            sh(2, 4)], axis=-1).astype(bf16)
        hss[rows(r, T), :] = _dot_balanced(g, lambda a, b: w2b[:, a:b], D, 4 if bal else 1)

    def mm_w2b(r, links=1):
        prev = [None] * links
        for n, o in enumerate(range(0, T, RG)):
            x1 = h2s[rows(r + o, RG), :] + hss[rows(r + o, RG), :]
            st = _stats(x1, prev[n % links], early=True)
            zb[o // 2:(o + RG) // 2, :] = pack_ln(x1, st)
            prev[n % links] = st[1]

    def mm_w3_main(bal=True):
        z = pltpu.bitcast(zb[...], bf16)
        return _gelu(_dot_balanced(z, lambda a, b: w3b[a:b, :], FM, 4 if bal else 1, nt=True)).astype(bf16)

    def mm_w3_tail():
        z = pltpu.bitcast(zb[...], bf16)
        tail = _gelu(jax.lax.dot_general(w3b[FM:F, :], z, NT_DIMS, preferred_element_type=f32))
        return tail.T.astype(bf16)

    def mm_w3(bal):
        tail = mm_w3_tail()
        return jnp.concatenate([mm_w3_main(bal), tail], axis=-1)

    def mm_w4(r, a, o=0, n=T, bal=True):
        h2 = _dot_balanced(a[o:o + n], lambda c0, c1: w4b[:, c0:c1], D, 2 if bal else 1)
        ob[rows(r + o, n), :] = (x2s[rows(r + o, n), :]
                                 + mvec(4) * ((h2s[rows(r + o, n), :] + hss[rows(r + o, n), :]) + h2)).astype(bf16)

    groups = list(range(0, P0 + P1, RG))
    with _scope("conv_last"):
        with _scope("w_modA"):
            mod_copies[0].wait()
        sa, ca, ga = mod_part(0, 1)
        modb[0] = ga * sa
        modb[1] = ga * (1.0 + ca)
        for a in desc:
            mac_inv(CT - 1, a, 0)
    with _scope("pre_a"):
        with _scope("w_q0"):
            q_copies[0].wait()
        st1 = {o: _stats(load_q(o)) for o in groups}
        zt[0:8, 0:128] = jnp.zeros((8, 128), u32)
        st2 = {}
        for o in groups:
            x2 = make_x2(o, load_q(o), st1[o])
            x2s[o:o + RG, :] = x2
            st2[o] = _stats(x2)

    def pass_c(os_, links):
        st3 = {}
        prev = [None] * max(links, 1)
        for n, o in enumerate(os_):
            h2 = make_h2(x2s[o:o + RG, :], st2[o])
            h2s[o:o + RG, :] = h2
            st3[o] = _stats(h2, prev[n % len(prev)], early=True)
            if links:
                prev[n % links] = st3[o][1]
                zt[o // 2:(o + RG) // 2, :] = pack_ln(h2, st3[o])
        if not links:
            for o in os_:
                zt[o // 2:(o + RG) // 2, :] = pack_ln(h2s[o:o + RG, :], st3[o])

    with _scope("pre_b"):
        with _scope("w_modB"):
            mod_copies[1].wait()
        sb, cb = mod_part(1, 2)
        modb[2] = sb
        modb[3] = 1.0 + cb
        pass_c([o for o in groups if o < P0], 0)
    with _scope("r1"):
        with _scope("w_w1"):
            w_copies[0].wait()
        mm_w1(0, P0)
        pass_c([o for o in groups if o >= P0], 2)
    with _scope("r2"):
        with _scope("w_w2"):
            w_copies[1].wait()
        mm_w2a(0)
        mm_w2b(0, 2)
        mm_w1(P0, P1, P0)
    with _scope("r3"):
        with _scope("w_w3"):
            w_copies[2].wait()
            q_copies[1].wait()
        a_chain(P0 + P1, P0 + P1)
        main = mm_w3_main()
        mm_w2a(T)
        act = jnp.concatenate([main, mm_w3_tail()], axis=-1)
    with _scope("r4"):
        with _scope("w_w4"):
            w_copies[3].wait()
            mod_copies[2].wait()
        modb[4] = mod_part(2, 1)[0]
        mm_w4(0, act)
        mm_w2b(T)
        out_copy(0).start()
        q_copies[2].wait()

    def mlp_body(i, carry):
        r1 = pl.multiple_of(P0 + P1 - PC + PC * i, 16)
        r = pl.multiple_of(i * T, T)
        mm_w1(r1, PC, bal=LBAL)
        a_chain(pl.multiple_of(jnp.minimum(r1 + PC, S - PC), 16), r1 + PC)
        act = mm_w3(LBAL)
        mm_w2a(r + T, bal=LBAL)
        mm_w2b(r + T)
        mm_w4(r, act, bal=LBAL)
        out_copy(i).start()
        return carry

    with _scope("loop"):
        jax.lax.fori_loop(1, NC - 1, mlp_body, 0)
    with _scope("last"):
        act = mm_w3(False)
        mm_w4(S - T, act, 0, LAST0, bal=False)
        out_tail[0].start()
        mm_w4(S - T, act, LAST0, T - LAST0, bal=False)
        out_tail[1].start()
    with _scope("fin"):
        for i in range(NC - 1):
            out_copy(i).wait()
        for cp in out_tail:
            cp.wait()


@jax.jit
def pallas_adaLN_cond__ssm_conv_h3__mixer_s_mlp__prompt_kernel(
    A_q: jax.Array,
    A_k: jax.Array,
    A_v: jax.Array,
    A_shift_k: jax.Array,
    A_ssm_k: jax.Array,
    A_ssm_D: jax.Array,
    B_x: jax.Array,
    B_w1: jax.Array,
    B_w2: jax.Array,
    B_w3: jax.Array,
    B_w4: jax.Array,
    c: jax.Array,
    w_mod: jax.Array,
):
    del B_x
    any_spec = pl.BlockSpec(memory_space=pl.ANY)
    vm = pltpu.VMEM
    dma = pltpu.SemaphoreType.DMA
    out = pl.pallas_call(
        _kernel,
        in_specs=[any_spec] * 12,
        out_specs=any_spec,
        out_shape=jax.ShapeDtypeStruct((S, D), bf16),
        scratch_shapes=[
            vm((CT, S + 16, 128), bf16), vm((CT, S, 128), bf16), vm((CT, 128, S), bf16),
            vm((S, D), bf16), vm((D, D), bf16), vm((D, D), bf16), vm((F, D), bf16), vm((F, D), bf16),
            vm((D, 6 * D), bf16), vm((4, D), bf16), vm((D,), bf16), vm((1, D), bf16),
            vm((4, 128, 128), u32), vm((4, 128, 128), u32), vm((4, 64, 256), u32),
            vm((CT, 5, 8, 128), f32),
            vm((2, NB, 4, 256, 128), f32), vm((2, NB, 4, 256, 128), f32), vm((4, 128, 128), f32),
            vm((CT, S, 128), f32), vm((5, 8, D), f32),
            vm((CT, S + 16, 128), f32), vm((S + PC, D), f32), vm((S + PC, D), f32), vm((S, D), f32),
            vm(((P0 + P1) // 2, D), u32), vm((T // 2, D), u32),
            vm((S, D), bf16),
            dma((28,)), dma((NC + 1,)),
        ],
        compiler_params=pltpu.CompilerParams(vmem_limit_bytes=110 << 20, disable_bounds_checks=True,
                                             disable_semaphore_checks=True),
    )(A_q.reshape(S, D), A_k.reshape(S, D), A_v.reshape(S, D), A_shift_k.T, A_ssm_k,
      A_ssm_D, B_w1, B_w2, B_w3.T, B_w4, c, w_mod)
    return out.reshape(1, S, D)
```

```python
import os
import numpy as np
import jax
import jax.numpy as jnp
import jax.experimental.pallas as pl
import jax.experimental.pallas.tpu as pltpu

f32, bf16, u32, i32 = jnp.float32, jnp.bfloat16, jnp.uint32, jnp.int32

S, D, F = 2048, 640, 1728
CT = D // 128
NB, BLK, NFFT = 4, 512, 1024
T = 256
NC = S // T
NL = int(os.environ.get('NL', '4'))
LBAL = bool(int(os.environ.get('LBAL', '0')))
LAST0 = int(os.environ.get('LAST0', '192'))
FM = (F // 128) * 128
E0 = int(os.environ.get('E0', '0'))
KGRP = [tuple(int(x) for x in g) for g in os.environ.get('KGRP', '0,12,34').split(',')]
TR = 8 * CT
P0, P1, PC = 320, 288, 240
RG = 16
EPS = 1e-5
NT_DIMS = (((1,), (1,)), ((), ()))
SCOPES = bool(int(os.environ.get("KSCOPES", "0")))


class _NoScope:
    def __enter__(self):
        return self

    def __exit__(self, *a):
        return False


def _scope(name):
    return jax.named_scope(name) if SCOPES else _NoScope()


def _lo(w):
    return pltpu.bitcast(w << 16, f32)


def _hi(w):
    return pltpu.bitcast(w & jnp.uint32(0xFFFF0000), f32)


def _cos_turn(n32, scale):
    x = 2.0 ** 30 - jnp.abs(n32.astype(f32))
    b = 2.0 * np.pi / 2.0 ** 32
    x = x * b
    x2 = x * x
    c = [scale * v for v in (1.0, -1.0 / 6, 1.0 / 120, -1.0 / 5040, 1.0 / 362880)]
    return x * (c[0] + x2 * (c[1] + x2 * (c[2] + x2 * (c[3] + x2 * c[4]))))


def _odd_freq(k):
    return jnp.where(k < 64, 4 * k + 1, 4 * k - 253) << 21


def _fwd_table(r):
    w = jax.lax.broadcasted_iota(i32, (128, 128), 0)
    halves = []
    for par in range(2):
        row = 2 * w + par
        k = ((row >> 4) << 3) + (row & 7)
        halves.append(_cos_turn(_odd_freq(k) * r + ((row & 8) << 27), 1.0))
    return pltpu.pack_elementwise(halves, packed_dtype=bf16)


def _inv_table(p):
    w = jax.lax.broadcasted_iota(i32, (64, 256), 0)
    col = jax.lax.broadcasted_iota(i32, (64, 256), 1)
    fr = _odd_freq(col >> 1)
    off = (col & 1) << 30
    halves = [_cos_turn(fr * (8 * w + 4 * par + p) + off, 2.0 / NFFT) for par in range(2)]
    return pltpu.pack_elementwise(halves, packed_dtype=bf16)


def _stats(x, link=None, early=False):
    zero = 0.0 if link is None else jnp.minimum(link, 0.0)
    part = x[:, 0:128]
    for c in range(1, CT):
        part = part + x[:, c * 128:(c + 1) * 128]
    if link is not None and early:
        part = part + zero
        zero = 0.0
    m = jnp.sum(part, axis=-1, keepdims=True) * (1.0 / D)
    v = jnp.maximum(jnp.sum(x * x, axis=-1, keepdims=True) * (1.0 / D) - m * m, zero)
    return m, jax.lax.rsqrt(v + EPS)


def _gelu(x):
    c = 0.7978845608028654
    u = c + (c * 0.044715) * (x * x)
    t = jnp.tanh(x * u)
    hx = 0.5 * x
    return hx + hx * t


def _row_parts(m, parts):
    base, extra = divmod(m // 16, parts)
    out, o = [], 0
    for i in range(parts):
        n = 16 * (base + (1 if i < extra else 0))
        out.append((o, n))
        o += n
    return out


def _dot_balanced(x, wslice, n_cols, parts, nt=False):
    def mm(a, c0, c1):
        if nt:
            return jax.lax.dot_general(a, wslice(c0, c1), NT_DIMS, preferred_element_type=f32)
        return jnp.dot(a, wslice(c0, c1), preferred_element_type=f32)
    if parts == 1:
        return mm(x, 0, n_cols)
    head = mm(x, 0, n_cols - 128)
    last = jnp.concatenate([mm(x[o:o + n], n_cols - 128, n_cols) for o, n in _row_parts(x.shape[0], parts)],
                           axis=0)
    return jnp.concatenate([head, last], axis=-1)


def _radix4(re, im, inverse):
    ar, ai = re[0] + re[2], im[0] + im[2]
    br, bi = re[0] - re[2], im[0] - im[2]
    cr, ci = re[1] + re[3], im[1] + im[3]
    dr, di = re[1] - re[3], im[1] - im[3]
    minus_i = (br + di, bi - dr)
    plus_i = (br - di, bi + dr)
    if inverse:
        return [(ar + cr, ai + ci), plus_i, (ar - cr, ai - ci), minus_i]
    return [(ar + cr, ai + ci), minus_i, (ar - cr, ai - ci), plus_i]


def _kernel(q_hbm, k_hbm, v_hbm, sh_hbm, sk_hbm, d_hbm, w1_hbm, w2_hbm, w3_hbm, w4_hbm,
            c_hbm, wm_hbm, o_hbm,
            kb, vb, skb, qb, w1b, w2b, w3b, w4b, wmb, shb, db, cb_, fub, fkb, gtb, par,
            US, KS, UR, YS, YP, ys, modb, h1s, h2s, x2s, hss, zt, zb, ob,
            sem, sem_o):
    def sk_copy(c):
        return pltpu.make_async_copy(sk_hbm.at[pl.ds(c * 128, 128), :], skb.at[c], sem.at[c])

    def kv_copies(a):
        n = BLK * CT
        return [
            pltpu.make_async_copy(k_hbm.at[pl.ds(a * n, n), :], kb.at[pl.ds(TR + a * n, n), :], sem.at[CT + a]),
            pltpu.make_async_copy(v_hbm.at[pl.ds(a * n, n), :], vb.at[pl.ds(a * n, n), :], sem.at[2 * CT + a]),
        ]

    small = [pltpu.make_async_copy(src, dst, sem.at[15 + i]) for i, (src, dst) in enumerate(
        [(d_hbm, db), (sh_hbm, shb), (c_hbm, cb_)])]

    mod_cols = [(0, 3 * D), (3 * D, 2 * D), (5 * D, D)]
    mod_copies = [pltpu.make_async_copy(wm_hbm.at[:, pl.ds(o, n)], wmb.at[:, pl.ds(o, n)], sem.at[18 + i])
                  for i, (o, n) in enumerate(mod_cols)]
    w_pairs = [(w1_hbm, w1b), (w2_hbm, w2b), (w3_hbm, w3b), (w4_hbm, w4b)]
    w_copies = [pltpu.make_async_copy(src, dst, sem.at[21 + i]) for i, (src, dst) in enumerate(w_pairs)]
    q_rows = [(0, P0 + P1), (P0 + P1, PC), (P0 + P1 + PC, S - P0 - P1 - PC)]
    q_copies = [pltpu.make_async_copy(q_hbm.at[pl.ds(o, n), :], qb.at[pl.ds(o, n), :], sem.at[25 + i])
                for i, (o, n) in enumerate(q_rows)]

    def out_copy(i):
        r = i * T if isinstance(i, int) else pl.multiple_of(i * T, T)
        return pltpu.make_async_copy(ob.at[pl.ds(r, T), :], o_hbm.at[pl.ds(r, T), :], sem_o.at[i])

    out_tail = [pltpu.make_async_copy(ob.at[pl.ds(o, n), :], o_hbm.at[pl.ds(o, n), :], sem_o.at[NC - 1 + i])
                for i, (o, n) in enumerate([(S - T, LAST0), (S - T + LAST0, T - LAST0)])]

    for cp in small + kv_copies(0):
        cp.start()
    for c in range(CT):
        sk_copy(c).start()
    for a in range(1, NB):
        for cp in kv_copies(a):
            cp.start()
    for cp in [mod_copies[0], q_copies[0], mod_copies[1], w_copies[0], w_copies[1],
               w_copies[2], q_copies[1], w_copies[3], mod_copies[2], q_copies[2]]:
        cp.start()

    with _scope("init"):
        def pin(i, carry):
            YP[i, 0:8, :] = jnp.zeros((8, 128), f32)
            US[i, 0, 0, 0:8, :] = jnp.zeros((8, 128), f32)
            KS[i, 0, 0, 0:8, :] = jnp.zeros((8, 128), f32)
            YS[i, 0, 0, 0:8, :] = jnp.zeros((8, 128), f32)
            UR[i, 0, 0:8, :] = jnp.zeros((8, 128), f32)
            return carry

        jax.lax.fori_loop(0, 2, pin, 0)
        lane = jax.lax.broadcasted_iota(i32, (128, 128), 1)
        for p in range(4):
            m = (lane - p) & 3
            fkb[p] = _fwd_table(128 * m + ((lane - m) & 127))
        for c in range(CT):
            kb[c * 8:(c + 1) * 8, :] = jnp.zeros((8, 128), bf16)
            h1s[c, 0:8, :] = jnp.zeros((8, 128), f32)
            h1s[c, S + 8:S + 16, :] = jnp.zeros((8, 128), f32)
        for p in range(4):
            fub[p] = _fwd_table(8 * (lane & 63) + ((lane >> 6) << 2) + p)
        for cp in small:
            cp.wait()
        dv = db[...].astype(f32).reshape(1, D)
        shv = shb[...].astype(f32)
        for c in range(CT):
            for i in range(4):
                par[c, i] = jnp.broadcast_to(shv[i:i + 1, c * 128:(c + 1) * 128], (8, 128))
            par[c, 4] = jnp.broadcast_to(dv[:, c * 128:(c + 1) * 128], (8, 128))
    def fence(i, carry):
        YP[i, 0:8, :] = jnp.zeros((8, 128), f32)
        return carry

    kw = kb.bitcast(u32)
    vw = vb.bitcast(u32)

    def re_(g):
        return slice(g * 16, g * 16 + 8)

    def im_(g):
        return slice(g * 16 + 8, g * 16 + 16)

    def fwd_k(c, j):
        lane = jax.lax.broadcasted_iota(i32, (64, 128), 1)
        even = (lane & 1) == 0
        l01 = (lane & 2) == 0
        l12 = ((lane + 3) & 2) == 0
        rm = []
        for m in range(4):
            w = pltpu.bitcast(skb[c, :, (4 * j + m) * 128:(4 * j + m + 1) * 128], u32)
            rm.append(pltpu.roll(w, m, 1) if m else w)
        e01 = jnp.where(even, rm[0], rm[1])
        o01 = jnp.where(even, rm[1], rm[0])
        e23 = jnp.where(even, rm[2], rm[3])
        o23 = jnp.where(even, rm[3], rm[2])
        kp = [jnp.where(l01, e01, e23), jnp.where(l12, o01, o23),
              jnp.where(l01, e23, e01), jnp.where(l12, o23, o01)]
        tt = [jax.lax.dot_general(pltpu.bitcast(fkb[p], bf16), pltpu.bitcast(kp[p], bf16), NT_DIMS,
                                  preferred_element_type=f32) for p in range(4)]
        dvec = par[c, 4] if j == 0 else None
        for g in range(16):
            re = [t[re_(g)] for t in tt]
            im = [t[im_(g)] for t in tt]
            if j == 0:
                re[0] = re[0] + dvec
            x = _radix4(re, im, False)
            for m in range(4):
                xr, xi = x[m]
                if j < NB - 1:
                    KS[c, j, m, re_(g), :] = xr
                    KS[c, j, m, im_(g), :] = xi
                ur, ui = US[c, 0, m, re_(g), :], US[c, 0, m, im_(g), :]
                YS[c, j, m, re_(g), :] = xr * ur - xi * ui
                YS[c, j, m, im_(g), :] = xr * ui + xi * ur

    def fwd_u(c, a):
        taps = [jnp.tile(par[c, i], (8, 1)) for i in range(4)]
        ws = TR // 2
        base = a * (BLK // 8) * ws + 4 * c

        def words(ref, start):
            return ref[pl.ds(start, BLK // 8, stride=ws), :]

        kk = {}
        for w in range(4):
            x = words(kw, ws + base + w)
            kk[2 * w], kk[2 * w + 1] = _lo(x), _hi(x)
        kk[-3] = _hi(words(kw, base + 2))
        x = words(kw, base + 3)
        kk[-2], kk[-1] = _lo(x), _hi(x)
        sub = []
        for w in range(4):
            x = words(vw, base + w)
            for r, vv in ((2 * w, _lo(x)), (2 * w + 1, _hi(x))):
                sh = taps[0] * kk[r] + taps[1] * kk[r - 1] + taps[2] * kk[r - 2] + taps[3] * kk[r - 3]
                sub.append(sh * vv)
        kv = [jnp.concatenate([sub[p], sub[p + 4]], axis=0) for p in range(4)]
        tt = [jnp.dot(pltpu.bitcast(fub[p], bf16), kv[p].astype(bf16), preferred_element_type=f32)
              for p in range(4)]
        for g in range(16):
            x = _radix4([t[re_(g)] for t in tt], [t[im_(g)] for t in tt], False)
            for m in range(4):
                xr, xi = x[m]
                if a:
                    if a == 1:
                        pr, pi = US[c, 0, m, re_(g), :], US[c, 0, m, im_(g), :]
                    else:
                        pr, pi = UR[c, m, re_(g), :], UR[c, m, im_(g), :]
                    if a < NB - 1:
                        UR[c, m, re_(g), :] = xr
                        UR[c, m, im_(g), :] = xi
                    if g < 8:
                        xr, xi = xr - pi, xi + pr
                    else:
                        xr, xi = xr + pi, xi - pr
                US[c, a, m, re_(g), :] = xr
                US[c, a, m, im_(g), :] = xi

    def mac_inv(c, a, halves=(0, 1)):
        for h in halves:
            words = [[] for _ in range(4)]
            for g in range(8 * h, 8 * h + 8):
                yre, yim = [], []
                for m in range(4):
                    yr, yi = YS[c, a, m, re_(g), :], YS[c, a, m, im_(g), :]
                    for j in range(a):
                        kr, ki = KS[c, j, m, re_(g), :], KS[c, j, m, im_(g), :]
                        ur, ui = US[c, a - j, m, re_(g), :], US[c, a - j, m, im_(g), :]
                        yr = yr + (kr * ur - ki * ui)
                        yi = yi + (kr * ui + ki * ur)
                    yre.append(yr)
                    yim.append(yi)
                pp = _radix4(yre, yim, True)
                for p in range(4):
                    words[p].append(pltpu.pack_elementwise([pp[p][0], pp[p][1]], packed_dtype=bf16))
            for p in range(4):
                pb = pltpu.bitcast(jnp.concatenate(words[p], axis=0), bf16)
                r = jnp.dot(pltpu.bitcast(gtb[p, :, h * 128:(h + 1) * 128], bf16), pb,
                            preferred_element_type=f32)
                if h == 0:
                    YP[p] = r
                else:
                    ys[c, pl.ds(a * BLK + p, 128, stride=4), :] = YP[p] + r

    desc = (3, 2, 1, 0)
    def k_tile(c):
        for j in desc:
            fwd_k(c, j)

    with _scope("conv_u0"):
        for p in range(4):
            gtb[p] = _inv_table(p)
        with _scope("w_kv"):
            for cp in kv_copies(0):
                cp.wait()
        for c in range(CT):
            fwd_u(c, 0)
    with _scope("conv_k"):
        done = 0
        for grp in KGRP:
            with _scope("w_sk"):
                for c in grp:
                    sk_copy(c).wait()
            for c in grp:
                k_tile(c)
            if grp is KGRP[-1]:
                for c in range(E0):
                    mac_inv(c, 0)
    for a in range(1, NB):
        with _scope("conv_u%d" % a):
            with _scope("w_kv"):
                for cp in kv_copies(a):
                    cp.wait()
            todo = [(c, a - 1) for c in range(CT)]
            if a == 1:
                todo = todo[E0:]
            late = len(todo) < CT
            for c in range(CT):
                fwd_u(c, a)
                if todo and (not late or c >= CT - len(todo)):
                    mac_inv(*todo.pop(0))

    def mod_cols_dot(o, n, extra):
        cvec = cb_[...].astype(f32)
        act = cvec * jax.nn.sigmoid(cvec)

        def sc(k0, k1):
            return jnp.broadcast_to(act[:, k0:k1], (16, k1 - k0)).astype(bf16)

        e = 128 * extra
        r = jnp.dot(sc(0, D), wmb[:, o + e:o + n], preferred_element_type=f32)
        if extra:
            r0 = (jnp.dot(sc(0, D - 64), wmb[0:D - 64, o:o + e], preferred_element_type=f32)
                  + jnp.dot(sc(D - 64, D), wmb[D - 64:D, o:o + e], preferred_element_type=f32))
            r = jnp.concatenate([r0, r], axis=-1)
        return r[0:8]

    def mod_part(part, extra):
        o, n = mod_cols[part]
        r = mod_cols_dot(o, n, extra)
        return [r[:, i * D:(i + 1) * D] for i in range(n // D)]

    def mvec(i):
        return modb[i, 0:1, :]

    def rows(r, n):
        return pl.ds(r, n)

    def load_q(r):
        return qb[rows(r, RG), :].astype(f32)

    def make_x2(r, q, st):
        y = jnp.concatenate([ys[c, rows(r, RG), :] for c in range(CT)], axis=-1)
        return q + (((q - st[0]) * st[1]) * mvec(1) + mvec(0)) * y

    def make_h2(x2, st):
        return ((x2 - st[0]) * st[1]) * mvec(3) + mvec(2)

    def pack_ln(x, st):
        return pltpu.bitcast(((x - st[0]) * st[1]).astype(bf16), u32)

    def a_chain(r_in, r_out):
        prev = None
        for o in range(0, PC, RG):
            q = load_q(r_in + o)
            x2 = make_x2(r_in + o, q, _stats(q, prev))
            x2s[rows(r_out + o, RG), :] = x2
            st = _stats(x2)
            h2 = make_h2(x2s[rows(r_out + o, RG), :], st)
            h2s[rows(r_out + o, RG), :] = h2
            st = _stats(h2)
            zt[o // 2:(o + RG) // 2, :] = pack_ln(h2s[rows(r_out + o, RG), :], st)
            prev = st[1]

    def mm_w1(r, n, o=0, bal=True):
        z = pltpu.bitcast(zt[o // 2:(o + n) // 2, :], bf16)
        h1 = _gelu(_dot_balanced(z, lambda a, b: w1b[:, a:b], D, 4 if bal else 1))
        for c in range(CT):
            h1s[c, rows(r + 8, n), :] = h1[:, c * 128:(c + 1) * 128]

    def mm_w2a(r, bal=True):
        lane = jax.lax.broadcasted_iota(i32, (T, 128), 1)

        def sh(k, c):
            return h1s[c, rows(r + 8 + k, T), :]

        g = jnp.concatenate([
            sh(-1, 0),
            jnp.where(lane < 32, sh(-1, 1), sh(1, 1)),
            jnp.where(lane < 64, sh(1, 2), sh(-2, 2)),
            jnp.where(lane < 96, sh(-2, 3), sh(2, 3)),
            sh(2, 4)], axis=-1).astype(bf16)
        hss[rows(r, T), :] = _dot_balanced(g, lambda a, b: w2b[:, a:b], D, 4 if bal else 1)

    def mm_w2b(r, links=1):
        prev = [None] * links
        for n, o in enumerate(range(0, T, RG)):
            x1 = h2s[rows(r + o, RG), :] + hss[rows(r + o, RG), :]
            st = _stats(x1, prev[n % links], early=True)
            zb[o // 2:(o + RG) // 2, :] = pack_ln(x1, st)
            prev[n % links] = st[1]

    def mm_w3_main(bal=True):
        z = pltpu.bitcast(zb[...], bf16)
        return _gelu(_dot_balanced(z, lambda a, b: w3b[a:b, :], FM, 4 if bal else 1, nt=True)).astype(bf16)

    def mm_w3_tail():
        z = pltpu.bitcast(zb[...], bf16)
        return _gelu(jax.lax.dot_general(w3b[FM:F, :], z, NT_DIMS, preferred_element_type=f32))

    def join_act(main, tail):
        return jnp.concatenate([main, tail.T.astype(bf16)], axis=-1)

    def mm_w3(bal):
        tail = mm_w3_tail()
        return join_act(mm_w3_main(bal), tail)

    def mm_w4(r, a, o=0, n=T, bal=True):
        h2 = _dot_balanced(a[o:o + n], lambda c0, c1: w4b[:, c0:c1], D, 2 if bal else 1)
        ob[rows(r + o, n), :] = (x2s[rows(r + o, n), :]
                                 + mvec(4) * ((h2s[rows(r + o, n), :] + hss[rows(r + o, n), :]) + h2)).astype(bf16)

    groups = list(range(0, P0 + P1, RG))
    with _scope("conv_last"):
        jax.lax.fori_loop(0, 2, fence, 0)
        for c in range(NL):
            mac_inv(c, NB - 1)
    with _scope("pre_a"):
        with _scope("w_q0"):
            mod_copies[0].wait()
            q_copies[0].wait()
        sa, ca, ga = mod_part(0, 1)
        modb[0] = ga * sa
        modb[1] = ga * (1.0 + ca)
        for c in range(NL, CT):
            mac_inv(c, NB - 1)
        st1 = {o: _stats(load_q(o)) for o in groups}
        zt[0:8, 0:128] = jnp.zeros((8, 128), u32)
        st2 = {}
        for o in groups:
            x2 = make_x2(o, load_q(o), st1[o])
            x2s[o:o + RG, :] = x2
            st2[o] = _stats(x2)

    def pass_c(os_, links):
        st3 = {}
        prev = [None] * max(links, 1)
        for n, o in enumerate(os_):
            h2 = make_h2(x2s[o:o + RG, :], st2[o])
            h2s[o:o + RG, :] = h2
            st3[o] = _stats(h2, prev[n % len(prev)], early=True)
            if links:
                prev[n % links] = st3[o][1]
                zt[o // 2:(o + RG) // 2, :] = pack_ln(h2, st3[o])
        if not links:
            for o in os_:
                zt[o // 2:(o + RG) // 2, :] = pack_ln(h2s[o:o + RG, :], st3[o])

    with _scope("pre_b"):
        with _scope("w_modB"):
            mod_copies[1].wait()
        sb, cb = mod_part(1, 2)
        modb[2] = sb
        modb[3] = 1.0 + cb
        pass_c([o for o in groups if o < P0], 0)
    with _scope("r1"):
        with _scope("w_w1"):
            w_copies[0].wait()
        mm_w1(0, P0)
        pass_c([o for o in groups if o >= P0], 2)
    with _scope("r2"):
        with _scope("w_w2"):
            w_copies[1].wait()
        mm_w2a(0)
        mm_w2b(0, 2)
        mm_w1(P0, P1, P0)
    with _scope("r3"):
        with _scope("w_w3"):
            w_copies[2].wait()
            q_copies[1].wait()
        a_chain(P0 + P1, P0 + P1)
        main = mm_w3_main()
        mm_w2a(T)
        tail = mm_w3_tail()
    with _scope("r4"):
        with _scope("w_w4"):
            w_copies[3].wait()
            mod_copies[2].wait()
        modb[4] = mod_part(2, 1)[0]
        mm_w4(0, join_act(main, tail))
        mm_w2b(T)
        out_copy(0).start()
        q_copies[2].wait()

    def mlp_iter(i):
        r1 = pl.multiple_of(P0 + P1 - PC + PC * i, 16)
        r = pl.multiple_of(i * T, T)
        mm_w1(r1, PC, bal=LBAL)
        a_chain(pl.multiple_of(jnp.minimum(r1 + PC, S - PC), 16), r1 + PC)
        act = mm_w3(LBAL)
        mm_w2a(r + T, bal=LBAL)
        mm_w2b(r + T)
        mm_w4(r, act, bal=LBAL)
        out_copy(i).start()

    def mlp_body(i, carry):
        with _scope("iter"):
            mlp_iter(i)
        return carry

    with _scope("loop"):
        jax.lax.fori_loop(1, NC - 1, mlp_body, 0)
    with _scope("last"):
        act = mm_w3(False)
        mm_w4(S - T, act, 0, LAST0, bal=False)
        out_tail[0].start()
        mm_w4(S - T, act, LAST0, T - LAST0, bal=False)
        out_tail[1].start()
    with _scope("fin"):
        for i in range(NC - 1):
            out_copy(i).wait()
        for cp in out_tail:
            cp.wait()


@jax.jit
def pallas_adaLN_cond__ssm_conv_h3__mixer_s_mlp__prompt_kernel(
    A_q: jax.Array,
    A_k: jax.Array,
    A_v: jax.Array,
    A_shift_k: jax.Array,
    A_ssm_k: jax.Array,
    A_ssm_D: jax.Array,
    B_x: jax.Array,
    B_w1: jax.Array,
    B_w2: jax.Array,
    B_w3: jax.Array,
    B_w4: jax.Array,
    c: jax.Array,
    w_mod: jax.Array,
):
    del B_x
    any_spec = pl.BlockSpec(memory_space=pl.ANY)

    def tile_view(x):
        return x.reshape(S // 8, 8, CT, 128).transpose(0, 2, 1, 3).reshape(S * CT, 128)

    vm = pltpu.VMEM
    dma = pltpu.SemaphoreType.DMA
    out = pl.pallas_call(
        _kernel,
        in_specs=[any_spec] * 12,
        out_specs=any_spec,
        out_shape=jax.ShapeDtypeStruct((S, D), bf16),
        scratch_shapes=[
            vm((S * CT + TR, 128), bf16), vm((S * CT, 128), bf16), vm((CT, 128, S), bf16),
            vm((S, D), bf16), vm((D, D), bf16), vm((D, D), bf16), vm((F, D), bf16), vm((F, D), bf16),
            vm((D, 6 * D), bf16), vm((4, D), bf16), vm((D,), bf16), vm((1, D), bf16),
            vm((4, 128, 128), u32), vm((4, 128, 128), u32), vm((4, 64, 256), u32),
            vm((CT, 5, 8, 128), f32),
            vm((CT, NB, 4, 256, 128), f32), vm((CT, NB - 1, 4, 256, 128), f32),
            vm((CT, 4, 256, 128), f32), vm((CT, NB, 4, 256, 128), f32), vm((4, 128, 128), f32),
            vm((CT, S, 128), f32), vm((5, 8, D), f32),
            vm((CT, S + 16, 128), f32), vm((S + PC, D), f32), vm((S + PC, D), f32), vm((S, D), f32),
            vm(((P0 + P1) // 2, D), u32), vm((T // 2, D), u32),
            vm((S, D), bf16),
            dma((28,)), dma((NC + 1,)),
        ],
        compiler_params=pltpu.CompilerParams(vmem_limit_bytes=110 << 20, disable_bounds_checks=True,
                                             disable_semaphore_checks=True),
    )(A_q.reshape(S, D), tile_view(A_k), tile_view(A_v), A_shift_k.T, A_ssm_k,
      A_ssm_D, B_w1, B_w2, B_w3.T, B_w4, c, w_mod)
    return out.reshape(1, S, D)
```

```python
import os
import numpy as np
import jax
import jax.numpy as jnp
import jax.experimental.pallas as pl
import jax.experimental.pallas.tpu as pltpu

f32, bf16, u32, i32 = jnp.float32, jnp.bfloat16, jnp.uint32, jnp.int32

S, D, F = 2048, 640, 1728
CT = D // 128
NB, BLK, NFFT = 4, 512, 1024
T = 256
NC = S // T
G2 = int(os.environ.get('G2', '1'))
NL = int(os.environ.get('NL', '4'))
LBAL = os.environ.get('LBAL', '')
BODY = os.environ.get('BODY', 't1c32l4')
SKIPCONV = int(os.environ.get('SKIPCONV', '0'))
RELOAD = int(os.environ.get('RELOAD', '1'))
W3S = int(os.environ.get('W3S', '512'))
LAST0 = int(os.environ.get('LAST0', '192'))
FM = (F // 128) * 128
E0 = int(os.environ.get('E0', '0'))
KGRP = [tuple(int(x) for x in g) for g in os.environ.get('KGRP', '0,12,34').split(',')]
TR = 8 * CT
P0, P1, PC = 320, 288, 240
RG = 16
EPS = 1e-5
NT_DIMS = (((1,), (1,)), ((), ()))
SCOPES = bool(int(os.environ.get("KSCOPES", "0")))


class _NoScope:
    def __enter__(self):
        return self

    def __exit__(self, *a):
        return False


def _scope(name):
    return jax.named_scope(name) if SCOPES else _NoScope()


def _lo(w):
    return pltpu.bitcast(w << 16, f32)


def _hi(w):
    return pltpu.bitcast(w & jnp.uint32(0xFFFF0000), f32)


def _cos_turn(n32, scale):
    x = 2.0 ** 30 - jnp.abs(n32.astype(f32))
    b = 2.0 * np.pi / 2.0 ** 32
    x = x * b
    x2 = x * x
    c = [scale * v for v in (1.0, -1.0 / 6, 1.0 / 120, -1.0 / 5040, 1.0 / 362880)]
    return x * (c[0] + x2 * (c[1] + x2 * (c[2] + x2 * (c[3] + x2 * c[4]))))


def _odd_freq(k):
    return jnp.where(k < 64, 4 * k + 1, 4 * k - 253) << 21


def _fwd_table(r):
    w = jax.lax.broadcasted_iota(i32, (128, 128), 0)
    halves = []
    for par in range(2):
        row = 2 * w + par
        k = ((row >> 4) << 3) + (row & 7)
        halves.append(_cos_turn(_odd_freq(k) * r + ((row & 8) << 27), 1.0))
    return pltpu.pack_elementwise(halves, packed_dtype=bf16)


def _inv_table(p):
    w = jax.lax.broadcasted_iota(i32, (64, 256), 0)
    col = jax.lax.broadcasted_iota(i32, (64, 256), 1)
    fr = _odd_freq(col >> 1)
    off = (col & 1) << 30
    halves = [_cos_turn(fr * (8 * w + 4 * par + p) + off, 2.0 / NFFT) for par in range(2)]
    return pltpu.pack_elementwise(halves, packed_dtype=bf16)


def _stats(x, link=None, early=False):
    zero = 0.0 if link is None else jnp.minimum(link, 0.0)
    part = x[:, 0:128]
    for c in range(1, CT):
        part = part + x[:, c * 128:(c + 1) * 128]
    if link is not None and early:
        part = part + zero
        zero = 0.0
    m = jnp.sum(part, axis=-1, keepdims=True) * (1.0 / D)
    v = jnp.maximum(jnp.sum(x * x, axis=-1, keepdims=True) * (1.0 / D) - m * m, zero)
    return m, jax.lax.rsqrt(v + EPS)


def _gelu2(x):
    c = 0.7978845608028654
    u = c + (c * 0.044715) * (x * x)
    return x + x * jnp.tanh(x * u)


def _gelu(x):
    c = 0.7978845608028654
    u = c + (c * 0.044715) * (x * x)
    t = jnp.tanh(x * u)
    hx = 0.5 * x
    return hx + hx * t


def _row_parts(m, parts):
    base, extra = divmod(m // 16, parts)
    out, o = [], 0
    for i in range(parts):
        n = 16 * (base + (1 if i < extra else 0))
        out.append((o, n))
        o += n
    return out


def _dot_balanced(x, wslice, n_cols, parts, nt=False):
    def mm(a, c0, c1):
        if nt:
            return jax.lax.dot_general(a, wslice(c0, c1), NT_DIMS, preferred_element_type=f32)
        return jnp.dot(a, wslice(c0, c1), preferred_element_type=f32)
    if parts == 1:
        return mm(x, 0, n_cols)
    head = mm(x, 0, n_cols - 128)
    last = jnp.concatenate([mm(x[o:o + n], n_cols - 128, n_cols) for o, n in _row_parts(x.shape[0], parts)],
                           axis=0)
    return jnp.concatenate([head, last], axis=-1)


def _radix4(re, im, inverse):
    ar, ai = re[0] + re[2], im[0] + im[2]
    br, bi = re[0] - re[2], im[0] - im[2]
    cr, ci = re[1] + re[3], im[1] + im[3]
    dr, di = re[1] - re[3], im[1] - im[3]
    minus_i = (br + di, bi - dr)
    plus_i = (br - di, bi + dr)
    if inverse:
        return [(ar + cr, ai + ci), plus_i, (ar - cr, ai - ci), minus_i]
    return [(ar + cr, ai + ci), minus_i, (ar - cr, ai - ci), plus_i]


def _kernel(q_hbm, k_hbm, v_hbm, sh_hbm, sk_hbm, d_hbm, w1_hbm, w2_hbm, w3_hbm, w4_hbm,
            c_hbm, wm_hbm, o_hbm,
            kb, vb, skb, qb, w1b, w2b, w3b, w4b, w1p, w2p, w3p, w4p, wmb, shb, db, cb_, fub, fkb, gtb, par,
            US, KS, UR, YS, YP, ys, modb, h1s, h2s, x2s, hss, zt, zb, ob,
            sem, sem_o):
    def sk_copy(c):
        return pltpu.make_async_copy(sk_hbm.at[pl.ds(c * 128, 128), :], skb.at[c], sem.at[c])

    def kv_copies(a):
        n = BLK * CT
        return [
            pltpu.make_async_copy(k_hbm.at[pl.ds(a * n, n), :], kb.at[pl.ds(TR + a * n, n), :], sem.at[CT + a]),
            pltpu.make_async_copy(v_hbm.at[pl.ds(a * n, n), :], vb.at[pl.ds(a * n, n), :], sem.at[2 * CT + a]),
        ]

    small = [pltpu.make_async_copy(src, dst, sem.at[15 + i]) for i, (src, dst) in enumerate(
        [(d_hbm, db), (sh_hbm, shb), (c_hbm, cb_)])]

    mod_cols = [(0, 3 * D), (3 * D, 2 * D), (5 * D, D)]
    mod_copies = [pltpu.make_async_copy(wm_hbm.at[:, pl.ds(o, n)], wmb.at[:, pl.ds(o, n)], sem.at[18 + i])
                  for i, (o, n) in enumerate(mod_cols)]
    w_pairs = [(w1_hbm, w1b), (w2_hbm, w2b), (w3_hbm, w3b), (w4_hbm, w4b)]
    w_copies = [pltpu.make_async_copy(src, dst, sem.at[21 + i]) for i, (src, dst) in enumerate(w_pairs)]
    q_rows = [(0, P0 + P1), (P0 + P1, PC), (P0 + P1 + PC, S - P0 - P1 - PC)]
    q_copies = [pltpu.make_async_copy(q_hbm.at[pl.ds(o, n), :], qb.at[pl.ds(o, n), :], sem.at[25 + i])
                for i, (o, n) in enumerate(q_rows)]

    def out_copy(i):
        r = i * T if isinstance(i, int) else pl.multiple_of(i * T, T)
        return pltpu.make_async_copy(ob.at[pl.ds(r, T), :], o_hbm.at[pl.ds(r, T), :], sem_o.at[i])

    out_tail = [pltpu.make_async_copy(ob.at[pl.ds(o, n), :], o_hbm.at[pl.ds(o, n), :], sem_o.at[NC - 1 + i])
                for i, (o, n) in enumerate([(S - T, LAST0), (S - T + LAST0, T - LAST0)])]

    for cp in small + kv_copies(0):
        cp.start()
    for c in range(CT):
        sk_copy(c).start()
    for a in range(1, NB):
        for cp in kv_copies(a):
            cp.start()
    for cp in [mod_copies[0], q_copies[0], mod_copies[1], w_copies[0], w_copies[1],
               w_copies[2], q_copies[1], w_copies[3], mod_copies[2], q_copies[2]]:
        cp.start()

    with _scope("init"):
        def pin(i, carry):
            YP[i, 0:8, :] = jnp.zeros((8, 128), f32)
            US[i, 0, 0, 0:8, :] = jnp.zeros((8, 128), f32)
            KS[i, 0, 0, 0:8, :] = jnp.zeros((8, 128), f32)
            YS[i, 0, 0, 0:8, :] = jnp.zeros((8, 128), f32)
            UR[i, 0, 0:8, :] = jnp.zeros((8, 128), f32)
            return carry

        jax.lax.fori_loop(0, 2, pin, 0)
        lane = jax.lax.broadcasted_iota(i32, (128, 128), 1)
        for p in range(4):
            m = (lane - p) & 3
            fkb[p] = _fwd_table(128 * m + ((lane - m) & 127))
        for c in range(CT):
            kb[c * 8:(c + 1) * 8, :] = jnp.zeros((8, 128), bf16)
            h1s[c, 0:8, :] = jnp.zeros((8, 128), f32)
            h1s[c, S + 8:S + 16, :] = jnp.zeros((8, 128), f32)
        for p in range(4):
            fub[p] = _fwd_table(8 * (lane & 63) + ((lane >> 6) << 2) + p)
        for cp in small:
            cp.wait()
        dv = db[...].astype(f32).reshape(1, D)
        shv = shb[...].astype(f32)
        for c in range(CT):
            for i in range(4):
                par[c, i] = jnp.broadcast_to(shv[i:i + 1, c * 128:(c + 1) * 128], (8, 128))
            par[c, 4] = jnp.broadcast_to(dv[:, c * 128:(c + 1) * 128], (8, 128))
    def fence(i, carry):
        YP[i, 0:8, :] = jnp.zeros((8, 128), f32)
        return carry

    kw = kb.bitcast(u32)
    vw = vb.bitcast(u32)

    def re_(g):
        return slice(g * 16, g * 16 + 8)

    def im_(g):
        return slice(g * 16 + 8, g * 16 + 16)

    def fwd_k(c, j):
        if SKIPCONV:
            return
        lane = jax.lax.broadcasted_iota(i32, (64, 128), 1)
        even = (lane & 1) == 0
        l01 = (lane & 2) == 0
        l12 = ((lane + 3) & 2) == 0
        rm = []
        for m in range(4):
            w = pltpu.bitcast(skb[c, :, (4 * j + m) * 128:(4 * j + m + 1) * 128], u32)
            rm.append(pltpu.roll(w, m, 1) if m else w)
        e01 = jnp.where(even, rm[0], rm[1])
        o01 = jnp.where(even, rm[1], rm[0])
        e23 = jnp.where(even, rm[2], rm[3])
        o23 = jnp.where(even, rm[3], rm[2])
        kp = [jnp.where(l01, e01, e23), jnp.where(l12, o01, o23),
              jnp.where(l01, e23, e01), jnp.where(l12, o23, o01)]
        tt = [jax.lax.dot_general(pltpu.bitcast(fkb[p], bf16), pltpu.bitcast(kp[p], bf16), NT_DIMS,
                                  preferred_element_type=f32) for p in range(4)]
        dvec = par[c, 4] if j == 0 else None
        for g in range(16):
            re = [t[re_(g)] for t in tt]
            im = [t[im_(g)] for t in tt]
            if j == 0:
                re[0] = re[0] + dvec
            x = _radix4(re, im, False)
            for m in range(4):
                xr, xi = x[m]
                if j < NB - 1:
                    KS[c, j, m, re_(g), :] = xr
                    KS[c, j, m, im_(g), :] = xi
                ur, ui = US[c, 0, m, re_(g), :], US[c, 0, m, im_(g), :]
                YS[c, j, m, re_(g), :] = xr * ur - xi * ui
                YS[c, j, m, im_(g), :] = xr * ui + xi * ur

    def fwd_u(c, a):
        if SKIPCONV:
            return
        taps = [jnp.tile(par[c, i], (8, 1)) for i in range(4)]
        ws = TR // 2
        base = a * (BLK // 8) * ws + 4 * c

        def words(ref, start):
            return ref[pl.ds(start, BLK // 8, stride=ws), :]

        kk = {}
        for w in range(4):
            x = words(kw, ws + base + w)
            kk[2 * w], kk[2 * w + 1] = _lo(x), _hi(x)
        kk[-3] = _hi(words(kw, base + 2))
        x = words(kw, base + 3)
        kk[-2], kk[-1] = _lo(x), _hi(x)
        sub = []
        for w in range(4):
            x = words(vw, base + w)
            for r, vv in ((2 * w, _lo(x)), (2 * w + 1, _hi(x))):
                sh = taps[0] * kk[r] + taps[1] * kk[r - 1] + taps[2] * kk[r - 2] + taps[3] * kk[r - 3]
                sub.append(sh * vv)
        kv = [jnp.concatenate([sub[p], sub[p + 4]], axis=0) for p in range(4)]
        tt = [jnp.dot(pltpu.bitcast(fub[p], bf16), kv[p].astype(bf16), preferred_element_type=f32)
              for p in range(4)]
        for g in range(16):
            x = _radix4([t[re_(g)] for t in tt], [t[im_(g)] for t in tt], False)
            for m in range(4):
                xr, xi = x[m]
                if a:
                    if a == 1:
                        pr, pi = US[c, 0, m, re_(g), :], US[c, 0, m, im_(g), :]
                    else:
                        pr, pi = UR[c, m, re_(g), :], UR[c, m, im_(g), :]
                    if a < NB - 1:
                        UR[c, m, re_(g), :] = xr
                        UR[c, m, im_(g), :] = xi
                    if g < 8:
                        xr, xi = xr - pi, xi + pr
                    else:
                        xr, xi = xr + pi, xi - pr
                US[c, a, m, re_(g), :] = xr
                US[c, a, m, im_(g), :] = xi

    def mac_inv(c, a, halves=(0, 1)):
        if SKIPCONV:
            return
        for h in halves:
            words = [[] for _ in range(4)]
            for g in range(8 * h, 8 * h + 8):
                yre, yim = [], []
                for m in range(4):
                    yr, yi = YS[c, a, m, re_(g), :], YS[c, a, m, im_(g), :]
                    for j in range(a):
                        kr, ki = KS[c, j, m, re_(g), :], KS[c, j, m, im_(g), :]
                        ur, ui = US[c, a - j, m, re_(g), :], US[c, a - j, m, im_(g), :]
                        yr = yr + (kr * ur - ki * ui)
                        yi = yi + (kr * ui + ki * ur)
                    yre.append(yr)
                    yim.append(yi)
                pp = _radix4(yre, yim, True)
                for p in range(4):
                    words[p].append(pltpu.pack_elementwise([pp[p][0], pp[p][1]], packed_dtype=bf16))
            for p in range(4):
                pb = pltpu.bitcast(jnp.concatenate(words[p], axis=0), bf16)
                r = jnp.dot(pltpu.bitcast(gtb[p, :, h * 128:(h + 1) * 128], bf16), pb,
                            preferred_element_type=f32)
                if h == 0:
                    YP[p] = r
                else:
                    ys[c, pl.ds(a * BLK + p, 128, stride=4), :] = YP[p] + r

    desc = (3, 2, 1, 0)
    def k_tile(c):
        for j in desc:
            fwd_k(c, j)

    with _scope("conv_u0"):
        for p in range(4):
            gtb[p] = _inv_table(p)
        with _scope("w_kv"):
            for cp in kv_copies(0):
                cp.wait()
        for c in range(CT):
            fwd_u(c, 0)
    with _scope("conv_k"):
        done = 0
        for grp in KGRP:
            with _scope("w_sk"):
                for c in grp:
                    sk_copy(c).wait()
            for c in grp:
                k_tile(c)
            if grp is KGRP[-1]:
                for c in range(E0):
                    mac_inv(c, 0)
    for a in range(1, NB):
        with _scope("conv_u%d" % a):
            with _scope("w_kv"):
                for cp in kv_copies(a):
                    cp.wait()
            todo = [(c, a - 1) for c in range(CT)]
            if a == 1:
                todo = todo[E0:]
            late = len(todo) < CT
            for c in range(CT):
                fwd_u(c, a)
                if todo and (not late or c >= CT - len(todo)):
                    mac_inv(*todo.pop(0))

    def mod_cols_dot(o, n, extra):
        cvec = cb_[...].astype(f32)
        act = cvec * jax.nn.sigmoid(cvec)

        def sc(k0, k1):
            return jnp.broadcast_to(act[:, k0:k1], (16, k1 - k0)).astype(bf16)

        e = 128 * extra
        r = jnp.dot(sc(0, D), wmb[:, o + e:o + n], preferred_element_type=f32)
        if extra:
            r0 = (jnp.dot(sc(0, D - 64), wmb[0:D - 64, o:o + e], preferred_element_type=f32)
                  + jnp.dot(sc(D - 64, D), wmb[D - 64:D, o:o + e], preferred_element_type=f32))
            r = jnp.concatenate([r0, r], axis=-1)
        return r[0:8]

    def mod_part(part, extra):
        o, n = mod_cols[part]
        r = mod_cols_dot(o, n, extra)
        return [r[:, i * D:(i + 1) * D] for i in range(n // D)]

    def mvec(i):
        return modb[i, 0:1, :]

    def rows(r, n):
        return pl.ds(r, n)

    def load_q(r):
        return qb[rows(r, RG), :].astype(f32)

    def make_x2(r, q, st):
        y = jnp.concatenate([ys[c, rows(r, RG), :] for c in range(CT)], axis=-1)
        return q + (((q - st[0]) * st[1]) * mvec(1) + mvec(0)) * y

    def make_h2(x2, st):
        return ((x2 - st[0]) * st[1]) * mvec(3) + mvec(2)

    def pack_ln(x, st):
        return pltpu.bitcast(((x - st[0]) * st[1]).astype(bf16), u32)

    def a_chain(r_in, r_out):
        prev = None
        for o in range(0, PC, RG):
            q = load_q(r_in + o)
            x2 = make_x2(r_in + o, q, _stats(q, prev))
            x2s[rows(r_out + o, RG), :] = x2
            st = _stats(x2)
            h2 = make_h2(x2s[rows(r_out + o, RG), :] if RELOAD else x2, st)
            h2s[rows(r_out + o, RG), :] = h2
            st = _stats(h2)
            zt[o // 2:(o + RG) // 2, :] = pack_ln(h2s[rows(r_out + o, RG), :] if RELOAD else h2, st)
            prev = st[1]

    def mm_w1(r, n, o=0, bal=True):
        z = pltpu.bitcast(zt[o // 2:(o + n) // 2, :], bf16)
        h1 = _gelu(_dot_balanced(z, lambda a, b: pltpu.bitcast(w1p[:, a:b], bf16), D, 4 if bal else 1))
        for c in range(CT):
            h1s[c, rows(r + 8, n), :] = h1[:, c * 128:(c + 1) * 128]

    def mm_w2a(r, bal=True):
        lane = jax.lax.broadcasted_iota(i32, (T, 128), 1)

        def sh(k, c):
            return h1s[c, rows(r + 8 + k, T), :]

        g = jnp.concatenate([
            sh(-1, 0),
            jnp.where(lane < 32, sh(-1, 1), sh(1, 1)),
            jnp.where(lane < 64, sh(1, 2), sh(-2, 2)),
            jnp.where(lane < 96, sh(-2, 3), sh(2, 3)),
            sh(2, 4)], axis=-1).astype(bf16)
        hss[rows(r, T), :] = _dot_balanced(g, lambda a, b: pltpu.bitcast(w2p[:, a:b], bf16), D, 4 if bal else 1)

    def mm_w2b(r, links=1):
        prev = [None] * links
        for n, o in enumerate(range(0, T, RG)):
            x1 = h2s[rows(r + o, RG), :] + hss[rows(r + o, RG), :]
            st = _stats(x1, prev[n % links], early=True)
            zb[o // 2:(o + RG) // 2, :] = pack_ln(x1, st)
            prev[n % links] = st[1]

    def mm_w3_main(bal=True):
        z = pltpu.bitcast(zb[...], bf16)
        return (_gelu2 if G2 else _gelu)(_dot_balanced(z, lambda a, b: pltpu.bitcast(w3p[a // 2:b // 2, :], bf16), FM, 4 if bal else 1, nt=True)).astype(bf16)

    def mm_w3_cols(a, b):
        z = pltpu.bitcast(zb[...], bf16)
        w = pltpu.bitcast(w3p[a // 2:b // 2, :], bf16)
        return _gelu2(jax.lax.dot_general(z, w, NT_DIMS, preferred_element_type=f32)).astype(bf16)

    def mm_w3_tail():
        z = pltpu.bitcast(zb[...], bf16)
        return (_gelu2 if G2 else _gelu)(jax.lax.dot_general(pltpu.bitcast(w3p[FM // 2:F // 2, :], bf16), z, NT_DIMS, preferred_element_type=f32))

    def join_act(main, tail):
        return jnp.concatenate([main, tail.T.astype(bf16)], axis=-1)

    def mm_w3(bal):
        tail = mm_w3_tail()
        return join_act(mm_w3_main(bal), tail)

    def mm_w4(r, a, o=0, n=T, bal=True):
        h2 = _dot_balanced(a[o:o + n], lambda c0, c1: pltpu.bitcast(w4p[:, c0:c1], bf16), D, 2 if bal else 1)
        ob[rows(r + o, n), :] = (x2s[rows(r + o, n), :]
                                 + mvec(4) * ((h2s[rows(r + o, n), :] + hss[rows(r + o, n), :]) + (0.5 * h2 if G2 else h2))).astype(bf16)

    groups = list(range(0, P0 + P1, RG))
    with _scope("conv_last"):
        jax.lax.fori_loop(0, 2, fence, 0)
        for c in range(NL):
            mac_inv(c, NB - 1)
    with _scope("pre_a"):
        with _scope("w_q0"):
            mod_copies[0].wait()
            q_copies[0].wait()
        sa, ca, ga = mod_part(0, 1)
        modb[0] = ga * sa
        modb[1] = ga * (1.0 + ca)
        for c in range(NL, CT):
            mac_inv(c, NB - 1)
        st1 = {o: _stats(load_q(o)) for o in groups}
        zt[0:8, 0:128] = jnp.zeros((8, 128), u32)
        st2 = {}
        for o in groups:
            x2 = make_x2(o, load_q(o), st1[o])
            x2s[o:o + RG, :] = x2
            st2[o] = _stats(x2)

    def pass_c(os_, links):
        st3 = {}
        prev = [None] * max(links, 1)
        for n, o in enumerate(os_):
            h2 = make_h2(x2s[o:o + RG, :], st2[o])
            h2s[o:o + RG, :] = h2
            st3[o] = _stats(h2, prev[n % len(prev)], early=True)
            if links:
                prev[n % links] = st3[o][1]
                zt[o // 2:(o + RG) // 2, :] = pack_ln(h2, st3[o])
        if not links:
            for o in os_:
                zt[o // 2:(o + RG) // 2, :] = pack_ln(h2s[o:o + RG, :], st3[o])

    with _scope("pre_b"):
        with _scope("w_modB"):
            mod_copies[1].wait()
        sb, cb = mod_part(1, 2)
        modb[2] = sb
        modb[3] = 1.0 + cb
        pass_c([o for o in groups if o < P0], 0)
    with _scope("r1"):
        with _scope("w_w1"):
            w_copies[0].wait()
        w1p[...] = pltpu.bitcast(w1b[...], u32)
        mm_w1(0, P0)
        pass_c([o for o in groups if o >= P0], 2)
    with _scope("r2"):
        with _scope("w_w2"):
            w_copies[1].wait()
        w2p[...] = pltpu.bitcast(w2b[...], u32)
        mm_w2a(0)
        mm_w2b(0, 2)
        mm_w1(P0, P1, P0)
    with _scope("r3"):
        with _scope("w_w3"):
            w_copies[2].wait()
            q_copies[1].wait()
        w3p[...] = pltpu.bitcast(w3b[...], u32)
        a_chain(P0 + P1, P0 + P1)
        main = mm_w3_main()
        mm_w2a(T)
        tail = mm_w3_tail()
    with _scope("r4"):
        with _scope("w_w4"):
            w_copies[3].wait()
            mod_copies[2].wait()
        w4p[...] = pltpu.bitcast(w4b[...], u32)
        modb[4] = mod_part(2, 1)[0]
        mm_w4(0, join_act(main, tail))
        mm_w2b(T)
        out_copy(0).start()
        q_copies[2].wait()

    def mlp_iter(i):
        r1 = pl.multiple_of(P0 + P1 - PC + PC * i, 16)
        r = pl.multiple_of(i * T, T)
        mains = []
        for tok in BODY:
            if tok == 't':
                tail = mm_w3_tail()
            elif tok == '1':
                mm_w1(r1, PC, bal='1' in LBAL)
            elif tok == 'c':
                a_chain(pl.multiple_of(jnp.minimum(r1 + PC, S - PC), 16), r1 + PC)
            elif tok == '3':
                mains.append(mm_w3_main('3' in LBAL))
            elif tok == 'x':
                mains.append(mm_w3_cols(0, W3S))
            elif tok == 'y':
                mains.append(mm_w3_cols(W3S, FM))
            elif tok == '2':
                mm_w2a(r + T, bal='2' in LBAL)
            elif tok == 'l':
                mm_w2b(r + T)
            elif tok == '4':
                mm_w4(r, join_act(jnp.concatenate(mains, axis=-1), tail), bal='4' in LBAL)
        out_copy(i).start()

    def mlp_body(i, carry):
        with _scope("iter"):
            mlp_iter(i)
        return carry

    with _scope("loop"):
        jax.lax.fori_loop(1, NC - 1, mlp_body, 0)
    with _scope("last"):
        act = mm_w3(False)
        mm_w4(S - T, act, 0, LAST0, bal=False)
        out_tail[0].start()
        mm_w4(S - T, act, LAST0, T - LAST0, bal=False)
        out_tail[1].start()
    with _scope("fin"):
        for i in range(NC - 1):
            out_copy(i).wait()
        for cp in out_tail:
            cp.wait()


@jax.jit
def pallas_adaLN_cond__ssm_conv_h3__mixer_s_mlp__prompt_kernel(
    A_q: jax.Array,
    A_k: jax.Array,
    A_v: jax.Array,
    A_shift_k: jax.Array,
    A_ssm_k: jax.Array,
    A_ssm_D: jax.Array,
    B_x: jax.Array,
    B_w1: jax.Array,
    B_w2: jax.Array,
    B_w3: jax.Array,
    B_w4: jax.Array,
    c: jax.Array,
    w_mod: jax.Array,
):
    del B_x
    any_spec = pl.BlockSpec(memory_space=pl.ANY)

    def tile_view(x):
        return x.reshape(S // 8, 8, CT, 128).transpose(0, 2, 1, 3).reshape(S * CT, 128)

    vm = pltpu.VMEM
    dma = pltpu.SemaphoreType.DMA
    out = pl.pallas_call(
        _kernel,
        in_specs=[any_spec] * 12,
        out_specs=any_spec,
        out_shape=jax.ShapeDtypeStruct((S, D), bf16),
        scratch_shapes=[
            vm((S * CT + TR, 128), bf16), vm((S * CT, 128), bf16), vm((CT, 128, S), bf16),
            vm((S, D), bf16), vm((D, D), bf16), vm((D, D), bf16), vm((F, D), bf16), vm((F, D), bf16),
            vm((D // 2, D), u32), vm((D // 2, D), u32), vm((F // 2, D), u32), vm((F // 2, D), u32),
            vm((D, 6 * D), bf16), vm((4, D), bf16), vm((D,), bf16), vm((1, D), bf16),
            vm((4, 128, 128), u32), vm((4, 128, 128), u32), vm((4, 64, 256), u32),
            vm((CT, 5, 8, 128), f32),
            vm((CT, NB, 4, 256, 128), f32), vm((CT, NB - 1, 4, 256, 128), f32),
            vm((CT, 4, 256, 128), f32), vm((CT, NB, 4, 256, 128), f32), vm((4, 128, 128), f32),
            vm((CT, S, 128), f32), vm((5, 8, D), f32),
            vm((CT, S + 16, 128), f32), vm((S + PC, D), f32), vm((S + PC, D), f32), vm((S, D), f32),
            vm(((P0 + P1) // 2, D), u32), vm((T // 2, D), u32),
            vm((S, D), bf16),
            dma((28,)), dma((NC + 1,)),
        ],
        compiler_params=pltpu.CompilerParams(vmem_limit_bytes=110 << 20, disable_bounds_checks=True,
                                             disable_semaphore_checks=True),
    )(A_q.reshape(S, D), tile_view(A_k), tile_view(A_v), A_shift_k.T, A_ssm_k,
      A_ssm_D, B_w1, B_w2, B_w3.T, B_w4, c, w_mod)
    return out.reshape(1, S, D)
```

```python
import os
import numpy as np
import jax
import jax.numpy as jnp
import jax.experimental.pallas as pl
import jax.experimental.pallas.tpu as pltpu

f32, bf16, u32, i32 = jnp.float32, jnp.bfloat16, jnp.uint32, jnp.int32

S, D, F = 2048, 640, 1728
CT = D // 128
NB, BLK, NFFT = 4, 512, 1024
T = 256
NC = S // T
CL1 = int(os.environ.get('CL1', '1'))
CLA = int(os.environ.get('CLA', '2'))
R3 = os.environ.get('R3', '1c3t')
G2 = int(os.environ.get('G2', '1'))
NL = int(os.environ.get('NL', '4'))
LBAL = os.environ.get('LBAL', '')
BODY = os.environ.get('BODY', 't1c32l4')
SKIPCONV = int(os.environ.get('SKIPCONV', '0'))
RELOAD = int(os.environ.get('RELOAD', '1'))
W3S = int(os.environ.get('W3S', '512'))
LAST0 = int(os.environ.get('LAST0', '192'))
FM = (F // 128) * 128
E0 = int(os.environ.get('E0', '0'))
KGRP = [tuple(int(x) for x in g) for g in os.environ.get('KGRP', '0,12,34').split(',')]
TR = 8 * CT
P0, P1, PC = int(os.environ.get('P0', '320')), 528 - int(os.environ.get('P0', '320')), int(os.environ.get('PC', '224'))
PA = S - P0 - P1 - 6 * PC
RG = 16
EPS = 1e-5
NT_DIMS = (((1,), (1,)), ((), ()))
SCOPES = bool(int(os.environ.get("KSCOPES", "0")))


class _NoScope:
    def __enter__(self):
        return self

    def __exit__(self, *a):
        return False


def _scope(name):
    return jax.named_scope(name) if SCOPES else _NoScope()


def _lo(w):
    return pltpu.bitcast(w << 16, f32)


def _hi(w):
    return pltpu.bitcast(w & jnp.uint32(0xFFFF0000), f32)


def _cos_turn(n32, scale):
    x = 2.0 ** 30 - jnp.abs(n32.astype(f32))
    b = 2.0 * np.pi / 2.0 ** 32
    x = x * b
    x2 = x * x
    c = [scale * v for v in (1.0, -1.0 / 6, 1.0 / 120, -1.0 / 5040, 1.0 / 362880)]
    return x * (c[0] + x2 * (c[1] + x2 * (c[2] + x2 * (c[3] + x2 * c[4]))))


def _odd_freq(k):
    return jnp.where(k < 64, 4 * k + 1, 4 * k - 253) << 21


def _fwd_table(r):
    w = jax.lax.broadcasted_iota(i32, (128, 128), 0)
    halves = []
    for par in range(2):
        row = 2 * w + par
        k = ((row >> 4) << 3) + (row & 7)
        halves.append(_cos_turn(_odd_freq(k) * r + ((row & 8) << 27), 1.0))
    return pltpu.pack_elementwise(halves, packed_dtype=bf16)


def _inv_table(p):
    w = jax.lax.broadcasted_iota(i32, (64, 256), 0)
    col = jax.lax.broadcasted_iota(i32, (64, 256), 1)
    fr = _odd_freq(col >> 1)
    off = (col & 1) << 30
    halves = [_cos_turn(fr * (8 * w + 4 * par + p) + off, 2.0 / NFFT) for par in range(2)]
    return pltpu.pack_elementwise(halves, packed_dtype=bf16)


def _stats(x, link=None, early=False):
    zero = 0.0 if link is None else jnp.minimum(link, 0.0)
    part = x[:, 0:128]
    for c in range(1, CT):
        part = part + x[:, c * 128:(c + 1) * 128]
    if link is not None and early:
        part = part + zero
        zero = 0.0
    m = jnp.sum(part, axis=-1, keepdims=True) * (1.0 / D)
    v = jnp.maximum(jnp.sum(x * x, axis=-1, keepdims=True) * (1.0 / D) - m * m, zero)
    return m, jax.lax.rsqrt(v + EPS)


def _gelu2(x):
    c = 0.7978845608028654
    u = c + (c * 0.044715) * (x * x)
    return x + x * jnp.tanh(x * u)


def _gelu(x):
    c = 0.7978845608028654
    u = c + (c * 0.044715) * (x * x)
    t = jnp.tanh(x * u)
    hx = 0.5 * x
    return hx + hx * t


def _row_parts(m, parts):
    base, extra = divmod(m // 16, parts)
    out, o = [], 0
    for i in range(parts):
        n = 16 * (base + (1 if i < extra else 0))
        out.append((o, n))
        o += n
    return out


def _dot_balanced(x, wslice, n_cols, parts, nt=False):
    def mm(a, c0, c1):
        if nt:
            return jax.lax.dot_general(a, wslice(c0, c1), NT_DIMS, preferred_element_type=f32)
        return jnp.dot(a, wslice(c0, c1), preferred_element_type=f32)
    if parts == 1:
        return mm(x, 0, n_cols)
    head = mm(x, 0, n_cols - 128)
    last = jnp.concatenate([mm(x[o:o + n], n_cols - 128, n_cols) for o, n in _row_parts(x.shape[0], parts)],
                           axis=0)
    return jnp.concatenate([head, last], axis=-1)


def _radix4(re, im, inverse):
    ar, ai = re[0] + re[2], im[0] + im[2]
    br, bi = re[0] - re[2], im[0] - im[2]
    cr, ci = re[1] + re[3], im[1] + im[3]
    dr, di = re[1] - re[3], im[1] - im[3]
    minus_i = (br + di, bi - dr)
    plus_i = (br - di, bi + dr)
    if inverse:
        return [(ar + cr, ai + ci), plus_i, (ar - cr, ai - ci), minus_i]
    return [(ar + cr, ai + ci), minus_i, (ar - cr, ai - ci), plus_i]


def _kernel(q_hbm, k_hbm, v_hbm, sh_hbm, sk_hbm, d_hbm, w1_hbm, w2_hbm, w3_hbm, w4_hbm,
            c_hbm, wm_hbm, o_hbm,
            kb, vb, skb, qb, w1b, w2b, w3b, w4b, w1p, w2p, w3p, w4p, wmb, shb, db, cb_, fub, fkb, gtb, par,
            US, KS, UR, YS, YP, ys, modb, h1s, h2s, x2s, hss, zt, zb, ob,
            sem, sem_o):
    def sk_copy(c):
        return pltpu.make_async_copy(sk_hbm.at[pl.ds(c * 128, 128), :], skb.at[c], sem.at[c])

    def kv_copies(a):
        n = BLK * CT
        return [
            pltpu.make_async_copy(k_hbm.at[pl.ds(a * n, n), :], kb.at[pl.ds(TR + a * n, n), :], sem.at[CT + a]),
            pltpu.make_async_copy(v_hbm.at[pl.ds(a * n, n), :], vb.at[pl.ds(a * n, n), :], sem.at[2 * CT + a]),
        ]

    small = [pltpu.make_async_copy(src, dst, sem.at[15 + i]) for i, (src, dst) in enumerate(
        [(d_hbm, db), (sh_hbm, shb), (c_hbm, cb_)])]

    mod_cols = [(0, 3 * D), (3 * D, 2 * D), (5 * D, D)]
    mod_copies = [pltpu.make_async_copy(wm_hbm.at[:, pl.ds(o, n)], wmb.at[:, pl.ds(o, n)], sem.at[18 + i])
                  for i, (o, n) in enumerate(mod_cols)]
    w_pairs = [(w1_hbm, w1b), (w2_hbm, w2b), (w3_hbm, w3b), (w4_hbm, w4b)]
    w_copies = [pltpu.make_async_copy(src, dst, sem.at[21 + i]) for i, (src, dst) in enumerate(w_pairs)]
    PB = P0 + P1 + PA
    q_rows = [(0, P0 + P1), (P0 + P1, PA), (PB, PC), (PB + PC, S - PB - PC)]
    q_copies = [pltpu.make_async_copy(q_hbm.at[pl.ds(o, n), :], qb.at[pl.ds(o, n), :], sem.at[25 + i])
                for i, (o, n) in enumerate(q_rows)]

    def out_copy(i):
        r = i * T if isinstance(i, int) else pl.multiple_of(i * T, T)
        return pltpu.make_async_copy(ob.at[pl.ds(r, T), :], o_hbm.at[pl.ds(r, T), :], sem_o.at[i])

    out_tail = [pltpu.make_async_copy(ob.at[pl.ds(o, n), :], o_hbm.at[pl.ds(o, n), :], sem_o.at[NC - 1 + i])
                for i, (o, n) in enumerate([(S - T, LAST0), (S - T + LAST0, T - LAST0)])]

    for cp in small + kv_copies(0):
        cp.start()
    for c in range(CT):
        sk_copy(c).start()
    for a in range(1, NB):
        for cp in kv_copies(a):
            cp.start()
    for cp in [mod_copies[0], q_copies[0], mod_copies[1], w_copies[0], w_copies[1], q_copies[1],
               w_copies[2], q_copies[2], w_copies[3], mod_copies[2], q_copies[3]]:
        cp.start()

    with _scope("init"):
        def pin(i, carry):
            YP[i, 0:8, :] = jnp.zeros((8, 128), f32)
            US[i, 0, 0, 0:8, :] = jnp.zeros((8, 128), f32)
            KS[i, 0, 0, 0:8, :] = jnp.zeros((8, 128), f32)
            YS[i, 0, 0, 0:8, :] = jnp.zeros((8, 128), f32)
            UR[i, 0, 0:8, :] = jnp.zeros((8, 128), f32)
            return carry

        jax.lax.fori_loop(0, 2, pin, 0)
        lane = jax.lax.broadcasted_iota(i32, (128, 128), 1)
        for p in range(4):
            m = (lane - p) & 3
            fkb[p] = _fwd_table(128 * m + ((lane - m) & 127))
        for c in range(CT):
            kb[c * 8:(c + 1) * 8, :] = jnp.zeros((8, 128), bf16)
            h1s[c, 0:8, :] = jnp.zeros((8, 128), f32)
            h1s[c, S + 8:S + 16, :] = jnp.zeros((8, 128), f32)
        for p in range(4):
            fub[p] = _fwd_table(8 * (lane & 63) + ((lane >> 6) << 2) + p)
        for cp in small:
            cp.wait()
        dv = db[...].astype(f32).reshape(1, D)
        shv = shb[...].astype(f32)
        for c in range(CT):
            for i in range(4):
                par[c, i] = jnp.broadcast_to(shv[i:i + 1, c * 128:(c + 1) * 128], (8, 128))
            par[c, 4] = jnp.broadcast_to(dv[:, c * 128:(c + 1) * 128], (8, 128))
    def fence(i, carry):
        YP[i, 0:8, :] = jnp.zeros((8, 128), f32)
        return carry

    kw = kb.bitcast(u32)
    vw = vb.bitcast(u32)

    def re_(g):
        return slice(g * 16, g * 16 + 8)

    def im_(g):
        return slice(g * 16 + 8, g * 16 + 16)

    def fwd_k(c, j):
        if SKIPCONV:
            return
        lane = jax.lax.broadcasted_iota(i32, (64, 128), 1)
        even = (lane & 1) == 0
        l01 = (lane & 2) == 0
        l12 = ((lane + 3) & 2) == 0
        rm = []
        for m in range(4):
            w = pltpu.bitcast(skb[c, :, (4 * j + m) * 128:(4 * j + m + 1) * 128], u32)
            rm.append(pltpu.roll(w, m, 1) if m else w)
        e01 = jnp.where(even, rm[0], rm[1])
        o01 = jnp.where(even, rm[1], rm[0])
        e23 = jnp.where(even, rm[2], rm[3])
        o23 = jnp.where(even, rm[3], rm[2])
        kp = [jnp.where(l01, e01, e23), jnp.where(l12, o01, o23),
              jnp.where(l01, e23, e01), jnp.where(l12, o23, o01)]
        tt = [jax.lax.dot_general(pltpu.bitcast(fkb[p], bf16), pltpu.bitcast(kp[p], bf16), NT_DIMS,
                                  preferred_element_type=f32) for p in range(4)]
        dvec = par[c, 4] if j == 0 else None
        for g in range(16):
            re = [t[re_(g)] for t in tt]
            im = [t[im_(g)] for t in tt]
            if j == 0:
                re[0] = re[0] + dvec
            x = _radix4(re, im, False)
            for m in range(4):
                xr, xi = x[m]
                if j < NB - 1:
                    KS[c, j, m, re_(g), :] = xr
                    KS[c, j, m, im_(g), :] = xi
                ur, ui = US[c, 0, m, re_(g), :], US[c, 0, m, im_(g), :]
                YS[c, j, m, re_(g), :] = xr * ur - xi * ui
                YS[c, j, m, im_(g), :] = xr * ui + xi * ur

    def fwd_u(c, a):
        if SKIPCONV:
            return
        taps = [jnp.tile(par[c, i], (8, 1)) for i in range(4)]
        ws = TR // 2
        base = a * (BLK // 8) * ws + 4 * c

        def words(ref, start):
            return ref[pl.ds(start, BLK // 8, stride=ws), :]

        kk = {}
        for w in range(4):
            x = words(kw, ws + base + w)
            kk[2 * w], kk[2 * w + 1] = _lo(x), _hi(x)
        kk[-3] = _hi(words(kw, base + 2))
        x = words(kw, base + 3)
        kk[-2], kk[-1] = _lo(x), _hi(x)
        sub = []
        for w in range(4):
            x = words(vw, base + w)
            for r, vv in ((2 * w, _lo(x)), (2 * w + 1, _hi(x))):
                sh = taps[0] * kk[r] + taps[1] * kk[r - 1] + taps[2] * kk[r - 2] + taps[3] * kk[r - 3]
                sub.append(sh * vv)
        kv = [jnp.concatenate([sub[p], sub[p + 4]], axis=0) for p in range(4)]
        tt = [jnp.dot(pltpu.bitcast(fub[p], bf16), kv[p].astype(bf16), preferred_element_type=f32)
              for p in range(4)]
        for g in range(16):
            x = _radix4([t[re_(g)] for t in tt], [t[im_(g)] for t in tt], False)
            for m in range(4):
                xr, xi = x[m]
                if a:
                    if a == 1:
                        pr, pi = US[c, 0, m, re_(g), :], US[c, 0, m, im_(g), :]
                    else:
                        pr, pi = UR[c, m, re_(g), :], UR[c, m, im_(g), :]
                    if a < NB - 1:
                        UR[c, m, re_(g), :] = xr
                        UR[c, m, im_(g), :] = xi
                    if g < 8:
                        xr, xi = xr - pi, xi + pr
                    else:
                        xr, xi = xr + pi, xi - pr
                US[c, a, m, re_(g), :] = xr
                US[c, a, m, im_(g), :] = xi

    def mac_inv(c, a, halves=(0, 1)):
        if SKIPCONV:
            return
        for h in halves:
            words = [[] for _ in range(4)]
            for g in range(8 * h, 8 * h + 8):
                yre, yim = [], []
                for m in range(4):
                    yr, yi = YS[c, a, m, re_(g), :], YS[c, a, m, im_(g), :]
                    for j in range(a):
                        kr, ki = KS[c, j, m, re_(g), :], KS[c, j, m, im_(g), :]
                        ur, ui = US[c, a - j, m, re_(g), :], US[c, a - j, m, im_(g), :]
                        yr = yr + (kr * ur - ki * ui)
                        yi = yi + (kr * ui + ki * ur)
                    yre.append(yr)
                    yim.append(yi)
                pp = _radix4(yre, yim, True)
                for p in range(4):
                    words[p].append(pltpu.pack_elementwise([pp[p][0], pp[p][1]], packed_dtype=bf16))
            for p in range(4):
                pb = pltpu.bitcast(jnp.concatenate(words[p], axis=0), bf16)
                r = jnp.dot(pltpu.bitcast(gtb[p, :, h * 128:(h + 1) * 128], bf16), pb,
                            preferred_element_type=f32)
                if h == 0:
                    YP[p] = r
                else:
                    ys[c, pl.ds(a * BLK + p, 128, stride=4), :] = YP[p] + r

    desc = (3, 2, 1, 0)
    def k_tile(c):
        for j in desc:
            fwd_k(c, j)

    with _scope("conv_u0"):
        for p in range(4):
            gtb[p] = _inv_table(p)
        with _scope("w_kv"):
            for cp in kv_copies(0):
                cp.wait()
        for c in range(CT):
            fwd_u(c, 0)
    with _scope("conv_k"):
        done = 0
        for grp in KGRP:
            with _scope("w_sk"):
                for c in grp:
                    sk_copy(c).wait()
            for c in grp:
                k_tile(c)
            if grp is KGRP[-1]:
                for c in range(E0):
                    mac_inv(c, 0)
    for a in range(1, NB):
        with _scope("conv_u%d" % a):
            with _scope("w_kv"):
                for cp in kv_copies(a):
                    cp.wait()
            todo = [(c, a - 1) for c in range(CT)]
            if a == 1:
                todo = todo[E0:]
            late = len(todo) < CT
            for c in range(CT):
                fwd_u(c, a)
                if todo and (not late or c >= CT - len(todo)):
                    mac_inv(*todo.pop(0))

    def mod_cols_dot(o, n, extra):
        cvec = cb_[...].astype(f32)
        act = cvec * jax.nn.sigmoid(cvec)

        def sc(k0, k1):
            return jnp.broadcast_to(act[:, k0:k1], (16, k1 - k0)).astype(bf16)

        e = 128 * extra
        r = jnp.dot(sc(0, D), wmb[:, o + e:o + n], preferred_element_type=f32)
        if extra:
            r0 = (jnp.dot(sc(0, D - 64), wmb[0:D - 64, o:o + e], preferred_element_type=f32)
                  + jnp.dot(sc(D - 64, D), wmb[D - 64:D, o:o + e], preferred_element_type=f32))
            r = jnp.concatenate([r0, r], axis=-1)
        return r[0:8]

    def mod_part(part, extra):
        o, n = mod_cols[part]
        r = mod_cols_dot(o, n, extra)
        return [r[:, i * D:(i + 1) * D] for i in range(n // D)]

    def mvec(i):
        return modb[i, 0:1, :]

    def rows(r, n):
        return pl.ds(r, n)

    def load_q(r):
        return qb[rows(r, RG), :].astype(f32)

    def make_x2(r, q, st):
        y = jnp.concatenate([ys[c, rows(r, RG), :] for c in range(CT)], axis=-1)
        return q + (((q - st[0]) * st[1]) * mvec(1) + mvec(0)) * y

    def make_h2(x2, st):
        return ((x2 - st[0]) * st[1]) * mvec(3) + mvec(2)

    def pack_ln(x, st):
        return pltpu.bitcast(((x - st[0]) * st[1]).astype(bf16), u32)

    def a_chain(r_in, r_out, n=PC, links=1):
        prevs = [None] * links
        for g, o in enumerate(range(0, n, RG)):
            prev = prevs[g % links]
            q = load_q(r_in + o)
            x2 = make_x2(r_in + o, q, _stats(q, prev))
            x2s[rows(r_out + o, RG), :] = x2
            st = _stats(x2)
            h2 = make_h2(x2s[rows(r_out + o, RG), :] if RELOAD else x2, st)
            h2s[rows(r_out + o, RG), :] = h2
            st = _stats(h2)
            zt[o // 2:(o + RG) // 2, :] = pack_ln(h2s[rows(r_out + o, RG), :] if RELOAD else h2, st)
            prevs[g % links] = st[1]

    def mm_w1(r, n, o=0, bal=True):
        z = pltpu.bitcast(zt[o // 2:(o + n) // 2, :], bf16)
        h1 = _gelu(_dot_balanced(z, lambda a, b: pltpu.bitcast(w1p[:, a:b], bf16), D, 4 if bal else 1))
        for c in range(CT):
            h1s[c, rows(r + 8, n), :] = h1[:, c * 128:(c + 1) * 128]

    def mm_w2a(r, bal=True):
        lane = jax.lax.broadcasted_iota(i32, (T, 128), 1)

        def sh(k, c):
            return h1s[c, rows(r + 8 + k, T), :]

        g = jnp.concatenate([
            sh(-1, 0),
            jnp.where(lane < 32, sh(-1, 1), sh(1, 1)),
            jnp.where(lane < 64, sh(1, 2), sh(-2, 2)),
            jnp.where(lane < 96, sh(-2, 3), sh(2, 3)),
            sh(2, 4)], axis=-1).astype(bf16)
        hss[rows(r, T), :] = _dot_balanced(g, lambda a, b: pltpu.bitcast(w2p[:, a:b], bf16), D, 4 if bal else 1)

    def mm_w2b(r, links=1):
        prev = [None] * links
        for n, o in enumerate(range(0, T, RG)):
            x1 = h2s[rows(r + o, RG), :] + hss[rows(r + o, RG), :]
            st = _stats(x1, prev[n % links], early=True)
            zb[o // 2:(o + RG) // 2, :] = pack_ln(x1, st)
            prev[n % links] = st[1]

    def mm_w3_main(bal=True):
        z = pltpu.bitcast(zb[...], bf16)
        return (_gelu2 if G2 else _gelu)(_dot_balanced(z, lambda a, b: pltpu.bitcast(w3p[a // 2:b // 2, :], bf16), FM, 4 if bal else 1, nt=True)).astype(bf16)

    def mm_w3_cols(a, b):
        z = pltpu.bitcast(zb[...], bf16)
        w = pltpu.bitcast(w3p[a // 2:b // 2, :], bf16)
        return _gelu2(jax.lax.dot_general(z, w, NT_DIMS, preferred_element_type=f32)).astype(bf16)

    def mm_w3_tail():
        z = pltpu.bitcast(zb[...], bf16)
        return (_gelu2 if G2 else _gelu)(jax.lax.dot_general(pltpu.bitcast(w3p[FM // 2:F // 2, :], bf16), z, NT_DIMS, preferred_element_type=f32))

    def join_act(main, tail):
        return jnp.concatenate([main, tail.T.astype(bf16)], axis=-1)

    def mm_w3(bal):
        tail = mm_w3_tail()
        return join_act(mm_w3_main(bal), tail)

    def mm_w4(r, a, o=0, n=T, bal=True):
        h2 = _dot_balanced(a[o:o + n], lambda c0, c1: pltpu.bitcast(w4p[:, c0:c1], bf16), D, 2 if bal else 1)
        ob[rows(r + o, n), :] = (x2s[rows(r + o, n), :]
                                 + mvec(4) * ((h2s[rows(r + o, n), :] + hss[rows(r + o, n), :]) + (0.5 * h2 if G2 else h2))).astype(bf16)

    groups = list(range(0, P0 + P1, RG))
    with _scope("conv_last"):
        jax.lax.fori_loop(0, 2, fence, 0)
        for c in range(NL):
            mac_inv(c, NB - 1)
    with _scope("pre_a"):
        with _scope("w_q0"):
            mod_copies[0].wait()
            q_copies[0].wait()
        sa, ca, ga = mod_part(0, 1)
        modb[0] = ga * sa
        modb[1] = ga * (1.0 + ca)
        for c in range(NL, CT):
            mac_inv(c, NB - 1)
        st1 = {o: _stats(load_q(o)) for o in groups}
        zt[0:8, 0:128] = jnp.zeros((8, 128), u32)
        st2 = {}
        for o in groups:
            x2 = make_x2(o, load_q(o), st1[o])
            x2s[o:o + RG, :] = x2
            st2[o] = _stats(x2)

    def pass_c(os_, links):
        st3 = {}
        prev = [None] * max(links, 1)
        for n, o in enumerate(os_):
            h2 = make_h2(x2s[o:o + RG, :], st2[o])
            h2s[o:o + RG, :] = h2
            st3[o] = _stats(h2, prev[n % len(prev)], early=True)
            if links:
                prev[n % links] = st3[o][1]
                zt[o // 2:(o + RG) // 2, :] = pack_ln(h2, st3[o])
        if not links:
            for o in os_:
                zt[o // 2:(o + RG) // 2, :] = pack_ln(h2s[o:o + RG, :], st3[o])

    with _scope("pre_b"):
        with _scope("w_modB"):
            mod_copies[1].wait()
        sb, cb = mod_part(1, 2)
        modb[2] = sb
        modb[3] = 1.0 + cb
        pass_c([o for o in groups if o < P0], 0)
    with _scope("r1"):
        with _scope("w_w1"):
            w_copies[0].wait()
        w1p[...] = pltpu.bitcast(w1b[...], u32)
        mm_w1(0, P0)
        pass_c([o for o in groups if o >= P0], CL1)
        mm_w1(P0, P1, P0)
    with _scope("r2"):
        with _scope("w_w2"):
            w_copies[1].wait()
            q_copies[1].wait()
        w2p[...] = pltpu.bitcast(w2b[...], u32)
        a_chain(P0 + P1, P0 + P1, PA, CLA)
        mm_w2a(0)
        mm_w2b(0, 2)
        mm_w2a(T)
    with _scope("r3"):
        with _scope("w_w3"):
            w_copies[2].wait()
            q_copies[2].wait()
        w3p[...] = pltpu.bitcast(w3b[...], u32)
        for tok in R3:
            if tok == '1':
                mm_w1(P0 + P1, PA)
            elif tok == 'c':
                a_chain(PB, PB)
            elif tok == '3':
                main = mm_w3_main()
            else:
                tail = mm_w3_tail()
    with _scope("r4"):
        with _scope("w_w4"):
            w_copies[3].wait()
            mod_copies[2].wait()
        w4p[...] = pltpu.bitcast(w4b[...], u32)
        modb[4] = mod_part(2, 1)[0]
        mm_w4(0, join_act(main, tail))
        mm_w2b(T)
        out_copy(0).start()
        q_copies[3].wait()

    def mlp_iter(i):
        r1 = pl.multiple_of(PB - PC + PC * i, 16)
        r = pl.multiple_of(i * T, T)
        mains = []
        for tok in BODY:
            if tok == 't':
                tail = mm_w3_tail()
            elif tok == '1':
                mm_w1(r1, PC, bal='1' in LBAL)
            elif tok == 'c':
                a_chain(pl.multiple_of(jnp.minimum(r1 + PC, S - PC), 16), r1 + PC)
            elif tok == '3':
                mains.append(mm_w3_main('3' in LBAL))
            elif tok == 'x':
                mains.append(mm_w3_cols(0, W3S))
            elif tok == 'y':
                mains.append(mm_w3_cols(W3S, FM))
            elif tok == '2':
                mm_w2a(r + T, bal='2' in LBAL)
            elif tok == 'l':
                mm_w2b(r + T)
            elif tok == '4':
                mm_w4(r, join_act(jnp.concatenate(mains, axis=-1), tail), bal='4' in LBAL)
        out_copy(i).start()

    def mlp_body(i, carry):
        with _scope("iter"):
            mlp_iter(i)
        return carry

    with _scope("loop"):
        jax.lax.fori_loop(1, NC - 1, mlp_body, 0)
    with _scope("last"):
        act = mm_w3(False)
        mm_w4(S - T, act, 0, LAST0, bal=False)
        out_tail[0].start()
        mm_w4(S - T, act, LAST0, T - LAST0, bal=False)
        out_tail[1].start()
    with _scope("fin"):
        for i in range(NC - 1):
            out_copy(i).wait()
        for cp in out_tail:
            cp.wait()


@jax.jit
def pallas_adaLN_cond__ssm_conv_h3__mixer_s_mlp__prompt_kernel(
    A_q: jax.Array,
    A_k: jax.Array,
    A_v: jax.Array,
    A_shift_k: jax.Array,
    A_ssm_k: jax.Array,
    A_ssm_D: jax.Array,
    B_x: jax.Array,
    B_w1: jax.Array,
    B_w2: jax.Array,
    B_w3: jax.Array,
    B_w4: jax.Array,
    c: jax.Array,
    w_mod: jax.Array,
):
    del B_x
    any_spec = pl.BlockSpec(memory_space=pl.ANY)

    def tile_view(x):
        return x.reshape(S // 8, 8, CT, 128).transpose(0, 2, 1, 3).reshape(S * CT, 128)

    vm = pltpu.VMEM
    dma = pltpu.SemaphoreType.DMA
    out = pl.pallas_call(
        _kernel,
        in_specs=[any_spec] * 12,
        out_specs=any_spec,
        out_shape=jax.ShapeDtypeStruct((S, D), bf16),
        scratch_shapes=[
            vm((S * CT + TR, 128), bf16), vm((S * CT, 128), bf16), vm((CT, 128, S), bf16),
            vm((S, D), bf16), vm((D, D), bf16), vm((D, D), bf16), vm((F, D), bf16), vm((F, D), bf16),
            vm((D // 2, D), u32), vm((D // 2, D), u32), vm((F // 2, D), u32), vm((F // 2, D), u32),
            vm((D, 6 * D), bf16), vm((4, D), bf16), vm((D,), bf16), vm((1, D), bf16),
            vm((4, 128, 128), u32), vm((4, 128, 128), u32), vm((4, 64, 256), u32),
            vm((CT, 5, 8, 128), f32),
            vm((CT, NB, 4, 256, 128), f32), vm((CT, NB - 1, 4, 256, 128), f32),
            vm((CT, 4, 256, 128), f32), vm((CT, NB, 4, 256, 128), f32), vm((4, 128, 128), f32),
            vm((CT, S, 128), f32), vm((5, 8, D), f32),
            vm((CT, S + 16, 128), f32), vm((S + PC, D), f32), vm((S + PC, D), f32), vm((S, D), f32),
            vm(((P0 + P1) // 2, D), u32), vm((T // 2, D), u32),
            vm((S, D), bf16),
            dma((29,)), dma((NC + 1,)),
        ],
        compiler_params=pltpu.CompilerParams(vmem_limit_bytes=110 << 20, disable_bounds_checks=True,
                                             disable_semaphore_checks=True),
    )(A_q.reshape(S, D), tile_view(A_k), tile_view(A_v), A_shift_k.T, A_ssm_k,
      A_ssm_D, B_w1, B_w2, B_w3.T, B_w4, c, w_mod)
    return out.reshape(1, S, D)
```

```python
import os
import numpy as np
import jax
import jax.numpy as jnp
import jax.experimental.pallas as pl
import jax.experimental.pallas.tpu as pltpu

f32, bf16, u32, i32 = jnp.float32, jnp.bfloat16, jnp.uint32, jnp.int32

S, D, F = 2048, 640, 1728
CT = D // 128
NB, BLK, NFFT = 4, 512, 1024
T = 256
NC = S // T
FILL = int(os.environ.get('FILL', '1792'))
VIEW = int(os.environ.get('VIEW', '1'))
CL1 = int(os.environ.get('CL1', '1'))
CLA = int(os.environ.get('CLA', '2'))
R3 = os.environ.get('R3', '1c3t')
G2 = int(os.environ.get('G2', '1'))
NL = int(os.environ.get('NL', '4'))
LBAL = os.environ.get('LBAL', '')
BODY = os.environ.get('BODY', '1ct32l4')
SKIPCONV = int(os.environ.get('SKIPCONV', '0'))
RELOAD = int(os.environ.get('RELOAD', '1'))
W3S = int(os.environ.get('W3S', '512'))
LAST0 = int(os.environ.get('LAST0', '192'))
FM = (F // 128) * 128
E0 = int(os.environ.get('E0', '0'))
KGRP = [tuple(int(x) for x in g) for g in os.environ.get('KGRP', '0,12,34').split(',')]
TR = 8 * CT
P0, P1, PC = int(os.environ.get('P0', '320')), 528 - int(os.environ.get('P0', '320')), int(os.environ.get('PC', '224'))
PA = S - P0 - P1 - 6 * PC
RG = 16
EPS = 1e-5
NT_DIMS = (((1,), (1,)), ((), ()))
SCOPES = bool(int(os.environ.get("KSCOPES", "0")))


class _NoScope:
    def __enter__(self):
        return self

    def __exit__(self, *a):
        return False


def _scope(name):
    return jax.named_scope(name) if SCOPES else _NoScope()


def _lo(w):
    return pltpu.bitcast(w << 16, f32)


def _hi(w):
    return pltpu.bitcast(w & jnp.uint32(0xFFFF0000), f32)


def _cos_turn(n32, scale):
    x = 2.0 ** 30 - jnp.abs(n32.astype(f32))
    b = 2.0 * np.pi / 2.0 ** 32
    x = x * b
    x2 = x * x
    c = [scale * v for v in (1.0, -1.0 / 6, 1.0 / 120, -1.0 / 5040, 1.0 / 362880)]
    return x * (c[0] + x2 * (c[1] + x2 * (c[2] + x2 * (c[3] + x2 * c[4]))))


def _odd_freq(k):
    return jnp.where(k < 64, 4 * k + 1, 4 * k - 253) << 21


def _slot_phase(idx):
    k = ((idx >> 4) << 3) + (idx & 7)
    return _odd_freq(k), (idx & 8) << 27


def _fwd_table(r):
    fr, off = _slot_phase(jax.lax.broadcasted_iota(i32, (256, 128), 0))
    return pltpu.bitcast(_cos_turn(fr * r + off, 1.0).astype(bf16), u32)


def _inv_table(p):
    row = jax.lax.broadcasted_iota(i32, (128, 256), 0)
    fr, off = _slot_phase(jax.lax.broadcasted_iota(i32, (128, 256), 1))
    return pltpu.bitcast(_cos_turn(fr * (4 * row + p) + off, 2.0 / NFFT).astype(bf16), u32)


def _stats(x, link=None, early=False):
    zero = 0.0 if link is None else jnp.minimum(link, 0.0)
    part = x[:, 0:128]
    for c in range(1, CT):
        part = part + x[:, c * 128:(c + 1) * 128]
    if link is not None and early:
        part = part + zero
        zero = 0.0
    m = jnp.sum(part, axis=-1, keepdims=True) * (1.0 / D)
    v = jnp.maximum(jnp.sum(x * x, axis=-1, keepdims=True) * (1.0 / D) - m * m, zero)
    return m, jax.lax.rsqrt(v + EPS)


def _gelu2(x):
    c = 0.7978845608028654
    u = c + (c * 0.044715) * (x * x)
    return x + x * jnp.tanh(x * u)


def _gelu(x):
    c = 0.7978845608028654
    u = c + (c * 0.044715) * (x * x)
    t = jnp.tanh(x * u)
    hx = 0.5 * x
    return hx + hx * t


def _row_parts(m, parts):
    base, extra = divmod(m // 16, parts)
    out, o = [], 0
    for i in range(parts):
        n = 16 * (base + (1 if i < extra else 0))
        out.append((o, n))
        o += n
    return out


def _dot_balanced(x, wslice, n_cols, parts, nt=False):
    def mm(a, c0, c1):
        a = a.astype(bf16)
        if nt:
            return jax.lax.dot_general(a, wslice(c0, c1), NT_DIMS, preferred_element_type=f32)
        return jnp.dot(a, wslice(c0, c1), preferred_element_type=f32)
    if parts == 1:
        return mm(x, 0, n_cols)
    head = mm(x, 0, n_cols - 128)
    last = jnp.concatenate([mm(x[o:o + n], n_cols - 128, n_cols) for o, n in _row_parts(x.shape[0], parts)],
                           axis=0)
    return jnp.concatenate([head, last], axis=-1)


def _radix4(re, im, inverse):
    ar, ai = re[0] + re[2], im[0] + im[2]
    br, bi = re[0] - re[2], im[0] - im[2]
    cr, ci = re[1] + re[3], im[1] + im[3]
    dr, di = re[1] - re[3], im[1] - im[3]
    minus_i = (br + di, bi - dr)
    plus_i = (br - di, bi + dr)
    if inverse:
        return [(ar + cr, ai + ci), plus_i, (ar - cr, ai - ci), minus_i]
    return [(ar + cr, ai + ci), minus_i, (ar - cr, ai - ci), plus_i]


def _kernel(q_hbm, k_hbm, v_hbm, sh_hbm, sk_hbm, d_hbm, w1_hbm, w2_hbm, w3_hbm, w4_hbm,
            c_hbm, wm_hbm, o_hbm,
            kb, vb, skb, qb, w1b, w2b, w3b, w4b, w1p, w2p, w3p, w4p, wmb, shb, db, cb_, fill, fub, fkb, gtb, par,
            US, KS, UR, YS, YP, ys, modb, h1s, h2s, x2s, hss, zt, zb, ob,
            sem, sem_o):
    def sk_copy(c):
        return pltpu.make_async_copy(sk_hbm.at[pl.ds(c * 128, 128), :], skb.at[c], sem.at[c])

    def kv_copies(a):
        n = BLK * CT
        return [
            pltpu.make_async_copy(k_hbm.at[pl.ds(a * n, n), :], kb.at[pl.ds(TR + a * n, n), :], sem.at[CT + a]),
            pltpu.make_async_copy(v_hbm.at[pl.ds(a * n, n), :], vb.at[pl.ds(a * n, n), :], sem.at[2 * CT + a]),
        ]

    small = [pltpu.make_async_copy(src, dst, sem.at[15 + i]) for i, (src, dst) in enumerate(
        [(d_hbm, db), (sh_hbm, shb), (c_hbm, cb_)])]

    mod_cols = [(0, 3 * D), (3 * D, 2 * D), (5 * D, D)]
    mod_copies = [pltpu.make_async_copy(wm_hbm.at[:, pl.ds(o, n)], wmb.at[:, pl.ds(o, n)], sem.at[18 + i])
                  for i, (o, n) in enumerate(mod_cols)]
    w_pairs = [(w1_hbm, w1b), (w2_hbm, w2b), (w3_hbm, w3b), (w4_hbm, w4b)]
    w_copies = [pltpu.make_async_copy(src, dst, sem.at[21 + i]) for i, (src, dst) in enumerate(w_pairs)]
    PB = P0 + P1 + PA
    q_rows = [(0, P0 + P1), (P0 + P1, PA), (PB, PC), (PB + PC, S - PB - PC)]
    q_copies = [pltpu.make_async_copy(q_hbm.at[pl.ds(o, n), :], qb.at[pl.ds(o, n), :], sem.at[25 + i])
                for i, (o, n) in enumerate(q_rows)]

    def out_copy(i):
        r = i * T if isinstance(i, int) else pl.multiple_of(i * T, T)
        return pltpu.make_async_copy(ob.at[pl.ds(r, T), :], o_hbm.at[pl.ds(r, T), :], sem_o.at[i])

    out_tail = [pltpu.make_async_copy(ob.at[pl.ds(o, n), :], o_hbm.at[pl.ds(o, n), :], sem_o.at[NC - 1 + i])
                for i, (o, n) in enumerate([(S - T, LAST0), (S - T + LAST0, T - LAST0)])]

    for cp in small + kv_copies(0):
        cp.start()
    for c in range(CT):
        sk_copy(c).start()
    for a in range(1, NB):
        for cp in kv_copies(a):
            cp.start()
    for cp in [mod_copies[0], q_copies[0], mod_copies[1], w_copies[0], w_copies[1], q_copies[1],
               w_copies[2], q_copies[2], w_copies[3], mod_copies[2], q_copies[3]]:
        cp.start()

    with _scope("init"):
        def pin(i, carry):
            fill[:, pl.ds(pl.multiple_of(i * 128, 128), 128)] = jnp.zeros((1, 128), f32)
            YP[i, 0:8, :] = jnp.zeros((8, 128), f32)
            US[i, 0, 0, 0:8, :] = jnp.zeros((8, 128), f32)
            KS[i, 0, 0, 0:8, :] = jnp.zeros((8, 128), f32)
            YS[i, 0, 0, 0:8, :] = jnp.zeros((8, 128), f32)
            UR[i, 0, 0:8, :] = jnp.zeros((8, 128), f32)
            return carry

        jax.lax.fori_loop(0, 2, pin, 0)
        lane = jax.lax.broadcasted_iota(i32, (256, 128), 1)
        for p in range(4):
            m = (lane - p) & 3
            fkb[p] = _fwd_table(128 * m + ((lane - m) & 127))
        for c in range(CT):
            kb[c * 8:(c + 1) * 8, :] = jnp.zeros((8, 128), bf16)
            h1s[c, 0:8, :] = jnp.zeros((8, 128), f32)
            h1s[c, S + 8:S + 16, :] = jnp.zeros((8, 128), f32)
        for p in range(4):
            fub[p] = _fwd_table(8 * (lane & 63) + ((lane >> 6) << 2) + p)
        for cp in small:
            cp.wait()
        cvec = cb_[...].astype(f32)
        fill[:, 0:D] = cvec * jax.nn.sigmoid(cvec)
        dv = db[...].astype(f32).reshape(1, D)
        shv = shb[...].astype(f32)
        for c in range(CT):
            for i in range(4):
                par[c, i] = jnp.broadcast_to(shv[i:i + 1, c * 128:(c + 1) * 128], (8, 128))
            par[c, 4] = jnp.broadcast_to(dv[:, c * 128:(c + 1) * 128], (8, 128))
    def fence(i, carry):
        YP[i, 0:8, :] = jnp.zeros((8, 128), f32)
        return carry

    kw = kb.bitcast(u32)
    vw = vb.bitcast(u32)

    def re_(g):
        return slice(g * 16, g * 16 + 8)

    def im_(g):
        return slice(g * 16 + 8, g * 16 + 16)

    def fwd_k(c, j):
        if SKIPCONV:
            return
        lane = jax.lax.broadcasted_iota(i32, (64, 128), 1)
        even = (lane & 1) == 0
        l01 = (lane & 2) == 0
        l12 = ((lane + 3) & 2) == 0
        rm = []
        for m in range(4):
            w = pltpu.bitcast(skb[c, :, (4 * j + m) * 128:(4 * j + m + 1) * 128], u32)
            rm.append(pltpu.roll(w, m, 1) if m else w)
        e01 = jnp.where(even, rm[0], rm[1])
        o01 = jnp.where(even, rm[1], rm[0])
        e23 = jnp.where(even, rm[2], rm[3])
        o23 = jnp.where(even, rm[3], rm[2])
        kp = [jnp.where(l01, e01, e23), jnp.where(l12, o01, o23),
              jnp.where(l01, e23, e01), jnp.where(l12, o23, o01)]
        tt = [jax.lax.dot_general(pltpu.bitcast(fkb[p], bf16), pltpu.bitcast(kp[p], bf16), NT_DIMS,
                                  preferred_element_type=f32) for p in range(4)]
        dvec = par[c, 4] if j == 0 else None
        for g in range(16):
            re = [t[re_(g)] for t in tt]
            im = [t[im_(g)] for t in tt]
            if j == 0:
                re[0] = re[0] + dvec
            x = _radix4(re, im, False)
            for m in range(4):
                xr, xi = x[m]
                if j < NB - 1:
                    KS[c, j, m, re_(g), :] = xr
                    KS[c, j, m, im_(g), :] = xi
                ur, ui = US[c, 0, m, re_(g), :], US[c, 0, m, im_(g), :]
                YS[c, j, m, re_(g), :] = xr * ur - xi * ui
                YS[c, j, m, im_(g), :] = xr * ui + xi * ur

    def fwd_u(c, a):
        if SKIPCONV:
            return
        taps = [jnp.tile(par[c, i], (8, 1)) for i in range(4)]
        ws = TR // 2
        base = a * (BLK // 8) * ws + 4 * c

        def words(ref, start):
            return ref[pl.ds(start, BLK // 8, stride=ws), :]

        kk = {}
        for w in range(4):
            x = words(kw, ws + base + w)
            kk[2 * w], kk[2 * w + 1] = _lo(x), _hi(x)
        kk[-3] = _hi(words(kw, base + 2))
        x = words(kw, base + 3)
        kk[-2], kk[-1] = _lo(x), _hi(x)
        sub = []
        for w in range(4):
            x = words(vw, base + w)
            for r, vv in ((2 * w, _lo(x)), (2 * w + 1, _hi(x))):
                sh = taps[0] * kk[r] + taps[1] * kk[r - 1] + taps[2] * kk[r - 2] + taps[3] * kk[r - 3]
                sub.append(sh * vv)
        kv = [jnp.concatenate([sub[p], sub[p + 4]], axis=0) for p in range(4)]
        tt = [jnp.dot(pltpu.bitcast(fub[p], bf16), kv[p].astype(bf16), preferred_element_type=f32)
              for p in range(4)]
        for g in range(16):
            x = _radix4([t[re_(g)] for t in tt], [t[im_(g)] for t in tt], False)
            for m in range(4):
                xr, xi = x[m]
                if a:
                    if a == 1:
                        pr, pi = US[c, 0, m, re_(g), :], US[c, 0, m, im_(g), :]
                    else:
                        pr, pi = UR[c, m, re_(g), :], UR[c, m, im_(g), :]
                    if a < NB - 1:
                        UR[c, m, re_(g), :] = xr
                        UR[c, m, im_(g), :] = xi
                    if g < 8:
                        xr, xi = xr - pi, xi + pr
                    else:
                        xr, xi = xr + pi, xi - pr
                US[c, a, m, re_(g), :] = xr
                US[c, a, m, im_(g), :] = xi

    def mac_inv(c, a, halves=(0, 1)):
        if SKIPCONV:
            return
        for h in halves:
            words = [[] for _ in range(4)]
            for g in range(8 * h, 8 * h + 8):
                yre, yim = [], []
                for m in range(4):
                    yr, yi = YS[c, a, m, re_(g), :], YS[c, a, m, im_(g), :]
                    for j in range(a):
                        kr, ki = KS[c, j, m, re_(g), :], KS[c, j, m, im_(g), :]
                        ur, ui = US[c, a - j, m, re_(g), :], US[c, a - j, m, im_(g), :]
                        yr = yr + (kr * ur - ki * ui)
                        yi = yi + (kr * ui + ki * ur)
                    yre.append(yr)
                    yim.append(yi)
                pp = _radix4(yre, yim, True)
                for p in range(4):
                    words[p].extend(pp[p])
            for p in range(4):
                pb = jnp.concatenate(words[p], axis=0).astype(bf16)
                r = jnp.dot(pltpu.bitcast(gtb[p, :, h * 128:(h + 1) * 128], bf16), pb,
                            preferred_element_type=f32)
                if h == 0:
                    YP[p] = r
                else:
                    ys[c, pl.ds(a * BLK + p, 128, stride=4), :] = YP[p] + r

    desc = (3, 2, 1, 0)
    def k_tile(c):
        for j in desc:
            fwd_k(c, j)

    with _scope("conv_u0"):
        for p in range(4):
            gtb[p] = _inv_table(p)
        with _scope("w_kv"):
            for cp in kv_copies(0):
                cp.wait()
        for c in range(CT):
            fwd_u(c, 0)
    with _scope("conv_k"):
        done = 0
        for grp in KGRP:
            with _scope("w_sk"):
                for c in grp:
                    sk_copy(c).wait()
            for c in grp:
                k_tile(c)
            if grp is KGRP[-1]:
                for c in range(E0):
                    mac_inv(c, 0)
    for a in range(1, NB):
        with _scope("conv_u%d" % a):
            with _scope("w_kv"):
                for cp in kv_copies(a):
                    cp.wait()
            todo = [(c, a - 1) for c in range(CT)]
            if a == 1:
                todo = todo[E0:]
            late = len(todo) < CT
            for c in range(CT):
                fwd_u(c, a)
                if todo and (not late or c >= CT - len(todo)):
                    mac_inv(*todo.pop(0))

    def mod_cols_dot(o, n, extra):
        act = fill[:, 0:D]

        def sc(k0, k1):
            return jnp.broadcast_to(act[:, k0:k1], (16, k1 - k0)).astype(bf16)

        e = 128 * extra
        r = jnp.dot(sc(0, D), wmb[:, o + e:o + n], preferred_element_type=f32)
        if extra:
            r0 = (jnp.dot(sc(0, D - 64), wmb[0:D - 64, o:o + e], preferred_element_type=f32)
                  + jnp.dot(sc(D - 64, D), wmb[D - 64:D, o:o + e], preferred_element_type=f32))
            r = jnp.concatenate([r0, r], axis=-1)
        return r[0:8]

    def mod_part(part, extra):
        o, n = mod_cols[part]
        r = mod_cols_dot(o, n, extra)
        return [r[:, i * D:(i + 1) * D] for i in range(n // D)]

    def mvec(i):
        return modb[i, 0:1, :]

    def rows(r, n):
        return pl.ds(r, n)

    def load_q(r, ref=qb):
        return ref[rows(r, RG), :].astype(f32)

    def make_x2(r, q, st, ref=ys):
        y = jnp.concatenate([ref[c, rows(r, RG), :] for c in range(CT)], axis=-1)
        return q + (((q - st[0]) * st[1]) * mvec(1) + mvec(0)) * y

    def make_h2(x2, st):
        return ((x2 - st[0]) * st[1]) * mvec(3) + mvec(2)

    def pack_ln(x, st):
        return pltpu.bitcast(((x - st[0]) * st[1]).astype(bf16), u32)

    def a_chain(r_in, r_out, n=PC, links=1):
        qv, yv = qb.at[rows(r_in, n), :], ys.at[:, rows(r_in, n), :]
        xv, hv = x2s.at[rows(r_out, n), :], h2s.at[rows(r_out, n), :]
        prevs = [None] * links
        for g, o in enumerate(range(0, n, RG)):
            q = load_q(o, qv)
            x2 = make_x2(o, q, _stats(q, prevs[g % links]), yv)
            xv[o:o + RG, :] = x2
            st = _stats(x2)
            h2 = make_h2(xv[o:o + RG, :], st)
            hv[o:o + RG, :] = h2
            st = _stats(h2)
            zt[o // 2:(o + RG) // 2, :] = pack_ln(hv[o:o + RG, :], st)
            prevs[g % links] = st[1]

    def mm_w1(r, n, o=0, bal=True):
        z = pltpu.bitcast(zt[o // 2:(o + n) // 2, :], bf16)
        h1 = _gelu(_dot_balanced(z, lambda a, b: pltpu.bitcast(w1p[:, a:b], bf16), D, 4 if bal else 1))
        for c in range(CT):
            h1s[c, rows(r + 8, n), :] = h1[:, c * 128:(c + 1) * 128]

    def mm_w2a(r, bal=True):
        lane = jax.lax.broadcasted_iota(i32, (T, 128), 1)

        def sh(k, c):
            return h1s[c, rows(r + 8 + k, T), :]

        g = jnp.concatenate([
            sh(-1, 0),
            jnp.where(lane < 32, sh(-1, 1), sh(1, 1)),
            jnp.where(lane < 64, sh(1, 2), sh(-2, 2)),
            jnp.where(lane < 96, sh(-2, 3), sh(2, 3)),
            sh(2, 4)], axis=-1)
        hss[rows(r, T), :] = _dot_balanced(g, lambda a, b: pltpu.bitcast(w2p[:, a:b], bf16), D, 4 if bal else 1)

    def mm_w2b(r, links=1):
        hv, sv = h2s.at[rows(r, T), :], hss.at[rows(r, T), :]
        prev = [None] * links
        for n, o in enumerate(range(0, T, RG)):
            x1 = hv[o:o + RG, :] + sv[o:o + RG, :]
            st = _stats(x1, prev[n % links], early=True)
            zb[o // 2:(o + RG) // 2, :] = pack_ln(x1, st)
            prev[n % links] = st[1]

    def mm_w3_main(bal=True):
        z = pltpu.bitcast(zb[...], bf16)
        return (_gelu2 if G2 else _gelu)(_dot_balanced(z, lambda a, b: pltpu.bitcast(w3p[a // 2:b // 2, :], bf16), FM, 4 if bal else 1, nt=True))

    def mm_w3_cols(a, b):
        z = pltpu.bitcast(zb[...], bf16)
        w = pltpu.bitcast(w3p[a // 2:b // 2, :], bf16)
        return _gelu2(jax.lax.dot_general(z, w, NT_DIMS, preferred_element_type=f32))

    def mm_w3_tail():
        z = pltpu.bitcast(zb[...], bf16)
        return (_gelu2 if G2 else _gelu)(jax.lax.dot_general(pltpu.bitcast(w3p[FM // 2:F // 2, :], bf16), z, NT_DIMS, preferred_element_type=f32))

    def join_act(main, tail):
        return jnp.concatenate([main, tail.T], axis=-1)

    def mm_w3(bal):
        tail = mm_w3_tail()
        return join_act(mm_w3_main(bal), tail)

    def mm_w4(r, a, o=0, n=T, bal=True):
        h2 = _dot_balanced(a[o:o + n], lambda c0, c1: pltpu.bitcast(w4p[:, c0:c1], bf16), D, 2 if bal else 1)
        ob[rows(r + o, n), :] = (x2s[rows(r + o, n), :]
                                 + mvec(4) * ((h2s[rows(r + o, n), :] + hss[rows(r + o, n), :]) + (0.5 * h2 if G2 else h2))).astype(bf16)

    groups = list(range(0, P0 + P1, RG))
    with _scope("conv_last"):
        jax.lax.fori_loop(0, 2, fence, 0)
        for c in range(NL):
            mac_inv(c, NB - 1)
    with _scope("pre_a"):
        with _scope("w_q0"):
            mod_copies[0].wait()
            q_copies[0].wait()
        sa, ca, ga = mod_part(0, 1)
        modb[0] = ga * sa
        modb[1] = ga * (1.0 + ca)
        for c in range(NL, CT):
            mac_inv(c, NB - 1)
        st1 = {o: _stats(load_q(o)) for o in groups}
        zt[0:8, 0:128] = jnp.zeros((8, 128), u32)
        st2 = {}
        for o in groups:
            x2 = make_x2(o, load_q(o), st1[o])
            x2s[o:o + RG, :] = x2
            st2[o] = _stats(x2)

    def pass_c(os_, links):
        st3 = {}
        prev = [None] * max(links, 1)
        for n, o in enumerate(os_):
            h2 = make_h2(x2s[o:o + RG, :], st2[o])
            h2s[o:o + RG, :] = h2
            st3[o] = _stats(h2, prev[n % len(prev)], early=True)
            if links:
                prev[n % links] = st3[o][1]
                zt[o // 2:(o + RG) // 2, :] = pack_ln(h2, st3[o])
        if not links:
            for o in os_:
                zt[o // 2:(o + RG) // 2, :] = pack_ln(h2s[o:o + RG, :], st3[o])

    with _scope("pre_b"):
        with _scope("w_modB"):
            mod_copies[1].wait()
        sb, cb = mod_part(1, 2)
        modb[2] = sb
        modb[3] = 1.0 + cb
        pass_c([o for o in groups if o < P0], 0)
    with _scope("r1"):
        with _scope("w_w1"):
            w_copies[0].wait()
        w1p[...] = pltpu.bitcast(w1b[...], u32)
        mm_w1(0, P0)
        pass_c([o for o in groups if o >= P0], CL1)
        mm_w1(P0, P1, P0)
    with _scope("r2"):
        with _scope("w_w2"):
            w_copies[1].wait()
            q_copies[1].wait()
        w2p[...] = pltpu.bitcast(w2b[...], u32)
        a_chain(P0 + P1, P0 + P1, PA, CLA)
        mm_w2a(0)
        mm_w2b(0, 2)
        mm_w2a(T)
    with _scope("r3"):
        with _scope("w_w3"):
            w_copies[2].wait()
            q_copies[2].wait()
        w3p[...] = pltpu.bitcast(w3b[...], u32)
        for tok in R3:
            if tok == '1':
                mm_w1(P0 + P1, PA)
            elif tok == 'c':
                a_chain(PB, PB)
            elif tok == '3':
                main = mm_w3_main()
            else:
                tail = mm_w3_tail()
    with _scope("r4"):
        with _scope("w_w4"):
            w_copies[3].wait()
            mod_copies[2].wait()
        w4p[...] = pltpu.bitcast(w4b[...], u32)
        modb[4] = mod_part(2, 1)[0]
        mm_w4(0, join_act(main, tail))
        mm_w2b(T)
        out_copy(0).start()
        q_copies[3].wait()

    def mlp_iter(i):
        r1 = pl.multiple_of(PB - PC + PC * i, 16)
        r = pl.multiple_of(i * T, T)
        mains = []
        for tok in BODY:
            if tok == 't':
                tail = mm_w3_tail()
            elif tok == '1':
                mm_w1(r1, PC, bal='1' in LBAL)
            elif tok == 'c':
                a_chain(pl.multiple_of(jnp.minimum(r1 + PC, S - PC), 16), r1 + PC)
            elif tok == '3':
                mains.append(mm_w3_main('3' in LBAL))
            elif tok == 'x':
                mains.append(mm_w3_cols(0, W3S))
            elif tok == 'y':
                mains.append(mm_w3_cols(W3S, FM))
            elif tok == '2':
                mm_w2a(r + T, bal='2' in LBAL)
            elif tok == 'l':
                mm_w2b(r + T)
            elif tok == '4':
                mm_w4(r, join_act(jnp.concatenate(mains, axis=-1), tail), bal='4' in LBAL)
        out_copy(i).start()

    def mlp_body(i, carry):
        with _scope("iter"):
            mlp_iter(i)
        return carry

    with _scope("loop"):
        jax.lax.fori_loop(1, NC - 1, mlp_body, 0)
    with _scope("last"):
        act = mm_w3(False)
        mm_w4(S - T, act, 0, LAST0, bal=False)
        out_tail[0].start()
        mm_w4(S - T, act, LAST0, T - LAST0, bal=False)
        out_tail[1].start()
    with _scope("fin"):
        for i in range(NC - 1):
            out_copy(i).wait()
        for cp in out_tail:
            cp.wait()


@jax.jit
def pallas_adaLN_cond__ssm_conv_h3__mixer_s_mlp__prompt_kernel(
    A_q: jax.Array,
    A_k: jax.Array,
    A_v: jax.Array,
    A_shift_k: jax.Array,
    A_ssm_k: jax.Array,
    A_ssm_D: jax.Array,
    B_x: jax.Array,
    B_w1: jax.Array,
    B_w2: jax.Array,
    B_w3: jax.Array,
    B_w4: jax.Array,
    c: jax.Array,
    w_mod: jax.Array,
):
    del B_x
    any_spec = pl.BlockSpec(memory_space=pl.ANY)

    def tile_view(x):
        return x.reshape(S // 8, 8, CT, 128).transpose(0, 2, 1, 3).reshape(S * CT, 128)

    vm = pltpu.VMEM
    dma = pltpu.SemaphoreType.DMA
    out = pl.pallas_call(
        _kernel,
        in_specs=[any_spec] * 12,
        out_specs=any_spec,
        out_shape=jax.ShapeDtypeStruct((S, D), bf16),
        scratch_shapes=[
            vm((S * CT + 128, 128), bf16), vm((S * CT + 64, 128), bf16), vm((CT, 128, S), bf16),
            vm((S, D), bf16), vm((D, D), bf16), vm((D, D), bf16), vm((F, D), bf16), vm((F, D), bf16),
            vm((D // 2, D), u32), vm((D // 2, D), u32), vm((F // 2, D), u32), vm((F // 2, D), u32),
            vm((D, 6 * D), bf16), vm((4, D), bf16), vm((D,), bf16), vm((1, D), bf16), vm((1, FILL), f32),
            vm((4, 128, 128), u32), vm((4, 128, 128), u32), vm((4, 64, 256), u32),
            vm((CT, 8, 8, 128), f32),
            vm((CT, NB, 4, 256, 128), f32), vm((CT, NB - 1, 4, 256, 128), f32),
            vm((CT, 4, 256, 128), f32), vm((CT, NB, 4, 256, 128), f32), vm((4, 128, 128), f32),
            vm((CT, S + 32, 128), f32), vm((8, 8, D), f32),
            vm((CT, S + 32, 128), f32), vm((S + 256, D), f32), vm((S + 256, D), f32),
            vm((S, D), f32),
            vm((288, D), u32), vm((T // 2, D), u32),
            vm((S, D), bf16),
            dma((29,)), dma((NC + 1,)),
        ],
        compiler_params=pltpu.CompilerParams(vmem_limit_bytes=110 << 20, disable_bounds_checks=True,
                                             disable_semaphore_checks=True),
    )(A_q.reshape(S, D), tile_view(A_k), tile_view(A_v), A_shift_k.T, A_ssm_k,
      A_ssm_D, B_w1, B_w2, B_w3.T, B_w4, c, w_mod)
    return out.reshape(1, S, D)
```

```python
import os
import numpy as np
import jax
import jax.numpy as jnp
import jax.experimental.pallas as pl
import jax.experimental.pallas.tpu as pltpu

f32, bf16, u32, i32 = jnp.float32, jnp.bfloat16, jnp.uint32, jnp.int32

S, D, F = 2048, 640, 1728
CT = D // 128
NB, BLK, NFFT = 4, 512, 1024
T = 256
NC = S // T
RSQ = int(os.environ.get('RSQ', '0'))
SAME = int(os.environ.get('SAME', '1'))
LL = int(os.environ.get('LL', '1'))
NS = [int(x) * 128 for x in os.environ.get('NS', '0125')]
R2 = os.environ.get('R2', 'x')
FILL = int(os.environ.get('FILL', '1792'))
VIEW = int(os.environ.get('VIEW', '1'))
CL1 = int(os.environ.get('CL1', '1'))
CLA = int(os.environ.get('CLA', '2'))
R3 = os.environ.get('R3', 'a31t')
G2 = int(os.environ.get('G2', '1'))
NL = int(os.environ.get('NL', '4'))
LBAL = os.environ.get('LBAL', '')
BODY = os.environ.get('BODY', 'ct3p1q2lr')
SKIPCONV = int(os.environ.get('SKIPCONV', '0'))
RELOAD = int(os.environ.get('RELOAD', '1'))
W3S = int(os.environ.get('W3S', '512'))
LAST0 = int(os.environ.get('LAST0', '192'))
FM = (F // 128) * 128
E0 = int(os.environ.get('E0', '0'))
KGRP = [tuple(int(x) for x in g) for g in os.environ.get('KGRP', '0,12,34').split(',')]
TR = 8 * CT
P0, P1, PC = int(os.environ.get('P0', '320')), 528 - int(os.environ.get('P0', '320')), int(os.environ.get('PC', '224'))
PA = S - P0 - P1 - 6 * PC
RG = 16
EPS = 1e-5
NT_DIMS = (((1,), (1,)), ((), ()))
SCOPES = bool(int(os.environ.get("KSCOPES", "0")))


class _NoScope:
    def __enter__(self):
        return self

    def __exit__(self, *a):
        return False


def _scope(name):
    return jax.named_scope(name) if SCOPES else _NoScope()


def _lo(w):
    return pltpu.bitcast(w << 16, f32)


def _hi(w):
    return pltpu.bitcast(w & jnp.uint32(0xFFFF0000), f32)


def _cos_turn(n32, scale):
    x = 2.0 ** 30 - jnp.abs(n32.astype(f32))
    b = 2.0 * np.pi / 2.0 ** 32
    x = x * b
    x2 = x * x
    c = [scale * v for v in (1.0, -1.0 / 6, 1.0 / 120, -1.0 / 5040, 1.0 / 362880)]
    return x * (c[0] + x2 * (c[1] + x2 * (c[2] + x2 * (c[3] + x2 * c[4]))))


def _odd_freq(k):
    return jnp.where(k < 64, 4 * k + 1, 4 * k - 253) << 21


def _slot_phase(idx):
    k = ((idx >> 4) << 3) + (idx & 7)
    return _odd_freq(k), (idx & 8) << 27


def _fwd_table(r):
    fr, off = _slot_phase(jax.lax.broadcasted_iota(i32, (256, 128), 0))
    return pltpu.bitcast(_cos_turn(fr * r + off, 1.0).astype(bf16), u32)


def _inv_table(p):
    row = jax.lax.broadcasted_iota(i32, (128, 256), 0)
    fr, off = _slot_phase(jax.lax.broadcasted_iota(i32, (128, 256), 1))
    return pltpu.bitcast(_cos_turn(fr * (4 * row + p) + off, 2.0 / NFFT).astype(bf16), u32)


def _stats(x, link=None, early=False):
    zero = 0.0 if link is None else jnp.minimum(link, 0.0)
    part = x[:, 0:128]
    for c in range(1, CT):
        part = part + x[:, c * 128:(c + 1) * 128]
    if link is not None and early:
        part = part + zero
        zero = 0.0
    m = jnp.sum(part, axis=-1, keepdims=True) * (1.0 / D)
    v = jnp.maximum(jnp.sum(x * x, axis=-1, keepdims=True) * (1.0 / D) - m * m, zero)
    if RSQ:
        return m, jnp.exp2(jnp.log(v + EPS) * (-0.5 / np.log(2.0)))
    return m, jax.lax.rsqrt(v + EPS)


def _gelu2(x):
    c = 0.7978845608028654
    u = c + (c * 0.044715) * (x * x)
    return x + x * jnp.tanh(x * u)


def _gelu(x):
    c = 0.7978845608028654
    u = c + (c * 0.044715) * (x * x)
    t = jnp.tanh(x * u)
    hx = 0.5 * x
    return hx + hx * t


def _row_parts(m, parts):
    base, extra = divmod(m // 16, parts)
    out, o = [], 0
    for i in range(parts):
        n = 16 * (base + (1 if i < extra else 0))
        out.append((o, n))
        o += n
    return out


def _dot_balanced(x, wslice, n_cols, parts, nt=False):
    def mm(a, c0, c1):
        a = a.astype(bf16)
        if nt:
            return jax.lax.dot_general(a, wslice(c0, c1), NT_DIMS, preferred_element_type=f32)
        return jnp.dot(a, wslice(c0, c1), preferred_element_type=f32)
    if parts == 1:
        return mm(x, 0, n_cols)
    head = mm(x, 0, n_cols - 128)
    last = jnp.concatenate([mm(x[o:o + n], n_cols - 128, n_cols) for o, n in _row_parts(x.shape[0], parts)],
                           axis=0)
    return jnp.concatenate([head, last], axis=-1)


def _radix4(re, im, inverse):
    ar, ai = re[0] + re[2], im[0] + im[2]
    br, bi = re[0] - re[2], im[0] - im[2]
    cr, ci = re[1] + re[3], im[1] + im[3]
    dr, di = re[1] - re[3], im[1] - im[3]
    minus_i = (br + di, bi - dr)
    plus_i = (br - di, bi + dr)
    if inverse:
        return [(ar + cr, ai + ci), plus_i, (ar - cr, ai - ci), minus_i]
    return [(ar + cr, ai + ci), minus_i, (ar - cr, ai - ci), plus_i]


def _kernel(q_hbm, k_hbm, v_hbm, sh_hbm, sk_hbm, d_hbm, w1_hbm, w2_hbm, w3_hbm, w4_hbm,
            c_hbm, wm_hbm, o_hbm,
            kb, vb, skb, qb, w1b, w2b, w3b, w4b, w1p, w2p, w3p, w4p, wmb, shb, db, cb_, fill, fub, fkb, gtb, par,
            US, KS, UR, YS, YP, ys, modb, h1s, h2s, x2s, hss, zt, zb, ob,
            sem, sem_o):
    def sk_copy(c):
        return pltpu.make_async_copy(sk_hbm.at[pl.ds(c * 128, 128), :], skb.at[c], sem.at[c])

    def kv_copies(a):
        n = BLK * CT
        return [
            pltpu.make_async_copy(k_hbm.at[pl.ds(a * n, n), :], kb.at[pl.ds(TR + a * n, n), :], sem.at[CT + a]),
            pltpu.make_async_copy(v_hbm.at[pl.ds(a * n, n), :], vb.at[pl.ds(a * n, n), :], sem.at[2 * CT + a]),
        ]

    small = [pltpu.make_async_copy(src, dst, sem.at[15 + i]) for i, (src, dst) in enumerate(
        [(d_hbm, db), (sh_hbm, shb), (c_hbm, cb_)])]

    mod_cols = [(0, 3 * D), (3 * D, 2 * D), (5 * D, D)]
    mod_copies = [pltpu.make_async_copy(wm_hbm.at[:, pl.ds(o, n)], wmb.at[:, pl.ds(o, n)], sem.at[18 + i])
                  for i, (o, n) in enumerate(mod_cols)]
    w_pairs = [(w1_hbm, w1b), (w2_hbm, w2b), (w3_hbm, w3b), (w4_hbm, w4b)]
    w_copies = [pltpu.make_async_copy(src, dst, sem.at[21 + i]) for i, (src, dst) in enumerate(w_pairs)]
    PB = P0 + P1 + PA
    q_rows = [(0, P0 + P1), (P0 + P1, PA), (PB, PC), (PB + PC, S - PB - PC)]
    q_copies = [pltpu.make_async_copy(q_hbm.at[pl.ds(o, n), :], qb.at[pl.ds(o, n), :], sem.at[25 + i])
                for i, (o, n) in enumerate(q_rows)]

    def out_copy(i):
        r = i * T if isinstance(i, int) else pl.multiple_of(i * T, T)
        return pltpu.make_async_copy(ob.at[pl.ds(r, T), :], o_hbm.at[pl.ds(r, T), :], sem_o.at[i])

    out_tail = [pltpu.make_async_copy(ob.at[pl.ds(o, n), :], o_hbm.at[pl.ds(o, n), :], sem_o.at[NC - 1 + i])
                for i, (o, n) in enumerate([(S - T, LAST0), (S - T + LAST0, T - LAST0)])]

    for cp in small + kv_copies(0):
        cp.start()
    for c in range(CT):
        sk_copy(c).start()
    for a in range(1, NB):
        for cp in kv_copies(a):
            cp.start()
    order = [mod_copies[0], q_copies[0], mod_copies[1], w_copies[0], w_copies[1], q_copies[1],
             w_copies[2], q_copies[2], w_copies[3], mod_copies[2], q_copies[3]]
    if SAME:
        order = [mod_copies[0], q_copies[0], mod_copies[1], w_copies[0], w_copies[1], q_copies[1],
                 w_copies[2], w_copies[3], mod_copies[2], q_copies[2], q_copies[3]]
    for cp in order:
        cp.start()

    with _scope("init"):
        def pin(i, carry):
            fill[:, pl.ds(pl.multiple_of(i * 128, 128), 128)] = jnp.zeros((1, 128), f32)
            YP[i, 0:8, :] = jnp.zeros((8, 128), f32)
            US[i, 0, 0, 0:8, :] = jnp.zeros((8, 128), f32)
            KS[i, 0, 0, 0:8, :] = jnp.zeros((8, 128), f32)
            YS[i, 0, 0, 0:8, :] = jnp.zeros((8, 128), f32)
            UR[i, 0, 0:8, :] = jnp.zeros((8, 128), f32)
            return carry

        jax.lax.fori_loop(0, 2, pin, 0)
        lane = jax.lax.broadcasted_iota(i32, (256, 128), 1)
        for p in range(4):
            m = (lane - p) & 3
            fkb[p] = _fwd_table(128 * m + ((lane - m) & 127))
        for c in range(CT):
            kb[c * 8:(c + 1) * 8, :] = jnp.zeros((8, 128), bf16)
            h1s[c, 0:8, :] = jnp.zeros((8, 128), f32)
            h1s[c, S + 8:S + 16, :] = jnp.zeros((8, 128), f32)
        for p in range(4):
            fub[p] = _fwd_table(8 * (lane & 63) + ((lane >> 6) << 2) + p)
        for cp in small:
            cp.wait()
        cvec = cb_[...].astype(f32)
        fill[:, 0:D] = cvec * jax.nn.sigmoid(cvec)
        dv = db[...].astype(f32).reshape(1, D)
        shv = shb[...].astype(f32)
        for c in range(CT):
            for i in range(4):
                par[c, i] = jnp.broadcast_to(shv[i:i + 1, c * 128:(c + 1) * 128], (8, 128))
            par[c, 4] = jnp.broadcast_to(dv[:, c * 128:(c + 1) * 128], (8, 128))
    def fence(i, carry):
        YP[i, 0:8, :] = jnp.zeros((8, 128), f32)
        return carry

    kw = kb.bitcast(u32)
    vw = vb.bitcast(u32)

    def re_(g):
        return slice(g * 16, g * 16 + 8)

    def im_(g):
        return slice(g * 16 + 8, g * 16 + 16)

    def fwd_k(c, j):
        if SKIPCONV:
            return
        lane = jax.lax.broadcasted_iota(i32, (64, 128), 1)
        even = (lane & 1) == 0
        l01 = (lane & 2) == 0
        l12 = ((lane + 3) & 2) == 0
        rm = []
        for m in range(4):
            w = pltpu.bitcast(skb[c, :, (4 * j + m) * 128:(4 * j + m + 1) * 128], u32)
            rm.append(pltpu.roll(w, m, 1) if m else w)
        e01 = jnp.where(even, rm[0], rm[1])
        o01 = jnp.where(even, rm[1], rm[0])
        e23 = jnp.where(even, rm[2], rm[3])
        o23 = jnp.where(even, rm[3], rm[2])
        kp = [jnp.where(l01, e01, e23), jnp.where(l12, o01, o23),
              jnp.where(l01, e23, e01), jnp.where(l12, o23, o01)]
        tt = [jax.lax.dot_general(pltpu.bitcast(fkb[p], bf16), pltpu.bitcast(kp[p], bf16), NT_DIMS,
                                  preferred_element_type=f32) for p in range(4)]
        dvec = par[c, 4] if j == 0 else None
        for g in range(16):
            re = [t[re_(g)] for t in tt]
            im = [t[im_(g)] for t in tt]
            if j == 0:
                re[0] = re[0] + dvec
            x = _radix4(re, im, False)
            for m in range(4):
                xr, xi = x[m]
                if j < NB - 1:
                    KS[c, j, m, re_(g), :] = xr
                    KS[c, j, m, im_(g), :] = xi
                ur, ui = US[c, 0, m, re_(g), :], US[c, 0, m, im_(g), :]
                YS[c, j, m, re_(g), :] = xr * ur - xi * ui
                YS[c, j, m, im_(g), :] = xr * ui + xi * ur

    def fwd_u(c, a):
        if SKIPCONV:
            return
        taps = [jnp.tile(par[c, i], (8, 1)) for i in range(4)]
        ws = TR // 2
        base = a * (BLK // 8) * ws + 4 * c

        def words(ref, start):
            return ref[pl.ds(start, BLK // 8, stride=ws), :]

        kk = {}
        for w in range(4):
            x = words(kw, ws + base + w)
            kk[2 * w], kk[2 * w + 1] = _lo(x), _hi(x)
        kk[-3] = _hi(words(kw, base + 2))
        x = words(kw, base + 3)
        kk[-2], kk[-1] = _lo(x), _hi(x)
        sub = []
        for w in range(4):
            x = words(vw, base + w)
            for r, vv in ((2 * w, _lo(x)), (2 * w + 1, _hi(x))):
                sh = taps[0] * kk[r] + taps[1] * kk[r - 1] + taps[2] * kk[r - 2] + taps[3] * kk[r - 3]
                sub.append(sh * vv)
        kv = [jnp.concatenate([sub[p], sub[p + 4]], axis=0) for p in range(4)]
        tt = [jnp.dot(pltpu.bitcast(fub[p], bf16), kv[p].astype(bf16), preferred_element_type=f32)
              for p in range(4)]
        for g in range(16):
            x = _radix4([t[re_(g)] for t in tt], [t[im_(g)] for t in tt], False)
            for m in range(4):
                xr, xi = x[m]
                if a:
                    if a == 1:
                        pr, pi = US[c, 0, m, re_(g), :], US[c, 0, m, im_(g), :]
                    else:
                        pr, pi = UR[c, m, re_(g), :], UR[c, m, im_(g), :]
                    if a < NB - 1:
                        UR[c, m, re_(g), :] = xr
                        UR[c, m, im_(g), :] = xi
                    if g < 8:
                        xr, xi = xr - pi, xi + pr
                    else:
                        xr, xi = xr + pi, xi - pr
                US[c, a, m, re_(g), :] = xr
                US[c, a, m, im_(g), :] = xi

    def mac_inv(c, a, halves=(0, 1)):
        if SKIPCONV:
            return
        for h in halves:
            words = [[] for _ in range(4)]
            for g in range(8 * h, 8 * h + 8):
                yre, yim = [], []
                for m in range(4):
                    yr, yi = YS[c, a, m, re_(g), :], YS[c, a, m, im_(g), :]
                    for j in range(a):
                        kr, ki = KS[c, j, m, re_(g), :], KS[c, j, m, im_(g), :]
                        ur, ui = US[c, a - j, m, re_(g), :], US[c, a - j, m, im_(g), :]
                        yr = yr + (kr * ur - ki * ui)
                        yi = yi + (kr * ui + ki * ur)
                    yre.append(yr)
                    yim.append(yi)
                pp = _radix4(yre, yim, True)
                for p in range(4):
                    words[p].extend(pp[p])
            for p in range(4):
                pb = jnp.concatenate(words[p], axis=0).astype(bf16)
                r = jnp.dot(pltpu.bitcast(gtb[p, :, h * 128:(h + 1) * 128], bf16), pb,
                            preferred_element_type=f32)
                if h == 0:
                    YP[p] = r
                else:
                    ys[c, pl.ds(a * BLK + p, 128, stride=4), :] = YP[p] + r

    desc = (3, 2, 1, 0)
    def k_tile(c):
        for j in desc:
            fwd_k(c, j)

    with _scope("conv_u0"):
        for p in range(4):
            gtb[p] = _inv_table(p)
        with _scope("w_kv"):
            for cp in kv_copies(0):
                cp.wait()
        for c in range(CT):
            fwd_u(c, 0)
    with _scope("conv_k"):
        done = 0
        for grp in KGRP:
            with _scope("w_sk"):
                for c in grp:
                    sk_copy(c).wait()
            for c in grp:
                k_tile(c)
            if grp is KGRP[-1]:
                for c in range(E0):
                    mac_inv(c, 0)
    for a in range(1, NB):
        with _scope("conv_u%d" % a):
            with _scope("w_kv"):
                for cp in kv_copies(a):
                    cp.wait()
            todo = [(c, a - 1) for c in range(CT)]
            if a == 1:
                todo = todo[E0:]
            late = len(todo) < CT
            for c in range(CT):
                fwd_u(c, a)
                if todo and (not late or c >= CT - len(todo)):
                    mac_inv(*todo.pop(0))

    def mod_cols_dot(o, n, extra):
        act = fill[:, 0:D]

        def sc(k0, k1):
            return jnp.broadcast_to(act[:, k0:k1], (16, k1 - k0)).astype(bf16)

        e = 128 * extra
        r = jnp.dot(sc(0, D), wmb[:, o + e:o + n], preferred_element_type=f32)
        if extra:
            r0 = (jnp.dot(sc(0, D - 64), wmb[0:D - 64, o:o + e], preferred_element_type=f32)
                  + jnp.dot(sc(D - 64, D), wmb[D - 64:D, o:o + e], preferred_element_type=f32))
            r = jnp.concatenate([r0, r], axis=-1)
        return r[0:8]

    def mod_part(part, extra):
        o, n = mod_cols[part]
        r = mod_cols_dot(o, n, extra)
        return [r[:, i * D:(i + 1) * D] for i in range(n // D)]

    def mvec(i, n=RG, c0=0, c1=D):
        return jnp.tile(modb[i, :, c0:c1], (n // 8, 1))

    def rows(r, n):
        return pl.ds(r, n)

    def load_q(r, ref=qb):
        return ref[rows(r, RG), :].astype(f32)

    def make_x2(r, q, st, ref=ys):
        y = jnp.concatenate([ref[c, rows(r, RG), :] for c in range(CT)], axis=-1)
        return q + (((q - st[0]) * st[1]) * mvec(1) + mvec(0)) * y

    def make_h2(x2, st):
        return ((x2 - st[0]) * st[1]) * mvec(3) + mvec(2)

    def pack_ln(x, st):
        return pltpu.bitcast(((x - st[0]) * st[1]).astype(bf16), u32)

    def a_chain(r_in, r_out, n=PC, links=1):
        qv, yv = qb.at[rows(r_in, n), :], ys.at[:, rows(r_in, n), :]
        xv, hv = x2s.at[rows(r_out, n), :], h2s.at[rows(r_out, n), :]
        prevs = [None] * links
        for g, o in enumerate(range(0, n, RG)):
            q = load_q(o, qv)
            x2 = make_x2(o, q, _stats(q, prevs[g % links]), yv)
            xv[o:o + RG, :] = x2
            st = _stats(x2)
            h2 = make_h2(xv[o:o + RG, :], st)
            hv[o:o + RG, :] = h2
            st = _stats(h2)
            zt[o // 2:(o + RG) // 2, :] = pack_ln(hv[o:o + RG, :], st)
            prevs[g % links] = st[1]

    def mm_w1(r, n, o=0, bal=True):
        z = pltpu.bitcast(zt[o // 2:(o + n) // 2, :], bf16)
        h1 = _gelu(_dot_balanced(z, lambda a, b: pltpu.bitcast(w1p[:, a:b], bf16), D, 4 if bal else 1))
        for c in range(CT):
            h1s[c, rows(r + 8, n), :] = h1[:, c * 128:(c + 1) * 128]

    def mm_w2a(r, bal=True):
        lane = jax.lax.broadcasted_iota(i32, (T, 128), 1)

        def sh(k, c):
            return h1s[c, rows(r + 8 + k, T), :]

        g = jnp.concatenate([
            sh(-1, 0),
            jnp.where(lane < 32, sh(-1, 1), sh(1, 1)),
            jnp.where(lane < 64, sh(1, 2), sh(-2, 2)),
            jnp.where(lane < 96, sh(-2, 3), sh(2, 3)),
            sh(2, 4)], axis=-1)
        hss[rows(r, T), :] = _dot_balanced(g, lambda a, b: pltpu.bitcast(w2p[:, a:b], bf16), D, 4 if bal else 1)

    def mm_w2b(r, links=1):
        hv, sv = h2s.at[rows(r, T), :], hss.at[rows(r, T), :]
        prev = [None] * links
        for n, o in enumerate(range(0, T, RG)):
            x1 = hv[o:o + RG, :] + sv[o:o + RG, :]
            st = _stats(x1, prev[n % links], early=True)
            zb[o // 2:(o + RG) // 2, :] = pack_ln(x1, st)
            prev[n % links] = st[1]

    def mm_w3_main(bal=True):
        z = pltpu.bitcast(zb[...], bf16)
        return (_gelu2 if G2 else _gelu)(_dot_balanced(z, lambda a, b: pltpu.bitcast(w3p[a // 2:b // 2, :], bf16), FM, 4 if bal else 1, nt=True))

    def mm_w3_cols(a, b):
        z = pltpu.bitcast(zb[...], bf16)
        w = pltpu.bitcast(w3p[a // 2:b // 2, :], bf16)
        return _gelu2(jax.lax.dot_general(z, w, NT_DIMS, preferred_element_type=f32))

    def mm_w3_tail():
        z = pltpu.bitcast(zb[...], bf16)
        return (_gelu2 if G2 else _gelu)(jax.lax.dot_general(pltpu.bitcast(w3p[FM // 2:F // 2, :], bf16), z, NT_DIMS, preferred_element_type=f32))

    def join_act(main, tail):
        return jnp.concatenate([main, tail.T], axis=-1)

    def mm_w3(bal):
        tail = mm_w3_tail()
        return join_act(mm_w3_main(bal), tail)

    def mm_w4(r, a, o=0, n=T, bal=True):
        h2 = _dot_balanced(a[o:o + n], lambda c0, c1: pltpu.bitcast(w4p[:, c0:c1], bf16), D, 2 if bal else 1)
        ob[rows(r + o, n), :] = (x2s[rows(r + o, n), :]
                                 + mvec(4, n) * ((h2s[rows(r + o, n), :] + hss[rows(r + o, n), :]) + (0.5 * h2 if G2 else h2))).astype(bf16)

    def mm_w4_cols(r, a, c0, c1):
        h2 = jnp.dot(a, pltpu.bitcast(w4p[:, c0:c1], bf16), preferred_element_type=f32)
        ob[rows(r, T), c0:c1] = (x2s[rows(r, T), c0:c1] + mvec(4, T, c0, c1) * (
            (h2s[rows(r, T), c0:c1] + hss[rows(r, T), c0:c1]) + 0.5 * h2)).astype(bf16)

    groups = list(range(0, P0 + P1, RG))
    with _scope("conv_last"):
        jax.lax.fori_loop(0, 2, fence, 0)
        for c in range(NL):
            mac_inv(c, NB - 1)
    with _scope("pre_a"):
        with _scope("w_q0"):
            mod_copies[0].wait()
            q_copies[0].wait()
        sa, ca, ga = mod_part(0, 1)
        modb[0] = ga * sa
        modb[1] = ga * (1.0 + ca)
        for c in range(NL, CT):
            mac_inv(c, NB - 1)
        st1 = {o: _stats(load_q(o)) for o in groups}
        zt[0:8, 0:128] = jnp.zeros((8, 128), u32)
        st2 = {}
        for o in groups:
            x2 = make_x2(o, load_q(o), st1[o])
            x2s[o:o + RG, :] = x2
            st2[o] = _stats(x2)

    def pass_c(os_, links):
        st3 = {}
        prev = [None] * max(links, 1)
        for n, o in enumerate(os_):
            h2 = make_h2(x2s[o:o + RG, :], st2[o])
            h2s[o:o + RG, :] = h2
            st3[o] = _stats(h2, prev[n % len(prev)], early=True)
            if links:
                prev[n % links] = st3[o][1]
                zt[o // 2:(o + RG) // 2, :] = pack_ln(h2, st3[o])
        if not links:
            for o in os_:
                zt[o // 2:(o + RG) // 2, :] = pack_ln(h2s[o:o + RG, :], st3[o])

    with _scope("pre_b"):
        with _scope("w_modB"):
            mod_copies[1].wait()
        sb, cb = mod_part(1, 2)
        modb[2] = sb
        modb[3] = 1.0 + cb
        pass_c([o for o in groups if o < P0], 0)
    with _scope("r1"):
        with _scope("w_w1"):
            w_copies[0].wait()
        w1p[...] = pltpu.bitcast(w1b[...], u32)
        mm_w1(0, P0)
        pass_c([o for o in groups if o >= P0], CL1)
        mm_w1(P0, P1, P0)
    with _scope("r2"):
        with _scope("w_w2"):
            w_copies[1].wait()
            q_copies[1].wait()
        w2p[...] = pltpu.bitcast(w2b[...], u32)
        if 'c' in R2:
            a_chain(P0 + P1, P0 + P1, PA, CLA)
        mm_w2a(0)
        mm_w2b(0, 2)
        mm_w2a(T)
    with _scope("r3"):
        with _scope("w_w3"):
            w_copies[2].wait()
            if not SAME:
                q_copies[2].wait()
        w3p[...] = pltpu.bitcast(w3b[...], u32)
        for tok in R3:
            if tok == '1':
                mm_w1(P0 + P1, PA)
            elif tok == 'c':
                a_chain(PB, PB)
            elif tok == 'a':
                a_chain(P0 + P1, P0 + P1, PA)
            elif tok == '3':
                main = mm_w3_main()
            else:
                tail = mm_w3_tail()
    with _scope("r4"):
        with _scope("w_w4"):
            w_copies[3].wait()
            mod_copies[2].wait()
        w4p[...] = pltpu.bitcast(w4b[...], u32)
        modb[4] = mod_part(2, 1)[0]
        mm_w4(0, join_act(main, tail))
        mm_w2b(T)
        out_copy(0).start()
        q_copies[3].wait()
        if SAME:
            q_copies[2].wait()

    def mlp_iter(i):
        r1 = pl.multiple_of(PB - PC + PC * i, 16)
        r = pl.multiple_of(i * T, T)
        mains = []
        for tok in BODY:
            if tok == 't':
                tail = mm_w3_tail()
            elif tok == '1':
                mm_w1(r1, PC, bal='1' in LBAL)
            elif tok == 'c':
                if SAME:
                    a_chain(r1, r1)
                else:
                    a_chain(pl.multiple_of(jnp.minimum(r1 + PC, S - PC), 16), r1 + PC)
            elif tok in 'pqr':
                if tok == 'p':
                    act = join_act(jnp.concatenate(mains, axis=-1), tail).astype(bf16)
                k = 'pqr'.index(tok)
                mm_w4_cols(r, act, NS[k], NS[k + 1])
            elif tok == '3':
                mains.append(mm_w3_main('3' in LBAL))
            elif tok == 'x':
                mains.append(mm_w3_cols(0, W3S))
            elif tok == 'y':
                mains.append(mm_w3_cols(W3S, FM))
            elif tok == '2':
                mm_w2a(r + T, bal='2' in LBAL)
            elif tok == 'l':
                mm_w2b(r + T, LL)
            elif tok == '4':
                mm_w4(r, join_act(jnp.concatenate(mains, axis=-1), tail), bal='4' in LBAL)
        out_copy(i).start()

    def mlp_body(i, carry):
        with _scope("iter"):
            mlp_iter(i)
        return carry

    with _scope("loop"):
        jax.lax.fori_loop(1, NC - 1, mlp_body, 0)
    with _scope("last"):
        act = mm_w3(False)
        mm_w4(S - T, act, 0, LAST0, bal=False)
        out_tail[0].start()
        mm_w4(S - T, act, LAST0, T - LAST0, bal=False)
        out_tail[1].start()
    with _scope("fin"):
        for i in range(NC - 1):
            out_copy(i).wait()
        for cp in out_tail:
            cp.wait()


@jax.jit
def pallas_adaLN_cond__ssm_conv_h3__mixer_s_mlp__prompt_kernel(
    A_q: jax.Array,
    A_k: jax.Array,
    A_v: jax.Array,
    A_shift_k: jax.Array,
    A_ssm_k: jax.Array,
    A_ssm_D: jax.Array,
    B_x: jax.Array,
    B_w1: jax.Array,
    B_w2: jax.Array,
    B_w3: jax.Array,
    B_w4: jax.Array,
    c: jax.Array,
    w_mod: jax.Array,
):
    del B_x
    any_spec = pl.BlockSpec(memory_space=pl.ANY)

    def tile_view(x):
        return x.reshape(S // 8, 8, CT, 128).transpose(0, 2, 1, 3).reshape(S * CT, 128)

    vm = pltpu.VMEM
    dma = pltpu.SemaphoreType.DMA
    out = pl.pallas_call(
        _kernel,
        in_specs=[any_spec] * 12,
        out_specs=any_spec,
        out_shape=jax.ShapeDtypeStruct((S, D), bf16),
        scratch_shapes=[
            vm((S * CT + 128, 128), bf16), vm((S * CT + 64, 128), bf16), vm((CT, 128, S), bf16),
            vm((S, D), bf16), vm((D, D), bf16), vm((D, D), bf16), vm((F, D), bf16), vm((F, D), bf16),
            vm((D // 2, D), u32), vm((D // 2, D), u32), vm((F // 2, D), u32), vm((F // 2, D), u32),
            vm((D, 6 * D), bf16), vm((4, D), bf16), vm((D,), bf16), vm((1, D), bf16), vm((1, FILL), f32),
            vm((4, 128, 128), u32), vm((4, 128, 128), u32), vm((4, 64, 256), u32),
            vm((CT, 8, 8, 128), f32),
            vm((CT, NB, 4, 256, 128), f32), vm((CT, NB - 1, 4, 256, 128), f32),
            vm((CT, 4, 256, 128), f32), vm((CT, NB, 4, 256, 128), f32), vm((4, 128, 128), f32),
            vm((CT, S + 32, 128), f32), vm((8, 8, D), f32),
            vm((CT, S + 32, 128), f32), vm((S + 256, D), f32), vm((S + 256, D), f32),
            vm((S, D), f32),
            vm((288, D), u32), vm((T // 2, D), u32),
            vm((S, D), bf16),
            dma((29,)), dma((NC + 1,)),
        ],
        compiler_params=pltpu.CompilerParams(vmem_limit_bytes=110 << 20, disable_bounds_checks=True,
                                             disable_semaphore_checks=True),
    )(A_q.reshape(S, D), tile_view(A_k), tile_view(A_v), A_shift_k.T, A_ssm_k,
      A_ssm_D, B_w1, B_w2, B_w3.T, B_w4, c, w_mod)
    return out.reshape(1, S, D)
```

```python
import os
import numpy as np
import jax
import jax.numpy as jnp
import jax.experimental.pallas as pl
import jax.experimental.pallas.tpu as pltpu

f32, bf16, u32, i32 = jnp.float32, jnp.bfloat16, jnp.uint32, jnp.int32

S, D, F = 2048, 640, 1728
CT = D // 128
NB, BLK, NFFT = 4, 512, 1024
T = 256
NC = S // T
RSQ = int(os.environ.get('RSQ', '0'))
SAME = int(os.environ.get('SAME', '1'))
LL = int(os.environ.get('LL', '1'))
NS = [int(x) * 128 for x in os.environ.get('NS', '0125')]
R2 = os.environ.get('R2', 'x')
FILL = int(os.environ.get('FILL', '1792'))
VIEW = int(os.environ.get('VIEW', '1'))
CL1 = int(os.environ.get('CL1', '1'))
CLA = int(os.environ.get('CLA', '2'))
R3 = os.environ.get('R3', 'a31t')
G2 = int(os.environ.get('G2', '1'))
NL = int(os.environ.get('NL', '4'))
LBAL = os.environ.get('LBAL', '')
BODY = os.environ.get('BODY', 'nctyp1q2lr')
SKIPCONV = int(os.environ.get('SKIPCONV', '0'))
RELOAD = int(os.environ.get('RELOAD', '1'))
W3S = int(os.environ.get('W3S', '128'))
LAST0 = int(os.environ.get('LAST0', '192'))
FM = (F // 128) * 128
E0 = int(os.environ.get('E0', '0'))
KGRP = [tuple(int(x) for x in g) for g in os.environ.get('KGRP', '0,12,34').split(',')]
TR = 8 * CT
P0, P1, PC = int(os.environ.get('P0', '320')), 528 - int(os.environ.get('P0', '320')), int(os.environ.get('PC', '224'))
PA = S - P0 - P1 - 6 * PC
RG = 16
EPS = 1e-5
NT_DIMS = (((1,), (1,)), ((), ()))
SCOPES = bool(int(os.environ.get("KSCOPES", "0")))


class _NoScope:
    def __enter__(self):
        return self

    def __exit__(self, *a):
        return False


def _scope(name):
    return jax.named_scope(name) if SCOPES else _NoScope()


def _lo(w):
    return pltpu.bitcast(w << 16, f32)


def _hi(w):
    return pltpu.bitcast(w & jnp.uint32(0xFFFF0000), f32)


def _cos_turn(n32, scale):
    x = 2.0 ** 30 - jnp.abs(n32.astype(f32))
    b = 2.0 * np.pi / 2.0 ** 32
    x = x * b
    x2 = x * x
    c = [scale * v for v in (1.0, -1.0 / 6, 1.0 / 120, -1.0 / 5040, 1.0 / 362880)]
    return x * (c[0] + x2 * (c[1] + x2 * (c[2] + x2 * (c[3] + x2 * c[4]))))


def _odd_freq(k):
    return jnp.where(k < 64, 4 * k + 1, 4 * k - 253) << 21


def _slot_phase(idx):
    k = ((idx >> 4) << 3) + (idx & 7)
    return _odd_freq(k), (idx & 8) << 27


def _fwd_table(r):
    fr, off = _slot_phase(jax.lax.broadcasted_iota(i32, (256, 128), 0))
    return pltpu.bitcast(_cos_turn(fr * r + off, 1.0).astype(bf16), u32)


def _inv_table(p):
    row = jax.lax.broadcasted_iota(i32, (128, 256), 0)
    fr, off = _slot_phase(jax.lax.broadcasted_iota(i32, (128, 256), 1))
    return pltpu.bitcast(_cos_turn(fr * (4 * row + p) + off, 2.0 / NFFT).astype(bf16), u32)


def _stats(x, link=None, early=False):
    zero = 0.0 if link is None else jnp.minimum(link, 0.0)
    part = x[:, 0:128]
    for c in range(1, CT):
        part = part + x[:, c * 128:(c + 1) * 128]
    if link is not None and early:
        part = part + zero
        zero = 0.0
    m = jnp.sum(part, axis=-1, keepdims=True) * (1.0 / D)
    v = jnp.maximum(jnp.sum(x * x, axis=-1, keepdims=True) * (1.0 / D) - m * m, zero)
    if RSQ:
        return m, jnp.exp2(jnp.log(v + EPS) * (-0.5 / np.log(2.0)))
    return m, jax.lax.rsqrt(v + EPS)


def _gelu2(x):
    c = 0.7978845608028654
    u = c + (c * 0.044715) * (x * x)
    return x + x * jnp.tanh(x * u)


def _gelu(x):
    c = 0.7978845608028654
    u = c + (c * 0.044715) * (x * x)
    t = jnp.tanh(x * u)
    hx = 0.5 * x
    return hx + hx * t


def _row_parts(m, parts):
    base, extra = divmod(m // 16, parts)
    out, o = [], 0
    for i in range(parts):
        n = 16 * (base + (1 if i < extra else 0))
        out.append((o, n))
        o += n
    return out


def _dot_balanced(x, wslice, n_cols, parts, nt=False):
    def mm(a, c0, c1):
        a = a.astype(bf16)
        if nt:
            return jax.lax.dot_general(a, wslice(c0, c1), NT_DIMS, preferred_element_type=f32)
        return jnp.dot(a, wslice(c0, c1), preferred_element_type=f32)
    if parts == 1:
        return mm(x, 0, n_cols)
    head = mm(x, 0, n_cols - 128)
    last = jnp.concatenate([mm(x[o:o + n], n_cols - 128, n_cols) for o, n in _row_parts(x.shape[0], parts)],
                           axis=0)
    return jnp.concatenate([head, last], axis=-1)


def _radix4(re, im, inverse):
    ar, ai = re[0] + re[2], im[0] + im[2]
    br, bi = re[0] - re[2], im[0] - im[2]
    cr, ci = re[1] + re[3], im[1] + im[3]
    dr, di = re[1] - re[3], im[1] - im[3]
    minus_i = (br + di, bi - dr)
    plus_i = (br - di, bi + dr)
    if inverse:
        return [(ar + cr, ai + ci), plus_i, (ar - cr, ai - ci), minus_i]
    return [(ar + cr, ai + ci), minus_i, (ar - cr, ai - ci), plus_i]


def _kernel(q_hbm, k_hbm, v_hbm, sh_hbm, sk_hbm, d_hbm, w1_hbm, w2_hbm, w3_hbm, w4_hbm,
            c_hbm, wm_hbm, o_hbm,
            kb, vb, skb, qb, w1b, w2b, w3b, w4b, w1p, w2p, w3p, w4p, wmb, shb, db, cb_, fill, fub, fkb, gtb, par,
            US, KS, UR, YS, YP, ys, modb, h1s, h2s, x2s, hss, zt, zb, w3n, ob,
            sem, sem_o):
    def sk_copy(c):
        return pltpu.make_async_copy(sk_hbm.at[pl.ds(c * 128, 128), :], skb.at[c], sem.at[c])

    def kv_copies(a):
        n = BLK * CT
        return [
            pltpu.make_async_copy(k_hbm.at[pl.ds(a * n, n), :], kb.at[pl.ds(TR + a * n, n), :], sem.at[CT + a]),
            pltpu.make_async_copy(v_hbm.at[pl.ds(a * n, n), :], vb.at[pl.ds(a * n, n), :], sem.at[2 * CT + a]),
        ]

    small = [pltpu.make_async_copy(src, dst, sem.at[15 + i]) for i, (src, dst) in enumerate(
        [(d_hbm, db), (sh_hbm, shb), (c_hbm, cb_)])]

    mod_cols = [(0, 3 * D), (3 * D, 2 * D), (5 * D, D)]
    mod_copies = [pltpu.make_async_copy(wm_hbm.at[:, pl.ds(o, n)], wmb.at[:, pl.ds(o, n)], sem.at[18 + i])
                  for i, (o, n) in enumerate(mod_cols)]
    w_pairs = [(w1_hbm, w1b), (w2_hbm, w2b), (w3_hbm, w3b), (w4_hbm, w4b)]
    w_copies = [pltpu.make_async_copy(src, dst, sem.at[21 + i]) for i, (src, dst) in enumerate(w_pairs)]
    PB = P0 + P1 + PA
    q_rows = [(0, P0 + P1), (P0 + P1, PA), (PB, PC), (PB + PC, S - PB - PC)]
    q_copies = [pltpu.make_async_copy(q_hbm.at[pl.ds(o, n), :], qb.at[pl.ds(o, n), :], sem.at[25 + i])
                for i, (o, n) in enumerate(q_rows)]

    def out_copy(i):
        r = i * T if isinstance(i, int) else pl.multiple_of(i * T, T)
        return pltpu.make_async_copy(ob.at[pl.ds(r, T), :], o_hbm.at[pl.ds(r, T), :], sem_o.at[i])

    out_tail = [pltpu.make_async_copy(ob.at[pl.ds(o, n), :], o_hbm.at[pl.ds(o, n), :], sem_o.at[NC - 1 + i])
                for i, (o, n) in enumerate([(S - T, LAST0), (S - T + LAST0, T - LAST0)])]

    for cp in small + kv_copies(0):
        cp.start()
    for c in range(CT):
        sk_copy(c).start()
    for a in range(1, NB):
        for cp in kv_copies(a):
            cp.start()
    order = [mod_copies[0], q_copies[0], mod_copies[1], w_copies[0], w_copies[1], q_copies[1],
             w_copies[2], q_copies[2], w_copies[3], mod_copies[2], q_copies[3]]
    if SAME:
        order = [mod_copies[0], q_copies[0], mod_copies[1], w_copies[0], w_copies[1], q_copies[1],
                 w_copies[2], w_copies[3], mod_copies[2], q_copies[2], q_copies[3]]
    for cp in order:
        cp.start()

    with _scope("init"):
        def pin(i, carry):
            fill[:, pl.ds(pl.multiple_of(i * 128, 128), 128)] = jnp.zeros((1, 128), f32)
            YP[i, 0:8, :] = jnp.zeros((8, 128), f32)
            US[i, 0, 0, 0:8, :] = jnp.zeros((8, 128), f32)
            KS[i, 0, 0, 0:8, :] = jnp.zeros((8, 128), f32)
            YS[i, 0, 0, 0:8, :] = jnp.zeros((8, 128), f32)
            UR[i, 0, 0:8, :] = jnp.zeros((8, 128), f32)
            return carry

        jax.lax.fori_loop(0, 2, pin, 0)
        lane = jax.lax.broadcasted_iota(i32, (256, 128), 1)
        for p in range(4):
            m = (lane - p) & 3
            fkb[p] = _fwd_table(128 * m + ((lane - m) & 127))
        for c in range(CT):
            kb[c * 8:(c + 1) * 8, :] = jnp.zeros((8, 128), bf16)
            h1s[c, 0:8, :] = jnp.zeros((8, 128), f32)
            h1s[c, S + 8:S + 16, :] = jnp.zeros((8, 128), f32)
        for p in range(4):
            fub[p] = _fwd_table(8 * (lane & 63) + ((lane >> 6) << 2) + p)
        for cp in small:
            cp.wait()
        cvec = cb_[...].astype(f32)
        fill[:, 0:D] = cvec * jax.nn.sigmoid(cvec)
        dv = db[...].astype(f32).reshape(1, D)
        shv = shb[...].astype(f32)
        for c in range(CT):
            for i in range(4):
                par[c, i] = jnp.broadcast_to(shv[i:i + 1, c * 128:(c + 1) * 128], (8, 128))
            par[c, 4] = jnp.broadcast_to(dv[:, c * 128:(c + 1) * 128], (8, 128))
    def fence(i, carry):
        YP[i, 0:8, :] = jnp.zeros((8, 128), f32)
        return carry

    kw = kb.bitcast(u32)
    vw = vb.bitcast(u32)

    def re_(g):
        return slice(g * 16, g * 16 + 8)

    def im_(g):
        return slice(g * 16 + 8, g * 16 + 16)

    def fwd_k(c, j):
        if SKIPCONV:
            return
        lane = jax.lax.broadcasted_iota(i32, (64, 128), 1)
        even = (lane & 1) == 0
        l01 = (lane & 2) == 0
        l12 = ((lane + 3) & 2) == 0
        rm = []
        for m in range(4):
            w = pltpu.bitcast(skb[c, :, (4 * j + m) * 128:(4 * j + m + 1) * 128], u32)
            rm.append(pltpu.roll(w, m, 1) if m else w)
        e01 = jnp.where(even, rm[0], rm[1])
        o01 = jnp.where(even, rm[1], rm[0])
        e23 = jnp.where(even, rm[2], rm[3])
        o23 = jnp.where(even, rm[3], rm[2])
        kp = [jnp.where(l01, e01, e23), jnp.where(l12, o01, o23),
              jnp.where(l01, e23, e01), jnp.where(l12, o23, o01)]
        tt = [jax.lax.dot_general(pltpu.bitcast(fkb[p], bf16), pltpu.bitcast(kp[p], bf16), NT_DIMS,
                                  preferred_element_type=f32) for p in range(4)]
        dvec = par[c, 4] if j == 0 else None
        for g in range(16):
            re = [t[re_(g)] for t in tt]
            im = [t[im_(g)] for t in tt]
            if j == 0:
                re[0] = re[0] + dvec
            x = _radix4(re, im, False)
            for m in range(4):
                xr, xi = x[m]
                if j < NB - 1:
                    KS[c, j, m, re_(g), :] = xr
                    KS[c, j, m, im_(g), :] = xi
                ur, ui = US[c, 0, m, re_(g), :], US[c, 0, m, im_(g), :]
                YS[c, j, m, re_(g), :] = xr * ur - xi * ui
                YS[c, j, m, im_(g), :] = xr * ui + xi * ur

    def fwd_u(c, a):
        if SKIPCONV:
            return
        taps = [jnp.tile(par[c, i], (8, 1)) for i in range(4)]
        ws = TR // 2
        base = a * (BLK // 8) * ws + 4 * c

        def words(ref, start):
            return ref[pl.ds(start, BLK // 8, stride=ws), :]

        kk = {}
        for w in range(4):
            x = words(kw, ws + base + w)
            kk[2 * w], kk[2 * w + 1] = _lo(x), _hi(x)
        kk[-3] = _hi(words(kw, base + 2))
        x = words(kw, base + 3)
        kk[-2], kk[-1] = _lo(x), _hi(x)
        sub = []
        for w in range(4):
            x = words(vw, base + w)
            for r, vv in ((2 * w, _lo(x)), (2 * w + 1, _hi(x))):
                sh = taps[0] * kk[r] + taps[1] * kk[r - 1] + taps[2] * kk[r - 2] + taps[3] * kk[r - 3]
                sub.append(sh * vv)
        kv = [jnp.concatenate([sub[p], sub[p + 4]], axis=0) for p in range(4)]
        tt = [jnp.dot(pltpu.bitcast(fub[p], bf16), kv[p].astype(bf16), preferred_element_type=f32)
              for p in range(4)]
        for g in range(16):
            x = _radix4([t[re_(g)] for t in tt], [t[im_(g)] for t in tt], False)
            for m in range(4):
                xr, xi = x[m]
                if a:
                    if a == 1:
                        pr, pi = US[c, 0, m, re_(g), :], US[c, 0, m, im_(g), :]
                    else:
                        pr, pi = UR[c, m, re_(g), :], UR[c, m, im_(g), :]
                    if a < NB - 1:
                        UR[c, m, re_(g), :] = xr
                        UR[c, m, im_(g), :] = xi
                    if g < 8:
                        xr, xi = xr - pi, xi + pr
                    else:
                        xr, xi = xr + pi, xi - pr
                US[c, a, m, re_(g), :] = xr
                US[c, a, m, im_(g), :] = xi

    def mac_inv(c, a, halves=(0, 1)):
        if SKIPCONV:
            return
        for h in halves:
            words = [[] for _ in range(4)]
            for g in range(8 * h, 8 * h + 8):
                yre, yim = [], []
                for m in range(4):
                    yr, yi = YS[c, a, m, re_(g), :], YS[c, a, m, im_(g), :]
                    for j in range(a):
                        kr, ki = KS[c, j, m, re_(g), :], KS[c, j, m, im_(g), :]
                        ur, ui = US[c, a - j, m, re_(g), :], US[c, a - j, m, im_(g), :]
                        yr = yr + (kr * ur - ki * ui)
                        yi = yi + (kr * ui + ki * ur)
                    yre.append(yr)
                    yim.append(yi)
                pp = _radix4(yre, yim, True)
                for p in range(4):
                    words[p].extend(pp[p])
            for p in range(4):
                pb = jnp.concatenate(words[p], axis=0).astype(bf16)
                r = jnp.dot(pltpu.bitcast(gtb[p, :, h * 128:(h + 1) * 128], bf16), pb,
                            preferred_element_type=f32)
                if h == 0:
                    YP[p] = r
                else:
                    ys[c, pl.ds(a * BLK + p, 128, stride=4), :] = YP[p] + r

    desc = (3, 2, 1, 0)
    def k_tile(c):
        for j in desc:
            fwd_k(c, j)

    with _scope("conv_u0"):
        for p in range(4):
            gtb[p] = _inv_table(p)
        with _scope("w_kv"):
            for cp in kv_copies(0):
                cp.wait()
        for c in range(CT):
            fwd_u(c, 0)
    with _scope("conv_k"):
        done = 0
        for grp in KGRP:
            with _scope("w_sk"):
                for c in grp:
                    sk_copy(c).wait()
            for c in grp:
                k_tile(c)
            if grp is KGRP[-1]:
                for c in range(E0):
                    mac_inv(c, 0)
    for a in range(1, NB):
        with _scope("conv_u%d" % a):
            with _scope("w_kv"):
                for cp in kv_copies(a):
                    cp.wait()
            todo = [(c, a - 1) for c in range(CT)]
            if a == 1:
                todo = todo[E0:]
            late = len(todo) < CT
            for c in range(CT):
                fwd_u(c, a)
                if todo and (not late or c >= CT - len(todo)):
                    mac_inv(*todo.pop(0))

    def mod_cols_dot(o, n, extra):
        act = fill[:, 0:D]

        def sc(k0, k1):
            return jnp.broadcast_to(act[:, k0:k1], (16, k1 - k0)).astype(bf16)

        e = 128 * extra
        r = jnp.dot(sc(0, D), wmb[:, o + e:o + n], preferred_element_type=f32)
        if extra:
            r0 = (jnp.dot(sc(0, D - 64), wmb[0:D - 64, o:o + e], preferred_element_type=f32)
                  + jnp.dot(sc(D - 64, D), wmb[D - 64:D, o:o + e], preferred_element_type=f32))
            r = jnp.concatenate([r0, r], axis=-1)
        return r[0:8]

    def mod_part(part, extra):
        o, n = mod_cols[part]
        r = mod_cols_dot(o, n, extra)
        return [r[:, i * D:(i + 1) * D] for i in range(n // D)]

    def mvec(i, n=RG, c0=0, c1=D):
        return jnp.tile(modb[i, :, c0:c1], (n // 8, 1))

    def rows(r, n):
        return pl.ds(r, n)

    def load_q(r, ref=qb):
        return ref[rows(r, RG), :].astype(f32)

    def make_x2(r, q, st, ref=ys):
        y = jnp.concatenate([ref[c, rows(r, RG), :] for c in range(CT)], axis=-1)
        return q + (((q - st[0]) * st[1]) * mvec(1) + mvec(0)) * y

    def make_h2(x2, st):
        return ((x2 - st[0]) * st[1]) * mvec(3) + mvec(2)

    def pack_ln(x, st):
        return pltpu.bitcast(((x - st[0]) * st[1]).astype(bf16), u32)

    def a_chain(r_in, r_out, n=PC, links=1):
        qv, yv = qb.at[rows(r_in, n), :], ys.at[:, rows(r_in, n), :]
        xv, hv = x2s.at[rows(r_out, n), :], h2s.at[rows(r_out, n), :]
        prevs = [None] * links
        for g, o in enumerate(range(0, n, RG)):
            q = load_q(o, qv)
            x2 = make_x2(o, q, _stats(q, prevs[g % links]), yv)
            xv[o:o + RG, :] = x2
            st = _stats(x2)
            h2 = make_h2(xv[o:o + RG, :], st)
            hv[o:o + RG, :] = h2
            st = _stats(h2)
            zt[o // 2:(o + RG) // 2, :] = pack_ln(hv[o:o + RG, :], st)
            prevs[g % links] = st[1]

    def mm_w1(r, n, o=0, bal=True):
        z = pltpu.bitcast(zt[o // 2:(o + n) // 2, :], bf16)
        h1 = _gelu(_dot_balanced(z, lambda a, b: pltpu.bitcast(w1p[:, a:b], bf16), D, 4 if bal else 1))
        for c in range(CT):
            h1s[c, rows(r + 8, n), :] = h1[:, c * 128:(c + 1) * 128]

    def mm_w2a(r, bal=True):
        lane = jax.lax.broadcasted_iota(i32, (T, 128), 1)

        def sh(k, c):
            return h1s[c, rows(r + 8 + k, T), :]

        g = jnp.concatenate([
            sh(-1, 0),
            jnp.where(lane < 32, sh(-1, 1), sh(1, 1)),
            jnp.where(lane < 64, sh(1, 2), sh(-2, 2)),
            jnp.where(lane < 96, sh(-2, 3), sh(2, 3)),
            sh(2, 4)], axis=-1)
        hss[rows(r, T), :] = _dot_balanced(g, lambda a, b: pltpu.bitcast(w2p[:, a:b], bf16), D, 4 if bal else 1)

    def mm_w2b(r, links=1):
        hv, sv = h2s.at[rows(r, T), :], hss.at[rows(r, T), :]
        prev = [None] * links
        for n, o in enumerate(range(0, T, RG)):
            x1 = hv[o:o + RG, :] + sv[o:o + RG, :]
            st = _stats(x1, prev[n % links], early=True)
            zb[o // 2:(o + RG) // 2, :] = pack_ln(x1, st)
            prev[n % links] = st[1]

    def mm_w3_main(bal=True):
        z = pltpu.bitcast(zb[...], bf16)
        return (_gelu2 if G2 else _gelu)(_dot_balanced(z, lambda a, b: pltpu.bitcast(w3p[a // 2:b // 2, :], bf16), FM, 4 if bal else 1, nt=True))

    def mm_w3_cols(a, b):
        z = pltpu.bitcast(zb[...], bf16)
        w = pltpu.bitcast(w3p[a // 2:b // 2, :], bf16)
        return _gelu2(jax.lax.dot_general(z, w, NT_DIMS, preferred_element_type=f32))

    def mm_w3_first():
        z = pltpu.bitcast(zb[...], bf16)
        return _gelu2(jnp.dot(z, pltpu.bitcast(w3n[...], bf16), preferred_element_type=f32))

    def mm_w3_tail():
        z = pltpu.bitcast(zb[...], bf16)
        return (_gelu2 if G2 else _gelu)(jax.lax.dot_general(pltpu.bitcast(w3p[FM // 2:F // 2, :], bf16), z, NT_DIMS, preferred_element_type=f32))

    def join_act(main, tail):
        return jnp.concatenate([main, tail.T], axis=-1)

    def mm_w3(bal):
        tail = mm_w3_tail()
        return join_act(mm_w3_main(bal), tail)

    def mm_w4(r, a, o=0, n=T, bal=True):
        h2 = _dot_balanced(a[o:o + n], lambda c0, c1: pltpu.bitcast(w4p[:, c0:c1], bf16), D, 2 if bal else 1)
        ob[rows(r + o, n), :] = (x2s[rows(r + o, n), :]
                                 + mvec(4, n) * ((h2s[rows(r + o, n), :] + hss[rows(r + o, n), :]) + (0.5 * h2 if G2 else h2))).astype(bf16)

    def mm_w4_cols(r, a, c0, c1):
        h2 = jnp.dot(a, pltpu.bitcast(w4p[:, c0:c1], bf16), preferred_element_type=f32)
        ob[rows(r, T), c0:c1] = (x2s[rows(r, T), c0:c1] + mvec(4, T, c0, c1) * (
            (h2s[rows(r, T), c0:c1] + hss[rows(r, T), c0:c1]) + 0.5 * h2)).astype(bf16)

    groups = list(range(0, P0 + P1, RG))
    with _scope("conv_last"):
        jax.lax.fori_loop(0, 2, fence, 0)
        for c in range(NL):
            mac_inv(c, NB - 1)
    with _scope("pre_a"):
        with _scope("w_q0"):
            mod_copies[0].wait()
            q_copies[0].wait()
        sa, ca, ga = mod_part(0, 1)
        modb[0] = ga * sa
        modb[1] = ga * (1.0 + ca)
        for c in range(NL, CT):
            mac_inv(c, NB - 1)
        st1 = {o: _stats(load_q(o)) for o in groups}
        zt[0:8, 0:128] = jnp.zeros((8, 128), u32)
        st2 = {}
        for o in groups:
            x2 = make_x2(o, load_q(o), st1[o])
            x2s[o:o + RG, :] = x2
            st2[o] = _stats(x2)

    def pass_c(os_, links):
        st3 = {}
        prev = [None] * max(links, 1)
        for n, o in enumerate(os_):
            h2 = make_h2(x2s[o:o + RG, :], st2[o])
            h2s[o:o + RG, :] = h2
            st3[o] = _stats(h2, prev[n % len(prev)], early=True)
            if links:
                prev[n % links] = st3[o][1]
                zt[o // 2:(o + RG) // 2, :] = pack_ln(h2, st3[o])
        if not links:
            for o in os_:
                zt[o // 2:(o + RG) // 2, :] = pack_ln(h2s[o:o + RG, :], st3[o])

    with _scope("pre_b"):
        with _scope("w_modB"):
            mod_copies[1].wait()
        sb, cb = mod_part(1, 2)
        modb[2] = sb
        modb[3] = 1.0 + cb
        pass_c([o for o in groups if o < P0], 0)
    with _scope("r1"):
        with _scope("w_w1"):
            w_copies[0].wait()
        w1p[...] = pltpu.bitcast(w1b[...], u32)
        mm_w1(0, P0)
        pass_c([o for o in groups if o >= P0], CL1)
        mm_w1(P0, P1, P0)
    with _scope("r2"):
        with _scope("w_w2"):
            w_copies[1].wait()
            q_copies[1].wait()
        w2p[...] = pltpu.bitcast(w2b[...], u32)
        if 'c' in R2:
            a_chain(P0 + P1, P0 + P1, PA, CLA)
        mm_w2a(0)
        mm_w2b(0, 2)
        mm_w2a(T)
    with _scope("r3"):
        with _scope("w_w3"):
            w_copies[2].wait()
            if not SAME:
                q_copies[2].wait()
        w3p[...] = pltpu.bitcast(w3b[...], u32)
        for tok in R3:
            if tok == '1':
                mm_w1(P0 + P1, PA)
            elif tok == 'c':
                a_chain(PB, PB)
            elif tok == 'a':
                a_chain(P0 + P1, P0 + P1, PA)
            elif tok == '3':
                main = mm_w3_main()
            else:
                tail = mm_w3_tail()
    with _scope("r4"):
        with _scope("w_w4"):
            w_copies[3].wait()
            mod_copies[2].wait()
        w4p[...] = pltpu.bitcast(w4b[...], u32)
        modb[4] = mod_part(2, 1)[0]
        w3n[...] = pltpu.bitcast(w3b[0:128, :].astype(f32).T.astype(bf16), u32)
        mm_w4(0, join_act(main, tail))
        mm_w2b(T)
        out_copy(0).start()
        q_copies[3].wait()
        if SAME:
            q_copies[2].wait()

    def mlp_iter(i):
        r1 = pl.multiple_of(PB - PC + PC * i, 16)
        r = pl.multiple_of(i * T, T)
        mains = []
        for tok in BODY:
            if tok == 't':
                tail = mm_w3_tail()
            elif tok == '1':
                mm_w1(r1, PC, bal='1' in LBAL)
            elif tok == 'c':
                if SAME:
                    a_chain(r1, r1)
                else:
                    a_chain(pl.multiple_of(jnp.minimum(r1 + PC, S - PC), 16), r1 + PC)
            elif tok in 'pqr':
                if tok == 'p':
                    act = join_act(jnp.concatenate(mains, axis=-1), tail).astype(bf16)
                k = 'pqr'.index(tok)
                mm_w4_cols(r, act, NS[k], NS[k + 1])
            elif tok == '3':
                mains.append(mm_w3_main('3' in LBAL))
            elif tok == 'n':
                mains.append(mm_w3_first())
            elif tok == 'w':
                mains.append(mm_w3_cols(128, W3S))
            elif tok == 'x':
                mains.append(mm_w3_cols(0, W3S))
            elif tok == 'y':
                mains.append(mm_w3_cols(W3S, FM))
            elif tok == '2':
                mm_w2a(r + T, bal='2' in LBAL)
            elif tok == 'l':
                mm_w2b(r + T, LL)
            elif tok == '4':
                mm_w4(r, join_act(jnp.concatenate(mains, axis=-1), tail), bal='4' in LBAL)
        out_copy(i).start()

    def mlp_body(i, carry):
        with _scope("iter"):
            mlp_iter(i)
        return carry

    with _scope("loop"):
        jax.lax.fori_loop(1, NC - 1, mlp_body, 0)
    with _scope("last"):
        first = mm_w3_first()
        tail = mm_w3_tail()
        act = join_act(jnp.concatenate([first, mm_w3_cols(128, FM)], axis=-1), tail)
        mm_w4(S - T, act, 0, LAST0, bal=False)
        out_tail[0].start()
        mm_w4(S - T, act, LAST0, T - LAST0, bal=False)
        out_tail[1].start()
    with _scope("fin"):
        for i in range(NC - 1):
            out_copy(i).wait()
        for cp in out_tail:
            cp.wait()


@jax.jit
def pallas_adaLN_cond__ssm_conv_h3__mixer_s_mlp__prompt_kernel(
    A_q: jax.Array,
    A_k: jax.Array,
    A_v: jax.Array,
    A_shift_k: jax.Array,
    A_ssm_k: jax.Array,
    A_ssm_D: jax.Array,
    B_x: jax.Array,
    B_w1: jax.Array,
    B_w2: jax.Array,
    B_w3: jax.Array,
    B_w4: jax.Array,
    c: jax.Array,
    w_mod: jax.Array,
):
    del B_x
    any_spec = pl.BlockSpec(memory_space=pl.ANY)

    def tile_view(x):
        return x.reshape(S // 8, 8, CT, 128).transpose(0, 2, 1, 3).reshape(S * CT, 128)

    vm = pltpu.VMEM
    dma = pltpu.SemaphoreType.DMA
    out = pl.pallas_call(
        _kernel,
        in_specs=[any_spec] * 12,
        out_specs=any_spec,
        out_shape=jax.ShapeDtypeStruct((S, D), bf16),
        scratch_shapes=[
            vm((S * CT + 128, 128), bf16), vm((S * CT + 64, 128), bf16), vm((CT, 128, S), bf16),
            vm((S, D), bf16), vm((D, D), bf16), vm((D, D), bf16), vm((F, D), bf16), vm((F, D), bf16),
            vm((D // 2, D), u32), vm((D // 2, D), u32), vm((F // 2, D), u32), vm((F // 2, D), u32),
            vm((D, 6 * D), bf16), vm((4, D), bf16), vm((D,), bf16), vm((1, D), bf16), vm((1, FILL), f32),
            vm((4, 128, 128), u32), vm((4, 128, 128), u32), vm((4, 64, 256), u32),
            vm((CT, 8, 8, 128), f32),
            vm((CT, NB, 4, 256, 128), f32), vm((CT, NB - 1, 4, 256, 128), f32),
            vm((CT, 4, 256, 128), f32), vm((CT, NB, 4, 256, 128), f32), vm((4, 128, 128), f32),
            vm((CT, S + 32, 128), f32), vm((8, 8, D), f32),
            vm((CT, S + 32, 128), f32), vm((S + 256, D), f32), vm((S + 256, D), f32),
            vm((S, D), f32),
            vm((288, D), u32), vm((T // 2, D), u32), vm((D // 2, 128), u32),
            vm((S, D), bf16),
            dma((29,)), dma((NC + 1,)),
        ],
        compiler_params=pltpu.CompilerParams(vmem_limit_bytes=110 << 20, disable_bounds_checks=True,
                                             disable_semaphore_checks=True),
    )(A_q.reshape(S, D), tile_view(A_k), tile_view(A_v), A_shift_k.T, A_ssm_k,
      A_ssm_D, B_w1, B_w2, B_w3.T, B_w4, c, w_mod)
    return out.reshape(1, S, D)
```

```python
import os
import numpy as np
import jax
import jax.numpy as jnp
import jax.experimental.pallas as pl
import jax.experimental.pallas.tpu as pltpu

f32, bf16, u32, i32 = jnp.float32, jnp.bfloat16, jnp.uint32, jnp.int32

S, D, F = 2048, 640, 1728
CT = D // 128
TR = 8 * CT
NB, BLK, NFFT = 4, 512, 1024
NG = 16
T = 256
NC = S // T
FM = (F // 128) * 128
P0, P1, PA, PC = 320, 208, 176, 224
PB = P0 + P1 + PA
LAST0 = 192
RG = 16
EPS = 1e-5
NT_DIMS = (((1,), (1,)), ((), ()))
GVF = int(os.environ.get("GVF", "8"))
GVI = int(os.environ.get("GVI", "8"))
NL = int(os.environ.get("NL", "4"))
SKIPCONV = int(os.environ.get("SKIPCONV", "0"))
SCOPES = bool(int(os.environ.get("KSCOPES", "0")))


class _NoScope:
    def __enter__(self):
        return self

    def __exit__(self, *a):
        return False


def _scope(name):
    return jax.named_scope(name) if SCOPES else _NoScope()


def _lo(w):
    return pltpu.bitcast(w << 16, f32)


def _hi(w):
    return pltpu.bitcast(w & jnp.uint32(0xFFFF0000), f32)


def _cos_turn(n32, scale):
    x = (2.0 ** 30 - jnp.abs(n32.astype(f32))) * (2.0 * np.pi / 2.0 ** 32)
    x2 = x * x
    c = [scale * v for v in (1.0, -1.0 / 6, 1.0 / 120, -1.0 / 5040, 1.0 / 362880)]
    return x * (c[0] + x2 * (c[1] + x2 * (c[2] + x2 * (c[3] + x2 * c[4]))))


def _slot_phase(idx):
    k = ((idx >> 4) << 3) + (idx & 7)
    return jnp.where(k < 64, 4 * k + 1, 4 * k - 253) << 21, (idx & 8) << 27


def _fwd_table(r):
    fr, off = _slot_phase(jax.lax.broadcasted_iota(i32, (256, 128), 0))
    return pltpu.bitcast(_cos_turn(fr * r + off, 1.0).astype(bf16), u32)


def _inv_table(p):
    row = jax.lax.broadcasted_iota(i32, (128, 256), 0)
    fr, off = _slot_phase(jax.lax.broadcasted_iota(i32, (128, 256), 1))
    return pltpu.bitcast(_cos_turn(fr * (4 * row + p) + off, 2.0 / NFFT).astype(bf16), u32)


def _radix4(re, im, inverse):
    ar, ai = re[0] + re[2], im[0] + im[2]
    br, bi = re[0] - re[2], im[0] - im[2]
    cr, ci = re[1] + re[3], im[1] + im[3]
    dr, di = re[1] - re[3], im[1] - im[3]
    minus_i = (br + di, bi - dr)
    plus_i = (br - di, bi + dr)
    if inverse:
        return [(ar + cr, ai + ci), plus_i, (ar - cr, ai - ci), minus_i]
    return [(ar + cr, ai + ci), minus_i, (ar - cr, ai - ci), plus_i]


def _stats(x, link=None, early=False):
    zero = 0.0 if link is None else jnp.minimum(link, 0.0)
    part = x[:, 0:128]
    for c in range(1, CT):
        part = part + x[:, c * 128:(c + 1) * 128]
    if link is not None and early:
        part = part + zero
        zero = 0.0
    m = jnp.sum(part, axis=-1, keepdims=True) * (1.0 / D)
    v = jnp.maximum(jnp.sum(x * x, axis=-1, keepdims=True) * (1.0 / D) - m * m, zero)
    return m, jax.lax.rsqrt(v + EPS)


def _gelu2(x):
    c = 0.7978845608028654
    u = c + (c * 0.044715) * (x * x)
    return x + x * jnp.tanh(x * u)


def _gelu(x):
    c = 0.7978845608028654
    u = c + (c * 0.044715) * (x * x)
    hx = 0.5 * x
    return hx + hx * jnp.tanh(x * u)


def _dot_balanced(x, wslice, n_cols, parts, nt=False):
    def mm(a, c0, c1):
        a, w = a.astype(bf16), pltpu.bitcast(wslice(c0, c1), bf16)
        if nt:
            return jax.lax.dot_general(a, w, NT_DIMS, preferred_element_type=f32)
        return jnp.dot(a, w, preferred_element_type=f32)

    if parts == 1:
        return mm(x, 0, n_cols)
    base, extra = divmod(x.shape[0] // 16, parts)
    last, o = [], 0
    head = mm(x, 0, n_cols - 128)
    for i in range(parts):
        n = 16 * (base + (1 if i < extra else 0))
        last.append(mm(x[o:o + n], n_cols - 128, n_cols))
        o += n
    return jnp.concatenate([head, jnp.concatenate(last, axis=0)], axis=-1)


def _kernel(q_hbm, k_hbm, v_hbm, sh_hbm, sk_hbm, d_hbm, w1_hbm, w2_hbm, w3_hbm, w4_hbm,
            c_hbm, wm_hbm, o_hbm,
            kb, vb, skb, qb, w1b, w2b, w3b, w4b, w1p, w2p, w3p, w4p, wmb, shb, db, cb_, scb,
            fub, fkb, gtb, par, US, KS, UR, YS, YP, ys, modb, h1s, h2s, x2s, hss, zt, zb, w3n, ob,
            sem, sem_o):
    n_in = [0]

    def load(src, dst):
        n_in[0] += 1
        return pltpu.make_async_copy(src, dst, sem.at[n_in[0] - 1])

    nkv = BLK * CT
    small = [load(d_hbm, db), load(sh_hbm, shb), load(c_hbm, cb_)]
    sk_copies = [load(sk_hbm.at[pl.ds(c * 128, 128), :], skb.at[c]) for c in range(CT)]
    kv_copies = [[load(k_hbm.at[pl.ds(a * nkv, nkv), :], kb.at[pl.ds(TR + a * nkv, nkv), :]),
                  load(v_hbm.at[pl.ds(a * nkv, nkv), :], vb.at[pl.ds(a * nkv, nkv), :])] for a in range(NB)]
    mod_cols = [(0, 3 * D), (3 * D, 2 * D), (5 * D, D)]
    mod_copies = [load(wm_hbm.at[:, pl.ds(o, n)], wmb.at[:, pl.ds(o, n)]) for o, n in mod_cols]
    w_copies = [load(w1_hbm, w1b), load(w2_hbm, w2b), load(w3_hbm, w3b), load(w4_hbm, w4b)]
    q_copies = [load(q_hbm.at[pl.ds(o, n), :], qb.at[pl.ds(o, n), :])
                for o, n in [(0, P0 + P1), (P0 + P1, PA), (PB, S - PB)]]

    def out_copy(i):
        r = i * T if isinstance(i, int) else pl.multiple_of(i * T, T)
        return pltpu.make_async_copy(ob.at[pl.ds(r, T), :], o_hbm.at[pl.ds(r, T), :], sem_o.at[i])

    out_tail = [pltpu.make_async_copy(ob.at[pl.ds(o, n), :], o_hbm.at[pl.ds(o, n), :], sem_o.at[NC - 1 + i])
                for i, (o, n) in enumerate([(S - T, LAST0), (S - T + LAST0, T - LAST0)])]

    for cp in (small + kv_copies[0] + sk_copies + kv_copies[1] + kv_copies[2] + kv_copies[3]
               + [mod_copies[0], q_copies[0], mod_copies[1], w_copies[0], w_copies[1], q_copies[1],
                  w_copies[2], w_copies[3], mod_copies[2], q_copies[2]]):
        cp.start()

    def wait(name, copies):
        with _scope(name):
            for cp in copies:
                cp.wait()

    def pin(i, carry):
        z = jnp.zeros((8, 128), f32)
        scb[:, pl.ds(pl.multiple_of(i * 128, 128), 128)] = z[0:1]
        YP[i, 0:8, :] = z
        US[i, 0, 0, 0, 0:8, :] = z
        KS[i, 0, 0, 0, 0:8, :] = z
        YS[i, 0, 0, 0, 0:8, :] = z
        UR[i, 0, 0, 0:8, :] = z
        return carry

    def fence(i, carry):
        YP[i, 0:8, :] = jnp.zeros((8, 128), f32)
        return carry

    with _scope("init"):
        jax.lax.fori_loop(0, 2, pin, 0)
        lane = jax.lax.broadcasted_iota(i32, (256, 128), 1)
        for p in range(4):
            m = (lane - p) & 3
            fkb[p] = _fwd_table(128 * m + ((lane - m) & 127))
        for c in range(CT):
            kb[c * 8:(c + 1) * 8, :] = jnp.zeros((8, 128), bf16)
            h1s[c, 0:8, :] = jnp.zeros((8, 128), f32)
            h1s[c, S + 8:S + 16, :] = jnp.zeros((8, 128), f32)
        for p in range(4):
            fub[p] = _fwd_table(8 * (lane & 63) + ((lane >> 6) << 2) + p)
        wait("w_small", small)
        cvec = cb_[...].astype(f32)
        scb[:, 0:D] = cvec * jax.nn.sigmoid(cvec)
        dv = db[...].astype(f32).reshape(1, D)
        shv = shb[...].astype(f32)
        for c in range(CT):
            for i in range(4):
                par[c, i] = jnp.broadcast_to(shv[i:i + 1, c * 128:(c + 1) * 128], (8, 128))
            par[c, 4] = jnp.broadcast_to(dv[:, c * 128:(c + 1) * 128], (8, 128))
        for p in range(4):
            gtb[p] = _inv_table(p)

    kw = kb.bitcast(u32)
    vw = vb.bitcast(u32)

    def get(ref, idx, g, n):
        return (ref[idx + (slice(g, g + n), slice(0, 8))], ref[idx + (slice(g, g + n), slice(8, 16))])

    def put(ref, idx, g, n, xr, xi):
        ref[idx + (slice(g, g + n), slice(0, 8))] = xr
        ref[idx + (slice(g, g + n), slice(8, 16))] = xi

    def split(tt, g, n):
        tt = [t[g * 16:(g + n) * 16].reshape(n, 16, 128) for t in tt]
        return [t[:, 0:8] for t in tt], [t[:, 8:16] for t in tt]

    def fwd_k(c, j):
        if SKIPCONV:
            return
        lane = jax.lax.broadcasted_iota(i32, (64, 128), 1)
        even = (lane & 1) == 0
        l01 = (lane & 2) == 0
        l12 = ((lane + 3) & 2) == 0
        rm = []
        for m in range(4):
            w = pltpu.bitcast(skb[c, :, (4 * j + m) * 128:(4 * j + m + 1) * 128], u32)
            rm.append(pltpu.roll(w, m, 1) if m else w)
        e01 = jnp.where(even, rm[0], rm[1])
        o01 = jnp.where(even, rm[1], rm[0])
        e23 = jnp.where(even, rm[2], rm[3])
        o23 = jnp.where(even, rm[3], rm[2])
        kp = [jnp.where(l01, e01, e23), jnp.where(l12, o01, o23),
              jnp.where(l01, e23, e01), jnp.where(l12, o23, o01)]
        tt = [jax.lax.dot_general(pltpu.bitcast(fkb[p], bf16), pltpu.bitcast(kp[p], bf16), NT_DIMS,
                                  preferred_element_type=f32) for p in range(4)]
        for g in range(0, NG, GVF):
            re, im = split(tt, g, GVF)
            if j == 0:
                re[0] = re[0] + par[c, 4][None]
            for m, (xr, xi) in enumerate(_radix4(re, im, False)):
                if j < NB - 1:
                    put(KS, (c, j, m), g, GVF, xr, xi)
                ur, ui = get(US, (c, 0, m), g, GVF)
                put(YS, (c, j, m), g, GVF, xr * ur - xi * ui, xr * ui + xi * ur)

    def fwd_u(c, a):
        if SKIPCONV:
            return
        taps = [jnp.tile(par[c, i], (8, 1)) for i in range(4)]
        ws = TR // 2
        base = a * (BLK // 8) * ws + 4 * c

        def words(ref, start):
            return ref[pl.ds(start, BLK // 8, stride=ws), :]

        kk = {}
        for w in range(4):
            x = words(kw, ws + base + w)
            kk[2 * w], kk[2 * w + 1] = _lo(x), _hi(x)
        kk[-3] = _hi(words(kw, base + 2))
        x = words(kw, base + 3)
        kk[-2], kk[-1] = _lo(x), _hi(x)
        sub = []
        for w in range(4):
            x = words(vw, base + w)
            for r, vv in ((2 * w, _lo(x)), (2 * w + 1, _hi(x))):
                sh = taps[0] * kk[r] + taps[1] * kk[r - 1] + taps[2] * kk[r - 2] + taps[3] * kk[r - 3]
                sub.append(sh * vv)
        kv = [jnp.concatenate([sub[p], sub[p + 4]], axis=0) for p in range(4)]
        tt = [jnp.dot(pltpu.bitcast(fub[p], bf16), kv[p].astype(bf16), preferred_element_type=f32)
              for p in range(4)]
        for g in range(0, NG, GVF):
            re, im = split(tt, g, GVF)
            for m, (xr, xi) in enumerate(_radix4(re, im, False)):
                if a:
                    pr, pi = get(US, (c, 0, m), g, GVF) if a == 1 else get(UR, (c, m), g, GVF)
                    if a < NB - 1:
                        put(UR, (c, m), g, GVF, xr, xi)
                    xr, xi = (xr - pi, xi + pr) if g < NG // 2 else (xr + pi, xi - pr)
                put(US, (c, a, m), g, GVF, xr, xi)

    def mac_inv(c, a):
        if SKIPCONV:
            return
        for h in range(2):
            vals = [[] for _ in range(4)]
            for g in range(8 * h, 8 * h + 8, GVI):
                yre, yim = [], []
                for m in range(4):
                    yr, yi = get(YS, (c, a, m), g, GVI)
                    for j in range(a):
                        kr, ki = get(KS, (c, j, m), g, GVI)
                        ur, ui = get(US, (c, a - j, m), g, GVI)
                        yr = yr + (kr * ur - ki * ui)
                        yi = yi + (kr * ui + ki * ur)
                    yre.append(yr)
                    yim.append(yi)
                for p, (pr, pi) in enumerate(_radix4(yre, yim, True)):
                    vals[p].append(jnp.concatenate([pr, pi], axis=1))
            for p in range(4):
                pb = jnp.concatenate(vals[p], axis=0).reshape(128, 128).astype(bf16)
                r = jnp.dot(pltpu.bitcast(gtb[p, :, h * 128:(h + 1) * 128], bf16), pb,
                            preferred_element_type=f32)
                if h == 0:
                    YP[p] = r
                else:
                    ys[c, pl.ds(a * BLK + p, 128, stride=4), :] = YP[p] + r

    with _scope("conv_u0"):
        wait("w_kv", kv_copies[0])
        for c in range(CT):
            fwd_u(c, 0)
    with _scope("conv_k"):
        for grp in ((0,), (1, 2), (3, 4)):
            wait("w_sk", [sk_copies[c] for c in grp])
            for c in grp:
                for j in (3, 2, 1, 0):
                    fwd_k(c, j)
    for a in range(1, NB):
        with _scope("conv_u%d" % a):
            wait("w_kv", kv_copies[a])
            for c in range(CT):
                fwd_u(c, a)
                mac_inv(c, a - 1)
    with _scope("conv_last"):
        jax.lax.fori_loop(0, 2, fence, 0)
        for c in range(NL):
            mac_inv(c, NB - 1)

    def mod_part(part, extra):
        o, n = mod_cols[part]
        act = scb[:, 0:D]

        def sc(k0, k1):
            return jnp.broadcast_to(act[:, k0:k1], (16, k1 - k0)).astype(bf16)

        e = 128 * extra
        r = jnp.dot(sc(0, D), wmb[:, o + e:o + n], preferred_element_type=f32)
        r0 = (jnp.dot(sc(0, D - 64), wmb[0:D - 64, o:o + e], preferred_element_type=f32)
              + jnp.dot(sc(D - 64, D), wmb[D - 64:D, o:o + e], preferred_element_type=f32))
        r = jnp.concatenate([r0, r], axis=-1)[0:8]
        return [r[:, i * D:(i + 1) * D] for i in range(n // D)]

    def mvec(i, n=RG, c0=0, c1=D):
        return jnp.tile(modb[i, :, c0:c1], (n // 8, 1))

    rows = pl.ds

    def load_q(r, ref=qb):
        return ref[rows(r, RG), :].astype(f32)

    def make_x2(r, q, st, ref=ys):
        y = jnp.concatenate([ref[c, rows(r, RG), :] for c in range(CT)], axis=-1)
        return q + (((q - st[0]) * st[1]) * mvec(1) + mvec(0)) * y

    def make_h2(x2, st):
        return ((x2 - st[0]) * st[1]) * mvec(3) + mvec(2)

    def pack_ln(x, st):
        return pltpu.bitcast(((x - st[0]) * st[1]).astype(bf16), u32)

    def ln_chain(r, n):
        qv, yv = qb.at[rows(r, n), :], ys.at[:, rows(r, n), :]
        xv, hv = x2s.at[rows(r, n), :], h2s.at[rows(r, n), :]
        prev = None
        for o in range(0, n, RG):
            q = load_q(o, qv)
            x2 = make_x2(o, q, _stats(q, prev), yv)
            xv[o:o + RG, :] = x2
            st = _stats(x2)
            h2 = make_h2(xv[o:o + RG, :], st)
            hv[o:o + RG, :] = h2
            st = _stats(h2)
            zt[o // 2:(o + RG) // 2, :] = pack_ln(hv[o:o + RG, :], st)
            prev = st[1]

    def mm_w1(r, n, o=0, parts=4):
        z = pltpu.bitcast(zt[o // 2:(o + n) // 2, :], bf16)
        h1 = _gelu(_dot_balanced(z, lambda a, b: w1p[:, a:b], D, parts))
        for c in range(CT):
            h1s[c, rows(r + 8, n), :] = h1[:, c * 128:(c + 1) * 128]

    def mm_w2(r, parts=4):
        lane = jax.lax.broadcasted_iota(i32, (T, 128), 1)

        def sh(k, c):
            return h1s[c, rows(r + 8 + k, T), :]

        g = jnp.concatenate([
            sh(-1, 0),
            jnp.where(lane < 32, sh(-1, 1), sh(1, 1)),
            jnp.where(lane < 64, sh(1, 2), sh(-2, 2)),
            jnp.where(lane < 96, sh(-2, 3), sh(2, 3)),
            sh(2, 4)], axis=-1)
        hss[rows(r, T), :] = _dot_balanced(g, lambda a, b: w2p[:, a:b], D, parts)

    def ln_x1(r, links=1):
        hv, sv = h2s.at[rows(r, T), :], hss.at[rows(r, T), :]
        prev = [None] * links
        for n, o in enumerate(range(0, T, RG)):
            x1 = hv[o:o + RG, :] + sv[o:o + RG, :]
            st = _stats(x1, prev[n % links], early=True)
            zb[o // 2:(o + RG) // 2, :] = pack_ln(x1, st)
            prev[n % links] = st[1]

    def mm_w3(f0, parts=1):
        z = pltpu.bitcast(zb[...], bf16)
        return _gelu2(_dot_balanced(z, lambda a, b: w3p[(f0 + a) // 2:(f0 + b) // 2, :], FM - f0, parts, nt=True))

    def mm_w3_first():
        z = pltpu.bitcast(zb[...], bf16)
        return _gelu2(jnp.dot(z, pltpu.bitcast(w3n[...], bf16), preferred_element_type=f32))

    def mm_w3_tail():
        z = pltpu.bitcast(zb[...], bf16)
        w = pltpu.bitcast(w3p[FM // 2:F // 2, :], bf16)
        return _gelu2(jax.lax.dot_general(w, z, NT_DIMS, preferred_element_type=f32))

    def mm_w4(r, n, act, c0=0, c1=D, parts=1):
        h = _dot_balanced(act, lambda a, b: w4p[:, c0 + a:c0 + b], c1 - c0, parts)
        x1 = h2s[rows(r, n), c0:c1] + hss[rows(r, n), c0:c1]
        ob[rows(r, n), c0:c1] = (x2s[rows(r, n), c0:c1] + mvec(4, n, c0, c1) * (x1 + 0.5 * h)).astype(bf16)

    groups = list(range(0, P0 + P1, RG))
    with _scope("pre_a"):
        wait("w_q0", [mod_copies[0], q_copies[0]])
        sa, ca, ga = mod_part(0, 1)
        modb[0] = ga * sa
        modb[1] = ga * (1.0 + ca)
        for c in range(NL, CT):
            mac_inv(c, NB - 1)
        st1 = {o: _stats(load_q(o)) for o in groups}
        zt[0:8, 0:128] = jnp.zeros((8, 128), u32)
        st2 = {}
        for o in groups:
            x2 = make_x2(o, load_q(o), st1[o])
            x2s[o:o + RG, :] = x2
            st2[o] = _stats(x2)
    with _scope("pre_b"):
        wait("w_modB", [mod_copies[1]])
        sb, cb = mod_part(1, 2)
        modb[2] = sb
        modb[3] = 1.0 + cb
        st3 = {}
        for o in range(0, P0, RG):
            h2 = make_h2(x2s[o:o + RG, :], st2[o])
            h2s[o:o + RG, :] = h2
            st3[o] = _stats(h2)
        for o in range(0, P0, RG):
            zt[o // 2:(o + RG) // 2, :] = pack_ln(h2s[o:o + RG, :], st3[o])
    with _scope("r1"):
        wait("w_w1", [w_copies[0]])
        w1p[...] = pltpu.bitcast(w1b[...], u32)
        mm_w1(0, P0)
        prev = None
        for o in range(P0, P0 + P1, RG):
            h2 = make_h2(x2s[o:o + RG, :], st2[o])
            h2s[o:o + RG, :] = h2
            st = _stats(h2, prev, early=True)
            zt[o // 2:(o + RG) // 2, :] = pack_ln(h2, st)
            prev = st[1]
        mm_w1(P0, P1, P0)
    with _scope("r2"):
        wait("w_w2", [w_copies[1]])
        w2p[...] = pltpu.bitcast(w2b[...], u32)
        mm_w2(0)
        ln_x1(0, 2)
        mm_w2(T)
    with _scope("r3"):
        wait("w_w3", [q_copies[1], w_copies[2]])
        w3p[...] = pltpu.bitcast(w3b[...], u32)
        ln_chain(P0 + P1, PA)
        main = mm_w3(0, 4)
        mm_w1(P0 + P1, PA)
        tail = mm_w3_tail()
    with _scope("r4"):
        wait("w_w4", [w_copies[3], mod_copies[2]])
        w4p[...] = pltpu.bitcast(w4b[...], u32)
        modb[4] = mod_part(2, 1)[0]
        w3n[...] = pltpu.bitcast(w3b[0:128, :].astype(f32).T.astype(bf16), u32)
        mm_w4(0, T, jnp.concatenate([main, tail.T], axis=-1), parts=2)
        ln_x1(T)
        out_copy(0).start()
        q_copies[2].wait()

    def mlp_body(i, carry):
        with _scope("iter"):
            r1 = pl.multiple_of(PB - PC + PC * i, 32)
            r = pl.multiple_of(i * T, T)
            first = mm_w3_first()
            ln_chain(r1, PC)
            tail = mm_w3_tail()
            act = jnp.concatenate([first, mm_w3(128), tail.T], axis=-1).astype(bf16)
            mm_w4(r, T, act, 0, 128)
            mm_w1(r1, PC, parts=1)
            mm_w4(r, T, act, 128, 256)
            mm_w2(r + T, parts=1)
            ln_x1(r + T)
            mm_w4(r, T, act, 256, D)
            out_copy(i).start()
        return carry

    with _scope("loop"):
        jax.lax.fori_loop(1, NC - 1, mlp_body, 0)
    with _scope("last"):
        first = mm_w3_first()
        tail = mm_w3_tail()
        act = jnp.concatenate([first, mm_w3(128), tail.T], axis=-1)
        mm_w4(S - T, LAST0, act[0:LAST0])
        out_tail[0].start()
        mm_w4(S - T + LAST0, T - LAST0, act[LAST0:T])
        out_tail[1].start()
    with _scope("fin"):
        for i in range(NC - 1):
            out_copy(i).wait()
        for cp in out_tail:
            cp.wait()


@jax.jit
def pallas_adaLN_cond__ssm_conv_h3__mixer_s_mlp__prompt_kernel(
    A_q: jax.Array,
    A_k: jax.Array,
    A_v: jax.Array,
    A_shift_k: jax.Array,
    A_ssm_k: jax.Array,
    A_ssm_D: jax.Array,
    B_x: jax.Array,
    B_w1: jax.Array,
    B_w2: jax.Array,
    B_w3: jax.Array,
    B_w4: jax.Array,
    c: jax.Array,
    w_mod: jax.Array,
):
    del B_x
    any_spec = pl.BlockSpec(memory_space=pl.ANY)

    def tile_view(x):
        return x.reshape(S // 8, 8, CT, 128).transpose(0, 2, 1, 3).reshape(S * CT, 128)

    vm = pltpu.VMEM
    dma = pltpu.SemaphoreType.DMA
    spec = (4, NG, 16, 128)
    out = pl.pallas_call(
        _kernel,
        in_specs=[any_spec] * 12,
        out_specs=any_spec,
        out_shape=jax.ShapeDtypeStruct((S, D), bf16),
        scratch_shapes=[
            vm((S * CT + 128, 128), bf16), vm((S * CT + 64, 128), bf16), vm((CT, 128, S), bf16),
            vm((S, D), bf16), vm((D, D), bf16), vm((D, D), bf16), vm((F, D), bf16), vm((F, D), bf16),
            vm((D // 2, D), u32), vm((D // 2, D), u32), vm((F // 2, D), u32), vm((F // 2, D), u32),
            vm((D, 6 * D), bf16), vm((4, D), bf16), vm((D,), bf16), vm((1, D), bf16), vm((1, 1792), f32),
            vm((4, 128, 128), u32), vm((4, 128, 128), u32), vm((4, 64, 256), u32),
            vm((CT, 8, 8, 128), f32),
            vm((CT, NB) + spec, f32), vm((CT, NB - 1) + spec, f32), vm((CT,) + spec, f32),
            vm((CT, NB) + spec, f32), vm((4, 128, 128), f32),
            vm((CT, S + 32, 128), f32), vm((8, 8, D), f32),
            vm((CT, S + 32, 128), f32), vm((S, D), f32), vm((S, D), f32), vm((S, D), f32),
            vm((288, D), u32), vm((T // 2, D), u32), vm((D // 2, 128), u32),
            vm((S, D), bf16),
            dma((26,)), dma((NC + 1,)),
        ],
        compiler_params=pltpu.CompilerParams(vmem_limit_bytes=110 << 20, disable_bounds_checks=True,
                                             disable_semaphore_checks=True),
    )(A_q.reshape(S, D), tile_view(A_k), tile_view(A_v), A_shift_k.T, A_ssm_k,
      A_ssm_D, B_w1, B_w2, B_w3.T, B_w4, c, w_mod)
    return out.reshape(1, S, D)
```

```python
import numpy as np
import jax
import jax.numpy as jnp
import jax.experimental.pallas as pl
import jax.experimental.pallas.tpu as pltpu

f32, bf16, u32, i32 = jnp.float32, jnp.bfloat16, jnp.uint32, jnp.int32

S, D, F = 2048, 640, 1728
CT = D // 128
TR = 8 * CT
NB, BLK, NFFT = 4, 512, 1024
NG = 16
T = 256
NC = S // T
FM = (F // 128) * 128
P0, P1, PA, PC = 320, 208, 176, 224
PB = P0 + P1 + PA
LAST0 = 208
RG = 16
EPS = 1e-5
NT_DIMS = (((1,), (1,)), ((), ()))
GV = 8
NL = 4


def _lo(w):
    return pltpu.bitcast(w << 16, f32)


def _hi(w):
    return pltpu.bitcast(w & jnp.uint32(0xFFFF0000), f32)


def _cos_turn(n32, scale):
    x = (2.0 ** 30 - jnp.abs(n32.astype(f32))) * (2.0 * np.pi / 2.0 ** 32)
    x2 = x * x
    c = [scale * v for v in (1.0, -1.0 / 6, 1.0 / 120, -1.0 / 5040, 1.0 / 362880)]
    return x * (c[0] + x2 * (c[1] + x2 * (c[2] + x2 * (c[3] + x2 * c[4]))))


def _slot_phase(idx):
    k = ((idx >> 4) << 3) + (idx & 7)
    return jnp.where(k < 64, 4 * k + 1, 4 * k - 253) << 21, (idx & 8) << 27


def _fwd_table(r):
    fr, off = _slot_phase(jax.lax.broadcasted_iota(i32, (256, 128), 0))
    return pltpu.bitcast(_cos_turn(fr * r + off, 1.0).astype(bf16), u32)


def _inv_table(p):
    row = jax.lax.broadcasted_iota(i32, (128, 256), 0)
    fr, off = _slot_phase(jax.lax.broadcasted_iota(i32, (128, 256), 1))
    return pltpu.bitcast(_cos_turn(fr * (4 * row + p) + off, 2.0 / NFFT).astype(bf16), u32)


def _radix4(re, im, inverse):
    ar, ai = re[0] + re[2], im[0] + im[2]
    br, bi = re[0] - re[2], im[0] - im[2]
    cr, ci = re[1] + re[3], im[1] + im[3]
    dr, di = re[1] - re[3], im[1] - im[3]
    minus_i = (br + di, bi - dr)
    plus_i = (br - di, bi + dr)
    if inverse:
        return [(ar + cr, ai + ci), plus_i, (ar - cr, ai - ci), minus_i]
    return [(ar + cr, ai + ci), minus_i, (ar - cr, ai - ci), plus_i]


def _stats(x, link=None, early=False):
    zero = 0.0 if link is None else jnp.minimum(link, 0.0)
    part = x[:, 0:128]
    for c in range(1, CT):
        part = part + x[:, c * 128:(c + 1) * 128]
    if link is not None and early:
        part = part + zero
        zero = 0.0
    m = jnp.sum(part, axis=-1, keepdims=True) * (1.0 / D)
    v = jnp.maximum(jnp.sum(x * x, axis=-1, keepdims=True) * (1.0 / D) - m * m, zero)
    return m, jax.lax.rsqrt(v + EPS)


def _gelu2(x):
    c = 0.7978845608028654
    u = c + (c * 0.044715) * (x * x)
    return x + x * jnp.tanh(x * u)


def _gelu(x):
    c = 0.7978845608028654
    u = c + (c * 0.044715) * (x * x)
    hx = 0.5 * x
    return hx + hx * jnp.tanh(x * u)


def _dot_balanced(x, wslice, n_cols, parts, nt=False):
    def mm(a, c0, c1):
        a, w = a.astype(bf16), pltpu.bitcast(wslice(c0, c1), bf16)
        if nt:
            return jax.lax.dot_general(a, w, NT_DIMS, preferred_element_type=f32)
        return jnp.dot(a, w, preferred_element_type=f32)

    if parts == 1:
        return mm(x, 0, n_cols)
    base, extra = divmod(x.shape[0] // 16, parts)
    last, o = [], 0
    head = mm(x, 0, n_cols - 128)
    for i in range(parts):
        n = 16 * (base + (1 if i < extra else 0))
        last.append(mm(x[o:o + n], n_cols - 128, n_cols))
        o += n
    return jnp.concatenate([head, jnp.concatenate(last, axis=0)], axis=-1)


def _kernel(q_hbm, k_hbm, v_hbm, sh_hbm, sk_hbm, d_hbm, w1_hbm, w2_hbm, w3_hbm, w4_hbm,
            c_hbm, wm_hbm, o_hbm,
            kb, vb, skb, qb, w1b, w2b, w3b, w4b, w1p, w2p, w3p, w4p, wmb, shb, db, cb_, scb,
            fub, fkb, gtb, par, US, KS, UR, YS, YP, ys, modb, h1s, h2s, x2s, hss, zt, zb, w3n, ob,
            sem, sem_o):
    n_in = [0]

    def load(src, dst):
        n_in[0] += 1
        return pltpu.make_async_copy(src, dst, sem.at[n_in[0] - 1])

    nkv = BLK * CT
    small = [load(d_hbm, db), load(sh_hbm, shb), load(c_hbm, cb_)]
    sk_copies = [load(sk_hbm.at[pl.ds(c * 128, 128), :], skb.at[c]) for c in range(CT)]
    kv_copies = [[load(k_hbm.at[pl.ds(a * nkv, nkv), :], kb.at[pl.ds(TR + a * nkv, nkv), :]),
                  load(v_hbm.at[pl.ds(a * nkv, nkv), :], vb.at[pl.ds(a * nkv, nkv), :])] for a in range(NB)]
    mod_cols = [(0, 3 * D), (3 * D, 2 * D), (5 * D, D)]
    mod_copies = [load(wm_hbm.at[:, pl.ds(o, n)], wmb.at[:, pl.ds(o, n)]) for o, n in mod_cols]
    w_copies = [load(w1_hbm, w1b), load(w2_hbm, w2b), load(w3_hbm, w3b), load(w4_hbm, w4b)]
    q_copies = [load(q_hbm.at[pl.ds(o, n), :], qb.at[pl.ds(o, n), :])
                for o, n in [(0, P0 + P1), (P0 + P1, PA), (PB, S - PB)]]

    def out_copy(i):
        r = i * T if isinstance(i, int) else pl.multiple_of(i * T, T)
        return pltpu.make_async_copy(ob.at[pl.ds(r, T), :], o_hbm.at[pl.ds(r, T), :], sem_o.at[i])

    out_tail = [pltpu.make_async_copy(ob.at[pl.ds(o, n), :], o_hbm.at[pl.ds(o, n), :], sem_o.at[NC - 1 + i])
                for i, (o, n) in enumerate([(S - T, LAST0), (S - T + LAST0, T - LAST0)])]

    for cp in (small + kv_copies[0] + sk_copies + kv_copies[1] + kv_copies[2] + kv_copies[3]
               + [mod_copies[0], q_copies[0], mod_copies[1], w_copies[0], w_copies[1], q_copies[1],
                  w_copies[2], w_copies[3], mod_copies[2], q_copies[2]]):
        cp.start()

    def wait(copies):
        for cp in copies:
            cp.wait()

    def pin(i, carry):
        z = jnp.zeros((8, 128), f32)
        scb[:, pl.ds(pl.multiple_of(i * 128, 128), 128)] = z[0:1]
        YP[i, 0:8, :] = z
        US[i, 0, 0, 0, 0:8, :] = z
        KS[i, 0, 0, 0, 0:8, :] = z
        YS[i, 0, 0, 0, 0:8, :] = z
        UR[i, 0, 0, 0:8, :] = z
        return carry

    def fence(i, carry):
        YP[i, 0:8, :] = jnp.zeros((8, 128), f32)
        return carry

    jax.lax.fori_loop(0, 2, pin, 0)
    lane = jax.lax.broadcasted_iota(i32, (256, 128), 1)
    for p in range(4):
        m = (lane - p) & 3
        fkb[p] = _fwd_table(128 * m + ((lane - m) & 127))
    for c in range(CT):
        kb[c * 8:(c + 1) * 8, :] = jnp.zeros((8, 128), bf16)
        h1s[c, 0:8, :] = jnp.zeros((8, 128), f32)
        h1s[c, S + 8:S + 16, :] = jnp.zeros((8, 128), f32)
    for p in range(4):
        fub[p] = _fwd_table(8 * (lane & 63) + ((lane >> 6) << 2) + p)
    wait(small)
    cvec = cb_[...].astype(f32)
    scb[:, 0:D] = cvec * jax.nn.sigmoid(cvec)
    dv = db[...].astype(f32).reshape(1, D)
    shv = shb[...].astype(f32)
    for c in range(CT):
        for i in range(4):
            par[c, i] = jnp.broadcast_to(shv[i:i + 1, c * 128:(c + 1) * 128], (8, 128))
        par[c, 4] = jnp.broadcast_to(dv[:, c * 128:(c + 1) * 128], (8, 128))
    for p in range(4):
        gtb[p] = _inv_table(p)

    kw = kb.bitcast(u32)
    vw = vb.bitcast(u32)

    def get(ref, idx, g, n):
        return (ref[idx + (slice(g, g + n), slice(0, 8))], ref[idx + (slice(g, g + n), slice(8, 16))])

    def put(ref, idx, g, n, xr, xi):
        ref[idx + (slice(g, g + n), slice(0, 8))] = xr
        ref[idx + (slice(g, g + n), slice(8, 16))] = xi

    def split(tt, g, n):
        tt = [t[g * 16:(g + n) * 16].reshape(n, 16, 128) for t in tt]
        return [t[:, 0:8] for t in tt], [t[:, 8:16] for t in tt]

    def fwd_k(c, j):
        lane = jax.lax.broadcasted_iota(i32, (64, 128), 1)
        even = (lane & 1) == 0
        l01 = (lane & 2) == 0
        l12 = ((lane + 3) & 2) == 0
        rm = []
        for m in range(4):
            w = pltpu.bitcast(skb[c, :, (4 * j + m) * 128:(4 * j + m + 1) * 128], u32)
            rm.append(pltpu.roll(w, m, 1) if m else w)
        e01 = jnp.where(even, rm[0], rm[1])
        o01 = jnp.where(even, rm[1], rm[0])
        e23 = jnp.where(even, rm[2], rm[3])
        o23 = jnp.where(even, rm[3], rm[2])
        kp = [jnp.where(l01, e01, e23), jnp.where(l12, o01, o23),
              jnp.where(l01, e23, e01), jnp.where(l12, o23, o01)]
        tt = [jax.lax.dot_general(pltpu.bitcast(fkb[p], bf16), pltpu.bitcast(kp[p], bf16), NT_DIMS,
                                  preferred_element_type=f32) for p in range(4)]
        for g in range(0, NG, GV):
            re, im = split(tt, g, GV)
            if j == 0:
                re[0] = re[0] + par[c, 4][None]
            for m, (xr, xi) in enumerate(_radix4(re, im, False)):
                if j < NB - 1:
                    put(KS, (c, j, m), g, GV, xr, xi)
                ur, ui = get(US, (c, 0, m), g, GV)
                put(YS, (c, j, m), g, GV, xr * ur - xi * ui, xr * ui + xi * ur)

    def fwd_u(c, a):
        taps = [jnp.tile(par[c, i], (8, 1)) for i in range(4)]
        ws = TR // 2
        base = a * (BLK // 8) * ws + 4 * c

        def words(ref, start):
            return ref[pl.ds(start, BLK // 8, stride=ws), :]

        kk = {}
        for w in range(4):
            x = words(kw, ws + base + w)
            kk[2 * w], kk[2 * w + 1] = _lo(x), _hi(x)
        kk[-3] = _hi(words(kw, base + 2))
        x = words(kw, base + 3)
        kk[-2], kk[-1] = _lo(x), _hi(x)
        sub = []
        for w in range(4):
            x = words(vw, base + w)
            for r, vv in ((2 * w, _lo(x)), (2 * w + 1, _hi(x))):
                sh = taps[0] * kk[r] + taps[1] * kk[r - 1] + taps[2] * kk[r - 2] + taps[3] * kk[r - 3]
                sub.append(sh * vv)
        kv = [jnp.concatenate([sub[p], sub[p + 4]], axis=0) for p in range(4)]
        tt = [jnp.dot(pltpu.bitcast(fub[p], bf16), kv[p].astype(bf16), preferred_element_type=f32)
              for p in range(4)]
        for g in range(0, NG, GV):
            re, im = split(tt, g, GV)
            for m, (xr, xi) in enumerate(_radix4(re, im, False)):
                if a:
                    pr, pi = get(US, (c, 0, m), g, GV) if a == 1 else get(UR, (c, m), g, GV)
                    if a < NB - 1:
                        put(UR, (c, m), g, GV, xr, xi)
                    xr, xi = (xr - pi, xi + pr) if g < NG // 2 else (xr + pi, xi - pr)
                put(US, (c, a, m), g, GV, xr, xi)

    def mac_inv(c, a):
        for h in range(2):
            vals = [[] for _ in range(4)]
            for g in range(8 * h, 8 * h + 8, GV):
                yre, yim = [], []
                for m in range(4):
                    yr, yi = get(YS, (c, a, m), g, GV)
                    for j in range(a):
                        kr, ki = get(KS, (c, j, m), g, GV)
                        ur, ui = get(US, (c, a - j, m), g, GV)
                        yr = yr + (kr * ur - ki * ui)
                        yi = yi + (kr * ui + ki * ur)
                    yre.append(yr)
                    yim.append(yi)
                for p, (pr, pi) in enumerate(_radix4(yre, yim, True)):
                    vals[p].append(jnp.concatenate([pr, pi], axis=1))
            for p in range(4):
                pb = jnp.concatenate(vals[p], axis=0).reshape(128, 128).astype(bf16)
                r = jnp.dot(pltpu.bitcast(gtb[p, :, h * 128:(h + 1) * 128], bf16), pb,
                            preferred_element_type=f32)
                if h == 0:
                    YP[p] = r
                else:
                    ys[c, pl.ds(a * BLK + p, 128, stride=4), :] = YP[p] + r

    wait(kv_copies[0])
    for c in range(CT):
        fwd_u(c, 0)

    for grp in ((0,), (1, 2), (3, 4)):
        wait([sk_copies[c] for c in grp])
        for c in grp:
            for j in (3, 2, 1, 0):
                fwd_k(c, j)
    for a in range(1, NB):
        wait(kv_copies[a])
        for c in range(CT):
            fwd_u(c, a)
            mac_inv(c, a - 1)

    jax.lax.fori_loop(0, 2, fence, 0)
    for c in range(NL):
        mac_inv(c, NB - 1)

    def mod_part(part, extra):
        o, n = mod_cols[part]
        act = scb[:, 0:D]

        def sc(k0, k1):
            return jnp.broadcast_to(act[:, k0:k1], (16, k1 - k0)).astype(bf16)

        e = 128 * extra
        r = jnp.dot(sc(0, D), wmb[:, o + e:o + n], preferred_element_type=f32)
        r0 = (jnp.dot(sc(0, D - 64), wmb[0:D - 64, o:o + e], preferred_element_type=f32)
              + jnp.dot(sc(D - 64, D), wmb[D - 64:D, o:o + e], preferred_element_type=f32))
        r = jnp.concatenate([r0, r], axis=-1)[0:8]
        return [r[:, i * D:(i + 1) * D] for i in range(n // D)]

    def mvec(i, n=RG, c0=0, c1=D):
        return jnp.tile(modb[i, :, c0:c1], (n // 8, 1))

    rows = pl.ds

    def load_q(r, ref=qb):
        return ref[rows(r, RG), :].astype(f32)

    def make_x2(r, q, st, ref=ys):
        y = jnp.concatenate([ref[c, rows(r, RG), :] for c in range(CT)], axis=-1)
        return q + (((q - st[0]) * st[1]) * mvec(1) + mvec(0)) * y

    def make_h2(x2, st):
        return ((x2 - st[0]) * st[1]) * mvec(3) + mvec(2)

    def pack_ln(x, st):
        return pltpu.bitcast(((x - st[0]) * st[1]).astype(bf16), u32)

    def ln_chain(r, n):
        qv, yv = qb.at[rows(r, n), :], ys.at[:, rows(r, n), :]
        xv, hv = x2s.at[rows(r, n), :], h2s.at[rows(r, n), :]
        prev = None
        for o in range(0, n, RG):
            q = load_q(o, qv)
            x2 = make_x2(o, q, _stats(q, prev), yv)
            xv[o:o + RG, :] = x2
            st = _stats(x2)
            h2 = make_h2(xv[o:o + RG, :], st)
            hv[o:o + RG, :] = h2
            st = _stats(h2)
            zt[o // 2:(o + RG) // 2, :] = pack_ln(hv[o:o + RG, :], st)
            prev = st[1]

    def mm_w1(r, n, o=0, parts=4):
        z = pltpu.bitcast(zt[o // 2:(o + n) // 2, :], bf16)
        h1 = _gelu(_dot_balanced(z, lambda a, b: w1p[:, a:b], D, parts))
        for c in range(CT):
            h1s[c, rows(r + 8, n), :] = h1[:, c * 128:(c + 1) * 128]

    def mm_w2(r, parts=4):
        lane = jax.lax.broadcasted_iota(i32, (T, 128), 1)

        def sh(k, c):
            return h1s[c, rows(r + 8 + k, T), :]

        g = jnp.concatenate([
            sh(-1, 0),
            jnp.where(lane < 32, sh(-1, 1), sh(1, 1)),
            jnp.where(lane < 64, sh(1, 2), sh(-2, 2)),
            jnp.where(lane < 96, sh(-2, 3), sh(2, 3)),
            sh(2, 4)], axis=-1)
        hss[rows(r, T), :] = _dot_balanced(g, lambda a, b: w2p[:, a:b], D, parts)

    def ln_x1(r, links=1):
        hv, sv = h2s.at[rows(r, T), :], hss.at[rows(r, T), :]
        prev = [None] * links
        for n, o in enumerate(range(0, T, RG)):
            x1 = hv[o:o + RG, :] + sv[o:o + RG, :]
            st = _stats(x1, prev[n % links], early=True)
            zb[o // 2:(o + RG) // 2, :] = pack_ln(x1, st)
            prev[n % links] = st[1]

    def mm_w3(f0, parts=1):
        z = pltpu.bitcast(zb[...], bf16)
        return _gelu2(_dot_balanced(z, lambda a, b: w3p[(f0 + a) // 2:(f0 + b) // 2, :], FM - f0, parts, nt=True))

    def mm_w3_first():
        z = pltpu.bitcast(zb[...], bf16)
        return _gelu2(jnp.dot(z, pltpu.bitcast(w3n[...], bf16), preferred_element_type=f32))

    def mm_w3_tail():
        z = pltpu.bitcast(zb[...], bf16)
        w = pltpu.bitcast(w3p[FM // 2:F // 2, :], bf16)
        return _gelu2(jax.lax.dot_general(w, z, NT_DIMS, preferred_element_type=f32))

    def mm_w4(r, n, act, c0=0, c1=D):
        h = _dot_balanced(act, lambda a, b: w4p[:, c0 + a:c0 + b], c1 - c0, 1)
        x1 = h2s[rows(r, n), c0:c1] + hss[rows(r, n), c0:c1]
        base = x2s[rows(r, n), c0:c1] + mvec(4, n, c0, c1) * x1
        ob[rows(r, n), c0:c1] = (base + mvec(5, n, c0, c1) * h).astype(bf16)

    groups = list(range(0, P0 + P1, RG))

    wait([mod_copies[0], q_copies[0]])
    sa, ca, ga = mod_part(0, 1)
    modb[0] = ga * sa
    modb[1] = ga * (1.0 + ca)
    for c in range(NL, CT):
        mac_inv(c, NB - 1)
    st1 = {o: _stats(load_q(o)) for o in groups}
    zt[0:8, 0:128] = jnp.zeros((8, 128), u32)
    st2 = {}
    for o in groups:
        x2 = make_x2(o, load_q(o), st1[o])
        x2s[o:o + RG, :] = x2
        st2[o] = _stats(x2)

    wait([mod_copies[1]])
    sb, cb = mod_part(1, 2)
    modb[2] = sb
    modb[3] = 1.0 + cb
    st3 = {}
    for o in range(0, P0, RG):
        h2 = make_h2(x2s[o:o + RG, :], st2[o])
        h2s[o:o + RG, :] = h2
        st3[o] = _stats(h2)
    for o in range(0, P0, RG):
        zt[o // 2:(o + RG) // 2, :] = pack_ln(h2s[o:o + RG, :], st3[o])

    wait([w_copies[0]])
    w1p[...] = pltpu.bitcast(w1b[...], u32)
    mm_w1(0, P0)
    prev = None
    for o in range(P0, P0 + P1, RG):
        h2 = make_h2(x2s[o:o + RG, :], st2[o])
        h2s[o:o + RG, :] = h2
        st = _stats(h2, prev, early=True)
        zt[o // 2:(o + RG) // 2, :] = pack_ln(h2, st)
        prev = st[1]
    mm_w1(P0, P1, P0)

    wait([w_copies[1]])
    w2p[...] = pltpu.bitcast(w2b[...], u32)
    mm_w2(0)
    ln_x1(0, 2)
    mm_w2(T)

    wait([q_copies[1], w_copies[2]])
    w3p[...] = pltpu.bitcast(w3b[...], u32)
    ln_chain(P0 + P1, PA)
    main = mm_w3(0, 4)
    mm_w1(P0 + P1, PA)
    tail = mm_w3_tail()

    wait([w_copies[3], mod_copies[2]])
    w4p[...] = pltpu.bitcast(w4b[...], u32)
    w3n[...] = pltpu.bitcast(w3b[0:128, :].astype(f32).T.astype(bf16), u32)
    act = jnp.concatenate([main, tail.T], axis=-1).astype(bf16)
    sc16 = jnp.broadcast_to(scb[:, 0:D], (16, D)).astype(bf16)
    for c0 in range(0, D, 128):
        gb = jnp.dot(sc16, wmb[:, 5 * D + c0:5 * D + c0 + 128], preferred_element_type=f32)[0:8]
        modb[4, :, c0:c0 + 128] = gb
        modb[5, :, c0:c0 + 128] = 0.5 * gb
        if c0 < D - 128:
            mm_w4(0, T, act, c0, c0 + 128)
        else:
            mm_w4(0, T // 2, act[0:T // 2], c0, c0 + 128)
            mm_w4(T // 2, T // 2, act[T // 2:T], c0, c0 + 128)
    ln_x1(T)
    out_copy(0).start()
    q_copies[2].wait()

    def mlp_body(i, carry):
        r1 = pl.multiple_of(PB - PC + PC * i, 32)
        r = pl.multiple_of(i * T, T)
        first = mm_w3_first()
        ln_chain(r1, PC)
        tail = mm_w3_tail()
        act = jnp.concatenate([first, mm_w3(128), tail.T], axis=-1).astype(bf16)
        mm_w4(r, T, act, 0, 128)
        mm_w1(r1, PC, parts=1)
        mm_w4(r, T, act, 128, 256)
        mm_w2(r + T, parts=1)
        ln_x1(r + T)
        mm_w4(r, T, act, 256, D)
        out_copy(i).start()
        return carry

    jax.lax.fori_loop(1, NC - 1, mlp_body, 0)

    first = mm_w3_first()
    tail = mm_w3_tail()
    act = jnp.concatenate([first, mm_w3(128), tail.T], axis=-1)
    mm_w4(S - T, LAST0, act[0:LAST0])
    out_tail[0].start()
    mm_w4(S - T + LAST0, T - LAST0, act[LAST0:T])
    out_tail[1].start()

    for i in range(NC - 1):
        out_copy(i).wait()
    for cp in out_tail:
        cp.wait()


@jax.jit
def pallas_adaLN_cond__ssm_conv_h3__mixer_s_mlp__prompt_kernel(
    A_q: jax.Array,
    A_k: jax.Array,
    A_v: jax.Array,
    A_shift_k: jax.Array,
    A_ssm_k: jax.Array,
    A_ssm_D: jax.Array,
    B_x: jax.Array,
    B_w1: jax.Array,
    B_w2: jax.Array,
    B_w3: jax.Array,
    B_w4: jax.Array,
    c: jax.Array,
    w_mod: jax.Array,
):
    del B_x
    any_spec = pl.BlockSpec(memory_space=pl.ANY)

    def tile_view(x):
        return x.reshape(S // 8, 8, CT, 128).transpose(0, 2, 1, 3).reshape(S * CT, 128)

    vm = pltpu.VMEM
    dma = pltpu.SemaphoreType.DMA
    spec = (4, NG, 16, 128)
    out = pl.pallas_call(
        _kernel,
        in_specs=[any_spec] * 12,
        out_specs=any_spec,
        out_shape=jax.ShapeDtypeStruct((S, D), bf16),
        scratch_shapes=[
            vm((S * CT + 128, 128), bf16), vm((S * CT + 64, 128), bf16), vm((CT, 128, S), bf16),
            vm((S, D), bf16), vm((D, D), bf16), vm((D, D), bf16), vm((F, D), bf16), vm((F, D), bf16),
            vm((D // 2, D), u32), vm((D // 2, D), u32), vm((F // 2, D), u32), vm((F // 2, D), u32),
            vm((D, 6 * D), bf16), vm((4, D), bf16), vm((D,), bf16), vm((1, D), bf16), vm((1, 1792), f32),
            vm((4, 128, 128), u32), vm((4, 128, 128), u32), vm((4, 64, 256), u32),
            vm((CT, 8, 8, 128), f32),
            vm((CT, NB) + spec, f32), vm((CT, NB - 1) + spec, f32), vm((CT,) + spec, f32),
            vm((CT, NB) + spec, f32), vm((4, 128, 128), f32),
            vm((CT, S + 32, 128), f32), vm((8, 8, D), f32),
            vm((CT, S + 32, 128), f32), vm((S, D), f32), vm((S, D), f32), vm((S, D), f32),
            vm((288, D), u32), vm((T // 2, D), u32), vm((D // 2, 128), u32),
            vm((S, D), bf16),
            dma((26,)), dma((NC + 1,)),
        ],
        compiler_params=pltpu.CompilerParams(vmem_limit_bytes=110 << 20, disable_bounds_checks=True,
                                             disable_semaphore_checks=True),
    )(A_q.reshape(S, D), tile_view(A_k), tile_view(A_v), A_shift_k.T, A_ssm_k,
      A_ssm_D, B_w1, B_w2, B_w3.T, B_w4, c, w_mod)
    return out.reshape(1, S, D)
```

```python
import numpy as np
import jax
import jax.numpy as jnp
import jax.experimental.pallas as pl
import jax.experimental.pallas.tpu as pltpu

f32, bf16, u32, i32 = jnp.float32, jnp.bfloat16, jnp.uint32, jnp.int32

S, D, F = 2048, 640, 1728
CT = D // 128
TR = 8 * CT
NB, BLK, NFFT = 4, 512, 1024
KROWS, VROWS = BLK * CT + 128, BLK * CT + 64
NG = 16
T = 256
NC = S // T
FM = (F // 128) * 128
P0, P1, PA, PC = 320, 208, 176, 224
PB = P0 + P1 + PA
LAST0 = 208
RG = 16
EPS = 1e-5
NT_DIMS = (((1,), (1,)), ((), ()))
GV = 8
NL = 4


def _lo(w):
    return pltpu.bitcast(w << 16, f32)


def _hi(w):
    return pltpu.bitcast(w & jnp.uint32(0xFFFF0000), f32)


def _cos_turn(n32, scale):
    x = (2.0 ** 30 - jnp.abs(n32.astype(f32))) * (2.0 * np.pi / 2.0 ** 32)
    x2 = x * x
    c = [scale * v for v in (1.0, -1.0 / 6, 1.0 / 120, -1.0 / 5040, 1.0 / 362880)]
    return x * (c[0] + x2 * (c[1] + x2 * (c[2] + x2 * (c[3] + x2 * c[4]))))


def _slot_phase(idx):
    k = ((idx >> 4) << 3) + (idx & 7)
    return jnp.where(k < 64, 4 * k + 1, 4 * k - 253) << 21, (idx & 8) << 27


def _fwd_table(r):
    fr, off = _slot_phase(jax.lax.broadcasted_iota(i32, (256, 128), 0))
    return pltpu.bitcast(_cos_turn(fr * r + off, 1.0).astype(bf16), u32)


def _inv_table(p):
    row = jax.lax.broadcasted_iota(i32, (128, 256), 0)
    fr, off = _slot_phase(jax.lax.broadcasted_iota(i32, (128, 256), 1))
    return pltpu.bitcast(_cos_turn(fr * (4 * row + p) + off, 2.0 / NFFT).astype(bf16), u32)


def _radix4(re, im, inverse):
    ar, ai = re[0] + re[2], im[0] + im[2]
    br, bi = re[0] - re[2], im[0] - im[2]
    cr, ci = re[1] + re[3], im[1] + im[3]
    dr, di = re[1] - re[3], im[1] - im[3]
    minus_i = (br + di, bi - dr)
    plus_i = (br - di, bi + dr)
    if inverse:
        return [(ar + cr, ai + ci), plus_i, (ar - cr, ai - ci), minus_i]
    return [(ar + cr, ai + ci), minus_i, (ar - cr, ai - ci), plus_i]


def _stats(x, link=None, early=False):
    zero = 0.0 if link is None else jnp.minimum(link, 0.0)
    part = x[:, 0:128]
    for c in range(1, CT):
        part = part + x[:, c * 128:(c + 1) * 128]
    if link is not None and early:
        part = part + zero
        zero = 0.0
    m = jnp.sum(part, axis=-1, keepdims=True) * (1.0 / D)
    v = jnp.maximum(jnp.sum(x * x, axis=-1, keepdims=True) * (1.0 / D) - m * m, zero)
    return m, jax.lax.rsqrt(v + EPS)


def _gelu2(x):
    c = 0.7978845608028654
    u = c + (c * 0.044715) * (x * x)
    return x + x * jnp.tanh(x * u)


def _gelu(x):
    c = 0.7978845608028654
    u = c + (c * 0.044715) * (x * x)
    hx = 0.5 * x
    return hx + hx * jnp.tanh(x * u)


def _dot_balanced(x, wslice, n_cols, parts, nt=False):
    def mm(a, c0, c1):
        a, w = a.astype(bf16), pltpu.bitcast(wslice(c0, c1), bf16)
        if nt:
            return jax.lax.dot_general(a, w, NT_DIMS, preferred_element_type=f32)
        return jnp.dot(a, w, preferred_element_type=f32)

    if parts == 1:
        return mm(x, 0, n_cols)
    base, extra = divmod(x.shape[0] // 16, parts)
    last, o = [], 0
    head = mm(x, 0, n_cols - 128)
    for i in range(parts):
        n = 16 * (base + (1 if i < extra else 0))
        last.append(mm(x[o:o + n], n_cols - 128, n_cols))
        o += n
    return jnp.concatenate([head, jnp.concatenate(last, axis=0)], axis=-1)


def _kernel(q_hbm, k_hbm, v_hbm, sh_hbm, sk_hbm, d_hbm, w1_hbm, w2_hbm, w3_hbm, w4_hbm,
            c_hbm, wm_hbm, o_hbm,
            kb0, kb1, kb2, kb3, vb0, vb1, vb2, vb3, skb, qb, w1b, w2b, w3b, w4b, w1p, w2p, w3p, w4p,
            wma, wmb, wmc, shb, db, cb_, scb,
            fub, fkb, gtb, par, US, KS, UR, YS, YP, ys, modb, h1s, h2s, x2s, hss, zt, zb, w3n, ob,
            sem, sem_o):
    n_in = [0]

    def load(src, dst):
        n_in[0] += 1
        return pltpu.make_async_copy(src, dst, sem.at[n_in[0] - 1])

    nkv = BLK * CT
    small = [load(d_hbm, db), load(sh_hbm, shb), load(c_hbm, cb_)]
    sk_copies = [load(sk_hbm.at[pl.ds(c * 128, 128), :], skb.at[c]) for c in range(CT)]
    kbs, vbs, wms = [kb0, kb1, kb2, kb3], [vb0, vb1, vb2, vb3], [wma, wmb, wmc]
    kv_copies = [[load(k_hbm.at[pl.ds(0, nkv), :], kb0.at[pl.ds(TR, nkv), :]) if a == 0 else
                  load(k_hbm.at[pl.ds(a * nkv - TR, nkv + TR), :], kbs[a].at[pl.ds(0, nkv + TR), :]),
                  load(v_hbm.at[pl.ds(a * nkv, nkv), :], vbs[a].at[pl.ds(0, nkv), :])] for a in range(NB)]
    mod_cols = [(0, 3 * D), (3 * D, 2 * D), (5 * D, D)]
    mod_copies = [load(wm_hbm.at[:, pl.ds(o, n)], w) for (o, n), w in zip(mod_cols, wms)]
    w_copies = [load(w1_hbm, w1b), load(w2_hbm, w2b), load(w3_hbm, w3b), load(w4_hbm, w4b)]
    q_copies = [load(q_hbm.at[pl.ds(o, n), :], qb.at[pl.ds(o, n), :])
                for o, n in [(0, P0 + P1), (P0 + P1, PA), (PB, S - PB)]]

    def out_copy(i):
        r = i * T if isinstance(i, int) else pl.multiple_of(i * T, T)
        return pltpu.make_async_copy(ob.at[pl.ds(r, T), :], o_hbm.at[pl.ds(r, T), :], sem_o.at[i])

    out_tail = [pltpu.make_async_copy(ob.at[pl.ds(o, n), :], o_hbm.at[pl.ds(o, n), :], sem_o.at[NC - 1 + i])
                for i, (o, n) in enumerate([(S - T, LAST0), (S - T + LAST0, T - LAST0)])]

    for cp in (small + kv_copies[0] + sk_copies + kv_copies[1] + kv_copies[2] + kv_copies[3]
               + [mod_copies[0], q_copies[0], mod_copies[1], w_copies[0], w_copies[1], q_copies[1],
                  w_copies[2], w_copies[3], mod_copies[2], q_copies[2]]):
        cp.start()

    def wait(copies):
        for cp in copies:
            cp.wait()

    def pin(i, carry):
        z = jnp.zeros((8, 128), f32)
        scb[:, pl.ds(pl.multiple_of(i * 128, 128), 128)] = z[0:1]
        YP[i, 0:8, :] = z
        US[i, 0, 0, 0, 0:8, :] = z
        KS[i, 0, 0, 0, 0:8, :] = z
        YS[i, 0, 0, 0, 0:8, :] = z
        UR[i, 0, 0, 0:8, :] = z
        return carry

    def fence(i, carry):
        YP[i, 0:8, :] = jnp.zeros((8, 128), f32)
        return carry

    jax.lax.fori_loop(0, 2, pin, 0)
    lane = jax.lax.broadcasted_iota(i32, (256, 128), 1)
    for p in range(4):
        m = (lane - p) & 3
        fkb[p] = _fwd_table(128 * m + ((lane - m) & 127))
    for c in range(CT):
        kb0[c * 8:(c + 1) * 8, :] = jnp.zeros((8, 128), bf16)
        h1s[c, 0:8, :] = jnp.zeros((8, 128), f32)
        h1s[c, S + 8:S + 16, :] = jnp.zeros((8, 128), f32)
    for a in range(NB):
        kbs[a][nkv + TR:KROWS, :] = jnp.zeros((KROWS - nkv - TR, 128), bf16)
        vbs[a][nkv:VROWS, :] = jnp.zeros((VROWS - nkv, 128), bf16)
    for p in range(4):
        fub[p] = _fwd_table(8 * (lane & 63) + ((lane >> 6) << 2) + p)
    wait(small)
    cvec = cb_[...].astype(f32)
    scb[:, 0:D] = cvec * jax.nn.sigmoid(cvec)
    dv = db[...].astype(f32).reshape(1, D)
    shv = shb[...].astype(f32)
    for c in range(CT):
        for i in range(4):
            par[c, i] = jnp.broadcast_to(shv[i:i + 1, c * 128:(c + 1) * 128], (8, 128))
        par[c, 4] = jnp.broadcast_to(dv[:, c * 128:(c + 1) * 128], (8, 128))
    for p in range(4):
        gtb[p] = _inv_table(p)

    def get(ref, idx, g, n):
        return (ref[idx + (slice(g, g + n), slice(0, 8))], ref[idx + (slice(g, g + n), slice(8, 16))])

    def put(ref, idx, g, n, xr, xi):
        ref[idx + (slice(g, g + n), slice(0, 8))] = xr
        ref[idx + (slice(g, g + n), slice(8, 16))] = xi

    def split(tt, g, n):
        tt = [t[g * 16:(g + n) * 16].reshape(n, 16, 128) for t in tt]
        return [t[:, 0:8] for t in tt], [t[:, 8:16] for t in tt]

    def fwd_k(c, j):
        lane = jax.lax.broadcasted_iota(i32, (64, 128), 1)
        even = (lane & 1) == 0
        l01 = (lane & 2) == 0
        l12 = ((lane + 3) & 2) == 0
        rm = []
        for m in range(4):
            w = pltpu.bitcast(skb[c, :, (4 * j + m) * 128:(4 * j + m + 1) * 128], u32)
            rm.append(pltpu.roll(w, m, 1) if m else w)
        e01 = jnp.where(even, rm[0], rm[1])
        o01 = jnp.where(even, rm[1], rm[0])
        e23 = jnp.where(even, rm[2], rm[3])
        o23 = jnp.where(even, rm[3], rm[2])
        kp = [jnp.where(l01, e01, e23), jnp.where(l12, o01, o23),
              jnp.where(l01, e23, e01), jnp.where(l12, o23, o01)]
        tt = [jax.lax.dot_general(pltpu.bitcast(fkb[p], bf16), pltpu.bitcast(kp[p], bf16), NT_DIMS,
                                  preferred_element_type=f32) for p in range(4)]
        for g in range(0, NG, GV):
            re, im = split(tt, g, GV)
            if j == 0:
                re[0] = re[0] + par[c, 4][None]
            for m, (xr, xi) in enumerate(_radix4(re, im, False)):
                if j < NB - 1:
                    put(KS, (c, j, m), g, GV, xr, xi)
                ur, ui = get(US, (c, 0, m), g, GV)
                put(YS, (c, j, m), g, GV, xr * ur - xi * ui, xr * ui + xi * ur)

    def fwd_u(c, a):
        taps = [jnp.tile(par[c, i], (8, 1)) for i in range(4)]
        ws = TR // 2
        base = 4 * c
        kw, vw = kbs[a].bitcast(u32), vbs[a].bitcast(u32)

        def words(ref, start):
            return ref[pl.ds(start, BLK // 8, stride=ws), :]

        kk = {}
        for w in range(4):
            x = words(kw, ws + base + w)
            kk[2 * w], kk[2 * w + 1] = _lo(x), _hi(x)
        kk[-3] = _hi(words(kw, base + 2))
        x = words(kw, base + 3)
        kk[-2], kk[-1] = _lo(x), _hi(x)
        sub = []
        for w in range(4):
            x = words(vw, base + w)
            for r, vv in ((2 * w, _lo(x)), (2 * w + 1, _hi(x))):
                sh = taps[0] * kk[r] + taps[1] * kk[r - 1] + taps[2] * kk[r - 2] + taps[3] * kk[r - 3]
                sub.append(sh * vv)
        kv = [jnp.concatenate([sub[p], sub[p + 4]], axis=0) for p in range(4)]
        tt = [jnp.dot(pltpu.bitcast(fub[p], bf16), kv[p].astype(bf16), preferred_element_type=f32)
              for p in range(4)]
        for g in range(0, NG, GV):
            re, im = split(tt, g, GV)
            for m, (xr, xi) in enumerate(_radix4(re, im, False)):
                if a:
                    pr, pi = get(US, (c, 0, m), g, GV) if a == 1 else get(UR, (c, m), g, GV)
                    if a < NB - 1:
                        put(UR, (c, m), g, GV, xr, xi)
                    xr, xi = (xr - pi, xi + pr) if g < NG // 2 else (xr + pi, xi - pr)
                put(US, (c, a, m), g, GV, xr, xi)

    def mac_inv(c, a):
        for h in range(2):
            vals = [[] for _ in range(4)]
            for g in range(8 * h, 8 * h + 8, GV):
                yre, yim = [], []
                for m in range(4):
                    yr, yi = get(YS, (c, a, m), g, GV)
                    for j in range(a):
                        kr, ki = get(KS, (c, j, m), g, GV)
                        ur, ui = get(US, (c, a - j, m), g, GV)
                        yr = yr + (kr * ur - ki * ui)
                        yi = yi + (kr * ui + ki * ur)
                    yre.append(yr)
                    yim.append(yi)
                for p, (pr, pi) in enumerate(_radix4(yre, yim, True)):
                    vals[p].append(jnp.concatenate([pr, pi], axis=1))
            for p in range(4):
                pb = jnp.concatenate(vals[p], axis=0).reshape(128, 128).astype(bf16)
                r = jnp.dot(pltpu.bitcast(gtb[p, :, h * 128:(h + 1) * 128], bf16), pb,
                            preferred_element_type=f32)
                if h == 0:
                    YP[p] = r
                else:
                    ys[c, pl.ds(a * BLK + p, 128, stride=4), :] = YP[p] + r

    wait(kv_copies[0])
    for c in range(CT):
        fwd_u(c, 0)

    for grp in ((0,), (1, 2), (3, 4)):
        wait([sk_copies[c] for c in grp])
        for c in grp:
            for j in (3, 2, 1, 0):
                fwd_k(c, j)
    for a in range(1, NB):
        wait(kv_copies[a])
        for c in range(CT):
            fwd_u(c, a)
            mac_inv(c, a - 1)

    jax.lax.fori_loop(0, 2, fence, 0)
    for c in range(NL):
        mac_inv(c, NB - 1)

    def mod_part(part, extra):
        n, wm = mod_cols[part][1], wms[part]
        act = scb[:, 0:D]

        def sc(k0, k1):
            return jnp.broadcast_to(act[:, k0:k1], (16, k1 - k0)).astype(bf16)

        e = 128 * extra
        r = jnp.dot(sc(0, D), wm[:, e:n], preferred_element_type=f32)
        r0 = (jnp.dot(sc(0, D - 64), wm[0:D - 64, 0:e], preferred_element_type=f32)
              + jnp.dot(sc(D - 64, D), wm[D - 64:D, 0:e], preferred_element_type=f32))
        r = jnp.concatenate([r0, r], axis=-1)[0:8]
        return [r[:, i * D:(i + 1) * D] for i in range(n // D)]

    def mvec(i, n=RG, c0=0, c1=D):
        return jnp.tile(modb[i, :, c0:c1], (n // 8, 1))

    rows = pl.ds

    def load_q(r, ref=qb):
        return ref[rows(r, RG), :].astype(f32)

    def make_x2(r, q, st, ref=ys):
        y = jnp.concatenate([ref[c, rows(r, RG), :] for c in range(CT)], axis=-1)
        return q + (((q - st[0]) * st[1]) * mvec(1) + mvec(0)) * y

    def make_h2(x2, st):
        return ((x2 - st[0]) * st[1]) * mvec(3) + mvec(2)

    def pack_ln(x, st):
        return pltpu.bitcast(((x - st[0]) * st[1]).astype(bf16), u32)

    def ln_chain(r, n):
        qv, yv = qb.at[rows(r, n), :], ys.at[:, rows(r, n), :]
        xv, hv = x2s.at[rows(r, n), :], h2s.at[rows(r, n), :]
        prev = None
        for o in range(0, n, RG):
            q = load_q(o, qv)
            x2 = make_x2(o, q, _stats(q, prev), yv)
            xv[o:o + RG, :] = x2
            st = _stats(x2)
            h2 = make_h2(xv[o:o + RG, :], st)
            hv[o:o + RG, :] = h2
            st = _stats(h2)
            zt[o // 2:(o + RG) // 2, :] = pack_ln(hv[o:o + RG, :], st)
            prev = st[1]

    def mm_w1(r, n, o=0, parts=4):
        z = pltpu.bitcast(zt[o // 2:(o + n) // 2, :], bf16)
        h1 = _gelu(_dot_balanced(z, lambda a, b: w1p[:, a:b], D, parts))
        for c in range(CT):
            h1s[c, rows(r + 8, n), :] = h1[:, c * 128:(c + 1) * 128]

    def mm_w2(r, parts=4):
        lane = jax.lax.broadcasted_iota(i32, (T, 128), 1)

        def sh(k, c):
            return h1s[c, rows(r + 8 + k, T), :]

        g = jnp.concatenate([
            sh(-1, 0),
            jnp.where(lane < 32, sh(-1, 1), sh(1, 1)),
            jnp.where(lane < 64, sh(1, 2), sh(-2, 2)),
            jnp.where(lane < 96, sh(-2, 3), sh(2, 3)),
            sh(2, 4)], axis=-1)
        hss[rows(r, T), :] = _dot_balanced(g, lambda a, b: w2p[:, a:b], D, parts)

    def ln_x1(r, links=1):
        hv, sv = h2s.at[rows(r, T), :], hss.at[rows(r, T), :]
        prev = [None] * links
        for n, o in enumerate(range(0, T, RG)):
            x1 = hv[o:o + RG, :] + sv[o:o + RG, :]
            st = _stats(x1, prev[n % links], early=True)
            zb[o // 2:(o + RG) // 2, :] = pack_ln(x1, st)
            prev[n % links] = st[1]

    def mm_w3(f0, parts=1):
        z = pltpu.bitcast(zb[...], bf16)
        return _gelu2(_dot_balanced(z, lambda a, b: w3p[(f0 + a) // 2:(f0 + b) // 2, :], FM - f0, parts, nt=True))

    def mm_w3_first():
        z = pltpu.bitcast(zb[...], bf16)
        return _gelu2(jnp.dot(z, pltpu.bitcast(w3n[...], bf16), preferred_element_type=f32))

    def mm_w3_tail():
        z = pltpu.bitcast(zb[...], bf16)
        w = pltpu.bitcast(w3p[FM // 2:F // 2, :], bf16)
        return _gelu2(jax.lax.dot_general(w, z, NT_DIMS, preferred_element_type=f32))

    def mm_w4(r, n, act, c0=0, c1=D):
        h = _dot_balanced(act, lambda a, b: w4p[:, c0 + a:c0 + b], c1 - c0, 1)
        x1 = h2s[rows(r, n), c0:c1] + hss[rows(r, n), c0:c1]
        base = x2s[rows(r, n), c0:c1] + mvec(4, n, c0, c1) * x1
        ob[rows(r, n), c0:c1] = (base + mvec(5, n, c0, c1) * h).astype(bf16)

    groups = list(range(0, P0 + P1, RG))

    wait([mod_copies[0], q_copies[0]])
    sa, ca, ga = mod_part(0, 1)
    modb[0] = ga * sa
    modb[1] = ga * (1.0 + ca)
    for c in range(NL, CT):
        mac_inv(c, NB - 1)
    st1 = {o: _stats(load_q(o)) for o in groups}
    zt[0:8, 0:128] = jnp.zeros((8, 128), u32)
    st2 = {}
    for o in groups:
        x2 = make_x2(o, load_q(o), st1[o])
        x2s[o:o + RG, :] = x2
        st2[o] = _stats(x2)

    wait([mod_copies[1]])
    sb, cb = mod_part(1, 2)
    modb[2] = sb
    modb[3] = 1.0 + cb
    st3 = {}
    for o in range(0, P0, RG):
        h2 = make_h2(x2s[o:o + RG, :], st2[o])
        h2s[o:o + RG, :] = h2
        st3[o] = _stats(h2)
    for o in range(0, P0, RG):
        zt[o // 2:(o + RG) // 2, :] = pack_ln(h2s[o:o + RG, :], st3[o])

    wait([w_copies[0]])
    w1p[...] = pltpu.bitcast(w1b[...], u32)
    mm_w1(0, P0)
    prev = None
    for o in range(P0, P0 + P1, RG):
        h2 = make_h2(x2s[o:o + RG, :], st2[o])
        h2s[o:o + RG, :] = h2
        st = _stats(h2, prev, early=True)
        zt[o // 2:(o + RG) // 2, :] = pack_ln(h2, st)
        prev = st[1]
    mm_w1(P0, P1, P0)

    wait([w_copies[1]])
    w2p[...] = pltpu.bitcast(w2b[...], u32)
    mm_w2(0)
    ln_x1(0, 2)
    mm_w2(T)

    wait([q_copies[1], w_copies[2]])
    w3p[...] = pltpu.bitcast(w3b[...], u32)
    ln_chain(P0 + P1, PA)
    main = mm_w3(0, 4)
    mm_w1(P0 + P1, PA)
    tail = mm_w3_tail()

    wait([w_copies[3], mod_copies[2]])
    w4p[...] = pltpu.bitcast(w4b[...], u32)
    w3n[...] = pltpu.bitcast(w3b[0:128, :].astype(f32).T.astype(bf16), u32)
    act = jnp.concatenate([main, tail.T], axis=-1).astype(bf16)
    sc16 = jnp.broadcast_to(scb[:, 0:D], (16, D)).astype(bf16)
    for c0 in range(0, D, 128):
        gb = jnp.dot(sc16, wmc[:, c0:c0 + 128], preferred_element_type=f32)[0:8]
        modb[4, :, c0:c0 + 128] = gb
        modb[5, :, c0:c0 + 128] = 0.5 * gb
        if c0 < D - 128:
            mm_w4(0, T, act, c0, c0 + 128)
        else:
            mm_w4(0, T // 2, act[0:T // 2], c0, c0 + 128)
            mm_w4(T // 2, T // 2, act[T // 2:T], c0, c0 + 128)
    ln_x1(T)
    out_copy(0).start()
    q_copies[2].wait()

    def mlp_body(i, carry):
        r1 = pl.multiple_of(PB - PC + PC * i, 32)
        r = pl.multiple_of(i * T, T)
        first = mm_w3_first()
        ln_chain(r1, PC)
        tail = mm_w3_tail()
        act = jnp.concatenate([first, mm_w3(128), tail.T], axis=-1).astype(bf16)
        mm_w4(r, T, act, 0, 128)
        mm_w1(r1, PC, parts=1)
        mm_w4(r, T, act, 128, 256)
        mm_w2(r + T, parts=1)
        ln_x1(r + T)
        mm_w4(r, T, act, 256, D)
        out_copy(i).start()
        return carry

    jax.lax.fori_loop(1, NC - 1, mlp_body, 0)

    first = mm_w3_first()
    tail = mm_w3_tail()
    act = jnp.concatenate([first, mm_w3(128), tail.T], axis=-1)
    mm_w4(S - T, LAST0, act[0:LAST0])
    out_tail[0].start()
    mm_w4(S - T + LAST0, T - LAST0, act[LAST0:T])
    out_tail[1].start()

    for i in range(NC - 1):
        out_copy(i).wait()
    for cp in out_tail:
        cp.wait()


@jax.jit
def pallas_adaLN_cond__ssm_conv_h3__mixer_s_mlp__prompt_kernel(
    A_q: jax.Array,
    A_k: jax.Array,
    A_v: jax.Array,
    A_shift_k: jax.Array,
    A_ssm_k: jax.Array,
    A_ssm_D: jax.Array,
    B_x: jax.Array,
    B_w1: jax.Array,
    B_w2: jax.Array,
    B_w3: jax.Array,
    B_w4: jax.Array,
    c: jax.Array,
    w_mod: jax.Array,
):
    del B_x
    any_spec = pl.BlockSpec(memory_space=pl.ANY)

    def tile_view(x):
        return x.reshape(S // 8, 8, CT, 128).transpose(0, 2, 1, 3).reshape(S * CT, 128)

    vm = pltpu.VMEM
    dma = pltpu.SemaphoreType.DMA
    spec = (4, NG, 16, 128)
    out = pl.pallas_call(
        _kernel,
        in_specs=[any_spec] * 12,
        out_specs=any_spec,
        out_shape=jax.ShapeDtypeStruct((S, D), bf16),
        scratch_shapes=[
            *[vm((KROWS, 128), bf16)] * NB, *[vm((VROWS, 128), bf16)] * NB, vm((CT, 128, S), bf16),
            vm((S, D), bf16), vm((D, D), bf16), vm((D, D), bf16), vm((F, D), bf16), vm((F, D), bf16),
            vm((D // 2, D), u32), vm((D // 2, D), u32), vm((F // 2, D), u32), vm((F // 2, D), u32),
            vm((D, 3 * D), bf16), vm((D, 2 * D), bf16), vm((D, D), bf16),
            vm((4, D), bf16), vm((D,), bf16), vm((1, D), bf16), vm((1, 1792), f32),
            vm((4, 128, 128), u32), vm((4, 128, 128), u32), vm((4, 64, 256), u32),
            vm((CT, 8, 8, 128), f32),
            vm((CT, NB) + spec, f32), vm((CT, NB - 1) + spec, f32), vm((CT,) + spec, f32),
            vm((CT, NB) + spec, f32), vm((4, 128, 128), f32),
            vm((CT, S + 32, 128), f32), vm((8, 8, D), f32),
            vm((CT, S + 32, 128), f32), vm((S, D), f32), vm((S, D), f32), vm((S, D), f32),
            vm((288, D), u32), vm((T // 2, D), u32), vm((D // 2, 128), u32),
            vm((S, D), bf16),
            dma((26,)), dma((NC + 1,)),
        ],
        compiler_params=pltpu.CompilerParams(vmem_limit_bytes=110 << 20, disable_bounds_checks=True,
                                             disable_semaphore_checks=True),
    )(A_q.reshape(S, D), tile_view(A_k), tile_view(A_v), A_shift_k.T, A_ssm_k,
      A_ssm_D, B_w1, B_w2, B_w3.T, B_w4, c, w_mod)
    return out.reshape(1, S, D)
```

```python
import numpy as np
import jax
import jax.numpy as jnp
import jax.experimental.pallas as pl
import jax.experimental.pallas.tpu as pltpu

f32, bf16, u32, i32 = jnp.float32, jnp.bfloat16, jnp.uint32, jnp.int32

S, D, F = 2048, 640, 1728
CT = D // 128
TR = 8 * CT
NB, BLK, NFFT = 4, 512, 1024
KROWS, VROWS = BLK * CT + 128, BLK * CT + 64
NG = 16
T = 256
NC = S // T
FM = (F // 128) * 128
P0, P1, PA, PC = 320, 208, 176, 224
PB = P0 + P1 + PA
LAST0 = 208
RG = 16
EPS = 1e-5
NT_DIMS = (((1,), (1,)), ((), ()))
GV = 8
NL = 4


def _lo(w):
    return pltpu.bitcast(w << 16, f32)


def _hi(w):
    return pltpu.bitcast(w & jnp.uint32(0xFFFF0000), f32)


def _cos_turn(n32, scale):
    x = (2.0 ** 30 - jnp.abs(n32.astype(f32))) * (2.0 * np.pi / 2.0 ** 32)
    x2 = x * x
    c = [scale * v for v in (1.0, -1.0 / 6, 1.0 / 120, -1.0 / 5040, 1.0 / 362880)]
    return x * (c[0] + x2 * (c[1] + x2 * (c[2] + x2 * (c[3] + x2 * c[4]))))


def _slot_phase(idx):
    k = ((idx >> 4) << 3) + (idx & 7)
    return jnp.where(k < 64, 4 * k + 1, 4 * k - 253) << 21, (idx & 8) << 27


def _fwd_table(r):
    fr, off = _slot_phase(jax.lax.broadcasted_iota(i32, (256, 128), 0))
    return pltpu.bitcast(_cos_turn(fr * r + off, 1.0).astype(bf16), u32)


def _inv_table(p):
    row = jax.lax.broadcasted_iota(i32, (128, 256), 0)
    fr, off = _slot_phase(jax.lax.broadcasted_iota(i32, (128, 256), 1))
    return pltpu.bitcast(_cos_turn(fr * (4 * row + p) + off, 2.0 / NFFT).astype(bf16), u32)


def _radix4(re, im, inverse):
    ar, ai = re[0] + re[2], im[0] + im[2]
    br, bi = re[0] - re[2], im[0] - im[2]
    cr, ci = re[1] + re[3], im[1] + im[3]
    dr, di = re[1] - re[3], im[1] - im[3]
    minus_i = (br + di, bi - dr)
    plus_i = (br - di, bi + dr)
    if inverse:
        return [(ar + cr, ai + ci), plus_i, (ar - cr, ai - ci), minus_i]
    return [(ar + cr, ai + ci), minus_i, (ar - cr, ai - ci), plus_i]


def _stats(x, link=None, early=False):
    zero = 0.0 if link is None else jnp.minimum(link, 0.0)
    part = x[:, 0:128]
    for c in range(1, CT):
        part = part + x[:, c * 128:(c + 1) * 128]
    if link is not None and early:
        part = part + zero
        zero = 0.0
    m = jnp.sum(part, axis=-1, keepdims=True) * (1.0 / D)
    v = jnp.maximum(jnp.sum(x * x, axis=-1, keepdims=True) * (1.0 / D) - m * m, zero)
    return m, jax.lax.rsqrt(v + EPS)


def _gelu2(x):
    c = 0.7978845608028654
    u = c + (c * 0.044715) * (x * x)
    return x + x * jnp.tanh(x * u)


def _gelu(x):
    c = 0.7978845608028654
    u = c + (c * 0.044715) * (x * x)
    hx = 0.5 * x
    return hx + hx * jnp.tanh(x * u)


def _dot_balanced(x, wslice, n_cols, parts, nt=False):
    def mm(a, c0, c1):
        a, w = a.astype(bf16), pltpu.bitcast(wslice(c0, c1), bf16)
        if nt:
            return jax.lax.dot_general(a, w, NT_DIMS, preferred_element_type=f32)
        return jnp.dot(a, w, preferred_element_type=f32)

    if parts == 1:
        return mm(x, 0, n_cols)
    base, extra = divmod(x.shape[0] // 16, parts)
    last, o = [], 0
    head = mm(x, 0, n_cols - 128)
    for i in range(parts):
        n = 16 * (base + (1 if i < extra else 0))
        last.append(mm(x[o:o + n], n_cols - 128, n_cols))
        o += n
    return jnp.concatenate([head, jnp.concatenate(last, axis=0)], axis=-1)


def _kernel(q_hbm, k_hbm, v_hbm, sh_hbm, sk_hbm, d_hbm, w1_hbm, w2_hbm, w3_hbm, w4_hbm,
            c_hbm, wm_hbm, o_hbm,
            kb0, kb1, kb2, kb3, vb0, vb1, vb2, vb3, skb, qb, w1b, w2b, w3b, w4b, w1p, w2p, w3p, w4p,
            wma, wmb, wmc, shb, db, cb_, scb,
            fub, fkb, gtb, par, US, KS, UR, YS, YP, ys, modb, h1s, h2s, x2s, hss, zt, zb, w3n, ob,
            sem, sem_o):
    n_in = [0]

    def load(src, dst):
        n_in[0] += 1
        return pltpu.make_async_copy(src, dst, sem.at[n_in[0] - 1])

    nkv = BLK * CT
    small = [load(d_hbm, db), load(sh_hbm, shb), load(c_hbm, cb_)]
    sk_copies = [load(sk_hbm.at[pl.ds(c * 128, 128), :], skb.at[c]) for c in range(CT)]
    kbs, vbs, wms = [kb0, kb1, kb2, kb3], [vb0, vb1, vb2, vb3], [wma, wmb, wmc]
    kv_copies = [[load(k_hbm.at[pl.ds(a * nkv, nkv), :], kbs[a].at[pl.ds(TR, nkv), :]),
                  load(v_hbm.at[pl.ds(a * nkv, nkv), :], vbs[a].at[pl.ds(0, nkv), :])] for a in range(NB)]
    mod_cols = [(0, 3 * D), (3 * D, 2 * D), (5 * D, D)]
    mod_copies = [load(wm_hbm.at[:, pl.ds(o, n)], w) for (o, n), w in zip(mod_cols, wms)]
    w_copies = [load(w1_hbm, w1b), load(w2_hbm, w2b), load(w3_hbm, w3b), load(w4_hbm, w4b)]
    q_copies = [load(q_hbm.at[pl.ds(o, n), :], qb.at[pl.ds(o, n), :])
                for o, n in [(0, P0 + P1), (P0 + P1, PA), (PB, S - PB)]]

    def out_copy(i):
        r = i * T if isinstance(i, int) else pl.multiple_of(i * T, T)
        return pltpu.make_async_copy(ob.at[pl.ds(r, T), :], o_hbm.at[pl.ds(r, T), :], sem_o.at[i])

    tail_parts = [(S - T, LAST0, 0, D), (S - T + LAST0, T - LAST0, 0, D - 128),
                  (S - T + LAST0, T - LAST0, D - 128, D)]
    out_tail = [pltpu.make_async_copy(ob.at[pl.ds(o, n), pl.ds(c0, c1 - c0)],
                                      o_hbm.at[pl.ds(o, n), pl.ds(c0, c1 - c0)], sem_o.at[NC - 1 + i])
                for i, (o, n, c0, c1) in enumerate(tail_parts)]

    for cp in (small + kv_copies[0] + sk_copies + kv_copies[1] + kv_copies[2] + kv_copies[3]
               + [mod_copies[0], q_copies[0], mod_copies[1], w_copies[0], w_copies[1], q_copies[1],
                  w_copies[2], w_copies[3], mod_copies[2], q_copies[2]]):
        cp.start()

    def wait(copies):
        for cp in copies:
            cp.wait()

    def pin(i, carry):
        z = jnp.zeros((8, 128), f32)
        scb[:, pl.ds(pl.multiple_of(i * 128, 128), 128)] = z[0:1]
        YP[i, 0:8, :] = z
        US[i, 0, 0, 0, 0:8, :] = z
        KS[i, 0, 0, 0, 0:8, :] = z
        YS[i, 0, 0, 0, 0:8, :] = z
        UR[i, 0, 0, 0:8, :] = z
        return carry

    def fence(i, carry):
        YP[i, 0:8, :] = jnp.zeros((8, 128), f32)
        return carry

    jax.lax.fori_loop(0, 2, pin, 0)
    lane = jax.lax.broadcasted_iota(i32, (256, 128), 1)
    for p in range(4):
        m = (lane - p) & 3
        fkb[p] = _fwd_table(128 * m + ((lane - m) & 127))
    for c in range(CT):
        kb0[c * 8:(c + 1) * 8, :] = jnp.zeros((8, 128), bf16)
        h1s[c, 0:8, :] = jnp.zeros((8, 128), f32)
        h1s[c, S + 8:S + 16, :] = jnp.zeros((8, 128), f32)
    for a in range(NB):
        kbs[a][nkv + TR:KROWS, :] = jnp.zeros((KROWS - nkv - TR, 128), bf16)
        vbs[a][nkv:VROWS, :] = jnp.zeros((VROWS - nkv, 128), bf16)
    for p in range(4):
        fub[p] = _fwd_table(8 * (lane & 63) + ((lane >> 6) << 2) + p)
    wait(small)
    cvec = cb_[...].astype(f32)
    scb[:, 0:D] = cvec * jax.nn.sigmoid(cvec)
    dv = db[...].astype(f32).reshape(1, D)
    shv = shb[...].astype(f32)
    for c in range(CT):
        for i in range(4):
            par[c, i] = jnp.broadcast_to(shv[i:i + 1, c * 128:(c + 1) * 128], (8, 128))
        par[c, 4] = jnp.broadcast_to(dv[:, c * 128:(c + 1) * 128], (8, 128))
    for p in range(4):
        gtb[p] = _inv_table(p)

    def get(ref, idx, g, n):
        return (ref[idx + (slice(g, g + n), slice(0, 8))], ref[idx + (slice(g, g + n), slice(8, 16))])

    def put(ref, idx, g, n, xr, xi):
        ref[idx + (slice(g, g + n), slice(0, 8))] = xr
        ref[idx + (slice(g, g + n), slice(8, 16))] = xi

    def split(tt, g, n):
        tt = [t[g * 16:(g + n) * 16].reshape(n, 16, 128) for t in tt]
        return [t[:, 0:8] for t in tt], [t[:, 8:16] for t in tt]

    def fwd_k(c, j):
        lane = jax.lax.broadcasted_iota(i32, (64, 128), 1)
        even = (lane & 1) == 0
        l01 = (lane & 2) == 0
        l12 = ((lane + 3) & 2) == 0
        rm = []
        for m in range(4):
            w = pltpu.bitcast(skb[c, :, (4 * j + m) * 128:(4 * j + m + 1) * 128], u32)
            rm.append(pltpu.roll(w, m, 1) if m else w)
        e01 = jnp.where(even, rm[0], rm[1])
        o01 = jnp.where(even, rm[1], rm[0])
        e23 = jnp.where(even, rm[2], rm[3])
        o23 = jnp.where(even, rm[3], rm[2])
        kp = [jnp.where(l01, e01, e23), jnp.where(l12, o01, o23),
              jnp.where(l01, e23, e01), jnp.where(l12, o23, o01)]
        tt = [jax.lax.dot_general(pltpu.bitcast(fkb[p], bf16), pltpu.bitcast(kp[p], bf16), NT_DIMS,
                                  preferred_element_type=f32) for p in range(4)]
        for g in range(0, NG, GV):
            re, im = split(tt, g, GV)
            if j == 0:
                re[0] = re[0] + par[c, 4][None]
            for m, (xr, xi) in enumerate(_radix4(re, im, False)):
                if j < NB - 1:
                    put(KS, (c, j, m), g, GV, xr, xi)
                ur, ui = get(US, (c, 0, m), g, GV)
                put(YS, (c, j, m), g, GV, xr * ur - xi * ui, xr * ui + xi * ur)

    def fwd_u(c, a):
        taps = [jnp.tile(par[c, i], (8, 1)) for i in range(4)]
        ws = TR // 2
        base = 4 * c
        kw, vw = kbs[a].bitcast(u32), vbs[a].bitcast(u32)

        def words(ref, start):
            return ref[pl.ds(start, BLK // 8, stride=ws), :]

        kk = {}
        for w in range(4):
            x = words(kw, ws + base + w)
            kk[2 * w], kk[2 * w + 1] = _lo(x), _hi(x)
        kk[-3] = _hi(words(kw, base + 2))
        x = words(kw, base + 3)
        kk[-2], kk[-1] = _lo(x), _hi(x)
        sub = []
        for w in range(4):
            x = words(vw, base + w)
            for r, vv in ((2 * w, _lo(x)), (2 * w + 1, _hi(x))):
                sh = taps[0] * kk[r] + taps[1] * kk[r - 1] + taps[2] * kk[r - 2] + taps[3] * kk[r - 3]
                sub.append(sh * vv)
        kv = [jnp.concatenate([sub[p], sub[p + 4]], axis=0) for p in range(4)]
        tt = [jnp.dot(pltpu.bitcast(fub[p], bf16), kv[p].astype(bf16), preferred_element_type=f32)
              for p in range(4)]
        for g in range(0, NG, GV):
            re, im = split(tt, g, GV)
            for m, (xr, xi) in enumerate(_radix4(re, im, False)):
                if a:
                    pr, pi = get(US, (c, 0, m), g, GV) if a == 1 else get(UR, (c, m), g, GV)
                    if a < NB - 1:
                        put(UR, (c, m), g, GV, xr, xi)
                    xr, xi = (xr - pi, xi + pr) if g < NG // 2 else (xr + pi, xi - pr)
                put(US, (c, a, m), g, GV, xr, xi)

    def mac_inv(c, a):
        for h in range(2):
            vals = [[] for _ in range(4)]
            for g in range(8 * h, 8 * h + 8, GV):
                yre, yim = [], []
                for m in range(4):
                    yr, yi = get(YS, (c, a, m), g, GV)
                    for j in range(a):
                        kr, ki = get(KS, (c, j, m), g, GV)
                        ur, ui = get(US, (c, a - j, m), g, GV)
                        yr = yr + (kr * ur - ki * ui)
                        yi = yi + (kr * ui + ki * ur)
                    yre.append(yr)
                    yim.append(yi)
                for p, (pr, pi) in enumerate(_radix4(yre, yim, True)):
                    vals[p].append(jnp.concatenate([pr, pi], axis=1))
            for p in range(4):
                pb = jnp.concatenate(vals[p], axis=0).reshape(128, 128).astype(bf16)
                r = jnp.dot(pltpu.bitcast(gtb[p, :, h * 128:(h + 1) * 128], bf16), pb,
                            preferred_element_type=f32)
                if h == 0:
                    YP[p] = r
                else:
                    ys[c, pl.ds(a * BLK + p, 128, stride=4), :] = YP[p] + r

    wait(kv_copies[0])
    for c in range(CT):
        fwd_u(c, 0)

    for grp in ((0,), (1, 2), (3, 4)):
        wait([sk_copies[c] for c in grp])
        for c in grp:
            for j in (3, 2, 1, 0):
                fwd_k(c, j)
    for a in range(1, NB):
        wait(kv_copies[a])
        for c in range(CT):
            kbs[a][c * 8:(c + 1) * 8, :] = kbs[a - 1][nkv + c * 8:nkv + (c + 1) * 8, :]
        for c in range(CT):
            fwd_u(c, a)
            mac_inv(c, a - 1)

    jax.lax.fori_loop(0, 2, fence, 0)
    for c in range(NL):
        mac_inv(c, NB - 1)

    def mod_part(part, extra):
        n, wm = mod_cols[part][1], wms[part]
        act = scb[:, 0:D]

        def sc(k0, k1):
            return jnp.broadcast_to(act[:, k0:k1], (16, k1 - k0)).astype(bf16)

        e = 128 * extra
        r = jnp.dot(sc(0, D), wm[:, e:n], preferred_element_type=f32)
        r0 = (jnp.dot(sc(0, D - 64), wm[0:D - 64, 0:e], preferred_element_type=f32)
              + jnp.dot(sc(D - 64, D), wm[D - 64:D, 0:e], preferred_element_type=f32))
        r = jnp.concatenate([r0, r], axis=-1)[0:8]
        return [r[:, i * D:(i + 1) * D] for i in range(n // D)]

    def mvec(i, n=RG, c0=0, c1=D):
        return jnp.tile(modb[i, :, c0:c1], (n // 8, 1))

    rows = pl.ds

    def load_q(r, ref=qb):
        return ref[rows(r, RG), :].astype(f32)

    def make_x2(r, q, st, ref=ys):
        y = jnp.concatenate([ref[c, rows(r, RG), :] for c in range(CT)], axis=-1)
        return q + (((q - st[0]) * st[1]) * mvec(1) + mvec(0)) * y

    def make_h2(x2, st):
        return ((x2 - st[0]) * st[1]) * mvec(3) + mvec(2)

    def pack_ln(x, st):
        return pltpu.bitcast(((x - st[0]) * st[1]).astype(bf16), u32)

    def ln_chain(r, n):
        qv, yv = qb.at[rows(r, n), :], ys.at[:, rows(r, n), :]
        xv, hv = x2s.at[rows(r, n), :], h2s.at[rows(r, n), :]
        prev = None
        for o in range(0, n, RG):
            q = load_q(o, qv)
            x2 = make_x2(o, q, _stats(q, prev), yv)
            xv[o:o + RG, :] = x2
            st = _stats(x2)
            h2 = make_h2(xv[o:o + RG, :], st)
            hv[o:o + RG, :] = h2
            st = _stats(h2)
            zt[o // 2:(o + RG) // 2, :] = pack_ln(hv[o:o + RG, :], st)
            prev = st[1]

    def mm_w1(r, n, o=0, parts=4):
        z = pltpu.bitcast(zt[o // 2:(o + n) // 2, :], bf16)
        h1 = _gelu(_dot_balanced(z, lambda a, b: w1p[:, a:b], D, parts))
        for c in range(CT):
            h1s[c, rows(r + 8, n), :] = h1[:, c * 128:(c + 1) * 128]

    def mm_w2(r, parts=4):
        lane = jax.lax.broadcasted_iota(i32, (T, 128), 1)

        def sh(k, c):
            return h1s[c, rows(r + 8 + k, T), :]

        g = jnp.concatenate([
            sh(-1, 0),
            jnp.where(lane < 32, sh(-1, 1), sh(1, 1)),
            jnp.where(lane < 64, sh(1, 2), sh(-2, 2)),
            jnp.where(lane < 96, sh(-2, 3), sh(2, 3)),
            sh(2, 4)], axis=-1)
        hss[rows(r, T), :] = _dot_balanced(g, lambda a, b: w2p[:, a:b], D, parts)

    def ln_x1(r, links=1):
        hv, sv = h2s.at[rows(r, T), :], hss.at[rows(r, T), :]
        prev = [None] * links
        for n, o in enumerate(range(0, T, RG)):
            x1 = hv[o:o + RG, :] + sv[o:o + RG, :]
            st = _stats(x1, prev[n % links], early=True)
            zb[o // 2:(o + RG) // 2, :] = pack_ln(x1, st)
            prev[n % links] = st[1]

    def mm_w3(f0, parts=1):
        z = pltpu.bitcast(zb[...], bf16)
        return _gelu2(_dot_balanced(z, lambda a, b: w3p[(f0 + a) // 2:(f0 + b) // 2, :], FM - f0, parts, nt=True))

    def mm_w3_first():
        z = pltpu.bitcast(zb[...], bf16)
        return _gelu2(jnp.dot(z, pltpu.bitcast(w3n[...], bf16), preferred_element_type=f32))

    def mm_w3_tail():
        z = pltpu.bitcast(zb[...], bf16)
        w = pltpu.bitcast(w3p[FM // 2:F // 2, :], bf16)
        return _gelu2(jax.lax.dot_general(w, z, NT_DIMS, preferred_element_type=f32))

    def mm_w4(r, n, act, c0=0, c1=D):
        h = _dot_balanced(act, lambda a, b: w4p[:, c0 + a:c0 + b], c1 - c0, 1)
        x1 = h2s[rows(r, n), c0:c1] + hss[rows(r, n), c0:c1]
        base = x2s[rows(r, n), c0:c1] + mvec(4, n, c0, c1) * x1
        ob[rows(r, n), c0:c1] = (base + mvec(5, n, c0, c1) * h).astype(bf16)

    groups = list(range(0, P0 + P1, RG))

    wait([mod_copies[0], q_copies[0]])
    sa, ca, ga = mod_part(0, 1)
    modb[0] = ga * sa
    modb[1] = ga * (1.0 + ca)
    for c in range(NL, CT):
        mac_inv(c, NB - 1)
    st1 = {o: _stats(load_q(o)) for o in groups}
    zt[0:8, 0:128] = jnp.zeros((8, 128), u32)
    st2 = {}
    for o in groups:
        x2 = make_x2(o, load_q(o), st1[o])
        x2s[o:o + RG, :] = x2
        st2[o] = _stats(x2)

    wait([mod_copies[1]])
    sb, cb = mod_part(1, 2)
    modb[2] = sb
    modb[3] = 1.0 + cb
    st3 = {}
    for o in range(0, P0, RG):
        h2 = make_h2(x2s[o:o + RG, :], st2[o])
        h2s[o:o + RG, :] = h2
        st3[o] = _stats(h2)
    for o in range(0, P0, RG):
        zt[o // 2:(o + RG) // 2, :] = pack_ln(h2s[o:o + RG, :], st3[o])

    wait([w_copies[0]])
    w1p[...] = pltpu.bitcast(w1b[...], u32)
    mm_w1(0, P0)
    prev = None
    for o in range(P0, P0 + P1, RG):
        h2 = make_h2(x2s[o:o + RG, :], st2[o])
        h2s[o:o + RG, :] = h2
        st = _stats(h2, prev, early=True)
        zt[o // 2:(o + RG) // 2, :] = pack_ln(h2, st)
        prev = st[1]
    mm_w1(P0, P1, P0)

    wait([w_copies[1]])
    w2p[...] = pltpu.bitcast(w2b[...], u32)
    mm_w2(0)
    ln_x1(0, 2)
    mm_w2(T)

    wait([q_copies[1], w_copies[2]])
    w3p[...] = pltpu.bitcast(w3b[...], u32)
    ln_chain(P0 + P1, PA)
    main = mm_w3(0, 4)
    mm_w1(P0 + P1, PA)
    tail = mm_w3_tail()

    wait([w_copies[3], mod_copies[2]])
    w4p[...] = pltpu.bitcast(w4b[...], u32)
    w3n[...] = pltpu.bitcast(w3b[0:128, :].astype(f32).T.astype(bf16), u32)
    act = jnp.concatenate([main, tail.T], axis=-1).astype(bf16)
    sc16 = jnp.broadcast_to(scb[:, 0:D], (16, D)).astype(bf16)
    for c0 in range(0, D, 128):
        gb = jnp.dot(sc16, wmc[:, c0:c0 + 128], preferred_element_type=f32)[0:8]
        modb[4, :, c0:c0 + 128] = gb
        modb[5, :, c0:c0 + 128] = 0.5 * gb
        if c0 < D - 128:
            mm_w4(0, T, act, c0, c0 + 128)
        else:
            mm_w4(0, T // 2, act[0:T // 2], c0, c0 + 128)
            mm_w4(T // 2, T // 2, act[T // 2:T], c0, c0 + 128)
    ln_x1(T)
    out_copy(0).start()
    q_copies[2].wait()

    def mlp_body(i, carry):
        r1 = pl.multiple_of(PB - PC + PC * i, 32)
        r = pl.multiple_of(i * T, T)
        first = mm_w3_first()
        ln_chain(r1, PC)
        tail = mm_w3_tail()
        act = jnp.concatenate([first, mm_w3(128), tail.T], axis=-1).astype(bf16)
        mm_w4(r, T, act, 0, 128)
        mm_w1(r1, PC, parts=1)
        mm_w4(r, T, act, 128, 256)
        mm_w2(r + T, parts=1)
        ln_x1(r + T)
        mm_w4(r, T, act, 256, D)
        out_copy(i).start()
        return carry

    jax.lax.fori_loop(1, NC - 1, mlp_body, 0)

    first = mm_w3_first()
    tail = mm_w3_tail()
    act = jnp.concatenate([first, mm_w3(128), tail.T], axis=-1)
    for cp, (o, n, c0, c1) in zip(out_tail, tail_parts):
        mm_w4(o, n, act[o - (S - T):o - (S - T) + n], c0, c1)
        cp.start()

    for i in range(NC - 1):
        out_copy(i).wait()
    for cp in out_tail:
        cp.wait()


@jax.jit
def pallas_adaLN_cond__ssm_conv_h3__mixer_s_mlp__prompt_kernel(
    A_q: jax.Array,
    A_k: jax.Array,
    A_v: jax.Array,
    A_shift_k: jax.Array,
    A_ssm_k: jax.Array,
    A_ssm_D: jax.Array,
    B_x: jax.Array,
    B_w1: jax.Array,
    B_w2: jax.Array,
    B_w3: jax.Array,
    B_w4: jax.Array,
    c: jax.Array,
    w_mod: jax.Array,
):
    del B_x
    any_spec = pl.BlockSpec(memory_space=pl.ANY)

    def tile_view(x):
        return x.reshape(S // 8, 8, CT, 128).transpose(0, 2, 1, 3).reshape(S * CT, 128)

    vm = pltpu.VMEM
    dma = pltpu.SemaphoreType.DMA
    spec = (4, NG, 16, 128)
    out = pl.pallas_call(
        _kernel,
        in_specs=[any_spec] * 12,
        out_specs=any_spec,
        out_shape=jax.ShapeDtypeStruct((S, D), bf16),
        scratch_shapes=[
            *[vm((KROWS, 128), bf16)] * NB, *[vm((VROWS, 128), bf16)] * NB, vm((CT, 128, S), bf16),
            vm((S, D), bf16), vm((D, D), bf16), vm((D, D), bf16), vm((F, D), bf16), vm((F, D), bf16),
            vm((D // 2, D), u32), vm((D // 2, D), u32), vm((F // 2, D), u32), vm((F // 2, D), u32),
            vm((D, 3 * D), bf16), vm((D, 2 * D), bf16), vm((D, D), bf16),
            vm((4, D), bf16), vm((D,), bf16), vm((1, D), bf16), vm((1, 1792), f32),
            vm((4, 128, 128), u32), vm((4, 128, 128), u32), vm((4, 64, 256), u32),
            vm((CT, 8, 8, 128), f32),
            vm((CT, NB) + spec, f32), vm((CT, NB - 1) + spec, f32), vm((CT,) + spec, f32),
            vm((CT, NB) + spec, f32), vm((4, 128, 128), f32),
            vm((CT, S + 32, 128), f32), vm((8, 8, D), f32),
            vm((CT, S + 32, 128), f32), vm((S, D), f32), vm((S, D), f32), vm((S, D), f32),
            vm((288, D), u32), vm((T // 2, D), u32), vm((D // 2, 128), u32),
            vm((S, D), bf16),
            dma((26,)), dma((NC + 2,)),
        ],
        compiler_params=pltpu.CompilerParams(vmem_limit_bytes=110 << 20, disable_bounds_checks=True,
                                             disable_semaphore_checks=True),
    )(A_q.reshape(S, D), tile_view(A_k), tile_view(A_v), A_shift_k.T, A_ssm_k,
      A_ssm_D, B_w1, B_w2, B_w3.T, B_w4, c, w_mod)
    return out.reshape(1, S, D)
```

```python
import numpy as np
import jax
import jax.numpy as jnp
import jax.experimental.pallas as pl
import jax.experimental.pallas.tpu as pltpu

f32, bf16, u32, i32 = jnp.float32, jnp.bfloat16, jnp.uint32, jnp.int32

S, D, F = 2048, 640, 1728
CT = D // 128
TR = 8 * CT
NB, BLK, NFFT = 4, 512, 1024
KROWS, VROWS = BLK * CT + 128, BLK * CT + 64
NG = 16
T = 256
NC = S // T
FM = (F // 128) * 128
P0, P1, PA, PC = 320, 208, 176, 224
PB = P0 + P1 + PA
LAST0 = 208
RG = 16
EPS = 1e-5
NT_DIMS = (((1,), (1,)), ((), ()))
GV = 8
NL = 4


def _lo(w):
    return pltpu.bitcast(w << 16, f32)


def _hi(w):
    return pltpu.bitcast(w & jnp.uint32(0xFFFF0000), f32)


def _cis(n):
    t = (n & (2 * NFFT - 1)).astype(f32) * (np.pi / NFFT)
    return jnp.cos(t), jnp.sin(t)


def _fwd_table(r):
    g = jax.lax.broadcasted_iota(i32, (NG, 128), 0)
    cg, sg = _cis(jnp.where(g < NG // 2, 32 * g + 1, 32 * g - 253) * r)
    cs, ss = _cis(4 * jax.lax.broadcasted_iota(i32, (8, 128), 0) * r)
    parts = []
    for i in range(NG):
        c, s = cg[i:i + 1], sg[i:i + 1]
        parts += [c * cs - s * ss, -(s * cs + c * ss)]
    return pltpu.bitcast(jnp.concatenate(parts, axis=0).astype(bf16), u32)


def _inv_tables():
    def phase(rows):
        col = jax.lax.broadcasted_iota(i32, (rows, 256), 1)
        k = ((col >> 4) << 3) + (col & 7)
        row = jax.lax.broadcasted_iota(i32, (rows, 256), 0)
        return jnp.where(k < 64, 4 * k + 1, 4 * k - 253), (col & 8) << 6, row

    fr, _, g = phase(16)
    cg, sg = _cis(fr * (32 * g))
    fr, off, s = phase(8)
    out = []
    for p in range(4):
        cs, ss = _cis(fr * (4 * s + p) + off)
        cs, ss = cs * (2.0 / NFFT), ss * (2.0 / NFFT)
        parts = [cg[i:i + 1] * cs - sg[i:i + 1] * ss for i in range(16)]
        out.append(pltpu.bitcast(jnp.concatenate(parts, axis=0).astype(bf16), u32))
    return out


def _radix4(re, im, inverse):
    ar, ai = re[0] + re[2], im[0] + im[2]
    br, bi = re[0] - re[2], im[0] - im[2]
    cr, ci = re[1] + re[3], im[1] + im[3]
    dr, di = re[1] - re[3], im[1] - im[3]
    minus_i = (br + di, bi - dr)
    plus_i = (br - di, bi + dr)
    if inverse:
        return [(ar + cr, ai + ci), plus_i, (ar - cr, ai - ci), minus_i]
    return [(ar + cr, ai + ci), minus_i, (ar - cr, ai - ci), plus_i]


def _stats(x, link=None, early=False):
    zero = 0.0 if link is None else jnp.minimum(link, 0.0)
    part = x[:, 0:128]
    for c in range(1, CT):
        part = part + x[:, c * 128:(c + 1) * 128]
    if link is not None and early:
        part = part + zero
        zero = 0.0
    m = jnp.sum(part, axis=-1, keepdims=True) * (1.0 / D)
    v = jnp.maximum(jnp.sum(x * x, axis=-1, keepdims=True) * (1.0 / D) - m * m, zero)
    return m, jax.lax.rsqrt(v + EPS)


def _gelu2(x):
    c = 0.7978845608028654
    u = c + (c * 0.044715) * (x * x)
    return x + x * jnp.tanh(x * u)


def _gelu(x):
    c = 0.7978845608028654
    u = c + (c * 0.044715) * (x * x)
    hx = 0.5 * x
    return hx + hx * jnp.tanh(x * u)


def _dot_balanced(x, wslice, n_cols, parts, nt=False):
    def mm(a, c0, c1):
        a, w = a.astype(bf16), pltpu.bitcast(wslice(c0, c1), bf16)
        if nt:
            return jax.lax.dot_general(a, w, NT_DIMS, preferred_element_type=f32)
        return jnp.dot(a, w, preferred_element_type=f32)

    if parts == 1:
        return mm(x, 0, n_cols)
    base, extra = divmod(x.shape[0] // 16, parts)
    last, o = [], 0
    head = mm(x, 0, n_cols - 128)
    for i in range(parts):
        n = 16 * (base + (1 if i < extra else 0))
        last.append(mm(x[o:o + n], n_cols - 128, n_cols))
        o += n
    return jnp.concatenate([head, jnp.concatenate(last, axis=0)], axis=-1)


def _kernel(q_hbm, k_hbm, v_hbm, sh_hbm, sk_hbm, d_hbm, w1_hbm, w2_hbm, w3_hbm, w4_hbm,
            c_hbm, wm_hbm, o_hbm,
            kb0, kb1, kb2, kb3, vb0, vb1, vb2, vb3, skb, qb, w1b, w2b, w3b, w4b, w1p, w2p, w3p, w4p,
            wma, wmb, wmc, shb, db, cb_, scb,
            fub, fkb, gtb, par, US, KS, UR, YS, YP, ys, modb, h1s, h2s, x2s, hss, zt, zb, w3n, ob,
            sem, sem_o):
    n_in = [0]

    def load(src, dst):
        n_in[0] += 1
        return pltpu.make_async_copy(src, dst, sem.at[n_in[0] - 1])

    nkv = BLK * CT
    small = [load(d_hbm, db), load(sh_hbm, shb), load(c_hbm, cb_)]
    sk_copies = [load(sk_hbm.at[pl.ds(c * 128, 128), :], skb.at[c]) for c in range(CT)]
    kbs, vbs, wms = [kb0, kb1, kb2, kb3], [vb0, vb1, vb2, vb3], [wma, wmb, wmc]
    kv_copies = [[load(k_hbm.at[pl.ds(a * nkv, nkv), :], kbs[a].at[pl.ds(TR, nkv), :]),
                  load(v_hbm.at[pl.ds(a * nkv, nkv), :], vbs[a].at[pl.ds(0, nkv), :])] for a in range(NB)]
    mod_cols = [(0, 3 * D), (3 * D, 2 * D), (5 * D, D)]
    mod_copies = [load(wm_hbm.at[:, pl.ds(o, n)], w) for (o, n), w in zip(mod_cols, wms)]
    w_copies = [load(w1_hbm, w1b), load(w2_hbm, w2b), load(w3_hbm, w3b), load(w4_hbm, w4b)]
    q_copies = [load(q_hbm.at[pl.ds(o, n), :], qb.at[pl.ds(o, n), :])
                for o, n in [(0, P0 + P1), (P0 + P1, PA), (PB, S - PB)]]

    def out_copy(i):
        r = i * T if isinstance(i, int) else pl.multiple_of(i * T, T)
        return pltpu.make_async_copy(ob.at[pl.ds(r, T), :], o_hbm.at[pl.ds(r, T), :], sem_o.at[i])

    tail_parts = [(S - T, LAST0, 0, D), (S - T + LAST0, T - LAST0, 0, D - 128),
                  (S - T + LAST0, T - LAST0, D - 128, D)]
    out_tail = [pltpu.make_async_copy(ob.at[pl.ds(o, n), pl.ds(c0, c1 - c0)],
                                      o_hbm.at[pl.ds(o, n), pl.ds(c0, c1 - c0)], sem_o.at[NC - 1 + i])
                for i, (o, n, c0, c1) in enumerate(tail_parts)]

    for cp in (small + kv_copies[0] + sk_copies + kv_copies[1] + kv_copies[2] + kv_copies[3]
               + [mod_copies[0], q_copies[0], mod_copies[1], w_copies[0], w_copies[1], q_copies[1],
                  w_copies[2], w_copies[3], mod_copies[2], q_copies[2]]):
        cp.start()

    def wait(copies):
        for cp in copies:
            cp.wait()

    def pin(i, carry):
        z = jnp.zeros((8, 128), f32)
        scb[:, pl.ds(pl.multiple_of(i * 128, 128), 128)] = z[0:1]
        YP[i, 0:8, :] = z
        US[i, 0, 0, 0, 0:8, :] = z
        KS[i, 0, 0, 0, 0:8, :] = z
        YS[i, 0, 0, 0, 0:8, :] = z
        UR[i, 0, 0, 0:8, :] = z
        return carry

    def fence(i, carry):
        YP[i, 0:8, :] = jnp.zeros((8, 128), f32)
        return carry

    jax.lax.fori_loop(0, 2, pin, 0)
    lane = jax.lax.broadcasted_iota(i32, (1, 128), 1)
    for p in range(4):
        m = (lane - p) & 3
        fkb[p] = _fwd_table(128 * m + ((lane - m) & 127))
    for c in range(CT):
        kb0[c * 8:(c + 1) * 8, :] = jnp.zeros((8, 128), bf16)
        h1s[c, 0:8, :] = jnp.zeros((8, 128), f32)
        h1s[c, S + 8:S + 16, :] = jnp.zeros((8, 128), f32)
    for a in range(NB):
        kbs[a][nkv + TR:KROWS, :] = jnp.zeros((KROWS - nkv - TR, 128), bf16)
        vbs[a][nkv:VROWS, :] = jnp.zeros((VROWS - nkv, 128), bf16)
    for p in range(4):
        fub[p] = _fwd_table(8 * (lane & 63) + ((lane >> 6) << 2) + p)
    wait(small)
    cvec = cb_[...].astype(f32)
    scb[:, 0:D] = cvec * jax.nn.sigmoid(cvec)
    dv = db[...].astype(f32).reshape(1, D)
    shv = shb[...].astype(f32)
    for c in range(CT):
        for i in range(4):
            par[c, i] = jnp.broadcast_to(shv[i:i + 1, c * 128:(c + 1) * 128], (8, 128))
        par[c, 4] = jnp.broadcast_to(dv[:, c * 128:(c + 1) * 128], (8, 128))
    for p, tab in enumerate(_inv_tables()):
        gtb[p] = tab

    def get(ref, idx, g, n):
        return (ref[idx + (slice(g, g + n), slice(0, 8))], ref[idx + (slice(g, g + n), slice(8, 16))])

    def put(ref, idx, g, n, xr, xi):
        ref[idx + (slice(g, g + n), slice(0, 8))] = xr
        ref[idx + (slice(g, g + n), slice(8, 16))] = xi

    def split(tt, g, n):
        tt = [t[g * 16:(g + n) * 16].reshape(n, 16, 128) for t in tt]
        return [t[:, 0:8] for t in tt], [t[:, 8:16] for t in tt]

    def fwd_k(c, j):
        lane = jax.lax.broadcasted_iota(i32, (64, 128), 1)
        even = (lane & 1) == 0
        l01 = (lane & 2) == 0
        l12 = ((lane + 3) & 2) == 0
        rm = []
        for m in range(4):
            w = pltpu.bitcast(skb[c, :, (4 * j + m) * 128:(4 * j + m + 1) * 128], u32)
            rm.append(pltpu.roll(w, m, 1) if m else w)
        e01 = jnp.where(even, rm[0], rm[1])
        o01 = jnp.where(even, rm[1], rm[0])
        e23 = jnp.where(even, rm[2], rm[3])
        o23 = jnp.where(even, rm[3], rm[2])
        kp = [jnp.where(l01, e01, e23), jnp.where(l12, o01, o23),
              jnp.where(l01, e23, e01), jnp.where(l12, o23, o01)]
        tt = [jax.lax.dot_general(pltpu.bitcast(fkb[p], bf16), pltpu.bitcast(kp[p], bf16), NT_DIMS,
                                  preferred_element_type=f32) for p in range(4)]
        for g in range(0, NG, GV):
            re, im = split(tt, g, GV)
            if j == 0:
                re[0] = re[0] + par[c, 4][None]
            for m, (xr, xi) in enumerate(_radix4(re, im, False)):
                if j < NB - 1:
                    put(KS, (c, j, m), g, GV, xr, xi)
                ur, ui = get(US, (c, 0, m), g, GV)
                put(YS, (c, j, m), g, GV, xr * ur - xi * ui, xr * ui + xi * ur)

    def fwd_u(c, a):
        taps = [jnp.tile(par[c, i], (8, 1)) for i in range(4)]
        ws = TR // 2
        base = 4 * c
        kw, vw = kbs[a].bitcast(u32), vbs[a].bitcast(u32)

        def words(ref, start):
            return ref[pl.ds(start, BLK // 8, stride=ws), :]

        kk = {}
        for w in range(4):
            x = words(kw, ws + base + w)
            kk[2 * w], kk[2 * w + 1] = _lo(x), _hi(x)
        kk[-3] = _hi(words(kw, base + 2))
        x = words(kw, base + 3)
        kk[-2], kk[-1] = _lo(x), _hi(x)
        sub = []
        for w in range(4):
            x = words(vw, base + w)
            for r, vv in ((2 * w, _lo(x)), (2 * w + 1, _hi(x))):
                sh = taps[0] * kk[r] + taps[1] * kk[r - 1] + taps[2] * kk[r - 2] + taps[3] * kk[r - 3]
                sub.append(sh * vv)
        kv = [jnp.concatenate([sub[p], sub[p + 4]], axis=0) for p in range(4)]
        tt = [jnp.dot(pltpu.bitcast(fub[p], bf16), kv[p].astype(bf16), preferred_element_type=f32)
              for p in range(4)]
        for g in range(0, NG, GV):
            re, im = split(tt, g, GV)
            for m, (xr, xi) in enumerate(_radix4(re, im, False)):
                if a:
                    pr, pi = get(US, (c, 0, m), g, GV) if a == 1 else get(UR, (c, m), g, GV)
                    if a < NB - 1:
                        put(UR, (c, m), g, GV, xr, xi)
                    xr, xi = (xr - pi, xi + pr) if g < NG // 2 else (xr + pi, xi - pr)
                put(US, (c, a, m), g, GV, xr, xi)

    def mac_inv(c, a):
        for h in range(2):
            vals = [[] for _ in range(4)]
            for g in range(8 * h, 8 * h + 8, GV):
                yre, yim = [], []
                for m in range(4):
                    yr, yi = get(YS, (c, a, m), g, GV)
                    for j in range(a):
                        kr, ki = get(KS, (c, j, m), g, GV)
                        ur, ui = get(US, (c, a - j, m), g, GV)
                        yr = yr + (kr * ur - ki * ui)
                        yi = yi + (kr * ui + ki * ur)
                    yre.append(yr)
                    yim.append(yi)
                for p, (pr, pi) in enumerate(_radix4(yre, yim, True)):
                    vals[p].append(jnp.concatenate([pr, pi], axis=1))
            for p in range(4):
                pb = jnp.concatenate(vals[p], axis=0).reshape(128, 128).astype(bf16)
                r = jnp.dot(pltpu.bitcast(gtb[p, :, h * 128:(h + 1) * 128], bf16), pb,
                            preferred_element_type=f32)
                if h == 0:
                    YP[p] = r
                else:
                    ys[c, pl.ds(a * BLK + p, 128, stride=4), :] = YP[p] + r

    wait(kv_copies[0])
    for c in range(CT):
        fwd_u(c, 0)
    for grp in ((0,), (1, 2), (3, 4)):
        wait([sk_copies[c] for c in grp])
        for c in grp:
            for j in (3, 2, 1, 0):
                fwd_k(c, j)
    for a in range(1, NB):
        wait(kv_copies[a])
        for c in range(CT):
            kbs[a][c * 8:(c + 1) * 8, :] = kbs[a - 1][nkv + c * 8:nkv + (c + 1) * 8, :]
        for c in range(CT):
            fwd_u(c, a)
            mac_inv(c, a - 1)
    jax.lax.fori_loop(0, 2, fence, 0)
    for c in range(NL):
        mac_inv(c, NB - 1)

    def mod_part(part, extra):
        n, wm = mod_cols[part][1], wms[part]
        act = scb[:, 0:D]

        def sc(k0, k1):
            return jnp.broadcast_to(act[:, k0:k1], (16, k1 - k0)).astype(bf16)

        e = 128 * extra
        r = jnp.dot(sc(0, D), wm[:, e:n], preferred_element_type=f32)
        r0 = (jnp.dot(sc(0, D - 64), wm[0:D - 64, 0:e], preferred_element_type=f32)
              + jnp.dot(sc(D - 64, D), wm[D - 64:D, 0:e], preferred_element_type=f32))
        r = jnp.concatenate([r0, r], axis=-1)[0:8]
        return [r[:, i * D:(i + 1) * D] for i in range(n // D)]

    def mvec(i, n=RG, c0=0, c1=D):
        return jnp.tile(modb[i, :, c0:c1], (n // 8, 1))

    rows = pl.ds

    def load_q(r, ref=qb):
        return ref[rows(r, RG), :].astype(f32)

    def make_x2(r, q, st, ref=ys):
        y = jnp.concatenate([ref[c, rows(r, RG), :] for c in range(CT)], axis=-1)
        return q + (((q - st[0]) * st[1]) * mvec(1) + mvec(0)) * y

    def make_h2(x2, st):
        return ((x2 - st[0]) * st[1]) * mvec(3) + mvec(2)

    def pack_ln(x, st):
        return pltpu.bitcast(((x - st[0]) * st[1]).astype(bf16), u32)

    def ln_chain(r, n):
        qv, yv = qb.at[rows(r, n), :], ys.at[:, rows(r, n), :]
        xv, hv = x2s.at[rows(r, n), :], h2s.at[rows(r, n), :]
        prev = None
        for o in range(0, n, RG):
            q = load_q(o, qv)
            x2 = make_x2(o, q, _stats(q, prev), yv)
            xv[o:o + RG, :] = x2
            st = _stats(x2)
            h2 = make_h2(xv[o:o + RG, :], st)
            hv[o:o + RG, :] = h2
            st = _stats(h2)
            zt[o // 2:(o + RG) // 2, :] = pack_ln(hv[o:o + RG, :], st)
            prev = st[1]

    def mm_w1(r, n, o=0, parts=4):
        z = pltpu.bitcast(zt[o // 2:(o + n) // 2, :], bf16)
        h1 = _gelu(_dot_balanced(z, lambda a, b: w1p[:, a:b], D, parts))
        for c in range(CT):
            h1s[c, rows(r + 8, n), :] = h1[:, c * 128:(c + 1) * 128]

    def mm_w2(r, parts=4):
        lane = jax.lax.broadcasted_iota(i32, (T, 128), 1)

        def sh(k, c):
            return h1s[c, rows(r + 8 + k, T), :]

        g = jnp.concatenate([
            sh(-1, 0),
            jnp.where(lane < 32, sh(-1, 1), sh(1, 1)),
            jnp.where(lane < 64, sh(1, 2), sh(-2, 2)),
            jnp.where(lane < 96, sh(-2, 3), sh(2, 3)),
            sh(2, 4)], axis=-1)
        hss[rows(r, T), :] = _dot_balanced(g, lambda a, b: w2p[:, a:b], D, parts)

    def ln_x1(r, links=1):
        hv, sv = h2s.at[rows(r, T), :], hss.at[rows(r, T), :]
        prev = [None] * links
        for n, o in enumerate(range(0, T, RG)):
            x1 = hv[o:o + RG, :] + sv[o:o + RG, :]
            st = _stats(x1, prev[n % links], early=True)
            zb[o // 2:(o + RG) // 2, :] = pack_ln(x1, st)
            prev[n % links] = st[1]

    def mm_w3(f0, parts=1):
        z = pltpu.bitcast(zb[...], bf16)
        return _gelu2(_dot_balanced(z, lambda a, b: w3p[(f0 + a) // 2:(f0 + b) // 2, :], FM - f0, parts, nt=True))

    def mm_w3_first():
        z = pltpu.bitcast(zb[...], bf16)
        return _gelu2(jnp.dot(z, pltpu.bitcast(w3n[...], bf16), preferred_element_type=f32))

    def mm_w3_tail():
        z = pltpu.bitcast(zb[...], bf16)
        w = pltpu.bitcast(w3p[FM // 2:F // 2, :], bf16)
        return _gelu2(jax.lax.dot_general(w, z, NT_DIMS, preferred_element_type=f32))

    def mm_w4(r, n, act, c0=0, c1=D):
        h = _dot_balanced(act, lambda a, b: w4p[:, c0 + a:c0 + b], c1 - c0, 1)
        x1 = h2s[rows(r, n), c0:c1] + hss[rows(r, n), c0:c1]
        base = x2s[rows(r, n), c0:c1] + mvec(4, n, c0, c1) * x1
        ob[rows(r, n), c0:c1] = (base + mvec(5, n, c0, c1) * h).astype(bf16)

    groups = list(range(0, P0 + P1, RG))

    wait([mod_copies[0], q_copies[0]])
    sa, ca, ga = mod_part(0, 1)
    modb[0] = ga * sa
    modb[1] = ga * (1.0 + ca)
    for c in range(NL, CT):
        mac_inv(c, NB - 1)
    st1 = {o: _stats(load_q(o)) for o in groups}
    zt[0:8, 0:128] = jnp.zeros((8, 128), u32)
    st2 = {}
    for o in groups:
        x2 = make_x2(o, load_q(o), st1[o])
        x2s[o:o + RG, :] = x2
        st2[o] = _stats(x2)

    wait([mod_copies[1]])
    sb, cb = mod_part(1, 2)
    modb[2] = sb
    modb[3] = 1.0 + cb
    st3 = {}
    for o in range(0, P0, RG):
        h2 = make_h2(x2s[o:o + RG, :], st2[o])
        h2s[o:o + RG, :] = h2
        st3[o] = _stats(h2)
    for o in range(0, P0, RG):
        zt[o // 2:(o + RG) // 2, :] = pack_ln(h2s[o:o + RG, :], st3[o])

    wait([w_copies[0]])
    w1p[...] = pltpu.bitcast(w1b[...], u32)
    mm_w1(0, P0)
    prev = None
    for o in range(P0, P0 + P1, RG):
        h2 = make_h2(x2s[o:o + RG, :], st2[o])
        h2s[o:o + RG, :] = h2
        st = _stats(h2, prev, early=True)
        zt[o // 2:(o + RG) // 2, :] = pack_ln(h2, st)
        prev = st[1]
    mm_w1(P0, P1, P0)

    wait([w_copies[1]])
    w2p[...] = pltpu.bitcast(w2b[...], u32)
    mm_w2(0)
    ln_x1(0, 2)
    mm_w2(T)

    wait([q_copies[1], w_copies[2]])
    w3p[...] = pltpu.bitcast(w3b[...], u32)
    ln_chain(P0 + P1, PA)
    main = mm_w3(0, 4)
    mm_w1(P0 + P1, PA)
    tail = mm_w3_tail()

    wait([w_copies[3], mod_copies[2]])
    w4p[...] = pltpu.bitcast(w4b[...], u32)
    w3n[...] = pltpu.bitcast(w3b[0:128, :].astype(f32).T.astype(bf16), u32)
    act = jnp.concatenate([main, tail.T], axis=-1).astype(bf16)
    sc16 = jnp.broadcast_to(scb[:, 0:D], (16, D)).astype(bf16)
    for c0 in range(0, D, 128):
        gb = jnp.dot(sc16, wmc[:, c0:c0 + 128], preferred_element_type=f32)[0:8]
        modb[4, :, c0:c0 + 128] = gb
        modb[5, :, c0:c0 + 128] = 0.5 * gb
        if c0 < D - 128:
            mm_w4(0, T, act, c0, c0 + 128)
        else:
            mm_w4(0, T // 2, act[0:T // 2], c0, c0 + 128)
            mm_w4(T // 2, T // 2, act[T // 2:T], c0, c0 + 128)
    ln_x1(T)
    out_copy(0).start()
    q_copies[2].wait()

    def mlp_body(i, carry):
        r1 = pl.multiple_of(PB - PC + PC * i, 32)
        r = pl.multiple_of(i * T, T)
        first = mm_w3_first()
        ln_chain(r1, PC)
        tail = mm_w3_tail()
        act = jnp.concatenate([first, mm_w3(128), tail.T], axis=-1).astype(bf16)
        mm_w4(r, T, act, 0, 128)
        mm_w1(r1, PC, parts=1)
        mm_w4(r, T, act, 128, 256)
        mm_w2(r + T, parts=1)
        ln_x1(r + T)
        mm_w4(r, T, act, 256, D)
        out_copy(i).start()
        return carry

    jax.lax.fori_loop(1, NC - 1, mlp_body, 0)

    first = mm_w3_first()
    tail = mm_w3_tail()
    act = jnp.concatenate([first, mm_w3(128), tail.T], axis=-1)
    for cp, (o, n, c0, c1) in zip(out_tail, tail_parts):
        mm_w4(o, n, act[o - (S - T):o - (S - T) + n], c0, c1)
        cp.start()
    for i in range(NC - 1):
        out_copy(i).wait()
    for cp in out_tail:
        cp.wait()


@jax.jit
def pallas_adaLN_cond__ssm_conv_h3__mixer_s_mlp__prompt_kernel(
    A_q: jax.Array,
    A_k: jax.Array,
    A_v: jax.Array,
    A_shift_k: jax.Array,
    A_ssm_k: jax.Array,
    A_ssm_D: jax.Array,
    B_x: jax.Array,
    B_w1: jax.Array,
    B_w2: jax.Array,
    B_w3: jax.Array,
    B_w4: jax.Array,
    c: jax.Array,
    w_mod: jax.Array,
):
    del B_x
    any_spec = pl.BlockSpec(memory_space=pl.ANY)

    def tile_view(x):
        return x.reshape(S // 8, 8, CT, 128).transpose(0, 2, 1, 3).reshape(S * CT, 128)

    vm = pltpu.VMEM
    dma = pltpu.SemaphoreType.DMA
    spec = (4, NG, 16, 128)
    out = pl.pallas_call(
        _kernel,
        in_specs=[any_spec] * 12,
        out_specs=any_spec,
        out_shape=jax.ShapeDtypeStruct((S, D), bf16),
        scratch_shapes=[
            *[vm((KROWS, 128), bf16)] * NB, *[vm((VROWS, 128), bf16)] * NB, vm((CT, 128, S), bf16),
            vm((S, D), bf16), vm((D, D), bf16), vm((D, D), bf16), vm((F, D), bf16), vm((F, D), bf16),
            vm((D // 2, D), u32), vm((D // 2, D), u32), vm((F // 2, D), u32), vm((F // 2, D), u32),
            vm((D, 3 * D), bf16), vm((D, 2 * D), bf16), vm((D, D), bf16),
            vm((4, D), bf16), vm((D,), bf16), vm((1, D), bf16), vm((1, 1792), f32),
            vm((4, 128, 128), u32), vm((4, 128, 128), u32), vm((4, 64, 256), u32),
            vm((CT, 8, 8, 128), f32),
            vm((CT, NB) + spec, f32), vm((CT, NB - 1) + spec, f32), vm((CT,) + spec, f32),
            vm((CT, NB) + spec, f32), vm((4, 128, 128), f32),
            vm((CT, S + 32, 128), f32), vm((8, 8, D), f32),
            vm((CT, S + 32, 128), f32), vm((S, D), f32), vm((S, D), f32), vm((S, D), f32),
            vm((288, D), u32), vm((T // 2, D), u32), vm((D // 2, 128), u32),
            vm((S, D), bf16),
            dma((26,)), dma((NC + 2,)),
        ],
        compiler_params=pltpu.CompilerParams(vmem_limit_bytes=110 << 20, disable_bounds_checks=True,
                                             disable_semaphore_checks=True),
    )(A_q.reshape(S, D), tile_view(A_k), tile_view(A_v), A_shift_k.T, A_ssm_k,
      A_ssm_D, B_w1, B_w2, B_w3.T, B_w4, c, w_mod)
    return out.reshape(1, S, D)
```

```python
import os
import numpy as np
import jax
import jax.numpy as jnp
import jax.experimental.pallas as pl
import jax.experimental.pallas.tpu as pltpu

f32, bf16, u32, i32 = jnp.float32, jnp.bfloat16, jnp.uint32, jnp.int32

S, D, F = 2048, 640, 1728
CT = D // 128
TR = 8 * CT
NB, BLK, NFFT = 4, 512, 1024
KROWS, VROWS = BLK * CT + 128, BLK * CT + 64
NG = 16
T = 256
NC = S // T
FM = (F // 128) * 128
P0, P1, PA, PC = 320, 224, 160, 224
PB = P0 + P1 + PA
LAST0 = int(os.environ.get('LAST0', '208'))
RG = 16
EPS = 1e-5
NT_DIMS = (((1,), (1,)), ((), ()))
OUTF = int(os.environ.get('OUTF', '1'))
MODI = int(os.environ.get('MODI', '1'))
NS = [int(x) * 128 for x in os.environ.get('NS', '12')]
R3 = os.environ.get('R3', 'a31t')
SM = int(os.environ.get('SM', '0'))
TC = int(os.environ.get('TC', '512'))
TMODE = int(os.environ.get('TMODE', '0'))
LB = os.environ.get('LB', 'nct3p1s2lssr')
W1P = int(os.environ.get('W1P', '1'))
W2P = int(os.environ.get('W2P', '1'))
RS = int(os.environ.get('RS', '0'))
W3S = int(os.environ.get('W3S', '640'))
ST3 = int(os.environ.get('ST3', '1'))
ST4 = int(os.environ.get('ST4', '1'))
LL = int(os.environ.get('LL', '1'))
H = T // 2
NP3 = 6
ST1 = int(os.environ.get('ST1', '1'))
ST2 = int(os.environ.get('ST2', '1'))
CL = int(os.environ.get('CL', '1'))
ACC = int(os.environ.get('ACC', '1'))
SORD = int(os.environ.get('SORD', '1'))
CE = int(os.environ.get('CE', '0'))
RSQ = int(os.environ.get('RSQ', '0'))
GM = int(os.environ.get('GM', '0'))
GVF = int(os.environ.get("GVF", "8"))
GVI = int(os.environ.get("GVI", "8"))
NL = int(os.environ.get("NL", "4"))
SKIPCONV = int(os.environ.get("SKIPCONV", "0"))
SCOPES = bool(int(os.environ.get("KSCOPES", "0")))


class _NoScope:
    def __enter__(self):
        return self

    def __exit__(self, *a):
        return False


def _scope(name):
    return jax.named_scope(name) if SCOPES else _NoScope()


def _lo(w):
    return pltpu.bitcast(w << 16, f32)


def _hi(w):
    return pltpu.bitcast(w & jnp.uint32(0xFFFF0000), f32)


def _cis(n):
    t = (n & (2 * NFFT - 1)).astype(f32) * (np.pi / NFFT)
    return jnp.cos(t), jnp.sin(t)


def _fwd_table(r):
    g = jax.lax.broadcasted_iota(i32, (NG, 128), 0)
    cg, sg = _cis(jnp.where(g < NG // 2, 32 * g + 1, 32 * g - 253) * r)
    cs, ss = _cis(4 * jax.lax.broadcasted_iota(i32, (8, 128), 0) * r)
    parts = []
    for i in range(NG):
        c, s = cg[i:i + 1], sg[i:i + 1]
        parts += [c * cs - s * ss, -(s * cs + c * ss)]
    return pltpu.bitcast(jnp.concatenate(parts, axis=0).astype(bf16), u32)


def _inv_tables():
    def phase(rows):
        col = jax.lax.broadcasted_iota(i32, (rows, 256), 1)
        k = ((col >> 4) << 3) + (col & 7)
        row = jax.lax.broadcasted_iota(i32, (rows, 256), 0)
        return jnp.where(k < 64, 4 * k + 1, 4 * k - 253), (col & 8) << 6, row

    fr, _, g = phase(16)
    cg, sg = _cis(fr * (32 * g))
    fr, off, s = phase(8)
    out = []
    for p in range(4):
        cs, ss = _cis(fr * (4 * s + p) + off)
        cs, ss = cs * (2.0 / NFFT), ss * (2.0 / NFFT)
        parts = [cg[i:i + 1] * cs - sg[i:i + 1] * ss for i in range(16)]
        out.append(pltpu.bitcast(jnp.concatenate(parts, axis=0).astype(bf16), u32))
    return out


def _radix4(re, im, inverse):
    ar, ai = re[0] + re[2], im[0] + im[2]
    br, bi = re[0] - re[2], im[0] - im[2]
    cr, ci = re[1] + re[3], im[1] + im[3]
    dr, di = re[1] - re[3], im[1] - im[3]
    minus_i = (br + di, bi - dr)
    plus_i = (br - di, bi + dr)
    if inverse:
        return [(ar + cr, ai + ci), plus_i, (ar - cr, ai - ci), minus_i]
    return [(ar + cr, ai + ci), minus_i, (ar - cr, ai - ci), plus_i]


def _stats(x, link=None, early=False):
    zero = 0.0 if link is None else jnp.minimum(link, 0.0)
    part = x[:, 0:128]
    for c in range(1, CT):
        part = part + x[:, c * 128:(c + 1) * 128]
    if link is not None and early:
        part = part + zero
        zero = 0.0
    m = jnp.sum(part, axis=-1, keepdims=True) * (1.0 / D)
    v = jnp.maximum(jnp.sum(x * x, axis=-1, keepdims=True) * (1.0 / D) - m * m, zero)
    if RSQ:
        return m, jnp.exp2(jnp.log(v + EPS) * (-0.5 / np.log(2.0)))
    return m, jax.lax.rsqrt(v + EPS)


def _gelu2(x):
    c = 0.7978845608028654
    u = c + (c * 0.044715) * (x * x)
    return x + x * jnp.tanh(x * u)


def _gelu(x):
    c = 0.7978845608028654
    u = c + (c * 0.044715) * (x * x)
    hx = 0.5 * x
    return hx + hx * jnp.tanh(x * u)


def _dot_balanced(x, wslice, n_cols, parts, nt=False):
    def mm(a, c0, c1):
        a, w = a.astype(bf16), pltpu.bitcast(wslice(c0, c1), bf16)
        if nt:
            return jax.lax.dot_general(a, w, NT_DIMS, preferred_element_type=f32)
        return jnp.dot(a, w, preferred_element_type=f32)

    if parts == 1:
        return mm(x, 0, n_cols)
    base, extra = divmod(x.shape[0] // 16, parts)
    last, o = [], 0
    head = mm(x, 0, n_cols - 128)
    for i in range(parts):
        n = 16 * (base + (1 if i < extra else 0))
        last.append(mm(x[o:o + n], n_cols - 128, n_cols))
        o += n
    return jnp.concatenate([head, jnp.concatenate(last, axis=0)], axis=-1)


def _kernel(q_hbm, k_hbm, v_hbm, sh_hbm, sk_hbm, d_hbm, w1_hbm, w2_hbm, w3_hbm, w4_hbm,
            c_hbm, wm_hbm, o_hbm,
            kb0, kb1, kb2, kb3, vb0, vb1, vb2, vb3, skb, qb, w1b, w2b, w3b, w4b, w1p, w2p, w3p, w4p,
            wma, wmb, wmc, shb, db, cb_, scb,
            fub, fkb, gtb, par, US, KS, UR, YS, YP, ys, modb, h1s, h2s, x2s, hss, zt, zb, w3n, s1, s2, s3, s4, p4, al, cq, zs, zu, gs, gu, ob,
            sem, sem_o):
    n_in = [0]

    def load(src, dst):
        n_in[0] += 1
        return pltpu.make_async_copy(src, dst, sem.at[n_in[0] - 1])

    nkv = BLK * CT
    small = [load(d_hbm, db), load(sh_hbm, shb), load(c_hbm, cb_)]
    sk_copies = [load(sk_hbm.at[pl.ds(c * 128, 128), :], skb.at[c]) for c in range(CT)]
    kbs, vbs, wms = [kb0, kb1, kb2, kb3], [vb0, vb1, vb2, vb3], [wma, wmb, wmc]
    kv_copies = [[load(k_hbm.at[pl.ds(0, nkv), :], kb0.at[pl.ds(TR, nkv), :]) if a == 0 else
                  load(k_hbm.at[pl.ds(a * nkv - TR, nkv + TR), :], kbs[a].at[pl.ds(0, nkv + TR), :]),
                  load(v_hbm.at[pl.ds(a * nkv, nkv), :], vbs[a].at[pl.ds(0, nkv), :])] for a in range(NB)]
    mod_cols = [(0, 3 * D), (3 * D, 2 * D), (5 * D, D)]
    mod_copies = [load(wm_hbm.at[:, pl.ds(o, n)], w) for (o, n), w in zip(mod_cols, wms)]
    w_copies = [load(w1_hbm, w1b), load(w2_hbm, w2b), load(w3_hbm, w3b), load(w4_hbm, w4b)]
    q_copies = [load(q_hbm.at[pl.ds(o, n), :], qb.at[pl.ds(o, n), :])
                for o, n in [(0, P0 + P1), (P0 + P1, PA), (PB, S - PB)]]

    def out_copy(i):
        r = i * T if isinstance(i, int) else pl.multiple_of(i * T, T)
        return pltpu.make_async_copy(ob.at[pl.ds(r, T), :], o_hbm.at[pl.ds(r, T), :], sem_o.at[i])

    tail_parts = [(S - T, T, 128, D), (S - T, LAST0, 0, 128), (S - T + LAST0, T - LAST0, 0, 128)]
    out_tail = [pltpu.make_async_copy(ob.at[pl.ds(o, n), pl.ds(c0, c1 - c0)], o_hbm.at[pl.ds(o, n), pl.ds(c0, c1 - c0)],
                                      sem_o.at[NC - 1 + i]) for i, (o, n, c0, c1) in enumerate(tail_parts)]

    first = small + kv_copies[0] if SM == 0 else [kv_copies[0][0]] + small + [kv_copies[0][1]]
    for cp in (first + sk_copies + kv_copies[1] + kv_copies[2] + kv_copies[3]
               + [mod_copies[0], q_copies[0], mod_copies[1], w_copies[0], w_copies[1], q_copies[1],
                  w_copies[2], w_copies[3], mod_copies[2], q_copies[2]]):
        cp.start()

    def wait(name, copies):
        with _scope(name):
            for cp in copies:
                cp.wait()

    def pin(i, carry):
        z = jnp.zeros((8, 128), f32)
        scb[:, pl.ds(pl.multiple_of(i * 128, 128), 128)] = z[0:1]
        YP[i, 0:8, :] = z
        US[i, 0, 0, 0, 0:8, :] = z
        KS[i, 0, 0, 0, 0:8, :] = z
        YS[i, 0, 0, 0, 0:8, :] = z
        UR[i, 0, 0, 0:8, :] = z
        cq[i, 0:8, :] = z
        r8 = pl.multiple_of(i * 8, 8)
        al[pl.ds(r8, 8), 0:128] = jnp.zeros((8, 128), u32)
        gs[pl.ds(r8, 8), 0:128] = jnp.zeros((8, 128), u32)
        gu[pl.ds(r8, 8), 0:128] = jnp.zeros((8, 128), u32)
        return carry

    def fence(i, carry):
        YP[i, 0:8, :] = jnp.zeros((8, 128), f32)
        return carry

    with _scope("init"):
        jax.lax.fori_loop(0, 2, pin, 0)
        lane = jax.lax.broadcasted_iota(i32, (1, 128), 1)
        for p in range(4):
            m = (lane - p) & 3
            fkb[p] = _fwd_table(128 * m + ((lane - m) & 127))
        for c in range(CT):
            kb0[c * 8:(c + 1) * 8, :] = jnp.zeros((8, 128), bf16)
            h1s[c, 0:8, :] = jnp.zeros((8, 128), f32)
            h1s[c, S + 8:S + 16, :] = jnp.zeros((8, 128), f32)
        for a in range(NB):
            kbs[a][nkv + TR:KROWS, :] = jnp.zeros((KROWS - nkv - TR, 128), bf16)
            vbs[a][nkv:VROWS, :] = jnp.zeros((VROWS - nkv, 128), bf16)
        for p in range(4):
            fub[p] = _fwd_table(8 * (lane & 63) + ((lane >> 6) << 2) + p)
        if SM:
            for p, tab in enumerate(_inv_tables()):
                gtb[p] = tab
        wait("w_small", small)
        cvec = cb_[...].astype(f32)
        scb[:, 0:D] = cvec * jax.nn.sigmoid(cvec)
        dv = db[...].astype(f32).reshape(1, D)
        shv = shb[...].astype(f32)
        for c in range(CT):
            for i in range(4):
                par[c, i] = jnp.broadcast_to(shv[i:i + 1, c * 128:(c + 1) * 128], (8, 128))
            par[c, 4] = jnp.broadcast_to(dv[:, c * 128:(c + 1) * 128], (8, 128))
        if not SM:
            for p, tab in enumerate(_inv_tables()):
                gtb[p] = tab

    def get(ref, idx, g, n):
        return (ref[idx + (slice(g, g + n), slice(0, 8))], ref[idx + (slice(g, g + n), slice(8, 16))])

    def put(ref, idx, g, n, xr, xi):
        ref[idx + (slice(g, g + n), slice(0, 8))] = xr
        ref[idx + (slice(g, g + n), slice(8, 16))] = xi

    def split(tt, g, n):
        tt = [t[g * 16:(g + n) * 16].reshape(n, 16, 128) for t in tt]
        return [t[:, 0:8] for t in tt], [t[:, 8:16] for t in tt]

    def fwd_k(c, j):
        if SKIPCONV:
            return
        lane = jax.lax.broadcasted_iota(i32, (64, 128), 1)
        even = (lane & 1) == 0
        l01 = (lane & 2) == 0
        l12 = ((lane + 3) & 2) == 0
        rm = []
        for m in range(4):
            w = pltpu.bitcast(skb[c, :, (4 * j + m) * 128:(4 * j + m + 1) * 128], u32)
            rm.append(pltpu.roll(w, m, 1) if m else w)
        e01 = jnp.where(even, rm[0], rm[1])
        o01 = jnp.where(even, rm[1], rm[0])
        e23 = jnp.where(even, rm[2], rm[3])
        o23 = jnp.where(even, rm[3], rm[2])
        kp = [jnp.where(l01, e01, e23), jnp.where(l12, o01, o23),
              jnp.where(l01, e23, e01), jnp.where(l12, o23, o01)]
        tt = [jax.lax.dot_general(pltpu.bitcast(fkb[p], bf16), pltpu.bitcast(kp[p], bf16), NT_DIMS,
                                  preferred_element_type=f32) for p in range(4)]
        for g in range(0, NG, GVF):
            re, im = split(tt, g, GVF)
            if j == 0:
                re[0] = re[0] + par[c, 4][None]
            for m, (xr, xi) in enumerate(_radix4(re, im, False)):
                if j < NB - 1:
                    put(KS, (c, j, m), g, GVF, xr, xi)
                ur, ui = get(US, (c, 0, m), g, GVF)
                put(YS, (c, j, m), g, GVF, xr * ur - xi * ui, xr * ui + xi * ur)

    def fwd_u(c, a):
        if SKIPCONV:
            return
        taps = [jnp.tile(par[c, i], (8, 1)) for i in range(4)]
        ws = TR // 2
        base = 4 * c
        kw, vw = kbs[a].bitcast(u32), vbs[a].bitcast(u32)

        def words(ref, start):
            return ref[pl.ds(start, BLK // 8, stride=ws), :]

        kk = {}
        for w in range(4):
            x = words(kw, ws + base + w)
            kk[2 * w], kk[2 * w + 1] = _lo(x), _hi(x)
        kk[-3] = _hi(words(kw, base + 2))
        x = words(kw, base + 3)
        kk[-2], kk[-1] = _lo(x), _hi(x)
        sub = []
        for w in range(4):
            x = words(vw, base + w)
            for r, vv in ((2 * w, _lo(x)), (2 * w + 1, _hi(x))):
                sh = taps[0] * kk[r] + taps[1] * kk[r - 1] + taps[2] * kk[r - 2] + taps[3] * kk[r - 3]
                sub.append(sh * vv)
        kv = [jnp.concatenate([sub[p], sub[p + 4]], axis=0) for p in range(4)]
        tt = [jnp.dot(pltpu.bitcast(fub[p], bf16), kv[p].astype(bf16), preferred_element_type=f32)
              for p in range(4)]
        for g in range(0, NG, GVF):
            re, im = split(tt, g, GVF)
            for m, (xr, xi) in enumerate(_radix4(re, im, False)):
                if a:
                    pr, pi = get(US, (c, 0, m), g, GVF) if a == 1 else get(UR, (c, m), g, GVF)
                    if a < NB - 1:
                        put(UR, (c, m), g, GVF, xr, xi)
                    xr, xi = (xr - pi, xi + pr) if g < NG // 2 else (xr + pi, xi - pr)
                put(US, (c, a, m), g, GVF, xr, xi)

    def mac_inv(c, a):
        if SKIPCONV:
            return
        for h in range(2):
            vals = [[] for _ in range(4)]
            for g in range(8 * h, 8 * h + 8, GVI):
                yre, yim = [], []
                for m in range(4):
                    yr, yi = get(YS, (c, a, m), g, GVI)
                    for j in range(a):
                        kr, ki = get(KS, (c, j, m), g, GVI)
                        ur, ui = get(US, (c, a - j, m), g, GVI)
                        yr = yr + (kr * ur - ki * ui)
                        yi = yi + (kr * ui + ki * ur)
                    yre.append(yr)
                    yim.append(yi)
                for p, (pr, pi) in enumerate(_radix4(yre, yim, True)):
                    vals[p].append(jnp.concatenate([pr, pi], axis=1))
            for p in range(4):
                pb = jnp.concatenate(vals[p], axis=0).reshape(128, 128).astype(bf16)
                r = jnp.dot(pltpu.bitcast(gtb[p, :, h * 128:(h + 1) * 128], bf16), pb,
                            preferred_element_type=f32)
                if h == 0:
                    YP[p] = r
                else:
                    ys[c, pl.ds(a * BLK + p, 128, stride=4), :] = YP[p] + r

    with _scope("conv_u0"):
        wait("w_kv", kv_copies[0])
        for c in range(CT):
            fwd_u(c, 0)
    with _scope("conv_k"):
        for grp in ((0,), (1, 2), (3, 4)):
            wait("w_sk", [sk_copies[c] for c in grp])
            for c in grp:
                for j in (3, 2, 1, 0):
                    fwd_k(c, j)
    for a in range(1, NB):
        with _scope("conv_u%d" % a):
            wait("w_kv", kv_copies[a])
            for c in range(CT):
                fwd_u(c, a)
                mac_inv(c, a - 1)
    with _scope("conv_last"):
        jax.lax.fori_loop(0, 2, fence, 0)
        for c in range(NL):
            mac_inv(c, NB - 1)

    def mod_part(part, extra):
        n, wm = mod_cols[part][1], wms[part]
        act = scb[:, 0:D]

        def sc(k0, k1):
            return jnp.broadcast_to(act[:, k0:k1], (16, k1 - k0)).astype(bf16)

        e = 128 * extra
        r = jnp.dot(sc(0, D), wm[:, e:n], preferred_element_type=f32)
        r0 = (jnp.dot(sc(0, D - 64), wm[0:D - 64, 0:e], preferred_element_type=f32)
              + jnp.dot(sc(D - 64, D), wm[D - 64:D, 0:e], preferred_element_type=f32))
        r = jnp.concatenate([r0, r], axis=-1)[0:8]
        return [r[:, i * D:(i + 1) * D] for i in range(n // D)]

    def mvec(i, n=RG, c0=0, c1=D):
        return jnp.tile(modb[i, :, c0:c1], (n // 8, 1))

    rows = pl.ds

    def load_q(r, ref=qb):
        return ref[rows(r, RG), :].astype(f32)

    def make_x2(r, q, st, ref=ys):
        y = jnp.concatenate([ref[c, rows(r, RG), :] for c in range(CT)], axis=-1)
        return q + (((q - st[0]) * st[1]) * mvec(1) + mvec(0)) * y

    def make_h2(x2, st):
        return ((x2 - st[0]) * st[1]) * mvec(3) + mvec(2)

    def pack_ln(x, st):
        return pltpu.bitcast(((x - st[0]) * st[1]).astype(bf16), u32)

    def lhs_sums(a11, a12, a21, a22):
        return [a11 + a22, a21 + a22, a11 + a12, a21 - a11, a12 - a22]

    def rhs_sums(b11, b12, b21, b22):
        return [b11 + b22, b12 - b22, b21 - b11, b11 + b12, b21 + b22]

    RHS = [(0, 3, 1), (1, 3, -1), (2, 0, -1), (0, 1, 1), (2, 3, 1)]

    def rhs_sum(k, block):
        a, b, sg = RHS[k]
        return block(a) + block(b) if sg > 0 else block(a) - block(b)

    def pk(x):
        return pltpu.bitcast(x.astype(bf16), u32)

    def pk_many(vals):
        return pk(jnp.concatenate(vals, axis=-1))

    def lanes(k):
        return slice(128 * k, 128 * (k + 1))

    def ub(x):
        return pltpu.bitcast(x, bf16)

    def strassen(dot, a11, a22, asum, ax1, ax2, b11, b22, bsum, bx1, bx2):
        if SORD:
            m2 = dot(asum[1], b11)
            m4 = dot(a22, bsum[2])
            c21 = (m4 + m2) + dot(ax2, bx1)
            m3 = dot(a11, bsum[1])
            m5 = dot(asum[2], b22)
            c12 = (m3 + m5) + dot(ax1, bx2)
            m1 = dot(asum[0], bsum[0])
            c11 = (((m4 - m5) + m1) + dot(asum[4], bsum[4])) + dot(ax1, bx1)
            c22 = (((m3 - m2) + m1) + dot(asum[3], bsum[3])) + dot(ax2, bx2)
            return [c11, c12, c21, c22]
        m1 = dot(asum[0], bsum[0])
        m4 = dot(a22, bsum[2])
        m2 = dot(asum[1], b11)
        m3 = dot(a11, bsum[1])
        m5 = dot(asum[2], b22)
        x12 = dot(ax1, bx2)
        x21 = dot(ax2, bx1)
        m7 = dot(asum[4], bsum[4])
        x11 = dot(ax1, bx1)
        m6 = dot(asum[3], bsum[3])
        x22 = dot(ax2, bx2)
        return [(((m1 + m4) - m5) + m7) + x11, (m3 + m5) + x12, (m4 + m2) + x21, (((m1 - m2) + m3) + m6) + x22]

    def nn(a, w):
        return jnp.dot(a.astype(bf16), w, preferred_element_type=f32)

    def both(ref, r0, r1, col):
        return jnp.concatenate([ref[r0:r1, lanes(1 + col)], ref[r0:r1, lanes(3 + col)]], axis=-1).astype(f32)

    def prep_sq(wb, sw):
        for k in (2, 1, 0, 4, 3):
            sw[128 * k:128 * (k + 1), :] = pk(rhs_sum(k, lambda b: both(wb, 256 * (b // 2), 256 * (b // 2 + 1), b % 2)))

    def sq_strassen(a, top, bot, asum, wp, sw):
        h = top.shape[0]
        c0 = nn(a, ub(wp[:, 0:128]))
        out = {0: (c0[0:h], c0[h:2 * h])}
        for n in range(2):
            c1, c2 = 128 + 256 * n, 256 + 256 * n
            q = strassen(nn, top[:, 0:256], bot[:, 256:512], asum, top[:, 512:D], bot[:, 512:D],
                         ub(wp[0:128, c1:c2]), ub(wp[128:256, c2:c2 + 128]), [ub(sw[128 * k:128 * (k + 1), lanes(n)]) for k in range(5)],
                         ub(wp[256:320, c1:c2]), ub(wp[256:320, c2:c2 + 128]))
            out[2 * n + 1] = (q[0], q[2])
            out[2 * n + 2] = (q[1], q[3])
        return out

    def ln_chain(r, n, links=1, r_out=None, early=False):
        qv, yv = qb.at[rows(r, n), :], ys.at[:, rows(r, n), :]
        r_out = r if r_out is None else r_out
        xv, hv = x2s.at[rows(r_out, n), :], h2s.at[rows(r_out, n), :]
        prev = [None] * links
        cnt = 0
        for o1 in range(0, n // 2, RG):
            zz = []
            for o in (o1, o1 + n // 2):
                q = load_q(o, qv)
                x2 = make_x2(o, q, _stats(q, prev[cnt % links], early), yv)
                xv[o:o + RG, :] = x2
                st = _stats(x2)
                h2 = make_h2(xv[o:o + RG, :], st)
                hv[o:o + RG, :] = h2
                st = _stats(h2)
                z = (hv[o:o + RG, :] - st[0]) * st[1]
                zt[o // 2:(o + RG) // 2, :] = pk(z)
                prev[cnt % links] = st[1]
                cnt += 1
                zz.append(z)
            if ST1:
                for k, v in enumerate(lhs_sums(zz[0][:, 0:256], zz[0][:, 256:512], zz[1][:, 0:256], zz[1][:, 256:512])):
                    zu.at[k][o1 // 2:(o1 + RG) // 2, :] = pk(v)

    def mm_w1s(r, n):
        h = n // 2
        res = sq_strassen(ub(zt[0:h, :]), ub(zt[0:h // 2, :]), ub(zt[h // 2:h, :]),
                          [ub(zu[k, 0:h // 2, :]) for k in range(5)], w1p, s1)
        for c, (ct, cb2) in res.items():
            h1s[c, rows(r + 8, h), :] = _gelu(ct)
            h1s[c, rows(r + 8 + h, h), :] = _gelu(cb2)

    def mm_w1(r, n, o=0, parts=4):
        z = pltpu.bitcast(zt[o // 2:(o + n) // 2, :], bf16)
        h1 = _gelu(_dot_balanced(z, lambda a, b: w1p[:, a:b], D, parts))
        for c in range(CT):
            h1s[c, rows(r + 8, n), :] = h1[:, c * 128:(c + 1) * 128]

    def mm_w2(r, parts=4, st=False):
        lane = jax.lax.broadcasted_iota(i32, (T, 128), 1)

        def sh(k, c):
            return h1s[c, rows(r + 8 + k, T), :]

        g = jnp.concatenate([
            sh(-1, 0),
            jnp.where(lane < 32, sh(-1, 1), sh(1, 1)),
            jnp.where(lane < 64, sh(1, 2), sh(-2, 2)),
            jnp.where(lane < 96, sh(-2, 3), sh(2, 3)),
            sh(2, 4)], axis=-1)
        if not st:
            hss[rows(r, T), :] = _dot_balanced(g, lambda a, b: w2p[:, a:b], D, parts)
            return
        top, bot = g[0:H], g[H:T]
        sums = lhs_sums(top[:, 0:256], top[:, 256:512], bot[:, 0:256], bot[:, 256:512])
        if GM == 0:
            res = sq_strassen(g, top, bot, sums, w2p, s2)
        else:
            gs[...] = pk(g)
            gu[...] = pk_many(sums)
            res = sq_strassen(ub(gs[...]), ub(gs[0:H // 2, :]), ub(gs[H // 2:H, :]),
                              [ub(gu[:, 256 * k:256 * (k + 1)]) for k in range(5)], w2p, s2)
        for c, (ct, cb2) in res.items():
            hss[rows(r, H), c * 128:(c + 1) * 128] = ct
            hss[rows(r + H, H), c * 128:(c + 1) * 128] = cb2

    def ln_x1(r, links=1):
        hv, sv = h2s.at[rows(r, T), :], hss.at[rows(r, T), :]
        prev = [None] * links
        n = 0
        for o in range(0, H, RG):
            zz = []
            for oo in (o, o + H):
                x1 = hv[oo:oo + RG, :] + sv[oo:oo + RG, :]
                st = _stats(x1, prev[n % links], early=True)
                z = (x1 - st[0]) * st[1]
                zb[oo // 2:(oo + RG) // 2, :] = pltpu.bitcast(z.astype(bf16), u32)
                prev[n % links] = st[1]
                n += 1
                zz.append(z)
            if ST3:
                a11, a12, a21, a22 = zz[0][:, 0:256], zz[0][:, 256:512], zz[1][:, 0:256], zz[1][:, 256:512]
                for k, v in enumerate([a11 + a22, a21 + a22, a11 + a12, a21 - a11, a12 - a22]):
                    zs.at[k][o // 2:(o + RG) // 2, :] = pk(v)

    def mm_w3(f0, parts=1, f1=FM):
        z = pltpu.bitcast(zb[...], bf16)
        return _gelu2(_dot_balanced(z, lambda a, b: w3p[(f0 + a) // 2:(f0 + b) // 2, :], f1 - f0, parts, nt=True))

    def mm_w3_first():
        z = pltpu.bitcast(zb[...], bf16)
        return _gelu2(jnp.dot(z, pltpu.bitcast(w3n[...], bf16), preferred_element_type=f32))

    def mm_w3_tail():
        z = pltpu.bitcast(zb[...], bf16)
        w = pltpu.bitcast(w3p[FM // 2:F // 2, :], bf16)
        return _gelu2(jax.lax.dot_general(w, z, NT_DIMS, preferred_element_type=f32))

    def mm_w4(r, n, act, c0=0, c1=D, parts=1):
        h = _dot_balanced(act, lambda a, b: w4p[:, c0 + a:c0 + b], c1 - c0, parts)
        x1 = h2s[rows(r, n), c0:c1] + hss[rows(r, n), c0:c1]
        if OUTF:
            base = x2s[rows(r, n), c0:c1] + mvec(4, n, c0, c1) * x1
            ob[rows(r, n), c0:c1] = (base + mvec(5, n, c0, c1) * h).astype(bf16)
        else:
            ob[rows(r, n), c0:c1] = (x2s[rows(r, n), c0:c1] + mvec(4, n, c0, c1) * (x1 + 0.5 * h)).astype(bf16)

    def prep_w3():
        for j in range(NP3):
            r0 = 128 * (2 * j + 1)
            for k in (2, 1, 0, 4, 3):
                s3[64 * j:64 * (j + 1), 256 * k:256 * (k + 1)] = pk(rhs_sum(k, lambda b: w3b[
                    r0 + 128 * (b % 2):r0 + 128 * (b % 2 + 1), 256 * (b // 2):256 * (b // 2 + 1)].astype(f32)))

    def prep_w4():
        for j in range(7):
            if j < NP3:
                r0 = 128 * (2 * j + 1)
                p4[0, 64 * j:64 * (j + 1), :] = pltpu.bitcast(w4b[r0:r0 + 128, 0:128], u32)
                p4[1, 64 * j:64 * (j + 1), :] = pltpu.bitcast(w4b[r0 + 128:r0 + 256, 0:128], u32)
            else:
                p4[0, 64 * j:64 * (j + 1), :] = pltpu.bitcast(w4b[0:128, 0:128], u32)
                p4[1, 64 * j:64 * j + 32, :] = pltpu.bitcast(w4b[FM:F, 0:128], u32)
                p4[1, 64 * j + 32:64 * (j + 1), :] = jnp.zeros((32, 128), u32)
        def block(j, b):
            if j < NP3:
                r0 = 128 * (2 * j + 1 + b // 2)
                return both(w4b, r0, r0 + 128, b % 2)
            if b < 2:
                return both(w4b, 0, 128, b % 2)
            return jnp.concatenate([both(w4b, FM, F, b % 2), jnp.zeros((64, 256), f32)], axis=0)

        for m, k in ((1, 0), (4, 2), (2, None), (3, 1), (5, None), (7, 4), (6, 3)):
            for j in range(7):
                v = block(j, 0 if m == 2 else 3) if k is None else rhs_sum(k, lambda b: block(j, b))
                o = 448 * (m - 1) + 64 * j
                s4[o:o + 64, :] = pk(v)

    def nt(a, w):
        return jax.lax.dot_general(a, w, NT_DIMS, preferred_element_type=f32)

    def w3_pair(j):
        r0 = 64 * (2 * j + 1)
        z1, z2 = ub(zb[0:H // 2, :]), ub(zb[H // 2:H, :])
        we, wo = ub(w3p[r0:r0 + 64, :]), ub(w3p[r0 + 64:r0 + 128, :])
        q = strassen(nt, z1[:, 0:256], z2[:, 256:512], [ub(zs[k]) for k in range(5)], z1[:, 512:D], z2[:, 512:D],
                     we[:, 0:256], wo[:, 256:512], [ub(s3[64 * j:64 * (j + 1), 256 * k:256 * (k + 1)]) for k in range(5)], we[:, 512:D], wo[:, 512:D])
        return [_gelu2(c) for c in q]

    def put_quads(j, q):
        l1, l2, l5, l6, l7 = lhs_sums(*q)
        al[64 * j:64 * (j + 1), :] = pk_many([l1, l2, q[0], q[3], l5, l6, l7, q[1], q[2]])

    def w3_all(first, tail):
        tp = jnp.concatenate([tail.T, jnp.zeros((T, 64), f32)], axis=-1)
        put_quads(NP3, [first[0:H], tp[0:H], first[H:T], tp[H:T]])
        for j in range(NP3):
            put_quads(j, w3_pair(j))

    def left(k):
        return jnp.concatenate([al[64 * j:64 * (j + 1), lanes(k)] for j in range(7)], axis=-1)

    def w4_plain(r, o=0, n=T):
        top = jnp.concatenate([left(2), left(7)], axis=-1)
        bot = jnp.concatenate([left(8), left(3)], axis=-1)
        a = jnp.concatenate([top, bot], axis=0)[o // 2:(o + n) // 2]
        h = nn(ub(a), ub(jnp.concatenate([p4[0], p4[1]], axis=0)))
        finish(r + o, n, h, 0, 128)

    def finish(r, n, h, c0, c1):
        x1 = h2s[rows(r, n), c0:c1] + hss[rows(r, n), c0:c1]
        base = x2s[rows(r, n), c0:c1] + mvec(4, n, c0, c1) * x1
        ob[rows(r, n), c0:c1] = (base + mvec(5, n, c0, c1) * h).astype(bf16)

    def w4_steps(r, n):
        c1 = 128 + 256 * n

        def m(k):
            return nn(ub(left(k - 1)), ub(s4[448 * (k - 1):448 * k, lanes(n)]))

        if ACC:
            m1 = m(1)
            cq[0] = m1
            m4 = m(4)
            cq[2] = m4
            cq[3] = cq[0] + m4
            m2 = m(2)
            cq[0] = cq[0] - m2
            finish(r + H, H, cq[2] + m2, c1, c1 + 128)
            yield
            m3 = m(3)
            cq[1] = m3
            cq[0] = cq[0] + m3
            m5 = m(5)
            cq[3] = cq[3] - m5
            finish(r, H, cq[1] + m5, c1 + 128, c1 + 256)
            yield
            finish(r, H, cq[3] + m(7), c1, c1 + 128)
            finish(r + H, H, cq[0] + m(6), c1 + 128, c1 + 256)
            yield
            return
        m1, m4 = m(1), m(4)
        m2 = m(2)
        finish(r + H, H, m4 + m2, c1, c1 + 128)
        yield
        m3, m5 = m(3), m(5)
        finish(r, H, m3 + m5, c1 + 128, c1 + 256)
        yield
        finish(r, H, ((m1 + m4) - m5) + m(7), c1, c1 + 128)
        finish(r + H, H, ((m1 - m2) + m3) + m(6), c1 + 128, c1 + 256)
        yield

    def w4_pair(r, n):
        for _ in w4_steps(r, n):
            pass

    groups = list(range(0, P0 + P1, RG))
    with _scope("pre_a"):
        wait("w_q0", [mod_copies[0], q_copies[0]])
        sa, ca, ga = mod_part(0, 1)
        modb[0] = ga * sa
        modb[1] = ga * (1.0 + ca)
        for c in range(NL, CT):
            mac_inv(c, NB - 1)
        st1 = {o: _stats(load_q(o)) for o in groups}
        zt[0:8, 0:128] = jnp.zeros((8, 128), u32)
        st2 = {}
        for o in groups:
            x2 = make_x2(o, load_q(o), st1[o])
            x2s[o:o + RG, :] = x2
            st2[o] = _stats(x2)
    with _scope("pre_b"):
        wait("w_modB", [mod_copies[1]])
        sb, cb = mod_part(1, 2)
        modb[2] = sb
        modb[3] = 1.0 + cb
        st3 = {}
        for o in range(0, P0, RG):
            h2 = make_h2(x2s[o:o + RG, :], st2[o])
            h2s[o:o + RG, :] = h2
            st3[o] = _stats(h2)
        for o in range(0, P0, RG):
            zt[o // 2:(o + RG) // 2, :] = pack_ln(h2s[o:o + RG, :], st3[o])
    with _scope("r1"):
        wait("w_w1", [w_copies[0]])
        w1p[...] = pltpu.bitcast(w1b[...], u32)
        mm_w1(0, P0)
        prev = None
        for o in range(P0, P0 + P1, RG):
            h2 = make_h2(x2s[o:o + RG, :], st2[o])
            h2s[o:o + RG, :] = h2
            st = _stats(h2, prev, early=True)
            zt[o // 2:(o + RG) // 2, :] = pack_ln(h2, st)
            prev = st[1]
        mm_w1(P0, P1, P0)
    with _scope("r2"):
        wait("w_w2", [w_copies[1]])
        w2p[...] = pltpu.bitcast(w2b[...], u32)
        if ST2:
            prep_sq(w2b, s2)
        mm_w2(0)
        ln_x1(0, 2)
        mm_w2(T, st=ST2)
    with _scope("r3"):
        wait("w_w3", [q_copies[1], w_copies[2]])
        w3p[...] = pltpu.bitcast(w3b[...], u32)
        if ST3:
            prep_w3()
        ln_chain(P0 + P1, PA)
        first = mm_w3(0, 1, 128)
        tail = mm_w3_tail()
        w3_all(first, tail)
        if ST1:
            prep_sq(w1b, s1)
            mm_w1s(P0 + P1, PA)
        else:
            mm_w1(P0 + P1, PA)
    with _scope("r4"):
        wait("w_w4", [w_copies[3], mod_copies[2]])
        prep_w4()
        w3n[...] = pltpu.bitcast(w3b[0:128, :].astype(f32).T.astype(bf16), u32)
        sc16 = jnp.broadcast_to(scb[:, 0:D], (16, D)).astype(bf16)

        def gate(c0, c1):
            gbc = jnp.dot(sc16, wmc[:, c0:c1], preferred_element_type=f32)[0:8]
            modb[4, :, c0:c1] = gbc
            modb[5, :, c0:c1] = 0.5 * gbc

        gate(0, 128)
        w4_plain(0)
        gate(128, 384)
        w4_pair(0, 0)
        gate(384, D)
        w4_pair(0, 1)
        ln_x1(T)
        out_copy(0).start()
        q_copies[2].wait()

    def mlp_body(i, carry):
        with _scope("iter"):
            r1 = pl.multiple_of(PB - PC + PC * i, 32)
            r = pl.multiple_of(i * T, T)
            for tok in LB:
                if tok == 'n':
                    first = mm_w3_first()
                elif tok == 'c':
                    ln_chain(r1, PC, CL)
                elif tok == 'd':
                    ln_chain(pl.multiple_of(jnp.minimum(r1 + PC, S - PC), 32), PC, CL, r1 + PC, CE)
                elif tok == 't':
                    tail = mm_w3_tail()
                elif tok == '3':
                    w3_all(first, tail)
                    steps = w4_steps(r, 0)
                elif tok == 's':
                    next(steps)
                elif tok == 'p':
                    w4_plain(r)
                elif tok == '1':
                    if ST1:
                        mm_w1s(r1, PC)
                    else:
                        mm_w1(r1, PC, parts=W1P)
                elif tok == 'q':
                    w4_pair(r, 0)
                elif tok == '2':
                    mm_w2(r + T, parts=W2P, st=ST2)
                elif tok == 'l':
                    ln_x1(r + T, LL)
                elif tok == 'r':
                    w4_pair(r, 1)
            out_copy(i).start()
        return carry

    with _scope("loop"):
        jax.lax.fori_loop(1, NC - 1, mlp_body, 0)
    with _scope("last"):
        first = mm_w3_first()
        tail = mm_w3_tail()
        w3_all(first, tail)
        w4_pair(S - T, 0)
        w4_pair(S - T, 1)
        out_tail[0].start()
        w4_plain(S - T, 0, LAST0)
        out_tail[1].start()
        w4_plain(S - T, LAST0, T - LAST0)
        out_tail[2].start()
    with _scope("fin"):
        for i in range(NC - 1):
            out_copy(i).wait()
        for cp in out_tail:
            cp.wait()


@jax.jit
def pallas_adaLN_cond__ssm_conv_h3__mixer_s_mlp__prompt_kernel(
    A_q: jax.Array,
    A_k: jax.Array,
    A_v: jax.Array,
    A_shift_k: jax.Array,
    A_ssm_k: jax.Array,
    A_ssm_D: jax.Array,
    B_x: jax.Array,
    B_w1: jax.Array,
    B_w2: jax.Array,
    B_w3: jax.Array,
    B_w4: jax.Array,
    c: jax.Array,
    w_mod: jax.Array,
):
    del B_x
    any_spec = pl.BlockSpec(memory_space=pl.ANY)

    def tile_view(x):
        return x.reshape(S // 8, 8, CT, 128).transpose(0, 2, 1, 3).reshape(S * CT, 128)

    vm = pltpu.VMEM
    dma = pltpu.SemaphoreType.DMA
    spec = (4, NG, 16, 128)
    out = pl.pallas_call(
        _kernel,
        in_specs=[any_spec] * 12,
        out_specs=any_spec,
        out_shape=jax.ShapeDtypeStruct((S, D), bf16),
        scratch_shapes=[
            *[vm((KROWS, 128), bf16)] * NB, *[vm((VROWS, 128), bf16)] * NB, vm((CT, 128, S), bf16),
            vm((S, D), bf16), vm((D, D), bf16), vm((D, D), bf16), vm((F, D), bf16), vm((F, D), bf16),
            vm((D // 2, D), u32), vm((D // 2, D), u32), vm((F // 2, D), u32), vm((F // 2, D), u32),
            vm((D, 3 * D), bf16), vm((D, 2 * D), bf16), vm((D, D), bf16),
            vm((4, D), bf16), vm((D,), bf16), vm((1, D), bf16), vm((1, 1792), f32),
            vm((4, 128, 128), u32), vm((4, 128, 128), u32), vm((4, 64, 256), u32),
            vm((CT, 8, 8, 128), f32),
            vm((CT, NB) + spec, f32), vm((CT, NB - 1) + spec, f32), vm((CT,) + spec, f32),
            vm((CT, NB) + spec, f32), vm((4, 128, 128), f32),
            vm((CT, S + 32, 128), f32), vm((8, 8, D), f32),
            vm((CT, S + 32, 128), f32), vm((S + 256, D), f32), vm((S + 256, D), f32), vm((S, D), f32),
            vm((288, D), u32), vm((T // 2, D), u32), vm((D // 2, 128), u32),
            vm((640, 256), u32), vm((640, 256), u32), vm((NP3 * 64, 1280), u32), vm((7 * 448, 256), u32), vm((2, 448, 128), u32), vm((7 * 64, 1152), u32),
            vm((4, H, 128), f32), vm((5, H // 2, 256), u32), vm((5, H // 2, 256), u32),
            vm((H, D), u32), vm((H // 2, 1280), u32),
            vm((S, D), bf16),
            dma((26,)), dma((NC + 2,)),
        ],
        compiler_params=pltpu.CompilerParams(vmem_limit_bytes=110 << 20, disable_bounds_checks=True,
                                             disable_semaphore_checks=True),
    )(A_q.reshape(S, D), tile_view(A_k), tile_view(A_v), A_shift_k.T, A_ssm_k,
      A_ssm_D, B_w1, B_w2, B_w3.T, B_w4, c, w_mod)
    return out.reshape(1, S, D)
```

```python
import os
import numpy as np
import jax
import jax.numpy as jnp
import jax.experimental.pallas as pl
import jax.experimental.pallas.tpu as pltpu

f32, bf16, u32, i32 = jnp.float32, jnp.bfloat16, jnp.uint32, jnp.int32

S, D, F = 2048, 640, 1728
CT = D // 128
TR = 8 * CT
NB, BLK, NFFT = 4, 512, 1024
KROWS, VROWS = BLK * CT + 128, BLK * CT + 64
NG = 16
T = 256
NC = S // T
FM = (F // 128) * 128
P0, P1, PA, PC = 320, 224, 160, 224
PB = P0 + P1 + PA
LAST0 = int(os.environ.get('LAST0', '208'))
RG = 16
EPS = 1e-5
NT_DIMS = (((1,), (1,)), ((), ()))
OUTF = int(os.environ.get('OUTF', '1'))
MODI = int(os.environ.get('MODI', '1'))
NS = [int(x) * 128 for x in os.environ.get('NS', '12')]
R3 = os.environ.get('R3', 'a31t')
SM = int(os.environ.get('SM', '0'))
TC = int(os.environ.get('TC', '512'))
TMODE = int(os.environ.get('TMODE', '0'))
LB = os.environ.get('LB', 'nct3p1s2lssr')
W1P = int(os.environ.get('W1P', '1'))
W2P = int(os.environ.get('W2P', '1'))
RS = int(os.environ.get('RS', '0'))
W3S = int(os.environ.get('W3S', '640'))
ST3 = int(os.environ.get('ST3', '1'))
ST4 = int(os.environ.get('ST4', '1'))
LL = int(os.environ.get('LL', '1'))
H = T // 2
NP3 = 6
ST1 = int(os.environ.get('ST1', '1'))
ST2 = int(os.environ.get('ST2', '1'))
CL = int(os.environ.get('CL', '1'))
ACC = int(os.environ.get('ACC', '1'))
SORD = int(os.environ.get('SORD', '1'))
CE = int(os.environ.get('CE', '0'))
RSQ = int(os.environ.get('RSQ', '1'))
GM = int(os.environ.get('GM', '0'))
FEN4 = int(os.environ.get('FEN4', '0'))
R2C = int(os.environ.get('R2C', '0'))
R3O = os.environ.get('R3O', 'ct3n1')
GVF = int(os.environ.get("GVF", "8"))
GVI = int(os.environ.get("GVI", "8"))
NL = int(os.environ.get("NL", "4"))
SKIPCONV = int(os.environ.get("SKIPCONV", "0"))
SCOPES = bool(int(os.environ.get("KSCOPES", "0")))


class _NoScope:
    def __enter__(self):
        return self

    def __exit__(self, *a):
        return False


def _scope(name):
    return jax.named_scope(name) if SCOPES else _NoScope()


def _lo(w):
    return pltpu.bitcast(w << 16, f32)


def _hi(w):
    return pltpu.bitcast(w & jnp.uint32(0xFFFF0000), f32)


def _cis(n):
    t = (n & (2 * NFFT - 1)).astype(f32) * (np.pi / NFFT)
    return jnp.cos(t), jnp.sin(t)


def _fwd_table(r):
    g = jax.lax.broadcasted_iota(i32, (NG, 128), 0)
    cg, sg = _cis(jnp.where(g < NG // 2, 32 * g + 1, 32 * g - 253) * r)
    cs, ss = _cis(4 * jax.lax.broadcasted_iota(i32, (8, 128), 0) * r)
    parts = []
    for i in range(NG):
        c, s = cg[i:i + 1], sg[i:i + 1]
        parts += [c * cs - s * ss, -(s * cs + c * ss)]
    return pltpu.bitcast(jnp.concatenate(parts, axis=0).astype(bf16), u32)


def _inv_tables():
    def phase(rows):
        col = jax.lax.broadcasted_iota(i32, (rows, 256), 1)
        k = ((col >> 4) << 3) + (col & 7)
        row = jax.lax.broadcasted_iota(i32, (rows, 256), 0)
        return jnp.where(k < 64, 4 * k + 1, 4 * k - 253), (col & 8) << 6, row

    fr, _, g = phase(16)
    cg, sg = _cis(fr * (32 * g))
    fr, off, s = phase(8)
    out = []
    for p in range(4):
        cs, ss = _cis(fr * (4 * s + p) + off)
        cs, ss = cs * (2.0 / NFFT), ss * (2.0 / NFFT)
        parts = [cg[i:i + 1] * cs - sg[i:i + 1] * ss for i in range(16)]
        out.append(pltpu.bitcast(jnp.concatenate(parts, axis=0).astype(bf16), u32))
    return out


def _radix4(re, im, inverse):
    ar, ai = re[0] + re[2], im[0] + im[2]
    br, bi = re[0] - re[2], im[0] - im[2]
    cr, ci = re[1] + re[3], im[1] + im[3]
    dr, di = re[1] - re[3], im[1] - im[3]
    minus_i = (br + di, bi - dr)
    plus_i = (br - di, bi + dr)
    if inverse:
        return [(ar + cr, ai + ci), plus_i, (ar - cr, ai - ci), minus_i]
    return [(ar + cr, ai + ci), minus_i, (ar - cr, ai - ci), plus_i]


def _stats(x, link=None, early=False):
    zero = 0.0 if link is None else jnp.minimum(link, 0.0)
    part = x[:, 0:128]
    for c in range(1, CT):
        part = part + x[:, c * 128:(c + 1) * 128]
    if link is not None and early:
        part = part + zero
        zero = 0.0
    m = jnp.sum(part, axis=-1, keepdims=True) * (1.0 / D)
    v = jnp.maximum(jnp.sum(x * x, axis=-1, keepdims=True) * (1.0 / D) - m * m, zero)
    if RSQ:
        return m, jnp.exp2(jnp.log(v + EPS) * (-0.5 / np.log(2.0)))
    return m, jax.lax.rsqrt(v + EPS)


def _gelu2(x):
    c = 0.7978845608028654
    u = c + (c * 0.044715) * (x * x)
    return x + x * jnp.tanh(x * u)


def _gelu(x):
    c = 0.7978845608028654
    u = c + (c * 0.044715) * (x * x)
    hx = 0.5 * x
    return hx + hx * jnp.tanh(x * u)


def _dot_balanced(x, wslice, n_cols, parts, nt=False):
    def mm(a, c0, c1):
        a, w = a.astype(bf16), pltpu.bitcast(wslice(c0, c1), bf16)
        if nt:
            return jax.lax.dot_general(a, w, NT_DIMS, preferred_element_type=f32)
        return jnp.dot(a, w, preferred_element_type=f32)

    if parts == 1:
        return mm(x, 0, n_cols)
    base, extra = divmod(x.shape[0] // 16, parts)
    last, o = [], 0
    head = mm(x, 0, n_cols - 128)
    for i in range(parts):
        n = 16 * (base + (1 if i < extra else 0))
        last.append(mm(x[o:o + n], n_cols - 128, n_cols))
        o += n
    return jnp.concatenate([head, jnp.concatenate(last, axis=0)], axis=-1)


def _kernel(q_hbm, k_hbm, v_hbm, sh_hbm, sk_hbm, d_hbm, w1_hbm, w2_hbm, w3_hbm, w4_hbm,
            c_hbm, wm_hbm, o_hbm,
            kb0, kb1, kb2, kb3, vb0, vb1, vb2, vb3, skb, qb, w1b, w2b, w3b, w4b, w1p, w2p, w3p, w4p,
            wma, wmb, wmc, shb, db, cb_, scb,
            fub, fkb, gtb, par, US, KS, UR, YS, YP, ys, modb, h1s, h2s, x2s, hss, zt, zb, w3n, s1, s2, s3, s4, p4, al, cq, zs, zu, gs, gu, ob,
            sem, sem_o):
    n_in = [0]

    def load(src, dst):
        n_in[0] += 1
        return pltpu.make_async_copy(src, dst, sem.at[n_in[0] - 1])

    nkv = BLK * CT
    small = [load(d_hbm, db), load(sh_hbm, shb), load(c_hbm, cb_)]
    sk_copies = [load(sk_hbm.at[pl.ds(c * 128, 128), :], skb.at[c]) for c in range(CT)]
    kbs, vbs, wms = [kb0, kb1, kb2, kb3], [vb0, vb1, vb2, vb3], [wma, wmb, wmc]
    kv_copies = [[load(k_hbm.at[pl.ds(0, nkv), :], kb0.at[pl.ds(TR, nkv), :]) if a == 0 else
                  load(k_hbm.at[pl.ds(a * nkv - TR, nkv + TR), :], kbs[a].at[pl.ds(0, nkv + TR), :]),
                  load(v_hbm.at[pl.ds(a * nkv, nkv), :], vbs[a].at[pl.ds(0, nkv), :])] for a in range(NB)]
    mod_cols = [(0, 3 * D), (3 * D, 2 * D), (5 * D, D)]
    mod_copies = [load(wm_hbm.at[:, pl.ds(o, n)], w) for (o, n), w in zip(mod_cols, wms)]
    w_copies = [load(w1_hbm, w1b), load(w2_hbm, w2b), load(w3_hbm, w3b), load(w4_hbm, w4b)]
    q_copies = [load(q_hbm.at[pl.ds(o, n), :], qb.at[pl.ds(o, n), :])
                for o, n in [(0, P0 + P1), (P0 + P1, PA), (PB, S - PB)]]

    def out_copy(i):
        r = i * T if isinstance(i, int) else pl.multiple_of(i * T, T)
        return pltpu.make_async_copy(ob.at[pl.ds(r, T), :], o_hbm.at[pl.ds(r, T), :], sem_o.at[i])

    tail_parts = [(S - T, T, 128, D), (S - T, LAST0, 0, 128), (S - T + LAST0, T - LAST0, 0, 128)]
    out_tail = [pltpu.make_async_copy(ob.at[pl.ds(o, n), pl.ds(c0, c1 - c0)], o_hbm.at[pl.ds(o, n), pl.ds(c0, c1 - c0)],
                                      sem_o.at[NC - 1 + i]) for i, (o, n, c0, c1) in enumerate(tail_parts)]

    first = small + kv_copies[0] if SM == 0 else [kv_copies[0][0]] + small + [kv_copies[0][1]]
    for cp in (first + sk_copies + kv_copies[1] + kv_copies[2] + kv_copies[3]
               + [mod_copies[0], q_copies[0], mod_copies[1], w_copies[0], w_copies[1], q_copies[1],
                  w_copies[2], w_copies[3], mod_copies[2], q_copies[2]]):
        cp.start()

    def wait(name, copies):
        with _scope(name):
            for cp in copies:
                cp.wait()

    def pin(i, carry):
        z = jnp.zeros((8, 128), f32)
        scb[:, pl.ds(pl.multiple_of(i * 128, 128), 128)] = z[0:1]
        YP[i, 0:8, :] = z
        US[i, 0, 0, 0, 0:8, :] = z
        KS[i, 0, 0, 0, 0:8, :] = z
        YS[i, 0, 0, 0, 0:8, :] = z
        UR[i, 0, 0, 0:8, :] = z
        cq[i, 0:8, :] = z
        r8 = pl.multiple_of(i * 8, 8)
        al[pl.ds(r8, 8), 0:128] = jnp.zeros((8, 128), u32)
        gs[pl.ds(r8, 8), 0:128] = jnp.zeros((8, 128), u32)
        gu[pl.ds(r8, 8), 0:128] = jnp.zeros((8, 128), u32)
        return carry

    def fence(i, carry):
        YP[i, 0:8, :] = jnp.zeros((8, 128), f32)
        return carry

    with _scope("init"):
        jax.lax.fori_loop(0, 2, pin, 0)
        lane = jax.lax.broadcasted_iota(i32, (1, 128), 1)
        for p in range(4):
            m = (lane - p) & 3
            fkb[p] = _fwd_table(128 * m + ((lane - m) & 127))
        for c in range(CT):
            kb0[c * 8:(c + 1) * 8, :] = jnp.zeros((8, 128), bf16)
            h1s[c, 0:8, :] = jnp.zeros((8, 128), f32)
            h1s[c, S + 8:S + 16, :] = jnp.zeros((8, 128), f32)
        for a in range(NB):
            kbs[a][nkv + TR:KROWS, :] = jnp.zeros((KROWS - nkv - TR, 128), bf16)
            vbs[a][nkv:VROWS, :] = jnp.zeros((VROWS - nkv, 128), bf16)
        for p in range(4):
            fub[p] = _fwd_table(8 * (lane & 63) + ((lane >> 6) << 2) + p)
        if SM:
            for p, tab in enumerate(_inv_tables()):
                gtb[p] = tab
        wait("w_small", small)
        cvec = cb_[...].astype(f32)
        scb[:, 0:D] = cvec * jax.nn.sigmoid(cvec)
        dv = db[...].astype(f32).reshape(1, D)
        shv = shb[...].astype(f32)
        for c in range(CT):
            for i in range(4):
                par[c, i] = jnp.broadcast_to(shv[i:i + 1, c * 128:(c + 1) * 128], (8, 128))
            par[c, 4] = jnp.broadcast_to(dv[:, c * 128:(c + 1) * 128], (8, 128))
        if not SM:
            for p, tab in enumerate(_inv_tables()):
                gtb[p] = tab

    def get(ref, idx, g, n):
        return (ref[idx + (slice(g, g + n), slice(0, 8))], ref[idx + (slice(g, g + n), slice(8, 16))])

    def put(ref, idx, g, n, xr, xi):
        ref[idx + (slice(g, g + n), slice(0, 8))] = xr
        ref[idx + (slice(g, g + n), slice(8, 16))] = xi

    def split(tt, g, n):
        tt = [t[g * 16:(g + n) * 16].reshape(n, 16, 128) for t in tt]
        return [t[:, 0:8] for t in tt], [t[:, 8:16] for t in tt]

    def fwd_k(c, j):
        if SKIPCONV:
            return
        lane = jax.lax.broadcasted_iota(i32, (64, 128), 1)
        even = (lane & 1) == 0
        l01 = (lane & 2) == 0
        l12 = ((lane + 3) & 2) == 0
        rm = []
        for m in range(4):
            w = pltpu.bitcast(skb[c, :, (4 * j + m) * 128:(4 * j + m + 1) * 128], u32)
            rm.append(pltpu.roll(w, m, 1) if m else w)
        e01 = jnp.where(even, rm[0], rm[1])
        o01 = jnp.where(even, rm[1], rm[0])
        e23 = jnp.where(even, rm[2], rm[3])
        o23 = jnp.where(even, rm[3], rm[2])
        kp = [jnp.where(l01, e01, e23), jnp.where(l12, o01, o23),
              jnp.where(l01, e23, e01), jnp.where(l12, o23, o01)]
        tt = [jax.lax.dot_general(pltpu.bitcast(fkb[p], bf16), pltpu.bitcast(kp[p], bf16), NT_DIMS,
                                  preferred_element_type=f32) for p in range(4)]
        for g in range(0, NG, GVF):
            re, im = split(tt, g, GVF)
            if j == 0:
                re[0] = re[0] + par[c, 4][None]
            for m, (xr, xi) in enumerate(_radix4(re, im, False)):
                if j < NB - 1:
                    put(KS, (c, j, m), g, GVF, xr, xi)
                ur, ui = get(US, (c, 0, m), g, GVF)
                put(YS, (c, j, m), g, GVF, xr * ur - xi * ui, xr * ui + xi * ur)

    def fwd_u(c, a):
        if SKIPCONV:
            return
        taps = [jnp.tile(par[c, i], (8, 1)) for i in range(4)]
        ws = TR // 2
        base = 4 * c
        kw, vw = kbs[a].bitcast(u32), vbs[a].bitcast(u32)

        def words(ref, start):
            return ref[pl.ds(start, BLK // 8, stride=ws), :]

        kk = {}
        for w in range(4):
            x = words(kw, ws + base + w)
            kk[2 * w], kk[2 * w + 1] = _lo(x), _hi(x)
        kk[-3] = _hi(words(kw, base + 2))
        x = words(kw, base + 3)
        kk[-2], kk[-1] = _lo(x), _hi(x)
        sub = []
        for w in range(4):
            x = words(vw, base + w)
            for r, vv in ((2 * w, _lo(x)), (2 * w + 1, _hi(x))):
                sh = taps[0] * kk[r] + taps[1] * kk[r - 1] + taps[2] * kk[r - 2] + taps[3] * kk[r - 3]
                sub.append(sh * vv)
        kv = [jnp.concatenate([sub[p], sub[p + 4]], axis=0) for p in range(4)]
        tt = [jnp.dot(pltpu.bitcast(fub[p], bf16), kv[p].astype(bf16), preferred_element_type=f32)
              for p in range(4)]
        for g in range(0, NG, GVF):
            re, im = split(tt, g, GVF)
            for m, (xr, xi) in enumerate(_radix4(re, im, False)):
                if a:
                    pr, pi = get(US, (c, 0, m), g, GVF) if a == 1 else get(UR, (c, m), g, GVF)
                    if a < NB - 1:
                        put(UR, (c, m), g, GVF, xr, xi)
                    xr, xi = (xr - pi, xi + pr) if g < NG // 2 else (xr + pi, xi - pr)
                put(US, (c, a, m), g, GVF, xr, xi)

    def mac_inv(c, a):
        if SKIPCONV:
            return
        for h in range(2):
            vals = [[] for _ in range(4)]
            for g in range(8 * h, 8 * h + 8, GVI):
                yre, yim = [], []
                for m in range(4):
                    yr, yi = get(YS, (c, a, m), g, GVI)
                    for j in range(a):
                        kr, ki = get(KS, (c, j, m), g, GVI)
                        ur, ui = get(US, (c, a - j, m), g, GVI)
                        yr = yr + (kr * ur - ki * ui)
                        yi = yi + (kr * ui + ki * ur)
                    yre.append(yr)
                    yim.append(yi)
                for p, (pr, pi) in enumerate(_radix4(yre, yim, True)):
                    vals[p].append(jnp.concatenate([pr, pi], axis=1))
            for p in range(4):
                pb = jnp.concatenate(vals[p], axis=0).reshape(128, 128).astype(bf16)
                r = jnp.dot(pltpu.bitcast(gtb[p, :, h * 128:(h + 1) * 128], bf16), pb,
                            preferred_element_type=f32)
                if h == 0:
                    YP[p] = r
                else:
                    ys[c, pl.ds(a * BLK + p, 128, stride=4), :] = YP[p] + r

    with _scope("conv_u0"):
        wait("w_kv", kv_copies[0])
        for c in range(CT):
            fwd_u(c, 0)
    with _scope("conv_k"):
        for grp in ((0,), (1, 2), (3, 4)):
            wait("w_sk", [sk_copies[c] for c in grp])
            for c in grp:
                for j in (3, 2, 1, 0):
                    fwd_k(c, j)
    for a in range(1, NB):
        with _scope("conv_u%d" % a):
            wait("w_kv", kv_copies[a])
            for c in range(CT):
                fwd_u(c, a)
                mac_inv(c, a - 1)
    with _scope("conv_last"):
        jax.lax.fori_loop(0, 2, fence, 0)
        for c in range(NL):
            mac_inv(c, NB - 1)

    def mod_part(part, extra):
        n, wm = mod_cols[part][1], wms[part]
        act = scb[:, 0:D]

        def sc(k0, k1):
            return jnp.broadcast_to(act[:, k0:k1], (16, k1 - k0)).astype(bf16)

        e = 128 * extra
        r = jnp.dot(sc(0, D), wm[:, e:n], preferred_element_type=f32)
        r0 = (jnp.dot(sc(0, D - 64), wm[0:D - 64, 0:e], preferred_element_type=f32)
              + jnp.dot(sc(D - 64, D), wm[D - 64:D, 0:e], preferred_element_type=f32))
        r = jnp.concatenate([r0, r], axis=-1)[0:8]
        return [r[:, i * D:(i + 1) * D] for i in range(n // D)]

    def mvec(i, n=RG, c0=0, c1=D):
        return jnp.tile(modb[i, :, c0:c1], (n // 8, 1))

    rows = pl.ds

    def load_q(r, ref=qb):
        return ref[rows(r, RG), :].astype(f32)

    def make_x2(r, q, st, ref=ys):
        y = jnp.concatenate([ref[c, rows(r, RG), :] for c in range(CT)], axis=-1)
        return q + (((q - st[0]) * st[1]) * mvec(1) + mvec(0)) * y

    def make_h2(x2, st):
        return ((x2 - st[0]) * st[1]) * mvec(3) + mvec(2)

    def pack_ln(x, st):
        return pltpu.bitcast(((x - st[0]) * st[1]).astype(bf16), u32)

    def lhs_sums(a11, a12, a21, a22):
        return [a11 + a22, a21 + a22, a11 + a12, a21 - a11, a12 - a22]

    def rhs_sums(b11, b12, b21, b22):
        return [b11 + b22, b12 - b22, b21 - b11, b11 + b12, b21 + b22]

    RHS = [(0, 3, 1), (1, 3, -1), (2, 0, -1), (0, 1, 1), (2, 3, 1)]

    def rhs_sum(k, block):
        a, b, sg = RHS[k]
        return block(a) + block(b) if sg > 0 else block(a) - block(b)

    def pk(x):
        return pltpu.bitcast(x.astype(bf16), u32)

    def pk_many(vals):
        return pk(jnp.concatenate(vals, axis=-1))

    def lanes(k):
        return slice(128 * k, 128 * (k + 1))

    def ub(x):
        return pltpu.bitcast(x, bf16)

    def strassen(dot, a11, a22, asum, ax1, ax2, b11, b22, bsum, bx1, bx2):
        if SORD:
            m2 = dot(asum[1], b11)
            m4 = dot(a22, bsum[2])
            c21 = (m4 + m2) + dot(ax2, bx1)
            m3 = dot(a11, bsum[1])
            m5 = dot(asum[2], b22)
            c12 = (m3 + m5) + dot(ax1, bx2)
            m1 = dot(asum[0], bsum[0])
            c11 = (((m4 - m5) + m1) + dot(asum[4], bsum[4])) + dot(ax1, bx1)
            c22 = (((m3 - m2) + m1) + dot(asum[3], bsum[3])) + dot(ax2, bx2)
            return [c11, c12, c21, c22]
        m1 = dot(asum[0], bsum[0])
        m4 = dot(a22, bsum[2])
        m2 = dot(asum[1], b11)
        m3 = dot(a11, bsum[1])
        m5 = dot(asum[2], b22)
        x12 = dot(ax1, bx2)
        x21 = dot(ax2, bx1)
        m7 = dot(asum[4], bsum[4])
        x11 = dot(ax1, bx1)
        m6 = dot(asum[3], bsum[3])
        x22 = dot(ax2, bx2)
        return [(((m1 + m4) - m5) + m7) + x11, (m3 + m5) + x12, (m4 + m2) + x21, (((m1 - m2) + m3) + m6) + x22]

    def nn(a, w):
        return jnp.dot(a.astype(bf16), w, preferred_element_type=f32)

    def both(ref, r0, r1, col):
        return jnp.concatenate([ref[r0:r1, lanes(1 + col)], ref[r0:r1, lanes(3 + col)]], axis=-1).astype(f32)

    def prep_sq(wb, sw):
        for k in (2, 1, 0, 4, 3):
            sw[128 * k:128 * (k + 1), :] = pk(rhs_sum(k, lambda b: both(wb, 256 * (b // 2), 256 * (b // 2 + 1), b % 2)))

    def sq_strassen(a, top, bot, asum, wp, sw):
        h = top.shape[0]
        c0 = nn(a, ub(wp[:, 0:128]))
        out = {0: (c0[0:h], c0[h:2 * h])}
        for n in range(2):
            c1, c2 = 128 + 256 * n, 256 + 256 * n
            q = strassen(nn, top[:, 0:256], bot[:, 256:512], asum, top[:, 512:D], bot[:, 512:D],
                         ub(wp[0:128, c1:c2]), ub(wp[128:256, c2:c2 + 128]), [ub(sw[128 * k:128 * (k + 1), lanes(n)]) for k in range(5)],
                         ub(wp[256:320, c1:c2]), ub(wp[256:320, c2:c2 + 128]))
            out[2 * n + 1] = (q[0], q[2])
            out[2 * n + 2] = (q[1], q[3])
        return out

    def ln_chain(r, n, links=1, r_out=None, early=False):
        qv, yv = qb.at[rows(r, n), :], ys.at[:, rows(r, n), :]
        r_out = r if r_out is None else r_out
        xv, hv = x2s.at[rows(r_out, n), :], h2s.at[rows(r_out, n), :]
        prev = [None] * links
        cnt = 0
        for o1 in range(0, n // 2, RG):
            zz = []
            for o in (o1, o1 + n // 2):
                q = load_q(o, qv)
                x2 = make_x2(o, q, _stats(q, prev[cnt % links], early), yv)
                xv[o:o + RG, :] = x2
                st = _stats(x2)
                h2 = make_h2(xv[o:o + RG, :], st)
                hv[o:o + RG, :] = h2
                st = _stats(h2)
                z = (hv[o:o + RG, :] - st[0]) * st[1]
                zt[o // 2:(o + RG) // 2, :] = pk(z)
                prev[cnt % links] = st[1]
                cnt += 1
                zz.append(z)
            if ST1:
                for k, v in enumerate(lhs_sums(zz[0][:, 0:256], zz[0][:, 256:512], zz[1][:, 0:256], zz[1][:, 256:512])):
                    zu.at[k][o1 // 2:(o1 + RG) // 2, :] = pk(v)

    def mm_w1s(r, n, o=0):
        h, o = n // 2, o // 2
        res = sq_strassen(ub(zt[o:o + h, :]), ub(zt[o:o + h // 2, :]), ub(zt[o + h // 2:o + h, :]),
                          [ub(zu[k, 0:h // 2, :]) for k in range(5)], w1p, s1)
        for c, (ct, cb2) in res.items():
            h1s[c, rows(r + 8, h), :] = _gelu(ct)
            h1s[c, rows(r + 8 + h, h), :] = _gelu(cb2)

    def mm_w1(r, n, o=0, parts=4):
        z = pltpu.bitcast(zt[o // 2:(o + n) // 2, :], bf16)
        h1 = _gelu(_dot_balanced(z, lambda a, b: w1p[:, a:b], D, parts))
        for c in range(CT):
            h1s[c, rows(r + 8, n), :] = h1[:, c * 128:(c + 1) * 128]

    def mm_w2(r, parts=4, st=False):
        lane = jax.lax.broadcasted_iota(i32, (T, 128), 1)

        def sh(k, c):
            return h1s[c, rows(r + 8 + k, T), :]

        g = jnp.concatenate([
            sh(-1, 0),
            jnp.where(lane < 32, sh(-1, 1), sh(1, 1)),
            jnp.where(lane < 64, sh(1, 2), sh(-2, 2)),
            jnp.where(lane < 96, sh(-2, 3), sh(2, 3)),
            sh(2, 4)], axis=-1)
        if not st:
            hss[rows(r, T), :] = _dot_balanced(g, lambda a, b: w2p[:, a:b], D, parts)
            return
        top, bot = g[0:H], g[H:T]
        sums = lhs_sums(top[:, 0:256], top[:, 256:512], bot[:, 0:256], bot[:, 256:512])
        if GM == 0:
            res = sq_strassen(g, top, bot, sums, w2p, s2)
        else:
            gs[...] = pk(g)
            gu[...] = pk_many(sums)
            res = sq_strassen(ub(gs[...]), ub(gs[0:H // 2, :]), ub(gs[H // 2:H, :]),
                              [ub(gu[:, 256 * k:256 * (k + 1)]) for k in range(5)], w2p, s2)
        for c, (ct, cb2) in res.items():
            hss[rows(r, H), c * 128:(c + 1) * 128] = ct
            hss[rows(r + H, H), c * 128:(c + 1) * 128] = cb2

    def ln_x1(r, links=1):
        hv, sv = h2s.at[rows(r, T), :], hss.at[rows(r, T), :]
        prev = [None] * links
        n = 0
        for o in range(0, H, RG):
            zz = []
            for oo in (o, o + H):
                x1 = hv[oo:oo + RG, :] + sv[oo:oo + RG, :]
                st = _stats(x1, prev[n % links], early=True)
                z = (x1 - st[0]) * st[1]
                zb[oo // 2:(oo + RG) // 2, :] = pltpu.bitcast(z.astype(bf16), u32)
                prev[n % links] = st[1]
                n += 1
                zz.append(z)
            if ST3:
                a11, a12, a21, a22 = zz[0][:, 0:256], zz[0][:, 256:512], zz[1][:, 0:256], zz[1][:, 256:512]
                for k, v in enumerate([a11 + a22, a21 + a22, a11 + a12, a21 - a11, a12 - a22]):
                    zs.at[k][o // 2:(o + RG) // 2, :] = pk(v)

    def mm_w3(f0, parts=1, f1=FM):
        z = pltpu.bitcast(zb[...], bf16)
        return _gelu2(_dot_balanced(z, lambda a, b: w3p[(f0 + a) // 2:(f0 + b) // 2, :], f1 - f0, parts, nt=True))

    def mm_w3_first():
        z = pltpu.bitcast(zb[...], bf16)
        return _gelu2(jnp.dot(z, pltpu.bitcast(w3n[...], bf16), preferred_element_type=f32))

    def mm_w3_tail():
        z = pltpu.bitcast(zb[...], bf16)
        w = pltpu.bitcast(w3p[FM // 2:F // 2, :], bf16)
        return _gelu2(jax.lax.dot_general(w, z, NT_DIMS, preferred_element_type=f32))

    def mm_w4(r, n, act, c0=0, c1=D, parts=1):
        h = _dot_balanced(act, lambda a, b: w4p[:, c0 + a:c0 + b], c1 - c0, parts)
        x1 = h2s[rows(r, n), c0:c1] + hss[rows(r, n), c0:c1]
        if OUTF:
            base = x2s[rows(r, n), c0:c1] + mvec(4, n, c0, c1) * x1
            ob[rows(r, n), c0:c1] = (base + mvec(5, n, c0, c1) * h).astype(bf16)
        else:
            ob[rows(r, n), c0:c1] = (x2s[rows(r, n), c0:c1] + mvec(4, n, c0, c1) * (x1 + 0.5 * h)).astype(bf16)

    def prep_w3():
        for j in range(NP3):
            r0 = 128 * (2 * j + 1)
            for k in (2, 1, 0, 4, 3):
                s3[64 * j:64 * (j + 1), 256 * k:256 * (k + 1)] = pk(rhs_sum(k, lambda b: w3b[
                    r0 + 128 * (b % 2):r0 + 128 * (b % 2 + 1), 256 * (b // 2):256 * (b // 2 + 1)].astype(f32)))

    def prep_w4():
        for j in range(7):
            if j < NP3:
                r0 = 128 * (2 * j + 1)
                p4[0, 64 * j:64 * (j + 1), :] = pltpu.bitcast(w4b[r0:r0 + 128, 0:128], u32)
                p4[1, 64 * j:64 * (j + 1), :] = pltpu.bitcast(w4b[r0 + 128:r0 + 256, 0:128], u32)
            else:
                p4[0, 64 * j:64 * (j + 1), :] = pltpu.bitcast(w4b[0:128, 0:128], u32)
                p4[1, 64 * j:64 * j + 32, :] = pltpu.bitcast(w4b[FM:F, 0:128], u32)
                p4[1, 64 * j + 32:64 * (j + 1), :] = jnp.zeros((32, 128), u32)
        def block(j, b):
            if j < NP3:
                r0 = 128 * (2 * j + 1 + b // 2)
                return both(w4b, r0, r0 + 128, b % 2)
            if b < 2:
                return both(w4b, 0, 128, b % 2)
            return jnp.concatenate([both(w4b, FM, F, b % 2), jnp.zeros((64, 256), f32)], axis=0)

        for m, k in ((1, 0), (4, 2), (2, None), (3, 1), (5, None), (7, 4), (6, 3)):
            for j in range(7):
                v = block(j, 0 if m == 2 else 3) if k is None else rhs_sum(k, lambda b: block(j, b))
                o = 448 * (m - 1) + 64 * j
                s4[o:o + 64, :] = pk(v)

    def nt(a, w):
        return jax.lax.dot_general(a, w, NT_DIMS, preferred_element_type=f32)

    def w3_pair(j):
        r0 = 64 * (2 * j + 1)
        z1, z2 = ub(zb[0:H // 2, :]), ub(zb[H // 2:H, :])
        q = strassen(nt, z1[:, 0:256], z2[:, 256:512], [ub(zs[k]) for k in range(5)], z1[:, 512:D], z2[:, 512:D],
                     ub(w3p[r0:r0 + 64, 0:256]), ub(w3p[r0 + 64:r0 + 128, 256:512]), [ub(s3[64 * j:64 * (j + 1), 256 * k:256 * (k + 1)]) for k in range(5)],
                     ub(w3p[r0:r0 + 64, 512:D]), ub(w3p[r0 + 64:r0 + 128, 512:D]))
        return [_gelu2(c) for c in q]

    def put_quads(j, q):
        l1, l2, l5, l6, l7 = lhs_sums(*q)
        al[64 * j:64 * (j + 1), :] = pk_many([l1, l2, q[0], q[3], l5, l6, l7, q[1], q[2]])

    def put_edge(first, tail):
        tp = jnp.concatenate([tail.T, jnp.zeros((T, 64), f32)], axis=-1)
        put_quads(NP3, [first[0:H], tp[0:H], first[H:T], tp[H:T]])

    def w3_all(first, tail):
        put_edge(first, tail)
        for j in range(NP3):
            put_quads(j, w3_pair(j))

    def left(k):
        return jnp.concatenate([al[64 * j:64 * (j + 1), lanes(k)] for j in range(7)], axis=-1)

    def w4_plain(r, o=0, n=T):
        top = jnp.concatenate([left(2), left(7)], axis=-1)
        bot = jnp.concatenate([left(8), left(3)], axis=-1)
        a = jnp.concatenate([top, bot], axis=0)[o // 2:(o + n) // 2]
        h = nn(ub(a), ub(jnp.concatenate([p4[0], p4[1]], axis=0)))
        finish(r + o, n, h, 0, 128)

    def finish(r, n, h, c0, c1):
        x1 = h2s[rows(r, n), c0:c1] + hss[rows(r, n), c0:c1]
        base = x2s[rows(r, n), c0:c1] + mvec(4, n, c0, c1) * x1
        ob[rows(r, n), c0:c1] = (base + mvec(5, n, c0, c1) * h).astype(bf16)

    def w4_steps(r, n):
        c1 = 128 + 256 * n

        def m(k):
            return nn(ub(left(k - 1)), ub(s4[448 * (k - 1):448 * k, lanes(n)]))

        if ACC:
            m1 = m(1)
            cq[0] = m1
            m4 = m(4)
            cq[2] = m4
            cq[3] = cq[0] + m4
            m2 = m(2)
            cq[0] = cq[0] - m2
            finish(r + H, H, cq[2] + m2, c1, c1 + 128)
            yield
            m3 = m(3)
            cq[1] = m3
            cq[0] = cq[0] + m3
            m5 = m(5)
            cq[3] = cq[3] - m5
            finish(r, H, cq[1] + m5, c1 + 128, c1 + 256)
            yield
            finish(r, H, cq[3] + m(7), c1, c1 + 128)
            finish(r + H, H, cq[0] + m(6), c1 + 128, c1 + 256)
            yield
            return
        m1, m4 = m(1), m(4)
        m2 = m(2)
        finish(r + H, H, m4 + m2, c1, c1 + 128)
        yield
        m3, m5 = m(3), m(5)
        finish(r, H, m3 + m5, c1 + 128, c1 + 256)
        yield
        finish(r, H, ((m1 + m4) - m5) + m(7), c1, c1 + 128)
        finish(r + H, H, ((m1 - m2) + m3) + m(6), c1 + 128, c1 + 256)
        yield

    def w4_pair(r, n):
        for _ in w4_steps(r, n):
            pass

    groups = list(range(0, P0 + P1, RG))
    with _scope("pre_a"):
        wait("w_q0", [mod_copies[0], q_copies[0]])
        sa, ca, ga = mod_part(0, 1)
        modb[0] = ga * sa
        modb[1] = ga * (1.0 + ca)
        for c in range(NL, CT):
            mac_inv(c, NB - 1)
        st1 = {o: _stats(load_q(o)) for o in groups}
        zt[0:8, 0:128] = jnp.zeros((8, 128), u32)
        st2 = {}
        for o in groups:
            x2 = make_x2(o, load_q(o), st1[o])
            x2s[o:o + RG, :] = x2
            st2[o] = _stats(x2)
    with _scope("pre_b"):
        wait("w_modB", [mod_copies[1]])
        sb, cb = mod_part(1, 2)
        modb[2] = sb
        modb[3] = 1.0 + cb
        st3 = {}
        for o in range(0, P0, RG):
            h2 = make_h2(x2s[o:o + RG, :], st2[o])
            h2s[o:o + RG, :] = h2
            st3[o] = _stats(h2)
        for o in range(0, P0, RG):
            zt[o // 2:(o + RG) // 2, :] = pack_ln(h2s[o:o + RG, :], st3[o])
    with _scope("r1"):
        wait("w_w1", [w_copies[0]])
        w1p[...] = pltpu.bitcast(w1b[...], u32)
        mm_w1(0, P0)
        prev = None
        for o1 in range(0, P1 // 2, RG):
            zz = []
            for o in (P0 + o1, P0 + o1 + P1 // 2):
                h2 = make_h2(x2s[o:o + RG, :], st2[o])
                h2s[o:o + RG, :] = h2
                st = _stats(h2, prev, early=True)
                z = (h2 - st[0]) * st[1]
                zt[o // 2:(o + RG) // 2, :] = pk(z)
                prev = st[1]
                zz.append(z)
            for k, v in enumerate(lhs_sums(zz[0][:, 0:256], zz[0][:, 256:512], zz[1][:, 0:256], zz[1][:, 256:512])):
                zu.at[k][o1 // 2:(o1 + RG) // 2, :] = pk(v)
        prep_sq(w1b, s1)
        mm_w1s(P0, P1, P0)
    with _scope("r2"):
        wait("w_w2", [w_copies[1]] + ([q_copies[1]] if R2C else []))
        w2p[...] = pltpu.bitcast(w2b[...], u32)
        prep_sq(w2b, s2)
        if R2C:
            ln_chain(P0 + P1, PA, R2C)
        mm_w2(0, st=True)
        ln_x1(0, 2)
        mm_w2(T, st=True)
    with _scope("r3"):
        wait("w_w3", ([] if R2C else [q_copies[1]]) + [w_copies[2]])
        for j in range(NP3):
            r0 = 128 * (2 * j + 1)
            w3p[r0 // 2:r0 // 2 + 64, 0:256] = pltpu.bitcast(w3b[r0:r0 + 128, 0:256], u32)
            w3p[r0 // 2:r0 // 2 + 64, 512:D] = pltpu.bitcast(w3b[r0:r0 + 128, 512:D], u32)
            w3p[r0 // 2 + 64:r0 // 2 + 128, 256:D] = pltpu.bitcast(w3b[r0 + 128:r0 + 256, 256:D], u32)
        w3p[FM // 2:F // 2, :] = pltpu.bitcast(w3b[FM:F, :], u32)
        w3n[...] = pltpu.bitcast(w3b[0:128, :].astype(f32).T.astype(bf16), u32)
        prep_w3()
        for tok in R3O:
            if tok == 'c':
                if not R2C:
                    ln_chain(P0 + P1, PA)
            elif tok == 't':
                tail = mm_w3_tail()
            elif tok == '3':
                for j in range(NP3):
                    put_quads(j, w3_pair(j))
            elif tok == 'n':
                put_edge(mm_w3_first(), tail)
            else:
                mm_w1s(P0 + P1, PA)
        if FEN4:
            jax.lax.fori_loop(0, 2, fence, 0)
    with _scope("r4"):
        wait("w_w4", [w_copies[3], mod_copies[2]])
        prep_w4()
        sc16 = jnp.broadcast_to(scb[:, 0:D], (16, D)).astype(bf16)

        def gate(c0, c1):
            gbc = jnp.dot(sc16, wmc[:, c0:c1], preferred_element_type=f32)[0:8]
            modb[4, :, c0:c1] = gbc
            modb[5, :, c0:c1] = 0.5 * gbc

        gate(0, 128)
        w4_plain(0)
        gate(128, 384)
        w4_pair(0, 0)
        gate(384, D)
        w4_pair(0, 1)
        ln_x1(T)
        out_copy(0).start()
        q_copies[2].wait()

    def mlp_body(i, carry):
        with _scope("iter"):
            r1 = pl.multiple_of(PB - PC + PC * i, 32)
            r = pl.multiple_of(i * T, T)
            for tok in LB:
                if tok == 'n':
                    first = mm_w3_first()
                elif tok == 'c':
                    ln_chain(r1, PC, CL)
                elif tok == 'd':
                    ln_chain(pl.multiple_of(jnp.minimum(r1 + PC, S - PC), 32), PC, CL, r1 + PC, CE)
                elif tok == 't':
                    tail = mm_w3_tail()
                elif tok == '3':
                    w3_all(first, tail)
                    steps = w4_steps(r, 0)
                elif tok == 's':
                    next(steps)
                elif tok == 'p':
                    w4_plain(r)
                elif tok == '1':
                    if ST1:
                        mm_w1s(r1, PC)
                    else:
                        mm_w1(r1, PC, parts=W1P)
                elif tok == 'q':
                    w4_pair(r, 0)
                elif tok == '2':
                    mm_w2(r + T, parts=W2P, st=ST2)
                elif tok == 'l':
                    ln_x1(r + T, LL)
                elif tok == 'r':
                    w4_pair(r, 1)
            out_copy(i).start()
        return carry

    with _scope("loop"):
        jax.lax.fori_loop(1, NC - 1, mlp_body, 0)
    with _scope("last"):
        first = mm_w3_first()
        tail = mm_w3_tail()
        w3_all(first, tail)
        w4_pair(S - T, 0)
        w4_pair(S - T, 1)
        out_tail[0].start()
        w4_plain(S - T, 0, LAST0)
        out_tail[1].start()
        w4_plain(S - T, LAST0, T - LAST0)
        out_tail[2].start()
    with _scope("fin"):
        for i in range(NC - 1):
            out_copy(i).wait()
        for cp in out_tail:
            cp.wait()


@jax.jit
def pallas_adaLN_cond__ssm_conv_h3__mixer_s_mlp__prompt_kernel(
    A_q: jax.Array,
    A_k: jax.Array,
    A_v: jax.Array,
    A_shift_k: jax.Array,
    A_ssm_k: jax.Array,
    A_ssm_D: jax.Array,
    B_x: jax.Array,
    B_w1: jax.Array,
    B_w2: jax.Array,
    B_w3: jax.Array,
    B_w4: jax.Array,
    c: jax.Array,
    w_mod: jax.Array,
):
    del B_x
    any_spec = pl.BlockSpec(memory_space=pl.ANY)

    def tile_view(x):
        return x.reshape(S // 8, 8, CT, 128).transpose(0, 2, 1, 3).reshape(S * CT, 128)

    vm = pltpu.VMEM
    dma = pltpu.SemaphoreType.DMA
    spec = (4, NG, 16, 128)
    out = pl.pallas_call(
        _kernel,
        in_specs=[any_spec] * 12,
        out_specs=any_spec,
        out_shape=jax.ShapeDtypeStruct((S, D), bf16),
        scratch_shapes=[
            *[vm((KROWS, 128), bf16)] * NB, *[vm((VROWS, 128), bf16)] * NB, vm((CT, 128, S), bf16),
            vm((S, D), bf16), vm((D, D), bf16), vm((D, D), bf16), vm((F, D), bf16), vm((F, D), bf16),
            vm((D // 2, D), u32), vm((D // 2, D), u32), vm((F // 2, D), u32), vm((F // 2, D), u32),
            vm((D, 3 * D), bf16), vm((D, 2 * D), bf16), vm((D, D), bf16),
            vm((4, D), bf16), vm((D,), bf16), vm((1, D), bf16), vm((1, 1792), f32),
            vm((4, 128, 128), u32), vm((4, 128, 128), u32), vm((4, 64, 256), u32),
            vm((CT, 8, 8, 128), f32),
            vm((CT, NB) + spec, f32), vm((CT, NB - 1) + spec, f32), vm((CT,) + spec, f32),
            vm((CT, NB) + spec, f32), vm((4, 128, 128), f32),
            vm((CT, S + 32, 128), f32), vm((8, 8, D), f32),
            vm((CT, S + 32, 128), f32), vm((S + 256, D), f32), vm((S + 256, D), f32), vm((S, D), f32),
            vm((288, D), u32), vm((T // 2, D), u32), vm((D // 2, 128), u32),
            vm((640, 256), u32), vm((640, 256), u32), vm((NP3 * 64, 1280), u32), vm((7 * 448, 256), u32), vm((2, 448, 128), u32), vm((7 * 64, 1152), u32),
            vm((4, H, 128), f32), vm((5, H // 2, 256), u32), vm((5, H // 2, 256), u32),
            vm((H, D), u32), vm((H // 2, 1280), u32),
            vm((S, D), bf16),
            dma((26,)), dma((NC + 2,)),
        ],
        compiler_params=pltpu.CompilerParams(vmem_limit_bytes=110 << 20, disable_bounds_checks=True,
                                             disable_semaphore_checks=True),
    )(A_q.reshape(S, D), tile_view(A_k), tile_view(A_v), A_shift_k.T, A_ssm_k,
      A_ssm_D, B_w1, B_w2, B_w3.T, B_w4, c, w_mod)
    return out.reshape(1, S, D)
```

```python
import os
import numpy as np
import jax
import jax.numpy as jnp
import jax.experimental.pallas as pl
import jax.experimental.pallas.tpu as pltpu

f32, bf16, u32, i32 = jnp.float32, jnp.bfloat16, jnp.uint32, jnp.int32

S, D, F = 2048, 640, 1728
CT = D // 128
TR = 8 * CT
NB, BLK, NFFT = 4, 512, 1024
KROWS, VROWS = BLK * CT + 128, BLK * CT + 64
NG = 16
T = 256
NC = S // T
FM = (F // 128) * 128
P0, P1, PA, PC = 320, 224, 160, 224
PB = P0 + P1 + PA
LAST0 = int(os.environ.get('LAST0', '208'))
RG = 16
EPS = 1e-5
NT_DIMS = (((1,), (1,)), ((), ()))
OUTF = int(os.environ.get('OUTF', '1'))
MODI = int(os.environ.get('MODI', '1'))
NS = [int(x) * 128 for x in os.environ.get('NS', '12')]
R3 = os.environ.get('R3', 'a31t')
SM = int(os.environ.get('SM', '0'))
TC = int(os.environ.get('TC', '512'))
TMODE = int(os.environ.get('TMODE', '0'))
LB = os.environ.get('LB', 'nct31p2lz')
W1P = int(os.environ.get('W1P', '1'))
W2P = int(os.environ.get('W2P', '1'))
RS = int(os.environ.get('RS', '0'))
W3S = int(os.environ.get('W3S', '640'))
ST3 = int(os.environ.get('ST3', '1'))
ST4 = int(os.environ.get('ST4', '1'))
LL = int(os.environ.get('LL', '1'))
H = T // 2
NP3 = 6
ST1 = int(os.environ.get('ST1', '1'))
ST2 = int(os.environ.get('ST2', '1'))
CL = int(os.environ.get('CL', '1'))
ACC = int(os.environ.get('ACC', '1'))
SORD = int(os.environ.get('SORD', '1'))
CE = int(os.environ.get('CE', '1'))
RSQ = int(os.environ.get('RSQ', '1'))
GM = int(os.environ.get('GM', '0'))
FEN4 = int(os.environ.get('FEN4', '0'))
R2C = int(os.environ.get('R2C', '2'))
R3O = os.environ.get('R3O', '1tn3')
LR = int(os.environ.get('LR', '0'))
CR = int(os.environ.get('CR', '0'))
L2 = int(os.environ.get('L2', '1'))
LA = int(os.environ.get('LA', '64'))
LX3 = int(os.environ.get('LX3', '1'))
IL4 = int(os.environ.get('IL4', '1'))
L2S = [int(x) for x in os.environ.get('L2S', '1234567')]
SAME = int(os.environ.get('SAME', '1'))
W2L2 = int(os.environ.get('W2L2', '0'))
J2 = int(os.environ.get('J2', '0'))
J0 = int(os.environ.get('J0', '2'))
JL = int(os.environ.get('JL', '2'))
STG = int(os.environ.get('STG', '0'))
D4 = int(os.environ.get('D4', '0'))
Q3 = int(os.environ.get('Q3', '0'))
CK = int(os.environ.get('CK', '5'))
LK = int(os.environ.get('LK', '0'))
GVF = int(os.environ.get("GVF", "8"))
GVI = int(os.environ.get("GVI", "8"))
NL = int(os.environ.get("NL", "4"))
SKIPCONV = int(os.environ.get("SKIPCONV", "0"))
SCOPES = bool(int(os.environ.get("KSCOPES", "0")))


class _NoScope:
    def __enter__(self):
        return self

    def __exit__(self, *a):
        return False


def _scope(name):
    return jax.named_scope(name) if SCOPES else _NoScope()


def _lo(w):
    return pltpu.bitcast(w << 16, f32)


def _hi(w):
    return pltpu.bitcast(w & jnp.uint32(0xFFFF0000), f32)


def _cis(n):
    t = (n & (2 * NFFT - 1)).astype(f32) * (np.pi / NFFT)
    return jnp.cos(t), jnp.sin(t)


def _fwd_table(r):
    g = jax.lax.broadcasted_iota(i32, (NG, 128), 0)
    cg, sg = _cis(jnp.where(g < NG // 2, 32 * g + 1, 32 * g - 253) * r)
    cs, ss = _cis(4 * jax.lax.broadcasted_iota(i32, (8, 128), 0) * r)
    parts = []
    for i in range(NG):
        c, s = cg[i:i + 1], sg[i:i + 1]
        parts += [c * cs - s * ss, -(s * cs + c * ss)]
    return pltpu.bitcast(jnp.concatenate(parts, axis=0).astype(bf16), u32)


def _inv_tables():
    def phase(rows):
        col = jax.lax.broadcasted_iota(i32, (rows, 256), 1)
        k = ((col >> 4) << 3) + (col & 7)
        row = jax.lax.broadcasted_iota(i32, (rows, 256), 0)
        return jnp.where(k < 64, 4 * k + 1, 4 * k - 253), (col & 8) << 6, row

    fr, _, g = phase(16)
    cg, sg = _cis(fr * (32 * g))
    fr, off, s = phase(8)
    out = []
    for p in range(4):
        cs, ss = _cis(fr * (4 * s + p) + off)
        cs, ss = cs * (2.0 / NFFT), ss * (2.0 / NFFT)
        parts = [cg[i:i + 1] * cs - sg[i:i + 1] * ss for i in range(16)]
        out.append(pltpu.bitcast(jnp.concatenate(parts, axis=0).astype(bf16), u32))
    return out


def _radix4(re, im, inverse):
    ar, ai = re[0] + re[2], im[0] + im[2]
    br, bi = re[0] - re[2], im[0] - im[2]
    cr, ci = re[1] + re[3], im[1] + im[3]
    dr, di = re[1] - re[3], im[1] - im[3]
    minus_i = (br + di, bi - dr)
    plus_i = (br - di, bi + dr)
    if inverse:
        return [(ar + cr, ai + ci), plus_i, (ar - cr, ai - ci), minus_i]
    return [(ar + cr, ai + ci), minus_i, (ar - cr, ai - ci), plus_i]


def _stats(x, link=None, early=False):
    zero = 0.0 if link is None else jnp.minimum(link, 0.0)
    part = x[:, 0:128]
    for c in range(1, CT):
        part = part + x[:, c * 128:(c + 1) * 128]
    if link is not None and early:
        part = part + zero
        zero = 0.0
    m = jnp.sum(part, axis=-1, keepdims=True) * (1.0 / D)
    v = jnp.maximum(jnp.sum(x * x, axis=-1, keepdims=True) * (1.0 / D) - m * m, zero)
    if RSQ:
        return m, jnp.exp2(jnp.log(v + EPS) * (-0.5 / np.log(2.0)))
    return m, jax.lax.rsqrt(v + EPS)


def _gelu2(x):
    c = 0.7978845608028654
    u = c + (c * 0.044715) * (x * x)
    return x + x * jnp.tanh(x * u)


def _gelu(x):
    c = 0.7978845608028654
    u = c + (c * 0.044715) * (x * x)
    hx = 0.5 * x
    return hx + hx * jnp.tanh(x * u)


def _dot_balanced(x, wslice, n_cols, parts, nt=False):
    def mm(a, c0, c1):
        a, w = a.astype(bf16), pltpu.bitcast(wslice(c0, c1), bf16)
        if nt:
            return jax.lax.dot_general(a, w, NT_DIMS, preferred_element_type=f32)
        return jnp.dot(a, w, preferred_element_type=f32)

    if parts == 1:
        return mm(x, 0, n_cols)
    base, extra = divmod(x.shape[0] // 16, parts)
    last, o = [], 0
    head = mm(x, 0, n_cols - 128)
    for i in range(parts):
        n = 16 * (base + (1 if i < extra else 0))
        last.append(mm(x[o:o + n], n_cols - 128, n_cols))
        o += n
    return jnp.concatenate([head, jnp.concatenate(last, axis=0)], axis=-1)


def _kernel(q_hbm, k_hbm, v_hbm, sh_hbm, sk_hbm, d_hbm, w1_hbm, w2_hbm, w3_hbm, w4_hbm,
            c_hbm, wm_hbm, o_hbm,
            kb0, kb1, kb2, kb3, vb0, vb1, vb2, vb3, skb, qb, w1b, w2b, w3b, w4b, w1p, w2p, w3p, w4p,
            wma, wmb, wmc, shb, db, cb_, scb,
            fub, fkb, gtb, par, US, KS, UR, YS, YP, ys, modb, h1s, h2s, x2s, hss, zt, zb, w3n, s1, s2, s3, s4, p4, al, cq, zs, zu, gs, gu, xt, s5, c2, t2, a2, ht, ob,
            sem, sem_o):
    n_in = [0]

    def load(src, dst):
        n_in[0] += 1
        return pltpu.make_async_copy(src, dst, sem.at[n_in[0] - 1])

    nkv = BLK * CT
    small = [load(d_hbm, db), load(sh_hbm, shb), load(c_hbm, cb_)]
    sk_copies = [load(sk_hbm.at[pl.ds(c * 128, 128), :], skb.at[c]) for c in range(CT)]
    kbs, vbs, wms = [kb0, kb1, kb2, kb3], [vb0, vb1, vb2, vb3], [wma, wmb, wmc]
    kv_copies = [[load(k_hbm.at[pl.ds(0, nkv), :], kb0.at[pl.ds(TR, nkv), :]) if a == 0 else
                  load(k_hbm.at[pl.ds(a * nkv - TR, nkv + TR), :], kbs[a].at[pl.ds(0, nkv + TR), :]),
                  load(v_hbm.at[pl.ds(a * nkv, nkv), :], vbs[a].at[pl.ds(0, nkv), :])] for a in range(NB)]
    mod_cols = [(0, 3 * D), (3 * D, 2 * D), (5 * D, D)]
    mod_copies = [load(wm_hbm.at[:, pl.ds(o, n)], w) for (o, n), w in zip(mod_cols, wms)]
    w_copies = [load(w1_hbm, w1b), load(w2_hbm, w2b), load(w3_hbm, w3b), load(w4_hbm, w4b)]
    q_copies = [load(q_hbm.at[pl.ds(o, n), :], qb.at[pl.ds(o, n), :])
                for o, n in [(0, P0 + P1), (P0 + P1, PA), (PB + PC, S - PB - PC), (PB, PC)]]

    def out_copy(i):
        r = i * T if isinstance(i, int) else pl.multiple_of(i * T, T)
        return pltpu.make_async_copy(ob.at[pl.ds(r, T), :], o_hbm.at[pl.ds(r, T), :], sem_o.at[i])

    tail_parts = [(S - T, T, 128, D), (S - T, LAST0, 0, 128), (S - T + LAST0, T - LAST0, 0, 128)]
    out_tail = [pltpu.make_async_copy(ob.at[pl.ds(o, n), pl.ds(c0, c1 - c0)], o_hbm.at[pl.ds(o, n), pl.ds(c0, c1 - c0)],
                                      sem_o.at[NC - 1 + i]) for i, (o, n, c0, c1) in enumerate(tail_parts)]

    first = small + kv_copies[0] if SM == 0 else [kv_copies[0][0]] + small + [kv_copies[0][1]]
    for cp in (first + sk_copies + kv_copies[1] + kv_copies[2] + kv_copies[3]
               + [mod_copies[0], q_copies[0], mod_copies[1], w_copies[0], w_copies[1], q_copies[1],
                  w_copies[2]] + ([w_copies[3], mod_copies[2], q_copies[3]] if (SAME or Q3) else [q_copies[3], w_copies[3], mod_copies[2]]) + [q_copies[2]]):
        cp.start()

    def wait(name, copies):
        with _scope(name):
            for cp in copies:
                cp.wait()

    def pin(i, carry):
        z = jnp.zeros((8, 128), f32)
        scb[:, pl.ds(pl.multiple_of(i * 128, 128), 128)] = z[0:1]
        YP[i, 0:8, :] = z
        US[i, 0, 0, 0, 0:8, :] = z
        KS[i, 0, 0, 0, 0:8, :] = z
        YS[i, 0, 0, 0, 0:8, :] = z
        UR[i, 0, 0, 0:8, :] = z
        cq[i, 0:8, :] = z
        r8 = pl.multiple_of(i * 8, 8)
        al[pl.ds(r8, 8), 0:128] = jnp.zeros((8, 128), u32)
        gs[pl.ds(r8, 8), 0:128] = jnp.zeros((8, 128), u32)
        xt[pl.ds(r8, 8), 0:128] = z
        c2[pl.ds(r8, 8), 0:128] = z
        ht[pl.ds(r8, 8), 0:128] = z
        a2[pl.ds(r8, 8), 0:128] = jnp.zeros((8, 128), u32)
        gu[pl.ds(r8, 8), 0:128] = jnp.zeros((8, 128), u32)
        return carry

    def fence(i, carry):
        YP[i, 0:8, :] = jnp.zeros((8, 128), f32)
        return carry

    with _scope("init"):
        jax.lax.fori_loop(0, 2, pin, 0)
        lane = jax.lax.broadcasted_iota(i32, (1, 128), 1)
        for p in range(4):
            m = (lane - p) & 3
            fkb[p] = _fwd_table(128 * m + ((lane - m) & 127))
        for c in range(CT):
            kb0[c * 8:(c + 1) * 8, :] = jnp.zeros((8, 128), bf16)
            h1s[c, 0:8, :] = jnp.zeros((8, 128), f32)
            h1s[c, S + 8:S + 16, :] = jnp.zeros((8, 128), f32)
        for a in range(NB):
            kbs[a][nkv + TR:KROWS, :] = jnp.zeros((KROWS - nkv - TR, 128), bf16)
            vbs[a][nkv:VROWS, :] = jnp.zeros((VROWS - nkv, 128), bf16)
        for p in range(4):
            fub[p] = _fwd_table(8 * (lane & 63) + ((lane >> 6) << 2) + p)
        if SM:
            for p, tab in enumerate(_inv_tables()):
                gtb[p] = tab
        wait("w_small", small)
        cvec = cb_[...].astype(f32)
        scb[:, 0:D] = cvec * jax.nn.sigmoid(cvec)
        dv = db[...].astype(f32).reshape(1, D)
        shv = shb[...].astype(f32)
        for c in range(CT):
            for i in range(4):
                par[c, i] = jnp.broadcast_to(shv[i:i + 1, c * 128:(c + 1) * 128], (8, 128))
            par[c, 4] = jnp.broadcast_to(dv[:, c * 128:(c + 1) * 128], (8, 128))
        if not SM:
            for p, tab in enumerate(_inv_tables()):
                gtb[p] = tab

    def get(ref, idx, g, n):
        return (ref[idx + (slice(g, g + n), slice(0, 8))], ref[idx + (slice(g, g + n), slice(8, 16))])

    def put(ref, idx, g, n, xr, xi):
        ref[idx + (slice(g, g + n), slice(0, 8))] = xr
        ref[idx + (slice(g, g + n), slice(8, 16))] = xi

    def split(tt, g, n):
        tt = [t[g * 16:(g + n) * 16].reshape(n, 16, 128) for t in tt]
        return [t[:, 0:8] for t in tt], [t[:, 8:16] for t in tt]

    def fwd_k(c, j):
        if SKIPCONV:
            return
        lane = jax.lax.broadcasted_iota(i32, (64, 128), 1)
        even = (lane & 1) == 0
        l01 = (lane & 2) == 0
        l12 = ((lane + 3) & 2) == 0
        rm = []
        for m in range(4):
            w = pltpu.bitcast(skb[c, :, (4 * j + m) * 128:(4 * j + m + 1) * 128], u32)
            rm.append(pltpu.roll(w, m, 1) if m else w)
        e01 = jnp.where(even, rm[0], rm[1])
        o01 = jnp.where(even, rm[1], rm[0])
        e23 = jnp.where(even, rm[2], rm[3])
        o23 = jnp.where(even, rm[3], rm[2])
        kp = [jnp.where(l01, e01, e23), jnp.where(l12, o01, o23),
              jnp.where(l01, e23, e01), jnp.where(l12, o23, o01)]
        tt = [jax.lax.dot_general(pltpu.bitcast(fkb[p], bf16), pltpu.bitcast(kp[p], bf16), NT_DIMS,
                                  preferred_element_type=f32) for p in range(4)]
        for g in range(0, NG, GVF):
            re, im = split(tt, g, GVF)
            if j == 0:
                re[0] = re[0] + par[c, 4][None]
            for m, (xr, xi) in enumerate(_radix4(re, im, False)):
                if j < NB - 1:
                    put(KS, (c, j, m), g, GVF, xr, xi)
                ur, ui = get(US, (c, 0, m), g, GVF)
                put(YS, (c, j, m), g, GVF, xr * ur - xi * ui, xr * ui + xi * ur)

    def fwd_u(c, a):
        if SKIPCONV:
            return
        taps = [jnp.tile(par[c, i], (8, 1)) for i in range(4)]
        ws = TR // 2
        base = 4 * c
        kw, vw = kbs[a].bitcast(u32), vbs[a].bitcast(u32)

        def words(ref, start):
            return ref[pl.ds(start, BLK // 8, stride=ws), :]

        kk = {}
        for w in range(4):
            x = words(kw, ws + base + w)
            kk[2 * w], kk[2 * w + 1] = _lo(x), _hi(x)
        kk[-3] = _hi(words(kw, base + 2))
        x = words(kw, base + 3)
        kk[-2], kk[-1] = _lo(x), _hi(x)
        sub = []
        for w in range(4):
            x = words(vw, base + w)
            for r, vv in ((2 * w, _lo(x)), (2 * w + 1, _hi(x))):
                sh = taps[0] * kk[r] + taps[1] * kk[r - 1] + taps[2] * kk[r - 2] + taps[3] * kk[r - 3]
                sub.append(sh * vv)
        kv = [jnp.concatenate([sub[p], sub[p + 4]], axis=0) for p in range(4)]
        tt = [jnp.dot(pltpu.bitcast(fub[p], bf16), kv[p].astype(bf16), preferred_element_type=f32)
              for p in range(4)]
        for g in range(0, NG, GVF):
            re, im = split(tt, g, GVF)
            for m, (xr, xi) in enumerate(_radix4(re, im, False)):
                if a:
                    pr, pi = get(US, (c, 0, m), g, GVF) if a == 1 else get(UR, (c, m), g, GVF)
                    if a < NB - 1:
                        put(UR, (c, m), g, GVF, xr, xi)
                    xr, xi = (xr - pi, xi + pr) if g < NG // 2 else (xr + pi, xi - pr)
                put(US, (c, a, m), g, GVF, xr, xi)

    def mac_inv(c, a):
        if SKIPCONV:
            return
        for h in range(2):
            vals = [[] for _ in range(4)]
            for g in range(8 * h, 8 * h + 8, GVI):
                yre, yim = [], []
                for m in range(4):
                    yr, yi = get(YS, (c, a, m), g, GVI)
                    for j in range(a):
                        kr, ki = get(KS, (c, j, m), g, GVI)
                        ur, ui = get(US, (c, a - j, m), g, GVI)
                        yr = yr + (kr * ur - ki * ui)
                        yi = yi + (kr * ui + ki * ur)
                    yre.append(yr)
                    yim.append(yi)
                for p, (pr, pi) in enumerate(_radix4(yre, yim, True)):
                    vals[p].append(jnp.concatenate([pr, pi], axis=1))
            for p in range(4):
                pb = jnp.concatenate(vals[p], axis=0).reshape(128, 128).astype(bf16)
                r = jnp.dot(pltpu.bitcast(gtb[p, :, h * 128:(h + 1) * 128], bf16), pb,
                            preferred_element_type=f32)
                if h == 0:
                    YP[p] = r
                else:
                    ys[c, pl.ds(a * BLK + p, 128, stride=4), :] = YP[p] + r

    with _scope("conv_u0"):
        wait("w_kv", kv_copies[0])
        for c in range(CT):
            fwd_u(c, 0)
    with _scope("conv_k"):
        for grp in ((0,), (1, 2), (3, 4)):
            wait("w_sk", [sk_copies[c] for c in grp])
            for c in grp:
                for j in (3, 2, 1, 0):
                    fwd_k(c, j)
    for a in range(1, NB):
        with _scope("conv_u%d" % a):
            wait("w_kv", kv_copies[a])
            for c in range(CT):
                fwd_u(c, a)
                mac_inv(c, a - 1)
    with _scope("conv_last"):
        jax.lax.fori_loop(0, 2, fence, 0)
        for c in range(NL):
            mac_inv(c, NB - 1)

    def mod_part(part, extra):
        n, wm = mod_cols[part][1], wms[part]
        act = scb[:, 0:D]

        def sc(k0, k1):
            return jnp.broadcast_to(act[:, k0:k1], (16, k1 - k0)).astype(bf16)

        e = 128 * extra
        r = jnp.dot(sc(0, D), wm[:, e:n], preferred_element_type=f32)
        r0 = (jnp.dot(sc(0, D - 64), wm[0:D - 64, 0:e], preferred_element_type=f32)
              + jnp.dot(sc(D - 64, D), wm[D - 64:D, 0:e], preferred_element_type=f32))
        r = jnp.concatenate([r0, r], axis=-1)[0:8]
        return [r[:, i * D:(i + 1) * D] for i in range(n // D)]

    def mvec(i, n=RG, c0=0, c1=D):
        return jnp.tile(modb[i, :, c0:c1], (n // 8, 1))

    rows = pl.ds

    def load_q(r, ref=qb):
        return ref[rows(r, RG), :].astype(f32)

    def make_x2(r, q, st, ref=ys):
        y = jnp.concatenate([ref[c, rows(r, RG), :] for c in range(CT)], axis=-1)
        return q + (((q - st[0]) * st[1]) * mvec(1) + mvec(0)) * y

    def make_h2(x2, st):
        return ((x2 - st[0]) * st[1]) * mvec(3) + mvec(2)

    def pack_ln(x, st):
        return pltpu.bitcast(((x - st[0]) * st[1]).astype(bf16), u32)

    def lhs_sums(a11, a12, a21, a22):
        return [a11 + a22, a21 + a22, a11 + a12, a21 - a11, a12 - a22]

    def rhs_sums(b11, b12, b21, b22):
        return [b11 + b22, b12 - b22, b21 - b11, b11 + b12, b21 + b22]

    RHS = [(0, 3, 1), (1, 3, -1), (2, 0, -1), (0, 1, 1), (2, 3, 1)]

    def rhs_sum(k, block):
        a, b, sg = RHS[k]
        return block(a) + block(b) if sg > 0 else block(a) - block(b)

    def pk(x):
        return pltpu.bitcast(x.astype(bf16), u32)

    def pk_many(vals):
        return pk(jnp.concatenate(vals, axis=-1))

    def lanes(k):
        return slice(128 * k, 128 * (k + 1))

    def ub(x):
        return pltpu.bitcast(x, bf16)

    def strassen(dot, a11, a22, asum, ax1, ax2, b11, b22, bsum, bx1, bx2):
        if SORD:
            m2 = dot(asum[1], b11)
            m4 = dot(a22, bsum[2])
            c21 = (m4 + m2) + dot(ax2, bx1)
            m3 = dot(a11, bsum[1])
            m5 = dot(asum[2], b22)
            c12 = (m3 + m5) + dot(ax1, bx2)
            m1 = dot(asum[0], bsum[0])
            c11 = (((m4 - m5) + m1) + dot(asum[4], bsum[4])) + dot(ax1, bx1)
            c22 = (((m3 - m2) + m1) + dot(asum[3], bsum[3])) + dot(ax2, bx2)
            return [c11, c12, c21, c22]
        m1 = dot(asum[0], bsum[0])
        m4 = dot(a22, bsum[2])
        m2 = dot(asum[1], b11)
        m3 = dot(a11, bsum[1])
        m5 = dot(asum[2], b22)
        x12 = dot(ax1, bx2)
        x21 = dot(ax2, bx1)
        m7 = dot(asum[4], bsum[4])
        x11 = dot(ax1, bx1)
        m6 = dot(asum[3], bsum[3])
        x22 = dot(ax2, bx2)
        return [(((m1 + m4) - m5) + m7) + x11, (m3 + m5) + x12, (m4 + m2) + x21, (((m1 - m2) + m3) + m6) + x22]

    def nn(a, w):
        return jnp.dot(a.astype(bf16), w, preferred_element_type=f32)

    def both(ref, r0, r1, col):
        return jnp.concatenate([ref[r0:r1, lanes(1 + col)].astype(f32), ref[r0:r1, lanes(3 + col)].astype(f32)], axis=-1)

    def prep_sq(wb, sw):
        for k in (2, 1, 0, 4, 3):
            sw[128 * k:128 * (k + 1), :] = pk(rhs_sum(k, lambda b: both(wb, 256 * (b // 2), 256 * (b // 2 + 1), b % 2)))

    def sq_strassen(a, top, bot, asum, wp, sw):
        h = top.shape[0]
        c0 = nn(a, ub(wp[:, 0:128]))
        out = {0: (c0[0:h], c0[h:2 * h])}
        for n in range(2):
            c1, c2 = 128 + 256 * n, 256 + 256 * n
            q = strassen(nn, top[:, 0:256], bot[:, 256:512], asum, top[:, 512:D], bot[:, 512:D],
                         ub(wp[0:128, c1:c2]), ub(wp[128:256, c2:c2 + 128]), [ub(sw[128 * k:128 * (k + 1), lanes(n)]) for k in range(5)],
                         ub(wp[256:320, c1:c2]), ub(wp[256:320, c2:c2 + 128]))
            out[2 * n + 1] = (q[0], q[2])
            out[2 * n + 2] = (q[1], q[3])
        return out

    ORDER = (2, 4, 3, 5, 1, 7, 6)
    LHS = {1: (0, 3, 1), 2: (2, 3, 1), 3: (0, None, 0), 4: (3, None, 0), 5: (0, 1, 1), 6: (2, 0, -1), 7: (1, 3, -1)}
    RHS7 = {1: (0, 3, 1), 2: (0, None, 0), 3: (1, 3, -1), 4: (2, 0, -1), 5: (3, None, 0), 6: (0, 1, 1), 7: (2, 3, 1)}

    def comb(rule, blk):
        a, b, sg = rule
        return blk(a) if b is None else blk(a) + blk(b) if sg > 0 else blk(a) - blk(b)

    def quad(x, b):
        h, w = x.shape[0] // 2, x.shape[1] // 2
        return x[h * (b // 2):h * (b // 2 + 1), w * (b % 2):w * (b % 2 + 1)]

    def join(m):
        c21 = m[4] + m[2]
        c12 = m[3] + m[5]
        c11 = ((m[4] - m[5]) + m[1]) + m[7]
        c22 = ((m[3] - m[2]) + m[1]) + m[6]
        return jnp.concatenate([jnp.concatenate([c11, c12], axis=-1), jnp.concatenate([c21, c22], axis=-1)], axis=0)

    def prep_sq2(wb, tab):
        for m in ORDER:
            b1 = comb(RHS7[m], lambda b: wb[256 * (b // 2):256 * (b // 2 + 1), 128 + 256 * (b % 2):384 + 256 * (b % 2)].astype(f32))
            tab[64 * (m - 1):64 * m, :] = pk_many([comb(RHS7[k], lambda b: quad(b1, b)) for k in range(1, 8)])

    def sq_strassen2(a, wp, tab):
        c0 = nn(a, ub(wp[:, 0:128]))
        prods = {}
        for m in ORDER:
            a1 = comb(LHS[m], lambda b: quad(a[:, 0:512], b))
            prods[m] = join({k: nn(comb(LHS[k], lambda b: quad(a1, b)), ub(tab[64 * (m - 1):64 * m, lanes(k - 1)]))
                             for k in ORDER})
        rest = nn(a[:, 512:D], ub(wp[256:320, 128:D]))
        return jnp.concatenate([c0, join(prods) + rest], axis=-1)

    def ln_chain(r, n, links=1, r_out=None, early=False, staged=False, skip=0):
        qv, yv = qb.at[rows(r, n), :], ys.at[:, rows(r, n), :]
        r_out = r if r_out is None else r_out
        xv, hv = (xt, ht) if staged else (x2s.at[rows(r_out, n), :], h2s.at[rows(r_out, n), :])
        prev = [None] * links
        cnt = 0
        for o1 in range(0, n // 2, RG):
            zz, sts = [], []
            for o in (o1, o1 + n // 2):
                q = load_q(o, qv)
                st = _stats(q, prev[cnt % links], early)
                if CR & 1:
                    xv[o:o + RG, :] = q
                    q = xv[o:o + RG, :]
                x2 = make_x2(o, q, st, yv)
                xv[o:o + RG, :] = x2
                st = _stats(x2)
                h2 = make_h2(xv[o:o + RG, :], st)
                hv[o:o + RG, :] = h2
                st = _stats(h2)
                if CR & 2:
                    sts.append(st)
                else:
                    z = (hv[o:o + RG, :] - st[0]) * st[1]
                    zt[o // 2:(o + RG) // 2, :] = pk(z)
                    zz.append(z)
                if skip and cnt % skip == 0:
                    pend = st[1]
                elif skip and cnt % skip == 1:
                    prev[0] = jnp.minimum(st[1], pend)
                else:
                    prev[cnt % links] = st[1]
                cnt += 1
            if CR & 2:
                for o, st in zip((o1, o1 + n // 2), sts):
                    z = (hv[o:o + RG, :] - st[0]) * st[1]
                    zt[o // 2:(o + RG) // 2, :] = pk(z)
                    zz.append(z)
            if ST1:
                for k, v in enumerate(lhs_sums(zz[0][:, 0:256], zz[0][:, 256:512], zz[1][:, 0:256], zz[1][:, 256:512])):
                    zu.at[k][o1 // 2:(o1 + RG) // 2, :] = pk(v)

    def mm_w1s(r, n, o=0):
        h, o = n // 2, o // 2
        res = sq_strassen(ub(zt[o:o + h, :]), ub(zt[o:o + h // 2, :]), ub(zt[o + h // 2:o + h, :]),
                          [ub(zu[k, 0:h // 2, :]) for k in range(5)], w1p, s1)
        for c, (ct, cb2) in res.items():
            h1s[c, rows(r + 8, h), :] = _gelu(ct)
            h1s[c, rows(r + 8 + h, h), :] = _gelu(cb2)

    def mm_w1(r, n, o=0, parts=4):
        z = pltpu.bitcast(zt[o // 2:(o + n) // 2, :], bf16)
        h1 = _gelu(_dot_balanced(z, lambda a, b: w1p[:, a:b], D, parts))
        for c in range(CT):
            h1s[c, rows(r + 8, n), :] = h1[:, c * 128:(c + 1) * 128]

    def mm_w2(r, parts=4, st=False):
        lane = jax.lax.broadcasted_iota(i32, (T, 128), 1)

        def sh(k, c):
            return h1s[c, rows(r + 8 + k, T), :]

        g = jnp.concatenate([
            sh(-1, 0),
            jnp.where(lane < 32, sh(-1, 1), sh(1, 1)),
            jnp.where(lane < 64, sh(1, 2), sh(-2, 2)),
            jnp.where(lane < 96, sh(-2, 3), sh(2, 3)),
            sh(2, 4)], axis=-1)
        if not st:
            hss[rows(r, T), :] = _dot_balanced(g, lambda a, b: w2p[:, a:b], D, parts)
            return
        if W2L2:
            hss[rows(r, T), :] = sq_strassen2(g, w2p, t2)
            return
        top, bot = g[0:H], g[H:T]
        sums = lhs_sums(top[:, 0:256], top[:, 256:512], bot[:, 0:256], bot[:, 256:512])
        if GM == 0:
            res = sq_strassen(g, top, bot, sums, w2p, s2)
        else:
            gs[...] = pk(g)
            gu[...] = pk_many(sums)
            res = sq_strassen(ub(gs[...]), ub(gs[0:H // 2, :]), ub(gs[H // 2:H, :]),
                              [ub(gu[:, 256 * k:256 * (k + 1)]) for k in range(5)], w2p, s2)
        for c, (ct, cb2) in res.items():
            hss[rows(r, H), c * 128:(c + 1) * 128] = ct
            hss[rows(r + H, H), c * 128:(c + 1) * 128] = cb2

    def ln_x1(r, links=1, skip=0):
        hv, sv = h2s.at[rows(r, T), :], hss.at[rows(r, T), :]
        prev = [None] * links
        n = 0
        for o in range(0, H, RG):
            zz, sts = [], []
            for oo in (o, o + H):
                x1 = hv[oo:oo + RG, :] + sv[oo:oo + RG, :]
                st = _stats(x1, prev[n % links], early=True)
                if LR:
                    xt[oo:oo + RG, :] = x1
                    sts.append(st)
                else:
                    z = (x1 - st[0]) * st[1]
                    zb[oo // 2:(oo + RG) // 2, :] = pk(z)
                    zz.append(z)
                if skip and n % skip == 0:
                    pend = st[1]
                elif skip and n % skip == 1:
                    prev[0] = jnp.minimum(st[1], pend)
                else:
                    prev[n % links] = st[1]
                n += 1
            if LR:
                for oo, st in zip((o, o + H), sts):
                    z = (xt[oo:oo + RG, :] - st[0]) * st[1]
                    zb[oo // 2:(oo + RG) // 2, :] = pk(z)
                    zz.append(z)
            for k, v in enumerate(lhs_sums(zz[0][:, 0:256], zz[0][:, 256:512], zz[1][:, 0:256], zz[1][:, 256:512])):
                zs.at[k][o // 2:(o + RG) // 2, :] = pk(v)

    def mm_w3(f0, parts=1, f1=FM):
        z = pltpu.bitcast(zb[...], bf16)
        return _gelu2(_dot_balanced(z, lambda a, b: w3p[(f0 + a) // 2:(f0 + b) // 2, :], f1 - f0, parts, nt=True))

    def mm_w3_first():
        z = pltpu.bitcast(zb[...], bf16)
        return _gelu2(jnp.dot(z, pltpu.bitcast(w3n[...], bf16), preferred_element_type=f32))

    def mm_w3_tail():
        z = pltpu.bitcast(zb[...], bf16)
        w = pltpu.bitcast(w3p[FM // 2:F // 2, :], bf16)
        return _gelu2(jax.lax.dot_general(w, z, NT_DIMS, preferred_element_type=f32))

    def mm_w4(r, n, act, c0=0, c1=D, parts=1):
        h = _dot_balanced(act, lambda a, b: w4p[:, c0 + a:c0 + b], c1 - c0, parts)
        x1 = h2s[rows(r, n), c0:c1] + hss[rows(r, n), c0:c1]
        if OUTF:
            base = x2s[rows(r, n), c0:c1] + mvec(4, n, c0, c1) * x1
            ob[rows(r, n), c0:c1] = (base + mvec(5, n, c0, c1) * h).astype(bf16)
        else:
            ob[rows(r, n), c0:c1] = (x2s[rows(r, n), c0:c1] + mvec(4, n, c0, c1) * (x1 + 0.5 * h)).astype(bf16)

    def prep_w3():
        for j in range(NP3):
            r0 = 128 * (2 * j + 1)
            for k in (2, 1, 0, 4, 3):
                s3[64 * j:64 * (j + 1), 256 * k:256 * (k + 1)] = pk(rhs_sum(k, lambda b: w3b[
                    r0 + 128 * (b % 2):r0 + 128 * (b % 2 + 1), 256 * (b // 2):256 * (b // 2 + 1)].astype(f32)))

    def r2_block(m, b, axis):
        o = 448 * (m - 1) + 64 * (b // 2)
        return jnp.concatenate([s4[o + 128 * i:o + 128 * i + 64, lanes(b % 2)] for i in range(3)], axis=axis)

    def w4_product(m, J2):
        if m not in L2S:
            return nn(ub(left(m - 1)), ub(s4[448 * (m - 1):448 * m, :]))

        def blk(b):
            o = 64 * (b % 2) + 32 * (b // 2)
            return ub(jnp.concatenate([al[o + 128 * i:o + 128 * i + 32, lanes(m - 1)] for i in range(3)], axis=-1))

        if J2:
            asum = [ub(jnp.concatenate([a2[32 * (3 * (m - 1) + i):32 * (3 * (m - 1) + i + 1), lanes(k)]
                                        for i in range(3)], axis=-1)) for k in range(5)]
        else:
            asum = lhs_sums(*[blk(b).astype(f32) for b in range(4)])
        bsum = [ub(jnp.concatenate([s5[64 * (5 * (m - 1) + k):64 * (5 * (m - 1) + k + 1), lanes(i)]
                                    for i in range(3)], axis=0)) for k in range(5)]
        ox = 448 * (m - 1) + 384
        q = strassen(nn, blk(0), blk(3), asum, ub(al[384:416, lanes(m - 1)]), ub(al[416:448, lanes(m - 1)]),
                     ub(r2_block(m, 0, 0)), ub(r2_block(m, 3, 0)), bsum,
                     ub(s4[ox:ox + 64, lanes(0)]), ub(s4[ox:ox + 64, lanes(1)]))
        return jnp.concatenate([jnp.concatenate(q[0:2], axis=-1), jnp.concatenate(q[2:4], axis=-1)], axis=0)

    def w4_steps2(r, J2):
        def acc(i):
            return c2.at[H * i:H * (i + 1), :]

        def fin2(rr, h, t):
            finish(rr, H, h[:, 0:128], 128 * t, 128 * (t + 1))
            finish(rr, H, h[:, 128:256], 128 * (t + 2), 128 * (t + 3))

        acc(0)[...] = w4_product(1, J2)
        yield
        m4 = w4_product(4, J2)
        acc(2)[...] = m4
        acc(3)[...] = acc(0)[...] + m4
        yield
        m2 = w4_product(2, J2)
        acc(0)[...] = acc(0)[...] - m2
        fin2(r + H, acc(2)[...] + m2, 1)
        yield
        m3 = w4_product(3, J2)
        acc(1)[...] = m3
        acc(0)[...] = acc(0)[...] + m3
        yield
        m5 = w4_product(5, J2)
        acc(3)[...] = acc(3)[...] - m5
        fin2(r, acc(1)[...] + m5, 2)
        yield
        fin2(r, acc(3)[...] + w4_product(7, J2), 1)
        yield
        fin2(r + H, acc(0)[...] + w4_product(6, J2), 2)
        yield

    def prep_w4():
        for j in range(7):
            if j < NP3:
                r0 = 128 * (2 * j + 1)
                p4[0, 64 * j:64 * (j + 1), :] = pltpu.bitcast(w4b[r0:r0 + 128, 0:128], u32)
                p4[1, 64 * j:64 * (j + 1), :] = pltpu.bitcast(w4b[r0 + 128:r0 + 256, 0:128], u32)
            else:
                p4[0, 64 * j:64 * (j + 1), :] = pltpu.bitcast(w4b[0:128, 0:128], u32)
                p4[1, 64 * j:64 * j + 32, :] = pltpu.bitcast(w4b[FM:F, 0:128], u32)
                p4[1, 64 * j + 32:64 * (j + 1), :] = jnp.zeros((32, 128), u32)
        def block(j, b):
            if j < NP3:
                r0 = 128 * (2 * j + 1 + b // 2)
                return both(w4b, r0, r0 + 128, b % 2)
            if b < 2:
                return both(w4b, 0, 128, b % 2)
            return jnp.concatenate([both(w4b, FM, F, b % 2), jnp.zeros((64, 256), f32)], axis=0)

        for m, k in ((1, 0), (4, 2), (2, None), (3, 1), (5, None), (7, 4), (6, 3)):
            for j in range(7):
                o = 448 * (m - 1) + 64 * j
                if k is None and (j < NP3 or m == 2):
                    r0 = 0 if j == NP3 else 128 * (2 * j + (1 if m == 2 else 2))
                    for n in range(2):
                        s4[o:o + 64, lanes(n)] = pltpu.bitcast(w4b[r0:r0 + 128, lanes(2 * n + (1 if m == 2 else 2))], u32)
                else:
                    s4[o:o + 64, :] = pk(block(j, 3) if k is None else rhs_sum(k, lambda b: block(j, b)))
            if m in L2S:
                for k2 in (2, 1, 0, 4, 3):
                    o = 64 * (5 * (m - 1) + k2)
                    s5[o:o + 64, :] = pk(rhs_sum(k2, lambda b: ub(r2_block(m, b, -1)).astype(f32)))

    def nt(a, w):
        return jax.lax.dot_general(a, w, NT_DIMS, preferred_element_type=f32)

    def w3_pair(j):
        r0 = 64 * (2 * j + 1)
        z1, z2 = ub(zb[0:H // 2, :]), ub(zb[H // 2:H, :])
        q = strassen(nt, z1[:, 0:256], z2[:, 256:512], [ub(zs[k]) for k in range(5)], z1[:, 512:D], z2[:, 512:D],
                     ub(w3p[r0:r0 + 64, 0:256]), ub(w3p[r0 + 64:r0 + 128, 256:512]), [ub(s3[64 * j:64 * (j + 1), 256 * k:256 * (k + 1)]) for k in range(5)],
                     ub(w3p[r0:r0 + 64, 512:D]), ub(w3p[r0 + 64:r0 + 128, 512:D]))
        return [_gelu2(c) for c in q]

    def put_quads(j, q):
        l1, l2, l5, l6, l7 = lhs_sums(*q)
        al[64 * j:64 * (j + 1), :] = pk_many([l1, l2, q[0], q[3], l5, l6, l7, q[1], q[2]])

    def put_two(i, qa, qb_):
        ops = []
        for j, q in ((2 * i, qa), (2 * i + 1, qb_)):
            l1, l2, l5, l6, l7 = lhs_sums(*q)
            ops.append([l1, l2, q[0], q[3], l5, l6, l7])
            half = slice(0, 64) if j % 2 == 0 else slice(64, 128)
            o = 64 * j + 32 * (j % 2)
            al[o:o + 32, 0:256] = pk_many([l1[half], l2[half]])
            al[o:o + 32, 512:896] = pk_many([l5[half], l6[half], l7[half]])
            al[64 * j:64 * (j + 1), 256:512] = pk_many([q[0], q[3]])
            al[64 * j:64 * (j + 1), 896:1152] = pk_many([q[1], q[2]])
        for m in range(7):
            e, o = ops[0][m], ops[1][m]
            r0 = 32 * (3 * m + i)
            a2[r0:r0 + 32, :] = pk_many(lhs_sums(e[0:64], o[0:64], e[64:128], o[64:128]))

    def w3_two(i):
        z1, z2 = ub(zb[0:H // 2, :]), ub(zb[H // 2:H, :])

        def wt(par, c0, c1):
            return ub(jnp.concatenate([w3p[64 * (2 * j + 1 + par):64 * (2 * j + 2 + par), c0:c1]
                                       for j in (2 * i, 2 * i + 1)], axis=0))

        q = strassen(nt, z1[:, 0:256], z2[:, 256:512], [ub(zs[k]) for k in range(5)], z1[:, 512:D], z2[:, 512:D],
                     wt(0, 0, 256), wt(1, 256, 512),
                     [ub(s3[128 * i:128 * (i + 1), 256 * k:256 * (k + 1)]) for k in range(5)], wt(0, 512, D), wt(1, 512, D))
        q = [_gelu2(c) for c in q]
        return [c[:, 0:128] for c in q], [c[:, 128:256] for c in q]

    def w3_pairs(J2):
        if J2 == 0:
            for j in range(NP3):
                put_quads(j, w3_pair(j))
        for i in range(3):
            if J2 == 1:
                put_two(i, *w3_two(i))
            elif J2 == 2:
                qa = w3_pair(2 * i)
                put_two(i, qa, w3_pair(2 * i + 1))

    def put_edge(first, tail):
        tp = jnp.concatenate([tail.T, jnp.zeros((T, 64), f32)], axis=-1)
        put_quads(NP3, [first[0:H], tp[0:H], first[H:T], tp[H:T]])

    def w3_all(first, tail, J2):
        put_edge(first, tail)
        w3_pairs(J2)

    def left(k):
        return jnp.concatenate([al[64 * j:64 * (j + 1), lanes(k)] for j in range(7)], axis=-1)

    def w4_plain(r, o=0, n=T):
        top = jnp.concatenate([left(2), left(7)], axis=-1)
        bot = jnp.concatenate([left(8), left(3)], axis=-1)
        a = jnp.concatenate([top, bot], axis=0)[o // 2:(o + n) // 2]
        h = nn(ub(a), ub(jnp.concatenate([p4[0], p4[1]], axis=0)))
        finish(r + o, n, h, 0, 128)

    def finish(r, n, h, c0, c1):
        x1 = h2s[rows(r, n), c0:c1] + hss[rows(r, n), c0:c1]
        base = x2s[rows(r, n), c0:c1] + mvec(4, n, c0, c1) * x1
        ob[rows(r, n), c0:c1] = (base + mvec(5, n, c0, c1) * h).astype(bf16)

    def w4_steps(r, n):
        c1 = 128 + 256 * n

        def m(k):
            return nn(ub(left(k - 1)), ub(s4[448 * (k - 1):448 * k, lanes(n)]))

        if ACC:
            m1 = m(1)
            cq[0] = m1
            m4 = m(4)
            cq[2] = m4
            cq[3] = cq[0] + m4
            m2 = m(2)
            cq[0] = cq[0] - m2
            finish(r + H, H, cq[2] + m2, c1, c1 + 128)
            yield
            m3 = m(3)
            cq[1] = m3
            cq[0] = cq[0] + m3
            m5 = m(5)
            cq[3] = cq[3] - m5
            finish(r, H, cq[1] + m5, c1 + 128, c1 + 256)
            yield
            finish(r, H, cq[3] + m(7), c1, c1 + 128)
            finish(r + H, H, cq[0] + m(6), c1 + 128, c1 + 256)
            yield
            return
        m1, m4 = m(1), m(4)
        m2 = m(2)
        finish(r + H, H, m4 + m2, c1, c1 + 128)
        yield
        m3, m5 = m(3), m(5)
        finish(r, H, m3 + m5, c1 + 128, c1 + 256)
        yield
        finish(r, H, ((m1 + m4) - m5) + m(7), c1, c1 + 128)
        finish(r + H, H, ((m1 - m2) + m3) + m(6), c1 + 128, c1 + 256)
        yield

    def w4_pair(r, n):
        for _ in w4_steps(r, n):
            pass

    groups = list(range(0, P0 + P1, RG))
    with _scope("pre_a"):
        wait("w_q0", [mod_copies[0], q_copies[0]])
        sa, ca, ga = mod_part(0, 1)
        modb[0] = ga * sa
        modb[1] = ga * (1.0 + ca)
        for c in range(NL, CT):
            mac_inv(c, NB - 1)
        st1 = {o: _stats(load_q(o)) for o in groups}
        zt[0:8, 0:128] = jnp.zeros((8, 128), u32)
        st2 = {}
        for o in groups:
            x2 = make_x2(o, load_q(o), st1[o])
            x2s[o:o + RG, :] = x2
            st2[o] = _stats(x2)
    with _scope("pre_b"):
        wait("w_modB", [mod_copies[1]])
        sb, cb = mod_part(1, 2)
        modb[2] = sb
        modb[3] = 1.0 + cb
        st3 = {}
        for o in range(0, P0, RG):
            h2 = make_h2(x2s[o:o + RG, :], st2[o])
            h2s[o:o + RG, :] = h2
            st3[o] = _stats(h2)
        for o in range(0, P0, RG):
            zt[o // 2:(o + RG) // 2, :] = pack_ln(h2s[o:o + RG, :], st3[o])
    with _scope("r1"):
        wait("w_w1", [w_copies[0]])
        w1p[...] = pltpu.bitcast(w1b[...], u32)
        mm_w1(0, P0)
        prev = None
        for o1 in range(0, P1 // 2, RG):
            zz = []
            for o in (P0 + o1, P0 + o1 + P1 // 2):
                h2 = make_h2(x2s[o:o + RG, :], st2[o])
                h2s[o:o + RG, :] = h2
                st = _stats(h2, prev, early=True)
                z = (h2 - st[0]) * st[1]
                zt[o // 2:(o + RG) // 2, :] = pk(z)
                prev = st[1]
                zz.append(z)
            for k, v in enumerate(lhs_sums(zz[0][:, 0:256], zz[0][:, 256:512], zz[1][:, 0:256], zz[1][:, 256:512])):
                zu.at[k][o1 // 2:(o1 + RG) // 2, :] = pk(v)
        prep_sq(w1b, s1)
        mm_w1s(P0, P1, P0)
    with _scope("r2"):
        wait("w_w2", [w_copies[1]] + ([q_copies[1]] if R2C else []))
        w2p[...] = pltpu.bitcast(w2b[...], u32)
        if W2L2:
            prep_sq2(w2b, t2)
        else:
            prep_sq(w2b, s2)
        if R2C:
            ln_chain(P0 + P1, PA, R2C)
        mm_w2(0, st=True)
        ln_x1(0, 2)
        mm_w2(T, st=True)
    with _scope("r3"):
        wait("w_w3", ([] if R2C else [q_copies[1]]) + [w_copies[2]] + ([] if (SAME or Q3) else [q_copies[3]]))
        for j in range(NP3):
            r0 = 128 * (2 * j + 1)
            w3p[r0 // 2:r0 // 2 + 64, 0:256] = pltpu.bitcast(w3b[r0:r0 + 128, 0:256], u32)
            w3p[r0 // 2:r0 // 2 + 64, 512:D] = pltpu.bitcast(w3b[r0:r0 + 128, 512:D], u32)
            w3p[r0 // 2 + 64:r0 // 2 + 128, 256:D] = pltpu.bitcast(w3b[r0 + 128:r0 + 256, 256:D], u32)
        w3p[FM // 2:F // 2, :] = pltpu.bitcast(w3b[FM:F, :], u32)
        w3n[...] = pltpu.bitcast(w3b[0:128, :].astype(f32).T.astype(bf16), u32)
        prep_w3()
        for tok in R3O:
            if tok == 'c':
                if not R2C:
                    ln_chain(P0 + P1, PA)
            elif tok == 'd':
                ln_chain(PB, PC, staged=STG)
            elif tok == 'l':
                ln_x1(T, 2)
            elif tok == 't':
                tail = mm_w3_tail()
            elif tok == '3':
                w3_pairs(J0)
            elif tok == 'n':
                put_edge(mm_w3_first(), tail)
            else:
                mm_w1s(P0 + P1, PA)
        if FEN4:
            jax.lax.fori_loop(0, 2, fence, 0)
    with _scope("r4"):
        wait("w_w4", [w_copies[3], mod_copies[2]] + ([q_copies[3]] if Q3 else []))
        prep_w4()
        sc16 = jnp.broadcast_to(scb[:, 0:D], (16, D)).astype(bf16)

        def gate(c0, c1):
            gbc = jnp.dot(sc16, wmc[:, c0:c1], preferred_element_type=f32)[0:8]
            modb[4, :, c0:c1] = gbc
            modb[5, :, c0:c1] = 0.5 * gbc

        if D4:
            ln_chain(PB, PC, D4)
        st0 = w4_steps2(0, J0)
        if IL4:
            h = None
            for j in range(7):
                a = jnp.concatenate([jnp.concatenate([al[64 * j:64 * (j + 1), lanes(2)], al[64 * j:64 * (j + 1), lanes(7)]], axis=-1),
                                     jnp.concatenate([al[64 * j:64 * (j + 1), lanes(8)], al[64 * j:64 * (j + 1), lanes(3)]], axis=-1)], axis=0)
                w = jnp.concatenate([p4[0, 64 * j:64 * (j + 1), :], p4[1, 64 * j:64 * (j + 1), :]], axis=0)
                d = [nn(ub(a[0:64]), ub(w)), nn(ub(a[64:128]), ub(w))]
                h = d if h is None else [h[0] + d[0], h[1] + d[1]]
                if j == 0:
                    gate(0, 384)
                if j == 1:
                    gate(384, D)
                if j == 6:
                    finish(0, H, h[0], 0, 128)
                    finish(H, H, h[1], 0, 128)
                next(st0)
        else:
            gate(0, 128)
            w4_plain(0)
            gate(128, 384)
            next(st0)
            gate(384, D)
            for _ in st0:
                pass
        if 'l' not in R3O:
            ln_x1(T)
        out_copy(0).start()
        q_copies[2].wait()
        if SAME:
            q_copies[3].wait()

    def mlp_body(i, carry):
        with _scope("iter"):
            r1 = pl.multiple_of(PB - PC + PC * i, 32)
            r = pl.multiple_of(i * T, T)
            for tok in LB:
                if tok == 'n':
                    first = mm_w3_first()
                elif tok == 'c':
                    ln_chain(r1, PC, CL, skip=CK)
                elif tok == 'd':
                    ln_chain(pl.multiple_of(jnp.minimum(r1 + PC, S - PC), 32), PC, CL, r1 + PC, CE, STG)
                elif tok == 'k':
                    x2s[rows(r1, PC), :] = xt[0:PC, :]
                    h2s[rows(r1, PC), :] = ht[0:PC, :]
                elif tok == 't':
                    tail = mm_w3_tail()
                elif tok == '3':
                    w3_all(first, tail, J2)
                    steps = w4_steps2(r, J2)
                elif tok == 'z':
                    for _ in steps:
                        pass
                elif tok == 's':
                    next(steps)
                elif tok == 'p':
                    w4_plain(r)
                elif tok == '1':
                    if ST1:
                        mm_w1s(r1, PC)
                    else:
                        mm_w1(r1, PC, parts=W1P)
                elif tok == 'q':
                    w4_pair(r, 0)
                elif tok == '2':
                    mm_w2(r + T, parts=W2P, st=ST2)
                elif tok == 'l':
                    ln_x1(r + T, LL, LK)
                elif tok == 'r':
                    w4_pair(r, 1)
            out_copy(i).start()
        return carry

    with _scope("loop"):
        jax.lax.fori_loop(1, NC - 1, mlp_body, 0)
    with _scope("last"):
        first = mm_w3_first()
        tail = mm_w3_tail()
        w3_all(first, tail, JL)
        w4_plain(S - T, 0, LA)
        for _ in w4_steps2(S - T, JL):
            pass
        out_tail[0].start()
        w4_plain(S - T, LA, LAST0 - LA)
        out_tail[1].start()
        w4_plain(S - T, LAST0, T - LAST0)
        out_tail[2].start()
    with _scope("fin"):
        for i in range(NC - 1):
            out_copy(i).wait()
        for cp in out_tail:
            cp.wait()


@jax.jit
def pallas_adaLN_cond__ssm_conv_h3__mixer_s_mlp__prompt_kernel(
    A_q: jax.Array,
    A_k: jax.Array,
    A_v: jax.Array,
    A_shift_k: jax.Array,
    A_ssm_k: jax.Array,
    A_ssm_D: jax.Array,
    B_x: jax.Array,
    B_w1: jax.Array,
    B_w2: jax.Array,
    B_w3: jax.Array,
    B_w4: jax.Array,
    c: jax.Array,
    w_mod: jax.Array,
):
    del B_x
    any_spec = pl.BlockSpec(memory_space=pl.ANY)

    def tile_view(x):
        return x.reshape(S // 8, 8, CT, 128).transpose(0, 2, 1, 3).reshape(S * CT, 128)

    vm = pltpu.VMEM
    dma = pltpu.SemaphoreType.DMA
    spec = (4, NG, 16, 128)
    out = pl.pallas_call(
        _kernel,
        in_specs=[any_spec] * 12,
        out_specs=any_spec,
        out_shape=jax.ShapeDtypeStruct((S, D), bf16),
        scratch_shapes=[
            *[vm((KROWS, 128), bf16)] * NB, *[vm((VROWS, 128), bf16)] * NB, vm((CT, 128, S), bf16),
            vm((S, D), bf16), vm((D, D), bf16), vm((D, D), bf16), vm((F, D), bf16), vm((F, D), bf16),
            vm((D // 2, D), u32), vm((D // 2, D), u32), vm((F // 2, D), u32), vm((F // 2, D), u32),
            vm((D, 3 * D), bf16), vm((D, 2 * D), bf16), vm((D, D), bf16),
            vm((4, D), bf16), vm((D,), bf16), vm((1, D), bf16), vm((1, 1792), f32),
            vm((4, 128, 128), u32), vm((4, 128, 128), u32), vm((4, 64, 256), u32),
            vm((CT, 8, 8, 128), f32),
            vm((CT, NB) + spec, f32), vm((CT, NB - 1) + spec, f32), vm((CT,) + spec, f32),
            vm((CT, NB) + spec, f32), vm((4, 128, 128), f32),
            vm((CT, S + 32, 128), f32), vm((8, 8, D), f32),
            vm((CT, S + 32, 128), f32), vm((S + 256, D), f32), vm((S + 256, D), f32), vm((S, D), f32),
            vm((288, D), u32), vm((T // 2, D), u32), vm((D // 2, 128), u32),
            vm((640, 256), u32), vm((640, 256), u32), vm((NP3 * 64, 1280), u32), vm((7 * 448, 256), u32), vm((2, 448, 128), u32), vm((7 * 64, 1152), u32),
            vm((4, H, 128), f32), vm((5, H // 2, 256), u32), vm((5, H // 2, 256), u32),
            vm((H, D), u32), vm((H // 2, 1280), u32), vm((T, D), f32),
            vm((35 * 64, 384), u32), vm((4 * H, 256), f32), vm((7 * 64, 896), u32), vm((21 * 32 + 32, 640), u32), vm((T, D), f32),
            vm((S, D), bf16),
            dma((27,)), dma((NC + 2,)),
        ],
        compiler_params=pltpu.CompilerParams(vmem_limit_bytes=110 << 20, disable_bounds_checks=True,
                                             disable_semaphore_checks=True),
    )(A_q.reshape(S, D), tile_view(A_k), tile_view(A_v), A_shift_k.T, A_ssm_k,
      A_ssm_D, B_w1, B_w2, B_w3.T, B_w4, c, w_mod)
    return out.reshape(1, S, D)
```

```python
import os
import numpy as np
import jax
import jax.numpy as jnp
import jax.experimental.pallas as pl
import jax.experimental.pallas.tpu as pltpu

f32, bf16, u32, i32 = jnp.float32, jnp.bfloat16, jnp.uint32, jnp.int32

S, D, F = 2048, 640, 1728
CT = D // 128
TR = 8 * CT
NB, BLK, NFFT = 4, 512, 1024
KROWS, VROWS = BLK * CT + 128, BLK * CT + 64
NG = 16
T = 256
NC = S // T
FM = (F // 128) * 128
P0, P1, PA, PC = 320, 224, 160, 224
PB = P0 + P1 + PA
LAST0 = int(os.environ.get('LAST0', '208'))
RG = 16
EPS = 1e-5
NT_DIMS = (((1,), (1,)), ((), ()))
OUTF = int(os.environ.get('OUTF', '1'))
MODI = int(os.environ.get('MODI', '1'))
NS = [int(x) * 128 for x in os.environ.get('NS', '12')]
R3 = os.environ.get('R3', 'a31t')
SM = int(os.environ.get('SM', '0'))
TC = int(os.environ.get('TC', '512'))
TMODE = int(os.environ.get('TMODE', '0'))
LB = os.environ.get('LB', 'nct31p2lz')
W1P = int(os.environ.get('W1P', '1'))
W2P = int(os.environ.get('W2P', '1'))
RS = int(os.environ.get('RS', '0'))
W3S = int(os.environ.get('W3S', '640'))
ST3 = int(os.environ.get('ST3', '1'))
ST4 = int(os.environ.get('ST4', '1'))
LL = int(os.environ.get('LL', '1'))
H = T // 2
NP3 = 6
ST1 = int(os.environ.get('ST1', '1'))
ST2 = int(os.environ.get('ST2', '1'))
CL = int(os.environ.get('CL', '1'))
ACC = int(os.environ.get('ACC', '1'))
SORD = int(os.environ.get('SORD', '1'))
CE = int(os.environ.get('CE', '1'))
RSQ = int(os.environ.get('RSQ', '1'))
GM = int(os.environ.get('GM', '0'))
FEN4 = int(os.environ.get('FEN4', '0'))
R2C = int(os.environ.get('R2C', '2'))
R3O = os.environ.get('R3O', '1tn3')
LR = int(os.environ.get('LR', '0'))
CR = int(os.environ.get('CR', '0'))
L2 = int(os.environ.get('L2', '1'))
LA = int(os.environ.get('LA', '64'))
LX3 = int(os.environ.get('LX3', '1'))
IL4 = int(os.environ.get('IL4', '1'))
L2S = [int(x) for x in os.environ.get('L2S', '1234567')]
SAME = int(os.environ.get('SAME', '1'))
W2L2 = int(os.environ.get('W2L2', '0'))
J2 = int(os.environ.get('J2', '0'))
J0 = int(os.environ.get('J0', '2'))
JL = int(os.environ.get('JL', '2'))
STG = int(os.environ.get('STG', '0'))
D4 = int(os.environ.get('D4', '0'))
Q3 = int(os.environ.get('Q3', '0'))
CK = os.environ.get('CM', '10000100001000')
LK = os.environ.get('LM', '')
SQL = int(os.environ.get('SQL', '0'))
SQ2 = int(os.environ.get('SQ2', '0'))
XMP = os.environ.get('XMP', '3g4s')
XML = os.environ.get('XML', '')
XMZ = os.environ.get('XMZ', 'g')
L3 = int(os.environ.get('L3', '2'))
L2R = int(os.environ.get('L2R', '2'))
R2O = os.environ.get('R2O', 'cAlB')
GVF = int(os.environ.get("GVF", "8"))
GVI = int(os.environ.get("GVI", "8"))
NL = int(os.environ.get("NL", "4"))
SKIPCONV = int(os.environ.get("SKIPCONV", "0"))
SCOPES = bool(int(os.environ.get("KSCOPES", "0")))


class _NoScope:
    def __enter__(self):
        return self

    def __exit__(self, *a):
        return False


def _scope(name):
    return jax.named_scope(name) if SCOPES else _NoScope()


def _lo(w):
    return pltpu.bitcast(w << 16, f32)


def _hi(w):
    return pltpu.bitcast(w & jnp.uint32(0xFFFF0000), f32)


def _cis(n):
    t = (n & (2 * NFFT - 1)).astype(f32) * (np.pi / NFFT)
    return jnp.cos(t), jnp.sin(t)


def _fwd_table(r):
    g = jax.lax.broadcasted_iota(i32, (NG, 128), 0)
    cg, sg = _cis(jnp.where(g < NG // 2, 32 * g + 1, 32 * g - 253) * r)
    cs, ss = _cis(4 * jax.lax.broadcasted_iota(i32, (8, 128), 0) * r)
    parts = []
    for i in range(NG):
        c, s = cg[i:i + 1], sg[i:i + 1]
        parts += [c * cs - s * ss, -(s * cs + c * ss)]
    return pltpu.bitcast(jnp.concatenate(parts, axis=0).astype(bf16), u32)


def _inv_tables():
    def phase(rows):
        col = jax.lax.broadcasted_iota(i32, (rows, 256), 1)
        k = ((col >> 4) << 3) + (col & 7)
        row = jax.lax.broadcasted_iota(i32, (rows, 256), 0)
        return jnp.where(k < 64, 4 * k + 1, 4 * k - 253), (col & 8) << 6, row

    fr, _, g = phase(16)
    cg, sg = _cis(fr * (32 * g))
    fr, off, s = phase(8)
    out = []
    for p in range(4):
        cs, ss = _cis(fr * (4 * s + p) + off)
        cs, ss = cs * (2.0 / NFFT), ss * (2.0 / NFFT)
        parts = [cg[i:i + 1] * cs - sg[i:i + 1] * ss for i in range(16)]
        out.append(pltpu.bitcast(jnp.concatenate(parts, axis=0).astype(bf16), u32))
    return out


def _radix4(re, im, inverse):
    ar, ai = re[0] + re[2], im[0] + im[2]
    br, bi = re[0] - re[2], im[0] - im[2]
    cr, ci = re[1] + re[3], im[1] + im[3]
    dr, di = re[1] - re[3], im[1] - im[3]
    minus_i = (br + di, bi - dr)
    plus_i = (br - di, bi + dr)
    if inverse:
        return [(ar + cr, ai + ci), plus_i, (ar - cr, ai - ci), minus_i]
    return [(ar + cr, ai + ci), minus_i, (ar - cr, ai - ci), plus_i]


def _stats(x, link=None, early=False):
    zero = 0.0 if link is None else jnp.minimum(link, 0.0)
    part = x[:, 0:128]
    for c in range(1, CT):
        part = part + x[:, c * 128:(c + 1) * 128]
    if link is not None and early:
        part = part + zero
        zero = 0.0
    m = jnp.sum(part, axis=-1, keepdims=True) * (1.0 / D)
    v = jnp.maximum(jnp.sum(x * x, axis=-1, keepdims=True) * (1.0 / D) - m * m, zero)
    if RSQ:
        return m, jnp.exp2(jnp.log(v + EPS) * (-0.5 / np.log(2.0)))
    return m, jax.lax.rsqrt(v + EPS)


def _gelu2(x):
    c = 0.7978845608028654
    u = c + (c * 0.044715) * (x * x)
    return x + x * jnp.tanh(x * u)


def _gelu(x):
    c = 0.7978845608028654
    u = c + (c * 0.044715) * (x * x)
    hx = 0.5 * x
    return hx + hx * jnp.tanh(x * u)


def _dot_balanced(x, wslice, n_cols, parts, nt=False):
    def mm(a, c0, c1):
        a, w = a.astype(bf16), pltpu.bitcast(wslice(c0, c1), bf16)
        if nt:
            return jax.lax.dot_general(a, w, NT_DIMS, preferred_element_type=f32)
        return jnp.dot(a, w, preferred_element_type=f32)

    if parts == 1:
        return mm(x, 0, n_cols)
    base, extra = divmod(x.shape[0] // 16, parts)
    last, o = [], 0
    head = mm(x, 0, n_cols - 128)
    for i in range(parts):
        n = 16 * (base + (1 if i < extra else 0))
        last.append(mm(x[o:o + n], n_cols - 128, n_cols))
        o += n
    return jnp.concatenate([head, jnp.concatenate(last, axis=0)], axis=-1)


def _kernel(q_hbm, k_hbm, v_hbm, sh_hbm, sk_hbm, d_hbm, w1_hbm, w2_hbm, w3_hbm, w4_hbm,
            c_hbm, wm_hbm, o_hbm,
            kb0, kb1, kb2, kb3, vb0, vb1, vb2, vb3, skb, qb, w1b, w2b, w3b, w4b, w1p, w2p, w3p, w4p,
            wma, wmb, wmc, shb, db, cb_, scb,
            fub, fkb, gtb, par, US, KS, UR, YS, YP, ys, modb, h10, h11, h12, h13, h14, h2s, x2s, hss, zt, zb, w3n, s1, s2, s3, s4, p4, al, cq, zs, zu, gs, gu, xt, s5, c2, t2, a2, ht, sp, ob,
            sem, sem_o):
    h1s = [h10, h11, h12, h13, h14]
    n_in = [0]

    def load(src, dst):
        n_in[0] += 1
        return pltpu.make_async_copy(src, dst, sem.at[n_in[0] - 1])

    nkv = BLK * CT
    small = [load(d_hbm, db), load(sh_hbm, shb), load(c_hbm, cb_)]
    sk_copies = [load(sk_hbm.at[pl.ds(c * 128, 128), :], skb.at[c]) for c in range(CT)]
    kbs, vbs, wms = [kb0, kb1, kb2, kb3], [vb0, vb1, vb2, vb3], [wma, wmb, wmc]
    kv_copies = [[load(k_hbm.at[pl.ds(0, nkv), :], kb0.at[pl.ds(TR, nkv), :]) if a == 0 else
                  load(k_hbm.at[pl.ds(a * nkv - TR, nkv + TR), :], kbs[a].at[pl.ds(0, nkv + TR), :]),
                  load(v_hbm.at[pl.ds(a * nkv, nkv), :], vbs[a].at[pl.ds(0, nkv), :])] for a in range(NB)]
    mod_cols = [(0, 3 * D), (3 * D, 2 * D), (5 * D, D)]
    mod_copies = [load(wm_hbm.at[:, pl.ds(o, n)], w) for (o, n), w in zip(mod_cols, wms)]
    w_copies = [load(w1_hbm, w1b), load(w2_hbm, w2b), load(w3_hbm, w3b), load(w4_hbm, w4b)]
    q_copies = [load(q_hbm.at[pl.ds(o, n), :], qb.at[pl.ds(o, n), :])
                for o, n in [(0, P0 + P1), (P0 + P1, PA), (PB + PC, S - PB - PC), (PB, PC)]]

    def out_copy(i):
        r = i * T if isinstance(i, int) else pl.multiple_of(i * T, T)
        return pltpu.make_async_copy(ob.at[pl.ds(r, T), :], o_hbm.at[pl.ds(r, T), :], sem_o.at[i])

    tail_parts = [(S - T, T, 128, D), (S - T, LAST0, 0, 128), (S - T + LAST0, T - LAST0, 0, 128)]
    out_tail = [pltpu.make_async_copy(ob.at[pl.ds(o, n), pl.ds(c0, c1 - c0)], o_hbm.at[pl.ds(o, n), pl.ds(c0, c1 - c0)],
                                      sem_o.at[NC - 1 + i]) for i, (o, n, c0, c1) in enumerate(tail_parts)]

    first = small + kv_copies[0] if SM == 0 else [kv_copies[0][0]] + small + [kv_copies[0][1]]
    for cp in (first + sk_copies + kv_copies[1] + kv_copies[2] + kv_copies[3]
               + [mod_copies[0], q_copies[0], mod_copies[1], w_copies[0], w_copies[1], q_copies[1],
                  w_copies[2]] + ([w_copies[3], mod_copies[2], q_copies[3]] if (SAME or Q3) else [q_copies[3], w_copies[3], mod_copies[2]]) + [q_copies[2]]):
        cp.start()

    def wait(name, copies):
        with _scope(name):
            for cp in copies:
                cp.wait()

    def pin(i, carry):
        z = jnp.zeros((8, 128), f32)
        scb[:, pl.ds(pl.multiple_of(i * 128, 128), 128)] = z[0:1]
        YP[i, 0:8, :] = z
        US[i, 0, 0, 0, 0:8, :] = z
        KS[i, 0, 0, 0, 0:8, :] = z
        YS[i, 0, 0, 0, 0:8, :] = z
        UR[i, 0, 0, 0:8, :] = z
        cq[i, 0:8, :] = z
        r8 = pl.multiple_of(i * 8, 8)
        al[pl.ds(r8, 8), 0:128] = jnp.zeros((8, 128), u32)
        gs[pl.ds(r8, 8), 0:128] = jnp.zeros((8, 128), u32)
        xt[pl.ds(r8, 8), 0:128] = z
        c2[pl.ds(r8, 8), 0:128] = z
        sp[pl.ds(r8, 8), 0:128] = z
        ht[pl.ds(r8, 8), 0:128] = z
        a2[pl.ds(r8, 8), 0:128] = jnp.zeros((8, 128), u32)
        gu[pl.ds(r8, 8), 0:128] = jnp.zeros((8, 128), u32)
        return carry

    def fence(i, carry):
        YP[i, 0:8, :] = jnp.zeros((8, 128), f32)
        return carry

    with _scope("init"):
        jax.lax.fori_loop(0, 2, pin, 0)
        lane = jax.lax.broadcasted_iota(i32, (1, 128), 1)
        for p in range(4):
            m = (lane - p) & 3
            fkb[p] = _fwd_table(128 * m + ((lane - m) & 127))
        for c in range(CT):
            kb0[c * 8:(c + 1) * 8, :] = jnp.zeros((8, 128), bf16)
            h1s[c][0:8, :] = jnp.zeros((8, 128), f32)
            h1s[c][S + 8:S + 16, :] = jnp.zeros((8, 128), f32)
        for a in range(NB):
            kbs[a][nkv + TR:KROWS, :] = jnp.zeros((KROWS - nkv - TR, 128), bf16)
            vbs[a][nkv:VROWS, :] = jnp.zeros((VROWS - nkv, 128), bf16)
        for p in range(4):
            fub[p] = _fwd_table(8 * (lane & 63) + ((lane >> 6) << 2) + p)
        if SM:
            for p, tab in enumerate(_inv_tables()):
                gtb[p] = tab
        wait("w_small", small)
        cvec = cb_[...].astype(f32)
        scb[:, 0:D] = cvec * jax.nn.sigmoid(cvec)
        dv = db[...].astype(f32).reshape(1, D)
        shv = shb[...].astype(f32)
        for c in range(CT):
            for i in range(4):
                par[c, i] = jnp.broadcast_to(shv[i:i + 1, c * 128:(c + 1) * 128], (8, 128))
            par[c, 4] = jnp.broadcast_to(dv[:, c * 128:(c + 1) * 128], (8, 128))
        if not SM:
            for p, tab in enumerate(_inv_tables()):
                gtb[p] = tab

    def get(ref, idx, g, n):
        return (ref[idx + (slice(g, g + n), slice(0, 8))], ref[idx + (slice(g, g + n), slice(8, 16))])

    def put(ref, idx, g, n, xr, xi):
        ref[idx + (slice(g, g + n), slice(0, 8))] = xr
        ref[idx + (slice(g, g + n), slice(8, 16))] = xi

    def split(tt, g, n):
        tt = [t[g * 16:(g + n) * 16].reshape(n, 16, 128) for t in tt]
        return [t[:, 0:8] for t in tt], [t[:, 8:16] for t in tt]

    def fwd_k(c, j):
        if SKIPCONV:
            return
        lane = jax.lax.broadcasted_iota(i32, (64, 128), 1)
        even = (lane & 1) == 0
        l01 = (lane & 2) == 0
        l12 = ((lane + 3) & 2) == 0
        rm = []
        for m in range(4):
            w = pltpu.bitcast(skb[c, :, (4 * j + m) * 128:(4 * j + m + 1) * 128], u32)
            rm.append(pltpu.roll(w, m, 1) if m else w)
        e01 = jnp.where(even, rm[0], rm[1])
        o01 = jnp.where(even, rm[1], rm[0])
        e23 = jnp.where(even, rm[2], rm[3])
        o23 = jnp.where(even, rm[3], rm[2])
        kp = [jnp.where(l01, e01, e23), jnp.where(l12, o01, o23),
              jnp.where(l01, e23, e01), jnp.where(l12, o23, o01)]
        tt = [jax.lax.dot_general(pltpu.bitcast(fkb[p], bf16), pltpu.bitcast(kp[p], bf16), NT_DIMS,
                                  preferred_element_type=f32) for p in range(4)]
        for g in range(0, NG, GVF):
            re, im = split(tt, g, GVF)
            if j == 0:
                re[0] = re[0] + par[c, 4][None]
            for m, (xr, xi) in enumerate(_radix4(re, im, False)):
                if j < NB - 1:
                    put(KS, (c, j, m), g, GVF, xr, xi)
                ur, ui = get(US, (c, 0, m), g, GVF)
                put(YS, (c, j, m), g, GVF, xr * ur - xi * ui, xr * ui + xi * ur)

    def fwd_u(c, a):
        if SKIPCONV:
            return
        taps = [jnp.tile(par[c, i], (8, 1)) for i in range(4)]
        ws = TR // 2
        base = 4 * c
        kw, vw = kbs[a].bitcast(u32), vbs[a].bitcast(u32)

        def words(ref, start):
            return ref[pl.ds(start, BLK // 8, stride=ws), :]

        kk = {}
        for w in range(4):
            x = words(kw, ws + base + w)
            kk[2 * w], kk[2 * w + 1] = _lo(x), _hi(x)
        kk[-3] = _hi(words(kw, base + 2))
        x = words(kw, base + 3)
        kk[-2], kk[-1] = _lo(x), _hi(x)
        sub = []
        for w in range(4):
            x = words(vw, base + w)
            for r, vv in ((2 * w, _lo(x)), (2 * w + 1, _hi(x))):
                sh = taps[0] * kk[r] + taps[1] * kk[r - 1] + taps[2] * kk[r - 2] + taps[3] * kk[r - 3]
                sub.append(sh * vv)
        kv = [jnp.concatenate([sub[p], sub[p + 4]], axis=0) for p in range(4)]
        tt = [jnp.dot(pltpu.bitcast(fub[p], bf16), kv[p].astype(bf16), preferred_element_type=f32)
              for p in range(4)]
        for g in range(0, NG, GVF):
            re, im = split(tt, g, GVF)
            for m, (xr, xi) in enumerate(_radix4(re, im, False)):
                if a:
                    pr, pi = get(US, (c, 0, m), g, GVF) if a == 1 else get(UR, (c, m), g, GVF)
                    if a < NB - 1:
                        put(UR, (c, m), g, GVF, xr, xi)
                    xr, xi = (xr - pi, xi + pr) if g < NG // 2 else (xr + pi, xi - pr)
                put(US, (c, a, m), g, GVF, xr, xi)

    def mac_inv(c, a):
        if SKIPCONV:
            return
        for h in range(2):
            vals = [[] for _ in range(4)]
            for g in range(8 * h, 8 * h + 8, GVI):
                yre, yim = [], []
                for m in range(4):
                    yr, yi = get(YS, (c, a, m), g, GVI)
                    for j in range(a):
                        kr, ki = get(KS, (c, j, m), g, GVI)
                        ur, ui = get(US, (c, a - j, m), g, GVI)
                        yr = yr + (kr * ur - ki * ui)
                        yi = yi + (kr * ui + ki * ur)
                    yre.append(yr)
                    yim.append(yi)
                for p, (pr, pi) in enumerate(_radix4(yre, yim, True)):
                    vals[p].append(jnp.concatenate([pr, pi], axis=1))
            for p in range(4):
                pb = jnp.concatenate(vals[p], axis=0).reshape(128, 128).astype(bf16)
                r = jnp.dot(pltpu.bitcast(gtb[p, :, h * 128:(h + 1) * 128], bf16), pb,
                            preferred_element_type=f32)
                if h == 0:
                    YP[p] = r
                else:
                    ys[c, pl.ds(a * BLK + p, 128, stride=4), :] = YP[p] + r

    with _scope("conv_u0"):
        wait("w_kv", kv_copies[0])
        for c in range(CT):
            fwd_u(c, 0)
    with _scope("conv_k"):
        for grp in ((0,), (1, 2), (3, 4)):
            wait("w_sk", [sk_copies[c] for c in grp])
            for c in grp:
                for j in (3, 2, 1, 0):
                    fwd_k(c, j)
    for a in range(1, NB):
        with _scope("conv_u%d" % a):
            wait("w_kv", kv_copies[a])
            for c in range(CT):
                fwd_u(c, a)
                mac_inv(c, a - 1)
    with _scope("conv_last"):
        jax.lax.fori_loop(0, 2, fence, 0)
        for c in range(NL):
            mac_inv(c, NB - 1)

    def mod_part(part, extra):
        n, wm = mod_cols[part][1], wms[part]
        act = scb[:, 0:D]

        def sc(k0, k1):
            return jnp.broadcast_to(act[:, k0:k1], (16, k1 - k0)).astype(bf16)

        e = 128 * extra
        r = jnp.dot(sc(0, D), wm[:, e:n], preferred_element_type=f32)
        r0 = (jnp.dot(sc(0, D - 64), wm[0:D - 64, 0:e], preferred_element_type=f32)
              + jnp.dot(sc(D - 64, D), wm[D - 64:D, 0:e], preferred_element_type=f32))
        r = jnp.concatenate([r0, r], axis=-1)[0:8]
        return [r[:, i * D:(i + 1) * D] for i in range(n // D)]

    def mvec(i, n=RG, c0=0, c1=D):
        return jnp.tile(modb[i, :, c0:c1], (n // 8, 1))

    rows = pl.ds

    def load_q(r, ref=qb):
        return ref[rows(r, RG), :].astype(f32)

    def make_x2(r, q, st, ref=ys):
        y = jnp.concatenate([ref[c, rows(r, RG), :] for c in range(CT)], axis=-1)
        return q + (((q - st[0]) * st[1]) * mvec(1) + mvec(0)) * y

    def make_h2(x2, st):
        return ((x2 - st[0]) * st[1]) * mvec(3) + mvec(2)

    def pack_ln(x, st):
        return pltpu.bitcast(((x - st[0]) * st[1]).astype(bf16), u32)

    def lhs_sums(a11, a12, a21, a22):
        return [a11 + a22, a21 + a22, a11 + a12, a21 - a11, a12 - a22]

    def rhs_sums(b11, b12, b21, b22):
        return [b11 + b22, b12 - b22, b21 - b11, b11 + b12, b21 + b22]

    RHS = [(0, 3, 1), (1, 3, -1), (2, 0, -1), (0, 1, 1), (2, 3, 1)]

    def rhs_sum(k, block):
        a, b, sg = RHS[k]
        return block(a) + block(b) if sg > 0 else block(a) - block(b)

    def pk(x):
        return pltpu.bitcast(x.astype(bf16), u32)

    def pk_many(vals):
        return pk(jnp.concatenate(vals, axis=-1))

    def lanes(k):
        return slice(128 * k, 128 * (k + 1))

    def ub(x):
        return pltpu.bitcast(x, bf16)

    slot = [0]
    XM = [XMP]

    def park(x):
        o = H * (slot[0] % 16)
        slot[0] += 1
        sp[o:o + x.shape[0], :] = x
        return lambda: sp[o:o + x.shape[0], :]

    def strassen(dot, a11, a22, asum, ax1, ax2, b11, b22, bsum, bx1, bx2, mem=False, post=None):
        if mem:
            post = post or (lambda x: x)
            m2 = dot(asum[1], b11)
            m4 = dot(a22, bsum[2])
            p2, p4 = park(m2), park(m4)
            c21 = post((p4() + p2()) + dot(ax2, bx1))
            m3 = dot(a11, bsum[1])
            p3, p32 = park(m3), park(m3 - p2())
            m5 = dot(asum[2], b22)
            p45 = park(p4() - m5)
            c12 = post((p3() + m5) + dot(ax1, bx2))
            m1 = dot(asum[0], bsum[0])
            p11, p22 = park(p45() + m1), park(p32() + m1)
            c11 = post((p11() + dot(asum[4], bsum[4])) + dot(ax1, bx1))
            c22 = post((p22() + dot(asum[3], bsum[3])) + dot(ax2, bx2))
            return [c11, c12, c21, c22]
        if SORD:
            m2 = dot(asum[1], b11)
            m4 = dot(a22, bsum[2])
            c21 = (m4 + m2) + dot(ax2, bx1)
            m3 = dot(a11, bsum[1])
            m5 = dot(asum[2], b22)
            c12 = (m3 + m5) + dot(ax1, bx2)
            m1 = dot(asum[0], bsum[0])
            c11 = (((m4 - m5) + m1) + dot(asum[4], bsum[4])) + dot(ax1, bx1)
            c22 = (((m3 - m2) + m1) + dot(asum[3], bsum[3])) + dot(ax2, bx2)
            return [c11, c12, c21, c22]
        m1 = dot(asum[0], bsum[0])
        m4 = dot(a22, bsum[2])
        m2 = dot(asum[1], b11)
        m3 = dot(a11, bsum[1])
        m5 = dot(asum[2], b22)
        x12 = dot(ax1, bx2)
        x21 = dot(ax2, bx1)
        m7 = dot(asum[4], bsum[4])
        x11 = dot(ax1, bx1)
        m6 = dot(asum[3], bsum[3])
        x22 = dot(ax2, bx2)
        return [(((m1 + m4) - m5) + m7) + x11, (m3 + m5) + x12, (m4 + m2) + x21, (((m1 - m2) + m3) + m6) + x22]

    def nn(a, w):
        return jnp.dot(a.astype(bf16), w, preferred_element_type=f32)

    def both(ref, r0, r1, col):
        return jnp.concatenate([ref[r0:r1, lanes(1 + col)].astype(f32), ref[r0:r1, lanes(3 + col)].astype(f32)], axis=-1)

    def prep_sq(wb, sw):
        for k in (2, 1, 0, 4, 3):
            sw[128 * k:128 * (k + 1), :] = pk(rhs_sum(k, lambda b: both(wb, 256 * (b // 2), 256 * (b // 2 + 1), b % 2)))

    def sq_strassen(a, top, bot, asum, wp, sw, last=None):
        h = top.shape[0]
        out = {}
        for n in range(3):
            if n == (SQL if last is None else last):
                c0 = nn(a, ub(wp[:, 0:128]))
                out[0] = (c0[0:h], c0[h:2 * h])
            if n == 2:
                break
            c1, c2 = 128 + 256 * n, 256 + 256 * n
            q = strassen(nn, top[:, 0:256], bot[:, 256:512], asum, top[:, 512:D], bot[:, 512:D],
                         ub(wp[0:128, c1:c2]), ub(wp[128:256, c2:c2 + 128]), [ub(sw[128 * k:128 * (k + 1), lanes(n)]) for k in range(5)],
                         ub(wp[256:320, c1:c2]), ub(wp[256:320, c2:c2 + 128]), mem='s' in XM[0])
            out[2 * n + 1] = (q[0], q[2])
            out[2 * n + 2] = (q[1], q[3])
        return out

    ORDER = (2, 4, 3, 5, 1, 7, 6)
    LHS = {1: (0, 3, 1), 2: (2, 3, 1), 3: (0, None, 0), 4: (3, None, 0), 5: (0, 1, 1), 6: (2, 0, -1), 7: (1, 3, -1)}
    RHS7 = {1: (0, 3, 1), 2: (0, None, 0), 3: (1, 3, -1), 4: (2, 0, -1), 5: (3, None, 0), 6: (0, 1, 1), 7: (2, 3, 1)}

    def comb(rule, blk):
        a, b, sg = rule
        return blk(a) if b is None else blk(a) + blk(b) if sg > 0 else blk(a) - blk(b)

    def quad(x, b):
        h, w = x.shape[0] // 2, x.shape[1] // 2
        return x[h * (b // 2):h * (b // 2 + 1), w * (b % 2):w * (b % 2 + 1)]

    def join(m):
        c21 = m[4] + m[2]
        c12 = m[3] + m[5]
        c11 = ((m[4] - m[5]) + m[1]) + m[7]
        c22 = ((m[3] - m[2]) + m[1]) + m[6]
        return jnp.concatenate([jnp.concatenate([c11, c12], axis=-1), jnp.concatenate([c21, c22], axis=-1)], axis=0)

    def prep_sq2(wb, tab):
        for m in ORDER:
            b1 = comb(RHS7[m], lambda b: wb[256 * (b // 2):256 * (b // 2 + 1), 128 + 256 * (b % 2):384 + 256 * (b % 2)].astype(f32))
            tab[64 * (m - 1):64 * m, :] = pk_many([comb(RHS7[k], lambda b: quad(b1, b)) for k in range(1, 8)])

    def sq_strassen2(a, wp, tab):
        c0 = nn(a, ub(wp[:, 0:128]))
        prods = {}
        for m in ORDER:
            a1 = comb(LHS[m], lambda b: quad(a[:, 0:512], b))
            prods[m] = join({k: nn(comb(LHS[k], lambda b: quad(a1, b)), ub(tab[64 * (m - 1):64 * m, lanes(k - 1)]))
                             for k in ORDER})
        rest = nn(a[:, 512:D], ub(wp[256:320, 128:D]))
        return jnp.concatenate([c0, join(prods) + rest], axis=-1)

    def ln_chain(r, n, links=1, r_out=None, early=False, staged=False, skip=0):
        qv, yv = qb.at[rows(r, n), :], ys.at[:, rows(r, n), :]
        r_out = r if r_out is None else r_out
        xv, hv = (xt, ht) if staged else (x2s.at[rows(r_out, n), :], h2s.at[rows(r_out, n), :])
        prev = [None] * links
        cnt = 0
        for o1 in range(0, n // 2, RG):
            zz, sts = [], []
            for o in (o1, o1 + n // 2):
                q = load_q(o, qv)
                st = _stats(q, prev[cnt % links], early)
                if CR & 1:
                    xv[o:o + RG, :] = q
                    q = xv[o:o + RG, :]
                x2 = make_x2(o, q, st, yv)
                xv[o:o + RG, :] = x2
                st = _stats(x2)
                h2 = make_h2(xv[o:o + RG, :], st)
                hv[o:o + RG, :] = h2
                st = _stats(h2)
                if CR & 2:
                    sts.append(st)
                else:
                    z = (hv[o:o + RG, :] - st[0]) * st[1]
                    zt[o // 2:(o + RG) // 2, :] = pk(z)
                    zz.append(z)
                if skip and skip[cnt] == '1':
                    pend = st[1]
                elif skip and cnt and skip[cnt - 1] == '1':
                    prev[0] = jnp.minimum(st[1], pend)
                else:
                    prev[cnt % links] = st[1]
                cnt += 1
            if CR & 2:
                for o, st in zip((o1, o1 + n // 2), sts):
                    z = (hv[o:o + RG, :] - st[0]) * st[1]
                    zt[o // 2:(o + RG) // 2, :] = pk(z)
                    zz.append(z)
            if ST1:
                for k, v in enumerate(lhs_sums(zz[0][:, 0:256], zz[0][:, 256:512], zz[1][:, 0:256], zz[1][:, 256:512])):
                    zu.at[k][o1 // 2:(o1 + RG) // 2, :] = pk(v)

    def mm_w1s(r, n, o=0):
        h, o = n // 2, o // 2
        res = sq_strassen(ub(zt[o:o + h, :]), ub(zt[o:o + h // 2, :]), ub(zt[o + h // 2:o + h, :]),
                          [ub(zu[k, 0:h // 2, :]) for k in range(5)], w1p, s1)
        for c, (ct, cb2) in res.items():
            h1s[c][rows(r + 8, h), :] = _gelu(ct)
            h1s[c][rows(r + 8 + h, h), :] = _gelu(cb2)

    def mm_w1(r, n, o=0, parts=4):
        z = pltpu.bitcast(zt[o // 2:(o + n) // 2, :], bf16)
        h1 = _gelu(_dot_balanced(z, lambda a, b: w1p[:, a:b], D, parts))
        for c in range(CT):
            h1s[c][rows(r + 8, n), :] = h1[:, c * 128:(c + 1) * 128]

    def mm_w2(r, parts=4, st=False):
        lane = jax.lax.broadcasted_iota(i32, (T, 128), 1)

        def sh(k, c):
            return h1s[c][rows(r + 8 + k, T), :]

        g = jnp.concatenate([
            sh(-1, 0),
            jnp.where(lane < 32, sh(-1, 1), sh(1, 1)),
            jnp.where(lane < 64, sh(1, 2), sh(-2, 2)),
            jnp.where(lane < 96, sh(-2, 3), sh(2, 3)),
            sh(2, 4)], axis=-1)
        if not st:
            hss[rows(r, T), :] = _dot_balanced(g, lambda a, b: w2p[:, a:b], D, parts)
            return
        if W2L2:
            hss[rows(r, T), :] = sq_strassen2(g, w2p, t2)
            return
        top, bot = g[0:H], g[H:T]
        sums = lhs_sums(top[:, 0:256], top[:, 256:512], bot[:, 0:256], bot[:, 256:512])
        if GM == 0:
            res = sq_strassen(g, top, bot, sums, w2p, s2, SQ2)
        else:
            gs[...] = pk(g)
            gu[...] = pk_many(sums)
            res = sq_strassen(ub(gs[...]), ub(gs[0:H // 2, :]), ub(gs[H // 2:H, :]),
                              [ub(gu[:, 256 * k:256 * (k + 1)]) for k in range(5)], w2p, s2)
        for c, (ct, cb2) in res.items():
            hss[rows(r, H), c * 128:(c + 1) * 128] = ct
            hss[rows(r + H, H), c * 128:(c + 1) * 128] = cb2

    def ln_x1(r, links=1, skip=0):
        hv, sv = h2s.at[rows(r, T), :], hss.at[rows(r, T), :]
        prev = [None] * links
        n = 0
        for o in range(0, H, RG):
            zz, sts = [], []
            for oo in (o, o + H):
                x1 = hv[oo:oo + RG, :] + sv[oo:oo + RG, :]
                st = _stats(x1, prev[n % links], early=True)
                if LR:
                    xt[oo:oo + RG, :] = x1
                    sts.append(st)
                else:
                    z = (x1 - st[0]) * st[1]
                    zb[oo // 2:(oo + RG) // 2, :] = pk(z)
                    zz.append(z)
                if skip and skip[n] == '1':
                    pend = st[1]
                elif skip and n and skip[n - 1] == '1':
                    prev[0] = jnp.minimum(st[1], pend)
                else:
                    prev[n % links] = st[1]
                n += 1
            if LR:
                for oo, st in zip((o, o + H), sts):
                    z = (xt[oo:oo + RG, :] - st[0]) * st[1]
                    zb[oo // 2:(oo + RG) // 2, :] = pk(z)
                    zz.append(z)
            for k, v in enumerate(lhs_sums(zz[0][:, 0:256], zz[0][:, 256:512], zz[1][:, 0:256], zz[1][:, 256:512])):
                zs.at[k][o // 2:(o + RG) // 2, :] = pk(v)

    def mm_w3(f0, parts=1, f1=FM):
        z = pltpu.bitcast(zb[...], bf16)
        return _gelu2(_dot_balanced(z, lambda a, b: w3p[(f0 + a) // 2:(f0 + b) // 2, :], f1 - f0, parts, nt=True))

    def mm_w3_first():
        z = pltpu.bitcast(zb[...], bf16)
        return _gelu2(jnp.dot(z, pltpu.bitcast(w3n[...], bf16), preferred_element_type=f32))

    def mm_w3_tail():
        z = pltpu.bitcast(zb[...], bf16)
        w = pltpu.bitcast(w3p[FM // 2:F // 2, :], bf16)
        return _gelu2(jax.lax.dot_general(w, z, NT_DIMS, preferred_element_type=f32))

    def mm_w4(r, n, act, c0=0, c1=D, parts=1):
        h = _dot_balanced(act, lambda a, b: w4p[:, c0 + a:c0 + b], c1 - c0, parts)
        x1 = h2s[rows(r, n), c0:c1] + hss[rows(r, n), c0:c1]
        if OUTF:
            base = x2s[rows(r, n), c0:c1] + mvec(4, n, c0, c1) * x1
            ob[rows(r, n), c0:c1] = (base + mvec(5, n, c0, c1) * h).astype(bf16)
        else:
            ob[rows(r, n), c0:c1] = (x2s[rows(r, n), c0:c1] + mvec(4, n, c0, c1) * (x1 + 0.5 * h)).astype(bf16)

    def prep_w3():
        for j in range(NP3):
            r0 = 128 * (2 * j + 1)
            for k in (2, 1, 0, 4, 3):
                s3[64 * j:64 * (j + 1), 256 * k:256 * (k + 1)] = pk(rhs_sum(k, lambda b: w3b[
                    r0 + 128 * (b % 2):r0 + 128 * (b % 2 + 1), 256 * (b // 2):256 * (b // 2 + 1)].astype(f32)))

    def r2_block(m, b, axis):
        o = 448 * (m - 1) + 64 * (b // 2)
        return jnp.concatenate([s4[o + 128 * i:o + 128 * i + 64, lanes(b % 2)] for i in range(3)], axis=axis)

    def w4_product(m, J2):
        if m not in L2S:
            return nn(ub(left(m - 1)), ub(s4[448 * (m - 1):448 * m, :]))

        def blk(b):
            o = 64 * (b % 2) + 32 * (b // 2)
            return ub(jnp.concatenate([al[o + 128 * i:o + 128 * i + 32, lanes(m - 1)] for i in range(3)], axis=-1))

        if J2:
            asum = [ub(jnp.concatenate([a2[32 * (3 * (m - 1) + i):32 * (3 * (m - 1) + i + 1), lanes(k)]
                                        for i in range(3)], axis=-1)) for k in range(5)]
        else:
            asum = lhs_sums(*[blk(b).astype(f32) for b in range(4)])
        bsum = [ub(jnp.concatenate([s5[64 * (5 * (m - 1) + k):64 * (5 * (m - 1) + k + 1), lanes(i)]
                                    for i in range(3)], axis=0)) for k in range(5)]
        ox = 448 * (m - 1) + 384
        q = strassen(nn, blk(0), blk(3), asum, ub(al[384:416, lanes(m - 1)]), ub(al[416:448, lanes(m - 1)]),
                     ub(r2_block(m, 0, 0)), ub(r2_block(m, 3, 0)), bsum,
                     ub(s4[ox:ox + 64, lanes(0)]), ub(s4[ox:ox + 64, lanes(1)]), mem='4' in XM[0])
        return jnp.concatenate([jnp.concatenate(q[0:2], axis=-1), jnp.concatenate(q[2:4], axis=-1)], axis=0)

    def w4_steps2(r, J2):
        def acc(i):
            return c2.at[H * i:H * (i + 1), :]

        def fin2(rr, h, t):
            finish(rr, H, h[:, 0:128], 128 * t, 128 * (t + 1))
            finish(rr, H, h[:, 128:256], 128 * (t + 2), 128 * (t + 3))

        acc(0)[...] = w4_product(1, J2)
        yield
        m4 = w4_product(4, J2)
        acc(2)[...] = m4
        acc(3)[...] = acc(0)[...] + m4
        yield
        m2 = w4_product(2, J2)
        acc(0)[...] = acc(0)[...] - m2
        fin2(r + H, acc(2)[...] + m2, 1)
        yield
        m3 = w4_product(3, J2)
        acc(1)[...] = m3
        acc(0)[...] = acc(0)[...] + m3
        yield
        m5 = w4_product(5, J2)
        acc(3)[...] = acc(3)[...] - m5
        fin2(r, acc(1)[...] + m5, 2)
        yield
        fin2(r, acc(3)[...] + w4_product(7, J2), 1)
        yield
        fin2(r + H, acc(0)[...] + w4_product(6, J2), 2)
        yield

    def prep_w4():
        for j in range(7):
            if j < NP3:
                r0 = 128 * (2 * j + 1)
                p4[0, 64 * j:64 * (j + 1), :] = pltpu.bitcast(w4b[r0:r0 + 128, 0:128], u32)
                p4[1, 64 * j:64 * (j + 1), :] = pltpu.bitcast(w4b[r0 + 128:r0 + 256, 0:128], u32)
            else:
                p4[0, 64 * j:64 * (j + 1), :] = pltpu.bitcast(w4b[0:128, 0:128], u32)
                p4[1, 64 * j:64 * j + 32, :] = pltpu.bitcast(w4b[FM:F, 0:128], u32)
                p4[1, 64 * j + 32:64 * (j + 1), :] = jnp.zeros((32, 128), u32)
        def block(j, b):
            if j < NP3:
                r0 = 128 * (2 * j + 1 + b // 2)
                return both(w4b, r0, r0 + 128, b % 2)
            if b < 2:
                return both(w4b, 0, 128, b % 2)
            return jnp.concatenate([both(w4b, FM, F, b % 2), jnp.zeros((64, 256), f32)], axis=0)

        for m, k in ((1, 0), (4, 2), (2, None), (3, 1), (5, None), (7, 4), (6, 3)):
            for j in range(7):
                o = 448 * (m - 1) + 64 * j
                if k is None and (j < NP3 or m == 2):
                    r0 = 0 if j == NP3 else 128 * (2 * j + (1 if m == 2 else 2))
                    for n in range(2):
                        s4[o:o + 64, lanes(n)] = pltpu.bitcast(w4b[r0:r0 + 128, lanes(2 * n + (1 if m == 2 else 2))], u32)
                else:
                    s4[o:o + 64, :] = pk(block(j, 3) if k is None else rhs_sum(k, lambda b: block(j, b)))
            if m in L2S:
                for k2 in (2, 1, 0, 4, 3):
                    o = 64 * (5 * (m - 1) + k2)
                    s5[o:o + 64, :] = pk(rhs_sum(k2, lambda b: ub(r2_block(m, b, -1)).astype(f32)))

    def nt(a, w):
        return jax.lax.dot_general(a, w, NT_DIMS, preferred_element_type=f32)

    def w3_pair(j):
        r0 = 64 * (2 * j + 1)
        z1, z2 = ub(zb[0:H // 2, :]), ub(zb[H // 2:H, :])
        q = strassen(nt, z1[:, 0:256], z2[:, 256:512], [ub(zs[k]) for k in range(5)], z1[:, 512:D], z2[:, 512:D],
                     ub(w3p[r0:r0 + 64, 0:256]), ub(w3p[r0 + 64:r0 + 128, 256:512]), [ub(s3[64 * j:64 * (j + 1), 256 * k:256 * (k + 1)]) for k in range(5)],
                     ub(w3p[r0:r0 + 64, 512:D]), ub(w3p[r0 + 64:r0 + 128, 512:D]), mem='3' in XM[0])
        q = [_gelu2(c) for c in q]
        if 'g' in XM[0]:
            q = [park(c)() for c in q[0:3]] + [q[3]]
        return q

    def put_quads(j, q):
        l1, l2, l5, l6, l7 = lhs_sums(*q)
        al[64 * j:64 * (j + 1), :] = pk_many([l1, l2, q[0], q[3], l5, l6, l7, q[1], q[2]])

    def put_two(i, qa, qb_):
        ops = []
        for j, q in ((2 * i, qa), (2 * i + 1, qb_)):
            l1, l2, l5, l6, l7 = lhs_sums(*q)
            ops.append([l1, l2, q[0], q[3], l5, l6, l7])
            half = slice(0, 64) if j % 2 == 0 else slice(64, 128)
            o = 64 * j + 32 * (j % 2)
            al[o:o + 32, 0:256] = pk_many([l1[half], l2[half]])
            al[o:o + 32, 512:896] = pk_many([l5[half], l6[half], l7[half]])
            al[64 * j:64 * (j + 1), 256:512] = pk_many([q[0], q[3]])
            al[64 * j:64 * (j + 1), 896:1152] = pk_many([q[1], q[2]])
        for m in range(7):
            e, o = ops[0][m], ops[1][m]
            r0 = 32 * (3 * m + i)
            a2[r0:r0 + 32, :] = pk_many(lhs_sums(e[0:64], o[0:64], e[64:128], o[64:128]))

    def w3_two(i):
        z1, z2 = ub(zb[0:H // 2, :]), ub(zb[H // 2:H, :])

        def wt(par, c0, c1):
            return ub(jnp.concatenate([w3p[64 * (2 * j + 1 + par):64 * (2 * j + 2 + par), c0:c1]
                                       for j in (2 * i, 2 * i + 1)], axis=0))

        q = strassen(nt, z1[:, 0:256], z2[:, 256:512], [ub(zs[k]) for k in range(5)], z1[:, 512:D], z2[:, 512:D],
                     wt(0, 0, 256), wt(1, 256, 512),
                     [ub(s3[128 * i:128 * (i + 1), 256 * k:256 * (k + 1)]) for k in range(5)], wt(0, 512, D), wt(1, 512, D))
        q = [_gelu2(c) for c in q]
        return [c[:, 0:128] for c in q], [c[:, 128:256] for c in q]

    def w3_pairs(J2):
        if J2 == 0:
            for j in range(NP3):
                put_quads(j, w3_pair(j))
        for i in range(3):
            if J2 == 1:
                put_two(i, *w3_two(i))
            elif J2 == 2:
                qa = w3_pair(2 * i)
                put_two(i, qa, w3_pair(2 * i + 1))

    def put_edge(first, tail):
        tp = jnp.concatenate([tail.T, jnp.zeros((T, 64), f32)], axis=-1)
        put_quads(NP3, [first[0:H], tp[0:H], first[H:T], tp[H:T]])

    def w3_all(first, tail, J2):
        put_edge(first, tail)
        w3_pairs(J2)

    def left(k):
        return jnp.concatenate([al[64 * j:64 * (j + 1), lanes(k)] for j in range(7)], axis=-1)

    def w4_plain(r, o=0, n=T):
        top = jnp.concatenate([left(2), left(7)], axis=-1)
        bot = jnp.concatenate([left(8), left(3)], axis=-1)
        a = jnp.concatenate([top, bot], axis=0)[o // 2:(o + n) // 2]
        h = nn(ub(a), ub(jnp.concatenate([p4[0], p4[1]], axis=0)))
        finish(r + o, n, h, 0, 128)

    def finish(r, n, h, c0, c1):
        x1 = h2s[rows(r, n), c0:c1] + hss[rows(r, n), c0:c1]
        base = x2s[rows(r, n), c0:c1] + mvec(4, n, c0, c1) * x1
        ob[rows(r, n), c0:c1] = (base + mvec(5, n, c0, c1) * h).astype(bf16)

    def w4_steps(r, n):
        c1 = 128 + 256 * n

        def m(k):
            return nn(ub(left(k - 1)), ub(s4[448 * (k - 1):448 * k, lanes(n)]))

        if ACC:
            m1 = m(1)
            cq[0] = m1
            m4 = m(4)
            cq[2] = m4
            cq[3] = cq[0] + m4
            m2 = m(2)
            cq[0] = cq[0] - m2
            finish(r + H, H, cq[2] + m2, c1, c1 + 128)
            yield
            m3 = m(3)
            cq[1] = m3
            cq[0] = cq[0] + m3
            m5 = m(5)
            cq[3] = cq[3] - m5
            finish(r, H, cq[1] + m5, c1 + 128, c1 + 256)
            yield
            finish(r, H, cq[3] + m(7), c1, c1 + 128)
            finish(r + H, H, cq[0] + m(6), c1 + 128, c1 + 256)
            yield
            return
        m1, m4 = m(1), m(4)
        m2 = m(2)
        finish(r + H, H, m4 + m2, c1, c1 + 128)
        yield
        m3, m5 = m(3), m(5)
        finish(r, H, m3 + m5, c1 + 128, c1 + 256)
        yield
        finish(r, H, ((m1 + m4) - m5) + m(7), c1, c1 + 128)
        finish(r + H, H, ((m1 - m2) + m3) + m(6), c1 + 128, c1 + 256)
        yield

    def w4_pair(r, n):
        for _ in w4_steps(r, n):
            pass

    groups = list(range(0, P0 + P1, RG))
    with _scope("pre_a"):
        wait("w_q0", [mod_copies[0], q_copies[0]])
        sa, ca, ga = mod_part(0, 1)
        modb[0] = ga * sa
        modb[1] = ga * (1.0 + ca)
        for c in range(NL, CT):
            mac_inv(c, NB - 1)
        st1 = {o: _stats(load_q(o)) for o in groups}
        zt[0:8, 0:128] = jnp.zeros((8, 128), u32)
        st2 = {}
        for o in groups:
            x2 = make_x2(o, load_q(o), st1[o])
            x2s[o:o + RG, :] = x2
            st2[o] = _stats(x2)
    with _scope("pre_b"):
        wait("w_modB", [mod_copies[1]])
        sb, cb = mod_part(1, 2)
        modb[2] = sb
        modb[3] = 1.0 + cb
        st3 = {}
        for o in range(0, P0, RG):
            h2 = make_h2(x2s[o:o + RG, :], st2[o])
            h2s[o:o + RG, :] = h2
            st3[o] = _stats(h2)
        for o in range(0, P0, RG):
            zt[o // 2:(o + RG) // 2, :] = pack_ln(h2s[o:o + RG, :], st3[o])
    with _scope("r1"):
        wait("w_w1", [w_copies[0]])
        w1p[...] = pltpu.bitcast(w1b[...], u32)
        mm_w1(0, P0)
        prev = None
        for o1 in range(0, P1 // 2, RG):
            zz = []
            for o in (P0 + o1, P0 + o1 + P1 // 2):
                h2 = make_h2(x2s[o:o + RG, :], st2[o])
                h2s[o:o + RG, :] = h2
                st = _stats(h2, prev, early=True)
                z = (h2 - st[0]) * st[1]
                zt[o // 2:(o + RG) // 2, :] = pk(z)
                prev = st[1]
                zz.append(z)
            for k, v in enumerate(lhs_sums(zz[0][:, 0:256], zz[0][:, 256:512], zz[1][:, 0:256], zz[1][:, 256:512])):
                zu.at[k][o1 // 2:(o1 + RG) // 2, :] = pk(v)
        prep_sq(w1b, s1)
        mm_w1s(P0, P1, P0)
    with _scope("r2"):
        wait("w_w2", [w_copies[1]] + ([q_copies[1]] if R2C else []))
        w2p[...] = pltpu.bitcast(w2b[...], u32)
        if W2L2:
            prep_sq2(w2b, t2)
        else:
            prep_sq(w2b, s2)
        for tok in R2O:
            if tok == 'c' and R2C:
                ln_chain(P0 + P1, PA, R2C)
            elif tok == 'A':
                mm_w2(0, st=True)
            elif tok == 'a':
                mm_w2(0)
            elif tok == 'l':
                ln_x1(0, L2R)
            elif tok == 'B':
                mm_w2(T, st=True)
            elif tok == 'b':
                mm_w2(T)
    with _scope("r3"):
        wait("w_w3", ([] if R2C else [q_copies[1]]) + [w_copies[2]] + ([] if (SAME or Q3) else [q_copies[3]]))
        for j in range(NP3):
            r0 = 128 * (2 * j + 1)
            w3p[r0 // 2:r0 // 2 + 64, 0:256] = pltpu.bitcast(w3b[r0:r0 + 128, 0:256], u32)
            w3p[r0 // 2:r0 // 2 + 64, 512:D] = pltpu.bitcast(w3b[r0:r0 + 128, 512:D], u32)
            w3p[r0 // 2 + 64:r0 // 2 + 128, 256:D] = pltpu.bitcast(w3b[r0 + 128:r0 + 256, 256:D], u32)
        w3p[FM // 2:F // 2, :] = pltpu.bitcast(w3b[FM:F, :], u32)
        w3n[...] = pltpu.bitcast(w3b[0:128, :].astype(f32).T.astype(bf16), u32)
        prep_w3()
        for tok in R3O:
            if tok == 'c':
                if not R2C:
                    ln_chain(P0 + P1, PA)
            elif tok == 'd':
                ln_chain(PB, PC, staged=STG)
            elif tok == 'l':
                ln_x1(T, L3)
            elif tok == 't':
                tail = mm_w3_tail()
            elif tok == '3':
                w3_pairs(J0)
            elif tok == 'n':
                put_edge(mm_w3_first(), tail)
            else:
                mm_w1s(P0 + P1, PA)
        if FEN4:
            jax.lax.fori_loop(0, 2, fence, 0)
    with _scope("r4"):
        wait("w_w4", [w_copies[3], mod_copies[2]] + ([q_copies[3]] if Q3 else []))
        prep_w4()
        sc16 = jnp.broadcast_to(scb[:, 0:D], (16, D)).astype(bf16)

        def gate(c0, c1):
            gbc = jnp.dot(sc16, wmc[:, c0:c1], preferred_element_type=f32)[0:8]
            modb[4, :, c0:c1] = gbc
            modb[5, :, c0:c1] = 0.5 * gbc

        if D4:
            ln_chain(PB, PC, D4)
        st0 = w4_steps2(0, J0)
        if IL4:
            h = None
            for j in range(7):
                a = jnp.concatenate([jnp.concatenate([al[64 * j:64 * (j + 1), lanes(2)], al[64 * j:64 * (j + 1), lanes(7)]], axis=-1),
                                     jnp.concatenate([al[64 * j:64 * (j + 1), lanes(8)], al[64 * j:64 * (j + 1), lanes(3)]], axis=-1)], axis=0)
                w = jnp.concatenate([p4[0, 64 * j:64 * (j + 1), :], p4[1, 64 * j:64 * (j + 1), :]], axis=0)
                d = [nn(ub(a[0:64]), ub(w)), nn(ub(a[64:128]), ub(w))]
                h = d if h is None else [h[0] + d[0], h[1] + d[1]]
                if j == 0:
                    gate(0, 384)
                if j == 1:
                    gate(384, D)
                if j == 6:
                    finish(0, H, h[0], 0, 128)
                    finish(H, H, h[1], 0, 128)
                next(st0)
        else:
            gate(0, 128)
            w4_plain(0)
            gate(128, 384)
            next(st0)
            gate(384, D)
            for _ in st0:
                pass
        if 'l' not in R3O:
            ln_x1(T)
        out_copy(0).start()
        q_copies[2].wait()
        if SAME:
            q_copies[3].wait()

    def mlp_body(i, carry):
        with _scope("iter"):
            r1 = pl.multiple_of(PB - PC + PC * i, 32)
            r = pl.multiple_of(i * T, T)
            for tok in LB:
                if tok == 'n':
                    first = mm_w3_first()
                elif tok == 'c':
                    ln_chain(r1, PC, CL, skip=CK)
                elif tok == 'd':
                    ln_chain(pl.multiple_of(jnp.minimum(r1 + PC, S - PC), 32), PC, CL, r1 + PC, CE, STG)
                elif tok == 'k':
                    x2s[rows(r1, PC), :] = xt[0:PC, :]
                    h2s[rows(r1, PC), :] = ht[0:PC, :]
                elif tok == 't':
                    tail = mm_w3_tail()
                elif tok == '3':
                    w3_all(first, tail, J2)
                    steps = w4_steps2(r, J2)
                elif tok == 'z':
                    for _ in steps:
                        pass
                elif tok == 's':
                    next(steps)
                elif tok == 'p':
                    w4_plain(r)
                elif tok == '1':
                    if ST1:
                        mm_w1s(r1, PC)
                    else:
                        mm_w1(r1, PC, parts=W1P)
                elif tok == 'q':
                    w4_pair(r, 0)
                elif tok == '2':
                    mm_w2(r + T, parts=W2P, st=ST2)
                elif tok == 'l':
                    ln_x1(r + T, LL, LK)
                elif tok == 'r':
                    w4_pair(r, 1)
            out_copy(i).start()
        return carry

    XM[0] = XML
    with _scope("loop"):
        jax.lax.fori_loop(1, NC - 1, mlp_body, 0)
    XM[0] = XMZ
    with _scope("last"):
        first = mm_w3_first()
        tail = mm_w3_tail()
        w3_all(first, tail, JL)
        w4_plain(S - T, 0, LA)
        for _ in w4_steps2(S - T, JL):
            pass
        out_tail[0].start()
        w4_plain(S - T, LA, LAST0 - LA)
        out_tail[1].start()
        w4_plain(S - T, LAST0, T - LAST0)
        out_tail[2].start()
    with _scope("fin"):
        for i in range(NC - 1):
            out_copy(i).wait()
        for cp in out_tail:
            cp.wait()


@jax.jit
def pallas_adaLN_cond__ssm_conv_h3__mixer_s_mlp__prompt_kernel(
    A_q: jax.Array,
    A_k: jax.Array,
    A_v: jax.Array,
    A_shift_k: jax.Array,
    A_ssm_k: jax.Array,
    A_ssm_D: jax.Array,
    B_x: jax.Array,
    B_w1: jax.Array,
    B_w2: jax.Array,
    B_w3: jax.Array,
    B_w4: jax.Array,
    c: jax.Array,
    w_mod: jax.Array,
):
    del B_x
    any_spec = pl.BlockSpec(memory_space=pl.ANY)

    def tile_view(x):
        return x.reshape(S // 8, 8, CT, 128).transpose(0, 2, 1, 3).reshape(S * CT, 128)

    vm = pltpu.VMEM
    dma = pltpu.SemaphoreType.DMA
    spec = (4, NG, 16, 128)
    out = pl.pallas_call(
        _kernel,
        in_specs=[any_spec] * 12,
        out_specs=any_spec,
        out_shape=jax.ShapeDtypeStruct((S, D), bf16),
        scratch_shapes=[
            *[vm((KROWS, 128), bf16)] * NB, *[vm((VROWS, 128), bf16)] * NB, vm((CT, 128, S), bf16),
            vm((S, D), bf16), vm((D, D), bf16), vm((D, D), bf16), vm((F, D), bf16), vm((F, D), bf16),
            vm((D // 2, D), u32), vm((D // 2, D), u32), vm((F // 2, D), u32), vm((F // 2, D), u32),
            vm((D, 3 * D), bf16), vm((D, 2 * D), bf16), vm((D, D), bf16),
            vm((4, D), bf16), vm((D,), bf16), vm((1, D), bf16), vm((1, 1792), f32),
            vm((4, 128, 128), u32), vm((4, 128, 128), u32), vm((4, 64, 256), u32),
            vm((CT, 8, 8, 128), f32),
            vm((CT, NB) + spec, f32), vm((CT, NB - 1) + spec, f32), vm((CT,) + spec, f32),
            vm((CT, NB) + spec, f32), vm((4, 128, 128), f32),
            vm((CT, S + 32, 128), f32), vm((8, 8, D), f32),
            *[vm((S + 32, 128), f32)] * CT, vm((S + 256, D), f32), vm((S + 256, D), f32), vm((S, D), f32),
            vm((288, D), u32), vm((T // 2, D), u32), vm((D // 2, 128), u32),
            vm((640, 256), u32), vm((640, 256), u32), vm((NP3 * 64, 1280), u32), vm((7 * 448, 256), u32), vm((2, 448, 128), u32), vm((7 * 64, 1152), u32),
            vm((4, H, 128), f32), vm((5, H // 2, 256), u32), vm((5, H // 2, 256), u32),
            vm((H, D), u32), vm((H // 2, 1280), u32), vm((T, D), f32),
            vm((35 * 64, 384), u32), vm((4 * H, 256), f32), vm((7 * 64, 896), u32), vm((21 * 32 + 32, 640), u32), vm((T, D), f32), vm((16 * H, 128), f32),
            vm((S, D), bf16),
            dma((27,)), dma((NC + 2,)),
        ],
        compiler_params=pltpu.CompilerParams(vmem_limit_bytes=110 << 20, disable_bounds_checks=True,
                                             disable_semaphore_checks=True),
    )(A_q.reshape(S, D), tile_view(A_k), tile_view(A_v), A_shift_k.T, A_ssm_k,
      A_ssm_D, B_w1, B_w2, B_w3.T, B_w4, c, w_mod)
    return out.reshape(1, S, D)
```

```python
import numpy as np
import jax
import jax.numpy as jnp
import jax.experimental.pallas as pl
import jax.experimental.pallas.tpu as pltpu

f32, bf16, u32, i32 = jnp.float32, jnp.bfloat16, jnp.uint32, jnp.int32

S, D, F = 2048, 640, 1728
CT = D // 128
TR = 8 * CT
NB, BLK, NFFT = 4, 512, 1024
KROWS, VROWS = BLK * CT + 128, BLK * CT + 64
NG = 16
T = 256
NC = S // T
H = T // 2
NP3 = 6
FM = (F // 128) * 128
P0, P1, PA, PC = 320, 224, 160, 224
PB = P0 + P1 + PA
LA, LAST0 = 64, 208
RG = 16
EPS = 1e-5
NT_DIMS = (((1,), (1,)), ((), ()))
PAIRED = "10000100001000"
GV = 8
NL = 4


def _lo(w):
    return pltpu.bitcast(w << 16, f32)


def _hi(w):
    return pltpu.bitcast(w & jnp.uint32(0xFFFF0000), f32)


def _cis(n):
    t = (n & (2 * NFFT - 1)).astype(f32) * (np.pi / NFFT)
    return jnp.cos(t), jnp.sin(t)


def _fwd_table(r):
    g = jax.lax.broadcasted_iota(i32, (NG, 128), 0)
    cg, sg = _cis(jnp.where(g < NG // 2, 32 * g + 1, 32 * g - 253) * r)
    cs, ss = _cis(4 * jax.lax.broadcasted_iota(i32, (8, 128), 0) * r)
    parts = []
    for i in range(NG):
        c, s = cg[i:i + 1], sg[i:i + 1]
        parts += [c * cs - s * ss, -(s * cs + c * ss)]
    return pltpu.bitcast(jnp.concatenate(parts, axis=0).astype(bf16), u32)


def _inv_tables():
    def phase(rows):
        col = jax.lax.broadcasted_iota(i32, (rows, 256), 1)
        k = ((col >> 4) << 3) + (col & 7)
        row = jax.lax.broadcasted_iota(i32, (rows, 256), 0)
        return jnp.where(k < 64, 4 * k + 1, 4 * k - 253), (col & 8) << 6, row

    fr, _, g = phase(16)
    cg, sg = _cis(fr * (32 * g))
    fr, off, s = phase(8)
    out = []
    for p in range(4):
        cs, ss = _cis(fr * (4 * s + p) + off)
        cs, ss = cs * (2.0 / NFFT), ss * (2.0 / NFFT)
        parts = [cg[i:i + 1] * cs - sg[i:i + 1] * ss for i in range(16)]
        out.append(pltpu.bitcast(jnp.concatenate(parts, axis=0).astype(bf16), u32))
    return out


def _radix4(re, im, inverse):
    ar, ai = re[0] + re[2], im[0] + im[2]
    br, bi = re[0] - re[2], im[0] - im[2]
    cr, ci = re[1] + re[3], im[1] + im[3]
    dr, di = re[1] - re[3], im[1] - im[3]
    minus_i = (br + di, bi - dr)
    plus_i = (br - di, bi + dr)
    if inverse:
        return [(ar + cr, ai + ci), plus_i, (ar - cr, ai - ci), minus_i]
    return [(ar + cr, ai + ci), minus_i, (ar - cr, ai - ci), plus_i]


def _stats(x, link=None, early=False):
    zero = 0.0 if link is None else jnp.minimum(link, 0.0)
    part = x[:, 0:128]
    for c in range(1, CT):
        part = part + x[:, c * 128:(c + 1) * 128]
    if link is not None and early:
        part = part + zero
        zero = 0.0
    m = jnp.sum(part, axis=-1, keepdims=True) * (1.0 / D)
    v = jnp.maximum(jnp.sum(x * x, axis=-1, keepdims=True) * (1.0 / D) - m * m, zero)
    return m, jnp.exp2(jnp.log(v + EPS) * (-0.5 / np.log(2.0)))


def _gelu2(x):
    c = 0.7978845608028654
    u = c + (c * 0.044715) * (x * x)
    return x + x * jnp.tanh(x * u)


def _gelu(x):
    c = 0.7978845608028654
    u = c + (c * 0.044715) * (x * x)
    hx = 0.5 * x
    return hx + hx * jnp.tanh(x * u)


def _pk(x):
    return pltpu.bitcast(x.astype(bf16), u32)


def _ub(x):
    return pltpu.bitcast(x, bf16)


def _cat(xs, axis=-1):
    return jnp.concatenate(xs, axis=axis)


def _lanes(k):
    return slice(128 * k, 128 * (k + 1))


def _nn(a, w):
    return jnp.dot(a.astype(bf16), w, preferred_element_type=f32)


def _nt(a, w):
    return jax.lax.dot_general(a, w, NT_DIMS, preferred_element_type=f32)


def _lhs_sums(a11, a12, a21, a22):
    return [a11 + a22, a21 + a22, a11 + a12, a21 - a11, a12 - a22]


def _rhs_sum(k, block):
    a, b, plus = [(0, 3, True), (1, 3, False), (2, 0, False), (0, 1, True), (2, 3, True)][k]
    return block(a) + block(b) if plus else block(a) - block(b)


def _strassen(dot, a11, a22, asum, ax1, ax2, b11, b22, bsum, bx1, bx2):
    m2 = dot(asum[1], b11)
    m4 = dot(a22, bsum[2])
    c21 = (m4 + m2) + dot(ax2, bx1)
    m3 = dot(a11, bsum[1])
    m5 = dot(asum[2], b22)
    c12 = (m3 + m5) + dot(ax1, bx2)
    m1 = dot(asum[0], bsum[0])
    c11 = (((m4 - m5) + m1) + dot(asum[4], bsum[4])) + dot(ax1, bx1)
    c22 = (((m3 - m2) + m1) + dot(asum[3], bsum[3])) + dot(ax2, bx2)
    return [c11, c12, c21, c22]


def _kernel(q_hbm, k_hbm, v_hbm, sh_hbm, sk_hbm, d_hbm, w1_hbm, w2_hbm, w3_hbm, w4_hbm,
            c_hbm, wm_hbm, o_hbm,
            kb0, kb1, kb2, kb3, vb0, vb1, vb2, vb3, skb, qb, w1b, w2b, w3b, w4b, w1p, w2p, w3p,
            wma, wmb, wmc, shb, db, cb_, scb,
            fub, fkb, gtb, par, US, KS, UR, YS, YP, ys, modb, h10, h11, h12, h13, h14, h2s, x2s, hss,
            zt, zu, zb, zs, w3n, s1, s2, s3, s4, s5, p4, al, a2, c2, ob,
            sem, sem_o):
    h1s = [h10, h11, h12, h13, h14]
    n_in = [0]

    def load(src, dst):
        n_in[0] += 1
        return pltpu.make_async_copy(src, dst, sem.at[n_in[0] - 1])

    nkv = BLK * CT
    small = [load(d_hbm, db), load(sh_hbm, shb), load(c_hbm, cb_)]
    sk_copies = [load(sk_hbm.at[pl.ds(c * 128, 128), :], skb.at[c]) for c in range(CT)]
    kbs, vbs, wms = [kb0, kb1, kb2, kb3], [vb0, vb1, vb2, vb3], [wma, wmb, wmc]
    kv_copies = [[load(k_hbm.at[pl.ds(a * nkv, nkv), :], kbs[a].at[pl.ds(TR, nkv), :]),
                  load(v_hbm.at[pl.ds(a * nkv, nkv), :], vbs[a].at[pl.ds(0, nkv), :])] for a in range(NB)]
    mod_cols = [(0, 3 * D), (3 * D, 2 * D), (5 * D, D)]
    mod_copies = [load(wm_hbm.at[:, pl.ds(o, n)], w) for (o, n), w in zip(mod_cols, wms)]
    w_copies = [load(w1_hbm, w1b), load(w2_hbm, w2b), load(w3_hbm, w3b), load(w4_hbm, w4b)]
    q_copies = [load(q_hbm.at[pl.ds(o, n), :], qb.at[pl.ds(o, n), :])
                for o, n in [(0, P0 + P1), (P0 + P1, PA), (PB, S - PB)]]

    def out_copy(i):
        r = i * T if isinstance(i, int) else pl.multiple_of(i * T, T)
        return pltpu.make_async_copy(ob.at[pl.ds(r, T), :], o_hbm.at[pl.ds(r, T), :], sem_o.at[i])

    tail_parts = [(S - T, T, 128, D), (S - T, LAST0, 0, 128), (S - T + LAST0, T - LAST0, 0, 128)]
    out_tail = [pltpu.make_async_copy(ob.at[pl.ds(o, n), pl.ds(c0, c1 - c0)],
                                      o_hbm.at[pl.ds(o, n), pl.ds(c0, c1 - c0)], sem_o.at[NC - 1 + i])
                for i, (o, n, c0, c1) in enumerate(tail_parts)]

    for cp in (small + kv_copies[0] + sk_copies + kv_copies[1] + kv_copies[2] + kv_copies[3]
               + [mod_copies[0], q_copies[0], mod_copies[1], w_copies[0], w_copies[1], q_copies[1],
                  w_copies[2], w_copies[3], mod_copies[2], q_copies[2]]):
        cp.start()

    def wait(copies):
        for cp in copies:
            cp.wait()

    def pin(i, carry):
        z = jnp.zeros((8, 128), f32)
        scb[:, pl.ds(pl.multiple_of(i * 128, 128), 128)] = z[0:1]
        YP[i, 0:8, :] = z
        US[i, 0, 0, 0, 0:8, :] = z
        KS[i, 0, 0, 0, 0:8, :] = z
        YS[i, 0, 0, 0, 0:8, :] = z
        UR[i, 0, 0, 0:8, :] = z
        r8 = pl.ds(pl.multiple_of(i * 8, 8), 8)
        c2[r8, 0:128] = z
        al[r8, 0:128] = jnp.zeros((8, 128), u32)
        a2[r8, 0:128] = jnp.zeros((8, 128), u32)
        return carry

    def fence(i, carry):
        YP[i, 0:8, :] = jnp.zeros((8, 128), f32)
        return carry

    jax.lax.fori_loop(0, 2, pin, 0)
    lane = jax.lax.broadcasted_iota(i32, (1, 128), 1)
    for p in range(4):
        m = (lane - p) & 3
        fkb[p] = _fwd_table(128 * m + ((lane - m) & 127))
    for c in range(CT):
        kb0[c * 8:(c + 1) * 8, :] = jnp.zeros((8, 128), bf16)
        h1s[c][0:8, :] = jnp.zeros((8, 128), f32)
        h1s[c][S + 8:S + 16, :] = jnp.zeros((8, 128), f32)
    for a in range(NB):
        kbs[a][nkv + TR:KROWS, :] = jnp.zeros((KROWS - nkv - TR, 128), bf16)
        vbs[a][nkv:VROWS, :] = jnp.zeros((VROWS - nkv, 128), bf16)
    for p in range(4):
        fub[p] = _fwd_table(8 * (lane & 63) + ((lane >> 6) << 2) + p)
    wait(small)
    cvec = cb_[...].astype(f32)
    scb[:, 0:D] = cvec * jax.nn.sigmoid(cvec)
    dv = db[...].astype(f32).reshape(1, D)
    shv = shb[...].astype(f32)
    for c in range(CT):
        for i in range(4):
            par[c, i] = jnp.broadcast_to(shv[i:i + 1, c * 128:(c + 1) * 128], (8, 128))
        par[c, 4] = jnp.broadcast_to(dv[:, c * 128:(c + 1) * 128], (8, 128))
    for p, tab in enumerate(_inv_tables()):
        gtb[p] = tab

    def get(ref, idx, g, n):
        return (ref[idx + (slice(g, g + n), slice(0, 8))], ref[idx + (slice(g, g + n), slice(8, 16))])

    def put(ref, idx, g, n, xr, xi):
        ref[idx + (slice(g, g + n), slice(0, 8))] = xr
        ref[idx + (slice(g, g + n), slice(8, 16))] = xi

    def split(tt, g, n):
        tt = [t[g * 16:(g + n) * 16].reshape(n, 16, 128) for t in tt]
        return [t[:, 0:8] for t in tt], [t[:, 8:16] for t in tt]

    def fwd_k(c, j):
        lane = jax.lax.broadcasted_iota(i32, (64, 128), 1)
        even = (lane & 1) == 0
        l01 = (lane & 2) == 0
        l12 = ((lane + 3) & 2) == 0
        rm = []
        for m in range(4):
            w = pltpu.bitcast(skb[c, :, (4 * j + m) * 128:(4 * j + m + 1) * 128], u32)
            rm.append(pltpu.roll(w, m, 1) if m else w)
        e01 = jnp.where(even, rm[0], rm[1])
        o01 = jnp.where(even, rm[1], rm[0])
        e23 = jnp.where(even, rm[2], rm[3])
        o23 = jnp.where(even, rm[3], rm[2])
        kp = [jnp.where(l01, e01, e23), jnp.where(l12, o01, o23),
              jnp.where(l01, e23, e01), jnp.where(l12, o23, o01)]
        tt = [jax.lax.dot_general(pltpu.bitcast(fkb[p], bf16), pltpu.bitcast(kp[p], bf16), NT_DIMS,
                                  preferred_element_type=f32) for p in range(4)]
        for g in range(0, NG, GV):
            re, im = split(tt, g, GV)
            if j == 0:
                re[0] = re[0] + par[c, 4][None]
            for m, (xr, xi) in enumerate(_radix4(re, im, False)):
                if j < NB - 1:
                    put(KS, (c, j, m), g, GV, xr, xi)
                ur, ui = get(US, (c, 0, m), g, GV)
                put(YS, (c, j, m), g, GV, xr * ur - xi * ui, xr * ui + xi * ur)

    def fwd_u(c, a):
        taps = [jnp.tile(par[c, i], (8, 1)) for i in range(4)]
        ws = TR // 2
        base = 4 * c
        kw, vw = kbs[a].bitcast(u32), vbs[a].bitcast(u32)

        def words(ref, start):
            return ref[pl.ds(start, BLK // 8, stride=ws), :]

        kk = {}
        for w in range(4):
            x = words(kw, ws + base + w)
            kk[2 * w], kk[2 * w + 1] = _lo(x), _hi(x)
        kk[-3] = _hi(words(kw, base + 2))
        x = words(kw, base + 3)
        kk[-2], kk[-1] = _lo(x), _hi(x)
        sub = []
        for w in range(4):
            x = words(vw, base + w)
            for r, vv in ((2 * w, _lo(x)), (2 * w + 1, _hi(x))):
                sh = taps[0] * kk[r] + taps[1] * kk[r - 1] + taps[2] * kk[r - 2] + taps[3] * kk[r - 3]
                sub.append(sh * vv)
        kv = [jnp.concatenate([sub[p], sub[p + 4]], axis=0) for p in range(4)]
        tt = [jnp.dot(pltpu.bitcast(fub[p], bf16), kv[p].astype(bf16), preferred_element_type=f32)
              for p in range(4)]
        for g in range(0, NG, GV):
            re, im = split(tt, g, GV)
            for m, (xr, xi) in enumerate(_radix4(re, im, False)):
                if a:
                    pr, pi = get(US, (c, 0, m), g, GV) if a == 1 else get(UR, (c, m), g, GV)
                    if a < NB - 1:
                        put(UR, (c, m), g, GV, xr, xi)
                    xr, xi = (xr - pi, xi + pr) if g < NG // 2 else (xr + pi, xi - pr)
                put(US, (c, a, m), g, GV, xr, xi)

    def mac_inv(c, a):
        for h in range(2):
            vals = [[] for _ in range(4)]
            for g in range(8 * h, 8 * h + 8, GV):
                yre, yim = [], []
                for m in range(4):
                    yr, yi = get(YS, (c, a, m), g, GV)
                    for j in range(a):
                        kr, ki = get(KS, (c, j, m), g, GV)
                        ur, ui = get(US, (c, a - j, m), g, GV)
                        yr = yr + (kr * ur - ki * ui)
                        yi = yi + (kr * ui + ki * ur)
                    yre.append(yr)
                    yim.append(yi)
                for p, (pr, pi) in enumerate(_radix4(yre, yim, True)):
                    vals[p].append(jnp.concatenate([pr, pi], axis=1))
            for p in range(4):
                pb = jnp.concatenate(vals[p], axis=0).reshape(128, 128).astype(bf16)
                r = jnp.dot(pltpu.bitcast(gtb[p, :, h * 128:(h + 1) * 128], bf16), pb,
                            preferred_element_type=f32)
                if h == 0:
                    YP[p] = r
                else:
                    ys[c, pl.ds(a * BLK + p, 128, stride=4), :] = YP[p] + r

    wait(kv_copies[0])
    for c in range(CT):
        fwd_u(c, 0)
    for grp in ((0,), (1, 2), (3, 4)):
        wait([sk_copies[c] for c in grp])
        for c in grp:
            for j in (3, 2, 1, 0):
                fwd_k(c, j)
    for a in range(1, NB):
        wait(kv_copies[a])
        for c in range(CT):
            kbs[a][c * 8:(c + 1) * 8, :] = kbs[a - 1][nkv + c * 8:nkv + (c + 1) * 8, :]
        for c in range(CT):
            fwd_u(c, a)
            mac_inv(c, a - 1)
    jax.lax.fori_loop(0, 2, fence, 0)
    for c in range(NL):
        mac_inv(c, NB - 1)

    def mod_part(part, extra):
        n, wm = mod_cols[part][1], wms[part]
        act = scb[:, 0:D]

        def sc(k0, k1):
            return jnp.broadcast_to(act[:, k0:k1], (16, k1 - k0)).astype(bf16)

        e = 128 * extra
        r = jnp.dot(sc(0, D), wm[:, e:n], preferred_element_type=f32)
        r0 = (jnp.dot(sc(0, D - 64), wm[0:D - 64, 0:e], preferred_element_type=f32)
              + jnp.dot(sc(D - 64, D), wm[D - 64:D, 0:e], preferred_element_type=f32))
        r = jnp.concatenate([r0, r], axis=-1)[0:8]
        return [r[:, i * D:(i + 1) * D] for i in range(n // D)]

    def mvec(i, n=RG, c0=0, c1=D):
        return jnp.tile(modb[i, :, c0:c1], (n // 8, 1))

    rows = pl.ds

    def load_q(r, ref=qb):
        return ref[rows(r, RG), :].astype(f32)

    def make_x2(r, q, st, ref=ys):
        y = _cat([ref[c, rows(r, RG), :] for c in range(CT)])
        return q + (((q - st[0]) * st[1]) * mvec(1) + mvec(0)) * y

    def make_h2(x2, st):
        return ((x2 - st[0]) * st[1]) * mvec(3) + mvec(2)

    def put_sums(ref, o, z1, z2):
        for k, v in enumerate(_lhs_sums(z1[:, 0:256], z1[:, 256:512], z2[:, 0:256], z2[:, 256:512])):
            ref.at[k][o // 2:(o + RG) // 2, :] = _pk(v)

    def ln_chain(r, n, links=1, paired=""):
        qv, yv = qb.at[rows(r, n), :], ys.at[:, rows(r, n), :]
        xv, hv = x2s.at[rows(r, n), :], h2s.at[rows(r, n), :]
        prev, pend, cnt = [None] * links, None, 0
        for o1 in range(0, n // 2, RG):
            zz = []
            for o in (o1, o1 + n // 2):
                q = load_q(o, qv)
                x2 = make_x2(o, q, _stats(q, prev[cnt % links]), yv)
                xv[o:o + RG, :] = x2
                st = _stats(x2)
                h2 = make_h2(xv[o:o + RG, :], st)
                hv[o:o + RG, :] = h2
                st = _stats(h2)
                z = (hv[o:o + RG, :] - st[0]) * st[1]
                zt[o // 2:(o + RG) // 2, :] = _pk(z)
                zz.append(z)
                if paired and paired[cnt] == "1":
                    pend = st[1]
                elif pend is not None:
                    prev[0], pend = jnp.minimum(st[1], pend), None
                else:
                    prev[cnt % links] = st[1]
                cnt += 1
            put_sums(zu, o1, zz[0], zz[1])

    def ln_x1(r, links=1):
        hv, sv = h2s.at[rows(r, T), :], hss.at[rows(r, T), :]
        prev, cnt = [None] * links, 0
        for o1 in range(0, H, RG):
            zz = []
            for o in (o1, o1 + H):
                x1 = hv[o:o + RG, :] + sv[o:o + RG, :]
                st = _stats(x1, prev[cnt % links], early=True)
                z = (x1 - st[0]) * st[1]
                zb[o // 2:(o + RG) // 2, :] = _pk(z)
                zz.append(z)
                prev[cnt % links] = st[1]
                cnt += 1
            put_sums(zs, o1, zz[0], zz[1])

    def both(ref, r0, r1, col):
        return _cat([ref[r0:r1, _lanes(1 + col)].astype(f32), ref[r0:r1, _lanes(3 + col)].astype(f32)])

    def prep_square(wb, wp, sw):
        wp[...] = pltpu.bitcast(wb[...], u32)
        for k in (2, 1, 0, 4, 3):
            sw[128 * k:128 * (k + 1), :] = _pk(_rhs_sum(
                k, lambda b: both(wb, 256 * (b // 2), 256 * (b // 2 + 1), b % 2)))

    def mm_square(a, top, bot, asum, wp, sw):
        h = top.shape[0]
        c0 = _nn(a, _ub(wp[:, 0:128]))
        out = [(c0[0:h], c0[h:2 * h])]
        for n in range(2):
            l1, l2 = _lanes(2 * n + 1), _lanes(2 * n + 2)
            q = _strassen(_nn, top[:, 0:256], bot[:, 256:512], asum, top[:, 512:D], bot[:, 512:D],
                          _ub(wp[0:128, l1]), _ub(wp[128:256, l2]),
                          [_ub(sw[128 * k:128 * (k + 1), _lanes(n)]) for k in range(5)],
                          _ub(wp[256:320, l1]), _ub(wp[256:320, l2]))
            out += [(q[0], q[2]), (q[1], q[3])]
        return out

    def mm_w1(r, n, o=0):
        h, o = n // 2, o // 2
        res = mm_square(_ub(zt[o:o + h, :]), _ub(zt[o:o + h // 2, :]), _ub(zt[o + h // 2:o + h, :]),
                        [_ub(zu[k, 0:h // 2, :]) for k in range(5)], w1p, s1)
        for c, (top, bot) in enumerate(res):
            h1s[c][rows(r + 8, h), :] = _gelu(top)
            h1s[c][rows(r + 8 + h, h), :] = _gelu(bot)

    def mm_w2(r):
        lane = jax.lax.broadcasted_iota(i32, (T, 128), 1)

        def sh(k, c):
            return h1s[c][rows(r + 8 + k, T), :]

        g = _cat([sh(-1, 0),
                  jnp.where(lane < 32, sh(-1, 1), sh(1, 1)),
                  jnp.where(lane < 64, sh(1, 2), sh(-2, 2)),
                  jnp.where(lane < 96, sh(-2, 3), sh(2, 3)),
                  sh(2, 4)])
        top, bot = g[0:H], g[H:T]
        sums = _lhs_sums(top[:, 0:256], top[:, 256:512], bot[:, 0:256], bot[:, 256:512])
        for c, (ct, cb) in enumerate(mm_square(g, top, bot, sums, w2p, s2)):
            hss[rows(r, H), _lanes(c)] = ct
            hss[rows(r + H, H), _lanes(c)] = cb

    def prep_w3():
        for j in range(NP3):
            r0 = 128 * (2 * j + 1)
            w3p[r0 // 2:r0 // 2 + 64, 0:256] = pltpu.bitcast(w3b[r0:r0 + 128, 0:256], u32)
            w3p[r0 // 2:r0 // 2 + 64, 512:D] = pltpu.bitcast(w3b[r0:r0 + 128, 512:D], u32)
            w3p[r0 // 2 + 64:r0 // 2 + 128, 256:D] = pltpu.bitcast(w3b[r0 + 128:r0 + 256, 256:D], u32)
        w3p[FM // 2:F // 2, :] = pltpu.bitcast(w3b[FM:F, :], u32)
        w3n[...] = _pk(w3b[0:128, :].astype(f32).T)
        for j in range(NP3):
            r0 = 128 * (2 * j + 1)
            for k in (2, 1, 0, 4, 3):
                s3[64 * j:64 * (j + 1), 256 * k:256 * (k + 1)] = _pk(_rhs_sum(k, lambda b: w3b[
                    r0 + 128 * (b % 2):r0 + 128 * (b % 2 + 1), 256 * (b // 2):256 * (b // 2 + 1)].astype(f32)))

    def w3_first():
        return _gelu2(_nn(_ub(zb[...]), _ub(w3n[...])))

    def w3_tail():
        return _gelu2(_nt(_ub(w3p[FM // 2:F // 2, :]), _ub(zb[...])))

    def w3_pair(j):
        e, o = slice(64 * (2 * j + 1), 64 * (2 * j + 2)), slice(64 * (2 * j + 2), 64 * (2 * j + 3))
        z1, z2 = _ub(zb[0:H // 2, :]), _ub(zb[H // 2:H, :])
        q = _strassen(_nt, z1[:, 0:256], z2[:, 256:512], [_ub(zs[k]) for k in range(5)], z1[:, 512:D], z2[:, 512:D],
                      _ub(w3p[e, 0:256]), _ub(w3p[o, 256:512]),
                      [_ub(s3[64 * j:64 * (j + 1), 256 * k:256 * (k + 1)]) for k in range(5)],
                      _ub(w3p[e, 512:D]), _ub(w3p[o, 512:D]))
        return [_gelu2(c) for c in q]

    def put_quads(j, q):
        l1, l2, l5, l6, l7 = _lhs_sums(*q)
        al[64 * j:64 * (j + 1), :] = _pk(_cat([l1, l2, q[0], q[3], l5, l6, l7, q[1], q[2]]))

    def put_edge(first, tail):
        tp = _cat([tail.T, jnp.zeros((T, 64), f32)])
        put_quads(NP3, [first[0:H], tp[0:H], first[H:T], tp[H:T]])

    def w3_pairs(ahead):
        for i in range(NP3 // 2):
            ops = []
            for j in (2 * i, 2 * i + 1):
                q = w3_pair(j)
                if not ahead:
                    put_quads(j, q)
                ops.append(q)
            if not ahead:
                continue
            for n, q in enumerate(ops):
                l1, l2, l5, l6, l7 = _lhs_sums(*q)
                ops[n] = [l1, l2, q[0], q[3], l5, l6, l7]
                j, half = 2 * i + n, slice(64 * n, 64 * (n + 1))
                o = 64 * j + 32 * n
                al[o:o + 32, 0:256] = _pk(_cat([l1[half], l2[half]]))
                al[o:o + 32, 512:896] = _pk(_cat([l5[half], l6[half], l7[half]]))
                al[64 * j:64 * (j + 1), 256:512] = _pk(_cat([q[0], q[3]]))
                al[64 * j:64 * (j + 1), 896:1152] = _pk(_cat([q[1], q[2]]))
            for m in range(7):
                e, o = ops[0][m], ops[1][m]
                r0 = 32 * (3 * m + i)
                a2[r0:r0 + 32, :] = _pk(_cat(_lhs_sums(e[0:64], o[0:64], e[64:128], o[64:128])))

    def s4_block(m, b, axis):
        o = 448 * (m - 1) + 64 * (b // 2)
        return _cat([s4[o + 128 * i:o + 128 * i + 64, _lanes(b % 2)] for i in range(3)], axis)

    def prep_w4():
        def krow(j, par):
            return 128 * (2 * j + 1 + par) if j < NP3 else FM * par

        for j in range(7):
            p4[0, 64 * j:64 * (j + 1), :] = pltpu.bitcast(w4b[krow(j, 0):krow(j, 0) + 128, 0:128], u32)
            if j < NP3:
                p4[1, 64 * j:64 * (j + 1), :] = pltpu.bitcast(w4b[krow(j, 1):krow(j, 1) + 128, 0:128], u32)
            else:
                p4[1, 64 * j:64 * j + 32, :] = pltpu.bitcast(w4b[FM:F, 0:128], u32)
                p4[1, 64 * j + 32:64 * (j + 1), :] = jnp.zeros((32, 128), u32)

        def block(j, b):
            if j == NP3 and b >= 2:
                return _cat([both(w4b, FM, F, b % 2), jnp.zeros((64, 256), f32)], 0)
            return both(w4b, krow(j, b // 2), krow(j, b // 2) + 128, b % 2)

        for m, k in ((1, 0), (4, 2), (2, None), (3, 1), (5, None), (7, 4), (6, 3)):
            for j in range(7):
                o = 448 * (m - 1) + 64 * j
                if k is None and (j < NP3 or m == 2):
                    par = 0 if m == 2 else 1
                    for n in range(2):
                        s4[o:o + 64, _lanes(n)] = pltpu.bitcast(
                            w4b[krow(j, par):krow(j, par) + 128, _lanes(2 * n + 1 + par)], u32)
                else:
                    s4[o:o + 64, :] = _pk(block(j, 3) if k is None else _rhs_sum(k, lambda b: block(j, b)))
            for k2 in (2, 1, 0, 4, 3):
                o = 64 * (5 * (m - 1) + k2)
                s5[o:o + 64, :] = _pk(_rhs_sum(k2, lambda b: _ub(s4_block(m, b, -1)).astype(f32)))

    def finish(r, n, h, c):
        c0, c1 = 128 * c, 128 * (c + 1)
        x1 = h2s[rows(r, n), c0:c1] + hss[rows(r, n), c0:c1]
        base = x2s[rows(r, n), c0:c1] + mvec(4, n, c0, c1) * x1
        ob[rows(r, n), c0:c1] = (base + mvec(5, n, c0, c1) * h).astype(bf16)

    def w4_plain(r, o=0, n=T):
        def left(k):
            return _cat([al[64 * j:64 * (j + 1), _lanes(k)] for j in range(7)])

        a = _cat([_cat([left(2), left(7)]), _cat([left(8), left(3)])], 0)[o // 2:(o + n) // 2]
        finish(r + o, n, _nn(_ub(a), _ub(_cat([p4[0], p4[1]], 0))), 0)

    def w4_product(m, ahead):
        def blk(b):
            o = 64 * (b % 2) + 32 * (b // 2)
            return _ub(_cat([al[o + 128 * i:o + 128 * i + 32, _lanes(m - 1)] for i in range(3)]))

        if ahead:
            asum = [_ub(_cat([a2[32 * (3 * (m - 1) + i):32 * (3 * (m - 1) + i + 1), _lanes(k)] for i in range(3)]))
                    for k in range(5)]
        else:
            asum = _lhs_sums(*[blk(b).astype(f32) for b in range(4)])
        bsum = [_ub(_cat([s5[64 * (5 * (m - 1) + k):64 * (5 * (m - 1) + k + 1), _lanes(i)] for i in range(3)], 0))
                for k in range(5)]
        ox = 448 * (m - 1) + 384
        q = _strassen(_nn, blk(0), blk(3), asum, _ub(al[384:416, _lanes(m - 1)]), _ub(al[416:448, _lanes(m - 1)]),
                      _ub(s4_block(m, 0, 0)), _ub(s4_block(m, 3, 0)), bsum,
                      _ub(s4[ox:ox + 64, _lanes(0)]), _ub(s4[ox:ox + 64, _lanes(1)]))
        return _cat([_cat(q[0:2]), _cat(q[2:4])], 0)

    def w4_steps(r, ahead):
        acc = [c2.at[H * i:H * (i + 1), :] for i in range(4)]

        def finish2(rr, h, c):
            finish(rr, H, h[:, 0:128], c)
            finish(rr, H, h[:, 128:256], c + 2)

        acc[0][...] = w4_product(1, ahead)
        yield
        m4 = w4_product(4, ahead)
        acc[2][...] = m4
        acc[3][...] = acc[0][...] + m4
        yield
        m2 = w4_product(2, ahead)
        acc[0][...] = acc[0][...] - m2
        finish2(r + H, acc[2][...] + m2, 1)
        yield
        m3 = w4_product(3, ahead)
        acc[1][...] = m3
        acc[0][...] = acc[0][...] + m3
        yield
        m5 = w4_product(5, ahead)
        acc[3][...] = acc[3][...] - m5
        finish2(r, acc[1][...] + m5, 2)
        yield
        finish2(r, acc[3][...] + w4_product(7, ahead), 1)
        yield
        finish2(r + H, acc[0][...] + w4_product(6, ahead), 2)
        yield

    groups = list(range(0, P0 + P1, RG))
    wait([mod_copies[0], q_copies[0]])
    sa, ca, ga = mod_part(0, 1)
    modb[0] = ga * sa
    modb[1] = ga * (1.0 + ca)
    for c in range(NL, CT):
        mac_inv(c, NB - 1)
    st1 = {o: _stats(load_q(o)) for o in groups}
    zt[0:8, 0:128] = jnp.zeros((8, 128), u32)
    st2 = {}
    for o in groups:
        x2 = make_x2(o, load_q(o), st1[o])
        x2s[o:o + RG, :] = x2
        st2[o] = _stats(x2)

    wait([mod_copies[1]])
    sb, cb = mod_part(1, 2)
    modb[2] = sb
    modb[3] = 1.0 + cb
    st3 = {}
    for o in range(0, P0, RG):
        h2 = make_h2(x2s[o:o + RG, :], st2[o])
        h2s[o:o + RG, :] = h2
        st3[o] = _stats(h2)
    for o in range(0, P0, RG):
        zt[o // 2:(o + RG) // 2, :] = _pk((h2s[o:o + RG, :] - st3[o][0]) * st3[o][1])

    wait([w_copies[0]])
    prep_square(w1b, w1p, s1)
    z0 = _ub(zt[0:P0 // 2, :])
    h1 = _gelu(_nn(z0, _ub(w1p[:, 0:512])))
    for c in range(CT - 1):
        h1s[c][8:8 + P0, :] = h1[:, _lanes(c)]
    for o in range(0, P0, P0 // 4):
        h1s[CT - 1][8 + o:8 + o + P0 // 4, :] = _gelu(_nn(z0[o:o + P0 // 4], _ub(w1p[:, 512:D])))
    prev = None
    for o1 in range(0, P1 // 2, RG):
        zz = []
        for o in (P0 + o1, P0 + o1 + P1 // 2):
            h2 = make_h2(x2s[o:o + RG, :], st2[o])
            h2s[o:o + RG, :] = h2
            st = _stats(h2, prev, early=True)
            z = (h2 - st[0]) * st[1]
            zt[o // 2:(o + RG) // 2, :] = _pk(z)
            prev = st[1]
            zz.append(z)
        put_sums(zu, o1, zz[0], zz[1])
    mm_w1(P0, P1, P0)

    wait([w_copies[1], q_copies[1]])
    prep_square(w2b, w2p, s2)
    ln_chain(P0 + P1, PA, 2)
    mm_w2(0)
    ln_x1(0, 2)
    mm_w2(T)

    wait([w_copies[2]])
    prep_w3()
    mm_w1(P0 + P1, PA)
    tail = w3_tail()
    put_edge(w3_first(), tail)
    w3_pairs(True)

    wait([w_copies[3], mod_copies[2]])
    prep_w4()
    sc16 = jnp.broadcast_to(scb[:, 0:D], (16, D)).astype(bf16)
    steps, h = w4_steps(0, True), None
    for j in range(7):
        blk = [al[64 * j:64 * (j + 1), _lanes(k)] for k in (2, 7, 8, 3)]
        w = _ub(_cat([p4[0, 64 * j:64 * (j + 1), :], p4[1, 64 * j:64 * (j + 1), :]], 0))
        d = [_nn(_ub(_cat(blk[0:2])), w), _nn(_ub(_cat(blk[2:4])), w)]
        h = d if h is None else [h[0] + d[0], h[1] + d[1]]
        if j < 2:
            c0, c1 = (0, 384) if j == 0 else (384, D)
            gb = jnp.dot(sc16, wmc[:, c0:c1], preferred_element_type=f32)[0:8]
            modb[4, :, c0:c1] = gb
            modb[5, :, c0:c1] = 0.5 * gb
        if j == 6:
            finish(0, H, h[0], 0)
            finish(H, H, h[1], 0)
        next(steps)
    ln_x1(T)
    out_copy(0).start()
    q_copies[2].wait()

    def mlp_body(i, carry):
        r1 = pl.multiple_of(PB - PC + PC * i, 32)
        r = pl.multiple_of(i * T, T)
        first = w3_first()
        ln_chain(r1, PC, paired=PAIRED)
        put_edge(first, w3_tail())
        w3_pairs(False)
        mm_w1(r1, PC)
        w4_plain(r)
        mm_w2(r + T)
        ln_x1(r + T)
        for _ in w4_steps(r, False):
            pass
        out_copy(i).start()
        return carry

    jax.lax.fori_loop(1, NC - 1, mlp_body, 0)

    first = w3_first()
    put_edge(first, w3_tail())
    w3_pairs(True)
    w4_plain(S - T, 0, LA)
    for _ in w4_steps(S - T, True):
        pass
    out_tail[0].start()
    w4_plain(S - T, LA, LAST0 - LA)
    out_tail[1].start()
    w4_plain(S - T, LAST0, T - LAST0)
    out_tail[2].start()
    for i in range(NC - 1):
        out_copy(i).wait()
    for cp in out_tail:
        cp.wait()


@jax.jit
def pallas_adaLN_cond__ssm_conv_h3__mixer_s_mlp__prompt_kernel(
    A_q: jax.Array,
    A_k: jax.Array,
    A_v: jax.Array,
    A_shift_k: jax.Array,
    A_ssm_k: jax.Array,
    A_ssm_D: jax.Array,
    B_x: jax.Array,
    B_w1: jax.Array,
    B_w2: jax.Array,
    B_w3: jax.Array,
    B_w4: jax.Array,
    c: jax.Array,
    w_mod: jax.Array,
):
    del B_x
    any_spec = pl.BlockSpec(memory_space=pl.ANY)

    def tile_view(x):
        return x.reshape(S // 8, 8, CT, 128).transpose(0, 2, 1, 3).reshape(S * CT, 128)

    vm = pltpu.VMEM
    dma = pltpu.SemaphoreType.DMA
    spec = (4, NG, 16, 128)
    out = pl.pallas_call(
        _kernel,
        in_specs=[any_spec] * 12,
        out_specs=any_spec,
        out_shape=jax.ShapeDtypeStruct((S, D), bf16),
        scratch_shapes=[
            *[vm((KROWS, 128), bf16)] * NB, *[vm((VROWS, 128), bf16)] * NB, vm((CT, 128, S), bf16),
            vm((S, D), bf16), vm((D, D), bf16), vm((D, D), bf16), vm((F, D), bf16), vm((F, D), bf16),
            vm((D // 2, D), u32), vm((D // 2, D), u32), vm((F // 2, D), u32),
            vm((D, 3 * D), bf16), vm((D, 2 * D), bf16), vm((D, D), bf16),
            vm((4, D), bf16), vm((D,), bf16), vm((1, D), bf16), vm((1, 1792), f32),
            vm((4, 128, 128), u32), vm((4, 128, 128), u32), vm((4, 64, 256), u32),
            vm((CT, 8, 8, 128), f32),
            vm((CT, NB) + spec, f32), vm((CT, NB - 1) + spec, f32), vm((CT,) + spec, f32),
            vm((CT, NB) + spec, f32), vm((4, 128, 128), f32),
            vm((CT, S + 32, 128), f32), vm((8, 8, D), f32),
            *[vm((S + 32, 128), f32)] * CT, vm((S, D), f32), vm((S, D), f32), vm((S, D), f32),
            vm((288, D), u32), vm((5, H // 2, 256), u32), vm((H, D), u32), vm((5, H // 2, 256), u32),
            vm((D // 2, 128), u32), vm((D, 256), u32), vm((D, 256), u32), vm((NP3 * 64, 1280), u32),
            vm((7 * 448, 256), u32), vm((35 * 64, 384), u32), vm((2, 448, 128), u32),
            vm((7 * 64, 1152), u32), vm((21 * 32, 640), u32), vm((4 * H, 256), f32),
            vm((S, D), bf16),
            dma((26,)), dma((NC + 2,)),
        ],
        compiler_params=pltpu.CompilerParams(vmem_limit_bytes=110 << 20, disable_bounds_checks=True,
                                             disable_semaphore_checks=True),
    )(A_q.reshape(S, D), tile_view(A_k), tile_view(A_v), A_shift_k.T, A_ssm_k,
      A_ssm_D, B_w1, B_w2, B_w3.T, B_w4, c, w_mod)
    return out.reshape(1, S, D)
```

```python
import numpy as np
import jax
import jax.numpy as jnp
import jax.experimental.pallas as pl
import jax.experimental.pallas.tpu as pltpu

f32, bf16, u32, i32 = jnp.float32, jnp.bfloat16, jnp.uint32, jnp.int32

S, D, F = 2048, 640, 1728
CT = D // 128
TR = 8 * CT
NB, BLK, NFFT = 4, 512, 1024
KROWS, VROWS = BLK * CT + 128, BLK * CT + 64
NG = 16
T = 256
NC = S // T
H = T // 2
NP3 = 6
FM = (F // 128) * 128
P0, P1, PA, PC = 320, 224, 160, 224
PB = P0 + P1 + PA
LA, LAST0 = 96, 208
RG = 16
EPS = 1e-5
NT_DIMS = (((1,), (1,)), ((), ()))
PAIRED = "10000100001000"
ORD = {"r1_1": "42351c7a6db", "r2_2": "4d2c63a71b5", "r3_1": "c7254b631ad", "r3_3": "c4a25173b6d",
       "r4_4": "215a7b4cd36", "l_1": "c7325ba61d4", "l_2": "2c43b517a6d", "l_3": "24c35b1a76d",
       "l_4": "24ca35b176d", "z_3": "2bc31457a6d", "z_4": "1b2354d7ca6"}
OUTER = {"r4": "7163245", "l": "1423567", "z": "1536427"}
BODY = "1p2lsssssss"
HEAD = "nte3c"
LM = "0100000000000000"
R2M = "1000001010"
R2L = "1010100010101010"
R3O = "1tn3e"
R4O = "ppgspspsGpsspssp"
SE = 1
ZO = "nt3e"
FEN4 = 1
FA = 3
GV = 8
NL = 4


def _lo(w):
    return pltpu.bitcast(w << 16, f32)


def _hi(w):
    return pltpu.bitcast(w & jnp.uint32(0xFFFF0000), f32)


def _cis(n):
    t = (n & (2 * NFFT - 1)).astype(f32) * (np.pi / NFFT)
    return jnp.cos(t), jnp.sin(t)


def _fwd_table(r):
    g = jax.lax.broadcasted_iota(i32, (NG, 128), 0)
    cg, sg = _cis(jnp.where(g < NG // 2, 32 * g + 1, 32 * g - 253) * r)
    cs, ss = _cis(4 * jax.lax.broadcasted_iota(i32, (8, 128), 0) * r)
    parts = []
    for i in range(NG):
        c, s = cg[i:i + 1], sg[i:i + 1]
        parts += [c * cs - s * ss, -(s * cs + c * ss)]
    return pltpu.bitcast(jnp.concatenate(parts, axis=0).astype(bf16), u32)


def _inv_tables():
    def phase(rows):
        col = jax.lax.broadcasted_iota(i32, (rows, 256), 1)
        k = ((col >> 4) << 3) + (col & 7)
        row = jax.lax.broadcasted_iota(i32, (rows, 256), 0)
        return jnp.where(k < 64, 4 * k + 1, 4 * k - 253), (col & 8) << 6, row

    fr, _, g = phase(16)
    cg, sg = _cis(fr * (32 * g))
    fr, off, s = phase(8)
    out = []
    for p in range(4):
        cs, ss = _cis(fr * (4 * s + p) + off)
        cs, ss = cs * (2.0 / NFFT), ss * (2.0 / NFFT)
        parts = [cg[i:i + 1] * cs - sg[i:i + 1] * ss for i in range(16)]
        out.append(pltpu.bitcast(jnp.concatenate(parts, axis=0).astype(bf16), u32))
    return out


def _radix4(re, im, inverse):
    ar, ai = re[0] + re[2], im[0] + im[2]
    br, bi = re[0] - re[2], im[0] - im[2]
    cr, ci = re[1] + re[3], im[1] + im[3]
    dr, di = re[1] - re[3], im[1] - im[3]
    minus_i = (br + di, bi - dr)
    plus_i = (br - di, bi + dr)
    if inverse:
        return [(ar + cr, ai + ci), plus_i, (ar - cr, ai - ci), minus_i]
    return [(ar + cr, ai + ci), minus_i, (ar - cr, ai - ci), plus_i]


def _stats(x, link=None, early=False):
    zero = 0.0 if link is None else jnp.minimum(link, 0.0)
    part = x[:, 0:128]
    for c in range(1, CT):
        part = part + x[:, c * 128:(c + 1) * 128]
    if link is not None and early:
        part = part + zero
        zero = 0.0
    m = jnp.sum(part, axis=-1, keepdims=True) * (1.0 / D)
    v = jnp.maximum(jnp.sum(x * x, axis=-1, keepdims=True) * (1.0 / D) - m * m, zero)
    return m, jnp.exp2(jnp.log(v + EPS) * (-0.5 / np.log(2.0)))


def _gelu2(x):
    c = 0.7978845608028654
    u = c + (c * 0.044715) * (x * x)
    return x + x * jnp.tanh(x * u)


def _gelu(x):
    c = 0.7978845608028654
    u = c + (c * 0.044715) * (x * x)
    hx = 0.5 * x
    return hx + hx * jnp.tanh(x * u)


def _pk(x):
    return pltpu.bitcast(x.astype(bf16), u32)


def _ub(x):
    return pltpu.bitcast(x, bf16)


def _cat(xs, axis=-1):
    return jnp.concatenate(xs, axis=axis)


def _lanes(k):
    return slice(128 * k, 128 * (k + 1))


def _nn(a, w):
    return jnp.dot(a.astype(bf16), w, preferred_element_type=f32)


def _nt(a, w):
    return jax.lax.dot_general(a, w, NT_DIMS, preferred_element_type=f32)


def _lhs_sums(a11, a12, a21, a22):
    return [a11 + a22, a21 + a22, a11 + a12, a21 - a11, a12 - a22]


def _rhs_sum(k, block):
    a, b, plus = [(0, 3, True), (1, 3, False), (2, 0, False), (0, 1, True), (2, 3, True)][k]
    return block(a) + block(b) if plus else block(a) - block(b)


def _strassen(dot, a11, a22, asum, ax1, ax2, b11, b22, bsum, bx1, bx2, order=""):
    if order:
        ops = {"1": (asum[0], bsum[0], (1, 0, 0, 1)), "2": (asum[1], b11, (0, 0, 1, -1)),
               "3": (a11, bsum[1], (0, 1, 0, 1)), "4": (a22, bsum[2], (1, 0, 1, 0)),
               "5": (asum[2], b22, (-1, 1, 0, 0)), "6": (asum[3], bsum[3], (0, 0, 0, 1)),
               "7": (asum[4], bsum[4], (1, 0, 0, 0)), "a": (ax1, bx1, (1, 0, 0, 0)),
               "b": (ax1, bx2, (0, 1, 0, 0)), "c": (ax2, bx1, (0, 0, 1, 0)), "d": (ax2, bx2, (0, 0, 0, 1))}
        c, neg = [None] * 4, [None] * 4
        for t in order:
            a, b, sg = ops[t]
            m = dot(a, b)
            for i in range(4):
                if sg[i] > 0:
                    c[i] = m if c[i] is None else c[i] + m
                    if neg[i] is not None:
                        c[i], neg[i] = c[i] - neg[i], None
                elif sg[i] < 0:
                    if c[i] is None:
                        neg[i] = m
                    else:
                        c[i] = c[i] - m
        return c
    m2 = dot(asum[1], b11)
    m4 = dot(a22, bsum[2])
    c21 = (m4 + m2) + dot(ax2, bx1)
    m3 = dot(a11, bsum[1])
    m5 = dot(asum[2], b22)
    c12 = (m3 + m5) + dot(ax1, bx2)
    m1 = dot(asum[0], bsum[0])
    c11 = (((m4 - m5) + m1) + dot(asum[4], bsum[4])) + dot(ax1, bx1)
    c22 = (((m3 - m2) + m1) + dot(asum[3], bsum[3])) + dot(ax2, bx2)
    return [c11, c12, c21, c22]


def _kernel(q_hbm, k_hbm, v_hbm, sh_hbm, sk_hbm, d_hbm, w1_hbm, w2_hbm, w3_hbm, w4_hbm,
            c_hbm, wm_hbm, o_hbm,
            kb0, kb1, kb2, kb3, vb0, vb1, vb2, vb3, skb, qb, w1b, w2b, w3b, w4b, w1p, w2p, w3p,
            wma, wmb, wmc, shb, db, cb_, scb,
            fub, fkb, gtb, par, US, KS, UR, YS, YP, ys, modb, h10, h11, h12, h13, h14, h2s, x2s, hss,
            zt, zu, zb, zs, w3n, s1, s2, s3, s4, s5, p4, al, a2, c2, ob,
            sem, sem_o):
    h1s = [h10, h11, h12, h13, h14]
    n_in = [0]

    def load(src, dst):
        n_in[0] += 1
        return pltpu.make_async_copy(src, dst, sem.at[n_in[0] - 1])

    nkv = BLK * CT
    small = [load(d_hbm, db), load(sh_hbm, shb), load(c_hbm, cb_)]
    sk_copies = [load(sk_hbm.at[pl.ds(c * 128, 128), :], skb.at[c]) for c in range(CT)]
    kbs, vbs, wms = [kb0, kb1, kb2, kb3], [vb0, vb1, vb2, vb3], [wma, wmb, wmc]
    kv_copies = [[load(k_hbm.at[pl.ds(a * nkv, nkv), :], kbs[a].at[pl.ds(TR, nkv), :]),
                  load(v_hbm.at[pl.ds(a * nkv, nkv), :], vbs[a].at[pl.ds(0, nkv), :])] for a in range(NB)]
    mod_cols = [(0, 3 * D), (3 * D, 2 * D), (5 * D, D)]
    mod_copies = [load(wm_hbm.at[:, pl.ds(o, n)], w) for (o, n), w in zip(mod_cols, wms)]
    w_copies = [load(w1_hbm, w1b), load(w2_hbm, w2b), load(w3_hbm, w3b), load(w4_hbm, w4b)]
    q_copies = [load(q_hbm.at[pl.ds(o, n), :], qb.at[pl.ds(o, n), :])
                for o, n in [(0, P0 + P1), (P0 + P1, PA), (PB, S - PB)]]

    def out_copy(i):
        r = i * T if isinstance(i, int) else pl.multiple_of(i * T, T)
        return pltpu.make_async_copy(ob.at[pl.ds(r, T), :], o_hbm.at[pl.ds(r, T), :], sem_o.at[i])

    tail_parts = [(S - T, T, 128, D), (S - T, LAST0, 0, 128), (S - T + LAST0, T - LAST0, 0, 128)]
    out_tail = [pltpu.make_async_copy(ob.at[pl.ds(o, n), pl.ds(c0, c1 - c0)],
                                      o_hbm.at[pl.ds(o, n), pl.ds(c0, c1 - c0)], sem_o.at[NC - 1 + i])
                for i, (o, n, c0, c1) in enumerate(tail_parts)]

    for cp in (small + kv_copies[0] + sk_copies + kv_copies[1] + kv_copies[2] + kv_copies[3]
               + [mod_copies[0], q_copies[0], mod_copies[1], w_copies[0], w_copies[1], q_copies[1],
                  w_copies[2], w_copies[3], mod_copies[2], q_copies[2]]):
        cp.start()

    def wait(copies):
        for cp in copies:
            cp.wait()

    def pin(i, carry):
        z = jnp.zeros((8, 128), f32)
        scb[:, pl.ds(pl.multiple_of(i * 128, 128), 128)] = z[0:1]
        YP[i, 0:8, :] = z
        US[i, 0, 0, 0, 0:8, :] = z
        KS[i, 0, 0, 0, 0:8, :] = z
        YS[i, 0, 0, 0, 0:8, :] = z
        UR[i, 0, 0, 0:8, :] = z
        r8 = pl.ds(pl.multiple_of(i * 8, 8), 8)
        c2[r8, 0:128] = z
        al[r8, 0:128] = jnp.zeros((8, 128), u32)
        a2[r8, 0:128] = jnp.zeros((8, 128), u32)
        return carry

    def fence(i, carry):
        YP[i, 0:8, :] = jnp.zeros((8, 128), f32)
        return carry

    jax.lax.fori_loop(0, 2, pin, 0)
    lane = jax.lax.broadcasted_iota(i32, (1, 128), 1)
    for p in range(4):
        m = (lane - p) & 3
        fkb[p] = _fwd_table(128 * m + ((lane - m) & 127))
    for c in range(CT):
        kb0[c * 8:(c + 1) * 8, :] = jnp.zeros((8, 128), bf16)
        h1s[c][0:8, :] = jnp.zeros((8, 128), f32)
        h1s[c][S + 8:S + 16, :] = jnp.zeros((8, 128), f32)
    for a in range(NB):
        kbs[a][nkv + TR:KROWS, :] = jnp.zeros((KROWS - nkv - TR, 128), bf16)
        vbs[a][nkv:VROWS, :] = jnp.zeros((VROWS - nkv, 128), bf16)
    for p in range(4):
        fub[p] = _fwd_table(8 * (lane & 63) + ((lane >> 6) << 2) + p)
    wait(small)
    cvec = cb_[...].astype(f32)
    scb[:, 0:D] = cvec * jax.nn.sigmoid(cvec)
    dv = db[...].astype(f32).reshape(1, D)
    shv = shb[...].astype(f32)
    for c in range(CT):
        for i in range(4):
            par[c, i] = jnp.broadcast_to(shv[i:i + 1, c * 128:(c + 1) * 128], (8, 128))
        par[c, 4] = jnp.broadcast_to(dv[:, c * 128:(c + 1) * 128], (8, 128))
    for p, tab in enumerate(_inv_tables()):
        gtb[p] = tab

    def get(ref, idx, g, n):
        return (ref[idx + (slice(g, g + n), slice(0, 8))], ref[idx + (slice(g, g + n), slice(8, 16))])

    def put(ref, idx, g, n, xr, xi):
        ref[idx + (slice(g, g + n), slice(0, 8))] = xr
        ref[idx + (slice(g, g + n), slice(8, 16))] = xi

    def split(tt, g, n):
        tt = [t[g * 16:(g + n) * 16].reshape(n, 16, 128) for t in tt]
        return [t[:, 0:8] for t in tt], [t[:, 8:16] for t in tt]

    def fwd_k(c, j):
        lane = jax.lax.broadcasted_iota(i32, (64, 128), 1)
        even = (lane & 1) == 0
        l01 = (lane & 2) == 0
        l12 = ((lane + 3) & 2) == 0
        rm = []
        for m in range(4):
            w = pltpu.bitcast(skb[c, :, (4 * j + m) * 128:(4 * j + m + 1) * 128], u32)
            rm.append(pltpu.roll(w, m, 1) if m else w)
        e01 = jnp.where(even, rm[0], rm[1])
        o01 = jnp.where(even, rm[1], rm[0])
        e23 = jnp.where(even, rm[2], rm[3])
        o23 = jnp.where(even, rm[3], rm[2])
        kp = [jnp.where(l01, e01, e23), jnp.where(l12, o01, o23),
              jnp.where(l01, e23, e01), jnp.where(l12, o23, o01)]
        tt = [jax.lax.dot_general(pltpu.bitcast(fkb[p], bf16), pltpu.bitcast(kp[p], bf16), NT_DIMS,
                                  preferred_element_type=f32) for p in range(4)]
        for g in range(0, NG, GV):
            re, im = split(tt, g, GV)
            if j == 0:
                re[0] = re[0] + par[c, 4][None]
            for m, (xr, xi) in enumerate(_radix4(re, im, False)):
                if j < NB - 1:
                    put(KS, (c, j, m), g, GV, xr, xi)
                ur, ui = get(US, (c, 0, m), g, GV)
                put(YS, (c, j, m), g, GV, xr * ur - xi * ui, xr * ui + xi * ur)

    def fwd_u(c, a):
        taps = [jnp.tile(par[c, i], (8, 1)) for i in range(4)]
        ws = TR // 2
        base = 4 * c
        kw, vw = kbs[a].bitcast(u32), vbs[a].bitcast(u32)

        def words(ref, start):
            return ref[pl.ds(start, BLK // 8, stride=ws), :]

        kk = {}
        for w in range(4):
            x = words(kw, ws + base + w)
            kk[2 * w], kk[2 * w + 1] = _lo(x), _hi(x)
        kk[-3] = _hi(words(kw, base + 2))
        x = words(kw, base + 3)
        kk[-2], kk[-1] = _lo(x), _hi(x)
        sub = []
        for w in range(4):
            x = words(vw, base + w)
            for r, vv in ((2 * w, _lo(x)), (2 * w + 1, _hi(x))):
                sh = taps[0] * kk[r] + taps[1] * kk[r - 1] + taps[2] * kk[r - 2] + taps[3] * kk[r - 3]
                sub.append(sh * vv)
        kv = [jnp.concatenate([sub[p], sub[p + 4]], axis=0) for p in range(4)]
        tt = [jnp.dot(pltpu.bitcast(fub[p], bf16), kv[p].astype(bf16), preferred_element_type=f32)
              for p in range(4)]
        for g in range(0, NG, GV):
            re, im = split(tt, g, GV)
            for m, (xr, xi) in enumerate(_radix4(re, im, False)):
                if a:
                    pr, pi = get(US, (c, 0, m), g, GV) if a == 1 else get(UR, (c, m), g, GV)
                    if a < NB - 1:
                        put(UR, (c, m), g, GV, xr, xi)
                    xr, xi = (xr - pi, xi + pr) if g < NG // 2 else (xr + pi, xi - pr)
                put(US, (c, a, m), g, GV, xr, xi)

    def mac_inv(c, a):
        for h in range(2):
            vals = [[] for _ in range(4)]
            for g in range(8 * h, 8 * h + 8, GV):
                yre, yim = [], []
                for m in range(4):
                    yr, yi = get(YS, (c, a, m), g, GV)
                    for j in range(a):
                        kr, ki = get(KS, (c, j, m), g, GV)
                        ur, ui = get(US, (c, a - j, m), g, GV)
                        yr = yr + (kr * ur - ki * ui)
                        yi = yi + (kr * ui + ki * ur)
                    yre.append(yr)
                    yim.append(yi)
                for p, (pr, pi) in enumerate(_radix4(yre, yim, True)):
                    vals[p].append(jnp.concatenate([pr, pi], axis=1))
            for p in range(4):
                pb = jnp.concatenate(vals[p], axis=0).reshape(128, 128).astype(bf16)
                r = jnp.dot(pltpu.bitcast(gtb[p, :, h * 128:(h + 1) * 128], bf16), pb,
                            preferred_element_type=f32)
                if h == 0:
                    YP[p] = r
                else:
                    ys[c, pl.ds(a * BLK + p, 128, stride=4), :] = YP[p] + r

    wait(kv_copies[0])
    for c in range(CT):
        fwd_u(c, 0)
    for grp in ((0,), (1, 2), (3, 4)):
        wait([sk_copies[c] for c in grp])
        for c in grp:
            for j in (3, 2, 1, 0):
                fwd_k(c, j)
    for a in range(1, NB):
        if a == FA:
            jax.lax.fori_loop(0, 2, fence, 0)
        wait(kv_copies[a])
        for c in range(CT):
            kbs[a][c * 8:(c + 1) * 8, :] = kbs[a - 1][nkv + c * 8:nkv + (c + 1) * 8, :]
        for c in range(CT):
            fwd_u(c, a)
            mac_inv(c, a - 1)
    wait([mod_copies[0]])
    for c in range(NL):
        mac_inv(c, NB - 1)

    def mod_part(part, extra):
        n, wm = mod_cols[part][1], wms[part]
        act = scb[:, 0:D]

        def sc(k0, k1):
            return jnp.broadcast_to(act[:, k0:k1], (16, k1 - k0)).astype(bf16)

        e = 128 * extra
        r = jnp.dot(sc(0, D), wm[:, e:n], preferred_element_type=f32)
        r0 = (jnp.dot(sc(0, D - 64), wm[0:D - 64, 0:e], preferred_element_type=f32)
              + jnp.dot(sc(D - 64, D), wm[D - 64:D, 0:e], preferred_element_type=f32))
        r = jnp.concatenate([r0, r], axis=-1)[0:8]
        return [r[:, i * D:(i + 1) * D] for i in range(n // D)]

    def mvec(i, n=RG, c0=0, c1=D):
        return jnp.tile(modb[i, :, c0:c1], (n // 8, 1))

    rows = pl.ds
    ctx = ["r1"]

    def load_q(r, ref=qb):
        return ref[rows(r, RG), :].astype(f32)

    def make_x2(r, q, st, ref=ys):
        y = _cat([ref[c, rows(r, RG), :] for c in range(CT)])
        return q + (((q - st[0]) * st[1]) * mvec(1) + mvec(0)) * y

    def make_h2(x2, st):
        return ((x2 - st[0]) * st[1]) * mvec(3) + mvec(2)

    def put_sums(ref, o, z1, z2):
        for k, v in enumerate(_lhs_sums(z1[:, 0:256], z1[:, 256:512], z2[:, 0:256], z2[:, 256:512])):
            ref.at[k][o // 2:(o + RG) // 2, :] = _pk(v)

    def ln_chain(r, n, links=1, paired=""):
        qv, yv = qb.at[rows(r, n), :], ys.at[:, rows(r, n), :]
        xv, hv = x2s.at[rows(r, n), :], h2s.at[rows(r, n), :]
        prev, pend, cnt = [None] * links, None, 0
        for o1 in range(0, n // 2, RG):
            zz = []
            for o in (o1, o1 + n // 2):
                q = load_q(o, qv)
                x2 = make_x2(o, q, _stats(q, prev[cnt % links]), yv)
                xv[o:o + RG, :] = x2
                st = _stats(x2)
                h2 = make_h2(xv[o:o + RG, :], st)
                hv[o:o + RG, :] = h2
                st = _stats(h2)
                z = (hv[o:o + RG, :] - st[0]) * st[1]
                zt[o // 2:(o + RG) // 2, :] = _pk(z)
                zz.append(z)
                if paired and paired[cnt] == "1":
                    pend = st[1]
                elif pend is not None:
                    prev[0], pend = jnp.minimum(st[1], pend), None
                else:
                    prev[cnt % links] = st[1]
                cnt += 1
            put_sums(zu, o1, zz[0], zz[1])

    def ln_x1(r, paired="", stats=None, stats_only=False):
        hv, sv = h2s.at[rows(r, T), :], hss.at[rows(r, T), :]
        prev, pend, cnt, out = None, None, 0, []
        for o1 in range(0, H, RG):
            zz = []
            for o in (o1, o1 + H):
                x1 = hv[o:o + RG, :] + sv[o:o + RG, :]
                st = _stats(x1, prev, early=True) if stats is None else stats[cnt]
                out.append(st)
                if not stats_only:
                    z = (x1 - st[0]) * st[1]
                    zb[o // 2:(o + RG) // 2, :] = _pk(z)
                    zz.append(z)
                if paired and paired[cnt] == "1":
                    pend = st[1]
                elif pend is not None:
                    prev, pend = jnp.minimum(st[1], pend), None
                else:
                    prev = st[1]
                cnt += 1
            if not stats_only:
                put_sums(zs, o1, zz[0], zz[1])
        return out

    def both(ref, r0, r1, col):
        return _cat([ref[r0:r1, _lanes(1 + col)].astype(f32), ref[r0:r1, _lanes(3 + col)].astype(f32)])

    def prep_square(wb, wp, sw):
        wp[...] = pltpu.bitcast(wb[...], u32)
        for k in (2, 1, 0, 4, 3):
            sw[128 * k:128 * (k + 1), :] = _pk(_rhs_sum(
                k, lambda b: both(wb, 256 * (b // 2), 256 * (b // 2 + 1), b % 2)))

    def mm_square(a, top, bot, asum, wp, sw, which):
        h = top.shape[0]
        c0 = _nn(a, _ub(wp[:, 0:128]))
        out = [(c0[0:h], c0[h:2 * h])]
        for n in range(2):
            l1, l2 = _lanes(2 * n + 1), _lanes(2 * n + 2)
            q = _strassen(_nn, top[:, 0:256], bot[:, 256:512], asum, top[:, 512:D], bot[:, 512:D],
                          _ub(wp[0:128, l1]), _ub(wp[128:256, l2]),
                          [_ub(sw[128 * k:128 * (k + 1), _lanes(n)]) for k in range(5)],
                          _ub(wp[256:320, l1]), _ub(wp[256:320, l2]), ORD[ctx[0] + "_" + which])
            out += [(q[0], q[2]), (q[1], q[3])]
        return out

    def mm_w1(r, n, o=0):
        h, o = n // 2, o // 2
        res = mm_square(_ub(zt[o:o + h, :]), _ub(zt[o:o + h // 2, :]), _ub(zt[o + h // 2:o + h, :]),
                        [_ub(zu[k, 0:h // 2, :]) for k in range(5)], w1p, s1, "1")
        for c, (top, bot) in enumerate(res):
            h1s[c][rows(r + 8, h), :] = _gelu(top)
            h1s[c][rows(r + 8 + h, h), :] = _gelu(bot)

    def mm_w2(r):
        lane = jax.lax.broadcasted_iota(i32, (T, 128), 1)

        def sh(k, c):
            return h1s[c][rows(r + 8 + k, T), :]

        g = _cat([sh(-1, 0),
                  jnp.where(lane < 32, sh(-1, 1), sh(1, 1)),
                  jnp.where(lane < 64, sh(1, 2), sh(-2, 2)),
                  jnp.where(lane < 96, sh(-2, 3), sh(2, 3)),
                  sh(2, 4)])
        top, bot = g[0:H], g[H:T]
        sums = _lhs_sums(top[:, 0:256], top[:, 256:512], bot[:, 0:256], bot[:, 256:512])
        for c, (ct, cb) in enumerate(mm_square(g, top, bot, sums, w2p, s2, "2")):
            hss[rows(r, H), _lanes(c)] = ct
            hss[rows(r + H, H), _lanes(c)] = cb

    def prep_w3():
        for j in range(NP3):
            r0 = 128 * (2 * j + 1)
            w3p[r0 // 2:r0 // 2 + 64, 0:256] = pltpu.bitcast(w3b[r0:r0 + 128, 0:256], u32)
            w3p[r0 // 2:r0 // 2 + 64, 512:D] = pltpu.bitcast(w3b[r0:r0 + 128, 512:D], u32)
            w3p[r0 // 2 + 64:r0 // 2 + 128, 256:D] = pltpu.bitcast(w3b[r0 + 128:r0 + 256, 256:D], u32)
        w3p[FM // 2:F // 2, :] = pltpu.bitcast(w3b[FM:F, :], u32)
        w3n[...] = _pk(w3b[0:128, :].astype(f32).T)
        for j in range(NP3):
            r0 = 128 * (2 * j + 1)
            for k in (2, 1, 0, 4, 3):
                s3[64 * j:64 * (j + 1), 256 * k:256 * (k + 1)] = _pk(_rhs_sum(k, lambda b: w3b[
                    r0 + 128 * (b % 2):r0 + 128 * (b % 2 + 1), 256 * (b // 2):256 * (b // 2 + 1)].astype(f32)))

    def w3_first():
        return _gelu2(_nn(_ub(zb[...]), _ub(w3n[...])))

    def w3_tail():
        return _gelu2(_nt(_ub(w3p[FM // 2:F // 2, :]), _ub(zb[...])))

    def w3_pair(j):
        e, o = slice(64 * (2 * j + 1), 64 * (2 * j + 2)), slice(64 * (2 * j + 2), 64 * (2 * j + 3))
        z1, z2 = _ub(zb[0:H // 2, :]), _ub(zb[H // 2:H, :])
        q = _strassen(_nt, z1[:, 0:256], z2[:, 256:512], [_ub(zs[k]) for k in range(5)], z1[:, 512:D], z2[:, 512:D],
                      _ub(w3p[e, 0:256]), _ub(w3p[o, 256:512]),
                      [_ub(s3[64 * j:64 * (j + 1), 256 * k:256 * (k + 1)]) for k in range(5)],
                      _ub(w3p[e, 512:D]), _ub(w3p[o, 512:D]), ORD[ctx[0] + "_3"])
        return [_gelu2(c) for c in q]

    def put_quads(j, q):
        l1, l2, l5, l6, l7 = _lhs_sums(*q)
        al[64 * j:64 * (j + 1), :] = _pk(_cat([l1, l2, q[0], q[3], l5, l6, l7, q[1], q[2]]))

    def put_edge(first, tail):
        tp = _cat([tail.T, jnp.zeros((T, 64), f32)])
        put_quads(NP3, [first[0:H], tp[0:H], first[H:T], tp[H:T]])

    def w3_pairs(ahead):
        for i in range(NP3 // 2):
            ops = []
            for j in (2 * i, 2 * i + 1):
                q = w3_pair(j)
                if not ahead:
                    put_quads(j, q)
                ops.append(q)
            if not ahead:
                continue
            for n, q in enumerate(ops):
                l1, l2, l5, l6, l7 = _lhs_sums(*q)
                ops[n] = [l1, l2, q[0], q[3], l5, l6, l7]
                j, half = 2 * i + n, slice(64 * n, 64 * (n + 1))
                o = 64 * j + 32 * n
                al[o:o + 32, 0:256] = _pk(_cat([l1[half], l2[half]]))
                al[o:o + 32, 512:896] = _pk(_cat([l5[half], l6[half], l7[half]]))
                al[64 * j:64 * (j + 1), 256:512] = _pk(_cat([q[0], q[3]]))
                al[64 * j:64 * (j + 1), 896:1152] = _pk(_cat([q[1], q[2]]))
            for m in range(7):
                e, o = ops[0][m], ops[1][m]
                r0 = 32 * (3 * m + i)
                a2[r0:r0 + 32, :] = _pk(_cat(_lhs_sums(e[0:64], o[0:64], e[64:128], o[64:128])))

    def s4_block(m, b, axis):
        o = 448 * (m - 1) + 64 * (b // 2)
        return _cat([s4[o + 128 * i:o + 128 * i + 64, _lanes(b % 2)] for i in range(3)], axis)

    def prep_w4():
        def krow(j, par):
            return 128 * (2 * j + 1 + par) if j < NP3 else FM * par

        for j in range(7):
            p4[0, 64 * j:64 * (j + 1), :] = pltpu.bitcast(w4b[krow(j, 0):krow(j, 0) + 128, 0:128], u32)
            if j < NP3:
                p4[1, 64 * j:64 * (j + 1), :] = pltpu.bitcast(w4b[krow(j, 1):krow(j, 1) + 128, 0:128], u32)
            else:
                p4[1, 64 * j:64 * j + 32, :] = pltpu.bitcast(w4b[FM:F, 0:128], u32)
                p4[1, 64 * j + 32:64 * (j + 1), :] = jnp.zeros((32, 128), u32)

        def block(j, b):
            if j == NP3 and b >= 2:
                return _cat([both(w4b, FM, F, b % 2), jnp.zeros((64, 256), f32)], 0)
            return both(w4b, krow(j, b // 2), krow(j, b // 2) + 128, b % 2)

        for m in [int(t) for t in OUTER['r4']]:
            k = {1: 0, 4: 2, 2: None, 3: 1, 5: None, 7: 4, 6: 3}[m]
            for j in range(7):
                o = 448 * (m - 1) + 64 * j
                if k is None and (j < NP3 or m == 2):
                    par = 0 if m == 2 else 1
                    for n in range(2):
                        s4[o:o + 64, _lanes(n)] = pltpu.bitcast(
                            w4b[krow(j, par):krow(j, par) + 128, _lanes(2 * n + 1 + par)], u32)
                else:
                    s4[o:o + 64, :] = _pk(block(j, 3) if k is None else _rhs_sum(k, lambda b: block(j, b)))
            for k2 in (2, 1, 0, 4, 3):
                o = 64 * (5 * (m - 1) + k2)
                s5[o:o + 64, :] = _pk(_rhs_sum(k2, lambda b: _ub(s4_block(m, b, -1)).astype(f32)))

    def finish(r, n, h, c):
        c0, c1 = 128 * c, 128 * (c + 1)
        x1 = h2s[rows(r, n), c0:c1] + hss[rows(r, n), c0:c1]
        base = x2s[rows(r, n), c0:c1] + mvec(4, n, c0, c1) * x1
        ob[rows(r, n), c0:c1] = (base + mvec(5, n, c0, c1) * h).astype(bf16)

    def w4_plain(r, o=0, n=T):
        def left(k):
            return _cat([al[64 * j:64 * (j + 1), _lanes(k)] for j in range(7)])

        a = _cat([_cat([left(2), left(7)]), _cat([left(8), left(3)])], 0)[o // 2:(o + n) // 2]
        finish(r + o, n, _nn(_ub(a), _ub(_cat([p4[0], p4[1]], 0))), 0)

    def w4_product(m, ahead, order=None):
        def blk(b):
            o = 64 * (b % 2) + 32 * (b // 2)
            return _ub(_cat([al[o + 128 * i:o + 128 * i + 32, _lanes(m - 1)] for i in range(3)]))

        if ahead:
            asum = [_ub(_cat([a2[32 * (3 * (m - 1) + i):32 * (3 * (m - 1) + i + 1), _lanes(k)] for i in range(3)]))
                    for k in range(5)]
        else:
            asum = _lhs_sums(*[blk(b).astype(f32) for b in range(4)])
        bsum = [_ub(_cat([s5[64 * (5 * (m - 1) + k):64 * (5 * (m - 1) + k + 1), _lanes(i)] for i in range(3)], 0))
                for k in range(5)]
        ox = 448 * (m - 1) + 384
        q = _strassen(_nn, blk(0), blk(3), asum, _ub(al[384:416, _lanes(m - 1)]), _ub(al[416:448, _lanes(m - 1)]),
                      _ub(s4_block(m, 0, 0)), _ub(s4_block(m, 3, 0)), bsum,
                      _ub(s4[ox:ox + 64, _lanes(0)]), _ub(s4[ox:ox + 64, _lanes(1)]), ORD[ctx[0] + "_4"])
        return _cat([_cat(q[0:2]), _cat(q[2:4])], 0)

    def w4_steps(r, ahead):
        acc = [c2.at[H * i:H * (i + 1), :] for i in range(4)]

        def finish2(rr, h, c):
            finish(rr, H, h[:, 0:128], c)
            finish(rr, H, h[:, 128:256], c + 2)

        sign = {1: (1, 0, 0, 1), 2: (0, 0, 1, -1), 3: (0, 1, 0, 1), 4: (1, 0, 1, 0), 5: (-1, 1, 0, 0),
                6: (0, 0, 0, 1), 7: (1, 0, 0, 0)}
        left_n, state = [4, 2, 2, 4], [None] * 4
        for m in [int(t) for t in OUTER[ctx[0]]]:
            x = w4_product(m, ahead)
            outs = [i for i in range(4) if sign[m][i]]
            olds = {i: None if state[i] is None else state[i][0][...] for i in outs}
            busy = [state[i][0] for i in range(4) if state[i] is not None and i not in outs]
            free = [a for a in acc if not any(a is b for b in busy)]
            shared = None
            for i in outs:
                sg = sign[m][i]
                left_n[i] -= 1
                if state[i] is None:
                    if shared is None:
                        shared = free.pop()
                        shared[...] = x
                    state[i] = (shared, sg)
                    continue
                v = olds[i] + x if (sg > 0) == (state[i][1] > 0) else (x - olds[i] if sg > 0 else olds[i] - x)
                if left_n[i] == 0:
                    finish2(r + H * (i // 2), v, 1 + i % 2)
                    state[i] = None
                else:
                    dst = free.pop()
                    dst[...] = v
                    state[i] = (dst, 1)
            yield

    def up(order, ahead, r1=None, n1=None):
        for tok in order:
            if tok == "n":
                first = w3_first()
            elif tok == "t":
                tail = w3_tail()
            elif tok == "e":
                put_edge(first, tail)
            elif tok == "3":
                w3_pairs(ahead)
            elif tok == "1":
                mm_w1(r1, n1)
            elif tok == "c":
                ln_chain(r1, n1, paired=PAIRED)

    groups = list(range(0, P0 + P1, RG))
    wait([q_copies[0]])
    sa, ca, ga = mod_part(0, 1)
    modb[0] = ga * sa
    modb[1] = ga * (1.0 + ca)
    for c in range(NL, CT):
        mac_inv(c, NB - 1)
    st1 = {o: _stats(load_q(o)) for o in groups}
    zt[0:8, 0:128] = jnp.zeros((8, 128), u32)
    st2 = {}
    for o in groups:
        x2 = make_x2(o, load_q(o), st1[o])
        x2s[o:o + RG, :] = x2
        st2[o] = _stats(x2)

    wait([mod_copies[1]])
    sb, cb = mod_part(1, 2)
    modb[2] = sb
    modb[3] = 1.0 + cb
    st3 = {}
    for o in range(0, P0, RG):
        h2 = make_h2(x2s[o:o + RG, :], st2[o])
        h2s[o:o + RG, :] = h2
        st3[o] = _stats(h2)
    for o in range(0, P0, RG):
        zt[o // 2:(o + RG) // 2, :] = _pk((h2s[o:o + RG, :] - st3[o][0]) * st3[o][1])

    wait([w_copies[0]])
    prep_square(w1b, w1p, s1)
    z0 = _ub(zt[0:P0 // 2, :])
    h1 = _gelu(_nn(z0, _ub(w1p[:, 0:512])))
    for c in range(CT - 1):
        h1s[c][8:8 + P0, :] = h1[:, _lanes(c)]
    for o in range(0, P0, P0 // 4):
        h1s[CT - 1][8 + o:8 + o + P0 // 4, :] = _gelu(_nn(z0[o:o + P0 // 4], _ub(w1p[:, 512:D])))
    prev = None
    for o1 in range(0, P1 // 2, RG):
        zz = []
        for o in (P0 + o1, P0 + o1 + P1 // 2):
            h2 = make_h2(x2s[o:o + RG, :], st2[o])
            h2s[o:o + RG, :] = h2
            st = _stats(h2, prev, early=True)
            z = (h2 - st[0]) * st[1]
            zt[o // 2:(o + RG) // 2, :] = _pk(z)
            prev = st[1]
            zz.append(z)
        put_sums(zu, o1, zz[0], zz[1])
    mm_w1(P0, P1, P0)

    ctx[0] = "r2"
    wait([w_copies[1], q_copies[1]])
    prep_square(w2b, w2p, s2)
    ln_chain(P0 + P1, PA, paired=R2M)
    mm_w2(0)
    ln_x1(0, R2L)
    mm_w2(T)

    ctx[0] = "r3"
    wait([w_copies[2]])
    prep_w3()
    early = ln_x1(T, stats_only=True) if SE else None
    up(R3O, True, P0 + P1, PA)

    ctx[0] = "r4"
    if FEN4:
        jax.lax.fori_loop(0, 2, fence, 0)
    wait([w_copies[3], mod_copies[2]])
    prep_w4()
    sc16 = jnp.broadcast_to(scb[:, 0:D], (16, D)).astype(bf16)
    steps, h, j = w4_steps(0, True), None, 0
    for tok in R4O:
        if tok == "p":
            blk = [al[64 * j:64 * (j + 1), _lanes(k)] for k in (2, 7, 8, 3)]
            w = _ub(_cat([p4[0, 64 * j:64 * (j + 1), :], p4[1, 64 * j:64 * (j + 1), :]], 0))
            d = [_nn(_ub(_cat(blk[0:2])), w), _nn(_ub(_cat(blk[2:4])), w)]
            h = d if h is None else [h[0] + d[0], h[1] + d[1]]
            j += 1
            if j == 7:
                finish(0, H, h[0], 0)
                finish(H, H, h[1], 0)
        elif tok == "s":
            next(steps)
        else:
            c0, c1 = (0, 384) if tok == "g" else (384, D)
            gb = jnp.dot(sc16, wmc[:, c0:c1], preferred_element_type=f32)[0:8]
            modb[4, :, c0:c1] = gb
            modb[5, :, c0:c1] = 0.5 * gb
    ln_x1(T, stats=early)
    out_copy(0).start()
    q_copies[2].wait()

    def mlp_body(i, carry):
        r1 = pl.multiple_of(PB - PC + PC * i, 32)
        r = pl.multiple_of(i * T, T)
        up(HEAD, False, r1, PC)
        steps = w4_steps(r, False)
        for tok in BODY:
            if tok == "1":
                mm_w1(r1, PC)
            elif tok == "p":
                w4_plain(r)
            elif tok == "2":
                mm_w2(r + T)
            elif tok == "l":
                ln_x1(r + T, LM)
            else:
                next(steps)
        out_copy(i).start()
        return carry

    ctx[0] = "l"
    jax.lax.fori_loop(1, NC - 1, mlp_body, 0)

    ctx[0] = "z"
    up(ZO, True)
    if LA:
        w4_plain(S - T, 0, LA)
    for _ in w4_steps(S - T, True):
        pass
    out_tail[0].start()
    w4_plain(S - T, LA, LAST0 - LA)
    out_tail[1].start()
    w4_plain(S - T, LAST0, T - LAST0)
    out_tail[2].start()
    for i in range(NC - 1):
        out_copy(i).wait()
    for cp in out_tail:
        cp.wait()


@jax.jit
def pallas_adaLN_cond__ssm_conv_h3__mixer_s_mlp__prompt_kernel(
    A_q: jax.Array,
    A_k: jax.Array,
    A_v: jax.Array,
    A_shift_k: jax.Array,
    A_ssm_k: jax.Array,
    A_ssm_D: jax.Array,
    B_x: jax.Array,
    B_w1: jax.Array,
    B_w2: jax.Array,
    B_w3: jax.Array,
    B_w4: jax.Array,
    c: jax.Array,
    w_mod: jax.Array,
):
    del B_x
    any_spec = pl.BlockSpec(memory_space=pl.ANY)

    def tile_view(x):
        return x.reshape(S // 8, 8, CT, 128).transpose(0, 2, 1, 3).reshape(S * CT, 128)

    vm = pltpu.VMEM
    dma = pltpu.SemaphoreType.DMA
    spec = (4, NG, 16, 128)
    out = pl.pallas_call(
        _kernel,
        in_specs=[any_spec] * 12,
        out_specs=any_spec,
        out_shape=jax.ShapeDtypeStruct((S, D), bf16),
        scratch_shapes=[
            *[vm((KROWS, 128), bf16)] * NB, *[vm((VROWS, 128), bf16)] * NB, vm((CT, 128, S), bf16),
            vm((S, D), bf16), vm((D, D), bf16), vm((D, D), bf16), vm((F, D), bf16), vm((F, D), bf16),
            vm((D // 2, D), u32), vm((D // 2, D), u32), vm((F // 2, D), u32),
            vm((D, 3 * D), bf16), vm((D, 2 * D), bf16), vm((D, D), bf16),
            vm((4, D), bf16), vm((D,), bf16), vm((1, D), bf16), vm((1, 1792), f32),
            vm((4, 128, 128), u32), vm((4, 128, 128), u32), vm((4, 64, 256), u32),
            vm((CT, 8, 8, 128), f32),
            vm((CT, NB) + spec, f32), vm((CT, NB - 1) + spec, f32), vm((CT,) + spec, f32),
            vm((CT, NB) + spec, f32), vm((4, 128, 128), f32),
            vm((CT, S + 32, 128), f32), vm((8, 8, D), f32),
            *[vm((S + 32, 128), f32)] * CT, vm((S, D), f32), vm((S, D), f32), vm((S, D), f32),
            vm((288, D), u32), vm((5, H // 2, 256), u32), vm((H, D), u32), vm((5, H // 2, 256), u32),
            vm((D // 2, 128), u32), vm((D, 256), u32), vm((D, 256), u32), vm((NP3 * 64, 1280), u32),
            vm((7 * 448, 256), u32), vm((35 * 64, 384), u32), vm((2, 448, 128), u32),
            vm((7 * 64, 1152), u32), vm((21 * 32, 640), u32), vm((4 * H, 256), f32),
            vm((S, D), bf16),
            dma((26,)), dma((NC + 2,)),
        ],
        compiler_params=pltpu.CompilerParams(vmem_limit_bytes=110 << 20, disable_bounds_checks=True,
                                             disable_semaphore_checks=True),
    )(A_q.reshape(S, D), tile_view(A_k), tile_view(A_v), A_shift_k.T, A_ssm_k,
      A_ssm_D, B_w1, B_w2, B_w3.T, B_w4, c, w_mod)
    return out.reshape(1, S, D)
```

```python
import numpy as np
import jax
import jax.numpy as jnp
import jax.experimental.pallas as pl
import jax.experimental.pallas.tpu as pltpu

f32, bf16, u32, i32 = jnp.float32, jnp.bfloat16, jnp.uint32, jnp.int32

S, D, F = 2048, 640, 1728
CT = D // 128
TR = 8 * CT
NB, BLK, NFFT = 4, 512, 1024
KROWS, VROWS = BLK * CT + 128, BLK * CT + 64
NG = 16
T = 256
NC = S // T
H = T // 2
NP3 = 6
FM = (F // 128) * 128
P0, P1, PA, PC = 320, 224, 160, 224
PB = P0 + P1 + PA
LA, LAST0 = 96, 208
RG = 16
EPS = 1e-5
NT_DIMS = (((1,), (1,)), ((), ()))
PAIRED = "10000100001000"
ORD = {"r1_1": "42351c7a6db", "r2_2": "4d2c36a71b5", "r3_1": "7254b6c31ad", "r3_3": "4c2a5173b6d",
       "r4_4": "215a7b4dc36", "l_1": "c7325ba61d4", "l_2": "2c43b517a6d", "l_3": "24c35b1a76d",
       "l_4": "24ca351b76d", "z_3": "c2b31457a6d", "z_4": "2354db17ca6"}
OUTER = {"r4": "7163245", "l": "1423657", "z": "1536472"}
BODY = "1p2lsssssss"
HEAD = "ncte3"
LM = "0100000000000000"
R2M = "1000001010"
R2L = "1010100100101010"
R3O = "1tne3"
R4O = "ppgspspsGpsspssp"
SE = 1
ZO = "nt3e"
FEN4 = 1
FA = 3
GV = 8
NL = 4


def _lo(w):
    return pltpu.bitcast(w << 16, f32)


def _hi(w):
    return pltpu.bitcast(w & jnp.uint32(0xFFFF0000), f32)


def _cis(n):
    t = (n & (2 * NFFT - 1)).astype(f32) * (np.pi / NFFT)
    return jnp.cos(t), jnp.sin(t)


def _fwd_table(r):
    g = jax.lax.broadcasted_iota(i32, (NG, 128), 0)
    cg, sg = _cis(jnp.where(g < NG // 2, 32 * g + 1, 32 * g - 253) * r)
    cs, ss = _cis(4 * jax.lax.broadcasted_iota(i32, (8, 128), 0) * r)
    parts = []
    for i in range(NG):
        c, s = cg[i:i + 1], sg[i:i + 1]
        parts += [c * cs - s * ss, -(s * cs + c * ss)]
    return pltpu.bitcast(jnp.concatenate(parts, axis=0).astype(bf16), u32)


def _inv_tables():
    def phase(rows):
        col = jax.lax.broadcasted_iota(i32, (rows, 256), 1)
        k = ((col >> 4) << 3) + (col & 7)
        row = jax.lax.broadcasted_iota(i32, (rows, 256), 0)
        return jnp.where(k < 64, 4 * k + 1, 4 * k - 253), (col & 8) << 6, row

    fr, _, g = phase(16)
    cg, sg = _cis(fr * (32 * g))
    fr, off, s = phase(8)
    out = []
    for p in range(4):
        cs, ss = _cis(fr * (4 * s + p) + off)
        cs, ss = cs * (2.0 / NFFT), ss * (2.0 / NFFT)
        parts = [cg[i:i + 1] * cs - sg[i:i + 1] * ss for i in range(16)]
        out.append(pltpu.bitcast(jnp.concatenate(parts, axis=0).astype(bf16), u32))
    return out


def _radix4(re, im, inverse):
    ar, ai = re[0] + re[2], im[0] + im[2]
    br, bi = re[0] - re[2], im[0] - im[2]
    cr, ci = re[1] + re[3], im[1] + im[3]
    dr, di = re[1] - re[3], im[1] - im[3]
    minus_i = (br + di, bi - dr)
    plus_i = (br - di, bi + dr)
    if inverse:
        return [(ar + cr, ai + ci), plus_i, (ar - cr, ai - ci), minus_i]
    return [(ar + cr, ai + ci), minus_i, (ar - cr, ai - ci), plus_i]


def _stats(x, link=None, early=False):
    zero = 0.0 if link is None else jnp.minimum(link, 0.0)
    part = x[:, 0:128]
    for c in range(1, CT):
        part = part + x[:, c * 128:(c + 1) * 128]
    if link is not None and early:
        part = part + zero
        zero = 0.0
    m = jnp.sum(part, axis=-1, keepdims=True) * (1.0 / D)
    v = jnp.maximum(jnp.sum(x * x, axis=-1, keepdims=True) * (1.0 / D) - m * m, zero)
    return m, jnp.exp2(jnp.log(v + EPS) * (-0.5 / np.log(2.0)))


def _gelu2(x):
    c = 0.7978845608028654
    u = c + (c * 0.044715) * (x * x)
    return x + x * jnp.tanh(x * u)


def _gelu(x):
    c = 0.7978845608028654
    u = c + (c * 0.044715) * (x * x)
    hx = 0.5 * x
    return hx + hx * jnp.tanh(x * u)


def _pk(x):
    return pltpu.bitcast(x.astype(bf16), u32)


def _ub(x):
    return pltpu.bitcast(x, bf16)


def _cat(xs, axis=-1):
    return jnp.concatenate(xs, axis=axis)


def _lanes(k):
    return slice(128 * k, 128 * (k + 1))


def _nn(a, w):
    return jnp.dot(a.astype(bf16), w, preferred_element_type=f32)


def _nt(a, w):
    return jax.lax.dot_general(a, w, NT_DIMS, preferred_element_type=f32)


def _lhs_sums(a11, a12, a21, a22):
    return [a11 + a22, a21 + a22, a11 + a12, a21 - a11, a12 - a22]


def _rhs_sum(k, block):
    a, b, plus = [(0, 3, True), (1, 3, False), (2, 0, False), (0, 1, True), (2, 3, True)][k]
    return block(a) + block(b) if plus else block(a) - block(b)


def _strassen(dot, a11, a22, asum, ax1, ax2, b11, b22, bsum, bx1, bx2, order=""):
    if order:
        ops = {"1": (asum[0], bsum[0], (1, 0, 0, 1)), "2": (asum[1], b11, (0, 0, 1, -1)),
               "3": (a11, bsum[1], (0, 1, 0, 1)), "4": (a22, bsum[2], (1, 0, 1, 0)),
               "5": (asum[2], b22, (-1, 1, 0, 0)), "6": (asum[3], bsum[3], (0, 0, 0, 1)),
               "7": (asum[4], bsum[4], (1, 0, 0, 0)), "a": (ax1, bx1, (1, 0, 0, 0)),
               "b": (ax1, bx2, (0, 1, 0, 0)), "c": (ax2, bx1, (0, 0, 1, 0)), "d": (ax2, bx2, (0, 0, 0, 1))}
        c, neg = [None] * 4, [None] * 4
        for t in order:
            a, b, sg = ops[t]
            m = dot(a, b)
            for i in range(4):
                if sg[i] > 0:
                    c[i] = m if c[i] is None else c[i] + m
                    if neg[i] is not None:
                        c[i], neg[i] = c[i] - neg[i], None
                elif sg[i] < 0:
                    if c[i] is None:
                        neg[i] = m
                    else:
                        c[i] = c[i] - m
        return c
    m2 = dot(asum[1], b11)
    m4 = dot(a22, bsum[2])
    c21 = (m4 + m2) + dot(ax2, bx1)
    m3 = dot(a11, bsum[1])
    m5 = dot(asum[2], b22)
    c12 = (m3 + m5) + dot(ax1, bx2)
    m1 = dot(asum[0], bsum[0])
    c11 = (((m4 - m5) + m1) + dot(asum[4], bsum[4])) + dot(ax1, bx1)
    c22 = (((m3 - m2) + m1) + dot(asum[3], bsum[3])) + dot(ax2, bx2)
    return [c11, c12, c21, c22]


def _kernel(q_hbm, k_hbm, v_hbm, sh_hbm, sk_hbm, d_hbm, w1_hbm, w2_hbm, w3_hbm, w4_hbm,
            c_hbm, wm_hbm, o_hbm,
            kb0, kb1, kb2, kb3, vb0, vb1, vb2, vb3, skb, qb, w1b, w2b, w3b, w4b, w1p, w2p, w3p,
            wma, wmb, wmc, shb, db, cb_, scb,
            fub, fkb, gtb, par, US, KS, UR, YS, YP, ys, modb, h10, h11, h12, h13, h14, h2s, x2s, hss,
            zt, zu, zb, zs, w3n, s1, s2, s3, s4, s5, p4, al, a2, c2, ob,
            sem, sem_o):
    h1s = [h10, h11, h12, h13, h14]
    n_in = [0]

    def load(src, dst):
        n_in[0] += 1
        return pltpu.make_async_copy(src, dst, sem.at[n_in[0] - 1])

    nkv = BLK * CT
    small = [load(d_hbm, db), load(sh_hbm, shb), load(c_hbm, cb_)]
    sk_copies = [load(sk_hbm.at[pl.ds(c * 128, 128), :], skb.at[c]) for c in range(CT)]
    kbs, vbs, wms = [kb0, kb1, kb2, kb3], [vb0, vb1, vb2, vb3], [wma, wmb, wmc]
    kv_copies = [[load(k_hbm.at[pl.ds(a * nkv, nkv), :], kbs[a].at[pl.ds(TR, nkv), :]),
                  load(v_hbm.at[pl.ds(a * nkv, nkv), :], vbs[a].at[pl.ds(0, nkv), :])] for a in range(NB)]
    mod_cols = [(0, 3 * D), (3 * D, 2 * D), (5 * D, D)]
    mod_copies = [load(wm_hbm.at[:, pl.ds(o, n)], w) for (o, n), w in zip(mod_cols, wms)]
    w_copies = [load(w1_hbm, w1b), load(w2_hbm, w2b), load(w3_hbm, w3b), load(w4_hbm, w4b)]
    q_copies = [load(q_hbm.at[pl.ds(o, n), :], qb.at[pl.ds(o, n), :])
                for o, n in [(0, P0 + P1), (P0 + P1, PA), (PB, S - PB)]]

    def out_copy(i):
        r = i * T if isinstance(i, int) else pl.multiple_of(i * T, T)
        return pltpu.make_async_copy(ob.at[pl.ds(r, T), :], o_hbm.at[pl.ds(r, T), :], sem_o.at[i])

    out_tail = []

    def send(r, n, c):
        cp = pltpu.make_async_copy(ob.at[pl.ds(r, n), pl.ds(128 * c, 128)], o_hbm.at[pl.ds(r, n), pl.ds(128 * c, 128)],
                                   sem_o.at[NC - 1 + len(out_tail)])
        out_tail.append(cp)
        cp.start()

    for cp in (small + kv_copies[0] + sk_copies + kv_copies[1] + kv_copies[2] + kv_copies[3]
               + [mod_copies[0], q_copies[0], mod_copies[1], w_copies[0], w_copies[1], q_copies[1],
                  w_copies[2], w_copies[3], mod_copies[2], q_copies[2]]):
        cp.start()

    def wait(copies):
        for cp in copies:
            cp.wait()

    def pin(i, carry):
        z = jnp.zeros((8, 128), f32)
        scb[:, pl.ds(pl.multiple_of(i * 128, 128), 128)] = z[0:1]
        YP[i, 0:8, :] = z
        US[i, 0, 0, 0, 0:8, :] = z
        KS[i, 0, 0, 0, 0:8, :] = z
        YS[i, 0, 0, 0, 0:8, :] = z
        UR[i, 0, 0, 0:8, :] = z
        r8 = pl.ds(pl.multiple_of(i * 8, 8), 8)
        c2[r8, 0:128] = z
        al[r8, 0:128] = jnp.zeros((8, 128), u32)
        a2[r8, 0:128] = jnp.zeros((8, 128), u32)
        return carry

    def fence(i, carry):
        YP[i, 0:8, :] = jnp.zeros((8, 128), f32)
        return carry

    jax.lax.fori_loop(0, 2, pin, 0)
    lane = jax.lax.broadcasted_iota(i32, (1, 128), 1)
    for p in range(4):
        m = (lane - p) & 3
        fkb[p] = _fwd_table(128 * m + ((lane - m) & 127))
    for c in range(CT):
        kb0[c * 8:(c + 1) * 8, :] = jnp.zeros((8, 128), bf16)
        h1s[c][0:8, :] = jnp.zeros((8, 128), f32)
        h1s[c][S + 8:S + 16, :] = jnp.zeros((8, 128), f32)
    for a in range(NB):
        kbs[a][nkv + TR:KROWS, :] = jnp.zeros((KROWS - nkv - TR, 128), bf16)
        vbs[a][nkv:VROWS, :] = jnp.zeros((VROWS - nkv, 128), bf16)
    for p in range(4):
        fub[p] = _fwd_table(8 * (lane & 63) + ((lane >> 6) << 2) + p)
    wait(small)
    cvec = cb_[...].astype(f32)
    scb[:, 0:D] = cvec * jax.nn.sigmoid(cvec)
    dv = db[...].astype(f32).reshape(1, D)
    shv = shb[...].astype(f32)
    for c in range(CT):
        for i in range(4):
            par[c, i] = jnp.broadcast_to(shv[i:i + 1, c * 128:(c + 1) * 128], (8, 128))
        par[c, 4] = jnp.broadcast_to(dv[:, c * 128:(c + 1) * 128], (8, 128))
    for p, tab in enumerate(_inv_tables()):
        gtb[p] = tab

    def get(ref, idx, g, n):
        return (ref[idx + (slice(g, g + n), slice(0, 8))], ref[idx + (slice(g, g + n), slice(8, 16))])

    def put(ref, idx, g, n, xr, xi):
        ref[idx + (slice(g, g + n), slice(0, 8))] = xr
        ref[idx + (slice(g, g + n), slice(8, 16))] = xi

    def split(tt, g, n):
        tt = [t[g * 16:(g + n) * 16].reshape(n, 16, 128) for t in tt]
        return [t[:, 0:8] for t in tt], [t[:, 8:16] for t in tt]

    def fwd_k(c, j):
        lane = jax.lax.broadcasted_iota(i32, (64, 128), 1)
        even = (lane & 1) == 0
        l01 = (lane & 2) == 0
        l12 = ((lane + 3) & 2) == 0
        rm = []
        for m in range(4):
            w = pltpu.bitcast(skb[c, :, (4 * j + m) * 128:(4 * j + m + 1) * 128], u32)
            rm.append(pltpu.roll(w, m, 1) if m else w)
        e01 = jnp.where(even, rm[0], rm[1])
        o01 = jnp.where(even, rm[1], rm[0])
        e23 = jnp.where(even, rm[2], rm[3])
        o23 = jnp.where(even, rm[3], rm[2])
        kp = [jnp.where(l01, e01, e23), jnp.where(l12, o01, o23),
              jnp.where(l01, e23, e01), jnp.where(l12, o23, o01)]
        tt = [jax.lax.dot_general(pltpu.bitcast(fkb[p], bf16), pltpu.bitcast(kp[p], bf16), NT_DIMS,
                                  preferred_element_type=f32) for p in range(4)]
        for g in range(0, NG, GV):
            re, im = split(tt, g, GV)
            if j == 0:
                re[0] = re[0] + par[c, 4][None]
            for m, (xr, xi) in enumerate(_radix4(re, im, False)):
                if j < NB - 1:
                    put(KS, (c, j, m), g, GV, xr, xi)
                ur, ui = get(US, (c, 0, m), g, GV)
                put(YS, (c, j, m), g, GV, xr * ur - xi * ui, xr * ui + xi * ur)

    def fwd_u(c, a):
        taps = [jnp.tile(par[c, i], (8, 1)) for i in range(4)]
        ws = TR // 2
        base = 4 * c
        kw, vw = kbs[a].bitcast(u32), vbs[a].bitcast(u32)

        def words(ref, start):
            return ref[pl.ds(start, BLK // 8, stride=ws), :]

        kk = {}
        for w in range(4):
            x = words(kw, ws + base + w)
            kk[2 * w], kk[2 * w + 1] = _lo(x), _hi(x)
        kk[-3] = _hi(words(kw, base + 2))
        x = words(kw, base + 3)
        kk[-2], kk[-1] = _lo(x), _hi(x)
        sub = []
        for w in range(4):
            x = words(vw, base + w)
            for r, vv in ((2 * w, _lo(x)), (2 * w + 1, _hi(x))):
                sh = taps[0] * kk[r] + taps[1] * kk[r - 1] + taps[2] * kk[r - 2] + taps[3] * kk[r - 3]
                sub.append(sh * vv)
        kv = [jnp.concatenate([sub[p], sub[p + 4]], axis=0) for p in range(4)]
        tt = [jnp.dot(pltpu.bitcast(fub[p], bf16), kv[p].astype(bf16), preferred_element_type=f32)
              for p in range(4)]
        for g in range(0, NG, GV):
            re, im = split(tt, g, GV)
            for m, (xr, xi) in enumerate(_radix4(re, im, False)):
                if a:
                    pr, pi = get(US, (c, 0, m), g, GV) if a == 1 else get(UR, (c, m), g, GV)
                    if a < NB - 1:
                        put(UR, (c, m), g, GV, xr, xi)
                    xr, xi = (xr - pi, xi + pr) if g < NG // 2 else (xr + pi, xi - pr)
                put(US, (c, a, m), g, GV, xr, xi)

    def mac_inv(c, a):
        for h in range(2):
            vals = [[] for _ in range(4)]
            for g in range(8 * h, 8 * h + 8, GV):
                yre, yim = [], []
                for m in range(4):
                    yr, yi = get(YS, (c, a, m), g, GV)
                    for j in range(a):
                        kr, ki = get(KS, (c, j, m), g, GV)
                        ur, ui = get(US, (c, a - j, m), g, GV)
                        yr = yr + (kr * ur - ki * ui)
                        yi = yi + (kr * ui + ki * ur)
                    yre.append(yr)
                    yim.append(yi)
                for p, (pr, pi) in enumerate(_radix4(yre, yim, True)):
                    vals[p].append(jnp.concatenate([pr, pi], axis=1))
            for p in range(4):
                pb = jnp.concatenate(vals[p], axis=0).reshape(128, 128).astype(bf16)
                r = jnp.dot(pltpu.bitcast(gtb[p, :, h * 128:(h + 1) * 128], bf16), pb,
                            preferred_element_type=f32)
                if h == 0:
                    YP[p] = r
                else:
                    ys[c, pl.ds(a * BLK + p, 128, stride=4), :] = YP[p] + r

    wait(kv_copies[0])
    for c in range(CT):
        fwd_u(c, 0)
    for grp in ((0,), (1, 2), (3, 4)):
        wait([sk_copies[c] for c in grp])
        for c in grp:
            for j in (3, 2, 1, 0):
                fwd_k(c, j)
    for a in range(1, NB):
        if a == FA:
            jax.lax.fori_loop(0, 2, fence, 0)
        wait(kv_copies[a])
        for c in range(CT):
            kbs[a][c * 8:(c + 1) * 8, :] = kbs[a - 1][nkv + c * 8:nkv + (c + 1) * 8, :]
        for c in range(CT):
            fwd_u(c, a)
            mac_inv(c, a - 1)
    wait([mod_copies[0]])
    for c in range(NL):
        mac_inv(c, NB - 1)

    def mod_part(part, extra):
        n, wm = mod_cols[part][1], wms[part]
        act = scb[:, 0:D]

        def sc(k0, k1):
            return jnp.broadcast_to(act[:, k0:k1], (16, k1 - k0)).astype(bf16)

        e = 128 * extra
        r = jnp.dot(sc(0, D), wm[:, e:n], preferred_element_type=f32)
        r0 = (jnp.dot(sc(0, D - 64), wm[0:D - 64, 0:e], preferred_element_type=f32)
              + jnp.dot(sc(D - 64, D), wm[D - 64:D, 0:e], preferred_element_type=f32))
        r = jnp.concatenate([r0, r], axis=-1)[0:8]
        return [r[:, i * D:(i + 1) * D] for i in range(n // D)]

    def mvec(i, n=RG, c0=0, c1=D):
        return jnp.tile(modb[i, :, c0:c1], (n // 8, 1))

    rows = pl.ds
    ctx = ["r1"]

    def load_q(r, ref=qb):
        return ref[rows(r, RG), :].astype(f32)

    def make_x2(r, q, st, ref=ys):
        y = _cat([ref[c, rows(r, RG), :] for c in range(CT)])
        return q + (((q - st[0]) * st[1]) * mvec(1) + mvec(0)) * y

    def make_h2(x2, st):
        return ((x2 - st[0]) * st[1]) * mvec(3) + mvec(2)

    def put_sums(ref, o, z1, z2):
        for k, v in enumerate(_lhs_sums(z1[:, 0:256], z1[:, 256:512], z2[:, 0:256], z2[:, 256:512])):
            ref.at[k][o // 2:(o + RG) // 2, :] = _pk(v)

    def ln_chain(r, n, links=1, paired=""):
        qv, yv = qb.at[rows(r, n), :], ys.at[:, rows(r, n), :]
        xv, hv = x2s.at[rows(r, n), :], h2s.at[rows(r, n), :]
        prev, pend, cnt = [None] * links, None, 0
        for o1 in range(0, n // 2, RG):
            zz = []
            for o in (o1, o1 + n // 2):
                q = load_q(o, qv)
                x2 = make_x2(o, q, _stats(q, prev[cnt % links]), yv)
                xv[o:o + RG, :] = x2
                st = _stats(x2)
                h2 = make_h2(xv[o:o + RG, :], st)
                hv[o:o + RG, :] = h2
                st = _stats(h2)
                z = (hv[o:o + RG, :] - st[0]) * st[1]
                zt[o // 2:(o + RG) // 2, :] = _pk(z)
                zz.append(z)
                if paired and paired[cnt] == "1":
                    pend = st[1]
                elif pend is not None:
                    prev[0], pend = jnp.minimum(st[1], pend), None
                else:
                    prev[cnt % links] = st[1]
                cnt += 1
            put_sums(zu, o1, zz[0], zz[1])

    def ln_x1(r, paired="", stats=None, stats_only=False):
        hv, sv = h2s.at[rows(r, T), :], hss.at[rows(r, T), :]
        prev, pend, cnt, out = None, None, 0, []
        for o1 in range(0, H, RG):
            zz = []
            for o in (o1, o1 + H):
                x1 = hv[o:o + RG, :] + sv[o:o + RG, :]
                st = _stats(x1, prev, early=True) if stats is None else stats[cnt]
                out.append(st)
                if not stats_only:
                    z = (x1 - st[0]) * st[1]
                    zb[o // 2:(o + RG) // 2, :] = _pk(z)
                    zz.append(z)
                if paired and paired[cnt] == "1":
                    pend = st[1]
                elif pend is not None:
                    prev, pend = jnp.minimum(st[1], pend), None
                else:
                    prev = st[1]
                cnt += 1
            if not stats_only:
                put_sums(zs, o1, zz[0], zz[1])
        return out

    def both(ref, r0, r1, col):
        return _cat([ref[r0:r1, _lanes(1 + col)].astype(f32), ref[r0:r1, _lanes(3 + col)].astype(f32)])

    def prep_square(wb, wp, sw):
        wp[...] = pltpu.bitcast(wb[...], u32)
        for k in (2, 1, 0, 4, 3):
            sw[128 * k:128 * (k + 1), :] = _pk(_rhs_sum(
                k, lambda b: both(wb, 256 * (b // 2), 256 * (b // 2 + 1), b % 2)))

    def mm_square(a, top, bot, asum, wp, sw, which):
        h = top.shape[0]
        c0 = _nn(a, _ub(wp[:, 0:128]))
        out = [(c0[0:h], c0[h:2 * h])]
        for n in range(2):
            l1, l2 = _lanes(2 * n + 1), _lanes(2 * n + 2)
            q = _strassen(_nn, top[:, 0:256], bot[:, 256:512], asum, top[:, 512:D], bot[:, 512:D],
                          _ub(wp[0:128, l1]), _ub(wp[128:256, l2]),
                          [_ub(sw[128 * k:128 * (k + 1), _lanes(n)]) for k in range(5)],
                          _ub(wp[256:320, l1]), _ub(wp[256:320, l2]), ORD[ctx[0] + "_" + which])
            out += [(q[0], q[2]), (q[1], q[3])]
        return out

    def mm_w1(r, n, o=0):
        h, o = n // 2, o // 2
        res = mm_square(_ub(zt[o:o + h, :]), _ub(zt[o:o + h // 2, :]), _ub(zt[o + h // 2:o + h, :]),
                        [_ub(zu[k, 0:h // 2, :]) for k in range(5)], w1p, s1, "1")
        for c, (top, bot) in enumerate(res):
            h1s[c][rows(r + 8, h), :] = _gelu(top)
            h1s[c][rows(r + 8 + h, h), :] = _gelu(bot)

    def mm_w2(r):
        lane = jax.lax.broadcasted_iota(i32, (T, 128), 1)

        def sh(k, c):
            return h1s[c][rows(r + 8 + k, T), :]

        g = _cat([sh(-1, 0),
                  jnp.where(lane < 32, sh(-1, 1), sh(1, 1)),
                  jnp.where(lane < 64, sh(1, 2), sh(-2, 2)),
                  jnp.where(lane < 96, sh(-2, 3), sh(2, 3)),
                  sh(2, 4)])
        top, bot = g[0:H], g[H:T]
        sums = _lhs_sums(top[:, 0:256], top[:, 256:512], bot[:, 0:256], bot[:, 256:512])
        for c, (ct, cb) in enumerate(mm_square(g, top, bot, sums, w2p, s2, "2")):
            hss[rows(r, H), _lanes(c)] = ct
            hss[rows(r + H, H), _lanes(c)] = cb

    def prep_w3():
        for j in range(NP3):
            r0 = 128 * (2 * j + 1)
            w3p[r0 // 2:r0 // 2 + 64, 0:256] = pltpu.bitcast(w3b[r0:r0 + 128, 0:256], u32)
            w3p[r0 // 2:r0 // 2 + 64, 512:D] = pltpu.bitcast(w3b[r0:r0 + 128, 512:D], u32)
            w3p[r0 // 2 + 64:r0 // 2 + 128, 256:D] = pltpu.bitcast(w3b[r0 + 128:r0 + 256, 256:D], u32)
        w3p[FM // 2:F // 2, :] = pltpu.bitcast(w3b[FM:F, :], u32)
        w3n[...] = _pk(w3b[0:128, :].astype(f32).T)
        for j in range(NP3):
            r0 = 128 * (2 * j + 1)
            for k in (2, 1, 0, 4, 3):
                s3[64 * j:64 * (j + 1), 256 * k:256 * (k + 1)] = _pk(_rhs_sum(k, lambda b: w3b[
                    r0 + 128 * (b % 2):r0 + 128 * (b % 2 + 1), 256 * (b // 2):256 * (b // 2 + 1)].astype(f32)))

    def w3_first():
        return _gelu2(_nn(_ub(zb[...]), _ub(w3n[...])))

    def w3_tail():
        return _gelu2(_nt(_ub(w3p[FM // 2:F // 2, :]), _ub(zb[...])))

    def w3_pair(j):
        e, o = slice(64 * (2 * j + 1), 64 * (2 * j + 2)), slice(64 * (2 * j + 2), 64 * (2 * j + 3))
        z1, z2 = _ub(zb[0:H // 2, :]), _ub(zb[H // 2:H, :])
        q = _strassen(_nt, z1[:, 0:256], z2[:, 256:512], [_ub(zs[k]) for k in range(5)], z1[:, 512:D], z2[:, 512:D],
                      _ub(w3p[e, 0:256]), _ub(w3p[o, 256:512]),
                      [_ub(s3[64 * j:64 * (j + 1), 256 * k:256 * (k + 1)]) for k in range(5)],
                      _ub(w3p[e, 512:D]), _ub(w3p[o, 512:D]), ORD[ctx[0] + "_3"])
        return [_gelu2(c) for c in q]

    def put_quads(j, q):
        l1, l2, l5, l6, l7 = _lhs_sums(*q)
        al[64 * j:64 * (j + 1), :] = _pk(_cat([l1, l2, q[0], q[3], l5, l6, l7, q[1], q[2]]))

    def put_edge(first, tail):
        tp = _cat([tail.T, jnp.zeros((T, 64), f32)])
        put_quads(NP3, [first[0:H], tp[0:H], first[H:T], tp[H:T]])

    def w3_pairs(ahead):
        for i in range(NP3 // 2):
            ops = []
            for j in (2 * i, 2 * i + 1):
                q = w3_pair(j)
                if not ahead:
                    put_quads(j, q)
                ops.append(q)
            if not ahead:
                continue
            for n, q in enumerate(ops):
                l1, l2, l5, l6, l7 = _lhs_sums(*q)
                ops[n] = [l1, l2, q[0], q[3], l5, l6, l7]
                j, half = 2 * i + n, slice(64 * n, 64 * (n + 1))
                o = 64 * j + 32 * n
                al[o:o + 32, 0:256] = _pk(_cat([l1[half], l2[half]]))
                al[o:o + 32, 512:896] = _pk(_cat([l5[half], l6[half], l7[half]]))
                al[64 * j:64 * (j + 1), 256:512] = _pk(_cat([q[0], q[3]]))
                al[64 * j:64 * (j + 1), 896:1152] = _pk(_cat([q[1], q[2]]))
            for m in range(7):
                e, o = ops[0][m], ops[1][m]
                r0 = 32 * (3 * m + i)
                a2[r0:r0 + 32, :] = _pk(_cat(_lhs_sums(e[0:64], o[0:64], e[64:128], o[64:128])))

    def s4_block(m, b, axis):
        o = 448 * (m - 1) + 64 * (b // 2)
        return _cat([s4[o + 128 * i:o + 128 * i + 64, _lanes(b % 2)] for i in range(3)], axis)

    def prep_w4():
        def krow(j, par):
            return 128 * (2 * j + 1 + par) if j < NP3 else FM * par

        for j in range(7):
            p4[0, 64 * j:64 * (j + 1), :] = pltpu.bitcast(w4b[krow(j, 0):krow(j, 0) + 128, 0:128], u32)
            if j < NP3:
                p4[1, 64 * j:64 * (j + 1), :] = pltpu.bitcast(w4b[krow(j, 1):krow(j, 1) + 128, 0:128], u32)
            else:
                p4[1, 64 * j:64 * j + 32, :] = pltpu.bitcast(w4b[FM:F, 0:128], u32)
                p4[1, 64 * j + 32:64 * (j + 1), :] = jnp.zeros((32, 128), u32)

        def block(j, b):
            if j == NP3 and b >= 2:
                return _cat([both(w4b, FM, F, b % 2), jnp.zeros((64, 256), f32)], 0)
            return both(w4b, krow(j, b // 2), krow(j, b // 2) + 128, b % 2)

        for m in [int(t) for t in OUTER['r4']]:
            k = {1: 0, 4: 2, 2: None, 3: 1, 5: None, 7: 4, 6: 3}[m]
            for j in range(7):
                o = 448 * (m - 1) + 64 * j
                if k is None and (j < NP3 or m == 2):
                    par = 0 if m == 2 else 1
                    for n in range(2):
                        s4[o:o + 64, _lanes(n)] = pltpu.bitcast(
                            w4b[krow(j, par):krow(j, par) + 128, _lanes(2 * n + 1 + par)], u32)
                else:
                    s4[o:o + 64, :] = _pk(block(j, 3) if k is None else _rhs_sum(k, lambda b: block(j, b)))
            for k2 in (2, 1, 0, 4, 3):
                o = 64 * (5 * (m - 1) + k2)
                s5[o:o + 64, :] = _pk(_rhs_sum(k2, lambda b: _ub(s4_block(m, b, -1)).astype(f32)))

    def finish(r, n, h, c):
        c0, c1 = 128 * c, 128 * (c + 1)
        x1 = h2s[rows(r, n), c0:c1] + hss[rows(r, n), c0:c1]
        base = x2s[rows(r, n), c0:c1] + mvec(4, n, c0, c1) * x1
        ob[rows(r, n), c0:c1] = (base + mvec(5, n, c0, c1) * h).astype(bf16)
        if ctx[0] == "z":
            send(r, n, c)

    def w4_plain(r, o=0, n=T):
        def left(k):
            return _cat([al[64 * j:64 * (j + 1), _lanes(k)] for j in range(7)])

        a = _cat([_cat([left(2), left(7)]), _cat([left(8), left(3)])], 0)[o // 2:(o + n) // 2]
        finish(r + o, n, _nn(_ub(a), _ub(_cat([p4[0], p4[1]], 0))), 0)

    def w4_product(m, ahead, order=None):
        def blk(b):
            o = 64 * (b % 2) + 32 * (b // 2)
            return _ub(_cat([al[o + 128 * i:o + 128 * i + 32, _lanes(m - 1)] for i in range(3)]))

        if ahead:
            asum = [_ub(_cat([a2[32 * (3 * (m - 1) + i):32 * (3 * (m - 1) + i + 1), _lanes(k)] for i in range(3)]))
                    for k in range(5)]
        else:
            asum = _lhs_sums(*[blk(b).astype(f32) for b in range(4)])
        bsum = [_ub(_cat([s5[64 * (5 * (m - 1) + k):64 * (5 * (m - 1) + k + 1), _lanes(i)] for i in range(3)], 0))
                for k in range(5)]
        ox = 448 * (m - 1) + 384
        q = _strassen(_nn, blk(0), blk(3), asum, _ub(al[384:416, _lanes(m - 1)]), _ub(al[416:448, _lanes(m - 1)]),
                      _ub(s4_block(m, 0, 0)), _ub(s4_block(m, 3, 0)), bsum,
                      _ub(s4[ox:ox + 64, _lanes(0)]), _ub(s4[ox:ox + 64, _lanes(1)]), ORD[ctx[0] + "_4"])
        return _cat([_cat(q[0:2]), _cat(q[2:4])], 0)

    def w4_steps(r, ahead):
        acc = [c2.at[H * i:H * (i + 1), :] for i in range(4)]

        def finish2(rr, h, c):
            finish(rr, H, h[:, 0:128], c)
            finish(rr, H, h[:, 128:256], c + 2)

        sign = {1: (1, 0, 0, 1), 2: (0, 0, 1, -1), 3: (0, 1, 0, 1), 4: (1, 0, 1, 0), 5: (-1, 1, 0, 0),
                6: (0, 0, 0, 1), 7: (1, 0, 0, 0)}
        left_n, state = [4, 2, 2, 4], [None] * 4
        for m in [int(t) for t in OUTER[ctx[0]]]:
            x = w4_product(m, ahead)
            outs = [i for i in range(4) if sign[m][i]]
            olds = {i: None if state[i] is None else state[i][0][...] for i in outs}
            busy = [state[i][0] for i in range(4) if state[i] is not None and i not in outs]
            free = [a for a in acc if not any(a is b for b in busy)]
            shared = None
            for i in outs:
                sg = sign[m][i]
                left_n[i] -= 1
                if state[i] is None:
                    if shared is None:
                        shared = free.pop()
                        shared[...] = x
                    state[i] = (shared, sg)
                    continue
                v = olds[i] + x if (sg > 0) == (state[i][1] > 0) else (x - olds[i] if sg > 0 else olds[i] - x)
                if left_n[i] == 0:
                    finish2(r + H * (i // 2), v, 1 + i % 2)
                    state[i] = None
                else:
                    dst = free.pop()
                    dst[...] = v
                    state[i] = (dst, 1)
            yield

    def up(order, ahead, r1=None, n1=None):
        for tok in order:
            if tok == "n":
                first = w3_first()
            elif tok == "t":
                tail = w3_tail()
            elif tok == "e":
                put_edge(first, tail)
            elif tok == "3":
                w3_pairs(ahead)
            elif tok == "1":
                mm_w1(r1, n1)
            elif tok == "c":
                ln_chain(r1, n1, paired=PAIRED)

    groups = list(range(0, P0 + P1, RG))
    wait([q_copies[0]])
    sa, ca, ga = mod_part(0, 1)
    modb[0] = ga * sa
    modb[1] = ga * (1.0 + ca)
    for c in range(NL, CT):
        mac_inv(c, NB - 1)
    st1 = {o: _stats(load_q(o)) for o in groups}
    zt[0:8, 0:128] = jnp.zeros((8, 128), u32)
    st2 = {}
    for o in groups:
        x2 = make_x2(o, load_q(o), st1[o])
        x2s[o:o + RG, :] = x2
        st2[o] = _stats(x2)

    wait([mod_copies[1]])
    sb, cb = mod_part(1, 2)
    modb[2] = sb
    modb[3] = 1.0 + cb
    st3 = {}
    for o in range(0, P0, RG):
        h2 = make_h2(x2s[o:o + RG, :], st2[o])
        h2s[o:o + RG, :] = h2
        st3[o] = _stats(h2)
    for o in range(0, P0, RG):
        zt[o // 2:(o + RG) // 2, :] = _pk((h2s[o:o + RG, :] - st3[o][0]) * st3[o][1])

    wait([w_copies[0]])
    prep_square(w1b, w1p, s1)
    z0 = _ub(zt[0:P0 // 2, :])
    h1 = _gelu(_nn(z0, _ub(w1p[:, 0:512])))
    for c in range(CT - 1):
        h1s[c][8:8 + P0, :] = h1[:, _lanes(c)]
    for o in range(0, P0, P0 // 4):
        h1s[CT - 1][8 + o:8 + o + P0 // 4, :] = _gelu(_nn(z0[o:o + P0 // 4], _ub(w1p[:, 512:D])))
    prev = None
    for o1 in range(0, P1 // 2, RG):
        zz = []
        for o in (P0 + o1, P0 + o1 + P1 // 2):
            h2 = make_h2(x2s[o:o + RG, :], st2[o])
            h2s[o:o + RG, :] = h2
            st = _stats(h2, prev, early=True)
            z = (h2 - st[0]) * st[1]
            zt[o // 2:(o + RG) // 2, :] = _pk(z)
            prev = st[1]
            zz.append(z)
        put_sums(zu, o1, zz[0], zz[1])
    mm_w1(P0, P1, P0)

    ctx[0] = "r2"
    wait([w_copies[1], q_copies[1]])
    prep_square(w2b, w2p, s2)
    ln_chain(P0 + P1, PA, paired=R2M)
    mm_w2(0)
    ln_x1(0, R2L)
    mm_w2(T)

    ctx[0] = "r3"
    wait([w_copies[2]])
    prep_w3()
    early = ln_x1(T, stats_only=True) if SE else None
    up(R3O, True, P0 + P1, PA)

    ctx[0] = "r4"
    if FEN4:
        jax.lax.fori_loop(0, 2, fence, 0)
    wait([w_copies[3], mod_copies[2]])
    prep_w4()
    sc16 = jnp.broadcast_to(scb[:, 0:D], (16, D)).astype(bf16)
    steps, h, j = w4_steps(0, True), None, 0
    for tok in R4O:
        if tok == "p":
            blk = [al[64 * j:64 * (j + 1), _lanes(k)] for k in (2, 7, 8, 3)]
            w = _ub(_cat([p4[0, 64 * j:64 * (j + 1), :], p4[1, 64 * j:64 * (j + 1), :]], 0))
            d = [_nn(_ub(_cat(blk[0:2])), w), _nn(_ub(_cat(blk[2:4])), w)]
            h = d if h is None else [h[0] + d[0], h[1] + d[1]]
            j += 1
            if j == 7:
                finish(0, H, h[0], 0)
                finish(H, H, h[1], 0)
        elif tok == "s":
            next(steps)
        else:
            c0, c1 = (0, 384) if tok == "g" else (384, D)
            gb = jnp.dot(sc16, wmc[:, c0:c1], preferred_element_type=f32)[0:8]
            modb[4, :, c0:c1] = gb
            modb[5, :, c0:c1] = 0.5 * gb
    ln_x1(T, stats=early)
    out_copy(0).start()
    q_copies[2].wait()

    def mlp_body(i, carry):
        r1 = pl.multiple_of(PB - PC + PC * i, 32)
        r = pl.multiple_of(i * T, T)
        up(HEAD, False, r1, PC)
        steps = w4_steps(r, False)
        for tok in BODY:
            if tok == "1":
                mm_w1(r1, PC)
            elif tok == "p":
                w4_plain(r)
            elif tok == "2":
                mm_w2(r + T)
            elif tok == "l":
                ln_x1(r + T, LM)
            else:
                next(steps)
        out_copy(i).start()
        return carry

    ctx[0] = "l"
    jax.lax.fori_loop(1, NC - 1, mlp_body, 0)

    ctx[0] = "z"
    up(ZO, True)
    w4_plain(S - T, 0, LA)
    for _ in w4_steps(S - T, True):
        pass
    if LAST0 > LA:
        w4_plain(S - T, LA, LAST0 - LA)
    w4_plain(S - T, LAST0, T - LAST0)
    for i in range(NC - 1):
        out_copy(i).wait()
    for cp in out_tail:
        cp.wait()


@jax.jit
def pallas_adaLN_cond__ssm_conv_h3__mixer_s_mlp__prompt_kernel(
    A_q: jax.Array,
    A_k: jax.Array,
    A_v: jax.Array,
    A_shift_k: jax.Array,
    A_ssm_k: jax.Array,
    A_ssm_D: jax.Array,
    B_x: jax.Array,
    B_w1: jax.Array,
    B_w2: jax.Array,
    B_w3: jax.Array,
    B_w4: jax.Array,
    c: jax.Array,
    w_mod: jax.Array,
):
    del B_x
    any_spec = pl.BlockSpec(memory_space=pl.ANY)

    def tile_view(x):
        return x.reshape(S // 8, 8, CT, 128).transpose(0, 2, 1, 3).reshape(S * CT, 128)

    vm = pltpu.VMEM
    dma = pltpu.SemaphoreType.DMA
    spec = (4, NG, 16, 128)
    out = pl.pallas_call(
        _kernel,
        in_specs=[any_spec] * 12,
        out_specs=any_spec,
        out_shape=jax.ShapeDtypeStruct((S, D), bf16),
        scratch_shapes=[
            *[vm((KROWS, 128), bf16)] * NB, *[vm((VROWS, 128), bf16)] * NB, vm((CT, 128, S), bf16),
            vm((S, D), bf16), vm((D, D), bf16), vm((D, D), bf16), vm((F, D), bf16), vm((F, D), bf16),
            vm((D // 2, D), u32), vm((D // 2, D), u32), vm((F // 2, D), u32),
            vm((D, 3 * D), bf16), vm((D, 2 * D), bf16), vm((D, D), bf16),
            vm((4, D), bf16), vm((D,), bf16), vm((1, D), bf16), vm((1, 1792), f32),
            vm((4, 128, 128), u32), vm((4, 128, 128), u32), vm((4, 64, 256), u32),
            vm((CT, 8, 8, 128), f32),
            vm((CT, NB) + spec, f32), vm((CT, NB - 1) + spec, f32), vm((CT,) + spec, f32),
            vm((CT, NB) + spec, f32), vm((4, 128, 128), f32),
            vm((CT, S + 32, 128), f32), vm((8, 8, D), f32),
            *[vm((S + 32, 128), f32)] * CT, vm((S, D), f32), vm((S, D), f32), vm((S, D), f32),
            vm((288, D), u32), vm((5, H // 2, 256), u32), vm((H, D), u32), vm((5, H // 2, 256), u32),
            vm((D // 2, 128), u32), vm((D, 256), u32), vm((D, 256), u32), vm((NP3 * 64, 1280), u32),
            vm((7 * 448, 256), u32), vm((35 * 64, 384), u32), vm((2, 448, 128), u32),
            vm((7 * 64, 1152), u32), vm((21 * 32, 640), u32), vm((4 * H, 256), f32),
            vm((S, D), bf16),
            dma((26,)), dma((NC + 10,)),
        ],
        compiler_params=pltpu.CompilerParams(vmem_limit_bytes=110 << 20, disable_bounds_checks=True,
                                             disable_semaphore_checks=True),
    )(A_q.reshape(S, D), tile_view(A_k), tile_view(A_v), A_shift_k.T, A_ssm_k,
      A_ssm_D, B_w1, B_w2, B_w3.T, B_w4, c, w_mod)
    return out.reshape(1, S, D)
```

```python
import numpy as np
import jax
import jax.numpy as jnp
import jax.experimental.pallas as pl
import jax.experimental.pallas.tpu as pltpu

f32, bf16, u32, i32 = jnp.float32, jnp.bfloat16, jnp.uint32, jnp.int32

S, D, F = 2048, 640, 1728
CT = D // 128
TR = 8 * CT
NB, BLK, NFFT = 4, 512, 1024
KROWS, VROWS = BLK * CT + 128, BLK * CT + 64
NG = 16
T = 256
NC = S // T
H = T // 2
NP3 = 6
FM = (F // 128) * 128
P0, P1, PA, PC = 320, 224, 160, 224
PB = P0 + P1 + PA
LA, LAST0 = 96, 208
RG = 16
EPS = 1e-5
NT_DIMS = (((1,), (1,)), ((), ()))
PAIRED = "10000100001000"
ORD = {"r1_1": "42351c7a6db", "r2_2": "42c3d6a71b5", "r3_1": "2754b6c3d1a", "r3_3": "4c2a5173b6d",
       "r4_4": "5b12a47cd63", "l_1": "7325bad4c61", "l_2": "24351ac7b6d", "l_3": "4bc3521a76d",
       "l_4": "243ac51b76d", "z_3": "c2b73145ad6", "z_4": "354d12b7ca6"}
OUTER = {"r4": "7123465", "l": "2135647", "z": "1537642"}
BODY = "1pp2slsppsspsppss"
HEAD = "cnte3"
LM = "0000000000000100"
R2M = "1000001010"
R2L = "1010100100101010"
R3O = "1tn3e"
R4O = "gsssGpspspppspps"
SE = 1
ZO = "nte3"
FEN4 = 1
FA = 3
TORD = "2435176"
TP0 = 1
TX = 1
TZ = 0
ZB = "ppsspspspspsps"
GV = 8
NL = 4


def _lo(w):
    return pltpu.bitcast(w << 16, f32)


def _hi(w):
    return pltpu.bitcast(w & jnp.uint32(0xFFFF0000), f32)


def _cis(n):
    t = (n & (2 * NFFT - 1)).astype(f32) * (np.pi / NFFT)
    return jnp.cos(t), jnp.sin(t)


def _fwd_table(r):
    g = jax.lax.broadcasted_iota(i32, (NG, 128), 0)
    cg, sg = _cis(jnp.where(g < NG // 2, 32 * g + 1, 32 * g - 253) * r)
    cs, ss = _cis(4 * jax.lax.broadcasted_iota(i32, (8, 128), 0) * r)
    parts = []
    for i in range(NG):
        c, s = cg[i:i + 1], sg[i:i + 1]
        parts += [c * cs - s * ss, -(s * cs + c * ss)]
    return pltpu.bitcast(jnp.concatenate(parts, axis=0).astype(bf16), u32)


def _inv_tables():
    def phase(rows):
        col = jax.lax.broadcasted_iota(i32, (rows, 256), 1)
        k = ((col >> 4) << 3) + (col & 7)
        row = jax.lax.broadcasted_iota(i32, (rows, 256), 0)
        return jnp.where(k < 64, 4 * k + 1, 4 * k - 253), (col & 8) << 6, row

    fr, _, g = phase(16)
    cg, sg = _cis(fr * (32 * g))
    fr, off, s = phase(8)
    out = []
    for p in range(4):
        cs, ss = _cis(fr * (4 * s + p) + off)
        cs, ss = cs * (2.0 / NFFT), ss * (2.0 / NFFT)
        parts = [cg[i:i + 1] * cs - sg[i:i + 1] * ss for i in range(16)]
        out.append(pltpu.bitcast(jnp.concatenate(parts, axis=0).astype(bf16), u32))
    return out


def _radix4(re, im, inverse):
    ar, ai = re[0] + re[2], im[0] + im[2]
    br, bi = re[0] - re[2], im[0] - im[2]
    cr, ci = re[1] + re[3], im[1] + im[3]
    dr, di = re[1] - re[3], im[1] - im[3]
    minus_i = (br + di, bi - dr)
    plus_i = (br - di, bi + dr)
    if inverse:
        return [(ar + cr, ai + ci), plus_i, (ar - cr, ai - ci), minus_i]
    return [(ar + cr, ai + ci), minus_i, (ar - cr, ai - ci), plus_i]


def _stats(x, link=None, early=False):
    zero = 0.0 if link is None else jnp.minimum(link, 0.0)
    part = x[:, 0:128]
    for c in range(1, CT):
        part = part + x[:, c * 128:(c + 1) * 128]
    if link is not None and early:
        part = part + zero
        zero = 0.0
    m = jnp.sum(part, axis=-1, keepdims=True) * (1.0 / D)
    v = jnp.maximum(jnp.sum(x * x, axis=-1, keepdims=True) * (1.0 / D) - m * m, zero)
    return m, jnp.exp2(jnp.log(v + EPS) * (-0.5 / np.log(2.0)))


def _gelu2(x):
    c = 0.7978845608028654
    u = c + (c * 0.044715) * (x * x)
    return x + x * jnp.tanh(x * u)


def _gelu(x):
    c = 0.7978845608028654
    u = c + (c * 0.044715) * (x * x)
    hx = 0.5 * x
    return hx + hx * jnp.tanh(x * u)


def _pk(x):
    return pltpu.bitcast(x.astype(bf16), u32)


def _ub(x):
    return pltpu.bitcast(x, bf16)


def _cat(xs, axis=-1):
    return jnp.concatenate(xs, axis=axis)


def _lanes(k):
    return slice(128 * k, 128 * (k + 1))


def _nn(a, w):
    return jnp.dot(a.astype(bf16), w, preferred_element_type=f32)


def _nt(a, w):
    return jax.lax.dot_general(a, w, NT_DIMS, preferred_element_type=f32)


def _lhs_sums(a11, a12, a21, a22):
    return [a11 + a22, a21 + a22, a11 + a12, a21 - a11, a12 - a22]


def _rhs_sum(k, block):
    a, b, plus = [(0, 3, True), (1, 3, False), (2, 0, False), (0, 1, True), (2, 3, True)][k]
    return block(a) + block(b) if plus else block(a) - block(b)


def _strassen(dot, a11, a22, asum, ax1, ax2, b11, b22, bsum, bx1, bx2, order=""):
    if order:
        ops = {"1": (asum[0], bsum[0], (1, 0, 0, 1)), "2": (asum[1], b11, (0, 0, 1, -1)),
               "3": (a11, bsum[1], (0, 1, 0, 1)), "4": (a22, bsum[2], (1, 0, 1, 0)),
               "5": (asum[2], b22, (-1, 1, 0, 0)), "6": (asum[3], bsum[3], (0, 0, 0, 1)),
               "7": (asum[4], bsum[4], (1, 0, 0, 0)), "a": (ax1, bx1, (1, 0, 0, 0)),
               "b": (ax1, bx2, (0, 1, 0, 0)), "c": (ax2, bx1, (0, 0, 1, 0)), "d": (ax2, bx2, (0, 0, 0, 1))}
        c, neg = [None] * 4, [None] * 4
        for t in order:
            a, b, sg = ops[t]
            m = dot(a, b)
            for i in range(4):
                if sg[i] > 0:
                    c[i] = m if c[i] is None else c[i] + m
                    if neg[i] is not None:
                        c[i], neg[i] = c[i] - neg[i], None
                elif sg[i] < 0:
                    if c[i] is None:
                        neg[i] = m
                    else:
                        c[i] = c[i] - m
        return c
    m2 = dot(asum[1], b11)
    m4 = dot(a22, bsum[2])
    c21 = (m4 + m2) + dot(ax2, bx1)
    m3 = dot(a11, bsum[1])
    m5 = dot(asum[2], b22)
    c12 = (m3 + m5) + dot(ax1, bx2)
    m1 = dot(asum[0], bsum[0])
    c11 = (((m4 - m5) + m1) + dot(asum[4], bsum[4])) + dot(ax1, bx1)
    c22 = (((m3 - m2) + m1) + dot(asum[3], bsum[3])) + dot(ax2, bx2)
    return [c11, c12, c21, c22]


def _kernel(q_hbm, k_hbm, v_hbm, sh_hbm, sk_hbm, d_hbm, w1_hbm, w2_hbm, w3_hbm, w4_hbm,
            c_hbm, wm_hbm, o_hbm,
            kb0, kb1, kb2, kb3, vb0, vb1, vb2, vb3, skb, qb, w1b, w2b, w3b, w4b, w1p, w2p, w3p,
            wma, wmb, wmc, shb, db, cb_, scb,
            fub, fkb, gtb, par, US, KS, UR, YS, YP, ys, modb, h10, h11, h12, h13, h14, h2s, x2s, hss,
            zt, zu, zb, zs, w3n, s1, s2, s3, s4, s5, p4, al, a2, c2, t4, ob,
            sem, sem_o):
    h1s = [h10, h11, h12, h13, h14]
    n_in = [0]

    def load(src, dst):
        n_in[0] += 1
        return pltpu.make_async_copy(src, dst, sem.at[n_in[0] - 1])

    nkv = BLK * CT
    small = [load(d_hbm, db), load(sh_hbm, shb), load(c_hbm, cb_)]
    sk_copies = [load(sk_hbm.at[pl.ds(c * 128, 128), :], skb.at[c]) for c in range(CT)]
    kbs, vbs, wms = [kb0, kb1, kb2, kb3], [vb0, vb1, vb2, vb3], [wma, wmb, wmc]
    kv_copies = [[load(k_hbm.at[pl.ds(a * nkv, nkv), :], kbs[a].at[pl.ds(TR, nkv), :]),
                  load(v_hbm.at[pl.ds(a * nkv, nkv), :], vbs[a].at[pl.ds(0, nkv), :])] for a in range(NB)]
    mod_cols = [(0, 3 * D), (3 * D, 2 * D), (5 * D, D)]
    mod_copies = [load(wm_hbm.at[:, pl.ds(o, n)], w) for (o, n), w in zip(mod_cols, wms)]
    w_copies = [load(w1_hbm, w1b), load(w2_hbm, w2b), load(w3_hbm, w3b), load(w4_hbm, w4b)]
    q_copies = [load(q_hbm.at[pl.ds(o, n), :], qb.at[pl.ds(o, n), :])
                for o, n in [(0, P0 + P1), (P0 + P1, PA), (PB, S - PB)]]

    def out_copy(i):
        r = i * T if isinstance(i, int) else pl.multiple_of(i * T, T)
        return pltpu.make_async_copy(ob.at[pl.ds(r, T), :], o_hbm.at[pl.ds(r, T), :], sem_o.at[i])

    out_tail = []

    def send(r, n, c):
        cp = pltpu.make_async_copy(ob.at[pl.ds(r, n), pl.ds(128 * c, 128)], o_hbm.at[pl.ds(r, n), pl.ds(128 * c, 128)],
                                   sem_o.at[NC - 1 + len(out_tail)])
        out_tail.append(cp)
        cp.start()

    for cp in (small + kv_copies[0] + sk_copies + kv_copies[1] + kv_copies[2] + kv_copies[3]
               + [mod_copies[0], q_copies[0], mod_copies[1], w_copies[0], w_copies[1], q_copies[1],
                  w_copies[2], w_copies[3], mod_copies[2], q_copies[2]]):
        cp.start()

    def wait(copies):
        for cp in copies:
            cp.wait()

    def pin(i, carry):
        z = jnp.zeros((8, 128), f32)
        scb[:, pl.ds(pl.multiple_of(i * 128, 128), 128)] = z[0:1]
        YP[i, 0:8, :] = z
        US[i, 0, 0, 0, 0:8, :] = z
        KS[i, 0, 0, 0, 0:8, :] = z
        YS[i, 0, 0, 0, 0:8, :] = z
        UR[i, 0, 0, 0:8, :] = z
        r8 = pl.ds(pl.multiple_of(i * 8, 8), 8)
        c2[r8, 0:128] = z
        al[r8, 0:128] = jnp.zeros((8, 128), u32)
        a2[r8, 0:128] = jnp.zeros((8, 128), u32)
        return carry

    def fence(i, carry):
        YP[i, 0:8, :] = jnp.zeros((8, 128), f32)
        return carry

    jax.lax.fori_loop(0, 2, pin, 0)
    lane = jax.lax.broadcasted_iota(i32, (1, 128), 1)
    for p in range(4):
        m = (lane - p) & 3
        fkb[p] = _fwd_table(128 * m + ((lane - m) & 127))
    for c in range(CT):
        kb0[c * 8:(c + 1) * 8, :] = jnp.zeros((8, 128), bf16)
        h1s[c][0:8, :] = jnp.zeros((8, 128), f32)
        h1s[c][S + 8:S + 16, :] = jnp.zeros((8, 128), f32)
    for a in range(NB):
        kbs[a][nkv + TR:KROWS, :] = jnp.zeros((KROWS - nkv - TR, 128), bf16)
        vbs[a][nkv:VROWS, :] = jnp.zeros((VROWS - nkv, 128), bf16)
    for p in range(4):
        fub[p] = _fwd_table(8 * (lane & 63) + ((lane >> 6) << 2) + p)
    wait(small)
    cvec = cb_[...].astype(f32)
    scb[:, 0:D] = cvec * jax.nn.sigmoid(cvec)
    dv = db[...].astype(f32).reshape(1, D)
    shv = shb[...].astype(f32)
    for c in range(CT):
        for i in range(4):
            par[c, i] = jnp.broadcast_to(shv[i:i + 1, c * 128:(c + 1) * 128], (8, 128))
        par[c, 4] = jnp.broadcast_to(dv[:, c * 128:(c + 1) * 128], (8, 128))
    for p, tab in enumerate(_inv_tables()):
        gtb[p] = tab

    def get(ref, idx, g, n):
        return (ref[idx + (slice(g, g + n), slice(0, 8))], ref[idx + (slice(g, g + n), slice(8, 16))])

    def put(ref, idx, g, n, xr, xi):
        ref[idx + (slice(g, g + n), slice(0, 8))] = xr
        ref[idx + (slice(g, g + n), slice(8, 16))] = xi

    def split(tt, g, n):
        tt = [t[g * 16:(g + n) * 16].reshape(n, 16, 128) for t in tt]
        return [t[:, 0:8] for t in tt], [t[:, 8:16] for t in tt]

    def fwd_k(c, j):
        lane = jax.lax.broadcasted_iota(i32, (64, 128), 1)
        even = (lane & 1) == 0
        l01 = (lane & 2) == 0
        l12 = ((lane + 3) & 2) == 0
        rm = []
        for m in range(4):
            w = pltpu.bitcast(skb[c, :, (4 * j + m) * 128:(4 * j + m + 1) * 128], u32)
            rm.append(pltpu.roll(w, m, 1) if m else w)
        e01 = jnp.where(even, rm[0], rm[1])
        o01 = jnp.where(even, rm[1], rm[0])
        e23 = jnp.where(even, rm[2], rm[3])
        o23 = jnp.where(even, rm[3], rm[2])
        kp = [jnp.where(l01, e01, e23), jnp.where(l12, o01, o23),
              jnp.where(l01, e23, e01), jnp.where(l12, o23, o01)]
        tt = [jax.lax.dot_general(pltpu.bitcast(fkb[p], bf16), pltpu.bitcast(kp[p], bf16), NT_DIMS,
                                  preferred_element_type=f32) for p in range(4)]
        for g in range(0, NG, GV):
            re, im = split(tt, g, GV)
            if j == 0:
                re[0] = re[0] + par[c, 4][None]
            for m, (xr, xi) in enumerate(_radix4(re, im, False)):
                if j < NB - 1:
                    put(KS, (c, j, m), g, GV, xr, xi)
                ur, ui = get(US, (c, 0, m), g, GV)
                put(YS, (c, j, m), g, GV, xr * ur - xi * ui, xr * ui + xi * ur)

    def fwd_u(c, a):
        taps = [jnp.tile(par[c, i], (8, 1)) for i in range(4)]
        ws = TR // 2
        base = 4 * c
        kw, vw = kbs[a].bitcast(u32), vbs[a].bitcast(u32)

        def words(ref, start):
            return ref[pl.ds(start, BLK // 8, stride=ws), :]

        kk = {}
        for w in range(4):
            x = words(kw, ws + base + w)
            kk[2 * w], kk[2 * w + 1] = _lo(x), _hi(x)
        kk[-3] = _hi(words(kw, base + 2))
        x = words(kw, base + 3)
        kk[-2], kk[-1] = _lo(x), _hi(x)
        sub = []
        for w in range(4):
            x = words(vw, base + w)
            for r, vv in ((2 * w, _lo(x)), (2 * w + 1, _hi(x))):
                sh = taps[0] * kk[r] + taps[1] * kk[r - 1] + taps[2] * kk[r - 2] + taps[3] * kk[r - 3]
                sub.append(sh * vv)
        kv = [jnp.concatenate([sub[p], sub[p + 4]], axis=0) for p in range(4)]
        tt = [jnp.dot(pltpu.bitcast(fub[p], bf16), kv[p].astype(bf16), preferred_element_type=f32)
              for p in range(4)]
        for g in range(0, NG, GV):
            re, im = split(tt, g, GV)
            for m, (xr, xi) in enumerate(_radix4(re, im, False)):
                if a:
                    pr, pi = get(US, (c, 0, m), g, GV) if a == 1 else get(UR, (c, m), g, GV)
                    if a < NB - 1:
                        put(UR, (c, m), g, GV, xr, xi)
                    xr, xi = (xr - pi, xi + pr) if g < NG // 2 else (xr + pi, xi - pr)
                put(US, (c, a, m), g, GV, xr, xi)

    def mac_inv(c, a):
        for h in range(2):
            vals = [[] for _ in range(4)]
            for g in range(8 * h, 8 * h + 8, GV):
                yre, yim = [], []
                for m in range(4):
                    yr, yi = get(YS, (c, a, m), g, GV)
                    for j in range(a):
                        kr, ki = get(KS, (c, j, m), g, GV)
                        ur, ui = get(US, (c, a - j, m), g, GV)
                        yr = yr + (kr * ur - ki * ui)
                        yi = yi + (kr * ui + ki * ur)
                    yre.append(yr)
                    yim.append(yi)
                for p, (pr, pi) in enumerate(_radix4(yre, yim, True)):
                    vals[p].append(jnp.concatenate([pr, pi], axis=1))
            for p in range(4):
                pb = jnp.concatenate(vals[p], axis=0).reshape(128, 128).astype(bf16)
                r = jnp.dot(pltpu.bitcast(gtb[p, :, h * 128:(h + 1) * 128], bf16), pb,
                            preferred_element_type=f32)
                if h == 0:
                    YP[p] = r
                else:
                    ys[c, pl.ds(a * BLK + p, 128, stride=4), :] = YP[p] + r

    wait(kv_copies[0])
    for c in range(CT):
        fwd_u(c, 0)
    for grp in ((0,), (1, 2), (3, 4)):
        wait([sk_copies[c] for c in grp])
        for c in grp:
            for j in (3, 2, 1, 0):
                fwd_k(c, j)
    for a in range(1, NB):
        if a == FA:
            jax.lax.fori_loop(0, 2, fence, 0)
        wait(kv_copies[a])
        for c in range(CT):
            kbs[a][c * 8:(c + 1) * 8, :] = kbs[a - 1][nkv + c * 8:nkv + (c + 1) * 8, :]
        for c in range(CT):
            fwd_u(c, a)
            mac_inv(c, a - 1)
    wait([mod_copies[0]])
    for c in range(NL):
        mac_inv(c, NB - 1)

    def mod_part(part, extra):
        n, wm = mod_cols[part][1], wms[part]
        act = scb[:, 0:D]

        def sc(k0, k1):
            return jnp.broadcast_to(act[:, k0:k1], (16, k1 - k0)).astype(bf16)

        e = 128 * extra
        r = jnp.dot(sc(0, D), wm[:, e:n], preferred_element_type=f32)
        r0 = (jnp.dot(sc(0, D - 64), wm[0:D - 64, 0:e], preferred_element_type=f32)
              + jnp.dot(sc(D - 64, D), wm[D - 64:D, 0:e], preferred_element_type=f32))
        r = jnp.concatenate([r0, r], axis=-1)[0:8]
        return [r[:, i * D:(i + 1) * D] for i in range(n // D)]

    def mvec(i, n=RG, c0=0, c1=D):
        return jnp.tile(modb[i, :, c0:c1], (n // 8, 1))

    rows = pl.ds
    ctx = ["r1"]

    def load_q(r, ref=qb):
        return ref[rows(r, RG), :].astype(f32)

    def make_x2(r, q, st, ref=ys):
        y = _cat([ref[c, rows(r, RG), :] for c in range(CT)])
        return q + (((q - st[0]) * st[1]) * mvec(1) + mvec(0)) * y

    def make_h2(x2, st):
        return ((x2 - st[0]) * st[1]) * mvec(3) + mvec(2)

    def put_sums(ref, o, z1, z2):
        for k, v in enumerate(_lhs_sums(z1[:, 0:256], z1[:, 256:512], z2[:, 0:256], z2[:, 256:512])):
            ref.at[k][o // 2:(o + RG) // 2, :] = _pk(v)

    def ln_chain(r, n, links=1, paired=""):
        qv, yv = qb.at[rows(r, n), :], ys.at[:, rows(r, n), :]
        xv, hv = x2s.at[rows(r, n), :], h2s.at[rows(r, n), :]
        prev, pend, cnt = [None] * links, None, 0
        for o1 in range(0, n // 2, RG):
            zz = []
            for o in (o1, o1 + n // 2):
                q = load_q(o, qv)
                x2 = make_x2(o, q, _stats(q, prev[cnt % links]), yv)
                xv[o:o + RG, :] = x2
                st = _stats(x2)
                h2 = make_h2(xv[o:o + RG, :], st)
                hv[o:o + RG, :] = h2
                st = _stats(h2)
                z = (hv[o:o + RG, :] - st[0]) * st[1]
                zt[o // 2:(o + RG) // 2, :] = _pk(z)
                zz.append(z)
                if paired and paired[cnt] == "1":
                    pend = st[1]
                elif pend is not None:
                    prev[0], pend = jnp.minimum(st[1], pend), None
                else:
                    prev[cnt % links] = st[1]
                cnt += 1
            put_sums(zu, o1, zz[0], zz[1])

    def ln_x1(r, paired="", stats=None, stats_only=False):
        hv, sv = h2s.at[rows(r, T), :], hss.at[rows(r, T), :]
        prev, pend, cnt, out = None, None, 0, []
        for o1 in range(0, H, RG):
            zz = []
            for o in (o1, o1 + H):
                x1 = hv[o:o + RG, :] + sv[o:o + RG, :]
                st = _stats(x1, prev, early=True) if stats is None else stats[cnt]
                out.append(st)
                if not stats_only:
                    z = (x1 - st[0]) * st[1]
                    zb[o // 2:(o + RG) // 2, :] = _pk(z)
                    zz.append(z)
                if paired and paired[cnt] == "1":
                    pend = st[1]
                elif pend is not None:
                    prev, pend = jnp.minimum(st[1], pend), None
                else:
                    prev = st[1]
                cnt += 1
            if not stats_only:
                put_sums(zs, o1, zz[0], zz[1])
        return out

    def both(ref, r0, r1, col):
        return _cat([ref[r0:r1, _lanes(1 + col)].astype(f32), ref[r0:r1, _lanes(3 + col)].astype(f32)])

    def prep_square(wb, wp, sw):
        wp[...] = pltpu.bitcast(wb[...], u32)
        for k in (2, 1, 0, 4, 3):
            sw[128 * k:128 * (k + 1), :] = _pk(_rhs_sum(
                k, lambda b: both(wb, 256 * (b // 2), 256 * (b // 2 + 1), b % 2)))

    def mm_square(a, top, bot, asum, wp, sw, which):
        h = top.shape[0]
        c0 = _nn(a, _ub(wp[:, 0:128]))
        out = [(c0[0:h], c0[h:2 * h])]
        for n in range(2):
            l1, l2 = _lanes(2 * n + 1), _lanes(2 * n + 2)
            q = _strassen(_nn, top[:, 0:256], bot[:, 256:512], asum, top[:, 512:D], bot[:, 512:D],
                          _ub(wp[0:128, l1]), _ub(wp[128:256, l2]),
                          [_ub(sw[128 * k:128 * (k + 1), _lanes(n)]) for k in range(5)],
                          _ub(wp[256:320, l1]), _ub(wp[256:320, l2]), ORD[ctx[0] + "_" + which])
            out += [(q[0], q[2]), (q[1], q[3])]
        return out

    def mm_w1(r, n, o=0):
        h, o = n // 2, o // 2
        res = mm_square(_ub(zt[o:o + h, :]), _ub(zt[o:o + h // 2, :]), _ub(zt[o + h // 2:o + h, :]),
                        [_ub(zu[k, 0:h // 2, :]) for k in range(5)], w1p, s1, "1")
        for c, (top, bot) in enumerate(res):
            h1s[c][rows(r + 8, h), :] = _gelu(top)
            h1s[c][rows(r + 8 + h, h), :] = _gelu(bot)

    def mm_w2(r):
        lane = jax.lax.broadcasted_iota(i32, (T, 128), 1)

        def sh(k, c):
            return h1s[c][rows(r + 8 + k, T), :]

        g = _cat([sh(-1, 0),
                  jnp.where(lane < 32, sh(-1, 1), sh(1, 1)),
                  jnp.where(lane < 64, sh(1, 2), sh(-2, 2)),
                  jnp.where(lane < 96, sh(-2, 3), sh(2, 3)),
                  sh(2, 4)])
        top, bot = g[0:H], g[H:T]
        sums = _lhs_sums(top[:, 0:256], top[:, 256:512], bot[:, 0:256], bot[:, 256:512])
        for c, (ct, cb) in enumerate(mm_square(g, top, bot, sums, w2p, s2, "2")):
            hss[rows(r, H), _lanes(c)] = ct
            hss[rows(r + H, H), _lanes(c)] = cb

    def prep_w3():
        for j in range(NP3):
            r0 = 128 * (2 * j + 1)
            w3p[r0 // 2:r0 // 2 + 64, 0:256] = pltpu.bitcast(w3b[r0:r0 + 128, 0:256], u32)
            w3p[r0 // 2:r0 // 2 + 64, 512:D] = pltpu.bitcast(w3b[r0:r0 + 128, 512:D], u32)
            w3p[r0 // 2 + 64:r0 // 2 + 128, 256:D] = pltpu.bitcast(w3b[r0 + 128:r0 + 256, 256:D], u32)
        w3p[FM // 2:F // 2, :] = pltpu.bitcast(w3b[FM:F, :], u32)
        w3n[...] = _pk(w3b[0:128, :].astype(f32).T)
        for j in range(NP3):
            r0 = 128 * (2 * j + 1)
            for k in (2, 1, 0, 4, 3):
                s3[64 * j:64 * (j + 1), 256 * k:256 * (k + 1)] = _pk(_rhs_sum(k, lambda b: w3b[
                    r0 + 128 * (b % 2):r0 + 128 * (b % 2 + 1), 256 * (b // 2):256 * (b // 2 + 1)].astype(f32)))

    def w3_first():
        return _gelu2(_nn(_ub(zb[...]), _ub(w3n[...])))

    def w3_tail():
        return _gelu2(_nt(_ub(w3p[FM // 2:F // 2, :]), _ub(zb[...])))

    def w3_pair(j):
        e, o = slice(64 * (2 * j + 1), 64 * (2 * j + 2)), slice(64 * (2 * j + 2), 64 * (2 * j + 3))
        z1, z2 = _ub(zb[0:H // 2, :]), _ub(zb[H // 2:H, :])
        q = _strassen(_nt, z1[:, 0:256], z2[:, 256:512], [_ub(zs[k]) for k in range(5)], z1[:, 512:D], z2[:, 512:D],
                      _ub(w3p[e, 0:256]), _ub(w3p[o, 256:512]),
                      [_ub(s3[64 * j:64 * (j + 1), 256 * k:256 * (k + 1)]) for k in range(5)],
                      _ub(w3p[e, 512:D]), _ub(w3p[o, 512:D]), ORD[ctx[0] + "_3"])
        return [_gelu2(c) for c in q]

    def plain_ctx():
        return (ctx[0] in ("r3", "r4") and not TP0) or (ctx[0] == "z" and not TZ)

    def put_quads(j, q):
        l1, l2, l5, l6, l7 = _lhs_sums(*q)
        if not plain_ctx():
            al[64 * j:64 * (j + 1), 0:896] = _pk(_cat([l1, l2, q[0], q[3], l5, l6, l7]))
        else:
            al[64 * j:64 * (j + 1), :] = _pk(_cat([l1, l2, q[0], q[3], l5, l6, l7, q[1], q[2]]))

    def put_edge(first, tail):
        tp = _cat([tail.T, jnp.zeros((T, 64), f32)])
        put_quads(NP3, [first[0:H], tp[0:H], first[H:T], tp[H:T]])

    def w3_pairs(ahead):
        for i in range(NP3 // 2):
            ops = []
            for j in (2 * i, 2 * i + 1):
                q = w3_pair(j)
                if not ahead:
                    put_quads(j, q)
                ops.append(q)
            if not ahead:
                continue
            for n, q in enumerate(ops):
                l1, l2, l5, l6, l7 = _lhs_sums(*q)
                ops[n] = [l1, l2, q[0], q[3], l5, l6, l7]
                j, half = 2 * i + n, slice(64 * n, 64 * (n + 1))
                if not plain_ctx():
                    al[64 * j:64 * (j + 1), 0:896] = _pk(_cat(ops[n]))
                    continue
                o = 64 * j + 32 * n
                al[o:o + 32, 0:256] = _pk(_cat([l1[half], l2[half]]))
                al[o:o + 32, 512:896] = _pk(_cat([l5[half], l6[half], l7[half]]))
                al[64 * j:64 * (j + 1), 256:512] = _pk(_cat([q[0], q[3]]))
                al[64 * j:64 * (j + 1), 896:1152] = _pk(_cat([q[1], q[2]]))
            for m in range(7):
                e, o = ops[0][m], ops[1][m]
                r0 = 32 * (3 * m + i)
                a2[r0:r0 + 32, :] = _pk(_cat(_lhs_sums(e[0:64], o[0:64], e[64:128], o[64:128])))

    def s4_block(m, b, axis):
        o = 448 * (m - 1) + 64 * (b // 2)
        return _cat([s4[o + 128 * i:o + 128 * i + 64, _lanes(b % 2)] for i in range(3)], axis)

    def krow(j, par):
        return 128 * (2 * j + 1 + par) if j < NP3 else FM * par

    def prep_p4():
        for j in range(7):
            p4[0, 64 * j:64 * (j + 1), :] = pltpu.bitcast(w4b[krow(j, 0):krow(j, 0) + 128, 0:128], u32)
            if j < NP3:
                p4[1, 64 * j:64 * (j + 1), :] = pltpu.bitcast(w4b[krow(j, 1):krow(j, 1) + 128, 0:128], u32)
            else:
                p4[1, 64 * j:64 * j + 32, :] = pltpu.bitcast(w4b[FM:F, 0:128], u32)
                p4[1, 64 * j + 32:64 * (j + 1), :] = jnp.zeros((32, 128), u32)

    def prep_w4():
        def block(j, b):
            if j == NP3 and b >= 2:
                return _cat([both(w4b, FM, F, b % 2), jnp.zeros((64, 256), f32)], 0)
            return both(w4b, krow(j, b // 2), krow(j, b // 2) + 128, b % 2)

        for m in [int(t) for t in OUTER['r4']]:
            k = {1: 0, 4: 2, 2: None, 3: 1, 5: None, 7: 4, 6: 3}[m]
            for j in range(7):
                o = 448 * (m - 1) + 64 * j
                if k is None and (j < NP3 or m == 2):
                    par = 0 if m == 2 else 1
                    for n in range(2):
                        s4[o:o + 64, _lanes(n)] = pltpu.bitcast(
                            w4b[krow(j, par):krow(j, par) + 128, _lanes(2 * n + 1 + par)], u32)
                else:
                    s4[o:o + 64, :] = _pk(block(j, 3) if k is None else _rhs_sum(k, lambda b: block(j, b)))
            for k2 in (2, 1, 0, 4, 3):
                o = 64 * (5 * (m - 1) + k2)
                s5[o:o + 64, :] = _pk(_rhs_sum(k2, lambda b: _ub(s4_block(m, b, -1)).astype(f32)))

    def prep_t4():
        eye = (jax.lax.broadcasted_iota(i32, (128, 128), 0)
               == jax.lax.broadcasted_iota(i32, (128, 128), 1)).astype(f32).astype(bf16)
        if TX:
            def tile(j, par):
                r0 = 128 * (2 * j + 1 + par) if j < NP3 else FM * par
                if j == NP3 and par:
                    return _cat([w4b[FM:F, 0:128].astype(f32), jnp.zeros((64, 128), f32)], 0).T
                return w4b[r0:r0 + 128, 0:128].astype(f32).T
            wt = [_cat([tile(j, par) for j in range(7)]) for par in range(2)]
        else:
            wt = [_nt(eye, _ub(p4[par])) for par in range(2)]
        for m, k in ((1, 0), (2, None), (3, 1), (4, 2), (5, None), (6, 3), (7, 4)):
            def blk(b):
                return wt[b // 2][64 * (b % 2):64 * (b % 2 + 1)]
            t4[32 * (m - 1):32 * m, :] = _pk(blk(0 if m == 2 else 3) if k is None else _rhs_sum(k, blk))

    def w4_tile0_steps(r):
        mm = {}
        for t in TORD:
            m = int(t)
            left = _cat([al[64 * j:64 * (j + 1), _lanes(m - 1)] for j in range(7)])
            mm[m] = _nt(_ub(t4[32 * (m - 1):32 * m, :]), _ub(left))
            if len(mm) == 7:
                c11 = ((mm[4] - mm[5]) + mm[1]) + mm[7]
                c22 = ((mm[3] - mm[2]) + mm[1]) + mm[6]
                finish(r, H, _cat([c11, mm[3] + mm[5]], 0).T, 0)
                finish(r + H, H, _cat([mm[4] + mm[2], c22], 0).T, 0)
            yield

    def finish(r, n, h, c):
        c0, c1 = 128 * c, 128 * (c + 1)
        x1 = h2s[rows(r, n), c0:c1] + hss[rows(r, n), c0:c1]
        base = x2s[rows(r, n), c0:c1] + mvec(4, n, c0, c1) * x1
        ob[rows(r, n), c0:c1] = (base + mvec(5, n, c0, c1) * h).astype(bf16)
        if ctx[0] == "z":
            send(r, n, c)

    def w4_plain(r, o=0, n=T):
        def left(k):
            return _cat([al[64 * j:64 * (j + 1), _lanes(k)] for j in range(7)])

        a = _cat([_cat([left(2), left(7)]), _cat([left(8), left(3)])], 0)[o // 2:(o + n) // 2]
        finish(r + o, n, _nn(_ub(a), _ub(_cat([p4[0], p4[1]], 0))), 0)

    def w4_product(m, ahead, order=None):
        def blk(b):
            o = 64 * (b % 2) + 32 * (b // 2)
            return _ub(_cat([al[o + 128 * i:o + 128 * i + 32, _lanes(m - 1)] for i in range(3)]))

        if ahead:
            asum = [_ub(_cat([a2[32 * (3 * (m - 1) + i):32 * (3 * (m - 1) + i + 1), _lanes(k)] for i in range(3)]))
                    for k in range(5)]
        else:
            asum = _lhs_sums(*[blk(b).astype(f32) for b in range(4)])
        bsum = [_ub(_cat([s5[64 * (5 * (m - 1) + k):64 * (5 * (m - 1) + k + 1), _lanes(i)] for i in range(3)], 0))
                for k in range(5)]
        ox = 448 * (m - 1) + 384
        q = _strassen(_nn, blk(0), blk(3), asum, _ub(al[384:416, _lanes(m - 1)]), _ub(al[416:448, _lanes(m - 1)]),
                      _ub(s4_block(m, 0, 0)), _ub(s4_block(m, 3, 0)), bsum,
                      _ub(s4[ox:ox + 64, _lanes(0)]), _ub(s4[ox:ox + 64, _lanes(1)]), ORD[ctx[0] + "_4"])
        return _cat([_cat(q[0:2]), _cat(q[2:4])], 0)

    def w4_steps(r, ahead):
        acc = [c2.at[H * i:H * (i + 1), :] for i in range(4)]

        def finish2(rr, h, c):
            finish(rr, H, h[:, 0:128], c)
            finish(rr, H, h[:, 128:256], c + 2)

        sign = {1: (1, 0, 0, 1), 2: (0, 0, 1, -1), 3: (0, 1, 0, 1), 4: (1, 0, 1, 0), 5: (-1, 1, 0, 0),
                6: (0, 0, 0, 1), 7: (1, 0, 0, 0)}
        left_n, state = [4, 2, 2, 4], [None] * 4
        for m in [int(t) for t in OUTER[ctx[0]]]:
            x = w4_product(m, ahead)
            outs = [i for i in range(4) if sign[m][i]]
            olds = {i: None if state[i] is None else state[i][0][...] for i in outs}
            busy = [state[i][0] for i in range(4) if state[i] is not None and i not in outs]
            free = [a for a in acc if not any(a is b for b in busy)]
            shared = None
            for i in outs:
                sg = sign[m][i]
                left_n[i] -= 1
                if state[i] is None:
                    if shared is None:
                        shared = free.pop()
                        shared[...] = x
                    state[i] = (shared, sg)
                    continue
                v = olds[i] + x if (sg > 0) == (state[i][1] > 0) else (x - olds[i] if sg > 0 else olds[i] - x)
                if left_n[i] == 0:
                    finish2(r + H * (i // 2), v, 1 + i % 2)
                    state[i] = None
                else:
                    dst = free.pop()
                    dst[...] = v
                    state[i] = (dst, 1)
            yield

    def up(order, ahead, r1=None, n1=None):
        for tok in order:
            if tok == "n":
                first = w3_first()
            elif tok == "t":
                tail = w3_tail()
            elif tok == "e":
                put_edge(first, tail)
            elif tok == "3":
                w3_pairs(ahead)
            elif tok == "1":
                mm_w1(r1, n1)
            elif tok == "c":
                ln_chain(r1, n1, paired=PAIRED)

    groups = list(range(0, P0 + P1, RG))
    wait([q_copies[0]])
    sa, ca, ga = mod_part(0, 1)
    modb[0] = ga * sa
    modb[1] = ga * (1.0 + ca)
    for c in range(NL, CT):
        mac_inv(c, NB - 1)
    st1 = {o: _stats(load_q(o)) for o in groups}
    zt[0:8, 0:128] = jnp.zeros((8, 128), u32)
    st2 = {}
    for o in groups:
        x2 = make_x2(o, load_q(o), st1[o])
        x2s[o:o + RG, :] = x2
        st2[o] = _stats(x2)

    wait([mod_copies[1]])
    sb, cb = mod_part(1, 2)
    modb[2] = sb
    modb[3] = 1.0 + cb
    st3 = {}
    for o in range(0, P0, RG):
        h2 = make_h2(x2s[o:o + RG, :], st2[o])
        h2s[o:o + RG, :] = h2
        st3[o] = _stats(h2)
    for o in range(0, P0, RG):
        zt[o // 2:(o + RG) // 2, :] = _pk((h2s[o:o + RG, :] - st3[o][0]) * st3[o][1])

    wait([w_copies[0]])
    prep_square(w1b, w1p, s1)
    z0 = _ub(zt[0:P0 // 2, :])
    h1 = _gelu(_nn(z0, _ub(w1p[:, 0:512])))
    for c in range(CT - 1):
        h1s[c][8:8 + P0, :] = h1[:, _lanes(c)]
    for o in range(0, P0, P0 // 4):
        h1s[CT - 1][8 + o:8 + o + P0 // 4, :] = _gelu(_nn(z0[o:o + P0 // 4], _ub(w1p[:, 512:D])))
    prev = None
    for o1 in range(0, P1 // 2, RG):
        zz = []
        for o in (P0 + o1, P0 + o1 + P1 // 2):
            h2 = make_h2(x2s[o:o + RG, :], st2[o])
            h2s[o:o + RG, :] = h2
            st = _stats(h2, prev, early=True)
            z = (h2 - st[0]) * st[1]
            zt[o // 2:(o + RG) // 2, :] = _pk(z)
            prev = st[1]
            zz.append(z)
        put_sums(zu, o1, zz[0], zz[1])
    mm_w1(P0, P1, P0)

    ctx[0] = "r2"
    wait([w_copies[1], q_copies[1]])
    prep_square(w2b, w2p, s2)
    ln_chain(P0 + P1, PA, paired=R2M)
    mm_w2(0)
    ln_x1(0, R2L)
    mm_w2(T)

    ctx[0] = "r3"
    wait([w_copies[2]])
    prep_w3()
    early = ln_x1(T, stats_only=True) if SE else None
    up(R3O, True, P0 + P1, PA)

    ctx[0] = "r4"
    if FEN4:
        jax.lax.fori_loop(0, 2, fence, 0)
    wait([w_copies[3], mod_copies[2]])
    prep_w4()
    sc16 = jnp.broadcast_to(scb[:, 0:D], (16, D)).astype(bf16)
    steps, h, j = w4_steps(0, True), None, 0
    if TP0:
        prep_t4()
        tile0 = w4_tile0_steps(0)
    for tok in R4O:
        if tok == "p" and TP0:
            next(tile0)
        elif tok == "T" and TP0:
            pass
        elif tok == "p":
            blk = [al[64 * j:64 * (j + 1), _lanes(k)] for k in (2, 7, 8, 3)]
            w = _ub(_cat([p4[0, 64 * j:64 * (j + 1), :], p4[1, 64 * j:64 * (j + 1), :]], 0))
            d = [_nn(_ub(_cat(blk[0:2])), w), _nn(_ub(_cat(blk[2:4])), w)]
            h = d if h is None else [h[0] + d[0], h[1] + d[1]]
            j += 1
            if j == 7:
                finish(0, H, h[0], 0)
                finish(H, H, h[1], 0)
        elif tok == "s":
            next(steps)
        elif tok == "T":
            prep_t4()
        else:
            c0, c1 = (0, 384) if tok == "g" else (384, D)
            gb = jnp.dot(sc16, wmc[:, c0:c1], preferred_element_type=f32)[0:8]
            modb[4, :, c0:c1] = gb
            modb[5, :, c0:c1] = 0.5 * gb
    ln_x1(T, stats=early)
    out_copy(0).start()
    q_copies[2].wait()

    def mlp_body(i, carry):
        r1 = pl.multiple_of(PB - PC + PC * i, 32)
        r = pl.multiple_of(i * T, T)
        up(HEAD, False, r1, PC)
        steps, tile0 = w4_steps(r, False), w4_tile0_steps(r)
        for tok in BODY:
            if tok == "1":
                mm_w1(r1, PC)
            elif tok == "p":
                next(tile0)
            elif tok == "2":
                mm_w2(r + T)
            elif tok == "l":
                ln_x1(r + T, LM)
            else:
                next(steps)
        out_copy(i).start()
        return carry

    ctx[0] = "l"
    jax.lax.fori_loop(1, NC - 1, mlp_body, 0)

    ctx[0] = "z"
    up(ZO, True)
    if TZ:
        steps, tile0 = w4_steps(S - T, True), w4_tile0_steps(S - T)
        for tok in ZB:
            next(steps if tok == "s" else tile0)
    else:
        prep_p4()
        w4_plain(S - T, 0, LA)
        for _ in w4_steps(S - T, True):
            pass
        if LAST0 > LA:
            w4_plain(S - T, LA, LAST0 - LA)
        w4_plain(S - T, LAST0, T - LAST0)
    for i in range(NC - 1):
        out_copy(i).wait()
    for cp in out_tail:
        cp.wait()


@jax.jit
def pallas_adaLN_cond__ssm_conv_h3__mixer_s_mlp__prompt_kernel(
    A_q: jax.Array,
    A_k: jax.Array,
    A_v: jax.Array,
    A_shift_k: jax.Array,
    A_ssm_k: jax.Array,
    A_ssm_D: jax.Array,
    B_x: jax.Array,
    B_w1: jax.Array,
    B_w2: jax.Array,
    B_w3: jax.Array,
    B_w4: jax.Array,
    c: jax.Array,
    w_mod: jax.Array,
):
    del B_x
    any_spec = pl.BlockSpec(memory_space=pl.ANY)

    def tile_view(x):
        return x.reshape(S // 8, 8, CT, 128).transpose(0, 2, 1, 3).reshape(S * CT, 128)

    vm = pltpu.VMEM
    dma = pltpu.SemaphoreType.DMA
    spec = (4, NG, 16, 128)
    out = pl.pallas_call(
        _kernel,
        in_specs=[any_spec] * 12,
        out_specs=any_spec,
        out_shape=jax.ShapeDtypeStruct((S, D), bf16),
        scratch_shapes=[
            *[vm((KROWS, 128), bf16)] * NB, *[vm((VROWS, 128), bf16)] * NB, vm((CT, 128, S), bf16),
            vm((S, D), bf16), vm((D, D), bf16), vm((D, D), bf16), vm((F, D), bf16), vm((F, D), bf16),
            vm((D // 2, D), u32), vm((D // 2, D), u32), vm((F // 2, D), u32),
            vm((D, 3 * D), bf16), vm((D, 2 * D), bf16), vm((D, D), bf16),
            vm((4, D), bf16), vm((D,), bf16), vm((1, D), bf16), vm((1, 1792), f32),
            vm((4, 128, 128), u32), vm((4, 128, 128), u32), vm((4, 64, 256), u32),
            vm((CT, 8, 8, 128), f32),
            vm((CT, NB) + spec, f32), vm((CT, NB - 1) + spec, f32), vm((CT,) + spec, f32),
            vm((CT, NB) + spec, f32), vm((4, 128, 128), f32),
            vm((CT, S + 32, 128), f32), vm((8, 8, D), f32),
            *[vm((S + 32, 128), f32)] * CT, vm((S, D), f32), vm((S, D), f32), vm((S, D), f32),
            vm((288, D), u32), vm((5, H // 2, 256), u32), vm((H, D), u32), vm((5, H // 2, 256), u32),
            vm((D // 2, 128), u32), vm((D, 256), u32), vm((D, 256), u32), vm((NP3 * 64, 1280), u32),
            vm((7 * 448, 256), u32), vm((35 * 64, 384), u32), vm((2, 448, 128), u32),
            vm((7 * 64, 1152), u32), vm((21 * 32, 640), u32), vm((4 * H, 256), f32), vm((7 * 32, 896), u32),
            vm((S, D), bf16),
            dma((26,)), dma((NC + 10,)),
        ],
        compiler_params=pltpu.CompilerParams(vmem_limit_bytes=110 << 20, disable_bounds_checks=True,
                                             disable_semaphore_checks=True),
    )(A_q.reshape(S, D), tile_view(A_k), tile_view(A_v), A_shift_k.T, A_ssm_k,
      A_ssm_D, B_w1, B_w2, B_w3.T, B_w4, c, w_mod)
    return out.reshape(1, S, D)
```

```python
import numpy as np
import jax
import jax.numpy as jnp
import jax.experimental.pallas as pl
import jax.experimental.pallas.tpu as pltpu

f32, bf16, u32, i32 = jnp.float32, jnp.bfloat16, jnp.uint32, jnp.int32

S, D, F = 2048, 640, 1728
CT = D // 128
TR = 8 * CT
NB, BLK, NFFT = 4, 512, 1024
KROWS, VROWS = BLK * CT + 128, BLK * CT + 64
NG = 16
T = 256
NC = S // T
H = T // 2
NP3 = 6
FM = (F // 128) * 128
P0, P1, PA, PC = 320, 224, 160, 224
PB = P0 + P1 + PA
LA, LAST0 = 96, 208
RG = 16
EPS = 1e-5
NT_DIMS = (((1,), (1,)), ((), ()))
PAIRED = "10000100001000"
ORD = {"r1_1": "4235a1c76db", "r2_2": "c72db4a3156", "r3_1": "15726b43cda", "r3_3": "c24a5173b6d",
       "r3_e": "23cb451a76d", "r3_0": "345217ba6cd", "r4_4": "5b12a47cd63", "l_1": "7325bad4c61",
       "l_2": "514d2ac67b3", "l_3": "4bc51a7d236", "l_4": "243ac571b6d", "l_e": "24bcd35176a",
       "l_0": "abcd2351746", "z_3": "b5c23147ad6", "z_4": "35d12cb74a6", "z_e": "cdb1237a465",
       "z_0": "acd231b4576"}
OUTER = {"r4": "1726435", "l": "5132647", "z": "1523674"}
BODY = "1pp2sslpsspspspps"
HEAD = "xecyz"
LM = "0000000000100000"
R2M = "0010101010"
R2L = "1010100010101010"
R3O = "1eyzx"
R4O = "gsssGpspsppppsps"
SE = 1
ZO = "xyez"
FEN4 = 1
FA = 3
TORD = "7621354"
TP0 = 1
TX = 1
TZ = 0
ZB = "ppsspspspspsps"
GV = 8
NL = 4


def _lo(w):
    return pltpu.bitcast(w << 16, f32)


def _hi(w):
    return pltpu.bitcast(w & jnp.uint32(0xFFFF0000), f32)


def _cis(n):
    t = (n & (2 * NFFT - 1)).astype(f32) * (np.pi / NFFT)
    return jnp.cos(t), jnp.sin(t)


def _fwd_table(r):
    g = jax.lax.broadcasted_iota(i32, (NG, 128), 0)
    cg, sg = _cis(jnp.where(g < NG // 2, 32 * g + 1, 32 * g - 253) * r)
    cs, ss = _cis(4 * jax.lax.broadcasted_iota(i32, (8, 128), 0) * r)
    parts = []
    for i in range(NG):
        c, s = cg[i:i + 1], sg[i:i + 1]
        parts += [c * cs - s * ss, -(s * cs + c * ss)]
    return pltpu.bitcast(jnp.concatenate(parts, axis=0).astype(bf16), u32)


def _inv_tables():
    def phase(rows):
        col = jax.lax.broadcasted_iota(i32, (rows, 256), 1)
        k = ((col >> 4) << 3) + (col & 7)
        row = jax.lax.broadcasted_iota(i32, (rows, 256), 0)
        return jnp.where(k < 64, 4 * k + 1, 4 * k - 253), (col & 8) << 6, row

    fr, _, g = phase(16)
    cg, sg = _cis(fr * (32 * g))
    fr, off, s = phase(8)
    out = []
    for p in range(4):
        cs, ss = _cis(fr * (4 * s + p) + off)
        cs, ss = cs * (2.0 / NFFT), ss * (2.0 / NFFT)
        parts = [cg[i:i + 1] * cs - sg[i:i + 1] * ss for i in range(16)]
        out.append(pltpu.bitcast(jnp.concatenate(parts, axis=0).astype(bf16), u32))
    return out


def _radix4(re, im, inverse):
    ar, ai = re[0] + re[2], im[0] + im[2]
    br, bi = re[0] - re[2], im[0] - im[2]
    cr, ci = re[1] + re[3], im[1] + im[3]
    dr, di = re[1] - re[3], im[1] - im[3]
    minus_i = (br + di, bi - dr)
    plus_i = (br - di, bi + dr)
    if inverse:
        return [(ar + cr, ai + ci), plus_i, (ar - cr, ai - ci), minus_i]
    return [(ar + cr, ai + ci), minus_i, (ar - cr, ai - ci), plus_i]


def _stats(x, link=None, early=False, scaled=False):
    zero = 0.0 if link is None else jnp.minimum(link, 0.0)
    part = x[:, 0:128]
    for c in range(1, CT):
        part = part + x[:, c * 128:(c + 1) * 128]
    if link is not None and early:
        part = part + zero
        zero = 0.0
    m = jnp.sum(part, axis=-1, keepdims=True) * (1.0 / D)
    v = jnp.maximum(jnp.sum(x * x, axis=-1, keepdims=True) * (1.0 / D) - m * m, zero)
    e = jnp.log(v + EPS) * (-0.5 / np.log(2.0))
    return m, jnp.exp2(e + np.log2(ALPHA) if scaled else e)


GC = 0.7978845608028654
ALPHA = (GC * 0.044715) ** (1.0 / 3.0)


def _gelu_scaled(y):
    return y + y * jnp.tanh(y * (y * y + GC / ALPHA))


def _pk(x):
    return pltpu.bitcast(x.astype(bf16), u32)


def _ub(x):
    return pltpu.bitcast(x, bf16)


def _cat(xs, axis=-1):
    return jnp.concatenate(xs, axis=axis)


def _lanes(k):
    return slice(128 * k, 128 * (k + 1))


def _nn(a, w):
    return jnp.dot(a.astype(bf16), w, preferred_element_type=f32)


def _nt(a, w):
    return jax.lax.dot_general(a, w, NT_DIMS, preferred_element_type=f32)


def _lhs_sums(a11, a12, a21, a22):
    return [a11 + a22, a21 + a22, a11 + a12, a21 - a11, a12 - a22]


def _rhs_sum(k, block):
    a, b, plus = [(0, 3, True), (1, 3, False), (2, 0, False), (0, 1, True), (2, 3, True)][k]
    return block(a) + block(b) if plus else block(a) - block(b)


def _strassen(dot, a11, a22, asum, ax1, ax2, b11, b22, bsum, bx1, bx2, order="", xdot=None):
    if order:
        ops = {"1": (asum[0], bsum[0], (1, 0, 0, 1)), "2": (asum[1], b11, (0, 0, 1, -1)),
               "3": (a11, bsum[1], (0, 1, 0, 1)), "4": (a22, bsum[2], (1, 0, 1, 0)),
               "5": (asum[2], b22, (-1, 1, 0, 0)), "6": (asum[3], bsum[3], (0, 0, 0, 1)),
               "7": (asum[4], bsum[4], (1, 0, 0, 0)), "a": (ax1, bx1, (1, 0, 0, 0)),
               "b": (ax1, bx2, (0, 1, 0, 0)), "c": (ax2, bx1, (0, 0, 1, 0)), "d": (ax2, bx2, (0, 0, 0, 1))}
        c, neg = [None] * 4, [None] * 4
        for t in order:
            a, b, sg = ops[t]
            m = (xdot if xdot and t in "abcd" else dot)(a, b)
            for i in range(4):
                if sg[i] > 0:
                    c[i] = m if c[i] is None else c[i] + m
                    if neg[i] is not None:
                        c[i], neg[i] = c[i] - neg[i], None
                elif sg[i] < 0:
                    if c[i] is None:
                        neg[i] = m
                    else:
                        c[i] = c[i] - m
        return c
    m2 = dot(asum[1], b11)
    m4 = dot(a22, bsum[2])
    c21 = (m4 + m2) + dot(ax2, bx1)
    m3 = dot(a11, bsum[1])
    m5 = dot(asum[2], b22)
    c12 = (m3 + m5) + dot(ax1, bx2)
    m1 = dot(asum[0], bsum[0])
    c11 = (((m4 - m5) + m1) + dot(asum[4], bsum[4])) + dot(ax1, bx1)
    c22 = (((m3 - m2) + m1) + dot(asum[3], bsum[3])) + dot(ax2, bx2)
    return [c11, c12, c21, c22]


def _kernel(q_hbm, k_hbm, v_hbm, sh_hbm, sk_hbm, d_hbm, w1_hbm, w2_hbm, w3_hbm, w4_hbm,
            c_hbm, wm_hbm, o_hbm,
            kb0, kb1, kb2, kb3, vb0, vb1, vb2, vb3, skb, qb, w1b, w2b, w3b, w4b, w1p, w2p, w3p,
            wma, wmb, wmc, shb, db, cb_, scb,
            fub, fkb, gtb, par, US, KS, UR, YS, YP, ys, modb, h10, h11, h12, h13, h14, h2s, x2s, hss,
            zt, zu, zb, zs, w3n, s1, s2, s3, s4, s5, p4, al, a2, c2, t4, e3, ob,
            sem, sem_o):
    h1s = [h10, h11, h12, h13, h14]
    n_in = [0]

    def load(src, dst):
        n_in[0] += 1
        return pltpu.make_async_copy(src, dst, sem.at[n_in[0] - 1])

    nkv = BLK * CT
    small = [load(d_hbm, db), load(sh_hbm, shb), load(c_hbm, cb_)]
    sk_copies = [load(sk_hbm.at[pl.ds(c * 128, 128), :], skb.at[c]) for c in range(CT)]
    kbs, vbs, wms = [kb0, kb1, kb2, kb3], [vb0, vb1, vb2, vb3], [wma, wmb, wmc]
    kv_copies = [[load(k_hbm.at[pl.ds(a * nkv, nkv), :], kbs[a].at[pl.ds(TR, nkv), :]),
                  load(v_hbm.at[pl.ds(a * nkv, nkv), :], vbs[a].at[pl.ds(0, nkv), :])] for a in range(NB)]
    mod_cols = [(0, 3 * D), (3 * D, 2 * D), (5 * D, D)]
    mod_copies = [load(wm_hbm.at[:, pl.ds(o, n)], w) for (o, n), w in zip(mod_cols, wms)]
    w_copies = [load(w1_hbm, w1b), load(w2_hbm, w2b), load(w3_hbm, w3b), load(w4_hbm, w4b)]
    q_copies = [load(q_hbm.at[pl.ds(o, n), :], qb.at[pl.ds(o, n), :])
                for o, n in [(0, P0 + P1), (P0 + P1, PA), (PB, S - PB)]]

    def out_copy(i):
        r = i * T if isinstance(i, int) else pl.multiple_of(i * T, T)
        return pltpu.make_async_copy(ob.at[pl.ds(r, T), :], o_hbm.at[pl.ds(r, T), :], sem_o.at[i])

    out_tail = []

    def send(r, n, c):
        cp = pltpu.make_async_copy(ob.at[pl.ds(r, n), pl.ds(128 * c, 128)], o_hbm.at[pl.ds(r, n), pl.ds(128 * c, 128)],
                                   sem_o.at[NC - 1 + len(out_tail)])
        out_tail.append(cp)
        cp.start()

    for cp in (small + kv_copies[0] + sk_copies + kv_copies[1] + kv_copies[2] + kv_copies[3]
               + [mod_copies[0], q_copies[0], mod_copies[1], w_copies[0], w_copies[1], q_copies[1],
                  w_copies[2], w_copies[3], mod_copies[2], q_copies[2]]):
        cp.start()

    def wait(copies):
        for cp in copies:
            cp.wait()

    def pin(i, carry):
        z = jnp.zeros((8, 128), f32)
        scb[:, pl.ds(pl.multiple_of(i * 128, 128), 128)] = z[0:1]
        YP[i, 0:8, :] = z
        US[i, 0, 0, 0, 0:8, :] = z
        KS[i, 0, 0, 0, 0:8, :] = z
        YS[i, 0, 0, 0, 0:8, :] = z
        UR[i, 0, 0, 0:8, :] = z
        r8 = pl.ds(pl.multiple_of(i * 8, 8), 8)
        c2[r8, 0:128] = z
        al[r8, 0:128] = jnp.zeros((8, 128), u32)
        a2[r8, 0:128] = jnp.zeros((8, 128), u32)
        return carry

    def fence(i, carry):
        YP[i, 0:8, :] = jnp.zeros((8, 128), f32)
        return carry

    jax.lax.fori_loop(0, 2, pin, 0)
    lane = jax.lax.broadcasted_iota(i32, (1, 128), 1)
    for p in range(4):
        m = (lane - p) & 3
        fkb[p] = _fwd_table(128 * m + ((lane - m) & 127))
    for c in range(CT):
        kb0[c * 8:(c + 1) * 8, :] = jnp.zeros((8, 128), bf16)
        h1s[c][0:8, :] = jnp.zeros((8, 128), f32)
        h1s[c][S + 8:S + 16, :] = jnp.zeros((8, 128), f32)
    for a in range(NB):
        kbs[a][nkv + TR:KROWS, :] = jnp.zeros((KROWS - nkv - TR, 128), bf16)
        vbs[a][nkv:VROWS, :] = jnp.zeros((VROWS - nkv, 128), bf16)
    for p in range(4):
        fub[p] = _fwd_table(8 * (lane & 63) + ((lane >> 6) << 2) + p)
    wait(small)
    cvec = cb_[...].astype(f32)
    scb[:, 0:D] = cvec * jax.nn.sigmoid(cvec)
    dv = db[...].astype(f32).reshape(1, D)
    shv = shb[...].astype(f32)
    for c in range(CT):
        for i in range(4):
            par[c, i] = jnp.broadcast_to(shv[i:i + 1, c * 128:(c + 1) * 128], (8, 128))
        par[c, 4] = jnp.broadcast_to(dv[:, c * 128:(c + 1) * 128], (8, 128))
    for p, tab in enumerate(_inv_tables()):
        gtb[p] = tab

    def get(ref, idx, g, n):
        return (ref[idx + (slice(g, g + n), slice(0, 8))], ref[idx + (slice(g, g + n), slice(8, 16))])

    def put(ref, idx, g, n, xr, xi):
        ref[idx + (slice(g, g + n), slice(0, 8))] = xr
        ref[idx + (slice(g, g + n), slice(8, 16))] = xi

    def split(tt, g, n):
        tt = [t[g * 16:(g + n) * 16].reshape(n, 16, 128) for t in tt]
        return [t[:, 0:8] for t in tt], [t[:, 8:16] for t in tt]

    def fwd_k(c, j):
        lane = jax.lax.broadcasted_iota(i32, (64, 128), 1)
        even = (lane & 1) == 0
        l01 = (lane & 2) == 0
        l12 = ((lane + 3) & 2) == 0
        rm = []
        for m in range(4):
            w = pltpu.bitcast(skb[c, :, (4 * j + m) * 128:(4 * j + m + 1) * 128], u32)
            rm.append(pltpu.roll(w, m, 1) if m else w)
        e01 = jnp.where(even, rm[0], rm[1])
        o01 = jnp.where(even, rm[1], rm[0])
        e23 = jnp.where(even, rm[2], rm[3])
        o23 = jnp.where(even, rm[3], rm[2])
        kp = [jnp.where(l01, e01, e23), jnp.where(l12, o01, o23),
              jnp.where(l01, e23, e01), jnp.where(l12, o23, o01)]
        tt = [jax.lax.dot_general(pltpu.bitcast(fkb[p], bf16), pltpu.bitcast(kp[p], bf16), NT_DIMS,
                                  preferred_element_type=f32) for p in range(4)]
        for g in range(0, NG, GV):
            re, im = split(tt, g, GV)
            if j == 0:
                re[0] = re[0] + par[c, 4][None]
            for m, (xr, xi) in enumerate(_radix4(re, im, False)):
                if j < NB - 1:
                    put(KS, (c, j, m), g, GV, xr, xi)
                ur, ui = get(US, (c, 0, m), g, GV)
                put(YS, (c, j, m), g, GV, xr * ur - xi * ui, xr * ui + xi * ur)

    def fwd_u(c, a):
        taps = [jnp.tile(par[c, i], (8, 1)) for i in range(4)]
        ws = TR // 2
        base = 4 * c
        kw, vw = kbs[a].bitcast(u32), vbs[a].bitcast(u32)

        def words(ref, start):
            return ref[pl.ds(start, BLK // 8, stride=ws), :]

        kk = {}
        for w in range(4):
            x = words(kw, ws + base + w)
            kk[2 * w], kk[2 * w + 1] = _lo(x), _hi(x)
        kk[-3] = _hi(words(kw, base + 2))
        x = words(kw, base + 3)
        kk[-2], kk[-1] = _lo(x), _hi(x)
        sub = []
        for w in range(4):
            x = words(vw, base + w)
            for r, vv in ((2 * w, _lo(x)), (2 * w + 1, _hi(x))):
                sh = taps[0] * kk[r] + taps[1] * kk[r - 1] + taps[2] * kk[r - 2] + taps[3] * kk[r - 3]
                sub.append(sh * vv)
        kv = [jnp.concatenate([sub[p], sub[p + 4]], axis=0) for p in range(4)]
        tt = [jnp.dot(pltpu.bitcast(fub[p], bf16), kv[p].astype(bf16), preferred_element_type=f32)
              for p in range(4)]
        for g in range(0, NG, GV):
            re, im = split(tt, g, GV)
            for m, (xr, xi) in enumerate(_radix4(re, im, False)):
                if a:
                    pr, pi = get(US, (c, 0, m), g, GV) if a == 1 else get(UR, (c, m), g, GV)
                    if a < NB - 1:
                        put(UR, (c, m), g, GV, xr, xi)
                    xr, xi = (xr - pi, xi + pr) if g < NG // 2 else (xr + pi, xi - pr)
                put(US, (c, a, m), g, GV, xr, xi)

    def mac_inv(c, a):
        for h in range(2):
            vals = [[] for _ in range(4)]
            for g in range(8 * h, 8 * h + 8, GV):
                yre, yim = [], []
                for m in range(4):
                    yr, yi = get(YS, (c, a, m), g, GV)
                    for j in range(a):
                        kr, ki = get(KS, (c, j, m), g, GV)
                        ur, ui = get(US, (c, a - j, m), g, GV)
                        yr = yr + (kr * ur - ki * ui)
                        yi = yi + (kr * ui + ki * ur)
                    yre.append(yr)
                    yim.append(yi)
                for p, (pr, pi) in enumerate(_radix4(yre, yim, True)):
                    vals[p].append(jnp.concatenate([pr, pi], axis=1))
            for p in range(4):
                pb = jnp.concatenate(vals[p], axis=0).reshape(128, 128).astype(bf16)
                r = jnp.dot(pltpu.bitcast(gtb[p, :, h * 128:(h + 1) * 128], bf16), pb,
                            preferred_element_type=f32)
                if h == 0:
                    YP[p] = r
                else:
                    ys[c, pl.ds(a * BLK + p, 128, stride=4), :] = YP[p] + r

    wait(kv_copies[0])
    for c in range(CT):
        fwd_u(c, 0)
    for grp in ((0,), (1, 2), (3, 4)):
        wait([sk_copies[c] for c in grp])
        for c in grp:
            for j in (3, 2, 1, 0):
                fwd_k(c, j)
    for a in range(1, NB):
        if a == FA:
            jax.lax.fori_loop(0, 2, fence, 0)
        wait(kv_copies[a])
        for c in range(CT):
            kbs[a][c * 8:(c + 1) * 8, :] = kbs[a - 1][nkv + c * 8:nkv + (c + 1) * 8, :]
        for c in range(CT):
            fwd_u(c, a)
            mac_inv(c, a - 1)
    wait([mod_copies[0]])
    for c in range(NL):
        mac_inv(c, NB - 1)

    def mod_part(part, extra):
        n, wm = mod_cols[part][1], wms[part]
        act = scb[:, 0:D]

        def sc(k0, k1):
            return jnp.broadcast_to(act[:, k0:k1], (16, k1 - k0)).astype(bf16)

        e = 128 * extra
        r = jnp.dot(sc(0, D), wm[:, e:n], preferred_element_type=f32)
        r0 = (jnp.dot(sc(0, D - 64), wm[0:D - 64, 0:e], preferred_element_type=f32)
              + jnp.dot(sc(D - 64, D), wm[D - 64:D, 0:e], preferred_element_type=f32))
        r = jnp.concatenate([r0, r], axis=-1)[0:8]
        return [r[:, i * D:(i + 1) * D] for i in range(n // D)]

    def mvec(i, n=RG, c0=0, c1=D):
        return jnp.tile(modb[i, :, c0:c1], (n // 8, 1))

    rows = pl.ds
    ctx = ["r1"]

    def load_q(r, ref=qb):
        return ref[rows(r, RG), :].astype(f32)

    def make_x2(r, q, st, ref=ys):
        y = _cat([ref[c, rows(r, RG), :] for c in range(CT)])
        return q + (((q - st[0]) * st[1]) * mvec(1) + mvec(0)) * y

    def make_h2(x2, st):
        return ((x2 - st[0]) * st[1]) * mvec(3) + mvec(2)

    def put_sums(ref, o, z1, z2):
        for k, v in enumerate(_lhs_sums(z1[:, 0:256], z1[:, 256:512], z2[:, 0:256], z2[:, 256:512])):
            ref.at[k][o // 2:(o + RG) // 2, :] = _pk(v)

    def ln_chain(r, n, links=1, paired=""):
        qv, yv = qb.at[rows(r, n), :], ys.at[:, rows(r, n), :]
        xv, hv = x2s.at[rows(r, n), :], h2s.at[rows(r, n), :]
        prev, pend, cnt = [None] * links, None, 0
        for o1 in range(0, n // 2, RG):
            zz = []
            for o in (o1, o1 + n // 2):
                q = load_q(o, qv)
                x2 = make_x2(o, q, _stats(q, prev[cnt % links]), yv)
                xv[o:o + RG, :] = x2
                st = _stats(x2)
                h2 = make_h2(xv[o:o + RG, :], st)
                hv[o:o + RG, :] = h2
                st = _stats(h2, scaled=True)
                z = (hv[o:o + RG, :] - st[0]) * st[1]
                zt[o // 2:(o + RG) // 2, :] = _pk(z)
                zz.append(z)
                if paired and paired[cnt] == "1":
                    pend = st[1]
                elif pend is not None:
                    prev[0], pend = jnp.minimum(st[1], pend), None
                else:
                    prev[cnt % links] = st[1]
                cnt += 1
            put_sums(zu, o1, zz[0], zz[1])

    def ln_x1(r, paired="", stats=None, stats_only=False):
        sv = hss.at[rows(r, T), :]
        prev, pend, cnt, out = None, None, 0, []
        for o1 in range(0, H, RG):
            zz = []
            for o in (o1, o1 + H):
                x1 = sv[o:o + RG, :]
                st = _stats(x1, prev, True, True) if stats is None else stats[cnt]
                out.append(st)
                if not stats_only:
                    z = (x1 - st[0]) * st[1]
                    zb[o // 2:(o + RG) // 2, :] = _pk(z)
                    zz.append(z)
                if paired and paired[cnt] == "1":
                    pend = st[1]
                elif pend is not None:
                    prev, pend = jnp.minimum(st[1], pend), None
                else:
                    prev = st[1]
                cnt += 1
            if not stats_only:
                put_sums(zs, o1, zz[0], zz[1])
        return out

    def both(ref, r0, r1, col):
        return _cat([ref[r0:r1, _lanes(1 + col)].astype(f32), ref[r0:r1, _lanes(3 + col)].astype(f32)])

    def prep_square(wb, wp, sw):
        wp[...] = pltpu.bitcast(wb[...], u32)
        for k in (2, 1, 0, 4, 3):
            sw[128 * k:128 * (k + 1), :] = _pk(_rhs_sum(
                k, lambda b: both(wb, 256 * (b // 2), 256 * (b // 2 + 1), b % 2)))

    def mm_square(a, top, bot, asum, wp, sw, which):
        h = top.shape[0]
        c0 = _nn(a, _ub(wp[:, 0:128]))
        out = [(c0[0:h], c0[h:2 * h])]
        for n in range(2):
            l1, l2 = _lanes(2 * n + 1), _lanes(2 * n + 2)
            q = _strassen(_nn, top[:, 0:256], bot[:, 256:512], asum, top[:, 512:D], bot[:, 512:D],
                          _ub(wp[0:128, l1]), _ub(wp[128:256, l2]),
                          [_ub(sw[128 * k:128 * (k + 1), _lanes(n)]) for k in range(5)],
                          _ub(wp[256:320, l1]), _ub(wp[256:320, l2]), ORD[ctx[0] + "_" + which])
            out += [(q[0], q[2]), (q[1], q[3])]
        return out

    def mm_w1(r, n, o=0):
        h, o = n // 2, o // 2
        res = mm_square(_ub(zt[o:o + h, :]), _ub(zt[o:o + h // 2, :]), _ub(zt[o + h // 2:o + h, :]),
                        [_ub(zu[k, 0:h // 2, :]) for k in range(5)], w1p, s1, "1")
        for c, (top, bot) in enumerate(res):
            h1s[c][rows(r + 8, h), :] = _gelu_scaled(top)
            h1s[c][rows(r + 8 + h, h), :] = _gelu_scaled(bot)

    def mm_w2(r):
        lane = jax.lax.broadcasted_iota(i32, (T, 128), 1)

        def sh(k, c):
            return h1s[c][rows(r + 8 + k, T), :]

        g = _cat([sh(-1, 0),
                  jnp.where(lane < 32, sh(-1, 1), sh(1, 1)),
                  jnp.where(lane < 64, sh(1, 2), sh(-2, 2)),
                  jnp.where(lane < 96, sh(-2, 3), sh(2, 3)),
                  sh(2, 4)])
        top, bot = g[0:H], g[H:T]
        sums = _lhs_sums(top[:, 0:256], top[:, 256:512], bot[:, 0:256], bot[:, 256:512])
        for c, (ct, cb) in enumerate(mm_square(g, top, bot, sums, w2p, s2, "2")):
            hss[rows(r, H), _lanes(c)] = h2s[rows(r, H), _lanes(c)] + ct * (0.5 / ALPHA)
            hss[rows(r + H, H), _lanes(c)] = h2s[rows(r + H, H), _lanes(c)] + cb * (0.5 / ALPHA)

    def prep_w3():
        for j in range(NP3):
            r0 = 128 * (2 * j + 1)
            w3p[r0 // 2:r0 // 2 + 64, 0:256] = pltpu.bitcast(w3b[r0:r0 + 128, 0:256], u32)
            w3p[r0 // 2:r0 // 2 + 64, 512:D] = pltpu.bitcast(w3b[r0:r0 + 128, 512:D], u32)
            w3p[r0 // 2 + 64:r0 // 2 + 128, 256:D] = pltpu.bitcast(w3b[r0 + 128:r0 + 256, 256:D], u32)
        w3p[0:64, :] = pltpu.bitcast(w3b[0:128, :], u32)
        w3p[FM // 2:F // 2, :] = pltpu.bitcast(w3b[FM:F, :], u32)
        w3n[0:64, :] = _pk(_cat([w3b[128:256, 512:D].astype(f32).T, w3b[256:384, 512:D].astype(f32).T]))

        def edge(b):
            c = slice(256 * (b // 2), 256 * (b // 2 + 1))
            if b % 2 == 0:
                return w3b[0:96, c].astype(f32)
            return _cat([w3b[96:128, c].astype(f32), w3b[FM:F, c].astype(f32)], 0)

        for k in (2, 1, 0, 4, 3):
            e3[0:48, 256 * k:256 * (k + 1)] = _pk(_rhs_sum(k, edge))
        for j in range(NP3):
            r0 = 128 * (2 * j + 1)
            for k in (2, 1, 0, 4, 3):
                s3[64 * j:64 * (j + 1), 256 * k:256 * (k + 1)] = _pk(_rhs_sum(k, lambda b: w3b[
                    r0 + 128 * (b % 2):r0 + 128 * (b % 2 + 1), 256 * (b // 2):256 * (b // 2 + 1)].astype(f32)))

    def w3_edge():
        def second(c0, c1):
            return _ub(_cat([w3p[48:64, c0:c1], w3p[FM // 2:F // 2, c0:c1]], 0))

        z1, z2 = _ub(zb[0:H // 2, :]), _ub(zb[H // 2:H, :])
        q = _strassen(lambda a, b: _nt(b, a), z1[:, 0:256], z2[:, 256:512], [_ub(zs[k]) for k in range(5)],
                      z1[:, 512:D], z2[:, 512:D], _ub(w3p[0:48, 0:256]), second(256, 512),
                      [_ub(e3[0:48, 256 * k:256 * (k + 1)]) for k in range(5)],
                      _ub(w3p[0:48, 512:D]), second(512, D), ORD[ctx[0] + "_e"])
        q = [_gelu_scaled(c) for c in q]
        out = []
        for x in (_cat(q[0:2], 0), _cat(q[2:4], 0)):
            out += [x[0:128].T, _cat([x[128:192], jnp.zeros((64, 128), f32)], 0).T]
        put_quads(NP3, out)

    def w3_pair(j):
        e, o = slice(64 * (2 * j + 1), 64 * (2 * j + 2)), slice(64 * (2 * j + 2), 64 * (2 * j + 3))
        z1, z2 = _ub(zb[0:H // 2, :]), _ub(zb[H // 2:H, :])
        q = _strassen(_nt, z1[:, 0:256], z2[:, 256:512], [_ub(zs[k]) for k in range(5)], z1[:, 512:D], z2[:, 512:D],
                      _ub(w3p[e, 0:256]), _ub(w3p[o, 256:512]),
                      [_ub(s3[64 * j:64 * (j + 1), 256 * k:256 * (k + 1)]) for k in range(5)],
                      *([_ub(w3n[0:64, 0:128]), _ub(w3n[0:64, 128:256]), ORD[ctx[0] + "_0"], _nn] if j == 0 else
                        [_ub(w3p[e, 512:D]), _ub(w3p[o, 512:D]), ORD[ctx[0] + "_3"]]))
        return [_gelu_scaled(c) for c in q]

    def plain_ctx():
        return (ctx[0] in ("r3", "r4") and not TP0) or (ctx[0] == "z" and not TZ)

    def put_quads(j, q):
        l1, l2, l5, l6, l7 = _lhs_sums(*q)
        if not plain_ctx():
            al[64 * j:64 * (j + 1), 0:896] = _pk(_cat([l1, l2, q[0], q[3], l5, l6, l7]))
        else:
            al[64 * j:64 * (j + 1), :] = _pk(_cat([l1, l2, q[0], q[3], l5, l6, l7, q[1], q[2]]))

    def w3_pairs(ahead, which):
        for i in which:
            ops = []
            for j in (2 * i, 2 * i + 1):
                q = w3_pair(j)
                if not ahead:
                    put_quads(j, q)
                ops.append(q)
            if not ahead:
                continue
            for n, q in enumerate(ops):
                l1, l2, l5, l6, l7 = _lhs_sums(*q)
                ops[n] = [l1, l2, q[0], q[3], l5, l6, l7]
                j, half = 2 * i + n, slice(64 * n, 64 * (n + 1))
                if not plain_ctx():
                    al[64 * j:64 * (j + 1), 0:896] = _pk(_cat(ops[n]))
                    continue
                o = 64 * j + 32 * n
                al[o:o + 32, 0:256] = _pk(_cat([l1[half], l2[half]]))
                al[o:o + 32, 512:896] = _pk(_cat([l5[half], l6[half], l7[half]]))
                al[64 * j:64 * (j + 1), 256:512] = _pk(_cat([q[0], q[3]]))
                al[64 * j:64 * (j + 1), 896:1152] = _pk(_cat([q[1], q[2]]))
            for m in range(7):
                e, o = ops[0][m], ops[1][m]
                r0 = 32 * (3 * m + i)
                a2[r0:r0 + 32, :] = _pk(_cat(_lhs_sums(e[0:64], o[0:64], e[64:128], o[64:128])))

    def s4_block(m, b, axis):
        o = 448 * (m - 1) + 64 * (b // 2)
        return _cat([s4[o + 128 * i:o + 128 * i + 64, _lanes(b % 2)] for i in range(3)], axis)

    def krow(j, par):
        return 128 * (2 * j + 1 + par) if j < NP3 else FM * par

    def prep_p4():
        for j in range(7):
            p4[0, 64 * j:64 * (j + 1), :] = pltpu.bitcast(w4b[krow(j, 0):krow(j, 0) + 128, 0:128], u32)
            if j < NP3:
                p4[1, 64 * j:64 * (j + 1), :] = pltpu.bitcast(w4b[krow(j, 1):krow(j, 1) + 128, 0:128], u32)
            else:
                p4[1, 64 * j:64 * j + 32, :] = pltpu.bitcast(w4b[FM:F, 0:128], u32)
                p4[1, 64 * j + 32:64 * (j + 1), :] = jnp.zeros((32, 128), u32)

    def prep_w4():
        def block(j, b):
            if j == NP3 and b >= 2:
                return _cat([both(w4b, FM, F, b % 2), jnp.zeros((64, 256), f32)], 0)
            return both(w4b, krow(j, b // 2), krow(j, b // 2) + 128, b % 2)

        for m in [int(t) for t in OUTER['r4']]:
            k = {1: 0, 4: 2, 2: None, 3: 1, 5: None, 7: 4, 6: 3}[m]
            for j in range(7):
                o = 448 * (m - 1) + 64 * j
                if k is None and (j < NP3 or m == 2):
                    par = 0 if m == 2 else 1
                    for n in range(2):
                        s4[o:o + 64, _lanes(n)] = pltpu.bitcast(
                            w4b[krow(j, par):krow(j, par) + 128, _lanes(2 * n + 1 + par)], u32)
                else:
                    s4[o:o + 64, :] = _pk(block(j, 3) if k is None else _rhs_sum(k, lambda b: block(j, b)))
            for k2 in (2, 1, 0, 4, 3):
                o = 64 * (5 * (m - 1) + k2)
                s5[o:o + 64, :] = _pk(_rhs_sum(k2, lambda b: _ub(s4_block(m, b, -1)).astype(f32)))

    def prep_t4():
        eye = (jax.lax.broadcasted_iota(i32, (128, 128), 0)
               == jax.lax.broadcasted_iota(i32, (128, 128), 1)).astype(f32).astype(bf16)
        if TX:
            def tile(j, par):
                r0 = 128 * (2 * j + 1 + par) if j < NP3 else FM * par
                if j == NP3 and par:
                    return _cat([w4b[FM:F, 0:128].astype(f32), jnp.zeros((64, 128), f32)], 0).T
                return w4b[r0:r0 + 128, 0:128].astype(f32).T
            wt = [_cat([tile(j, par) for j in range(7)]) for par in range(2)]
        else:
            wt = [_nt(eye, _ub(p4[par])) for par in range(2)]
        for m, k in ((1, 0), (2, None), (3, 1), (4, 2), (5, None), (6, 3), (7, 4)):
            def blk(b):
                return wt[b // 2][64 * (b % 2):64 * (b % 2 + 1)]
            t4[32 * (m - 1):32 * m, :] = _pk(blk(0 if m == 2 else 3) if k is None else _rhs_sum(k, blk))

    def w4_tile0_steps(r):
        mm = {}
        for t in TORD:
            m = int(t)
            left = _cat([al[64 * j:64 * (j + 1), _lanes(m - 1)] for j in range(7)])
            mm[m] = _nt(_ub(t4[32 * (m - 1):32 * m, :]), _ub(left))
            if len(mm) == 7:
                c11 = ((mm[4] - mm[5]) + mm[1]) + mm[7]
                c22 = ((mm[3] - mm[2]) + mm[1]) + mm[6]
                finish(r, H, _cat([c11, mm[3] + mm[5]], 0).T, 0)
                finish(r + H, H, _cat([mm[4] + mm[2], c22], 0).T, 0)
            yield

    def finish(r, n, h, c):
        c0, c1 = 128 * c, 128 * (c + 1)
        x1 = hss[rows(r, n), c0:c1]
        base = x2s[rows(r, n), c0:c1] + mvec(4, n, c0, c1) * x1
        ob[rows(r, n), c0:c1] = (base + mvec(5, n, c0, c1) * h).astype(bf16)
        if ctx[0] == "z":
            send(r, n, c)

    def w4_plain(r, o=0, n=T):
        def left(k):
            return _cat([al[64 * j:64 * (j + 1), _lanes(k)] for j in range(7)])

        a = _cat([_cat([left(2), left(7)]), _cat([left(8), left(3)])], 0)[o // 2:(o + n) // 2]
        finish(r + o, n, _nn(_ub(a), _ub(_cat([p4[0], p4[1]], 0))), 0)

    def w4_product(m, ahead, order=None):
        def blk(b):
            o = 64 * (b % 2) + 32 * (b // 2)
            return _ub(_cat([al[o + 128 * i:o + 128 * i + 32, _lanes(m - 1)] for i in range(3)]))

        if ahead:
            asum = [_ub(_cat([a2[32 * (3 * (m - 1) + i):32 * (3 * (m - 1) + i + 1), _lanes(k)] for i in range(3)]))
                    for k in range(5)]
        else:
            asum = _lhs_sums(*[blk(b).astype(f32) for b in range(4)])
        bsum = [_ub(_cat([s5[64 * (5 * (m - 1) + k):64 * (5 * (m - 1) + k + 1), _lanes(i)] for i in range(3)], 0))
                for k in range(5)]
        ox = 448 * (m - 1) + 384
        q = _strassen(_nn, blk(0), blk(3), asum, _ub(al[384:416, _lanes(m - 1)]), _ub(al[416:448, _lanes(m - 1)]),
                      _ub(s4_block(m, 0, 0)), _ub(s4_block(m, 3, 0)), bsum,
                      _ub(s4[ox:ox + 64, _lanes(0)]), _ub(s4[ox:ox + 64, _lanes(1)]), ORD[ctx[0] + "_4"])
        return _cat([_cat(q[0:2]), _cat(q[2:4])], 0)

    def w4_steps(r, ahead):
        acc = [c2.at[H * i:H * (i + 1), :] for i in range(4)]

        def finish2(rr, h, c):
            finish(rr, H, h[:, 0:128], c)
            finish(rr, H, h[:, 128:256], c + 2)

        sign = {1: (1, 0, 0, 1), 2: (0, 0, 1, -1), 3: (0, 1, 0, 1), 4: (1, 0, 1, 0), 5: (-1, 1, 0, 0),
                6: (0, 0, 0, 1), 7: (1, 0, 0, 0)}
        left_n, state = [4, 2, 2, 4], [None] * 4
        for m in [int(t) for t in OUTER[ctx[0]]]:
            x = w4_product(m, ahead)
            outs = [i for i in range(4) if sign[m][i]]
            olds = {i: None if state[i] is None else state[i][0][...] for i in outs}
            busy = [state[i][0] for i in range(4) if state[i] is not None and i not in outs]
            free = [a for a in acc if not any(a is b for b in busy)]
            shared = None
            for i in outs:
                sg = sign[m][i]
                left_n[i] -= 1
                if state[i] is None:
                    if shared is None:
                        shared = free.pop()
                        shared[...] = x
                    state[i] = (shared, sg)
                    continue
                v = olds[i] + x if (sg > 0) == (state[i][1] > 0) else (x - olds[i] if sg > 0 else olds[i] - x)
                if left_n[i] == 0:
                    finish2(r + H * (i // 2), v, 1 + i % 2)
                    state[i] = None
                else:
                    dst = free.pop()
                    dst[...] = v
                    state[i] = (dst, 1)
            yield

    def up(order, ahead, r1=None, n1=None):
        for tok in order:
            if tok == "e":
                w3_edge()
            elif tok in "xyz":
                w3_pairs(ahead, ["xyz".index(tok)])
            elif tok == "1":
                mm_w1(r1, n1)
            elif tok == "c":
                ln_chain(r1, n1, paired=PAIRED)

    groups = list(range(0, P0 + P1, RG))
    wait([q_copies[0]])
    sa, ca, ga = mod_part(0, 1)
    modb[0] = ga * sa
    modb[1] = ga * (1.0 + ca)
    for c in range(NL, CT):
        mac_inv(c, NB - 1)
    st1 = {o: _stats(load_q(o)) for o in groups}
    zt[0:8, 0:128] = jnp.zeros((8, 128), u32)
    st2 = {}
    for o in groups:
        x2 = make_x2(o, load_q(o), st1[o])
        x2s[o:o + RG, :] = x2
        st2[o] = _stats(x2)

    wait([mod_copies[1]])
    sb, cb = mod_part(1, 2)
    modb[2] = sb
    modb[3] = 1.0 + cb
    st3 = {}
    for o in range(0, P0, RG):
        h2 = make_h2(x2s[o:o + RG, :], st2[o])
        h2s[o:o + RG, :] = h2
        st3[o] = _stats(h2, scaled=True)
    for o in range(0, P0, RG):
        zt[o // 2:(o + RG) // 2, :] = _pk((h2s[o:o + RG, :] - st3[o][0]) * st3[o][1])

    wait([w_copies[0]])
    prep_square(w1b, w1p, s1)
    z0 = _ub(zt[0:P0 // 2, :])
    h1 = _gelu_scaled(_nn(z0, _ub(w1p[:, 0:512])))
    for c in range(CT - 1):
        h1s[c][8:8 + P0, :] = h1[:, _lanes(c)]
    for o in range(0, P0, P0 // 4):
        h1s[CT - 1][8 + o:8 + o + P0 // 4, :] = _gelu_scaled(_nn(z0[o:o + P0 // 4], _ub(w1p[:, 512:D])))
    prev = None
    for o1 in range(0, P1 // 2, RG):
        zz = []
        for o in (P0 + o1, P0 + o1 + P1 // 2):
            h2 = make_h2(x2s[o:o + RG, :], st2[o])
            h2s[o:o + RG, :] = h2
            st = _stats(h2, prev, True, True)
            z = (h2 - st[0]) * st[1]
            zt[o // 2:(o + RG) // 2, :] = _pk(z)
            prev = st[1]
            zz.append(z)
        put_sums(zu, o1, zz[0], zz[1])
    mm_w1(P0, P1, P0)

    ctx[0] = "r2"
    wait([w_copies[1], q_copies[1]])
    prep_square(w2b, w2p, s2)
    ln_chain(P0 + P1, PA, paired=R2M)
    mm_w2(0)
    ln_x1(0, R2L)
    mm_w2(T)

    ctx[0] = "r3"
    wait([w_copies[2]])
    prep_w3()
    early = ln_x1(T, stats_only=True) if SE else None
    up(R3O, True, P0 + P1, PA)

    ctx[0] = "r4"
    if FEN4:
        jax.lax.fori_loop(0, 2, fence, 0)
    wait([w_copies[3], mod_copies[2]])
    prep_w4()
    sc16 = jnp.broadcast_to(scb[:, 0:D], (16, D)).astype(bf16)
    steps, h, j = w4_steps(0, True), None, 0
    if TP0:
        prep_t4()
        tile0 = w4_tile0_steps(0)
    for tok in R4O:
        if tok == "p" and TP0:
            next(tile0)
        elif tok == "T" and TP0:
            pass
        elif tok == "p":
            blk = [al[64 * j:64 * (j + 1), _lanes(k)] for k in (2, 7, 8, 3)]
            w = _ub(_cat([p4[0, 64 * j:64 * (j + 1), :], p4[1, 64 * j:64 * (j + 1), :]], 0))
            d = [_nn(_ub(_cat(blk[0:2])), w), _nn(_ub(_cat(blk[2:4])), w)]
            h = d if h is None else [h[0] + d[0], h[1] + d[1]]
            j += 1
            if j == 7:
                finish(0, H, h[0], 0)
                finish(H, H, h[1], 0)
        elif tok == "s":
            next(steps)
        elif tok == "T":
            prep_t4()
        else:
            c0, c1 = (0, 384) if tok == "g" else (384, D)
            gb = jnp.dot(sc16, wmc[:, c0:c1], preferred_element_type=f32)[0:8]
            modb[4, :, c0:c1] = gb
            modb[5, :, c0:c1] = (0.5 / ALPHA) * gb
    ln_x1(T, stats=early)
    out_copy(0).start()
    q_copies[2].wait()

    def mlp_body(i, carry):
        r1 = pl.multiple_of(PB - PC + PC * i, 32)
        r = pl.multiple_of(i * T, T)
        up(HEAD, False, r1, PC)
        steps, tile0 = w4_steps(r, False), w4_tile0_steps(r)
        for tok in BODY:
            if tok == "1":
                mm_w1(r1, PC)
            elif tok == "p":
                next(tile0)
            elif tok == "2":
                mm_w2(r + T)
            elif tok == "l":
                ln_x1(r + T, LM)
            else:
                next(steps)
        out_copy(i).start()
        return carry

    ctx[0] = "l"
    jax.lax.fori_loop(1, NC - 1, mlp_body, 0)

    ctx[0] = "z"
    up(ZO, True)
    if TZ:
        steps, tile0 = w4_steps(S - T, True), w4_tile0_steps(S - T)
        for tok in ZB:
            next(steps if tok == "s" else tile0)
    else:
        prep_p4()
        w4_plain(S - T, 0, LA)
        for _ in w4_steps(S - T, True):
            pass
        if LAST0 > LA:
            w4_plain(S - T, LA, LAST0 - LA)
        w4_plain(S - T, LAST0, T - LAST0)
    for i in range(NC - 1):
        out_copy(i).wait()
    for cp in out_tail:
        cp.wait()


@jax.jit
def pallas_adaLN_cond__ssm_conv_h3__mixer_s_mlp__prompt_kernel(
    A_q: jax.Array,
    A_k: jax.Array,
    A_v: jax.Array,
    A_shift_k: jax.Array,
    A_ssm_k: jax.Array,
    A_ssm_D: jax.Array,
    B_x: jax.Array,
    B_w1: jax.Array,
    B_w2: jax.Array,
    B_w3: jax.Array,
    B_w4: jax.Array,
    c: jax.Array,
    w_mod: jax.Array,
):
    del B_x
    any_spec = pl.BlockSpec(memory_space=pl.ANY)

    def tile_view(x):
        return x.reshape(S // 8, 8, CT, 128).transpose(0, 2, 1, 3).reshape(S * CT, 128)

    vm = pltpu.VMEM
    dma = pltpu.SemaphoreType.DMA
    spec = (4, NG, 16, 128)
    out = pl.pallas_call(
        _kernel,
        in_specs=[any_spec] * 12,
        out_specs=any_spec,
        out_shape=jax.ShapeDtypeStruct((S, D), bf16),
        scratch_shapes=[
            *[vm((KROWS, 128), bf16)] * NB, *[vm((VROWS, 128), bf16)] * NB, vm((CT, 128, S), bf16),
            vm((S, D), bf16), vm((D, D), bf16), vm((D, D), bf16), vm((F, D), bf16), vm((F, D), bf16),
            vm((D // 2, D), u32), vm((D // 2, D), u32), vm((F // 2, D), u32),
            vm((D, 3 * D), bf16), vm((D, 2 * D), bf16), vm((D, D), bf16),
            vm((4, D), bf16), vm((D,), bf16), vm((1, D), bf16), vm((1, 1792), f32),
            vm((4, 128, 128), u32), vm((4, 128, 128), u32), vm((4, 64, 256), u32),
            vm((CT, 8, 8, 128), f32),
            vm((CT, NB) + spec, f32), vm((CT, NB - 1) + spec, f32), vm((CT,) + spec, f32),
            vm((CT, NB) + spec, f32), vm((4, 128, 128), f32),
            vm((CT, S + 32, 128), f32), vm((8, 8, D), f32),
            *[vm((S + 32, 128), f32)] * CT, vm((S, D), f32), vm((S, D), f32), vm((S, D), f32),
            vm((288, D), u32), vm((5, H // 2, 256), u32), vm((H, D), u32), vm((5, H // 2, 256), u32),
            vm((64, 256), u32), vm((D, 256), u32), vm((D, 256), u32), vm((NP3 * 64, 1280), u32),
            vm((7 * 448, 256), u32), vm((35 * 64, 384), u32), vm((2, 448, 128), u32),
            vm((7 * 64, 1152), u32), vm((21 * 32, 640), u32), vm((4 * H, 256), f32), vm((7 * 32, 896), u32), vm((64, 1280), u32),
            vm((S, D), bf16),
            dma((26,)), dma((NC + 10,)),
        ],
        compiler_params=pltpu.CompilerParams(vmem_limit_bytes=110 << 20, disable_bounds_checks=True,
                                             disable_semaphore_checks=True),
    )(A_q.reshape(S, D), tile_view(A_k), tile_view(A_v), A_shift_k.T, A_ssm_k,
      A_ssm_D, B_w1, B_w2, B_w3.T, B_w4, c, w_mod)
    return out.reshape(1, S, D)
```

```python
import numpy as np
import jax
import jax.numpy as jnp
import jax.experimental.pallas as pl
import jax.experimental.pallas.tpu as pltpu

f32, bf16, u32, i32 = jnp.float32, jnp.bfloat16, jnp.uint32, jnp.int32

S, D, F = 2048, 640, 1728
CT = D // 128
TR = 8 * CT
NB, BLK, NFFT = 4, 512, 1024
KROWS, VROWS = BLK * CT + 128, BLK * CT + 64
NG = 16
T = 256
NC = S // T
H = T // 2
NP3 = 6
FM = (F // 128) * 128
P0, P1, PA, PC = 320, 224, 160, 224
PB = P0 + P1 + PA
LA, LAST0 = 96, 208
RG = 16
EPS = 1e-5
NT_DIMS = (((1,), (1,)), ((), ()))
PAIRED = "10000100001000"
ORD = {"r1_1": "4235a1c76db", "r2_2": "d7b24ac3156", "r3_1": "1576b432acd", "r3_3": "c24a5173b6d",
       "r3_e": "23bc451a76d", "r3_0": "345217ba6cd", "r4_4": "5b12a47dc63", "l_1": "7325bad4c61",
       "l_2": "5164d2ac7b3", "l_3": "4bc51a7d236", "l_4": "243ac571b6d", "l_e": "24bcd35176a",
       "l_0": "acbd2351746", "z_3": "b5c231a47d6", "z_4": "c35d12b74a6", "z_e": "cd1237ab465",
       "z_0": "acd231b4576"}
OUTER = {"r4": "1723645", "l": "5132647", "z": "1523467"}
BODY = "1pp2sslpsspspspps"
HEAD = "cxeyz"
LM = "0000000000100000"
R2M = "0010101010"
R2L = "1010100010101010"
R3O = "1eyzx"
R4O = "gsssGpspspppspps"
ZO = "xeyz"
FA = 3
TORD = "7621354"
AHEAD = {"r3": "111", "r4": "111", "l": "000", "z": "110"}
GV = 8
NL = 4


def _lo(w):
    return pltpu.bitcast(w << 16, f32)


def _hi(w):
    return pltpu.bitcast(w & jnp.uint32(0xFFFF0000), f32)


def _cis(n):
    t = (n & (2 * NFFT - 1)).astype(f32) * (np.pi / NFFT)
    return jnp.cos(t), jnp.sin(t)


def _fwd_table(r):
    g = jax.lax.broadcasted_iota(i32, (NG, 128), 0)
    cg, sg = _cis(jnp.where(g < NG // 2, 32 * g + 1, 32 * g - 253) * r)
    cs, ss = _cis(4 * jax.lax.broadcasted_iota(i32, (8, 128), 0) * r)
    parts = []
    for i in range(NG):
        c, s = cg[i:i + 1], sg[i:i + 1]
        parts += [c * cs - s * ss, -(s * cs + c * ss)]
    return pltpu.bitcast(jnp.concatenate(parts, axis=0).astype(bf16), u32)


def _inv_tables():
    def phase(rows):
        col = jax.lax.broadcasted_iota(i32, (rows, 256), 1)
        k = ((col >> 4) << 3) + (col & 7)
        row = jax.lax.broadcasted_iota(i32, (rows, 256), 0)
        return jnp.where(k < 64, 4 * k + 1, 4 * k - 253), (col & 8) << 6, row

    fr, _, g = phase(16)
    cg, sg = _cis(fr * (32 * g))
    fr, off, s = phase(8)
    out = []
    for p in range(4):
        cs, ss = _cis(fr * (4 * s + p) + off)
        cs, ss = cs * (2.0 / NFFT), ss * (2.0 / NFFT)
        parts = [cg[i:i + 1] * cs - sg[i:i + 1] * ss for i in range(16)]
        out.append(pltpu.bitcast(jnp.concatenate(parts, axis=0).astype(bf16), u32))
    return out


def _radix4(re, im, inverse):
    ar, ai = re[0] + re[2], im[0] + im[2]
    br, bi = re[0] - re[2], im[0] - im[2]
    cr, ci = re[1] + re[3], im[1] + im[3]
    dr, di = re[1] - re[3], im[1] - im[3]
    minus_i = (br + di, bi - dr)
    plus_i = (br - di, bi + dr)
    if inverse:
        return [(ar + cr, ai + ci), plus_i, (ar - cr, ai - ci), minus_i]
    return [(ar + cr, ai + ci), minus_i, (ar - cr, ai - ci), plus_i]


def _stats(x, link=None, early=False, scaled=False):
    zero = 0.0 if link is None else jnp.minimum(link, 0.0)
    part = x[:, 0:128]
    for c in range(1, CT):
        part = part + x[:, c * 128:(c + 1) * 128]
    if link is not None and early:
        part = part + zero
        zero = 0.0
    m = jnp.sum(part, axis=-1, keepdims=True) * (1.0 / D)
    v = jnp.maximum(jnp.sum(x * x, axis=-1, keepdims=True) * (1.0 / D) - m * m, zero)
    e = jnp.log(v + EPS) * (-0.5 / np.log(2.0))
    return m, jnp.exp2(e + np.log2(ALPHA) if scaled else e)


GC = 0.7978845608028654
ALPHA = (GC * 0.044715) ** (1.0 / 3.0)


def _gelu_scaled(y):
    return y + y * jnp.tanh(y * (y * y + GC / ALPHA))


def _pk(x):
    return pltpu.bitcast(x.astype(bf16), u32)


def _ub(x):
    return pltpu.bitcast(x, bf16)


def _cat(xs, axis=-1):
    return jnp.concatenate(xs, axis=axis)


def _lanes(k):
    return slice(128 * k, 128 * (k + 1))


def _nn(a, w):
    return jnp.dot(a.astype(bf16), w, preferred_element_type=f32)


def _nt(a, w):
    return jax.lax.dot_general(a, w, NT_DIMS, preferred_element_type=f32)


def _lhs_sums(a11, a12, a21, a22):
    return [a11 + a22, a21 + a22, a11 + a12, a21 - a11, a12 - a22]


def _rhs_sum(k, block):
    a, b, plus = [(0, 3, True), (1, 3, False), (2, 0, False), (0, 1, True), (2, 3, True)][k]
    return block(a) + block(b) if plus else block(a) - block(b)


def _strassen(dot, a11, a22, asum, ax1, ax2, b11, b22, bsum, bx1, bx2, order, xdot=None):
    ops = {"1": (asum[0], bsum[0], (1, 0, 0, 1)), "2": (asum[1], b11, (0, 0, 1, -1)),
           "3": (a11, bsum[1], (0, 1, 0, 1)), "4": (a22, bsum[2], (1, 0, 1, 0)),
           "5": (asum[2], b22, (-1, 1, 0, 0)), "6": (asum[3], bsum[3], (0, 0, 0, 1)),
           "7": (asum[4], bsum[4], (1, 0, 0, 0)), "a": (ax1, bx1, (1, 0, 0, 0)),
           "b": (ax1, bx2, (0, 1, 0, 0)), "c": (ax2, bx1, (0, 0, 1, 0)), "d": (ax2, bx2, (0, 0, 0, 1))}
    c, neg = [None] * 4, [None] * 4
    for t in order:
        a, b, sg = ops[t]
        m = (xdot if xdot and t in "abcd" else dot)(a, b)
        for i in range(4):
            if sg[i] > 0:
                c[i] = m if c[i] is None else c[i] + m
                if neg[i] is not None:
                    c[i], neg[i] = c[i] - neg[i], None
            elif sg[i] < 0:
                if c[i] is None:
                    neg[i] = m
                else:
                    c[i] = c[i] - m
    return c


def _kernel(q_hbm, k_hbm, v_hbm, sh_hbm, sk_hbm, d_hbm, w1_hbm, w2_hbm, w3_hbm, w4_hbm,
            c_hbm, wm_hbm, o_hbm,
            kb0, kb1, kb2, kb3, vb0, vb1, vb2, vb3, skb, qb, w1b, w2b, w3b, w4b, w1p, w2p, w3p,
            wma, wmb, wmc, shb, db, cb_, scb,
            fub, fkb, gtb, par, US, KS, UR, YS, YP, ys, modb, h10, h11, h12, h13, h14, h2s, x2s, x1s,
            zt, zu, zb, zs, w3n, s1, s2, s3, s4, s5, p4, al, a2, c2, t4, e3, ob,
            sem, sem_o):
    h1s = [h10, h11, h12, h13, h14]
    n_in = [0]

    def load(src, dst):
        n_in[0] += 1
        return pltpu.make_async_copy(src, dst, sem.at[n_in[0] - 1])

    nkv = BLK * CT
    small = [load(d_hbm, db), load(sh_hbm, shb), load(c_hbm, cb_)]
    sk_copies = [load(sk_hbm.at[pl.ds(c * 128, 128), :], skb.at[c]) for c in range(CT)]
    kbs, vbs, wms = [kb0, kb1, kb2, kb3], [vb0, vb1, vb2, vb3], [wma, wmb, wmc]
    kv_copies = [[load(k_hbm.at[pl.ds(a * nkv, nkv), :], kbs[a].at[pl.ds(TR, nkv), :]),
                  load(v_hbm.at[pl.ds(a * nkv, nkv), :], vbs[a].at[pl.ds(0, nkv), :])] for a in range(NB)]
    mod_cols = [(0, 3 * D), (3 * D, 2 * D), (5 * D, D)]
    mod_copies = [load(wm_hbm.at[:, pl.ds(o, n)], w) for (o, n), w in zip(mod_cols, wms)]
    w_copies = [load(w1_hbm, w1b), load(w2_hbm, w2b), load(w3_hbm, w3b), load(w4_hbm, w4b)]
    q_copies = [load(q_hbm.at[pl.ds(o, n), :], qb.at[pl.ds(o, n), :])
                for o, n in [(0, P0 + P1), (P0 + P1, PA), (PB, S - PB)]]

    def out_copy(i):
        r = i * T if isinstance(i, int) else pl.multiple_of(i * T, T)
        return pltpu.make_async_copy(ob.at[pl.ds(r, T), :], o_hbm.at[pl.ds(r, T), :], sem_o.at[i])

    out_tail = []

    def send(r, n, c):
        cp = pltpu.make_async_copy(ob.at[pl.ds(r, n), pl.ds(128 * c, 128)], o_hbm.at[pl.ds(r, n), pl.ds(128 * c, 128)],
                                   sem_o.at[NC - 1 + len(out_tail)])
        out_tail.append(cp)
        cp.start()

    for cp in (small + kv_copies[0] + sk_copies + kv_copies[1] + kv_copies[2] + kv_copies[3]
               + [mod_copies[0], q_copies[0], mod_copies[1], w_copies[0], w_copies[1], q_copies[1],
                  w_copies[2], w_copies[3], mod_copies[2], q_copies[2]]):
        cp.start()

    def wait(copies):
        for cp in copies:
            cp.wait()

    def pin(i, carry):
        z = jnp.zeros((8, 128), f32)
        scb[:, pl.ds(pl.multiple_of(i * 128, 128), 128)] = z[0:1]
        YP[i, 0:8, :] = z
        US[i, 0, 0, 0, 0:8, :] = z
        KS[i, 0, 0, 0, 0:8, :] = z
        YS[i, 0, 0, 0, 0:8, :] = z
        UR[i, 0, 0, 0:8, :] = z
        r8 = pl.ds(pl.multiple_of(i * 8, 8), 8)
        c2[r8, 0:128] = z
        al[r8, 0:128] = jnp.zeros((8, 128), u32)
        a2[r8, 0:128] = jnp.zeros((8, 128), u32)
        return carry

    def fence(i, carry):
        YP[i, 0:8, :] = jnp.zeros((8, 128), f32)
        return carry

    jax.lax.fori_loop(0, 2, pin, 0)
    lane = jax.lax.broadcasted_iota(i32, (1, 128), 1)
    for p in range(4):
        m = (lane - p) & 3
        fkb[p] = _fwd_table(128 * m + ((lane - m) & 127))
    for c in range(CT):
        kb0[c * 8:(c + 1) * 8, :] = jnp.zeros((8, 128), bf16)
        h1s[c][0:8, :] = jnp.zeros((8, 128), f32)
        h1s[c][S + 8:S + 16, :] = jnp.zeros((8, 128), f32)
    for a in range(NB):
        kbs[a][nkv + TR:KROWS, :] = jnp.zeros((KROWS - nkv - TR, 128), bf16)
        vbs[a][nkv:VROWS, :] = jnp.zeros((VROWS - nkv, 128), bf16)
    for p in range(4):
        fub[p] = _fwd_table(8 * (lane & 63) + ((lane >> 6) << 2) + p)
    wait(small)
    cvec = cb_[...].astype(f32)
    scb[:, 0:D] = cvec * jax.nn.sigmoid(cvec)
    dv = db[...].astype(f32).reshape(1, D)
    shv = shb[...].astype(f32)
    for c in range(CT):
        for i in range(4):
            par[c, i] = jnp.broadcast_to(shv[i:i + 1, c * 128:(c + 1) * 128], (8, 128))
        par[c, 4] = jnp.broadcast_to(dv[:, c * 128:(c + 1) * 128], (8, 128))
    for p, tab in enumerate(_inv_tables()):
        gtb[p] = tab

    def get(ref, idx, g, n):
        return (ref[idx + (slice(g, g + n), slice(0, 8))], ref[idx + (slice(g, g + n), slice(8, 16))])

    def put(ref, idx, g, n, xr, xi):
        ref[idx + (slice(g, g + n), slice(0, 8))] = xr
        ref[idx + (slice(g, g + n), slice(8, 16))] = xi

    def split(tt, g, n):
        tt = [t[g * 16:(g + n) * 16].reshape(n, 16, 128) for t in tt]
        return [t[:, 0:8] for t in tt], [t[:, 8:16] for t in tt]

    def fwd_k(c, j):
        lane = jax.lax.broadcasted_iota(i32, (64, 128), 1)
        even = (lane & 1) == 0
        l01 = (lane & 2) == 0
        l12 = ((lane + 3) & 2) == 0
        rm = []
        for m in range(4):
            w = pltpu.bitcast(skb[c, :, (4 * j + m) * 128:(4 * j + m + 1) * 128], u32)
            rm.append(pltpu.roll(w, m, 1) if m else w)
        e01 = jnp.where(even, rm[0], rm[1])
        o01 = jnp.where(even, rm[1], rm[0])
        e23 = jnp.where(even, rm[2], rm[3])
        o23 = jnp.where(even, rm[3], rm[2])
        kp = [jnp.where(l01, e01, e23), jnp.where(l12, o01, o23),
              jnp.where(l01, e23, e01), jnp.where(l12, o23, o01)]
        tt = [jax.lax.dot_general(pltpu.bitcast(fkb[p], bf16), pltpu.bitcast(kp[p], bf16), NT_DIMS,
                                  preferred_element_type=f32) for p in range(4)]
        for g in range(0, NG, GV):
            re, im = split(tt, g, GV)
            if j == 0:
                re[0] = re[0] + par[c, 4][None]
            for m, (xr, xi) in enumerate(_radix4(re, im, False)):
                if j < NB - 1:
                    put(KS, (c, j, m), g, GV, xr, xi)
                ur, ui = get(US, (c, 0, m), g, GV)
                put(YS, (c, j, m), g, GV, xr * ur - xi * ui, xr * ui + xi * ur)

    def fwd_u(c, a):
        taps = [jnp.tile(par[c, i], (8, 1)) for i in range(4)]
        ws = TR // 2
        base = 4 * c
        kw, vw = kbs[a].bitcast(u32), vbs[a].bitcast(u32)

        def words(ref, start):
            return ref[pl.ds(start, BLK // 8, stride=ws), :]

        kk = {}
        for w in range(4):
            x = words(kw, ws + base + w)
            kk[2 * w], kk[2 * w + 1] = _lo(x), _hi(x)
        kk[-3] = _hi(words(kw, base + 2))
        x = words(kw, base + 3)
        kk[-2], kk[-1] = _lo(x), _hi(x)
        sub = []
        for w in range(4):
            x = words(vw, base + w)
            for r, vv in ((2 * w, _lo(x)), (2 * w + 1, _hi(x))):
                sh = taps[0] * kk[r] + taps[1] * kk[r - 1] + taps[2] * kk[r - 2] + taps[3] * kk[r - 3]
                sub.append(sh * vv)
        kv = [jnp.concatenate([sub[p], sub[p + 4]], axis=0) for p in range(4)]
        tt = [jnp.dot(pltpu.bitcast(fub[p], bf16), kv[p].astype(bf16), preferred_element_type=f32)
              for p in range(4)]
        for g in range(0, NG, GV):
            re, im = split(tt, g, GV)
            for m, (xr, xi) in enumerate(_radix4(re, im, False)):
                if a:
                    pr, pi = get(US, (c, 0, m), g, GV) if a == 1 else get(UR, (c, m), g, GV)
                    if a < NB - 1:
                        put(UR, (c, m), g, GV, xr, xi)
                    xr, xi = (xr - pi, xi + pr) if g < NG // 2 else (xr + pi, xi - pr)
                put(US, (c, a, m), g, GV, xr, xi)

    def mac_inv(c, a):
        for h in range(2):
            vals = [[] for _ in range(4)]
            for g in range(8 * h, 8 * h + 8, GV):
                yre, yim = [], []
                for m in range(4):
                    yr, yi = get(YS, (c, a, m), g, GV)
                    for j in range(a):
                        kr, ki = get(KS, (c, j, m), g, GV)
                        ur, ui = get(US, (c, a - j, m), g, GV)
                        yr = yr + (kr * ur - ki * ui)
                        yi = yi + (kr * ui + ki * ur)
                    yre.append(yr)
                    yim.append(yi)
                for p, (pr, pi) in enumerate(_radix4(yre, yim, True)):
                    vals[p].append(jnp.concatenate([pr, pi], axis=1))
            for p in range(4):
                pb = jnp.concatenate(vals[p], axis=0).reshape(128, 128).astype(bf16)
                r = jnp.dot(pltpu.bitcast(gtb[p, :, h * 128:(h + 1) * 128], bf16), pb,
                            preferred_element_type=f32)
                if h == 0:
                    YP[p] = r
                else:
                    ys[c, pl.ds(a * BLK + p, 128, stride=4), :] = YP[p] + r

    wait(kv_copies[0])
    for c in range(CT):
        fwd_u(c, 0)
    for grp in ((0,), (1, 2), (3, 4)):
        wait([sk_copies[c] for c in grp])
        for c in grp:
            for j in (3, 2, 1, 0):
                fwd_k(c, j)
    for a in range(1, NB):
        if a == FA:
            jax.lax.fori_loop(0, 2, fence, 0)
        wait(kv_copies[a])
        for c in range(CT):
            kbs[a][c * 8:(c + 1) * 8, :] = kbs[a - 1][nkv + c * 8:nkv + (c + 1) * 8, :]
        for c in range(CT):
            fwd_u(c, a)
            mac_inv(c, a - 1)
    wait([mod_copies[0]])
    for c in range(NL):
        mac_inv(c, NB - 1)

    def mod_part(part, extra):
        n, wm = mod_cols[part][1], wms[part]
        act = scb[:, 0:D]

        def sc(k0, k1):
            return jnp.broadcast_to(act[:, k0:k1], (16, k1 - k0)).astype(bf16)

        e = 128 * extra
        r = jnp.dot(sc(0, D), wm[:, e:n], preferred_element_type=f32)
        r0 = (jnp.dot(sc(0, D - 64), wm[0:D - 64, 0:e], preferred_element_type=f32)
              + jnp.dot(sc(D - 64, D), wm[D - 64:D, 0:e], preferred_element_type=f32))
        r = jnp.concatenate([r0, r], axis=-1)[0:8]
        return [r[:, i * D:(i + 1) * D] for i in range(n // D)]

    def mvec(i, n=RG, c0=0, c1=D):
        return jnp.tile(modb[i, :, c0:c1], (n // 8, 1))

    rows = pl.ds
    ctx = ["r1"]

    def load_q(r, ref=qb):
        return ref[rows(r, RG), :].astype(f32)

    def make_x2(r, q, st, ref=ys):
        y = _cat([ref[c, rows(r, RG), :] for c in range(CT)])
        return q + (((q - st[0]) * st[1]) * mvec(1) + mvec(0)) * y

    def make_h2(x2, st):
        return ((x2 - st[0]) * st[1]) * mvec(3) + mvec(2)

    def put_sums(ref, o, z1, z2):
        for k, v in enumerate(_lhs_sums(z1[:, 0:256], z1[:, 256:512], z2[:, 0:256], z2[:, 256:512])):
            ref.at[k][o // 2:(o + RG) // 2, :] = _pk(v)

    def ln_chain(r, n, paired):
        qv, yv = qb.at[rows(r, n), :], ys.at[:, rows(r, n), :]
        xv, hv = x2s.at[rows(r, n), :], h2s.at[rows(r, n), :]
        prev, pend, cnt = None, None, 0
        for o1 in range(0, n // 2, RG):
            zz = []
            for o in (o1, o1 + n // 2):
                q = load_q(o, qv)
                x2 = make_x2(o, q, _stats(q, prev), yv)
                xv[o:o + RG, :] = x2
                st = _stats(x2)
                h2 = make_h2(xv[o:o + RG, :], st)
                hv[o:o + RG, :] = h2
                st = _stats(h2, scaled=True)
                z = (hv[o:o + RG, :] - st[0]) * st[1]
                zt[o // 2:(o + RG) // 2, :] = _pk(z)
                zz.append(z)
                if paired[cnt] == "1":
                    pend = st[1]
                elif pend is not None:
                    prev, pend = jnp.minimum(st[1], pend), None
                else:
                    prev = st[1]
                cnt += 1
            put_sums(zu, o1, zz[0], zz[1])

    def ln_x1(r, paired="", stats=None, stats_only=False):
        sv = x1s.at[rows(r, T), :]
        prev, pend, cnt, out = None, None, 0, []
        for o1 in range(0, H, RG):
            zz = []
            for o in (o1, o1 + H):
                x1 = sv[o:o + RG, :]
                st = _stats(x1, prev, True, True) if stats is None else stats[cnt]
                out.append(st)
                if not stats_only:
                    z = (x1 - st[0]) * st[1]
                    zb[o // 2:(o + RG) // 2, :] = _pk(z)
                    zz.append(z)
                if paired and paired[cnt] == "1":
                    pend = st[1]
                elif pend is not None:
                    prev, pend = jnp.minimum(st[1], pend), None
                else:
                    prev = st[1]
                cnt += 1
            if not stats_only:
                put_sums(zs, o1, zz[0], zz[1])
        return out

    def both(ref, r0, r1, col):
        return _cat([ref[r0:r1, _lanes(1 + col)].astype(f32), ref[r0:r1, _lanes(3 + col)].astype(f32)])

    def prep_square(wb, wp, sw):
        wp[...] = pltpu.bitcast(wb[...], u32)
        for k in (2, 1, 0, 4, 3):
            sw[128 * k:128 * (k + 1), :] = _pk(_rhs_sum(
                k, lambda b: both(wb, 256 * (b // 2), 256 * (b // 2 + 1), b % 2)))

    def mm_square(a, top, bot, asum, wp, sw, which):
        h = top.shape[0]
        c0 = _nn(a, _ub(wp[:, 0:128]))
        out = [(c0[0:h], c0[h:2 * h])]
        for n in range(2):
            l1, l2 = _lanes(2 * n + 1), _lanes(2 * n + 2)
            q = _strassen(_nn, top[:, 0:256], bot[:, 256:512], asum, top[:, 512:D], bot[:, 512:D],
                          _ub(wp[0:128, l1]), _ub(wp[128:256, l2]),
                          [_ub(sw[128 * k:128 * (k + 1), _lanes(n)]) for k in range(5)],
                          _ub(wp[256:320, l1]), _ub(wp[256:320, l2]), ORD[ctx[0] + "_" + which])
            out += [(q[0], q[2]), (q[1], q[3])]
        return out

    def mm_w1(r, n, o=0):
        h, o = n // 2, o // 2
        res = mm_square(_ub(zt[o:o + h, :]), _ub(zt[o:o + h // 2, :]), _ub(zt[o + h // 2:o + h, :]),
                        [_ub(zu[k, 0:h // 2, :]) for k in range(5)], w1p, s1, "1")
        for c, (top, bot) in enumerate(res):
            h1s[c][rows(r + 8, h), :] = _gelu_scaled(top)
            h1s[c][rows(r + 8 + h, h), :] = _gelu_scaled(bot)

    def mm_w2(r):
        lane = jax.lax.broadcasted_iota(i32, (T, 128), 1)

        def sh(k, c):
            return h1s[c][rows(r + 8 + k, T), :]

        g = _cat([sh(-1, 0),
                  jnp.where(lane < 32, sh(-1, 1), sh(1, 1)),
                  jnp.where(lane < 64, sh(1, 2), sh(-2, 2)),
                  jnp.where(lane < 96, sh(-2, 3), sh(2, 3)),
                  sh(2, 4)])
        top, bot = g[0:H], g[H:T]
        sums = _lhs_sums(top[:, 0:256], top[:, 256:512], bot[:, 0:256], bot[:, 256:512])
        for c, (ct, cb) in enumerate(mm_square(g, top, bot, sums, w2p, s2, "2")):
            x1s[rows(r, H), _lanes(c)] = h2s[rows(r, H), _lanes(c)] + ct * (0.5 / ALPHA)
            x1s[rows(r + H, H), _lanes(c)] = h2s[rows(r + H, H), _lanes(c)] + cb * (0.5 / ALPHA)

    def prep_w3():
        for j in range(NP3):
            r0 = 128 * (2 * j + 1)
            w3p[r0 // 2:r0 // 2 + 64, 0:256] = pltpu.bitcast(w3b[r0:r0 + 128, 0:256], u32)
            w3p[r0 // 2:r0 // 2 + 64, 512:D] = pltpu.bitcast(w3b[r0:r0 + 128, 512:D], u32)
            w3p[r0 // 2 + 64:r0 // 2 + 128, 256:D] = pltpu.bitcast(w3b[r0 + 128:r0 + 256, 256:D], u32)
        w3p[0:64, :] = pltpu.bitcast(w3b[0:128, :], u32)
        w3p[FM // 2:F // 2, :] = pltpu.bitcast(w3b[FM:F, :], u32)
        w3n[0:64, :] = _pk(_cat([w3b[128:256, 512:D].astype(f32).T, w3b[256:384, 512:D].astype(f32).T]))

        def edge(b):
            c = slice(256 * (b // 2), 256 * (b // 2 + 1))
            if b % 2 == 0:
                return w3b[0:96, c].astype(f32)
            return _cat([w3b[96:128, c].astype(f32), w3b[FM:F, c].astype(f32)], 0)

        for k in (2, 1, 0, 4, 3):
            e3[0:48, 256 * k:256 * (k + 1)] = _pk(_rhs_sum(k, edge))
        for j in range(NP3):
            r0 = 128 * (2 * j + 1)
            for k in (2, 1, 0, 4, 3):
                s3[64 * j:64 * (j + 1), 256 * k:256 * (k + 1)] = _pk(_rhs_sum(k, lambda b: w3b[
                    r0 + 128 * (b % 2):r0 + 128 * (b % 2 + 1), 256 * (b // 2):256 * (b // 2 + 1)].astype(f32)))

    def w3_edge():
        def second(c0, c1):
            return _ub(_cat([w3p[48:64, c0:c1], w3p[FM // 2:F // 2, c0:c1]], 0))

        z1, z2 = _ub(zb[0:H // 2, :]), _ub(zb[H // 2:H, :])
        q = _strassen(lambda a, b: _nt(b, a), z1[:, 0:256], z2[:, 256:512], [_ub(zs[k]) for k in range(5)],
                      z1[:, 512:D], z2[:, 512:D], _ub(w3p[0:48, 0:256]), second(256, 512),
                      [_ub(e3[0:48, 256 * k:256 * (k + 1)]) for k in range(5)],
                      _ub(w3p[0:48, 512:D]), second(512, D), ORD[ctx[0] + "_e"])
        q = [_gelu_scaled(c) for c in q]
        out = []
        for x in (_cat(q[0:2], 0), _cat(q[2:4], 0)):
            out += [x[0:128].T, _cat([x[128:192], jnp.zeros((64, 128), f32)], 0).T]
        put_quads(NP3, out)

    def w3_pair(j):
        e, o = slice(64 * (2 * j + 1), 64 * (2 * j + 2)), slice(64 * (2 * j + 2), 64 * (2 * j + 3))
        z1, z2 = _ub(zb[0:H // 2, :]), _ub(zb[H // 2:H, :])
        q = _strassen(_nt, z1[:, 0:256], z2[:, 256:512], [_ub(zs[k]) for k in range(5)], z1[:, 512:D], z2[:, 512:D],
                      _ub(w3p[e, 0:256]), _ub(w3p[o, 256:512]),
                      [_ub(s3[64 * j:64 * (j + 1), 256 * k:256 * (k + 1)]) for k in range(5)],
                      *([_ub(w3n[0:64, 0:128]), _ub(w3n[0:64, 128:256]), ORD[ctx[0] + "_0"], _nn] if j == 0 else
                        [_ub(w3p[e, 512:D]), _ub(w3p[o, 512:D]), ORD[ctx[0] + "_3"]]))
        return [_gelu_scaled(c) for c in q]

    def plain_ctx():
        return ctx[0] == "z"

    def put_quads(j, q):
        l1, l2, l5, l6, l7 = _lhs_sums(*q)
        if not plain_ctx():
            al[64 * j:64 * (j + 1), 0:896] = _pk(_cat([l1, l2, q[0], q[3], l5, l6, l7]))
        else:
            al[64 * j:64 * (j + 1), :] = _pk(_cat([l1, l2, q[0], q[3], l5, l6, l7, q[1], q[2]]))

    def w3_pairs(i):
        ahead = AHEAD[ctx[0]][i] == "1"
        ops = []
        for j in (2 * i, 2 * i + 1):
            q = w3_pair(j)
            if not ahead:
                put_quads(j, q)
            ops.append(q)
        if not ahead:
            return
        for n, q in enumerate(ops):
            l1, l2, l5, l6, l7 = _lhs_sums(*q)
            ops[n] = [l1, l2, q[0], q[3], l5, l6, l7]
            j, half = 2 * i + n, slice(64 * n, 64 * (n + 1))
            if not plain_ctx():
                al[64 * j:64 * (j + 1), 0:896] = _pk(_cat(ops[n]))
                continue
            o = 64 * j + 32 * n
            al[o:o + 32, 0:256] = _pk(_cat([l1[half], l2[half]]))
            al[o:o + 32, 512:896] = _pk(_cat([l5[half], l6[half], l7[half]]))
            al[64 * j:64 * (j + 1), 256:512] = _pk(_cat([q[0], q[3]]))
            al[64 * j:64 * (j + 1), 896:1152] = _pk(_cat([q[1], q[2]]))
        for m in range(7):
            e, o = ops[0][m], ops[1][m]
            r0 = 32 * (3 * m + i)
            a2[r0:r0 + 32, :] = _pk(_cat(_lhs_sums(e[0:64], o[0:64], e[64:128], o[64:128])))

    def s4_block(m, b, axis):
        o = 448 * (m - 1) + 64 * (b // 2)
        return _cat([s4[o + 128 * i:o + 128 * i + 64, _lanes(b % 2)] for i in range(3)], axis)

    def krow(j, par):
        return 128 * (2 * j + 1 + par) if j < NP3 else FM * par

    def prep_p4():
        for j in range(7):
            p4[0, 64 * j:64 * (j + 1), :] = pltpu.bitcast(w4b[krow(j, 0):krow(j, 0) + 128, 0:128], u32)
            if j < NP3:
                p4[1, 64 * j:64 * (j + 1), :] = pltpu.bitcast(w4b[krow(j, 1):krow(j, 1) + 128, 0:128], u32)
            else:
                p4[1, 64 * j:64 * j + 32, :] = pltpu.bitcast(w4b[FM:F, 0:128], u32)
                p4[1, 64 * j + 32:64 * (j + 1), :] = jnp.zeros((32, 128), u32)

    def prep_w4():
        def block(j, b):
            if j == NP3 and b >= 2:
                return _cat([both(w4b, FM, F, b % 2), jnp.zeros((64, 256), f32)], 0)
            return both(w4b, krow(j, b // 2), krow(j, b // 2) + 128, b % 2)

        for m in [int(t) for t in OUTER['r4']]:
            k = {1: 0, 4: 2, 2: None, 3: 1, 5: None, 7: 4, 6: 3}[m]
            for j in range(7):
                o = 448 * (m - 1) + 64 * j
                if k is None and (j < NP3 or m == 2):
                    par = 0 if m == 2 else 1
                    for n in range(2):
                        s4[o:o + 64, _lanes(n)] = pltpu.bitcast(
                            w4b[krow(j, par):krow(j, par) + 128, _lanes(2 * n + 1 + par)], u32)
                else:
                    s4[o:o + 64, :] = _pk(block(j, 3) if k is None else _rhs_sum(k, lambda b: block(j, b)))
            for k2 in (2, 1, 0, 4, 3):
                o = 64 * (5 * (m - 1) + k2)
                s5[o:o + 64, :] = _pk(_rhs_sum(k2, lambda b: _ub(s4_block(m, b, -1)).astype(f32)))

    def prep_t4():
        def tile(j, par):
            if j == NP3 and par:
                return _cat([w4b[FM:F, 0:128].astype(f32), jnp.zeros((64, 128), f32)], 0).T
            return w4b[krow(j, par):krow(j, par) + 128, 0:128].astype(f32).T

        wt = [_cat([tile(j, par) for j in range(7)]) for par in range(2)]
        for m, k in ((1, 0), (2, None), (3, 1), (4, 2), (5, None), (6, 3), (7, 4)):
            def blk(b):
                return wt[b // 2][64 * (b % 2):64 * (b % 2 + 1)]
            t4[32 * (m - 1):32 * m, :] = _pk(blk(0 if m == 2 else 3) if k is None else _rhs_sum(k, blk))

    def w4_tile0_steps(r):
        mm = {}
        for t in TORD:
            m = int(t)
            left = _cat([al[64 * j:64 * (j + 1), _lanes(m - 1)] for j in range(7)])
            mm[m] = _nt(_ub(t4[32 * (m - 1):32 * m, :]), _ub(left))
            if len(mm) == 7:
                c11 = ((mm[4] - mm[5]) + mm[1]) + mm[7]
                c22 = ((mm[3] - mm[2]) + mm[1]) + mm[6]
                finish(r, H, _cat([c11, mm[3] + mm[5]], 0).T, 0)
                finish(r + H, H, _cat([mm[4] + mm[2], c22], 0).T, 0)
            yield

    def finish(r, n, h, c):
        c0, c1 = 128 * c, 128 * (c + 1)
        x1 = x1s[rows(r, n), c0:c1]
        base = x2s[rows(r, n), c0:c1] + mvec(4, n, c0, c1) * x1
        ob[rows(r, n), c0:c1] = (base + mvec(5, n, c0, c1) * h).astype(bf16)
        if ctx[0] == "z":
            send(r, n, c)

    def w4_plain(r, o=0, n=T):
        def left(k):
            return _cat([al[64 * j:64 * (j + 1), _lanes(k)] for j in range(7)])

        a = _cat([_cat([left(2), left(7)]), _cat([left(8), left(3)])], 0)[o // 2:(o + n) // 2]
        finish(r + o, n, _nn(_ub(a), _ub(_cat([p4[0], p4[1]], 0))), 0)

    def w4_product(m):
        def blk(b, grp=range(3)):
            o = 64 * (b % 2) + 32 * (b // 2)
            return _ub(_cat([al[o + 128 * i:o + 128 * i + 32, _lanes(m - 1)] for i in grp]))

        pre = [i for i in range(3) if AHEAD[ctx[0]][i] == "1"]
        now = [i for i in range(3) if i not in pre]
        asum = [[] for _ in range(5)]
        if pre:
            for k in range(5):
                asum[k].append((pre, _ub(_cat([a2[32 * (3 * (m - 1) + i):32 * (3 * (m - 1) + i + 1), _lanes(k)]
                                               for i in pre]))))
        if now:
            for k, v in enumerate(_lhs_sums(*[blk(b, now).astype(f32) for b in range(4)])):
                asum[k].append((now, v))

        def dot(a, w):
            if not isinstance(a, list):
                return _nn(a, w)
            parts = [_nn(v, w if len(grp) == 3 else _cat([w[128 * i:128 * (i + 1)] for i in grp], 0)) for grp, v in a]
            return parts[0] if len(parts) == 1 else parts[0] + parts[1]

        bsum = [_ub(_cat([s5[64 * (5 * (m - 1) + k):64 * (5 * (m - 1) + k + 1), _lanes(i)] for i in range(3)], 0))
                for k in range(5)]
        ox = 448 * (m - 1) + 384
        q = _strassen(dot, blk(0), blk(3), asum, _ub(al[384:416, _lanes(m - 1)]), _ub(al[416:448, _lanes(m - 1)]),
                      _ub(s4_block(m, 0, 0)), _ub(s4_block(m, 3, 0)), bsum,
                      _ub(s4[ox:ox + 64, _lanes(0)]), _ub(s4[ox:ox + 64, _lanes(1)]), ORD[ctx[0] + "_4"])
        return _cat([_cat(q[0:2]), _cat(q[2:4])], 0)

    def w4_steps(r):
        acc = [c2.at[H * i:H * (i + 1), :] for i in range(4)]

        def finish2(rr, h, c):
            finish(rr, H, h[:, 0:128], c)
            finish(rr, H, h[:, 128:256], c + 2)

        sign = {1: (1, 0, 0, 1), 2: (0, 0, 1, -1), 3: (0, 1, 0, 1), 4: (1, 0, 1, 0), 5: (-1, 1, 0, 0),
                6: (0, 0, 0, 1), 7: (1, 0, 0, 0)}
        left_n, state = [4, 2, 2, 4], [None] * 4
        for m in [int(t) for t in OUTER[ctx[0]]]:
            x = w4_product(m)
            outs = [i for i in range(4) if sign[m][i]]
            olds = {i: None if state[i] is None else state[i][0][...] for i in outs}
            busy = [state[i][0] for i in range(4) if state[i] is not None and i not in outs]
            free = [a for a in acc if not any(a is b for b in busy)]
            shared = None
            for i in outs:
                sg = sign[m][i]
                left_n[i] -= 1
                if state[i] is None:
                    if shared is None:
                        shared = free.pop()
                        shared[...] = x
                    state[i] = (shared, sg)
                    continue
                v = olds[i] + x if (sg > 0) == (state[i][1] > 0) else (x - olds[i] if sg > 0 else olds[i] - x)
                if left_n[i] == 0:
                    finish2(r + H * (i // 2), v, 1 + i % 2)
                    state[i] = None
                else:
                    dst = free.pop()
                    dst[...] = v
                    state[i] = (dst, 1)
            yield

    def up(order, r1=None, n1=None):
        for tok in order:
            if tok == "e":
                w3_edge()
            elif tok in "xyz":
                w3_pairs("xyz".index(tok))
            elif tok == "1":
                mm_w1(r1, n1)
            elif tok == "c":
                ln_chain(r1, n1, paired=PAIRED)

    groups = list(range(0, P0 + P1, RG))
    wait([q_copies[0]])
    sa, ca, ga = mod_part(0, 1)
    modb[0] = ga * sa
    modb[1] = ga * (1.0 + ca)
    for c in range(NL, CT):
        mac_inv(c, NB - 1)
    st1 = {o: _stats(load_q(o)) for o in groups}
    zt[0:8, 0:128] = jnp.zeros((8, 128), u32)
    st2 = {}
    for o in groups:
        x2 = make_x2(o, load_q(o), st1[o])
        x2s[o:o + RG, :] = x2
        st2[o] = _stats(x2)

    wait([mod_copies[1]])
    sb, cb = mod_part(1, 2)
    modb[2] = sb
    modb[3] = 1.0 + cb
    st3 = {}
    for o in range(0, P0, RG):
        h2 = make_h2(x2s[o:o + RG, :], st2[o])
        h2s[o:o + RG, :] = h2
        st3[o] = _stats(h2, scaled=True)
    for o in range(0, P0, RG):
        zt[o // 2:(o + RG) // 2, :] = _pk((h2s[o:o + RG, :] - st3[o][0]) * st3[o][1])

    wait([w_copies[0]])
    prep_square(w1b, w1p, s1)
    z0 = _ub(zt[0:P0 // 2, :])
    h1 = _gelu_scaled(_nn(z0, _ub(w1p[:, 0:512])))
    for c in range(CT - 1):
        h1s[c][8:8 + P0, :] = h1[:, _lanes(c)]
    for o in range(0, P0, P0 // 4):
        h1s[CT - 1][8 + o:8 + o + P0 // 4, :] = _gelu_scaled(_nn(z0[o:o + P0 // 4], _ub(w1p[:, 512:D])))
    prev = None
    for o1 in range(0, P1 // 2, RG):
        zz = []
        for o in (P0 + o1, P0 + o1 + P1 // 2):
            h2 = make_h2(x2s[o:o + RG, :], st2[o])
            h2s[o:o + RG, :] = h2
            st = _stats(h2, prev, True, True)
            z = (h2 - st[0]) * st[1]
            zt[o // 2:(o + RG) // 2, :] = _pk(z)
            prev = st[1]
            zz.append(z)
        put_sums(zu, o1, zz[0], zz[1])
    mm_w1(P0, P1, P0)

    ctx[0] = "r2"
    wait([w_copies[1], q_copies[1]])
    prep_square(w2b, w2p, s2)
    ln_chain(P0 + P1, PA, paired=R2M)
    mm_w2(0)
    ln_x1(0, R2L)
    mm_w2(T)

    ctx[0] = "r3"
    wait([w_copies[2]])
    prep_w3()
    early = ln_x1(T, stats_only=True)
    up(R3O, P0 + P1, PA)

    ctx[0] = "r4"
    jax.lax.fori_loop(0, 2, fence, 0)
    wait([w_copies[3], mod_copies[2]])
    prep_w4()
    sc16 = jnp.broadcast_to(scb[:, 0:D], (16, D)).astype(bf16)
    prep_t4()
    steps, tile0 = w4_steps(0), w4_tile0_steps(0)
    for tok in R4O:
        if tok == "p":
            next(tile0)
        elif tok == "s":
            next(steps)
        else:
            c0, c1 = (0, 384) if tok == "g" else (384, D)
            gb = jnp.dot(sc16, wmc[:, c0:c1], preferred_element_type=f32)[0:8]
            modb[4, :, c0:c1] = gb
            modb[5, :, c0:c1] = (0.5 / ALPHA) * gb
    ln_x1(T, stats=early)
    out_copy(0).start()
    q_copies[2].wait()

    def mlp_body(i, carry):
        r1 = pl.multiple_of(PB - PC + PC * i, 32)
        r = pl.multiple_of(i * T, T)
        up(HEAD, r1, PC)
        steps, tile0 = w4_steps(r), w4_tile0_steps(r)
        for tok in BODY:
            if tok == "1":
                mm_w1(r1, PC)
            elif tok == "p":
                next(tile0)
            elif tok == "2":
                mm_w2(r + T)
            elif tok == "l":
                ln_x1(r + T, LM)
            else:
                next(steps)
        out_copy(i).start()
        return carry

    ctx[0] = "l"
    jax.lax.fori_loop(1, NC - 1, mlp_body, 0)

    ctx[0] = "z"
    up(ZO)
    prep_p4()
    w4_plain(S - T, 0, LA)
    for _ in w4_steps(S - T):
        pass
    w4_plain(S - T, LA, LAST0 - LA)
    w4_plain(S - T, LAST0, T - LAST0)
    for i in range(NC - 1):
        out_copy(i).wait()
    for cp in out_tail:
        cp.wait()


@jax.jit
def pallas_adaLN_cond__ssm_conv_h3__mixer_s_mlp__prompt_kernel(
    A_q: jax.Array,
    A_k: jax.Array,
    A_v: jax.Array,
    A_shift_k: jax.Array,
    A_ssm_k: jax.Array,
    A_ssm_D: jax.Array,
    B_x: jax.Array,
    B_w1: jax.Array,
    B_w2: jax.Array,
    B_w3: jax.Array,
    B_w4: jax.Array,
    c: jax.Array,
    w_mod: jax.Array,
):
    del B_x
    any_spec = pl.BlockSpec(memory_space=pl.ANY)

    def tile_view(x):
        return x.reshape(S // 8, 8, CT, 128).transpose(0, 2, 1, 3).reshape(S * CT, 128)

    vm = pltpu.VMEM
    dma = pltpu.SemaphoreType.DMA
    spec = (4, NG, 16, 128)
    out = pl.pallas_call(
        _kernel,
        in_specs=[any_spec] * 12,
        out_specs=any_spec,
        out_shape=jax.ShapeDtypeStruct((S, D), bf16),
        scratch_shapes=[
            *[vm((KROWS, 128), bf16)] * NB, *[vm((VROWS, 128), bf16)] * NB, vm((CT, 128, S), bf16),
            vm((S, D), bf16), vm((D, D), bf16), vm((D, D), bf16), vm((F, D), bf16), vm((F, D), bf16),
            vm((D // 2, D), u32), vm((D // 2, D), u32), vm((F // 2, D), u32),
            vm((D, 3 * D), bf16), vm((D, 2 * D), bf16), vm((D, D), bf16),
            vm((4, D), bf16), vm((D,), bf16), vm((1, D), bf16), vm((1, 1792), f32),
            vm((4, 128, 128), u32), vm((4, 128, 128), u32), vm((4, 64, 256), u32),
            vm((CT, 8, 8, 128), f32),
            vm((CT, NB) + spec, f32), vm((CT, NB - 1) + spec, f32), vm((CT,) + spec, f32),
            vm((CT, NB) + spec, f32), vm((4, 128, 128), f32),
            vm((CT, S + 32, 128), f32), vm((8, 8, D), f32),
            *[vm((S + 32, 128), f32)] * CT, vm((S, D), f32), vm((S, D), f32), vm((S, D), f32),
            vm((288, D), u32), vm((5, H // 2, 256), u32), vm((H, D), u32), vm((5, H // 2, 256), u32),
            vm((64, 256), u32), vm((D, 256), u32), vm((D, 256), u32), vm((NP3 * 64, 1280), u32),
            vm((7 * 448, 256), u32), vm((35 * 64, 384), u32), vm((2, 448, 128), u32),
            vm((7 * 64, 1152), u32), vm((21 * 32, 640), u32), vm((4 * H, 256), f32), vm((7 * 32, 896), u32), vm((64, 1280), u32),
            vm((S, D), bf16),
            dma((26,)), dma((NC + 10,)),
        ],
        compiler_params=pltpu.CompilerParams(vmem_limit_bytes=110 << 20, disable_bounds_checks=True,
                                             disable_semaphore_checks=True),
    )(A_q.reshape(S, D), tile_view(A_k), tile_view(A_v), A_shift_k.T, A_ssm_k,
      A_ssm_D, B_w1, B_w2, B_w3.T, B_w4, c, w_mod)
    return out.reshape(1, S, D)
```

```python
import numpy as np
import jax
import jax.numpy as jnp
import jax.experimental.pallas as pl
import jax.experimental.pallas.tpu as pltpu

f32, bf16, u32, i32 = jnp.float32, jnp.bfloat16, jnp.uint32, jnp.int32

S, D, F = 2048, 640, 1728
CT = D // 128
TR = 8 * CT
NB, BLK, NFFT = 4, 512, 1024
KROWS, VROWS = BLK * CT + 128, BLK * CT + 64
NG = 16
T = 256
NC = S // T
H = T // 2
NP3 = 6
FM = (F // 128) * 128
P0, P1, PA, PC = 320, 224, 160, 224
PB = P0 + P1 + PA
LA, LAST0 = 96, 208
RG = 16
EPS = 1e-5
NT_DIMS = (((1,), (1,)), ((), ()))
PAIRED = "10000100001000"
ORD = {"r1_1": "4235ba16cd7", "r1_0": "4c5213db7a6", "r2_2": "d274c3ab156", "r3_1": "576b432acd1",
       "r3_3": "c245a173b6d", "r3_e": "32bca41d576", "r3_0": "345217ba6cd", "r4_4": "5b21a74dc63",
       "l_1": "7ba325cd461", "l_2": "45c1627ab3d", "l_3": "4bc51a7d236", "l_4": "243ac571b6d",
       "l_e": "24bdc35176a", "l_0": "acbd2351746", "z_3": "b5c231a47d6", "z_4": "c35d12b74a6",
       "z_e": "6cd3127ab45", "z_0": "acd231b4576"}
OUTER = {"r4": "2617345", "l": "5132647", "z": "1523467"}
BODY = "1pp2sslpsspspspps"
HEAD = "xecyz"
LM = "0000000000100000"
R2M = "0010101010"
R2L = "1010100010101010"
R3O = "1ezyx"
R4O = "sgGpspspspsppsps"
SE = 2
ZO = "xeyz"
FEN4 = 1
FA = 3
TORD = "7621354"
TP0 = 1
TX = 1
TZ = 0
ZB = "ppsspspspspsps"
AHEAD = {"r3": "111", "r4": "111", "l": "000", "z": "110"}
S1 = 1
GV = 8
NL = 4


def _lo(w):
    return pltpu.bitcast(w << 16, f32)


def _hi(w):
    return pltpu.bitcast(w & jnp.uint32(0xFFFF0000), f32)


def _cis(n):
    t = (n & (2 * NFFT - 1)).astype(f32) * (np.pi / NFFT)
    return jnp.cos(t), jnp.sin(t)


def _fwd_table(r):
    g = jax.lax.broadcasted_iota(i32, (NG, 128), 0)
    cg, sg = _cis(jnp.where(g < NG // 2, 32 * g + 1, 32 * g - 253) * r)
    cs, ss = _cis(4 * jax.lax.broadcasted_iota(i32, (8, 128), 0) * r)
    parts = []
    for i in range(NG):
        c, s = cg[i:i + 1], sg[i:i + 1]
        parts += [c * cs - s * ss, -(s * cs + c * ss)]
    return pltpu.bitcast(jnp.concatenate(parts, axis=0).astype(bf16), u32)


def _inv_tables():
    def phase(rows):
        col = jax.lax.broadcasted_iota(i32, (rows, 256), 1)
        k = ((col >> 4) << 3) + (col & 7)
        row = jax.lax.broadcasted_iota(i32, (rows, 256), 0)
        return jnp.where(k < 64, 4 * k + 1, 4 * k - 253), (col & 8) << 6, row

    fr, _, g = phase(16)
    cg, sg = _cis(fr * (32 * g))
    fr, off, s = phase(8)
    out = []
    for p in range(4):
        cs, ss = _cis(fr * (4 * s + p) + off)
        cs, ss = cs * (2.0 / NFFT), ss * (2.0 / NFFT)
        parts = [cg[i:i + 1] * cs - sg[i:i + 1] * ss for i in range(16)]
        out.append(pltpu.bitcast(jnp.concatenate(parts, axis=0).astype(bf16), u32))
    return out


def _radix4(re, im, inverse):
    ar, ai = re[0] + re[2], im[0] + im[2]
    br, bi = re[0] - re[2], im[0] - im[2]
    cr, ci = re[1] + re[3], im[1] + im[3]
    dr, di = re[1] - re[3], im[1] - im[3]
    minus_i = (br + di, bi - dr)
    plus_i = (br - di, bi + dr)
    if inverse:
        return [(ar + cr, ai + ci), plus_i, (ar - cr, ai - ci), minus_i]
    return [(ar + cr, ai + ci), minus_i, (ar - cr, ai - ci), plus_i]


def _stats(x, link=None, early=False, scaled=False):
    zero = 0.0 if link is None else jnp.minimum(link, 0.0)
    part = x[:, 0:128]
    for c in range(1, CT):
        part = part + x[:, c * 128:(c + 1) * 128]
    if link is not None and early:
        part = part + zero
        zero = 0.0
    m = jnp.sum(part, axis=-1, keepdims=True) * (1.0 / D)
    v = jnp.maximum(jnp.sum(x * x, axis=-1, keepdims=True) * (1.0 / D) - m * m, zero)
    e = jnp.log(v + EPS) * (-0.5 / np.log(2.0))
    return m, jnp.exp2(e + np.log2(ALPHA) if scaled else e)


GC = 0.7978845608028654
ALPHA = (GC * 0.044715) ** (1.0 / 3.0)


def _gelu_scaled(y):
    return y + y * jnp.tanh(y * (y * y + GC / ALPHA))


def _pk(x):
    return pltpu.bitcast(x.astype(bf16), u32)


def _ub(x):
    return pltpu.bitcast(x, bf16)


def _cat(xs, axis=-1):
    return jnp.concatenate(xs, axis=axis)


def _lanes(k):
    return slice(128 * k, 128 * (k + 1))


def _nn(a, w):
    return jnp.dot(a.astype(bf16), w, preferred_element_type=f32)


def _nt(a, w):
    return jax.lax.dot_general(a, w, NT_DIMS, preferred_element_type=f32)


def _lhs_sums(a11, a12, a21, a22):
    return [a11 + a22, a21 + a22, a11 + a12, a21 - a11, a12 - a22]


def _rhs_sum(k, block):
    a, b, plus = [(0, 3, True), (1, 3, False), (2, 0, False), (0, 1, True), (2, 3, True)][k]
    return block(a) + block(b) if plus else block(a) - block(b)


def _strassen(dot, a11, a22, asum, ax1, ax2, b11, b22, bsum, bx1, bx2, order="", xdot=None):
    if order:
        ops = {"1": (asum[0], bsum[0], (1, 0, 0, 1)), "2": (asum[1], b11, (0, 0, 1, -1)),
               "3": (a11, bsum[1], (0, 1, 0, 1)), "4": (a22, bsum[2], (1, 0, 1, 0)),
               "5": (asum[2], b22, (-1, 1, 0, 0)), "6": (asum[3], bsum[3], (0, 0, 0, 1)),
               "7": (asum[4], bsum[4], (1, 0, 0, 0)), "a": (ax1, bx1, (1, 0, 0, 0)),
               "b": (ax1, bx2, (0, 1, 0, 0)), "c": (ax2, bx1, (0, 0, 1, 0)), "d": (ax2, bx2, (0, 0, 0, 1))}
        c, neg = [None] * 4, [None] * 4
        for t in order:
            a, b, sg = ops[t]
            m = (xdot if xdot and t in "abcd" else dot)(a, b)
            for i in range(4):
                if sg[i] > 0:
                    c[i] = m if c[i] is None else c[i] + m
                    if neg[i] is not None:
                        c[i], neg[i] = c[i] - neg[i], None
                elif sg[i] < 0:
                    if c[i] is None:
                        neg[i] = m
                    else:
                        c[i] = c[i] - m
        return c
    m2 = dot(asum[1], b11)
    m4 = dot(a22, bsum[2])
    c21 = (m4 + m2) + dot(ax2, bx1)
    m3 = dot(a11, bsum[1])
    m5 = dot(asum[2], b22)
    c12 = (m3 + m5) + dot(ax1, bx2)
    m1 = dot(asum[0], bsum[0])
    c11 = (((m4 - m5) + m1) + dot(asum[4], bsum[4])) + dot(ax1, bx1)
    c22 = (((m3 - m2) + m1) + dot(asum[3], bsum[3])) + dot(ax2, bx2)
    return [c11, c12, c21, c22]


def _kernel(q_hbm, k_hbm, v_hbm, sh_hbm, sk_hbm, d_hbm, w1_hbm, w2_hbm, w3_hbm, w4_hbm,
            c_hbm, wm_hbm, o_hbm,
            kb0, kb1, kb2, kb3, vb0, vb1, vb2, vb3, skb, qb, w1b, w2b, w3b, w4b, w1p, w2p, w3p,
            wma, wmb, wmc, shb, db, cb_, scb,
            fub, fkb, gtb, par, US, KS, UR, YS, YP, ys, modb, h10, h11, h12, h13, h14, h2s, x2s, hss,
            zt, zu, zb1, zs1, zb0, zs0, zu0, w3n, s1, s2, s3, s4, s5, p4, al, a2, c2, t4, e3, ob,
            sem, sem_o):
    h1s = [h10, h11, h12, h13, h14]
    n_in = [0]

    def load(src, dst):
        n_in[0] += 1
        return pltpu.make_async_copy(src, dst, sem.at[n_in[0] - 1])

    nkv = BLK * CT
    small = [load(d_hbm, db), load(sh_hbm, shb), load(c_hbm, cb_)]
    sk_copies = [load(sk_hbm.at[pl.ds(c * 128, 128), :], skb.at[c]) for c in range(CT)]
    kbs, vbs, wms = [kb0, kb1, kb2, kb3], [vb0, vb1, vb2, vb3], [wma, wmb, wmc]
    kv_copies = [[load(k_hbm.at[pl.ds(a * nkv, nkv), :], kbs[a].at[pl.ds(TR, nkv), :]),
                  load(v_hbm.at[pl.ds(a * nkv, nkv), :], vbs[a].at[pl.ds(0, nkv), :])] for a in range(NB)]
    mod_cols = [(0, 3 * D), (3 * D, 2 * D), (5 * D, D)]
    mod_copies = [load(wm_hbm.at[:, pl.ds(o, n)], w) for (o, n), w in zip(mod_cols, wms)]
    w_copies = [load(w1_hbm, w1b), load(w2_hbm, w2b), load(w3_hbm, w3b), load(w4_hbm, w4b)]
    q_copies = [load(q_hbm.at[pl.ds(o, n), :], qb.at[pl.ds(o, n), :])
                for o, n in [(0, P0 + P1), (P0 + P1, PA), (PB, S - PB)]]

    def out_copy(i):
        r = i * T if isinstance(i, int) else pl.multiple_of(i * T, T)
        return pltpu.make_async_copy(ob.at[pl.ds(r, T), :], o_hbm.at[pl.ds(r, T), :], sem_o.at[i])

    out_tail = []

    def send(r, n, c):
        cp = pltpu.make_async_copy(ob.at[pl.ds(r, n), pl.ds(128 * c, 128)], o_hbm.at[pl.ds(r, n), pl.ds(128 * c, 128)],
                                   sem_o.at[NC - 1 + len(out_tail)])
        out_tail.append(cp)
        cp.start()

    for cp in (small + kv_copies[0] + sk_copies + kv_copies[1] + kv_copies[2] + kv_copies[3]
               + [mod_copies[0], q_copies[0], mod_copies[1], w_copies[0], w_copies[1], q_copies[1],
                  w_copies[2], w_copies[3], mod_copies[2], q_copies[2]]):
        cp.start()

    def wait(copies):
        for cp in copies:
            cp.wait()

    def pin(i, carry):
        z = jnp.zeros((8, 128), f32)
        scb[:, pl.ds(pl.multiple_of(i * 128, 128), 128)] = z[0:1]
        YP[i, 0:8, :] = z
        US[i, 0, 0, 0, 0:8, :] = z
        KS[i, 0, 0, 0, 0:8, :] = z
        YS[i, 0, 0, 0, 0:8, :] = z
        UR[i, 0, 0, 0:8, :] = z
        r8 = pl.ds(pl.multiple_of(i * 8, 8), 8)
        c2[r8, 0:128] = z
        al[r8, 0:128] = jnp.zeros((8, 128), u32)
        zb0[r8, 0:128] = jnp.zeros((8, 128), u32)
        zs0[i, 0:8, 0:128] = jnp.zeros((8, 128), u32)
        zu0[i, 0:8, 0:128] = jnp.zeros((8, 128), u32)
        a2[r8, 0:128] = jnp.zeros((8, 128), u32)
        return carry

    def fence(i, carry):
        YP[i, 0:8, :] = jnp.zeros((8, 128), f32)
        return carry

    jax.lax.fori_loop(0, 2, pin, 0)
    lane = jax.lax.broadcasted_iota(i32, (1, 128), 1)
    for p in range(4):
        m = (lane - p) & 3
        fkb[p] = _fwd_table(128 * m + ((lane - m) & 127))
    for c in range(CT):
        kb0[c * 8:(c + 1) * 8, :] = jnp.zeros((8, 128), bf16)
        h1s[c][0:8, :] = jnp.zeros((8, 128), f32)
        h1s[c][S + 8:S + 16, :] = jnp.zeros((8, 128), f32)
    for a in range(NB):
        kbs[a][nkv + TR:KROWS, :] = jnp.zeros((KROWS - nkv - TR, 128), bf16)
        vbs[a][nkv:VROWS, :] = jnp.zeros((VROWS - nkv, 128), bf16)
    for p in range(4):
        fub[p] = _fwd_table(8 * (lane & 63) + ((lane >> 6) << 2) + p)
    wait(small)
    cvec = cb_[...].astype(f32)
    scb[:, 0:D] = cvec * jax.nn.sigmoid(cvec)
    dv = db[...].astype(f32).reshape(1, D)
    shv = shb[...].astype(f32)
    for c in range(CT):
        for i in range(4):
            par[c, i] = jnp.broadcast_to(shv[i:i + 1, c * 128:(c + 1) * 128], (8, 128))
        par[c, 4] = jnp.broadcast_to(dv[:, c * 128:(c + 1) * 128], (8, 128))
    for p, tab in enumerate(_inv_tables()):
        gtb[p] = tab

    def get(ref, idx, g, n):
        return (ref[idx + (slice(g, g + n), slice(0, 8))], ref[idx + (slice(g, g + n), slice(8, 16))])

    def put(ref, idx, g, n, xr, xi):
        ref[idx + (slice(g, g + n), slice(0, 8))] = xr
        ref[idx + (slice(g, g + n), slice(8, 16))] = xi

    def split(tt, g, n):
        tt = [t[g * 16:(g + n) * 16].reshape(n, 16, 128) for t in tt]
        return [t[:, 0:8] for t in tt], [t[:, 8:16] for t in tt]

    def fwd_k(c, j):
        lane = jax.lax.broadcasted_iota(i32, (64, 128), 1)
        even = (lane & 1) == 0
        l01 = (lane & 2) == 0
        l12 = ((lane + 3) & 2) == 0
        rm = []
        for m in range(4):
            w = pltpu.bitcast(skb[c, :, (4 * j + m) * 128:(4 * j + m + 1) * 128], u32)
            rm.append(pltpu.roll(w, m, 1) if m else w)
        e01 = jnp.where(even, rm[0], rm[1])
        o01 = jnp.where(even, rm[1], rm[0])
        e23 = jnp.where(even, rm[2], rm[3])
        o23 = jnp.where(even, rm[3], rm[2])
        kp = [jnp.where(l01, e01, e23), jnp.where(l12, o01, o23),
              jnp.where(l01, e23, e01), jnp.where(l12, o23, o01)]
        tt = [jax.lax.dot_general(pltpu.bitcast(fkb[p], bf16), pltpu.bitcast(kp[p], bf16), NT_DIMS,
                                  preferred_element_type=f32) for p in range(4)]
        for g in range(0, NG, GV):
            re, im = split(tt, g, GV)
            if j == 0:
                re[0] = re[0] + par[c, 4][None]
            for m, (xr, xi) in enumerate(_radix4(re, im, False)):
                if j < NB - 1:
                    put(KS, (c, j, m), g, GV, xr, xi)
                ur, ui = get(US, (c, 0, m), g, GV)
                put(YS, (c, j, m), g, GV, xr * ur - xi * ui, xr * ui + xi * ur)

    def fwd_u(c, a):
        taps = [jnp.tile(par[c, i], (8, 1)) for i in range(4)]
        ws = TR // 2
        base = 4 * c
        kw, vw = kbs[a].bitcast(u32), vbs[a].bitcast(u32)

        def words(ref, start):
            return ref[pl.ds(start, BLK // 8, stride=ws), :]

        kk = {}
        for w in range(4):
            x = words(kw, ws + base + w)
            kk[2 * w], kk[2 * w + 1] = _lo(x), _hi(x)
        kk[-3] = _hi(words(kw, base + 2))
        x = words(kw, base + 3)
        kk[-2], kk[-1] = _lo(x), _hi(x)
        sub = []
        for w in range(4):
            x = words(vw, base + w)
            for r, vv in ((2 * w, _lo(x)), (2 * w + 1, _hi(x))):
                sh = taps[0] * kk[r] + taps[1] * kk[r - 1] + taps[2] * kk[r - 2] + taps[3] * kk[r - 3]
                sub.append(sh * vv)
        kv = [jnp.concatenate([sub[p], sub[p + 4]], axis=0) for p in range(4)]
        tt = [jnp.dot(pltpu.bitcast(fub[p], bf16), kv[p].astype(bf16), preferred_element_type=f32)
              for p in range(4)]
        for g in range(0, NG, GV):
            re, im = split(tt, g, GV)
            for m, (xr, xi) in enumerate(_radix4(re, im, False)):
                if a:
                    pr, pi = get(US, (c, 0, m), g, GV) if a == 1 else get(UR, (c, m), g, GV)
                    if a < NB - 1:
                        put(UR, (c, m), g, GV, xr, xi)
                    xr, xi = (xr - pi, xi + pr) if g < NG // 2 else (xr + pi, xi - pr)
                put(US, (c, a, m), g, GV, xr, xi)

    def mac_inv(c, a):
        for h in range(2):
            vals = [[] for _ in range(4)]
            for g in range(8 * h, 8 * h + 8, GV):
                yre, yim = [], []
                for m in range(4):
                    yr, yi = get(YS, (c, a, m), g, GV)
                    for j in range(a):
                        kr, ki = get(KS, (c, j, m), g, GV)
                        ur, ui = get(US, (c, a - j, m), g, GV)
                        yr = yr + (kr * ur - ki * ui)
                        yi = yi + (kr * ui + ki * ur)
                    yre.append(yr)
                    yim.append(yi)
                for p, (pr, pi) in enumerate(_radix4(yre, yim, True)):
                    vals[p].append(jnp.concatenate([pr, pi], axis=1))
            for p in range(4):
                pb = jnp.concatenate(vals[p], axis=0).reshape(128, 128).astype(bf16)
                r = jnp.dot(pltpu.bitcast(gtb[p, :, h * 128:(h + 1) * 128], bf16), pb,
                            preferred_element_type=f32)
                if h == 0:
                    YP[p] = r
                else:
                    ys[c, pl.ds(a * BLK + p, 128, stride=4), :] = YP[p] + r

    wait(kv_copies[0])
    for c in range(CT):
        fwd_u(c, 0)
    for grp in ((0,), (1, 2), (3, 4)):
        wait([sk_copies[c] for c in grp])
        for c in grp:
            for j in (3, 2, 1, 0):
                fwd_k(c, j)
    for a in range(1, NB):
        if a == FA:
            jax.lax.fori_loop(0, 2, fence, 0)
        wait(kv_copies[a])
        for c in range(CT):
            kbs[a][c * 8:(c + 1) * 8, :] = kbs[a - 1][nkv + c * 8:nkv + (c + 1) * 8, :]
        for c in range(CT):
            fwd_u(c, a)
            mac_inv(c, a - 1)
    wait([mod_copies[0]])
    for c in range(NL):
        mac_inv(c, NB - 1)

    def mod_part(part, extra):
        n, wm = mod_cols[part][1], wms[part]
        act = scb[:, 0:D]

        def sc(k0, k1):
            return jnp.broadcast_to(act[:, k0:k1], (16, k1 - k0)).astype(bf16)

        e = 128 * extra
        r = jnp.dot(sc(0, D), wm[:, e:n], preferred_element_type=f32)
        r0 = (jnp.dot(sc(0, D - 64), wm[0:D - 64, 0:e], preferred_element_type=f32)
              + jnp.dot(sc(D - 64, D), wm[D - 64:D, 0:e], preferred_element_type=f32))
        r = jnp.concatenate([r0, r], axis=-1)[0:8]
        return [r[:, i * D:(i + 1) * D] for i in range(n // D)]

    def mvec(i, n=RG, c0=0, c1=D):
        return jnp.tile(modb[i, :, c0:c1], (n // 8, 1))

    rows = pl.ds
    ctx = ["r1"]

    def load_q(r, ref=qb):
        return ref[rows(r, RG), :].astype(f32)

    def make_x2(r, q, st, ref=ys):
        y = _cat([ref[c, rows(r, RG), :] for c in range(CT)])
        return q + (((q - st[0]) * st[1]) * mvec(1) + mvec(0)) * y

    def make_h2(x2, st):
        return ((x2 - st[0]) * st[1]) * mvec(3) + mvec(2)

    def put_sums(ref, o, z1, z2):
        for k, v in enumerate(_lhs_sums(z1[:, 0:256], z1[:, 256:512], z2[:, 0:256], z2[:, 256:512])):
            ref.at[k][o // 2:(o + RG) // 2, :] = _pk(v)

    def ln_chain(r, n, links=1, paired=""):
        qv, yv = qb.at[rows(r, n), :], ys.at[:, rows(r, n), :]
        xv, hv = x2s.at[rows(r, n), :], h2s.at[rows(r, n), :]
        prev, pend, cnt = [None] * links, None, 0
        for o1 in range(0, n // 2, RG):
            zz = []
            for o in (o1, o1 + n // 2):
                q = load_q(o, qv)
                x2 = make_x2(o, q, _stats(q, prev[cnt % links]), yv)
                xv[o:o + RG, :] = x2
                st = _stats(x2)
                h2 = make_h2(xv[o:o + RG, :], st)
                hv[o:o + RG, :] = h2
                st = _stats(h2, scaled=True)
                z = (hv[o:o + RG, :] - st[0]) * st[1]
                zt[o // 2:(o + RG) // 2, :] = _pk(z)
                zz.append(z)
                if paired and paired[cnt] == "1":
                    pend = st[1]
                elif pend is not None:
                    prev[0], pend = jnp.minimum(st[1], pend), None
                else:
                    prev[cnt % links] = st[1]
                cnt += 1
            put_sums(zu, o1, zz[0], zz[1])

    def ln_x1(r, paired="", stats=None, stats_only=False):
        zb, zs = (zb0, zs0) if ctx[0] == "r2" else (zb1, zs1)
        sv = hss.at[rows(r, T), :]
        prev, pend, cnt, out = None, None, 0, []
        for o1 in range(0, H, RG):
            zz = []
            for o in (o1, o1 + H):
                x1 = sv[o:o + RG, :]
                st = _stats(x1, prev, True, True) if stats is None else stats[cnt]
                out.append(st)
                if not stats_only:
                    z = (x1 - st[0]) * st[1]
                    zb[o // 2:(o + RG) // 2, :] = _pk(z)
                    zz.append(z)
                if paired and paired[cnt] == "1":
                    pend = st[1]
                elif pend is not None:
                    prev, pend = jnp.minimum(st[1], pend), None
                else:
                    prev = st[1]
                cnt += 1
            if not stats_only:
                put_sums(zs, o1, zz[0], zz[1])
        return out

    def both(ref, r0, r1, col):
        return _cat([ref[r0:r1, _lanes(1 + col)].astype(f32), ref[r0:r1, _lanes(3 + col)].astype(f32)])

    def prep_square(wb, wp, sw, full=False):
        if full:
            wp[...] = pltpu.bitcast(wb[...], u32)
        else:
            wp[:, 0:128] = pltpu.bitcast(wb[:, 0:128], u32)
            wp[256:320, 128:D] = pltpu.bitcast(wb[512:D, 128:D], u32)
            for n in range(2):
                wp[0:128, _lanes(2 * n + 1)] = pltpu.bitcast(wb[0:256, _lanes(2 * n + 1)], u32)
                wp[128:256, _lanes(2 * n + 2)] = pltpu.bitcast(wb[256:512, _lanes(2 * n + 2)], u32)
        for k in (2, 1, 0, 4, 3):
            sw[128 * k:128 * (k + 1), :] = _pk(_rhs_sum(
                k, lambda b: both(wb, 256 * (b // 2), 256 * (b // 2 + 1), b % 2)))

    def mm_square(a, top, bot, asum, wp, sw, which):
        h = top.shape[0]
        c0 = _nn(a, _ub(wp[:, 0:128]))
        out = [(c0[0:h], c0[h:2 * h])]
        for n in range(2):
            l1, l2 = _lanes(2 * n + 1), _lanes(2 * n + 2)
            q = _strassen(_nn, top[:, 0:256], bot[:, 256:512], asum, top[:, 512:D], bot[:, 512:D],
                          _ub(wp[0:128, l1]), _ub(wp[128:256, l2]),
                          [_ub(sw[128 * k:128 * (k + 1), _lanes(n)]) for k in range(5)],
                          _ub(wp[256:320, l1]), _ub(wp[256:320, l2]), ORD[ctx[0] + "_" + which])
            out += [(q[0], q[2]), (q[1], q[3])]
        return out

    def mm_w1(r, n, o=0, zu=zu, which="1"):
        h, o = n // 2, o // 2
        res = mm_square(_ub(zt[o:o + h, :]), _ub(zt[o:o + h // 2, :]), _ub(zt[o + h // 2:o + h, :]),
                        [_ub(zu[k, 0:h // 2, :]) for k in range(5)], w1p, s1, which)
        for c, (top, bot) in enumerate(res):
            h1s[c][rows(r + 8, h), :] = _gelu_scaled(top)
            h1s[c][rows(r + 8 + h, h), :] = _gelu_scaled(bot)

    def mm_w2(r):
        lane = jax.lax.broadcasted_iota(i32, (T, 128), 1)

        def sh(k, c):
            return h1s[c][rows(r + 8 + k, T), :]

        g = _cat([sh(-1, 0),
                  jnp.where(lane < 32, sh(-1, 1), sh(1, 1)),
                  jnp.where(lane < 64, sh(1, 2), sh(-2, 2)),
                  jnp.where(lane < 96, sh(-2, 3), sh(2, 3)),
                  sh(2, 4)])
        top, bot = g[0:H], g[H:T]
        sums = _lhs_sums(top[:, 0:256], top[:, 256:512], bot[:, 0:256], bot[:, 256:512])
        for c, (ct, cb) in enumerate(mm_square(g, top, bot, sums, w2p, s2, "2")):
            hss[rows(r, H), _lanes(c)] = h2s[rows(r, H), _lanes(c)] + ct * (0.5 / ALPHA)
            hss[rows(r + H, H), _lanes(c)] = h2s[rows(r + H, H), _lanes(c)] + cb * (0.5 / ALPHA)

    def prep_w3():
        for j in range(NP3):
            r0 = 128 * (2 * j + 1)
            w3p[r0 // 2:r0 // 2 + 64, 0:256] = pltpu.bitcast(w3b[r0:r0 + 128, 0:256], u32)
            if j:
                w3p[r0 // 2:r0 // 2 + 64, 512:D] = pltpu.bitcast(w3b[r0:r0 + 128, 512:D], u32)
            c1 = D if j else 512
            w3p[r0 // 2 + 64:r0 // 2 + 128, 256:c1] = pltpu.bitcast(w3b[r0 + 128:r0 + 256, 256:c1], u32)
        w3p[0:48, 0:256] = pltpu.bitcast(w3b[0:96, 0:256], u32)
        w3p[0:48, 512:D] = pltpu.bitcast(w3b[0:96, 512:D], u32)
        w3p[48:64, 256:D] = pltpu.bitcast(w3b[96:128, 256:D], u32)
        w3p[FM // 2:F // 2, 256:D] = pltpu.bitcast(w3b[FM:F, 256:D], u32)
        w3n[0:64, :] = _pk(_cat([w3b[128:256, 512:D].astype(f32).T, w3b[256:384, 512:D].astype(f32).T]))

        def edge(b):
            c = slice(256 * (b // 2), 256 * (b // 2 + 1))
            if b % 2 == 0:
                return w3b[0:96, c].astype(f32)
            return _cat([w3b[96:128, c].astype(f32), w3b[FM:F, c].astype(f32)], 0)

        for k in (2, 1, 0, 4, 3):
            e3[0:48, 256 * k:256 * (k + 1)] = _pk(_rhs_sum(k, edge))
        for j in range(NP3):
            r0 = 128 * (2 * j + 1)
            for k in (2, 1, 0, 4, 3):
                s3[64 * j:64 * (j + 1), 256 * k:256 * (k + 1)] = _pk(_rhs_sum(k, lambda b: w3b[
                    r0 + 128 * (b % 2):r0 + 128 * (b % 2 + 1), 256 * (b // 2):256 * (b // 2 + 1)].astype(f32)))

    def w3_edge():
        def second(c0, c1):
            return _ub(_cat([w3p[48:64, c0:c1], w3p[FM // 2:F // 2, c0:c1]], 0))

        zb, zs = (zb0, zs0) if ctx[0] == "r3" else (zb1, zs1)
        z1, z2 = _ub(zb[0:H // 2, :]), _ub(zb[H // 2:H, :])
        q = _strassen(lambda a, b: _nt(b, a), z1[:, 0:256], z2[:, 256:512], [_ub(zs[k]) for k in range(5)],
                      z1[:, 512:D], z2[:, 512:D], _ub(w3p[0:48, 0:256]), second(256, 512),
                      [_ub(e3[0:48, 256 * k:256 * (k + 1)]) for k in range(5)],
                      _ub(w3p[0:48, 512:D]), second(512, D), ORD[ctx[0] + "_e"])
        q = [_gelu_scaled(c) for c in q]
        out = []
        for x in (_cat(q[0:2], 0), _cat(q[2:4], 0)):
            out += [x[0:128].T, _cat([x[128:192], jnp.zeros((64, 128), f32)], 0).T]
        put_quads(NP3, out)

    def w3_pair(j):
        e, o = slice(64 * (2 * j + 1), 64 * (2 * j + 2)), slice(64 * (2 * j + 2), 64 * (2 * j + 3))
        zb, zs = (zb0, zs0) if ctx[0] == "r3" else (zb1, zs1)
        z1, z2 = _ub(zb[0:H // 2, :]), _ub(zb[H // 2:H, :])
        q = _strassen(_nt, z1[:, 0:256], z2[:, 256:512], [_ub(zs[k]) for k in range(5)], z1[:, 512:D], z2[:, 512:D],
                      _ub(w3p[e, 0:256]), _ub(w3p[o, 256:512]),
                      [_ub(s3[64 * j:64 * (j + 1), 256 * k:256 * (k + 1)]) for k in range(5)],
                      *([_ub(w3n[0:64, 0:128]), _ub(w3n[0:64, 128:256]), ORD[ctx[0] + "_0"], _nn] if j == 0 else
                        [_ub(w3p[e, 512:D]), _ub(w3p[o, 512:D]), ORD[ctx[0] + "_3"]]))
        return [_gelu_scaled(c) for c in q]

    def plain_ctx():
        return (ctx[0] in ("r3", "r4") and not TP0) or (ctx[0] == "z" and not TZ)

    def put_quads(j, q):
        l1, l2, l5, l6, l7 = _lhs_sums(*q)
        if not plain_ctx():
            al[64 * j:64 * (j + 1), 0:896] = _pk(_cat([l1, l2, q[0], q[3], l5, l6, l7]))
        else:
            al[64 * j:64 * (j + 1), :] = _pk(_cat([l1, l2, q[0], q[3], l5, l6, l7, q[1], q[2]]))

    def w3_pairs(ahead, which):
        for i in which:
            ahead = AHEAD[ctx[0]][i] == "1"
            ops = []
            for j in (2 * i, 2 * i + 1):
                q = w3_pair(j)
                if not ahead:
                    put_quads(j, q)
                ops.append(q)
            if not ahead:
                continue
            for n, q in enumerate(ops):
                l1, l2, l5, l6, l7 = _lhs_sums(*q)
                ops[n] = [l1, l2, q[0], q[3], l5, l6, l7]
                j, half = 2 * i + n, slice(64 * n, 64 * (n + 1))
                if not plain_ctx():
                    al[64 * j:64 * (j + 1), 0:896] = _pk(_cat(ops[n]))
                    continue
                o = 64 * j + 32 * n
                al[o:o + 32, 0:256] = _pk(_cat([l1[half], l2[half]]))
                al[o:o + 32, 512:896] = _pk(_cat([l5[half], l6[half], l7[half]]))
                al[64 * j:64 * (j + 1), 256:512] = _pk(_cat([q[0], q[3]]))
                al[64 * j:64 * (j + 1), 896:1152] = _pk(_cat([q[1], q[2]]))
            for m in range(7):
                e, o = ops[0][m], ops[1][m]
                r0 = 32 * (3 * m + i)
                a2[r0:r0 + 32, :] = _pk(_cat(_lhs_sums(e[0:64], o[0:64], e[64:128], o[64:128])))

    def s4_block(m, b, axis):
        o = 448 * (m - 1) + 64 * (b // 2)
        return _cat([s4[o + 128 * i:o + 128 * i + 64, _lanes(b % 2)] for i in range(3)], axis)

    def krow(j, par):
        return 128 * (2 * j + 1 + par) if j < NP3 else FM * par

    def prep_p4():
        for j in range(7):
            p4[0, 64 * j:64 * (j + 1), :] = pltpu.bitcast(w4b[krow(j, 0):krow(j, 0) + 128, 0:128], u32)
            if j < NP3:
                p4[1, 64 * j:64 * (j + 1), :] = pltpu.bitcast(w4b[krow(j, 1):krow(j, 1) + 128, 0:128], u32)
            else:
                p4[1, 64 * j:64 * j + 32, :] = pltpu.bitcast(w4b[FM:F, 0:128], u32)
                p4[1, 64 * j + 32:64 * (j + 1), :] = jnp.zeros((32, 128), u32)

    def prep_w4():
        def block(j, b):
            if j == NP3 and b >= 2:
                return _cat([both(w4b, FM, F, b % 2), jnp.zeros((64, 256), f32)], 0)
            return both(w4b, krow(j, b // 2), krow(j, b // 2) + 128, b % 2)

        for m in [int(t) for t in OUTER['r4']]:
            k = {1: 0, 4: 2, 2: None, 3: 1, 5: None, 7: 4, 6: 3}[m]
            for j in range(7):
                o = 448 * (m - 1) + 64 * j
                if k is None and (j < NP3 or m == 2):
                    par = 0 if m == 2 else 1
                    for n in range(2):
                        s4[o:o + 64, _lanes(n)] = pltpu.bitcast(
                            w4b[krow(j, par):krow(j, par) + 128, _lanes(2 * n + 1 + par)], u32)
                else:
                    s4[o:o + 64, :] = _pk(block(j, 3) if k is None else _rhs_sum(k, lambda b: block(j, b)))
            for k2 in (2, 1, 0, 4, 3):
                o = 64 * (5 * (m - 1) + k2)
                s5[o:o + 64, :] = _pk(_rhs_sum(k2, lambda b: _ub(s4_block(m, b, -1)).astype(f32)))

    def prep_t4():
        eye = (jax.lax.broadcasted_iota(i32, (128, 128), 0)
               == jax.lax.broadcasted_iota(i32, (128, 128), 1)).astype(f32).astype(bf16)
        if TX:
            def tile(j, par):
                r0 = 128 * (2 * j + 1 + par) if j < NP3 else FM * par
                if j == NP3 and par:
                    return _cat([w4b[FM:F, 0:128].astype(f32), jnp.zeros((64, 128), f32)], 0).T
                return w4b[r0:r0 + 128, 0:128].astype(f32).T
            wt = [_cat([tile(j, par) for j in range(7)]) for par in range(2)]
        else:
            wt = [_nt(eye, _ub(p4[par])) for par in range(2)]
        for m, k in ((1, 0), (2, None), (3, 1), (4, 2), (5, None), (6, 3), (7, 4)):
            def blk(b):
                return wt[b // 2][64 * (b % 2):64 * (b % 2 + 1)]
            t4[32 * (m - 1):32 * m, :] = _pk(blk(0 if m == 2 else 3) if k is None else _rhs_sum(k, blk))

    def w4_tile0_steps(r):
        mm = {}
        for t in TORD:
            m = int(t)
            left = _cat([al[64 * j:64 * (j + 1), _lanes(m - 1)] for j in range(7)])
            mm[m] = _nt(_ub(t4[32 * (m - 1):32 * m, :]), _ub(left))
            if len(mm) == 7:
                c11 = ((mm[4] - mm[5]) + mm[1]) + mm[7]
                c22 = ((mm[3] - mm[2]) + mm[1]) + mm[6]
                finish(r, H, _cat([c11, mm[3] + mm[5]], 0).T, 0)
                finish(r + H, H, _cat([mm[4] + mm[2], c22], 0).T, 0)
            yield

    def finish(r, n, h, c):
        c0, c1 = 128 * c, 128 * (c + 1)
        x1 = hss[rows(r, n), c0:c1]
        base = x2s[rows(r, n), c0:c1] + mvec(4, n, c0, c1) * x1
        ob[rows(r, n), c0:c1] = (base + mvec(5, n, c0, c1) * h).astype(bf16)
        if ctx[0] == "z":
            send(r, n, c)

    def w4_plain(r, o=0, n=T):
        def left(k):
            return _cat([al[64 * j:64 * (j + 1), _lanes(k)] for j in range(7)])

        a = _cat([_cat([left(2), left(7)]), _cat([left(8), left(3)])], 0)[o // 2:(o + n) // 2]
        finish(r + o, n, _nn(_ub(a), _ub(_cat([p4[0], p4[1]], 0))), 0)

    def w4_product(m, ahead, order=None):
        def blk(b, grp=range(3)):
            o = 64 * (b % 2) + 32 * (b // 2)
            return _ub(_cat([al[o + 128 * i:o + 128 * i + 32, _lanes(m - 1)] for i in grp]))

        pre = [i for i in range(3) if AHEAD[ctx[0]][i] == "1"]
        now = [i for i in range(3) if i not in pre]
        asum = [[] for _ in range(5)]
        if pre:
            for k in range(5):
                asum[k].append((pre, _ub(_cat([a2[32 * (3 * (m - 1) + i):32 * (3 * (m - 1) + i + 1), _lanes(k)]
                                               for i in pre]))))
        if now:
            for k, v in enumerate(_lhs_sums(*[blk(b, now).astype(f32) for b in range(4)])):
                asum[k].append((now, v))

        def dot(a, w):
            if not isinstance(a, list):
                return _nn(a, w)
            parts = [_nn(v, w if len(grp) == 3 else _cat([w[128 * i:128 * (i + 1)] for i in grp], 0)) for grp, v in a]
            return parts[0] if len(parts) == 1 else parts[0] + parts[1]

        bsum = [_ub(_cat([s5[64 * (5 * (m - 1) + k):64 * (5 * (m - 1) + k + 1), _lanes(i)] for i in range(3)], 0))
                for k in range(5)]
        ox = 448 * (m - 1) + 384
        q = _strassen(dot, blk(0), blk(3), asum, _ub(al[384:416, _lanes(m - 1)]), _ub(al[416:448, _lanes(m - 1)]),
                      _ub(s4_block(m, 0, 0)), _ub(s4_block(m, 3, 0)), bsum,
                      _ub(s4[ox:ox + 64, _lanes(0)]), _ub(s4[ox:ox + 64, _lanes(1)]), ORD[ctx[0] + "_4"])
        return _cat([_cat(q[0:2]), _cat(q[2:4])], 0)

    def w4_steps(r, ahead):
        acc = [c2.at[H * i:H * (i + 1), :] for i in range(4)]

        def finish2(rr, h, c):
            finish(rr, H, h[:, 0:128], c)
            finish(rr, H, h[:, 128:256], c + 2)

        sign = {1: (1, 0, 0, 1), 2: (0, 0, 1, -1), 3: (0, 1, 0, 1), 4: (1, 0, 1, 0), 5: (-1, 1, 0, 0),
                6: (0, 0, 0, 1), 7: (1, 0, 0, 0)}
        left_n, state = [4, 2, 2, 4], [None] * 4
        for m in [int(t) for t in OUTER[ctx[0]]]:
            x = w4_product(m, ahead)
            outs = [i for i in range(4) if sign[m][i]]
            olds = {i: None if state[i] is None else state[i][0][...] for i in outs}
            busy = [state[i][0] for i in range(4) if state[i] is not None and i not in outs]
            free = [a for a in acc if not any(a is b for b in busy)]
            shared = None
            for i in outs:
                sg = sign[m][i]
                left_n[i] -= 1
                if state[i] is None:
                    if shared is None:
                        shared = free.pop()
                        shared[...] = x
                    state[i] = (shared, sg)
                    continue
                v = olds[i] + x if (sg > 0) == (state[i][1] > 0) else (x - olds[i] if sg > 0 else olds[i] - x)
                if left_n[i] == 0:
                    finish2(r + H * (i // 2), v, 1 + i % 2)
                    state[i] = None
                else:
                    dst = free.pop()
                    dst[...] = v
                    state[i] = (dst, 1)
            yield

    def up(order, ahead, r1=None, n1=None):
        for tok in order:
            if tok == "e":
                w3_edge()
            elif tok in "xyz":
                w3_pairs(ahead, ["xyz".index(tok)])
            elif tok == "1":
                mm_w1(r1, n1)
            elif tok == "c":
                ln_chain(r1, n1, paired=PAIRED)

    groups = list(range(0, P0 + P1, RG))
    wait([q_copies[0]])
    sa, ca, ga = mod_part(0, 1)
    modb[0] = ga * sa
    modb[1] = ga * (1.0 + ca)
    for c in range(NL, CT):
        mac_inv(c, NB - 1)
    st1 = {o: _stats(load_q(o)) for o in groups}
    zt[0:8, 0:128] = jnp.zeros((8, 128), u32)
    st2 = {}
    for o in groups:
        x2 = make_x2(o, load_q(o), st1[o])
        x2s[o:o + RG, :] = x2
        st2[o] = _stats(x2)

    wait([mod_copies[1]])
    sb, cb = mod_part(1, 2)
    modb[2] = sb
    modb[3] = 1.0 + cb
    st3 = {}
    for o in range(0, P0, RG):
        h2 = make_h2(x2s[o:o + RG, :], st2[o])
        h2s[o:o + RG, :] = h2
        st3[o] = _stats(h2, scaled=True)
    for o1 in range(0, P0 // 2, RG):
        zz = []
        for o in (o1, o1 + P0 // 2):
            zz.append((h2s[o:o + RG, :] - st3[o][0]) * st3[o][1])
            zt[o // 2:(o + RG) // 2, :] = _pk(zz[-1])
        if S1:
            put_sums(zu0, o1, zz[0], zz[1])

    wait([w_copies[0]])
    prep_square(w1b, w1p, s1, not S1)
    if S1:
        mm_w1(0, P0, 0, zu0, "0")
    else:
        z0 = _ub(zt[0:P0 // 2, :])
        h1 = _gelu_scaled(_nn(z0, _ub(w1p[:, 0:512])))
        for c in range(CT - 1):
            h1s[c][8:8 + P0, :] = h1[:, _lanes(c)]
        for o in range(0, P0, P0 // 4):
            h1s[CT - 1][8 + o:8 + o + P0 // 4, :] = _gelu_scaled(_nn(z0[o:o + P0 // 4], _ub(w1p[:, 512:D])))
    prev = None
    for o1 in range(0, P1 // 2, RG):
        zz = []
        for o in (P0 + o1, P0 + o1 + P1 // 2):
            h2 = make_h2(x2s[o:o + RG, :], st2[o])
            h2s[o:o + RG, :] = h2
            st = _stats(h2, prev, True, True)
            z = (h2 - st[0]) * st[1]
            zt[o // 2:(o + RG) // 2, :] = _pk(z)
            prev = st[1]
            zz.append(z)
        put_sums(zu, o1, zz[0], zz[1])
    mm_w1(P0, P1, P0)

    ctx[0] = "r2"
    wait([w_copies[1], q_copies[1]])
    prep_square(w2b, w2p, s2)
    ln_chain(P0 + P1, PA, paired=R2M)
    mm_w2(0)
    ln_x1(0, R2L)
    mm_w2(T)

    ctx[0] = "r3"
    wait([w_copies[2]])
    prep_w3()
    early = ln_x1(T, stats_only=SE == 1) if SE else None
    up(R3O, True, P0 + P1, PA)

    ctx[0] = "r4"
    if FEN4:
        jax.lax.fori_loop(0, 2, fence, 0)
    wait([w_copies[3], mod_copies[2]])
    prep_w4()
    sc16 = jnp.broadcast_to(scb[:, 0:D], (16, D)).astype(bf16)
    steps, h, j = w4_steps(0, True), None, 0
    if TP0:
        prep_t4()
        tile0 = w4_tile0_steps(0)
    for tok in R4O:
        if tok == "p" and TP0:
            next(tile0)
        elif tok == "T" and TP0:
            pass
        elif tok == "p":
            blk = [al[64 * j:64 * (j + 1), _lanes(k)] for k in (2, 7, 8, 3)]
            w = _ub(_cat([p4[0, 64 * j:64 * (j + 1), :], p4[1, 64 * j:64 * (j + 1), :]], 0))
            d = [_nn(_ub(_cat(blk[0:2])), w), _nn(_ub(_cat(blk[2:4])), w)]
            h = d if h is None else [h[0] + d[0], h[1] + d[1]]
            j += 1
            if j == 7:
                finish(0, H, h[0], 0)
                finish(H, H, h[1], 0)
        elif tok == "s":
            next(steps)
        elif tok == "T":
            prep_t4()
        else:
            c0, c1 = (0, 384) if tok == "g" else (384, D)
            gb = jnp.dot(sc16, wmc[:, c0:c1], preferred_element_type=f32)[0:8]
            modb[4, :, c0:c1] = gb
            modb[5, :, c0:c1] = (0.5 / ALPHA) * gb
    if SE < 2:
        ln_x1(T, stats=early)
    out_copy(0).start()
    q_copies[2].wait()

    def mlp_body(i, carry):
        r1 = pl.multiple_of(PB - PC + PC * i, 32)
        r = pl.multiple_of(i * T, T)
        up(HEAD, False, r1, PC)
        steps, tile0 = w4_steps(r, False), w4_tile0_steps(r)
        for tok in BODY:
            if tok == "1":
                mm_w1(r1, PC)
            elif tok == "p":
                next(tile0)
            elif tok == "2":
                mm_w2(r + T)
            elif tok == "l":
                ln_x1(r + T, LM)
            else:
                next(steps)
        out_copy(i).start()
        return carry

    ctx[0] = "l"
    jax.lax.fori_loop(1, NC - 1, mlp_body, 0)

    ctx[0] = "z"
    up(ZO, True)
    if TZ:
        steps, tile0 = w4_steps(S - T, True), w4_tile0_steps(S - T)
        for tok in ZB:
            next(steps if tok == "s" else tile0)
    else:
        prep_p4()
        w4_plain(S - T, 0, LA)
        for _ in w4_steps(S - T, True):
            pass
        if LAST0 > LA:
            w4_plain(S - T, LA, LAST0 - LA)
        w4_plain(S - T, LAST0, T - LAST0)
    for i in range(NC - 1):
        out_copy(i).wait()
    for cp in out_tail:
        cp.wait()


@jax.jit
def pallas_adaLN_cond__ssm_conv_h3__mixer_s_mlp__prompt_kernel(
    A_q: jax.Array,
    A_k: jax.Array,
    A_v: jax.Array,
    A_shift_k: jax.Array,
    A_ssm_k: jax.Array,
    A_ssm_D: jax.Array,
    B_x: jax.Array,
    B_w1: jax.Array,
    B_w2: jax.Array,
    B_w3: jax.Array,
    B_w4: jax.Array,
    c: jax.Array,
    w_mod: jax.Array,
):
    del B_x
    any_spec = pl.BlockSpec(memory_space=pl.ANY)

    def tile_view(x):
        return x.reshape(S // 8, 8, CT, 128).transpose(0, 2, 1, 3).reshape(S * CT, 128)

    vm = pltpu.VMEM
    dma = pltpu.SemaphoreType.DMA
    spec = (4, NG, 16, 128)
    out = pl.pallas_call(
        _kernel,
        in_specs=[any_spec] * 12,
        out_specs=any_spec,
        out_shape=jax.ShapeDtypeStruct((S, D), bf16),
        scratch_shapes=[
            *[vm((KROWS, 128), bf16)] * NB, *[vm((VROWS, 128), bf16)] * NB, vm((CT, 128, S), bf16),
            vm((S, D), bf16), vm((D, D), bf16), vm((D, D), bf16), vm((F, D), bf16), vm((F, D), bf16),
            vm((D // 2, D), u32), vm((D // 2, D), u32), vm((F // 2, D), u32),
            vm((D, 3 * D), bf16), vm((D, 2 * D), bf16), vm((D, D), bf16),
            vm((4, D), bf16), vm((D,), bf16), vm((1, D), bf16), vm((1, 1792), f32),
            vm((4, 128, 128), u32), vm((4, 128, 128), u32), vm((4, 64, 256), u32),
            vm((CT, 8, 8, 128), f32),
            vm((CT, NB) + spec, f32), vm((CT, NB - 1) + spec, f32), vm((CT,) + spec, f32),
            vm((CT, NB) + spec, f32), vm((4, 128, 128), f32),
            vm((CT, S + 32, 128), f32), vm((8, 8, D), f32),
            *[vm((S + 32, 128), f32)] * CT, vm((S, D), f32), vm((S, D), f32), vm((S, D), f32),
            vm((288, D), u32), vm((5, H // 2, 256), u32), vm((H, D), u32), vm((5, H // 2, 256), u32),
            vm((H, D), u32), vm((5, H // 2, 256), u32), vm((5, 96, 256), u32),
            vm((64, 256), u32), vm((D, 256), u32), vm((D, 256), u32), vm((NP3 * 64, 1280), u32),
            vm((7 * 448, 256), u32), vm((35 * 64, 384), u32), vm((2, 448, 128), u32),
            vm((7 * 64, 1152), u32), vm((21 * 32, 640), u32), vm((4 * H, 256), f32), vm((7 * 32, 896), u32), vm((64, 1280), u32),
            vm((S, D), bf16),
            dma((26,)), dma((NC + 10,)),
        ],
        compiler_params=pltpu.CompilerParams(vmem_limit_bytes=110 << 20, disable_bounds_checks=True,
                                             disable_semaphore_checks=True),
    )(A_q.reshape(S, D), tile_view(A_k), tile_view(A_v), A_shift_k.T, A_ssm_k,
      A_ssm_D, B_w1, B_w2, B_w3.T, B_w4, c, w_mod)
    return out.reshape(1, S, D)
```

```python
import numpy as np
import jax
import jax.numpy as jnp
import jax.experimental.pallas as pl
import jax.experimental.pallas.tpu as pltpu

f32, bf16, u32, i32 = jnp.float32, jnp.bfloat16, jnp.uint32, jnp.int32

S, D, F = 2048, 640, 1728
CT = D // 128
TR = 8 * CT
NB, BLK, NFFT = 4, 512, 1024
KROWS, VROWS = BLK * CT + 128, BLK * CT + 64
NG = 16
T = 256
NC = S // T
H = T // 2
NP3 = 6
FM = (F // 128) * 128
P0, P1, PA, PC = 320, 224, 160, 224
PB = P0 + P1 + PA
LA, LAST0 = 96, 208
RG = 16
EPS = 1e-5
NT_DIMS = (((1,), (1,)), ((), ()))
PAIRED = "10000100001000"
ORD = {"r1_1": "4235ba16cd7", "r1_0": "4c5213db7a6", "r2_2": "d274c3ab156", "r3_1": "576b432acd1",
       "r3_3": "c245a173b6d", "r3_e": "32bca41d576", "r3_0": "345217ba6cd", "r4_4": "5b21a74dc63",
       "l_1": "7ba325cd461", "l_2": "45c1627ab3d", "l_3": "4bc51a7d236", "l_4": "243ac571b6d",
       "l_e": "24bdc35176a", "l_0": "acbd2351746", "z_3": "b5c231a47d6", "z_4": "c35d12b74a6",
       "z_e": "6cd3127ab45", "z_0": "acd231b4576"}
OUTER = {"r4": "2617345", "l": "5132647", "z": "1523467"}
BODY = "1pp2sslpsspspspps"
HEAD = "xecyz"
LM = "0000000000100000"
R2M = "0010101010"
R2L = "1010100010101010"
R3O = "1ezyx"
R4O = "sgGpspspspsppsps"
ZO = "xeyz"
FA = 3
TORD = "7621354"
AHEAD = {"r3": "111", "r4": "111", "l": "000", "z": "110"}
GV = 8
NL = 4


def _lo(w):
    return pltpu.bitcast(w << 16, f32)


def _hi(w):
    return pltpu.bitcast(w & jnp.uint32(0xFFFF0000), f32)


def _cis(n):
    t = (n & (2 * NFFT - 1)).astype(f32) * (np.pi / NFFT)
    return jnp.cos(t), jnp.sin(t)


def _fwd_table(r):
    g = jax.lax.broadcasted_iota(i32, (NG, 128), 0)
    cg, sg = _cis(jnp.where(g < NG // 2, 32 * g + 1, 32 * g - 253) * r)
    cs, ss = _cis(4 * jax.lax.broadcasted_iota(i32, (8, 128), 0) * r)
    parts = []
    for i in range(NG):
        c, s = cg[i:i + 1], sg[i:i + 1]
        parts += [c * cs - s * ss, -(s * cs + c * ss)]
    return pltpu.bitcast(jnp.concatenate(parts, axis=0).astype(bf16), u32)


def _inv_tables():
    def phase(rows):
        col = jax.lax.broadcasted_iota(i32, (rows, 256), 1)
        k = ((col >> 4) << 3) + (col & 7)
        row = jax.lax.broadcasted_iota(i32, (rows, 256), 0)
        return jnp.where(k < 64, 4 * k + 1, 4 * k - 253), (col & 8) << 6, row

    fr, _, g = phase(16)
    cg, sg = _cis(fr * (32 * g))
    fr, off, s = phase(8)
    out = []
    for p in range(4):
        cs, ss = _cis(fr * (4 * s + p) + off)
        cs, ss = cs * (2.0 / NFFT), ss * (2.0 / NFFT)
        parts = [cg[i:i + 1] * cs - sg[i:i + 1] * ss for i in range(16)]
        out.append(pltpu.bitcast(jnp.concatenate(parts, axis=0).astype(bf16), u32))
    return out


def _radix4(re, im, inverse):
    ar, ai = re[0] + re[2], im[0] + im[2]
    br, bi = re[0] - re[2], im[0] - im[2]
    cr, ci = re[1] + re[3], im[1] + im[3]
    dr, di = re[1] - re[3], im[1] - im[3]
    minus_i = (br + di, bi - dr)
    plus_i = (br - di, bi + dr)
    if inverse:
        return [(ar + cr, ai + ci), plus_i, (ar - cr, ai - ci), minus_i]
    return [(ar + cr, ai + ci), minus_i, (ar - cr, ai - ci), plus_i]


def _stats(x, link=None, early=False, scaled=False):
    zero = 0.0 if link is None else jnp.minimum(link, 0.0)
    part = x[:, 0:128]
    for c in range(1, CT):
        part = part + x[:, c * 128:(c + 1) * 128]
    if link is not None and early:
        part = part + zero
        zero = 0.0
    m = jnp.sum(part, axis=-1, keepdims=True) * (1.0 / D)
    v = jnp.maximum(jnp.sum(x * x, axis=-1, keepdims=True) * (1.0 / D) - m * m, zero)
    e = jnp.log(v + EPS) * (-0.5 / np.log(2.0))
    return m, jnp.exp2(e + np.log2(ALPHA) if scaled else e)


GC = 0.7978845608028654
ALPHA = (GC * 0.044715) ** (1.0 / 3.0)


def _gelu_scaled(y):
    return y + y * jnp.tanh(y * (y * y + GC / ALPHA))


def _pk(x):
    return pltpu.bitcast(x.astype(bf16), u32)


def _ub(x):
    return pltpu.bitcast(x, bf16)


def _cat(xs, axis=-1):
    return jnp.concatenate(xs, axis=axis)


def _lanes(k):
    return slice(128 * k, 128 * (k + 1))


def _nn(a, w):
    return jnp.dot(a.astype(bf16), w, preferred_element_type=f32)


def _nt(a, w):
    return jax.lax.dot_general(a, w, NT_DIMS, preferred_element_type=f32)


def _lhs_sums(a11, a12, a21, a22):
    return [a11 + a22, a21 + a22, a11 + a12, a21 - a11, a12 - a22]


def _rhs_sum(k, block):
    a, b, plus = [(0, 3, True), (1, 3, False), (2, 0, False), (0, 1, True), (2, 3, True)][k]
    return block(a) + block(b) if plus else block(a) - block(b)


def _strassen(dot, a11, a22, asum, ax1, ax2, b11, b22, bsum, bx1, bx2, order, xdot=None):
    ops = {"1": (asum[0], bsum[0], (1, 0, 0, 1)), "2": (asum[1], b11, (0, 0, 1, -1)),
           "3": (a11, bsum[1], (0, 1, 0, 1)), "4": (a22, bsum[2], (1, 0, 1, 0)),
           "5": (asum[2], b22, (-1, 1, 0, 0)), "6": (asum[3], bsum[3], (0, 0, 0, 1)),
           "7": (asum[4], bsum[4], (1, 0, 0, 0)), "a": (ax1, bx1, (1, 0, 0, 0)),
           "b": (ax1, bx2, (0, 1, 0, 0)), "c": (ax2, bx1, (0, 0, 1, 0)), "d": (ax2, bx2, (0, 0, 0, 1))}
    c, neg = [None] * 4, [None] * 4
    for t in order:
        a, b, sg = ops[t]
        m = (xdot if xdot and t in "abcd" else dot)(a, b)
        for i in range(4):
            if sg[i] > 0:
                c[i] = m if c[i] is None else c[i] + m
                if neg[i] is not None:
                    c[i], neg[i] = c[i] - neg[i], None
            elif sg[i] < 0:
                if c[i] is None:
                    neg[i] = m
                else:
                    c[i] = c[i] - m
    return c


def _kernel(q_hbm, k_hbm, v_hbm, sh_hbm, sk_hbm, d_hbm, w1_hbm, w2_hbm, w3_hbm, w4_hbm,
            c_hbm, wm_hbm, o_hbm,
            kb0, kb1, kb2, kb3, vb0, vb1, vb2, vb3, skb, qb, w1b, w2b, w3b, w4b, w1p, w2p, w3p,
            wma, wmb, wmc, shb, db, cb_, scb,
            fub, fkb, gtb, par, US, KS, UR, YS, YP, ys, modb, h10, h11, h12, h13, h14, h2s, x2s, x1s,
            zt, zu, zb1, zs1, zb0, zs0, zu0, w3n, s1, s2, s3, s4, s5, p4, al, a2, c2, t4, e3, ob,
            sem, sem_o):
    h1s = [h10, h11, h12, h13, h14]
    n_in = [0]

    def load(src, dst):
        n_in[0] += 1
        return pltpu.make_async_copy(src, dst, sem.at[n_in[0] - 1])

    nkv = BLK * CT
    small = [load(d_hbm, db), load(sh_hbm, shb), load(c_hbm, cb_)]
    sk_copies = [load(sk_hbm.at[pl.ds(c * 128, 128), :], skb.at[c]) for c in range(CT)]
    kbs, vbs, wms = [kb0, kb1, kb2, kb3], [vb0, vb1, vb2, vb3], [wma, wmb, wmc]
    kv_copies = [[load(k_hbm.at[pl.ds(a * nkv, nkv), :], kbs[a].at[pl.ds(TR, nkv), :]),
                  load(v_hbm.at[pl.ds(a * nkv, nkv), :], vbs[a].at[pl.ds(0, nkv), :])] for a in range(NB)]
    mod_cols = [(0, 3 * D), (3 * D, 2 * D), (5 * D, D)]
    mod_copies = [load(wm_hbm.at[:, pl.ds(o, n)], w) for (o, n), w in zip(mod_cols, wms)]
    w_copies = [load(w1_hbm, w1b), load(w2_hbm, w2b), load(w3_hbm, w3b), load(w4_hbm, w4b)]
    q_copies = [load(q_hbm.at[pl.ds(o, n), :], qb.at[pl.ds(o, n), :])
                for o, n in [(0, P0 + P1), (P0 + P1, PA), (PB, S - PB)]]

    def out_copy(i):
        r = i * T if isinstance(i, int) else pl.multiple_of(i * T, T)
        return pltpu.make_async_copy(ob.at[pl.ds(r, T), :], o_hbm.at[pl.ds(r, T), :], sem_o.at[i])

    out_tail = []

    def send(r, n, c):
        cp = pltpu.make_async_copy(ob.at[pl.ds(r, n), pl.ds(128 * c, 128)], o_hbm.at[pl.ds(r, n), pl.ds(128 * c, 128)],
                                   sem_o.at[NC - 1 + len(out_tail)])
        out_tail.append(cp)
        cp.start()

    for cp in (small + kv_copies[0] + sk_copies + kv_copies[1] + kv_copies[2] + kv_copies[3]
               + [mod_copies[0], q_copies[0], mod_copies[1], w_copies[0], w_copies[1], q_copies[1],
                  w_copies[2], w_copies[3], mod_copies[2], q_copies[2]]):
        cp.start()

    def wait(copies):
        for cp in copies:
            cp.wait()

    def pin(i, carry):
        z = jnp.zeros((8, 128), f32)
        scb[:, pl.ds(pl.multiple_of(i * 128, 128), 128)] = z[0:1]
        YP[i, 0:8, :] = z
        US[i, 0, 0, 0, 0:8, :] = z
        KS[i, 0, 0, 0, 0:8, :] = z
        YS[i, 0, 0, 0, 0:8, :] = z
        UR[i, 0, 0, 0:8, :] = z
        r8 = pl.ds(pl.multiple_of(i * 8, 8), 8)
        c2[r8, 0:128] = z
        al[r8, 0:128] = jnp.zeros((8, 128), u32)
        zb0[r8, 0:128] = jnp.zeros((8, 128), u32)
        zs0[i, 0:8, 0:128] = jnp.zeros((8, 128), u32)
        zu0[i, 0:8, 0:128] = jnp.zeros((8, 128), u32)
        a2[r8, 0:128] = jnp.zeros((8, 128), u32)
        return carry

    def fence(i, carry):
        YP[i, 0:8, :] = jnp.zeros((8, 128), f32)
        return carry

    jax.lax.fori_loop(0, 2, pin, 0)
    lane = jax.lax.broadcasted_iota(i32, (1, 128), 1)
    for p in range(4):
        m = (lane - p) & 3
        fkb[p] = _fwd_table(128 * m + ((lane - m) & 127))
    for c in range(CT):
        kb0[c * 8:(c + 1) * 8, :] = jnp.zeros((8, 128), bf16)
        h1s[c][0:8, :] = jnp.zeros((8, 128), f32)
        h1s[c][S + 8:S + 16, :] = jnp.zeros((8, 128), f32)
    for a in range(NB):
        kbs[a][nkv + TR:KROWS, :] = jnp.zeros((KROWS - nkv - TR, 128), bf16)
        vbs[a][nkv:VROWS, :] = jnp.zeros((VROWS - nkv, 128), bf16)
    for p in range(4):
        fub[p] = _fwd_table(8 * (lane & 63) + ((lane >> 6) << 2) + p)
    wait(small)
    cvec = cb_[...].astype(f32)
    scb[:, 0:D] = cvec * jax.nn.sigmoid(cvec)
    dv = db[...].astype(f32).reshape(1, D)
    shv = shb[...].astype(f32)
    for c in range(CT):
        for i in range(4):
            par[c, i] = jnp.broadcast_to(shv[i:i + 1, c * 128:(c + 1) * 128], (8, 128))
        par[c, 4] = jnp.broadcast_to(dv[:, c * 128:(c + 1) * 128], (8, 128))
    for p, tab in enumerate(_inv_tables()):
        gtb[p] = tab

    def get(ref, idx, g, n):
        return (ref[idx + (slice(g, g + n), slice(0, 8))], ref[idx + (slice(g, g + n), slice(8, 16))])

    def put(ref, idx, g, n, xr, xi):
        ref[idx + (slice(g, g + n), slice(0, 8))] = xr
        ref[idx + (slice(g, g + n), slice(8, 16))] = xi

    def split(tt, g, n):
        tt = [t[g * 16:(g + n) * 16].reshape(n, 16, 128) for t in tt]
        return [t[:, 0:8] for t in tt], [t[:, 8:16] for t in tt]

    def fwd_k(c, j):
        lane = jax.lax.broadcasted_iota(i32, (64, 128), 1)
        even = (lane & 1) == 0
        l01 = (lane & 2) == 0
        l12 = ((lane + 3) & 2) == 0
        rm = []
        for m in range(4):
            w = pltpu.bitcast(skb[c, :, (4 * j + m) * 128:(4 * j + m + 1) * 128], u32)
            rm.append(pltpu.roll(w, m, 1) if m else w)
        e01 = jnp.where(even, rm[0], rm[1])
        o01 = jnp.where(even, rm[1], rm[0])
        e23 = jnp.where(even, rm[2], rm[3])
        o23 = jnp.where(even, rm[3], rm[2])
        kp = [jnp.where(l01, e01, e23), jnp.where(l12, o01, o23),
              jnp.where(l01, e23, e01), jnp.where(l12, o23, o01)]
        tt = [jax.lax.dot_general(pltpu.bitcast(fkb[p], bf16), pltpu.bitcast(kp[p], bf16), NT_DIMS,
                                  preferred_element_type=f32) for p in range(4)]
        for g in range(0, NG, GV):
            re, im = split(tt, g, GV)
            if j == 0:
                re[0] = re[0] + par[c, 4][None]
            for m, (xr, xi) in enumerate(_radix4(re, im, False)):
                if j < NB - 1:
                    put(KS, (c, j, m), g, GV, xr, xi)
                ur, ui = get(US, (c, 0, m), g, GV)
                put(YS, (c, j, m), g, GV, xr * ur - xi * ui, xr * ui + xi * ur)

    def fwd_u(c, a):
        taps = [jnp.tile(par[c, i], (8, 1)) for i in range(4)]
        ws = TR // 2
        base = 4 * c
        kw, vw = kbs[a].bitcast(u32), vbs[a].bitcast(u32)

        def words(ref, start):
            return ref[pl.ds(start, BLK // 8, stride=ws), :]

        kk = {}
        for w in range(4):
            x = words(kw, ws + base + w)
            kk[2 * w], kk[2 * w + 1] = _lo(x), _hi(x)
        kk[-3] = _hi(words(kw, base + 2))
        x = words(kw, base + 3)
        kk[-2], kk[-1] = _lo(x), _hi(x)
        sub = []
        for w in range(4):
            x = words(vw, base + w)
            for r, vv in ((2 * w, _lo(x)), (2 * w + 1, _hi(x))):
                sh = taps[0] * kk[r] + taps[1] * kk[r - 1] + taps[2] * kk[r - 2] + taps[3] * kk[r - 3]
                sub.append(sh * vv)
        kv = [jnp.concatenate([sub[p], sub[p + 4]], axis=0) for p in range(4)]
        tt = [jnp.dot(pltpu.bitcast(fub[p], bf16), kv[p].astype(bf16), preferred_element_type=f32)
              for p in range(4)]
        for g in range(0, NG, GV):
            re, im = split(tt, g, GV)
            for m, (xr, xi) in enumerate(_radix4(re, im, False)):
                if a:
                    pr, pi = get(US, (c, 0, m), g, GV) if a == 1 else get(UR, (c, m), g, GV)
                    if a < NB - 1:
                        put(UR, (c, m), g, GV, xr, xi)
                    xr, xi = (xr - pi, xi + pr) if g < NG // 2 else (xr + pi, xi - pr)
                put(US, (c, a, m), g, GV, xr, xi)

    def mac_inv(c, a):
        for h in range(2):
            vals = [[] for _ in range(4)]
            for g in range(8 * h, 8 * h + 8, GV):
                yre, yim = [], []
                for m in range(4):
                    yr, yi = get(YS, (c, a, m), g, GV)
                    for j in range(a):
                        kr, ki = get(KS, (c, j, m), g, GV)
                        ur, ui = get(US, (c, a - j, m), g, GV)
                        yr = yr + (kr * ur - ki * ui)
                        yi = yi + (kr * ui + ki * ur)
                    yre.append(yr)
                    yim.append(yi)
                for p, (pr, pi) in enumerate(_radix4(yre, yim, True)):
                    vals[p].append(jnp.concatenate([pr, pi], axis=1))
            for p in range(4):
                pb = jnp.concatenate(vals[p], axis=0).reshape(128, 128).astype(bf16)
                r = jnp.dot(pltpu.bitcast(gtb[p, :, h * 128:(h + 1) * 128], bf16), pb,
                            preferred_element_type=f32)
                if h == 0:
                    YP[p] = r
                else:
                    ys[c, pl.ds(a * BLK + p, 128, stride=4), :] = YP[p] + r

    wait(kv_copies[0])
    for c in range(CT):
        fwd_u(c, 0)
    for grp in ((0,), (1, 2), (3, 4)):
        wait([sk_copies[c] for c in grp])
        for c in grp:
            for j in (3, 2, 1, 0):
                fwd_k(c, j)
    for a in range(1, NB):
        if a == FA:
            jax.lax.fori_loop(0, 2, fence, 0)
        wait(kv_copies[a])
        for c in range(CT):
            kbs[a][c * 8:(c + 1) * 8, :] = kbs[a - 1][nkv + c * 8:nkv + (c + 1) * 8, :]
        for c in range(CT):
            fwd_u(c, a)
            mac_inv(c, a - 1)
    wait([mod_copies[0]])
    for c in range(NL):
        mac_inv(c, NB - 1)

    def mod_part(part, extra):
        n, wm = mod_cols[part][1], wms[part]
        act = scb[:, 0:D]

        def sc(k0, k1):
            return jnp.broadcast_to(act[:, k0:k1], (16, k1 - k0)).astype(bf16)

        e = 128 * extra
        r = jnp.dot(sc(0, D), wm[:, e:n], preferred_element_type=f32)
        r0 = (jnp.dot(sc(0, D - 64), wm[0:D - 64, 0:e], preferred_element_type=f32)
              + jnp.dot(sc(D - 64, D), wm[D - 64:D, 0:e], preferred_element_type=f32))
        r = jnp.concatenate([r0, r], axis=-1)[0:8]
        return [r[:, i * D:(i + 1) * D] for i in range(n // D)]

    def mvec(i, n=RG, c0=0, c1=D):
        return jnp.tile(modb[i, :, c0:c1], (n // 8, 1))

    rows = pl.ds
    ctx = ["r1"]

    def load_q(r, ref=qb):
        return ref[rows(r, RG), :].astype(f32)

    def make_x2(r, q, st, ref=ys):
        y = _cat([ref[c, rows(r, RG), :] for c in range(CT)])
        return q + (((q - st[0]) * st[1]) * mvec(1) + mvec(0)) * y

    def make_h2(x2, st):
        return ((x2 - st[0]) * st[1]) * mvec(3) + mvec(2)

    def put_sums(ref, o, z1, z2):
        for k, v in enumerate(_lhs_sums(z1[:, 0:256], z1[:, 256:512], z2[:, 0:256], z2[:, 256:512])):
            ref.at[k][o // 2:(o + RG) // 2, :] = _pk(v)

    def ln_chain(r, n, paired):
        qv, yv = qb.at[rows(r, n), :], ys.at[:, rows(r, n), :]
        xv, hv = x2s.at[rows(r, n), :], h2s.at[rows(r, n), :]
        prev, pend, cnt = None, None, 0
        for o1 in range(0, n // 2, RG):
            zz = []
            for o in (o1, o1 + n // 2):
                q = load_q(o, qv)
                x2 = make_x2(o, q, _stats(q, prev), yv)
                xv[o:o + RG, :] = x2
                st = _stats(x2)
                h2 = make_h2(xv[o:o + RG, :], st)
                hv[o:o + RG, :] = h2
                st = _stats(h2, scaled=True)
                z = (hv[o:o + RG, :] - st[0]) * st[1]
                zt[o // 2:(o + RG) // 2, :] = _pk(z)
                zz.append(z)
                if paired and paired[cnt] == "1":
                    pend = st[1]
                elif pend is not None:
                    prev, pend = jnp.minimum(st[1], pend), None
                else:
                    prev = st[1]
                cnt += 1
            put_sums(zu, o1, zz[0], zz[1])

    def ln_x1(r, paired=""):
        zb, zs = (zb0, zs0) if ctx[0] == "r2" else (zb1, zs1)
        sv = x1s.at[rows(r, T), :]
        prev, pend, cnt = None, None, 0
        for o1 in range(0, H, RG):
            zz = []
            for o in (o1, o1 + H):
                x1 = sv[o:o + RG, :]
                st = _stats(x1, prev, True, True)
                z = (x1 - st[0]) * st[1]
                zb[o // 2:(o + RG) // 2, :] = _pk(z)
                zz.append(z)
                if paired and paired[cnt] == "1":
                    pend = st[1]
                elif pend is not None:
                    prev, pend = jnp.minimum(st[1], pend), None
                else:
                    prev = st[1]
                cnt += 1
            put_sums(zs, o1, zz[0], zz[1])

    def both(ref, r0, r1, col):
        return _cat([ref[r0:r1, _lanes(1 + col)].astype(f32), ref[r0:r1, _lanes(3 + col)].astype(f32)])

    def prep_square(wb, wp, sw):
        wp[:, 0:128] = pltpu.bitcast(wb[:, 0:128], u32)
        wp[256:320, 128:D] = pltpu.bitcast(wb[512:D, 128:D], u32)
        for n in range(2):
            wp[0:128, _lanes(2 * n + 1)] = pltpu.bitcast(wb[0:256, _lanes(2 * n + 1)], u32)
            wp[128:256, _lanes(2 * n + 2)] = pltpu.bitcast(wb[256:512, _lanes(2 * n + 2)], u32)
        for k in (2, 1, 0, 4, 3):
            sw[128 * k:128 * (k + 1), :] = _pk(_rhs_sum(
                k, lambda b: both(wb, 256 * (b // 2), 256 * (b // 2 + 1), b % 2)))

    def mm_square(a, top, bot, asum, wp, sw, which):
        h = top.shape[0]
        c0 = _nn(a, _ub(wp[:, 0:128]))
        out = [(c0[0:h], c0[h:2 * h])]
        for n in range(2):
            l1, l2 = _lanes(2 * n + 1), _lanes(2 * n + 2)
            q = _strassen(_nn, top[:, 0:256], bot[:, 256:512], asum, top[:, 512:D], bot[:, 512:D],
                          _ub(wp[0:128, l1]), _ub(wp[128:256, l2]),
                          [_ub(sw[128 * k:128 * (k + 1), _lanes(n)]) for k in range(5)],
                          _ub(wp[256:320, l1]), _ub(wp[256:320, l2]), ORD[ctx[0] + "_" + which])
            out += [(q[0], q[2]), (q[1], q[3])]
        return out

    def mm_w1(r, n, o=0, zu=zu, which="1"):
        h, o = n // 2, o // 2
        res = mm_square(_ub(zt[o:o + h, :]), _ub(zt[o:o + h // 2, :]), _ub(zt[o + h // 2:o + h, :]),
                        [_ub(zu[k, 0:h // 2, :]) for k in range(5)], w1p, s1, which)
        for c, (top, bot) in enumerate(res):
            h1s[c][rows(r + 8, h), :] = _gelu_scaled(top)
            h1s[c][rows(r + 8 + h, h), :] = _gelu_scaled(bot)

    def mm_w2(r):
        lane = jax.lax.broadcasted_iota(i32, (T, 128), 1)

        def sh(k, c):
            return h1s[c][rows(r + 8 + k, T), :]

        g = _cat([sh(-1, 0),
                  jnp.where(lane < 32, sh(-1, 1), sh(1, 1)),
                  jnp.where(lane < 64, sh(1, 2), sh(-2, 2)),
                  jnp.where(lane < 96, sh(-2, 3), sh(2, 3)),
                  sh(2, 4)])
        top, bot = g[0:H], g[H:T]
        sums = _lhs_sums(top[:, 0:256], top[:, 256:512], bot[:, 0:256], bot[:, 256:512])
        for c, (ct, cb) in enumerate(mm_square(g, top, bot, sums, w2p, s2, "2")):
            x1s[rows(r, H), _lanes(c)] = h2s[rows(r, H), _lanes(c)] + ct * (0.5 / ALPHA)
            x1s[rows(r + H, H), _lanes(c)] = h2s[rows(r + H, H), _lanes(c)] + cb * (0.5 / ALPHA)

    def prep_w3():
        for j in range(NP3):
            r0 = 128 * (2 * j + 1)
            w3p[r0 // 2:r0 // 2 + 64, 0:256] = pltpu.bitcast(w3b[r0:r0 + 128, 0:256], u32)
            if j:
                w3p[r0 // 2:r0 // 2 + 64, 512:D] = pltpu.bitcast(w3b[r0:r0 + 128, 512:D], u32)
            c1 = D if j else 512
            w3p[r0 // 2 + 64:r0 // 2 + 128, 256:c1] = pltpu.bitcast(w3b[r0 + 128:r0 + 256, 256:c1], u32)
        w3p[0:48, 0:256] = pltpu.bitcast(w3b[0:96, 0:256], u32)
        w3p[0:48, 512:D] = pltpu.bitcast(w3b[0:96, 512:D], u32)
        w3p[48:64, 256:D] = pltpu.bitcast(w3b[96:128, 256:D], u32)
        w3p[FM // 2:F // 2, 256:D] = pltpu.bitcast(w3b[FM:F, 256:D], u32)
        w3n[0:64, :] = _pk(_cat([w3b[128:256, 512:D].astype(f32).T, w3b[256:384, 512:D].astype(f32).T]))

        def edge(b):
            c = slice(256 * (b // 2), 256 * (b // 2 + 1))
            if b % 2 == 0:
                return w3b[0:96, c].astype(f32)
            return _cat([w3b[96:128, c].astype(f32), w3b[FM:F, c].astype(f32)], 0)

        for k in (2, 1, 0, 4, 3):
            e3[0:48, 256 * k:256 * (k + 1)] = _pk(_rhs_sum(k, edge))
        for j in range(NP3):
            r0 = 128 * (2 * j + 1)
            for k in (2, 1, 0, 4, 3):
                s3[64 * j:64 * (j + 1), 256 * k:256 * (k + 1)] = _pk(_rhs_sum(k, lambda b: w3b[
                    r0 + 128 * (b % 2):r0 + 128 * (b % 2 + 1), 256 * (b // 2):256 * (b // 2 + 1)].astype(f32)))

    def w3_edge():
        def second(c0, c1):
            return _ub(_cat([w3p[48:64, c0:c1], w3p[FM // 2:F // 2, c0:c1]], 0))

        zb, zs = (zb0, zs0) if ctx[0] == "r3" else (zb1, zs1)
        z1, z2 = _ub(zb[0:H // 2, :]), _ub(zb[H // 2:H, :])
        q = _strassen(lambda a, b: _nt(b, a), z1[:, 0:256], z2[:, 256:512], [_ub(zs[k]) for k in range(5)],
                      z1[:, 512:D], z2[:, 512:D], _ub(w3p[0:48, 0:256]), second(256, 512),
                      [_ub(e3[0:48, 256 * k:256 * (k + 1)]) for k in range(5)],
                      _ub(w3p[0:48, 512:D]), second(512, D), ORD[ctx[0] + "_e"])
        q = [_gelu_scaled(c) for c in q]
        out = []
        for x in (_cat(q[0:2], 0), _cat(q[2:4], 0)):
            out += [x[0:128].T, _cat([x[128:192], jnp.zeros((64, 128), f32)], 0).T]
        put_quads(NP3, out)

    def w3_pair(j):
        e, o = slice(64 * (2 * j + 1), 64 * (2 * j + 2)), slice(64 * (2 * j + 2), 64 * (2 * j + 3))
        zb, zs = (zb0, zs0) if ctx[0] == "r3" else (zb1, zs1)
        z1, z2 = _ub(zb[0:H // 2, :]), _ub(zb[H // 2:H, :])
        q = _strassen(_nt, z1[:, 0:256], z2[:, 256:512], [_ub(zs[k]) for k in range(5)], z1[:, 512:D], z2[:, 512:D],
                      _ub(w3p[e, 0:256]), _ub(w3p[o, 256:512]),
                      [_ub(s3[64 * j:64 * (j + 1), 256 * k:256 * (k + 1)]) for k in range(5)],
                      *([_ub(w3n[0:64, 0:128]), _ub(w3n[0:64, 128:256]), ORD[ctx[0] + "_0"], _nn] if j == 0 else
                        [_ub(w3p[e, 512:D]), _ub(w3p[o, 512:D]), ORD[ctx[0] + "_3"]]))
        return [_gelu_scaled(c) for c in q]

    def plain_ctx():
        return ctx[0] == "z"

    def put_quads(j, q):
        l1, l2, l5, l6, l7 = _lhs_sums(*q)
        if not plain_ctx():
            al[64 * j:64 * (j + 1), 0:896] = _pk(_cat([l1, l2, q[0], q[3], l5, l6, l7]))
        else:
            al[64 * j:64 * (j + 1), :] = _pk(_cat([l1, l2, q[0], q[3], l5, l6, l7, q[1], q[2]]))

    def w3_pairs(i):
        ahead = AHEAD[ctx[0]][i] == "1"
        ops = []
        for j in (2 * i, 2 * i + 1):
            q = w3_pair(j)
            if not ahead:
                put_quads(j, q)
            ops.append(q)
        if not ahead:
            return
        for n, q in enumerate(ops):
            l1, l2, l5, l6, l7 = _lhs_sums(*q)
            ops[n] = [l1, l2, q[0], q[3], l5, l6, l7]
            j, half = 2 * i + n, slice(64 * n, 64 * (n + 1))
            if not plain_ctx():
                al[64 * j:64 * (j + 1), 0:896] = _pk(_cat(ops[n]))
                continue
            o = 64 * j + 32 * n
            al[o:o + 32, 0:256] = _pk(_cat([l1[half], l2[half]]))
            al[o:o + 32, 512:896] = _pk(_cat([l5[half], l6[half], l7[half]]))
            al[64 * j:64 * (j + 1), 256:512] = _pk(_cat([q[0], q[3]]))
            al[64 * j:64 * (j + 1), 896:1152] = _pk(_cat([q[1], q[2]]))
        for m in range(7):
            e, o = ops[0][m], ops[1][m]
            r0 = 32 * (3 * m + i)
            a2[r0:r0 + 32, :] = _pk(_cat(_lhs_sums(e[0:64], o[0:64], e[64:128], o[64:128])))

    def s4_block(m, b, axis):
        o = 448 * (m - 1) + 64 * (b // 2)
        return _cat([s4[o + 128 * i:o + 128 * i + 64, _lanes(b % 2)] for i in range(3)], axis)

    def krow(j, par):
        return 128 * (2 * j + 1 + par) if j < NP3 else FM * par

    def prep_p4():
        for j in range(7):
            p4[0, 64 * j:64 * (j + 1), :] = pltpu.bitcast(w4b[krow(j, 0):krow(j, 0) + 128, 0:128], u32)
            if j < NP3:
                p4[1, 64 * j:64 * (j + 1), :] = pltpu.bitcast(w4b[krow(j, 1):krow(j, 1) + 128, 0:128], u32)
            else:
                p4[1, 64 * j:64 * j + 32, :] = pltpu.bitcast(w4b[FM:F, 0:128], u32)
                p4[1, 64 * j + 32:64 * (j + 1), :] = jnp.zeros((32, 128), u32)

    def prep_w4():
        def block(j, b):
            if j == NP3 and b >= 2:
                return _cat([both(w4b, FM, F, b % 2), jnp.zeros((64, 256), f32)], 0)
            return both(w4b, krow(j, b // 2), krow(j, b // 2) + 128, b % 2)

        for m in [int(t) for t in OUTER['r4']]:
            k = {1: 0, 4: 2, 2: None, 3: 1, 5: None, 7: 4, 6: 3}[m]
            for j in range(7):
                o = 448 * (m - 1) + 64 * j
                if k is None and (j < NP3 or m == 2):
                    par = 0 if m == 2 else 1
                    for n in range(2):
                        s4[o:o + 64, _lanes(n)] = pltpu.bitcast(
                            w4b[krow(j, par):krow(j, par) + 128, _lanes(2 * n + 1 + par)], u32)
                else:
                    s4[o:o + 64, :] = _pk(block(j, 3) if k is None else _rhs_sum(k, lambda b: block(j, b)))
            for k2 in (2, 1, 0, 4, 3):
                o = 64 * (5 * (m - 1) + k2)
                s5[o:o + 64, :] = _pk(_rhs_sum(k2, lambda b: _ub(s4_block(m, b, -1)).astype(f32)))

    def prep_t4():
        def tile(j, par):
            if j == NP3 and par:
                return _cat([w4b[FM:F, 0:128].astype(f32), jnp.zeros((64, 128), f32)], 0).T
            return w4b[krow(j, par):krow(j, par) + 128, 0:128].astype(f32).T

        wt = [_cat([tile(j, par) for j in range(7)]) for par in range(2)]
        for m, k in ((1, 0), (2, None), (3, 1), (4, 2), (5, None), (6, 3), (7, 4)):
            def blk(b):
                return wt[b // 2][64 * (b % 2):64 * (b % 2 + 1)]
            t4[32 * (m - 1):32 * m, :] = _pk(blk(0 if m == 2 else 3) if k is None else _rhs_sum(k, blk))

    def w4_tile0_steps(r):
        mm = {}
        for t in TORD:
            m = int(t)
            left = _cat([al[64 * j:64 * (j + 1), _lanes(m - 1)] for j in range(7)])
            mm[m] = _nt(_ub(t4[32 * (m - 1):32 * m, :]), _ub(left))
            if len(mm) == 7:
                c11 = ((mm[4] - mm[5]) + mm[1]) + mm[7]
                c22 = ((mm[3] - mm[2]) + mm[1]) + mm[6]
                finish(r, H, _cat([c11, mm[3] + mm[5]], 0).T, 0)
                finish(r + H, H, _cat([mm[4] + mm[2], c22], 0).T, 0)
            yield

    def finish(r, n, h, c):
        c0, c1 = 128 * c, 128 * (c + 1)
        x1 = x1s[rows(r, n), c0:c1]
        base = x2s[rows(r, n), c0:c1] + mvec(4, n, c0, c1) * x1
        ob[rows(r, n), c0:c1] = (base + mvec(5, n, c0, c1) * h).astype(bf16)
        if ctx[0] == "z":
            send(r, n, c)

    def w4_plain(r, o=0, n=T):
        def left(k):
            return _cat([al[64 * j:64 * (j + 1), _lanes(k)] for j in range(7)])

        a = _cat([_cat([left(2), left(7)]), _cat([left(8), left(3)])], 0)[o // 2:(o + n) // 2]
        finish(r + o, n, _nn(_ub(a), _ub(_cat([p4[0], p4[1]], 0))), 0)

    def w4_product(m):
        def blk(b, grp=range(3)):
            o = 64 * (b % 2) + 32 * (b // 2)
            return _ub(_cat([al[o + 128 * i:o + 128 * i + 32, _lanes(m - 1)] for i in grp]))

        pre = [i for i in range(3) if AHEAD[ctx[0]][i] == "1"]
        now = [i for i in range(3) if i not in pre]
        asum = [[] for _ in range(5)]
        if pre:
            for k in range(5):
                asum[k].append((pre, _ub(_cat([a2[32 * (3 * (m - 1) + i):32 * (3 * (m - 1) + i + 1), _lanes(k)]
                                               for i in pre]))))
        if now:
            for k, v in enumerate(_lhs_sums(*[blk(b, now).astype(f32) for b in range(4)])):
                asum[k].append((now, v))

        def dot(a, w):
            if not isinstance(a, list):
                return _nn(a, w)
            parts = [_nn(v, w if len(grp) == 3 else _cat([w[128 * i:128 * (i + 1)] for i in grp], 0)) for grp, v in a]
            return parts[0] if len(parts) == 1 else parts[0] + parts[1]

        bsum = [_ub(_cat([s5[64 * (5 * (m - 1) + k):64 * (5 * (m - 1) + k + 1), _lanes(i)] for i in range(3)], 0))
                for k in range(5)]
        ox = 448 * (m - 1) + 384
        q = _strassen(dot, blk(0), blk(3), asum, _ub(al[384:416, _lanes(m - 1)]), _ub(al[416:448, _lanes(m - 1)]),
                      _ub(s4_block(m, 0, 0)), _ub(s4_block(m, 3, 0)), bsum,
                      _ub(s4[ox:ox + 64, _lanes(0)]), _ub(s4[ox:ox + 64, _lanes(1)]), ORD[ctx[0] + "_4"])
        return _cat([_cat(q[0:2]), _cat(q[2:4])], 0)

    def w4_steps(r):
        acc = [c2.at[H * i:H * (i + 1), :] for i in range(4)]

        def finish2(rr, h, c):
            finish(rr, H, h[:, 0:128], c)
            finish(rr, H, h[:, 128:256], c + 2)

        sign = {1: (1, 0, 0, 1), 2: (0, 0, 1, -1), 3: (0, 1, 0, 1), 4: (1, 0, 1, 0), 5: (-1, 1, 0, 0),
                6: (0, 0, 0, 1), 7: (1, 0, 0, 0)}
        left_n, state = [4, 2, 2, 4], [None] * 4
        for m in [int(t) for t in OUTER[ctx[0]]]:
            x = w4_product(m)
            outs = [i for i in range(4) if sign[m][i]]
            olds = {i: None if state[i] is None else state[i][0][...] for i in outs}
            busy = [state[i][0] for i in range(4) if state[i] is not None and i not in outs]
            free = [a for a in acc if not any(a is b for b in busy)]
            shared = None
            for i in outs:
                sg = sign[m][i]
                left_n[i] -= 1
                if state[i] is None:
                    if shared is None:
                        shared = free.pop()
                        shared[...] = x
                    state[i] = (shared, sg)
                    continue
                v = olds[i] + x if (sg > 0) == (state[i][1] > 0) else (x - olds[i] if sg > 0 else olds[i] - x)
                if left_n[i] == 0:
                    finish2(r + H * (i // 2), v, 1 + i % 2)
                    state[i] = None
                else:
                    dst = free.pop()
                    dst[...] = v
                    state[i] = (dst, 1)
            yield

    def up(order, r1=None, n1=None):
        for tok in order:
            if tok == "e":
                w3_edge()
            elif tok in "xyz":
                w3_pairs("xyz".index(tok))
            elif tok == "1":
                mm_w1(r1, n1)
            elif tok == "c":
                ln_chain(r1, n1, paired=PAIRED)

    groups = list(range(0, P0 + P1, RG))
    wait([q_copies[0]])
    sa, ca, ga = mod_part(0, 1)
    modb[0] = ga * sa
    modb[1] = ga * (1.0 + ca)
    for c in range(NL, CT):
        mac_inv(c, NB - 1)
    st1 = {o: _stats(load_q(o)) for o in groups}
    zt[0:8, 0:128] = jnp.zeros((8, 128), u32)
    st2 = {}
    for o in groups:
        x2 = make_x2(o, load_q(o), st1[o])
        x2s[o:o + RG, :] = x2
        st2[o] = _stats(x2)

    wait([mod_copies[1]])
    sb, cb = mod_part(1, 2)
    modb[2] = sb
    modb[3] = 1.0 + cb
    st3 = {}
    for o in range(0, P0, RG):
        h2 = make_h2(x2s[o:o + RG, :], st2[o])
        h2s[o:o + RG, :] = h2
        st3[o] = _stats(h2, scaled=True)
    for o1 in range(0, P0 // 2, RG):
        zz = []
        for o in (o1, o1 + P0 // 2):
            zz.append((h2s[o:o + RG, :] - st3[o][0]) * st3[o][1])
            zt[o // 2:(o + RG) // 2, :] = _pk(zz[-1])
        put_sums(zu0, o1, zz[0], zz[1])

    wait([w_copies[0]])
    prep_square(w1b, w1p, s1)
    mm_w1(0, P0, 0, zu0, "0")
    prev = None
    for o1 in range(0, P1 // 2, RG):
        zz = []
        for o in (P0 + o1, P0 + o1 + P1 // 2):
            h2 = make_h2(x2s[o:o + RG, :], st2[o])
            h2s[o:o + RG, :] = h2
            st = _stats(h2, prev, True, True)
            z = (h2 - st[0]) * st[1]
            zt[o // 2:(o + RG) // 2, :] = _pk(z)
            prev = st[1]
            zz.append(z)
        put_sums(zu, o1, zz[0], zz[1])
    mm_w1(P0, P1, P0)

    ctx[0] = "r2"
    wait([w_copies[1], q_copies[1]])
    prep_square(w2b, w2p, s2)
    ln_chain(P0 + P1, PA, paired=R2M)
    mm_w2(0)
    ln_x1(0, R2L)
    mm_w2(T)

    ctx[0] = "r3"
    wait([w_copies[2]])
    prep_w3()
    ln_x1(T)
    up(R3O, P0 + P1, PA)

    ctx[0] = "r4"
    jax.lax.fori_loop(0, 2, fence, 0)
    wait([w_copies[3], mod_copies[2]])
    prep_w4()
    sc16 = jnp.broadcast_to(scb[:, 0:D], (16, D)).astype(bf16)
    prep_t4()
    steps, tile0 = w4_steps(0), w4_tile0_steps(0)
    for tok in R4O:
        if tok == "p":
            next(tile0)
        elif tok == "s":
            next(steps)
        else:
            c0, c1 = (0, 384) if tok == "g" else (384, D)
            gb = jnp.dot(sc16, wmc[:, c0:c1], preferred_element_type=f32)[0:8]
            modb[4, :, c0:c1] = gb
            modb[5, :, c0:c1] = (0.5 / ALPHA) * gb
    out_copy(0).start()
    q_copies[2].wait()

    def mlp_body(i, carry):
        r1 = pl.multiple_of(PB - PC + PC * i, 32)
        r = pl.multiple_of(i * T, T)
        up(HEAD, r1, PC)
        steps, tile0 = w4_steps(r), w4_tile0_steps(r)
        for tok in BODY:
            if tok == "1":
                mm_w1(r1, PC)
            elif tok == "p":
                next(tile0)
            elif tok == "2":
                mm_w2(r + T)
            elif tok == "l":
                ln_x1(r + T, LM)
            else:
                next(steps)
        out_copy(i).start()
        return carry

    ctx[0] = "l"
    jax.lax.fori_loop(1, NC - 1, mlp_body, 0)

    ctx[0] = "z"
    up(ZO)
    prep_p4()
    w4_plain(S - T, 0, LA)
    for _ in w4_steps(S - T):
        pass
    w4_plain(S - T, LA, LAST0 - LA)
    w4_plain(S - T, LAST0, T - LAST0)
    for i in range(NC - 1):
        out_copy(i).wait()
    for cp in out_tail:
        cp.wait()


@jax.jit
def pallas_adaLN_cond__ssm_conv_h3__mixer_s_mlp__prompt_kernel(
    A_q: jax.Array,
    A_k: jax.Array,
    A_v: jax.Array,
    A_shift_k: jax.Array,
    A_ssm_k: jax.Array,
    A_ssm_D: jax.Array,
    B_x: jax.Array,
    B_w1: jax.Array,
    B_w2: jax.Array,
    B_w3: jax.Array,
    B_w4: jax.Array,
    c: jax.Array,
    w_mod: jax.Array,
):
    del B_x
    any_spec = pl.BlockSpec(memory_space=pl.ANY)

    def tile_view(x):
        return x.reshape(S // 8, 8, CT, 128).transpose(0, 2, 1, 3).reshape(S * CT, 128)

    vm = pltpu.VMEM
    dma = pltpu.SemaphoreType.DMA
    spec = (4, NG, 16, 128)
    out = pl.pallas_call(
        _kernel,
        in_specs=[any_spec] * 12,
        out_specs=any_spec,
        out_shape=jax.ShapeDtypeStruct((S, D), bf16),
        scratch_shapes=[
            *[vm((KROWS, 128), bf16)] * NB, *[vm((VROWS, 128), bf16)] * NB, vm((CT, 128, S), bf16),
            vm((S, D), bf16), vm((D, D), bf16), vm((D, D), bf16), vm((F, D), bf16), vm((F, D), bf16),
            vm((D // 2, D), u32), vm((D // 2, D), u32), vm((F // 2, D), u32),
            vm((D, 3 * D), bf16), vm((D, 2 * D), bf16), vm((D, D), bf16),
            vm((4, D), bf16), vm((D,), bf16), vm((1, D), bf16), vm((1, 1792), f32),
            vm((4, 128, 128), u32), vm((4, 128, 128), u32), vm((4, 64, 256), u32),
            vm((CT, 8, 8, 128), f32),
            vm((CT, NB) + spec, f32), vm((CT, NB - 1) + spec, f32), vm((CT,) + spec, f32),
            vm((CT, NB) + spec, f32), vm((4, 128, 128), f32),
            vm((CT, S + 32, 128), f32), vm((8, 8, D), f32),
            *[vm((S + 32, 128), f32)] * CT, vm((S, D), f32), vm((S, D), f32), vm((S, D), f32),
            vm((288, D), u32), vm((5, H // 2, 256), u32), vm((H, D), u32), vm((5, H // 2, 256), u32),
            vm((H, D), u32), vm((5, H // 2, 256), u32), vm((5, 96, 256), u32),
            vm((64, 256), u32), vm((D, 256), u32), vm((D, 256), u32), vm((NP3 * 64, 1280), u32),
            vm((7 * 448, 256), u32), vm((35 * 64, 384), u32), vm((2, 448, 128), u32),
            vm((7 * 64, 1152), u32), vm((21 * 32, 640), u32), vm((4 * H, 256), f32), vm((7 * 32, 896), u32), vm((64, 1280), u32),
            vm((S, D), bf16),
            dma((26,)), dma((NC + 10,)),
        ],
        compiler_params=pltpu.CompilerParams(vmem_limit_bytes=110 << 20, disable_bounds_checks=True,
                                             disable_semaphore_checks=True),
    )(A_q.reshape(S, D), tile_view(A_k), tile_view(A_v), A_shift_k.T, A_ssm_k,
      A_ssm_D, B_w1, B_w2, B_w3.T, B_w4, c, w_mod)
    return out.reshape(1, S, D)
```

```python
import numpy as np
import jax
import jax.numpy as jnp
import jax.experimental.pallas as pl
import jax.experimental.pallas.tpu as pltpu

f32, bf16, u32, i32 = jnp.float32, jnp.bfloat16, jnp.uint32, jnp.int32

S, D, F = 2048, 640, 1728
CT = D // 128
TR = 8 * CT
NB, BLK, NFFT = 4, 512, 1024
KROWS, VROWS = BLK * CT + 128, BLK * CT + 64
NG = 16
T = 256
NC = S // T
H = T // 2
NP3 = 6
FM = (F // 128) * 128
P0, P1, PA, PC = 320, 224, 160, 224
PB = P0 + P1 + PA
LA, LAST0 = 112, 208
RG = 16
EPS = 1e-5
NT_DIMS = (((1,), (1,)), ((), ()))
PAIRED = "10000100001000"
ORD = {"r1_1": "42536ba1cd7", "r1_0": "4c5213db7a6", "r2_2": "a2174c3db56", "r3_1": "b76532a4cd1",
       "r3_3": "c245a173b6d", "r3_e": "163cba72d45", "r3_0": "571cab4236d", "r4_41": "5b2a174dc63",
       "r4_42": "a57bd64c321", "r4_43": "b21a574dc63", "r4_44": "52ba174dc63", "r4_45": "5217a4dcb63",
       "r4_46": "52ab174dc36", "r4_47": "b52a174dc63", "l_1": "7a325cbd461", "l_2": "5ca72b1436d",
       "l_e": "24cbd35176a", "l_30": "abd23c51746", "l_31": "acbd2357146", "l_32": "5bc1a74d236",
       "l_33": "bc51a74d236", "l_34": "bc51a74d236", "l_35": "bc15a74d236", "l_41": "243ac571b6d",
       "l_42": "243ac571b6d", "l_43": "243ac571b6d", "l_44": "243ac571b6d", "l_45": "43a17c5b26d",
       "l_46": "243ac571b6d", "l_47": "243ac571b6d", "z_3": "2b5c31a47d6", "z_4": "c35d127b4a6",
       "z_e": "c1d3527ab46", "z_0": "a2d1cb43576"}
OUTER = {"r4": "2637145", "l": "5321647", "z": "4152367"}
BODY = "1pp2sslpsspspspps"
HEAD = "hzcxey"
LM = "0000000100000000"
R2M = "0010101010"
R2L = "1010100010101010"
R3O = "1ezyhx"
R4O = "sGgpspspspsppsps"
ZO = "hxeyz"
FA = 3
TORD = "7624513"
AHEAD = {"r3": "111", "r4": "111", "l": "000", "z": "110"}
GV = 8
NL = 4


def _lo(w):
    return pltpu.bitcast(w << 16, f32)


def _hi(w):
    return pltpu.bitcast(w & jnp.uint32(0xFFFF0000), f32)


def _cis(n):
    t = (n & (2 * NFFT - 1)).astype(f32) * (np.pi / NFFT)
    return jnp.cos(t), jnp.sin(t)


def _fwd_table(r):
    g = jax.lax.broadcasted_iota(i32, (NG, 128), 0)
    cg, sg = _cis(jnp.where(g < NG // 2, 32 * g + 1, 32 * g - 253) * r)
    cs, ss = _cis(4 * jax.lax.broadcasted_iota(i32, (8, 128), 0) * r)
    parts = []
    for i in range(NG):
        c, s = cg[i:i + 1], sg[i:i + 1]
        parts += [c * cs - s * ss, -(s * cs + c * ss)]
    return pltpu.bitcast(jnp.concatenate(parts, axis=0).astype(bf16), u32)


def _inv_tables():
    def phase(rows):
        col = jax.lax.broadcasted_iota(i32, (rows, 256), 1)
        k = ((col >> 4) << 3) + (col & 7)
        row = jax.lax.broadcasted_iota(i32, (rows, 256), 0)
        return jnp.where(k < 64, 4 * k + 1, 4 * k - 253), (col & 8) << 6, row

    fr, _, g = phase(16)
    cg, sg = _cis(fr * (32 * g))
    fr, off, s = phase(8)
    out = []
    for p in range(4):
        cs, ss = _cis(fr * (4 * s + p) + off)
        cs, ss = cs * (2.0 / NFFT), ss * (2.0 / NFFT)
        parts = [cg[i:i + 1] * cs - sg[i:i + 1] * ss for i in range(16)]
        out.append(pltpu.bitcast(jnp.concatenate(parts, axis=0).astype(bf16), u32))
    return out


def _radix4(re, im, inverse):
    ar, ai = re[0] + re[2], im[0] + im[2]
    br, bi = re[0] - re[2], im[0] - im[2]
    cr, ci = re[1] + re[3], im[1] + im[3]
    dr, di = re[1] - re[3], im[1] - im[3]
    minus_i = (br + di, bi - dr)
    plus_i = (br - di, bi + dr)
    if inverse:
        return [(ar + cr, ai + ci), plus_i, (ar - cr, ai - ci), minus_i]
    return [(ar + cr, ai + ci), minus_i, (ar - cr, ai - ci), plus_i]


def _stats(x, link=None, early=False, scaled=False):
    zero = 0.0 if link is None else jnp.minimum(link, 0.0)
    part = x[:, 0:128]
    for c in range(1, CT):
        part = part + x[:, c * 128:(c + 1) * 128]
    if link is not None and early:
        part = part + zero
        zero = 0.0
    m = jnp.sum(part, axis=-1, keepdims=True) * (1.0 / D)
    v = jnp.maximum(jnp.sum(x * x, axis=-1, keepdims=True) * (1.0 / D) - m * m, zero)
    e = jnp.log(v + EPS) * (-0.5 / np.log(2.0))
    return m, jnp.exp2(e + np.log2(ALPHA) if scaled else e)


GC = 0.7978845608028654
ALPHA = (GC * 0.044715) ** (1.0 / 3.0)


def _gelu_scaled(y):
    return y + y * jnp.tanh(y * (y * y + GC / ALPHA))


def _pk(x):
    return pltpu.bitcast(x.astype(bf16), u32)


def _ub(x):
    return pltpu.bitcast(x, bf16)


def _cat(xs, axis=-1):
    return jnp.concatenate(xs, axis=axis)


def _lanes(k):
    return slice(128 * k, 128 * (k + 1))


def _nn(a, w):
    return jnp.dot(a.astype(bf16), w, preferred_element_type=f32)


def _nt(a, w):
    return jax.lax.dot_general(a, w, NT_DIMS, preferred_element_type=f32)


def _lhs_sums(a11, a12, a21, a22):
    return [a11 + a22, a21 + a22, a11 + a12, a21 - a11, a12 - a22]


def _rhs_sum(k, block):
    a, b, plus = [(0, 3, True), (1, 3, False), (2, 0, False), (0, 1, True), (2, 3, True)][k]
    return block(a) + block(b) if plus else block(a) - block(b)


def _strassen(dot, a11, a22, asum, ax1, ax2, b11, b22, bsum, bx1, bx2, order, xdot=None):
    ops = {"1": (asum[0], bsum[0], (1, 0, 0, 1)), "2": (asum[1], b11, (0, 0, 1, -1)),
           "3": (a11, bsum[1], (0, 1, 0, 1)), "4": (a22, bsum[2], (1, 0, 1, 0)),
           "5": (asum[2], b22, (-1, 1, 0, 0)), "6": (asum[3], bsum[3], (0, 0, 0, 1)),
           "7": (asum[4], bsum[4], (1, 0, 0, 0)), "a": (ax1, bx1, (1, 0, 0, 0)),
           "b": (ax1, bx2, (0, 1, 0, 0)), "c": (ax2, bx1, (0, 0, 1, 0)), "d": (ax2, bx2, (0, 0, 0, 1))}
    c, neg = [None] * 4, [None] * 4
    for t in order:
        a, b, sg = ops[t]
        m = (xdot if xdot and t in "abcd" else dot)(a, b)
        for i in range(4):
            if sg[i] > 0:
                c[i] = m if c[i] is None else c[i] + m
                if neg[i] is not None:
                    c[i], neg[i] = c[i] - neg[i], None
            elif sg[i] < 0:
                if c[i] is None:
                    neg[i] = m
                else:
                    c[i] = c[i] - m
    return c


def _kernel(q_hbm, k_hbm, v_hbm, sh_hbm, sk_hbm, d_hbm, w1_hbm, w2_hbm, w3_hbm, w4_hbm,
            c_hbm, wm_hbm, o_hbm,
            kb0, kb1, kb2, kb3, vb0, vb1, vb2, vb3, skb, qb, w1b, w2b, w3b, w4b, w1p, w2p, w3p,
            wma, wmb, wmc, shb, db, cb_, scb,
            fub, fkb, gtb, par, US, KS, UR, YS, YP, ys, modb, h10, h11, h12, h13, h14, h2s, x2s, x1s,
            zt, zu, zb1, zs1, zb0, zs0, zu0, w3n, s1, s2, s3, s4, s5, p4, al, a2, c2, t4, e3, ob,
            sem, sem_o):
    h1s = [h10, h11, h12, h13, h14]
    n_in = [0]

    def load(src, dst):
        n_in[0] += 1
        return pltpu.make_async_copy(src, dst, sem.at[n_in[0] - 1])

    nkv = BLK * CT
    small = [load(d_hbm, db), load(sh_hbm, shb), load(c_hbm, cb_)]
    sk_copies = [load(sk_hbm.at[pl.ds(c * 128, 128), :], skb.at[c]) for c in range(CT)]
    kbs, vbs, wms = [kb0, kb1, kb2, kb3], [vb0, vb1, vb2, vb3], [wma, wmb, wmc]
    kv_copies = [[load(k_hbm.at[pl.ds(a * nkv, nkv), :], kbs[a].at[pl.ds(TR, nkv), :]),
                  load(v_hbm.at[pl.ds(a * nkv, nkv), :], vbs[a].at[pl.ds(0, nkv), :])] for a in range(NB)]
    mod_cols = [(0, 3 * D), (3 * D, 2 * D), (5 * D, D)]
    mod_copies = [load(wm_hbm.at[:, pl.ds(o, n)], w) for (o, n), w in zip(mod_cols, wms)]
    w_copies = [load(w1_hbm, w1b), load(w2_hbm, w2b), load(w3_hbm, w3b), load(w4_hbm, w4b)]
    q_copies = [load(q_hbm.at[pl.ds(o, n), :], qb.at[pl.ds(o, n), :])
                for o, n in [(0, P0 + P1), (P0 + P1, PA), (PB, S - PB)]]

    def out_copy(i):
        r = i * T if isinstance(i, int) else pl.multiple_of(i * T, T)
        return pltpu.make_async_copy(ob.at[pl.ds(r, T), :], o_hbm.at[pl.ds(r, T), :], sem_o.at[i])

    out_tail = []

    def send(r, n, c):
        cp = pltpu.make_async_copy(ob.at[pl.ds(r, n), pl.ds(128 * c, 128)], o_hbm.at[pl.ds(r, n), pl.ds(128 * c, 128)],
                                   sem_o.at[NC - 1 + len(out_tail)])
        out_tail.append(cp)
        cp.start()

    for cp in (small + kv_copies[0] + sk_copies + kv_copies[1] + kv_copies[2] + kv_copies[3]
               + [mod_copies[0], q_copies[0], mod_copies[1], w_copies[0], w_copies[1], q_copies[1],
                  w_copies[2], w_copies[3], mod_copies[2], q_copies[2]]):
        cp.start()

    def wait(copies):
        for cp in copies:
            cp.wait()

    def pin(i, carry):
        z = jnp.zeros((8, 128), f32)
        scb[:, pl.ds(pl.multiple_of(i * 128, 128), 128)] = z[0:1]
        YP[i, 0:8, :] = z
        US[i, 0, 0, 0, 0:8, :] = z
        KS[i, 0, 0, 0, 0:8, :] = z
        YS[i, 0, 0, 0, 0:8, :] = z
        UR[i, 0, 0, 0:8, :] = z
        r8 = pl.ds(pl.multiple_of(i * 8, 8), 8)
        c2[r8, 0:128] = z
        al[r8, 0:128] = jnp.zeros((8, 128), u32)
        zb0[r8, 0:128] = jnp.zeros((8, 128), u32)
        zs0[i, 0:8, 0:128] = jnp.zeros((8, 128), u32)
        zu0[i, 0:8, 0:128] = jnp.zeros((8, 128), u32)
        a2[r8, 0:128] = jnp.zeros((8, 128), u32)
        return carry

    def fence(i, carry):
        YP[i, 0:8, :] = jnp.zeros((8, 128), f32)
        return carry

    jax.lax.fori_loop(0, 2, pin, 0)
    lane = jax.lax.broadcasted_iota(i32, (1, 128), 1)
    for p in range(4):
        m = (lane - p) & 3
        fkb[p] = _fwd_table(128 * m + ((lane - m) & 127))
    for c in range(CT):
        kb0[c * 8:(c + 1) * 8, :] = jnp.zeros((8, 128), bf16)
        h1s[c][0:8, :] = jnp.zeros((8, 128), f32)
        h1s[c][S + 8:S + 16, :] = jnp.zeros((8, 128), f32)
    for a in range(NB):
        kbs[a][nkv + TR:KROWS, :] = jnp.zeros((KROWS - nkv - TR, 128), bf16)
        vbs[a][nkv:VROWS, :] = jnp.zeros((VROWS - nkv, 128), bf16)
    for p in range(4):
        fub[p] = _fwd_table(8 * (lane & 63) + ((lane >> 6) << 2) + p)
    wait(small)
    cvec = cb_[...].astype(f32)
    scb[:, 0:D] = cvec * jax.nn.sigmoid(cvec)
    dv = db[...].astype(f32).reshape(1, D)
    shv = shb[...].astype(f32)
    for c in range(CT):
        for i in range(4):
            par[c, i] = jnp.broadcast_to(shv[i:i + 1, c * 128:(c + 1) * 128], (8, 128))
        par[c, 4] = jnp.broadcast_to(dv[:, c * 128:(c + 1) * 128], (8, 128))
    for p, tab in enumerate(_inv_tables()):
        gtb[p] = tab

    def get(ref, idx, g, n):
        return (ref[idx + (slice(g, g + n), slice(0, 8))], ref[idx + (slice(g, g + n), slice(8, 16))])

    def put(ref, idx, g, n, xr, xi):
        ref[idx + (slice(g, g + n), slice(0, 8))] = xr
        ref[idx + (slice(g, g + n), slice(8, 16))] = xi

    def split(tt, g, n):
        tt = [t[g * 16:(g + n) * 16].reshape(n, 16, 128) for t in tt]
        return [t[:, 0:8] for t in tt], [t[:, 8:16] for t in tt]

    def fwd_k(c, j):
        lane = jax.lax.broadcasted_iota(i32, (64, 128), 1)
        even = (lane & 1) == 0
        l01 = (lane & 2) == 0
        l12 = ((lane + 3) & 2) == 0
        rm = []
        for m in range(4):
            w = pltpu.bitcast(skb[c, :, (4 * j + m) * 128:(4 * j + m + 1) * 128], u32)
            rm.append(pltpu.roll(w, m, 1) if m else w)
        e01 = jnp.where(even, rm[0], rm[1])
        o01 = jnp.where(even, rm[1], rm[0])
        e23 = jnp.where(even, rm[2], rm[3])
        o23 = jnp.where(even, rm[3], rm[2])
        kp = [jnp.where(l01, e01, e23), jnp.where(l12, o01, o23),
              jnp.where(l01, e23, e01), jnp.where(l12, o23, o01)]
        tt = [jax.lax.dot_general(pltpu.bitcast(fkb[p], bf16), pltpu.bitcast(kp[p], bf16), NT_DIMS,
                                  preferred_element_type=f32) for p in range(4)]
        for g in range(0, NG, GV):
            re, im = split(tt, g, GV)
            if j == 0:
                re[0] = re[0] + par[c, 4][None]
            for m, (xr, xi) in enumerate(_radix4(re, im, False)):
                if j < NB - 1:
                    put(KS, (c, j, m), g, GV, xr, xi)
                ur, ui = get(US, (c, 0, m), g, GV)
                put(YS, (c, j, m), g, GV, xr * ur - xi * ui, xr * ui + xi * ur)

    def fwd_u(c, a):
        taps = [jnp.tile(par[c, i], (8, 1)) for i in range(4)]
        ws = TR // 2
        base = 4 * c
        kw, vw = kbs[a].bitcast(u32), vbs[a].bitcast(u32)

        def words(ref, start):
            return ref[pl.ds(start, BLK // 8, stride=ws), :]

        kk = {}
        for w in range(4):
            x = words(kw, ws + base + w)
            kk[2 * w], kk[2 * w + 1] = _lo(x), _hi(x)
        kk[-3] = _hi(words(kw, base + 2))
        x = words(kw, base + 3)
        kk[-2], kk[-1] = _lo(x), _hi(x)
        sub = []
        for w in range(4):
            x = words(vw, base + w)
            for r, vv in ((2 * w, _lo(x)), (2 * w + 1, _hi(x))):
                sh = taps[0] * kk[r] + taps[1] * kk[r - 1] + taps[2] * kk[r - 2] + taps[3] * kk[r - 3]
                sub.append(sh * vv)
        kv = [jnp.concatenate([sub[p], sub[p + 4]], axis=0) for p in range(4)]
        tt = [jnp.dot(pltpu.bitcast(fub[p], bf16), kv[p].astype(bf16), preferred_element_type=f32)
              for p in range(4)]
        for g in range(0, NG, GV):
            re, im = split(tt, g, GV)
            for m, (xr, xi) in enumerate(_radix4(re, im, False)):
                if a:
                    pr, pi = get(US, (c, 0, m), g, GV) if a == 1 else get(UR, (c, m), g, GV)
                    if a < NB - 1:
                        put(UR, (c, m), g, GV, xr, xi)
                    xr, xi = (xr - pi, xi + pr) if g < NG // 2 else (xr + pi, xi - pr)
                put(US, (c, a, m), g, GV, xr, xi)

    def mac_inv(c, a):
        for h in range(2):
            vals = [[] for _ in range(4)]
            for g in range(8 * h, 8 * h + 8, GV):
                yre, yim = [], []
                for m in range(4):
                    yr, yi = get(YS, (c, a, m), g, GV)
                    for j in range(a):
                        kr, ki = get(KS, (c, j, m), g, GV)
                        ur, ui = get(US, (c, a - j, m), g, GV)
                        yr = yr + (kr * ur - ki * ui)
                        yi = yi + (kr * ui + ki * ur)
                    yre.append(yr)
                    yim.append(yi)
                for p, (pr, pi) in enumerate(_radix4(yre, yim, True)):
                    vals[p].append(jnp.concatenate([pr, pi], axis=1))
            for p in range(4):
                pb = jnp.concatenate(vals[p], axis=0).reshape(128, 128).astype(bf16)
                r = jnp.dot(pltpu.bitcast(gtb[p, :, h * 128:(h + 1) * 128], bf16), pb,
                            preferred_element_type=f32)
                if h == 0:
                    YP[p] = r
                else:
                    ys[c, pl.ds(a * BLK + p, 128, stride=4), :] = YP[p] + r

    wait(kv_copies[0])
    for c in range(CT):
        fwd_u(c, 0)
    for grp in ((0,), (1, 2), (3, 4)):
        wait([sk_copies[c] for c in grp])
        for c in grp:
            for j in (3, 2, 1, 0):
                fwd_k(c, j)
    for a in range(1, NB):
        if a == FA:
            jax.lax.fori_loop(0, 2, fence, 0)
        wait(kv_copies[a])
        for c in range(CT):
            kbs[a][c * 8:(c + 1) * 8, :] = kbs[a - 1][nkv + c * 8:nkv + (c + 1) * 8, :]
        for c in range(CT):
            fwd_u(c, a)
            mac_inv(c, a - 1)
    wait([mod_copies[0]])
    for c in range(NL):
        mac_inv(c, NB - 1)

    def mod_part(part, extra):
        n, wm = mod_cols[part][1], wms[part]
        act = scb[:, 0:D]

        def sc(k0, k1):
            return jnp.broadcast_to(act[:, k0:k1], (16, k1 - k0)).astype(bf16)

        e = 128 * extra
        r = jnp.dot(sc(0, D), wm[:, e:n], preferred_element_type=f32)
        r0 = (jnp.dot(sc(0, D - 64), wm[0:D - 64, 0:e], preferred_element_type=f32)
              + jnp.dot(sc(D - 64, D), wm[D - 64:D, 0:e], preferred_element_type=f32))
        r = jnp.concatenate([r0, r], axis=-1)[0:8]
        return [r[:, i * D:(i + 1) * D] for i in range(n // D)]

    def mvec(i, n=RG, c0=0, c1=D):
        return jnp.tile(modb[i, :, c0:c1], (n // 8, 1))

    rows = pl.ds
    ctx = ["r1"]

    def load_q(r, ref=qb):
        return ref[rows(r, RG), :].astype(f32)

    def make_x2(r, q, st, ref=ys):
        y = _cat([ref[c, rows(r, RG), :] for c in range(CT)])
        return q + (((q - st[0]) * st[1]) * mvec(1) + mvec(0)) * y

    def make_h2(x2, st):
        return ((x2 - st[0]) * st[1]) * mvec(3) + mvec(2)

    def put_sums(ref, o, z1, z2):
        for k, v in enumerate(_lhs_sums(z1[:, 0:256], z1[:, 256:512], z2[:, 0:256], z2[:, 256:512])):
            ref.at[k][o // 2:(o + RG) // 2, :] = _pk(v)

    def ln_chain(r, n, paired):
        qv, yv = qb.at[rows(r, n), :], ys.at[:, rows(r, n), :]
        xv, hv = x2s.at[rows(r, n), :], h2s.at[rows(r, n), :]
        prev, pend, cnt = None, None, 0
        for o1 in range(0, n // 2, RG):
            zz = []
            for o in (o1, o1 + n // 2):
                q = load_q(o, qv)
                x2 = make_x2(o, q, _stats(q, prev), yv)
                xv[o:o + RG, :] = x2
                st = _stats(x2)
                h2 = make_h2(xv[o:o + RG, :], st)
                hv[o:o + RG, :] = h2
                st = _stats(h2, scaled=True)
                z = (hv[o:o + RG, :] - st[0]) * st[1]
                zt[o // 2:(o + RG) // 2, :] = _pk(z)
                zz.append(z)
                if paired and paired[cnt] == "1":
                    pend = st[1]
                elif pend is not None:
                    prev, pend = jnp.minimum(st[1], pend), None
                else:
                    prev = st[1]
                cnt += 1
            put_sums(zu, o1, zz[0], zz[1])

    def ln_x1(r, paired=""):
        zb, zs = (zb0, zs0) if ctx[0] == "r2" else (zb1, zs1)
        sv = x1s.at[rows(r, T), :]
        prev, pend, cnt = None, None, 0
        for o1 in range(0, H, RG):
            zz = []
            for o in (o1, o1 + H):
                x1 = sv[o:o + RG, :]
                st = _stats(x1, prev, True, True)
                z = (x1 - st[0]) * st[1]
                zb[o // 2:(o + RG) // 2, :] = _pk(z)
                zz.append(z)
                if paired and paired[cnt] == "1":
                    pend = st[1]
                elif pend is not None:
                    prev, pend = jnp.minimum(st[1], pend), None
                else:
                    prev = st[1]
                cnt += 1
            put_sums(zs, o1, zz[0], zz[1])

    def both(ref, r0, r1, col):
        return _cat([ref[r0:r1, _lanes(1 + col)].astype(f32), ref[r0:r1, _lanes(3 + col)].astype(f32)])

    def prep_square(wb, wp, sw):
        wp[:, 0:128] = pltpu.bitcast(wb[:, 0:128], u32)
        wp[256:320, 128:D] = pltpu.bitcast(wb[512:D, 128:D], u32)
        for n in range(2):
            wp[0:128, _lanes(2 * n + 1)] = pltpu.bitcast(wb[0:256, _lanes(2 * n + 1)], u32)
            wp[128:256, _lanes(2 * n + 2)] = pltpu.bitcast(wb[256:512, _lanes(2 * n + 2)], u32)
        for k in (2, 1, 0, 4, 3):
            sw[128 * k:128 * (k + 1), :] = _pk(_rhs_sum(
                k, lambda b: both(wb, 256 * (b // 2), 256 * (b // 2 + 1), b % 2)))

    def mm_square(a, top, bot, asum, wp, sw, which):
        h = top.shape[0]
        c0 = _nn(a, _ub(wp[:, 0:128]))
        out = [(c0[0:h], c0[h:2 * h])]
        for n in range(2):
            l1, l2 = _lanes(2 * n + 1), _lanes(2 * n + 2)
            q = _strassen(_nn, top[:, 0:256], bot[:, 256:512], asum, top[:, 512:D], bot[:, 512:D],
                          _ub(wp[0:128, l1]), _ub(wp[128:256, l2]),
                          [_ub(sw[128 * k:128 * (k + 1), _lanes(n)]) for k in range(5)],
                          _ub(wp[256:320, l1]), _ub(wp[256:320, l2]), ORD[ctx[0] + "_" + which])
            out += [(q[0], q[2]), (q[1], q[3])]
        return out

    def mm_w1(r, n, o=0, zu=zu, which="1"):
        h, o = n // 2, o // 2
        res = mm_square(_ub(zt[o:o + h, :]), _ub(zt[o:o + h // 2, :]), _ub(zt[o + h // 2:o + h, :]),
                        [_ub(zu[k, 0:h // 2, :]) for k in range(5)], w1p, s1, which)
        for c, (top, bot) in enumerate(res):
            h1s[c][rows(r + 8, h), :] = _gelu_scaled(top)
            h1s[c][rows(r + 8 + h, h), :] = _gelu_scaled(bot)

    def mm_w2(r):
        lane = jax.lax.broadcasted_iota(i32, (T, 128), 1)

        def sh(k, c):
            return h1s[c][rows(r + 8 + k, T), :]

        g = _cat([sh(-1, 0),
                  jnp.where(lane < 32, sh(-1, 1), sh(1, 1)),
                  jnp.where(lane < 64, sh(1, 2), sh(-2, 2)),
                  jnp.where(lane < 96, sh(-2, 3), sh(2, 3)),
                  sh(2, 4)])
        top, bot = g[0:H], g[H:T]
        sums = _lhs_sums(top[:, 0:256], top[:, 256:512], bot[:, 0:256], bot[:, 256:512])
        for c, (ct, cb) in enumerate(mm_square(g, top, bot, sums, w2p, s2, "2")):
            x1s[rows(r, H), _lanes(c)] = h2s[rows(r, H), _lanes(c)] + ct * (0.5 / ALPHA)
            x1s[rows(r + H, H), _lanes(c)] = h2s[rows(r + H, H), _lanes(c)] + cb * (0.5 / ALPHA)

    def prep_w3():
        for j in range(NP3):
            r0 = 128 * (2 * j + 1)
            w3p[r0 // 2:r0 // 2 + 64, 0:256] = pltpu.bitcast(w3b[r0:r0 + 128, 0:256], u32)
            if j > 1:
                w3p[r0 // 2:r0 // 2 + 64, 512:D] = pltpu.bitcast(w3b[r0:r0 + 128, 512:D], u32)
            c1 = D if j > 1 else 512
            w3p[r0 // 2 + 64:r0 // 2 + 128, 256:c1] = pltpu.bitcast(w3b[r0 + 128:r0 + 256, 256:c1], u32)
        w3p[0:48, 0:256] = pltpu.bitcast(w3b[0:96, 0:256], u32)
        w3p[0:48, 512:D] = pltpu.bitcast(w3b[0:96, 512:D], u32)
        w3p[48:64, 256:D] = pltpu.bitcast(w3b[96:128, 256:D], u32)
        w3p[FM // 2:F // 2, 256:D] = pltpu.bitcast(w3b[FM:F, 256:D], u32)
        w3n[0:64, :] = _pk(_cat([w3b[128 * t:128 * (t + 1), 512:D].astype(f32).T for t in range(1, 5)]))

        def edge(b):
            c = slice(256 * (b // 2), 256 * (b // 2 + 1))
            if b % 2 == 0:
                return w3b[0:96, c].astype(f32)
            return _cat([w3b[96:128, c].astype(f32), w3b[FM:F, c].astype(f32)], 0)

        for k in (2, 1, 0, 4, 3):
            e3[0:48, 256 * k:256 * (k + 1)] = _pk(_rhs_sum(k, edge))
        for j in range(NP3):
            r0 = 128 * (2 * j + 1)
            for k in (2, 1, 0, 4, 3):
                s3[64 * j:64 * (j + 1), 256 * k:256 * (k + 1)] = _pk(_rhs_sum(k, lambda b: w3b[
                    r0 + 128 * (b % 2):r0 + 128 * (b % 2 + 1), 256 * (b // 2):256 * (b // 2 + 1)].astype(f32)))

    def w3_edge():
        def second(c0, c1):
            return _ub(_cat([w3p[48:64, c0:c1], w3p[FM // 2:F // 2, c0:c1]], 0))

        zb, zs = (zb0, zs0) if ctx[0] == "r3" else (zb1, zs1)
        z1, z2 = _ub(zb[0:H // 2, :]), _ub(zb[H // 2:H, :])
        q = _strassen(lambda a, b: _nt(b, a), z1[:, 0:256], z2[:, 256:512], [_ub(zs[k]) for k in range(5)],
                      z1[:, 512:D], z2[:, 512:D], _ub(w3p[0:48, 0:256]), second(256, 512),
                      [_ub(e3[0:48, 256 * k:256 * (k + 1)]) for k in range(5)],
                      _ub(w3p[0:48, 512:D]), second(512, D), ORD[ctx[0] + "_e"])
        q = [_gelu_scaled(c) for c in q]
        out = []
        for x in (_cat(q[0:2], 0), _cat(q[2:4], 0)):
            out += [x[0:128].T, _cat([x[128:192], jnp.zeros((64, 128), f32)], 0).T]
        put_quads(NP3, out)

    xpre = [None]

    def w3_head():
        zb = zb0 if ctx[0] == "r3" else zb1
        xpre[0] = _nn(_ub(zb[:, 512:D]), _ub(w3n[...]))

    def w3_pair(j):
        e, o = slice(64 * (2 * j + 1), 64 * (2 * j + 2)), slice(64 * (2 * j + 2), 64 * (2 * j + 3))
        zb, zs = (zb0, zs0) if ctx[0] == "r3" else (zb1, zs1)
        z1, z2 = _ub(zb[0:H // 2, :]), _ub(zb[H // 2:H, :])
        q = _strassen(_nt, z1[:, 0:256], z2[:, 256:512], [_ub(zs[k]) for k in range(5)],
                      *([0, 1] if j < 2 else [z1[:, 512:D], z2[:, 512:D]]),
                      _ub(w3p[e, 0:256]), _ub(w3p[o, 256:512]),
                      [_ub(s3[64 * j:64 * (j + 1), 256 * k:256 * (k + 1)]) for k in range(5)],
                      *([2 * j, 2 * j + 1, ORD.get(ctx[0] + "_3%d" % j, ORD.get(ctx[0] + "_0")), lambda a, b: xpre[0][H * a:H * (a + 1), _lanes(b)]] if j < 2 else
                        [_ub(w3p[e, 512:D]), _ub(w3p[o, 512:D]), ORD.get(ctx[0] + "_3%d" % j, ORD.get(ctx[0] + "_3"))]))
        return [_gelu_scaled(c) for c in q]

    def plain_ctx():
        return ctx[0] == "z"

    def put_quads(j, q):
        l1, l2, l5, l6, l7 = _lhs_sums(*q)
        if not plain_ctx():
            al[64 * j:64 * (j + 1), 0:896] = _pk(_cat([l1, l2, q[0], q[3], l5, l6, l7]))
        else:
            al[64 * j:64 * (j + 1), :] = _pk(_cat([l1, l2, q[0], q[3], l5, l6, l7, q[1], q[2]]))

    def w3_pairs(i):
        ahead = AHEAD[ctx[0]][i] == "1"
        ops = []
        for j in (2 * i, 2 * i + 1):
            q = w3_pair(j)
            if not ahead:
                put_quads(j, q)
            ops.append(q)
        if not ahead:
            return
        for n, q in enumerate(ops):
            l1, l2, l5, l6, l7 = _lhs_sums(*q)
            ops[n] = [l1, l2, q[0], q[3], l5, l6, l7]
            j, half = 2 * i + n, slice(64 * n, 64 * (n + 1))
            if not plain_ctx():
                al[64 * j:64 * (j + 1), 0:896] = _pk(_cat(ops[n]))
                continue
            o = 64 * j + 32 * n
            al[o:o + 32, 0:256] = _pk(_cat([l1[half], l2[half]]))
            al[o:o + 32, 512:896] = _pk(_cat([l5[half], l6[half], l7[half]]))
            al[64 * j:64 * (j + 1), 256:512] = _pk(_cat([q[0], q[3]]))
            al[64 * j:64 * (j + 1), 896:1152] = _pk(_cat([q[1], q[2]]))
        for m in range(7):
            e, o = ops[0][m], ops[1][m]
            r0 = 32 * (3 * m + i)
            a2[r0:r0 + 32, :] = _pk(_cat(_lhs_sums(e[0:64], o[0:64], e[64:128], o[64:128])))

    def s4_block(m, b, axis):
        o = 448 * (m - 1) + 64 * (b // 2)
        return _cat([s4[o + 128 * i:o + 128 * i + 64, _lanes(b % 2)] for i in range(3)], axis)

    def krow(j, par):
        return 128 * (2 * j + 1 + par) if j < NP3 else FM * par

    def prep_p4():
        for j in range(7):
            p4[0, 64 * j:64 * (j + 1), :] = pltpu.bitcast(w4b[krow(j, 0):krow(j, 0) + 128, 0:128], u32)
            if j < NP3:
                p4[1, 64 * j:64 * (j + 1), :] = pltpu.bitcast(w4b[krow(j, 1):krow(j, 1) + 128, 0:128], u32)
            else:
                p4[1, 64 * j:64 * j + 32, :] = pltpu.bitcast(w4b[FM:F, 0:128], u32)
                p4[1, 64 * j + 32:64 * (j + 1), :] = jnp.zeros((32, 128), u32)

    def prep_w4():
        def block(j, b):
            if j == NP3 and b >= 2:
                return _cat([both(w4b, FM, F, b % 2), jnp.zeros((64, 256), f32)], 0)
            return both(w4b, krow(j, b // 2), krow(j, b // 2) + 128, b % 2)

        for m in [int(t) for t in OUTER['r4']]:
            k = {1: 0, 4: 2, 2: None, 3: 1, 5: None, 7: 4, 6: 3}[m]
            for j in range(7):
                o = 448 * (m - 1) + 64 * j
                if k is None and (j < NP3 or m == 2):
                    par = 0 if m == 2 else 1
                    for n in range(2):
                        s4[o:o + 64, _lanes(n)] = pltpu.bitcast(
                            w4b[krow(j, par):krow(j, par) + 128, _lanes(2 * n + 1 + par)], u32)
                else:
                    s4[o:o + 64, :] = _pk(block(j, 3) if k is None else _rhs_sum(k, lambda b: block(j, b)))
            for k2 in (2, 1, 0, 4, 3):
                o = 64 * (5 * (m - 1) + k2)
                s5[o:o + 64, :] = _pk(_rhs_sum(k2, lambda b: _ub(s4_block(m, b, -1)).astype(f32)))

    def prep_t4():
        def tile(j, par):
            if j == NP3 and par:
                return _cat([w4b[FM:F, 0:128].astype(f32), jnp.zeros((64, 128), f32)], 0).T
            return w4b[krow(j, par):krow(j, par) + 128, 0:128].astype(f32).T

        wt = [_cat([tile(j, par) for j in range(7)]) for par in range(2)]
        for m, k in ((1, 0), (2, None), (3, 1), (4, 2), (5, None), (6, 3), (7, 4)):
            def blk(b):
                return wt[b // 2][64 * (b % 2):64 * (b % 2 + 1)]
            t4[32 * (m - 1):32 * m, :] = _pk(blk(0 if m == 2 else 3) if k is None else _rhs_sum(k, blk))

    def w4_tile0_steps(r):
        mm = {}
        for t in TORD:
            m = int(t)
            left = _cat([al[64 * j:64 * (j + 1), _lanes(m - 1)] for j in range(7)])
            mm[m] = _nt(_ub(t4[32 * (m - 1):32 * m, :]), _ub(left))
            if len(mm) == 7:
                c11 = ((mm[4] - mm[5]) + mm[1]) + mm[7]
                c22 = ((mm[3] - mm[2]) + mm[1]) + mm[6]
                finish(r, H, _cat([c11, mm[3] + mm[5]], 0).T, 0)
                finish(r + H, H, _cat([mm[4] + mm[2], c22], 0).T, 0)
            yield

    def finish(r, n, h, c):
        c0, c1 = 128 * c, 128 * (c + 1)
        x1 = x1s[rows(r, n), c0:c1]
        base = x2s[rows(r, n), c0:c1] + mvec(4, n, c0, c1) * x1
        ob[rows(r, n), c0:c1] = (base + mvec(5, n, c0, c1) * h).astype(bf16)
        if ctx[0] == "z":
            send(r, n, c)

    def w4_plain(r, o=0, n=T):
        def left(k):
            return _cat([al[64 * j:64 * (j + 1), _lanes(k)] for j in range(7)])

        a = _cat([_cat([left(2), left(7)]), _cat([left(8), left(3)])], 0)[o // 2:(o + n) // 2]
        finish(r + o, n, _nn(_ub(a), _ub(_cat([p4[0], p4[1]], 0))), 0)

    def w4_product(m):
        def blk(b, grp=range(3)):
            o = 64 * (b % 2) + 32 * (b // 2)
            return _ub(_cat([al[o + 128 * i:o + 128 * i + 32, _lanes(m - 1)] for i in grp]))

        pre = [i for i in range(3) if AHEAD[ctx[0]][i] == "1"]
        now = [i for i in range(3) if i not in pre]
        asum = [[] for _ in range(5)]
        if pre:
            for k in range(5):
                asum[k].append((pre, _ub(_cat([a2[32 * (3 * (m - 1) + i):32 * (3 * (m - 1) + i + 1), _lanes(k)]
                                               for i in pre]))))
        if now:
            for k, v in enumerate(_lhs_sums(*[blk(b, now).astype(f32) for b in range(4)])):
                asum[k].append((now, v))

        def dot(a, w):
            if not isinstance(a, list):
                return _nn(a, w)
            parts = [_nn(v, w if len(grp) == 3 else _cat([w[128 * i:128 * (i + 1)] for i in grp], 0)) for grp, v in a]
            return parts[0] if len(parts) == 1 else parts[0] + parts[1]

        bsum = [_ub(_cat([s5[64 * (5 * (m - 1) + k):64 * (5 * (m - 1) + k + 1), _lanes(i)] for i in range(3)], 0))
                for k in range(5)]
        ox = 448 * (m - 1) + 384
        q = _strassen(dot, blk(0), blk(3), asum, _ub(al[384:416, _lanes(m - 1)]), _ub(al[416:448, _lanes(m - 1)]),
                      _ub(s4_block(m, 0, 0)), _ub(s4_block(m, 3, 0)), bsum,
                      _ub(s4[ox:ox + 64, _lanes(0)]), _ub(s4[ox:ox + 64, _lanes(1)]), ORD.get(ctx[0] + "_4%d" % m, ORD.get(ctx[0] + "_4")))
        return _cat([_cat(q[0:2]), _cat(q[2:4])], 0)

    def w4_steps(r):
        acc = [c2.at[H * i:H * (i + 1), :] for i in range(4)]

        def finish2(rr, h, c):
            finish(rr, H, h[:, 0:128], c)
            finish(rr, H, h[:, 128:256], c + 2)

        sign = {1: (1, 0, 0, 1), 2: (0, 0, 1, -1), 3: (0, 1, 0, 1), 4: (1, 0, 1, 0), 5: (-1, 1, 0, 0),
                6: (0, 0, 0, 1), 7: (1, 0, 0, 0)}
        left_n, state = [4, 2, 2, 4], [None] * 4
        for m in [int(t) for t in OUTER[ctx[0]]]:
            x = w4_product(m)
            outs = [i for i in range(4) if sign[m][i]]
            olds = {i: None if state[i] is None else state[i][0][...] for i in outs}
            busy = [state[i][0] for i in range(4) if state[i] is not None and i not in outs]
            free = [a for a in acc if not any(a is b for b in busy)]
            shared = None
            for i in outs:
                sg = sign[m][i]
                left_n[i] -= 1
                if state[i] is None:
                    if shared is None:
                        shared = free.pop()
                        shared[...] = x
                    state[i] = (shared, sg)
                    continue
                v = olds[i] + x if (sg > 0) == (state[i][1] > 0) else (x - olds[i] if sg > 0 else olds[i] - x)
                if left_n[i] == 0:
                    finish2(r + H * (i // 2), v, 1 + i % 2)
                    state[i] = None
                else:
                    dst = free.pop()
                    dst[...] = v
                    state[i] = (dst, 1)
            yield

    def up(order, r1=None, n1=None):
        for tok in order:
            if tok == "h":
                w3_head()
            elif tok == "e":
                w3_edge()
            elif tok in "xyz":
                w3_pairs("xyz".index(tok))
            elif tok == "1":
                mm_w1(r1, n1)
            elif tok == "c":
                ln_chain(r1, n1, paired=PAIRED)

    groups = list(range(0, P0 + P1, RG))
    wait([q_copies[0]])
    sa, ca, ga = mod_part(0, 1)
    modb[0] = ga * sa
    modb[1] = ga * (1.0 + ca)
    for c in range(NL, CT):
        mac_inv(c, NB - 1)
    st1 = {o: _stats(load_q(o)) for o in groups}
    zt[0:8, 0:128] = jnp.zeros((8, 128), u32)
    st2 = {}
    for o in groups:
        x2 = make_x2(o, load_q(o), st1[o])
        x2s[o:o + RG, :] = x2
        st2[o] = _stats(x2)

    wait([mod_copies[1]])
    sb, cb = mod_part(1, 2)
    modb[2] = sb
    modb[3] = 1.0 + cb
    st3 = {}
    for o in range(0, P0, RG):
        h2 = make_h2(x2s[o:o + RG, :], st2[o])
        h2s[o:o + RG, :] = h2
        st3[o] = _stats(h2, scaled=True)
    for o1 in range(0, P0 // 2, RG):
        zz = []
        for o in (o1, o1 + P0 // 2):
            zz.append((h2s[o:o + RG, :] - st3[o][0]) * st3[o][1])
            zt[o // 2:(o + RG) // 2, :] = _pk(zz[-1])
        put_sums(zu0, o1, zz[0], zz[1])

    wait([w_copies[0]])
    prep_square(w1b, w1p, s1)
    mm_w1(0, P0, 0, zu0, "0")
    prev = None
    for o1 in range(0, P1 // 2, RG):
        zz = []
        for o in (P0 + o1, P0 + o1 + P1 // 2):
            h2 = make_h2(x2s[o:o + RG, :], st2[o])
            h2s[o:o + RG, :] = h2
            st = _stats(h2, prev, True, True)
            z = (h2 - st[0]) * st[1]
            zt[o // 2:(o + RG) // 2, :] = _pk(z)
            prev = st[1]
            zz.append(z)
        put_sums(zu, o1, zz[0], zz[1])
    mm_w1(P0, P1, P0)

    ctx[0] = "r2"
    wait([w_copies[1], q_copies[1]])
    prep_square(w2b, w2p, s2)
    ln_chain(P0 + P1, PA, paired=R2M)
    mm_w2(0)
    ln_x1(0, R2L)
    mm_w2(T)

    ctx[0] = "r3"
    wait([w_copies[2]])
    prep_w3()
    ln_x1(T)
    up(R3O, P0 + P1, PA)

    ctx[0] = "r4"
    jax.lax.fori_loop(0, 2, fence, 0)
    wait([w_copies[3], mod_copies[2]])
    prep_w4()
    sc16 = jnp.broadcast_to(scb[:, 0:D], (16, D)).astype(bf16)
    prep_t4()
    steps, tile0 = w4_steps(0), w4_tile0_steps(0)
    for tok in R4O:
        if tok == "p":
            next(tile0)
        elif tok == "s":
            next(steps)
        else:
            c0, c1 = (0, 384) if tok == "g" else (384, D)
            gb = jnp.dot(sc16, wmc[:, c0:c1], preferred_element_type=f32)[0:8]
            modb[4, :, c0:c1] = gb
            modb[5, :, c0:c1] = (0.5 / ALPHA) * gb
    out_copy(0).start()
    q_copies[2].wait()

    def mlp_body(i, carry):
        r1 = pl.multiple_of(PB - PC + PC * i, 32)
        r = pl.multiple_of(i * T, T)
        up(HEAD, r1, PC)
        steps, tile0 = w4_steps(r), w4_tile0_steps(r)
        for tok in BODY:
            if tok == "1":
                mm_w1(r1, PC)
            elif tok == "p":
                next(tile0)
            elif tok == "2":
                mm_w2(r + T)
            elif tok == "l":
                ln_x1(r + T, LM)
            else:
                next(steps)
        out_copy(i).start()
        return carry

    ctx[0] = "l"
    jax.lax.fori_loop(1, NC - 1, mlp_body, 0)

    ctx[0] = "z"
    up(ZO)
    prep_p4()
    w4_plain(S - T, 0, LA)
    for _ in w4_steps(S - T):
        pass
    w4_plain(S - T, LA, LAST0 - LA)
    w4_plain(S - T, LAST0, T - LAST0)
    for i in range(NC - 1):
        out_copy(i).wait()
    for cp in out_tail:
        cp.wait()


@jax.jit
def pallas_adaLN_cond__ssm_conv_h3__mixer_s_mlp__prompt_kernel(
    A_q: jax.Array,
    A_k: jax.Array,
    A_v: jax.Array,
    A_shift_k: jax.Array,
    A_ssm_k: jax.Array,
    A_ssm_D: jax.Array,
    B_x: jax.Array,
    B_w1: jax.Array,
    B_w2: jax.Array,
    B_w3: jax.Array,
    B_w4: jax.Array,
    c: jax.Array,
    w_mod: jax.Array,
):
    del B_x
    any_spec = pl.BlockSpec(memory_space=pl.ANY)

    def tile_view(x):
        return x.reshape(S // 8, 8, CT, 128).transpose(0, 2, 1, 3).reshape(S * CT, 128)

    vm = pltpu.VMEM
    dma = pltpu.SemaphoreType.DMA
    spec = (4, NG, 16, 128)
    out = pl.pallas_call(
        _kernel,
        in_specs=[any_spec] * 12,
        out_specs=any_spec,
        out_shape=jax.ShapeDtypeStruct((S, D), bf16),
        scratch_shapes=[
            *[vm((KROWS, 128), bf16)] * NB, *[vm((VROWS, 128), bf16)] * NB, vm((CT, 128, S), bf16),
            vm((S, D), bf16), vm((D, D), bf16), vm((D, D), bf16), vm((F, D), bf16), vm((F, D), bf16),
            vm((D // 2, D), u32), vm((D // 2, D), u32), vm((F // 2, D), u32),
            vm((D, 3 * D), bf16), vm((D, 2 * D), bf16), vm((D, D), bf16),
            vm((4, D), bf16), vm((D,), bf16), vm((1, D), bf16), vm((1, 1792), f32),
            vm((4, 128, 128), u32), vm((4, 128, 128), u32), vm((4, 64, 256), u32),
            vm((CT, 8, 8, 128), f32),
            vm((CT, NB) + spec, f32), vm((CT, NB - 1) + spec, f32), vm((CT,) + spec, f32),
            vm((CT, NB) + spec, f32), vm((4, 128, 128), f32),
            vm((CT, S + 32, 128), f32), vm((8, 8, D), f32),
            *[vm((S + 32, 128), f32)] * CT, vm((S, D), f32), vm((S, D), f32), vm((S, D), f32),
            vm((288, D), u32), vm((5, H // 2, 256), u32), vm((H, D), u32), vm((5, H // 2, 256), u32),
            vm((H, D), u32), vm((5, H // 2, 256), u32), vm((5, 96, 256), u32),
            vm((64, 512), u32), vm((D, 256), u32), vm((D, 256), u32), vm((NP3 * 64, 1280), u32),
            vm((7 * 448, 256), u32), vm((35 * 64, 384), u32), vm((2, 448, 128), u32),
            vm((7 * 64, 1152), u32), vm((21 * 32, 640), u32), vm((4 * H, 256), f32), vm((7 * 32, 896), u32), vm((64, 1280), u32),
            vm((S, D), bf16),
            dma((26,)), dma((NC + 10,)),
        ],
        compiler_params=pltpu.CompilerParams(vmem_limit_bytes=110 << 20, disable_bounds_checks=True,
                                             disable_semaphore_checks=True),
    )(A_q.reshape(S, D), tile_view(A_k), tile_view(A_v), A_shift_k.T, A_ssm_k,
      A_ssm_D, B_w1, B_w2, B_w3.T, B_w4, c, w_mod)
    return out.reshape(1, S, D)
```
